```python
import jax
import jax.numpy as jnp

def _softmax(x, axis=-1):
    return jax.nn.softmax(x, axis=axis)

def _gelu(x):
    return jax.nn.gelu(x, approximate=True)

def _silu(x):
    return jax.nn.silu(x)

def _sigmoid(x):
    return jax.nn.sigmoid(x)

def _layernorm(x, axis=-1, eps=1e-05):
    m = jnp.mean(x, axis=axis, keepdims=True)
    v = jnp.var(x, axis=axis, keepdims=True)
    return (x - m) / jnp.sqrt(v + eps)

def _scatter_add(tgt, idx, src, axis=0):
    return tgt.at[idx].add(src)

def _segment_sum(src, seg, n):
    return jax.ops.segment_sum(src, seg, n)

class _Rng:

    def __init__(self, key):
        self._k = key

    def _next(self):
        self._k, sub = jax.random.split(self._k)
        return sub

    def normal(self, shape):
        return jax.random.normal(self._next(), shape, dtype=jnp.bfloat16)

    def randint(self, lo, hi, shape):
        return jax.random.randint(self._next(), shape, lo, hi, dtype=jnp.int32)

    def uniform(self, shape, lo=0.0, hi=1.0):
        return jax.random.uniform(self._next(), shape, jnp.bfloat16, lo, hi)

    def permutation(self, n):
        return jax.random.permutation(self._next(), n)
kernel_name = 'adaLN_cond__compressed_kv_cla__mixer_s_mlp__prompt'

def setup_inputs():
    _rng = _Rng(jax.random.key(int.from_bytes(__import__("os").urandom(4), "little")))
    _w = lambda a: (lambda t: t.astype(jnp.bfloat16) if jnp.issubdtype(t.dtype, jnp.floating) else t)(jnp.asarray(a))

    def _A_setup():
        B, H, Sq, Sk, D, M = (1, 32, 2048, 2048, 128, 640)
        Dc = 4 * D
        return {'x': _w((lambda *s: _rng.normal(s) * 0.05)(B, Sq, M)), 'c_kv': _w((lambda *s: _rng.normal(s) * 0.05)(B, Sk, Dc)), 'w_q': _w((lambda *s: _rng.normal(s) * 0.05)(M, H, D) * M ** (-0.5)), 'w_uk': _w((lambda *s: _rng.normal(s) * 0.05)(Dc, H, D) * Dc ** (-0.5)), 'w_uv': _w((lambda *s: _rng.normal(s) * 0.05)(Dc, H, D) * Dc ** (-0.5)), 'w_o': _w((lambda *s: _rng.normal(s) * 0.05)(H, D, M) * (H * D) ** (-0.5))}
    _A_in = _A_setup()

    def _B_setup():
        B, S, D, F = (1, 2048, 640, 1728)
        return {'x': _w((lambda *s: _rng.normal(s) * 0.05)(B, S, D)), 'w1': _w((lambda *s: _rng.normal(s) * 0.05)(D, D) * D ** (-0.5)), 'w2': _w((lambda *s: _rng.normal(s) * 0.05)(D, D) * D ** (-0.5)), 'w3': _w((lambda *s: _rng.normal(s) * 0.05)(D, F) * D ** (-0.5)), 'w4': _w((lambda *s: _rng.normal(s) * 0.05)(F, D) * F ** (-0.5))}
    _B_in = _B_setup()
    return {'A_x': _A_in['x'], 'A_c_kv': _A_in['c_kv'], 'A_w_q': _A_in['w_q'], 'A_w_uk': _A_in['w_uk'], 'A_w_uv': _A_in['w_uv'], 'A_w_o': _A_in['w_o'], 'B_x': _B_in['x'], 'B_w1': _B_in['w1'], 'B_w2': _B_in['w2'], 'B_w3': _B_in['w3'], 'B_w4': _B_in['w4'], 'c': _w((lambda *s: _rng.normal(s) * 0.05)(1, 640)), 'w_mod': _w((lambda *s: _rng.normal(s) * 0.05)(640, 6 * 640) * 640 ** (-0.5))}

def reference(A_x, A_c_kv, A_w_q, A_w_uk, A_w_uv, A_w_o, B_x, B_w1, B_w2, B_w3, B_w4, c, w_mod):

    def _A_ref(x, c_kv, w_q, w_uk, w_uv, w_o):
        B, Sq, M = (x.shape[0], x.shape[1], x.shape[2])
        Sk = c_kv.shape[1]
        H, D = (w_q.shape[1], w_q.shape[2])
        q = jnp.einsum('bqm,mhd->bhqd', x, w_q)
        k = jnp.einsum('bkc,chd->bhkd', c_kv, w_uk)
        v = jnp.einsum('bkc,chd->bhkd', c_kv, w_uv)
        scores = jnp.einsum('bhqd,bhkd->bhqk', q, k) * D ** (-0.5)
        off = Sk - Sq
        qi = jnp.arange(Sq)[:, None]
        kj = jnp.arange(Sk)[None, :]
        cmask = kj <= qi + off
        scores = jnp.where(cmask[None, None], scores, -1000000000.0)
        p = _softmax(scores, axis=-1)
        ctx = jnp.einsum('bhqk,bhkd->bhqd', p, v)
        return jnp.einsum('bhqd,hdm->bqm', ctx, w_o)

    def _B_ref(x, w1, w2, w3, w4):
        B, S, D = x.shape
        h = _gelu(_layernorm(x, axis=-1) @ w1)
        c = D // 4
        g0 = jnp.pad(h[:, :, 0 * c:1 * c], ((0, 0), (1, 0), (0, 0)))[:, :S, :]
        g1 = jnp.pad(h[:, :, 1 * c:2 * c], ((0, 0), (0, 1), (0, 0)))[:, 1:, :]
        g2 = jnp.pad(h[:, :, 2 * c:3 * c], ((0, 0), (2, 0), (0, 0)))[:, :S, :]
        g3 = jnp.pad(h[:, :, 3 * c:], ((0, 0), (0, 2), (0, 0)))[:, 2:, :]
        hs = jnp.concatenate([g0, g1, g2, g3], axis=-1) @ w2
        x1 = x + hs
        h2 = _gelu(_layernorm(x1, axis=-1) @ w3) @ w4
        return x1 + h2
    x = A_x
    mod = (_silu(c) @ w_mod).reshape(c.shape[0], 6, 1, -1)
    sa, ca, ga, sb, cb, gb = (mod[:, 0].copy(), mod[:, 1].copy(), mod[:, 2].copy(), mod[:, 3].copy(), mod[:, 4].copy(), mod[:, 5].copy())
    h = _layernorm(x, axis=-1) * (1 + ca) + sa
    x = x + ga * _A_ref(h, A_c_kv, A_w_q, A_w_uk, A_w_uv, A_w_o)
    h = _layernorm(x, axis=-1) * (1 + cb) + sb
    x = x + gb * _B_ref(h, B_w1, B_w2, B_w3, B_w4)
    return x
```

```python
import functools
import math
import os

import jax
import jax.numpy as jnp
import jax.experimental.pallas as pl
import jax.experimental.pallas.tpu as pltpu

F32 = jnp.float32
BF16 = jnp.bfloat16
U32 = jnp.uint32
NT = (((1,), (1,)), ((), ()))
T = 128
EPS = 1e-5

LAG_M = int(os.environ.get('LAG_M', 10))
GRP = int(os.environ.get('GRP', 4))
LEAD = int(os.environ.get('LEAD', 12))
PROW = int(os.environ.get('PROW', 0))
LVAR = int(os.environ.get('LVAR', 3))


def _dot(a, b):
    return jnp.dot(a, b, preferred_element_type=F32)


def _dot_nt(a, b):
    return jax.lax.dot_general(a, b, NT, preferred_element_type=F32)


def _ln(x):
    m = jnp.mean(x, axis=-1, keepdims=True)
    xc = x - m
    v = jnp.mean(xc * xc, axis=-1, keepdims=True)
    return xc * jax.lax.rsqrt(v + EPS)


def _gelu(x):
    c0 = math.sqrt(2.0 / math.pi)
    return 0.5 * x * (1.0 + jnp.tanh(c0 * (x + 0.044715 * (x * x * x))))


def _tie(x, dep):
    xu = pltpu.bitcast(x, U32)
    first = jnp.where(dep > jnp.inf, jnp.uint32(0), xu[:8])
    return pltpu.bitcast(jnp.concatenate([first, xu[8:]], axis=0), BF16)


def _unpack_pair(wu):
    lo = pltpu.bitcast(wu << 16, F32)
    hi = pltpu.bitcast(wu & jnp.uint32(0xFFFF0000), F32)
    return lo, hi


def _ld(ref, *idx):
    return pltpu.bitcast(ref[idx], BF16)


def _pk(x):
    return pltpu.bitcast(x, U32)


def _attention_step(h_scr, c_scr, wq_ref, wuk_ref, wuv_ref, wo_ref, acc_scr,
                    w_scr, q_scr, k_scr, v_scr, s_scr,
                    *, S, M, Dc, H, scale, neg):
    nb = S // T
    km, kc = M // T, Dc // T
    T2 = T // 2
    for j in range(kc):
        for hd, w in enumerate(_unpack_pair(wuk_ref[j * T:(j + 1) * T, :])):
            w_scr[hd, km + j] = _pk(w.astype(BF16))
    for j in range(km):
        for hd, w in enumerate(_unpack_pair(wq_ref[j * T:(j + 1) * T, :])):
            w_scr[hd, j] = _pk(w.astype(BF16))
    for j in range(kc):
        for hd, w in enumerate(_unpack_pair(wuv_ref[j * T:(j + 1) * T, :])):
            w_scr[hd, km + kc + j] = _pk(w.astype(BF16).T)
    for hd in range(2):
        for j in range(km):
            w_scr[hd, km + 2 * kc + j] = _pk(wo_ref[hd * T:(hd + 1) * T, j * T:(j + 1) * T])

    tri = (jax.lax.broadcasted_iota(jnp.int32, (T, T), 0)
           <= jax.lax.broadcasted_iota(jnp.int32, (T, T), 1))

    mx = {}; mfin = {}; lsum = {}; o = {}
    part = {}
    st = dict(n=0)
    pend = []
    NS = s_scr.shape[0]
    NQ = q_scr.shape[0]

    def lhs(x, extra=None):
        deps = [] if extra is None else [extra]
        while LAG_M and pend and pend[0][0] + LAG_M <= st['n']:
            d = pend.pop(0)
            if pend and pend[0][0] + LAG_M <= st['n'] and pend[0][2] == d[2]:
                continue
            deps.append(d[1])
        st['n'] += 1
        if not deps:
            return x
        z = deps[0]
        for d in deps[1:]:
            z = jnp.maximum(z, d)
        return _tie(x, z)

    res = []

    def rec(v):
        res.append(v)
        return v

    def accum(key, val):
        rec(val)
        part[key] = val if key not in part else val + part[key]
        return part[key]

    def job_q(u, j):
        r, hd = divmod(u, 2)
        v = accum(('q', u), _dot(lhs(_ld(h_scr, r, j)), _ld(w_scr, hd, j)))
        if j == km - 1:
            q_scr[u % NQ] = _pk((v * scale).astype(BF16))

    def job_k(u, j):
        r, hd = divmod(u, 2)
        v = accum(('k', u), _dot(lhs(_ld(c_scr, r, j)), _ld(w_scr, hd, km + j)))
        if j == kc - 1:
            k_scr[u] = _pk(v.astype(BF16))

    def job_v(u, j):
        r, hd = divmod(u, 2)
        v = accum(('v', u), _dot_nt(lhs(_ld(w_scr, hd, km + kc + j)), _ld(c_scr, r, j)))
        if j == kc - 1:
            v_scr[u] = _pk(v.astype(BF16))

    def job_a(u, cidx):
        r, hd = divmod(u, 2)
        n = st['n']
        s = rec(_dot_nt(lhs(_ld(k_scr, 2 * cidx + hd)), _ld(q_scr, u % NQ)))
        if cidx == r:
            s = jnp.where(tri, s, neg)
        s_scr[u % NS, cidx] = s
        pm = jnp.max(s.reshape(T // 8, 8, T), axis=0)
        mx[u] = pm if u not in mx else jnp.maximum(mx[u], pm)
        pend.append((n, mx[u], u))

    def job_b(u, cidx):
        r, hd = divmod(u, 2)
        if u not in mfin:
            mfin[u] = jnp.broadcast_to(jnp.max(mx[u], axis=0, keepdims=True), (8, T))
        m = mfin[u]
        if LEAD and st['n'] >= LEAD:
            assert len(res) == st['n']
            r0 = 8 * (PROW * (cidx % 4) % 16)
            src = res[st['n'] - LEAD][r0:r0 + 8, :]
            m = jnp.where(src > jnp.inf, src, m)
        p = jnp.exp2(s_scr[u % NS, cidx].reshape(T // 8, 8, T) - m[None])
        if LVAR in (2, 4):
            ls = lsum.get(u)
            for i in range(T // 8):
                ls = p[i] if ls is None else ls + p[i]
            lsum[u] = ls
        else:
            ls = jnp.sum(p, axis=0)
            lsum[u] = ls if u not in lsum else lsum[u] + ls
        if LVAR == 0:
            ls = lsum[u]
        if LVAR == 3:
            ls = None
        if LVAR == 4:
            last = jnp.where(ls > jnp.inf, 0.0, p[T // 8 - 1])
            p = jnp.concatenate([p[:T // 8 - 1], last[None]], axis=0)
            ls = None
        pb = p.reshape(T, T).astype(BF16)
        v = accum(('o', u), _dot(lhs(_ld(v_scr, 2 * cidx + hd), ls), pb))
        if cidx == r:
            l = jnp.sum(lsum[u], axis=0, keepdims=True)
            o[u] = (v * (1.0 / l)).astype(BF16).T

    def job_o(u, j):
        r, hd = divmod(u, 2)
        v = rec(_dot(lhs(o[u]), _ld(w_scr, hd, km + 2 * kc + j)))
        acc_scr[r * T:(r + 1) * T, j * T:(j + 1) * T] += v

    nu = 2 * nb
    for slot in range(-2, nu + 1):
        A = [(job_a, slot + 1, c) for c in range((slot + 1) // 2 + 1)] if 0 <= slot + 1 < nu else []
        B = [(job_b, slot, c) for c in range(slot // 2 + 1)] if 0 <= slot < nu else []
        Fj = []
        if slot + 2 < nu:
            Fj += [(job_q, slot + 2, j) for j in range(km)]
            Fj += [(job_k, slot + 2, j) for j in range(kc)]
            Fj += [(job_v, slot + 2, j) for j in range(kc)]
        if slot - 1 >= 0:
            Fj += [(job_o, slot - 1, j) for j in range(km)]
        if slot == -1:
            seq = Fj + A
        else:
            seq = []
            while A or B:
                seq += A[:GRP]; A = A[GRP:]
                seq += B[:GRP]; B = B[GRP:]
            seq += Fj
        for fn, u, j in seq:
            fn(u, j)


def _kernel(x_ref, c_ref, wq_ref, wuk_ref, wuv_ref, wo_ref, w1_ref, w2_ref, w3_ref, w4_ref,
            cond_ref, wmod_ref, out_ref,
            h_scr, acc_scr, mod_scr, x1_scr, hb_scr, t_scr, wq_buf, wk_buf, wv_buf, wsem,
            c_scr, w_scr, q_scr, k_scr, v_scr, s_scr,
            *, S, M, Dc, H, D, RB):
    step = pl.program_id(0)
    nattn = H // 2
    scale = float(D) ** -0.5 * math.log2(math.e)
    neg = -1e9 * math.log2(math.e)
    nrb = S // RB

    def wcopies(g, slot):
        return [pltpu.make_async_copy(src.bitcast(U32).at[:, g, :], dst.at[slot], wsem.at[slot, j])
                for j, (src, dst) in enumerate(((wuk_ref, wk_buf), (wuv_ref, wv_buf), (wq_ref, wq_buf)))]

    @pl.when(step == 0)
    def _():
        for cp in wcopies(0, 0):
            cp.start()
        cf = cond_ref[...].astype(F32)
        sc = (cf * jax.nn.sigmoid(cf)).astype(BF16)
        mod_scr[...] = _dot(jnp.broadcast_to(sc, (8, M)), wmod_ref[...])
        sa = mod_scr[0:1, 0:M]
        ca = mod_scr[0:1, M:2 * M]

        def body(r, carry):
            rows = pl.ds(pl.multiple_of(r * T, T), T)
            hh = (_ln(x_ref[rows, :].astype(F32)) * (1.0 + ca) + sa).astype(BF16)
            for j in range(M // T):
                h_scr[r, j] = _pk(hh[:, j * T:(j + 1) * T])
            for j in range(Dc // T):
                c_scr[r, j] = _pk(c_ref[rows, j * T:(j + 1) * T])
            acc_scr[rows, :] = jnp.zeros((T, M), F32)
            return carry

        jax.lax.fori_loop(0, S // T, body, 0)

    @pl.when(step < nattn)
    def _():
        slot = step % 2

        @pl.when(step + 1 < nattn)
        def _():
            for cp in wcopies(step + 1, 1 - slot):
                cp.start()

        for cp in wcopies(step, slot):
            cp.wait()
        _attention_step(h_scr, c_scr, wq_buf.at[slot], wk_buf.at[slot], wv_buf.at[slot], wo_ref, acc_scr,
                        w_scr, q_scr, k_scr, v_scr, s_scr,
                        S=S, M=M, Dc=Dc, H=H, scale=scale, neg=neg)

    @pl.when(step == nattn)
    def _():
        ga = mod_scr[0:1, 2 * M:3 * M]
        sb = mod_scr[0:1, 3 * M:4 * M]
        cb = mod_scr[0:1, 4 * M:5 * M]
        t_scr[0:8, :] = jnp.zeros((8, M), F32)
        t_scr[S + 8:S + 16, :] = jnp.zeros((8, M), F32)

        def body(r, carry):
            rows = pl.ds(pl.multiple_of(r * RB, RB), RB)
            x1 = x_ref[rows, :].astype(F32) + ga * acc_scr[rows, :]
            x1_scr[rows, :] = x1
            hb = _ln(x1) * (1.0 + cb) + sb
            hb_scr[rows, :] = hb
            t_scr[pl.ds(pl.multiple_of(r * RB + 8, 8), RB), :] = _gelu(_dot(_ln(hb).astype(BF16), w1_ref[...]))
            return carry

        jax.lax.fori_loop(0, nrb, body, 0)

    @pl.when(step > nattn)
    def _():
        gb = mod_scr[0:1, 5 * M:6 * M]
        r0 = pl.multiple_of((step - nattn - 1) * RB, RB)
        cq = M // 4
        col = jax.lax.broadcasted_iota(jnp.int32, (RB, M), 1)
        blk = t_scr[pl.ds(r0, RB + 16), :]
        tm1 = blk[7:7 + RB]
        tp1 = blk[9:9 + RB]
        tm2 = blk[6:6 + RB]
        tp2 = blk[10:10 + RB]
        sh = jnp.where(col < 2 * cq, jnp.where(col < cq, tm1, tp1), jnp.where(col < 3 * cq, tm2, tp2))
        y1 = hb_scr[pl.ds(r0, RB), :] + _dot(sh.astype(BF16), w2_ref[...])
        h3 = _gelu(_dot_nt(_ln(y1).astype(BF16), w3_ref[...]))
        y2 = y1 + _dot(h3.astype(BF16), w4_ref[...])
        out_ref[...] = (x1_scr[pl.ds(r0, RB), :] + gb * y2).astype(out_ref.dtype)


@jax.jit
def pallas_adaLN_cond__compressed_kv_cla__mixer_s_mlp__prompt_kernel(
    A_x: jax.Array,
    A_c_kv: jax.Array,
    A_w_q: jax.Array,
    A_w_uk: jax.Array,
    A_w_uv: jax.Array,
    A_w_o: jax.Array,
    B_x: jax.Array,
    B_w1: jax.Array,
    B_w2: jax.Array,
    B_w3: jax.Array,
    B_w4: jax.Array,
    c: jax.Array,
    w_mod: jax.Array,
):
    _, S, M = A_x.shape
    Dc = A_c_kv.shape[2]
    H, D = A_w_q.shape[1], A_w_q.shape[2]
    Fd = B_w3.shape[1]
    RB = int(os.environ.get('RB', 256))
    nattn = H // 2
    nrb = S // RB
    full = lambda shp: pl.BlockSpec(shp, lambda i: (0,) * len(shp))
    out = pl.pallas_call(
        functools.partial(_kernel, S=S, M=M, Dc=Dc, H=H, D=D, RB=RB),
        grid=(nattn + 1 + nrb,),
        in_specs=[
            full((S, M)), full((S, Dc)),
            pl.BlockSpec(memory_space=pltpu.HBM), pl.BlockSpec(memory_space=pltpu.HBM),
            pl.BlockSpec(memory_space=pltpu.HBM),
            pl.BlockSpec((2 * D, M), lambda i: (jnp.minimum(i, nattn - 1), 0)),
            full((M, M)), full((M, M)), full((Fd, M)), full((Fd, M)),
            full((1, M)), full((M, 6 * M)),
        ],
        out_specs=pl.BlockSpec((RB, M), lambda i: (jnp.maximum(i - nattn - 1, 0), 0)),
        out_shape=jax.ShapeDtypeStruct((S, M), A_x.dtype),
        scratch_shapes=[
            pltpu.VMEM((S // T, M // T, T // 2, T), U32),
            pltpu.VMEM((S, M), F32),
            pltpu.VMEM((8, 6 * M), F32),
            pltpu.VMEM((S, M), F32),
            pltpu.VMEM((S, M), F32),
            pltpu.VMEM((S + 16, M), F32),
            pltpu.VMEM((2, M, D), U32),
            pltpu.VMEM((2, Dc, D), U32),
            pltpu.VMEM((2, Dc, D), U32),
            pltpu.SemaphoreType.DMA((2, 3)),
            pltpu.VMEM((S // T, Dc // T, T // 2, T), U32),
            pltpu.VMEM((2, 2 * (M // T) + 2 * (Dc // T), T // 2, T), U32),
            pltpu.VMEM((4, T // 2, T), U32),
            pltpu.VMEM((2 * S // T, T // 2, T), U32),
            pltpu.VMEM((2 * S // T, T // 2, T), U32),
            pltpu.VMEM((4, S // T, T, T), F32),
        ],
        compiler_params=pltpu.CompilerParams(
            dimension_semantics=("arbitrary",),
            vmem_limit_bytes=120 * 1024 * 1024,
        ),
    )(
        A_x.reshape(S, M), A_c_kv.reshape(S, Dc),
        A_w_q, A_w_uk, A_w_uv,
        A_w_o.reshape(H * D, M),
        B_w1, B_w2, B_w3.T, B_w4, c, w_mod,
    )
    return out.reshape(1, S, M)
```

```python
import functools
import math
import os

import jax
import jax.numpy as jnp
import jax.experimental.pallas as pl
import jax.experimental.pallas.tpu as pltpu

F32 = jnp.float32
BF16 = jnp.bfloat16
U32 = jnp.uint32
NT = (((1,), (1,)), ((), ()))
T = 128
EPS = 1e-5

LAG_M = int(os.environ.get('LAG_M', 0))
GRP = int(os.environ.get('GRP', 4))
LEAD = int(os.environ.get('LEAD', 12))
PROW = int(os.environ.get('PROW', 0))
VXP = int(os.environ.get('VXP', 0))
VT = int(os.environ.get('VT', 8))
RES = int(os.environ.get('RES', 5))
LAT_Q = int(os.environ.get('LAT_Q', 12))
LAT_K = int(os.environ.get('LAT_K', 10))
LAT_A = int(os.environ.get('LAT_A', 16))
LAT_B = int(os.environ.get('LAT_B', 14))
LNR = int(os.environ.get('LNR', 128))
LVAR = int(os.environ.get('LVAR', 3))


def _dot(a, b):
    return jnp.dot(a, b, preferred_element_type=F32)


def _dot_nt(a, b):
    return jax.lax.dot_general(a, b, NT, preferred_element_type=F32)


def _ln(x):
    m = jnp.mean(x, axis=-1, keepdims=True)
    xc = x - m
    v = jnp.mean(xc * xc, axis=-1, keepdims=True)
    return xc * jax.lax.rsqrt(v + EPS)


def _gelu(x):
    c0 = math.sqrt(2.0 / math.pi)
    return 0.5 * x * (1.0 + jnp.tanh(c0 * (x + 0.044715 * (x * x * x))))


def _tie(x, dep):
    xu = pltpu.bitcast(x, U32)
    first = jnp.where(dep > jnp.inf, jnp.uint32(0), xu[:8])
    return pltpu.bitcast(jnp.concatenate([first, xu[8:]], axis=0), BF16)


def _unpack_pair(wu):
    lo = pltpu.bitcast(wu << 16, F32)
    hi = pltpu.bitcast(wu & jnp.uint32(0xFFFF0000), F32)
    return lo, hi


def _ld(ref, *idx):
    return pltpu.bitcast(ref[idx], BF16)


def _pk(x):
    return pltpu.bitcast(x, U32)


def _attention_step(h_scr, c_scr, wq_ref, wuk_ref, wuv_ref, wo_ref, acc_scr,
                    w_scr, q_scr, k_scr, v_scr, s_scr,
                    *, S, M, Dc, H, scale, neg):
    nb = S // T
    km, kc = M // T, Dc // T
    T2 = T // 2
    for j in range(kc):
        for hd, w in enumerate(_unpack_pair(wuk_ref[j * T:(j + 1) * T, :])):
            w_scr[hd, km + j] = _pk(w.astype(BF16))
    for j in range(km):
        for hd, w in enumerate(_unpack_pair(wq_ref[j * T:(j + 1) * T, :])):
            w_scr[hd, j] = _pk(w.astype(BF16))
    for j in range(kc):
        for hd, w in enumerate(_unpack_pair(wuv_ref[j * T:(j + 1) * T, :])):
            w_scr[hd, km + kc + j] = _pk(w.astype(BF16) if VXP else w.astype(BF16).T)
    for hd in range(2):
        for j in range(km):
            w_scr[hd, km + 2 * kc + j] = _pk(wo_ref[hd * T:(hd + 1) * T, j * T:(j + 1) * T])

    tri = (jax.lax.broadcasted_iota(jnp.int32, (T, T), 0)
           <= jax.lax.broadcasted_iota(jnp.int32, (T, T), 1))

    mx = {}; mfin = {}; lsum = {}; o = {}
    part = {}
    st = dict(n=0)
    pend = []
    NS = s_scr.shape[0]
    NQ = q_scr.shape[0]

    def lhs(x, extra=None):
        deps = [] if extra is None else [extra]
        while LAG_M and pend and pend[0][0] + LAG_M <= st['n']:
            d = pend.pop(0)
            if pend and pend[0][0] + LAG_M <= st['n'] and pend[0][2] == d[2]:
                continue
            deps.append(d[1])
        st['n'] += 1
        if not deps:
            return x
        z = deps[0]
        for d in deps[1:]:
            z = jnp.maximum(z, d)
        return _tie(x, z)

    res = []

    def rec(v):
        res.append(v)
        return v

    def accum(key, val):
        rec(val)
        part[key] = val if key not in part else val + part[key]
        return part[key]

    def job_q(u, j):
        r, hd = divmod(u, 2)
        v = accum(('q', u), _dot(lhs(_ld(h_scr, r, j)), _ld(w_scr, hd, j)))
        if j == km - 1:
            q_scr[u % NQ] = _pk((v * scale).astype(BF16))

    def job_k(u, j):
        r, hd = divmod(u, 2)
        v = accum(('k', u), _dot(lhs(_ld(c_scr, r, j)), _ld(w_scr, hd, km + j)))
        if j == kc - 1:
            k_scr[u] = _pk(v.astype(BF16))

    def job_v(u, j):
        r, hd = divmod(u, 2)
        if VXP:
            v = accum(('v', u), _dot(lhs(_ld(c_scr, r, j)), _ld(w_scr, hd, km + kc + j)))
        else:
            ex = res[st['n'] - VT][0:8, :] if VT and st['n'] >= VT else None
            v = accum(('v', u), _dot_nt(lhs(_ld(w_scr, hd, km + kc + j), ex), _ld(c_scr, r, j)))
        if j == kc - 1:
            v_scr[u] = _pk(v.astype(BF16).T if VXP else v.astype(BF16))

    def job_a(u, cidx):
        r, hd = divmod(u, 2)
        n = st['n']
        s = rec(_dot_nt(lhs(_ld(k_scr, 2 * cidx + hd)), _ld(q_scr, u % NQ)))
        if cidx == r:
            s = jnp.where(tri, s, neg)
        s_scr[u % NS, cidx] = s
        pm = jnp.max(s.reshape(T // 8, 8, T), axis=0)
        mx[u] = pm if u not in mx else jnp.maximum(mx[u], pm)
        pend.append((n, mx[u], u))

    def job_b(u, cidx):
        r, hd = divmod(u, 2)
        if u not in mfin:
            mfin[u] = jnp.broadcast_to(jnp.max(mx[u], axis=0, keepdims=True), (8, T))
        m = mfin[u]
        if LEAD and st['n'] >= LEAD:
            assert len(res) == st['n']
            r0 = 8 * (PROW * (cidx % 4) % 16)
            src = res[st['n'] - LEAD][r0:r0 + 8, :]
            m = jnp.where(src > jnp.inf, src, m)
        p = jnp.exp2(s_scr[u % NS, cidx].reshape(T // 8, 8, T) - m[None])
        if LVAR in (2, 4):
            ls = lsum.get(u)
            for i in range(T // 8):
                ls = p[i] if ls is None else ls + p[i]
            lsum[u] = ls
        else:
            ls = jnp.sum(p, axis=0)
            lsum[u] = ls if u not in lsum else lsum[u] + ls
        if LVAR == 0:
            ls = lsum[u]
        if LVAR == 3:
            ls = None
        if LVAR == 4:
            last = jnp.where(ls > jnp.inf, 0.0, p[T // 8 - 1])
            p = jnp.concatenate([p[:T // 8 - 1], last[None]], axis=0)
            ls = None
        pb = p.reshape(T, T).astype(BF16)
        v = accum(('o', u), _dot(lhs(_ld(v_scr, 2 * cidx + hd), ls), pb))
        if cidx == r:
            l = jnp.sum(lsum[u], axis=0, keepdims=True)
            o[u] = (v * (1.0 / l)).astype(BF16).T

    def job_o(u, j):
        r, hd = divmod(u, 2)
        v = rec(_dot(lhs(o[u]), _ld(w_scr, hd, km + 2 * kc + j)))
        acc_scr[r * T:(r + 1) * T, j * T:(j + 1) * T] += v

    fns = dict(q=job_q, k=job_k, v=job_v, a=job_a, b=job_b, o=job_o)
    for kind, u, j in _job_order(nb, km, kc):
        fns[kind](u, j)


def _job_order(nb, km, kc):
    nu = 2 * nb
    nominal = []
    tail = []
    for slot in range(-2, nu + 1):
        A = [('a', slot + 1, c) for c in range((slot + 1) // 2 + 1)] if 0 <= slot + 1 < nu else []
        B = [('b', slot, c) for c in range(slot // 2 + 1)] if 0 <= slot < nu else []
        Fj = []
        if slot + 2 < nu:
            Fj += [('q', slot + 2, j) for j in range(km)]
            Fj += [('k', slot + 2, j) for j in range(kc)]
            Fj += [('v', slot + 2, j) for j in range(kc)]
        if slot - 1 >= 0:
            oj = [('o', slot - 1, j) for j in range(km)]
            if slot - 1 >= nu - 1 - RES:
                tail += oj
            else:
                Fj += oj
        while A or B:
            nominal += A[:GRP]; A = A[GRP:]
            nominal += B[:GRP]; B = B[GRP:]
        nominal += Fj
    nominal += tail
    last = dict(q=km - 1, k=kc - 1, v=kc - 1)
    done = {}

    def ready_at(job):
        kind, u, j = job
        hd = u % 2
        if kind == 'a':
            deps = [(('q', u), LAT_Q), (('k', 2 * j + hd), LAT_K)]
        elif kind == 'b':
            deps = [(('a', u), LAT_A), (('v', 2 * j + hd), LAT_K)]
        elif kind == 'o':
            deps = [(('b', u), LAT_B)]
        else:
            deps = []
        t = 0
        for key, lat in deps:
            if key not in done:
                return None
            t = max(t, done[key] + lat)
        return t

    order = []
    while nominal:
        n = len(order)
        seen = set()
        pick = None
        best = None
        for i, job in enumerate(nominal):
            cls = 'p' if job[0] in 'qkv' else job[0]
            if cls in seen:
                continue
            seen.add(cls)
            t = ready_at(job)
            if t is not None and t <= n:
                pick = i
                break
            if t is not None and (best is None or t < best[0]):
                best = (t, i)
            if len(seen) == 4:
                break
        if pick is None:
            pick = best[1]
        job = nominal.pop(pick)
        order.append(job)
        kind, u, j = job
        if j == last.get(kind, u // 2):
            done[(kind, u)] = n
    return order


def _kernel(x_hbm, c_hbm, wq_hbm, wuk_hbm, wuv_hbm, wo_hbm, w1_hbm, w2_hbm, w3_hbm, w4_hbm,
            cond_hbm, wmod_hbm, out_ref,
            h_scr, acc_scr, mod_scr, x1_scr, hb_scr, t_scr, wq_buf, wk_buf, wv_buf, wo_buf, wsem,
            c_scr, w_scr, q_scr, k_scr, v_scr, s_scr,
            x_ref, c_ref, cond_ref, wma_ref, wmb_ref, w1_ref, w2_ref, w3_ref, w4_ref, sem,
            *, S, M, Dc, H, D, RB):
    step = pl.program_id(0)
    nattn = H // 2
    scale = float(D) ** -0.5 * math.log2(math.e)
    neg = -1e9 * math.log2(math.e)
    nrb = S // RB
    NX = 4
    XR = S // NX

    def wcopies(g, slot):
        cps = [pltpu.make_async_copy(src.bitcast(U32).at[:, g, :], dst.at[slot], wsem.at[slot, j])
               for j, (src, dst) in enumerate(((wq_hbm, wq_buf), (wuk_hbm, wk_buf), (wuv_hbm, wv_buf)))]
        cps.append(pltpu.make_async_copy(wo_hbm.at[g], wo_buf.at[slot], wsem.at[slot, 3]))
        return cps

    cp_cond = pltpu.make_async_copy(cond_hbm, cond_ref, sem.at[0])
    cp_wma = pltpu.make_async_copy(wmod_hbm.at[:, 0:2 * M], wma_ref, sem.at[1])
    cp_c = pltpu.make_async_copy(c_hbm, c_ref, sem.at[2])
    cp_late = [pltpu.make_async_copy(src, dst, sem.at[3 + j]) for j, (src, dst) in enumerate((
        (wmod_hbm.at[:, 2 * M:6 * M], wmb_ref), (w1_hbm, w1_ref), (w2_hbm, w2_ref),
        (w3_hbm, w3_ref), (w4_hbm, w4_ref)))]
    cp_x = [pltpu.make_async_copy(x_hbm.at[i * XR:(i + 1) * XR, :], x_ref.at[i * XR:(i + 1) * XR, :],
                                  sem.at[8 + i]) for i in range(NX)]

    def silu_cond():
        cf = cond_ref[...].astype(F32)
        return jnp.broadcast_to((cf * jax.nn.sigmoid(cf)).astype(BF16), (8, M))

    @pl.when(step == 0)
    def _():
        cp_cond.start()
        cp_wma.start()
        for cp in cp_x:
            cp.start()
        cp_c.start()
        for cp in wcopies(0, 0):
            cp.start()

        def zero(r, carry):
            acc_scr[pl.ds(pl.multiple_of(r * T, T), T), :] = jnp.zeros((T, M), F32)
            return carry

        jax.lax.fori_loop(0, S // T, zero, 0)
        cp_cond.wait()
        cp_wma.wait()
        mod_scr[:, 0:2 * M] = _dot(silu_cond(), wma_ref[...])
        sa = mod_scr[0:1, 0:M]
        ca = mod_scr[0:1, M:2 * M]

        def body(r, carry):
            rows = pl.ds(pl.multiple_of(r * LNR, LNR), LNR)
            hh = (_ln(x_ref[rows, :].astype(F32)) * (1.0 + ca) + sa).astype(BF16)
            for i in range(LNR // T):
                for j in range(M // T):
                    h_scr[r * (LNR // T) + i, j] = _pk(hh[i * T:(i + 1) * T, j * T:(j + 1) * T])
            return carry

        for i in range(NX):
            cp_x[i].wait()
            jax.lax.fori_loop(i * (XR // LNR), (i + 1) * (XR // LNR), body, 0)

        cp_c.wait()

        def cbody(r, carry):
            rows = pl.ds(pl.multiple_of(r * T, T), T)
            for j in range(Dc // T):
                c_scr[r, j] = _pk(c_ref[rows, j * T:(j + 1) * T])
            return carry

        jax.lax.fori_loop(0, S // T, cbody, 0)

    @pl.when(step == 1)
    def _():
        for cp in cp_late:
            cp.start()

    @pl.when(step < nattn)
    def _():
        slot = step % 2
        for cp in wcopies(step, slot):
            cp.wait()

        @pl.when(step + 1 < nattn)
        def _():
            for cp in wcopies(step + 1, 1 - slot):
                cp.start()

        _attention_step(h_scr, c_scr, wq_buf.at[slot], wk_buf.at[slot], wv_buf.at[slot],
                        wo_buf.at[slot], acc_scr,
                        w_scr, q_scr, k_scr, v_scr, s_scr,
                        S=S, M=M, Dc=Dc, H=H, scale=scale, neg=neg)

    @pl.when(step == nattn)
    def _():
        for cp in cp_late:
            cp.wait()
        mod_scr[:, 2 * M:6 * M] = _dot(silu_cond(), wmb_ref[...])
        ga = mod_scr[0:1, 2 * M:3 * M]
        sb = mod_scr[0:1, 3 * M:4 * M]
        cb = mod_scr[0:1, 4 * M:5 * M]
        t_scr[0:8, :] = jnp.zeros((8, M), F32)
        t_scr[S + 8:S + 16, :] = jnp.zeros((8, M), F32)

        def body(r, carry):
            rows = pl.ds(pl.multiple_of(r * RB, RB), RB)
            x1 = x_ref[rows, :].astype(F32) + ga * acc_scr[rows, :]
            x1_scr[rows, :] = x1
            hb = _ln(x1) * (1.0 + cb) + sb
            hb_scr[rows, :] = hb
            t_scr[pl.ds(pl.multiple_of(r * RB + 8, 8), RB), :] = _gelu(_dot(_ln(hb).astype(BF16), w1_ref[...]))
            return carry

        jax.lax.fori_loop(0, nrb, body, 0)

    @pl.when(step > nattn)
    def _():
        gb = mod_scr[0:1, 5 * M:6 * M]
        r0 = pl.multiple_of((step - nattn - 1) * RB, RB)
        cq = M // 4
        col = jax.lax.broadcasted_iota(jnp.int32, (RB, M), 1)
        blk = t_scr[pl.ds(r0, RB + 16), :]
        tm1 = blk[7:7 + RB]
        tp1 = blk[9:9 + RB]
        tm2 = blk[6:6 + RB]
        tp2 = blk[10:10 + RB]
        sh = jnp.where(col < 2 * cq, jnp.where(col < cq, tm1, tp1), jnp.where(col < 3 * cq, tm2, tp2))
        y1 = hb_scr[pl.ds(r0, RB), :] + _dot(sh.astype(BF16), w2_ref[...])
        h3 = _gelu(_dot_nt(_ln(y1).astype(BF16), w3_ref[...]))
        y2 = y1 + _dot(h3.astype(BF16), w4_ref[...])
        out_ref[...] = (x1_scr[pl.ds(r0, RB), :] + gb * y2).astype(out_ref.dtype)


@jax.jit
def pallas_adaLN_cond__compressed_kv_cla__mixer_s_mlp__prompt_kernel(
    A_x: jax.Array,
    A_c_kv: jax.Array,
    A_w_q: jax.Array,
    A_w_uk: jax.Array,
    A_w_uv: jax.Array,
    A_w_o: jax.Array,
    B_x: jax.Array,
    B_w1: jax.Array,
    B_w2: jax.Array,
    B_w3: jax.Array,
    B_w4: jax.Array,
    c: jax.Array,
    w_mod: jax.Array,
):
    _, S, M = A_x.shape
    Dc = A_c_kv.shape[2]
    H, D = A_w_q.shape[1], A_w_q.shape[2]
    Fd = B_w3.shape[1]
    RB = int(os.environ.get('RB', 256))
    nattn = H // 2
    nrb = S // RB
    out = pl.pallas_call(
        functools.partial(_kernel, S=S, M=M, Dc=Dc, H=H, D=D, RB=RB),
        grid=(nattn + 1 + nrb,),
        in_specs=[pl.BlockSpec(memory_space=pltpu.HBM)] * 12,
        out_specs=pl.BlockSpec((RB, M), lambda i: (jnp.maximum(i - nattn - 1, 0), 0)),
        out_shape=jax.ShapeDtypeStruct((S, M), A_x.dtype),
        scratch_shapes=[
            pltpu.VMEM((S // T, M // T, T // 2, T), U32),
            pltpu.VMEM((S, M), F32),
            pltpu.VMEM((8, 6 * M), F32),
            pltpu.VMEM((S, M), F32),
            pltpu.VMEM((S, M), F32),
            pltpu.VMEM((S + 16, M), F32),
            pltpu.VMEM((2, M, D), U32),
            pltpu.VMEM((2, Dc, D), U32),
            pltpu.VMEM((2, Dc, D), U32),
            pltpu.VMEM((2, 2 * D, M), BF16),
            pltpu.SemaphoreType.DMA((2, 4)),
            pltpu.VMEM((S // T, Dc // T, T // 2, T), U32),
            pltpu.VMEM((2, 2 * (M // T) + 2 * (Dc // T), T // 2, T), U32),
            pltpu.VMEM((4, T // 2, T), U32),
            pltpu.VMEM((2 * S // T, T // 2, T), U32),
            pltpu.VMEM((2 * S // T, T // 2, T), U32),
            pltpu.VMEM((4, S // T, T, T), F32),
            pltpu.VMEM((S, M), BF16),
            pltpu.VMEM((S, Dc), BF16),
            pltpu.VMEM((1, M), BF16),
            pltpu.VMEM((M, 2 * M), BF16),
            pltpu.VMEM((M, 4 * M), BF16),
            pltpu.VMEM((M, M), BF16),
            pltpu.VMEM((M, M), BF16),
            pltpu.VMEM((Fd, M), BF16),
            pltpu.VMEM((Fd, M), BF16),
            pltpu.SemaphoreType.DMA((12,)),
        ],
        compiler_params=pltpu.CompilerParams(
            dimension_semantics=("arbitrary",),
            vmem_limit_bytes=100 * 1024 * 1024,
        ),
    )(
        A_x.reshape(S, M), A_c_kv.reshape(S, Dc),
        A_w_q, A_w_uk, A_w_uv,
        A_w_o.reshape(H // 2, 2 * D, M),
        B_w1, B_w2, B_w3.T, B_w4, c, w_mod,
    )
    return out.reshape(1, S, M)
```

```python
import functools
import math
import os

import jax
import jax.numpy as jnp
import jax.experimental.pallas as pl
import jax.experimental.pallas.tpu as pltpu

F32 = jnp.float32
BF16 = jnp.bfloat16
U32 = jnp.uint32
NT = (((1,), (1,)), ((), ()))
T = 128
EPS = 1e-5

GRP = int(os.environ.get('GRP', 4))
LEAD = int(os.environ.get('LEAD', 10))
PROW = int(os.environ.get('PROW', 3))
VT = int(os.environ.get('VT', 8))
RES = int(os.environ.get('RES', 5))
LAT_Q = int(os.environ.get('LAT_Q', 12))
LAT_K = int(os.environ.get('LAT_K', 10))
LAT_A = int(os.environ.get('LAT_A', 16))
LAT_B = int(os.environ.get('LAT_B', 14))
LNR = int(os.environ.get('LNR', 128))
MID = int(os.environ.get('MID', 120))
MINMASK = int(os.environ.get('MINMASK', 1))
OPAIR = int(os.environ.get('OPAIR', 0))
NSUB = int(os.environ.get('NSUB', 1))
PSUB = int(os.environ.get('PSUB', 1))


def _dot(a, b):
    return jnp.dot(a, b, preferred_element_type=F32)


def _dot_nt(a, b):
    return jax.lax.dot_general(a, b, NT, preferred_element_type=F32)


def _ln(x):
    m = jnp.mean(x, axis=-1, keepdims=True)
    xc = x - m
    v = jnp.mean(xc * xc, axis=-1, keepdims=True)
    return xc * jax.lax.rsqrt(v + EPS)


def _gelu(x):
    c0 = math.sqrt(2.0 / math.pi)
    return 0.5 * x * (1.0 + jnp.tanh(c0 * (x + 0.044715 * (x * x * x))))


def _tie(x, dep):
    xu = pltpu.bitcast(x, U32)
    first = jnp.where(dep > jnp.inf, jnp.uint32(0), xu[:8])
    return pltpu.bitcast(jnp.concatenate([first, xu[8:]], axis=0), BF16)


def _unpack_pair(wu):
    lo = pltpu.bitcast(wu << 16, F32)
    hi = pltpu.bitcast(wu & jnp.uint32(0xFFFF0000), F32)
    return lo, hi


def _ld(ref, *idx):
    return pltpu.bitcast(ref[idx], BF16)


def _pk(x):
    return pltpu.bitcast(x, U32)


def _attention_step(h_scr, c_scr, wq_ref, wuk_ref, wuv_ref, wo_ref, acc_scr, cap_ref, mid,
                    *, S, M, Dc, H, scale, neg):
    nb = S // T
    km, kc = M // T, Dc // T
    tile = lambda j: slice(j * T, (j + 1) * T)
    wq = [[w.astype(BF16) for w in _unpack_pair(wq_ref[tile(j), :])] for j in range(km)]
    wk = [[w.astype(BF16) for w in _unpack_pair(wuk_ref[tile(j), :])] for j in range(kc)]
    wvT = [[w.astype(BF16).T for w in _unpack_pair(wuv_ref[tile(j), :])] for j in range(kc)]
    if not MINMASK:
        tri = (jax.lax.broadcasted_iota(jnp.int32, (T, T), 0)
               <= jax.lax.broadcasted_iota(jnp.int32, (T, T), 1))

    q = {}; k = {}; vT = {}; sv = {}; mx = {}; mfin = {}; lsum = {}; o = {}
    part = {}
    res = []

    def accum(key, val):
        res.append(val)
        part[key] = val if key not in part else val + part[key]
        return part[key]

    def job_q(u, j):
        r, hd = divmod(u, 2)
        v = accum(('q', u), _dot(_ld(h_scr, r, j), wq[j][hd]))
        if j == km - 1:
            q[u] = (v * scale).astype(BF16)

    def job_k(u, j):
        r, hd = divmod(u, 2)
        v = accum(('k', u), _dot(_ld(c_scr, r, j), wk[j][hd]))
        if j == kc - 1:
            k[u] = v.astype(BF16)

    def job_v(u, j):
        r, hd = divmod(u, 2)
        a = wvT[j][hd]
        if VT and len(res) >= VT:
            a = _tie(a, res[len(res) - VT][0:8, :])
        v = accum(('v', u), _dot_nt(a, _ld(c_scr, r, j)))
        if j == kc - 1:
            vT[u] = v.astype(BF16)

    def job_a(u, cidx):
        r, hd = divmod(u, 2)
        s = _dot_nt(k[2 * cidx + hd], q[u])
        res.append(s)
        if cidx == r:
            s = jnp.minimum(s, cap_ref[...]) if MINMASK else jnp.where(tri, s, neg)
        s = s.reshape(T // 8, 8, T)
        sv[(u, cidx)] = s
        pm = jnp.max(s, axis=0)
        mx[u] = pm if u not in mx else jnp.maximum(mx[u], pm)

    def job_b(u, cidx):
        r, hd = divmod(u, 2)
        if u not in mfin:
            mfin[u] = jnp.broadcast_to(jnp.max(mx[u], axis=0, keepdims=True), (8, T))
        s = sv.pop((u, cidx))
        ps = []
        g = T // 8 // NSUB
        for i in range(NSUB):
            m = mfin[u]
            if LEAD and len(res) >= LEAD:
                r0 = 8 * ((PROW * (cidx % 4) + PSUB * (NSUB - 1 - i)) % 16)
                src = res[len(res) - LEAD][r0:r0 + 8, :]
                m = jnp.where(src > jnp.inf, src, m)
            ps.append(jnp.exp2(s[i * g:(i + 1) * g] - m[None]))
        p = ps[0] if NSUB == 1 else jnp.concatenate(ps, axis=0)
        ls = jnp.sum(p, axis=0)
        lsum[u] = ls if u not in lsum else lsum[u] + ls
        v = accum(('o', u), _dot(vT[2 * cidx + hd], p.reshape(T, T).astype(BF16)))
        if cidx == r:
            l = jnp.sum(lsum[u], axis=0, keepdims=True)
            o[u] = (v * (1.0 / l)).astype(BF16).T

    def job_o(u, j):
        r, hd = divmod(u, 2)
        v = _dot(o[u], wo_ref[tile(hd), tile(j)])
        if OPAIR:
            v = accum(('out', r, j), v)
            if hd == 1:
                acc_scr[tile(r), tile(j)] += v
        else:
            res.append(v)
            acc_scr[tile(r), tile(j)] += v

    fns = dict(q=job_q, k=job_k, v=job_v, a=job_a, b=job_b, o=job_o)
    for n, (kind, u, j) in enumerate(_job_order(nb, km, kc)):
        if n == MID:
            mid()
        fns[kind](u, j)


def _job_order(nb, km, kc):
    nu = 2 * nb
    nominal = []
    tail = []
    for slot in range(-2, nu + 1):
        A = [('a', slot + 1, c) for c in range((slot + 1) // 2 + 1)] if 0 <= slot + 1 < nu else []
        B = [('b', slot, c) for c in range(slot // 2 + 1)] if 0 <= slot < nu else []
        Fj = []
        if slot + 2 < nu:
            Fj += [('q', slot + 2, j) for j in range(km)]
            Fj += [('k', slot + 2, j) for j in range(kc)]
            Fj += [('v', slot + 2, j) for j in range(kc)]
        if slot - 1 >= 0:
            oj = [('o', slot - 1, j) for j in range(km)]
            if OPAIR:
                oj = [('o', slot - 2 + hd, j) for j in range(km) for hd in range(2)] if slot % 2 == 0 else []
            if slot - 1 >= nu - 1 - RES:
                tail += oj
            else:
                Fj += oj
        while A or B:
            nominal += A[:GRP]; A = A[GRP:]
            nominal += B[:GRP]; B = B[GRP:]
        nominal += Fj
    nominal += tail
    last = dict(q=km - 1, k=kc - 1, v=kc - 1)
    done = {}

    def ready_at(job):
        kind, u, j = job
        hd = u % 2
        if kind == 'a':
            deps = [(('q', u), LAT_Q), (('k', 2 * j + hd), LAT_K)]
        elif kind == 'b':
            deps = [(('a', u), LAT_A), (('v', 2 * j + hd), LAT_K)]
        elif kind == 'o':
            deps = [(('b', u), LAT_B)]
        else:
            deps = []
        t = 0
        for key, lat in deps:
            if key not in done:
                return None
            t = max(t, done[key] + lat)
        return t

    order = []
    while nominal:
        n = len(order)
        seen = set()
        pick = None
        best = None
        for i, job in enumerate(nominal):
            cls = 'p' if job[0] in 'qkv' else job[0]
            if cls in seen:
                continue
            seen.add(cls)
            t = ready_at(job)
            if t is not None and t <= n:
                pick = i
                break
            if t is not None and (best is None or t < best[0]):
                best = (t, i)
            if len(seen) == 4:
                break
        if pick is None:
            pick = best[1]
        job = nominal.pop(pick)
        order.append(job)
        kind, u, j = job
        if j == last.get(kind, u // 2):
            done[(kind, u)] = n
    return order


def _kernel(x_hbm, c_hbm, wq_hbm, wuk_hbm, wuv_hbm, wo_hbm, w1_hbm, w2_hbm, w3_hbm, w4_hbm,
            cond_hbm, wmod_hbm, out_hbm,
            h_scr, acc_scr, mod_scr, x1_scr, hb_scr, t_scr, wq_buf, wk_buf, wv_buf, wo_buf, wsem,
            c_scr, cap_scr,
            x_ref, c_ref, cond_ref, wma_ref, wmb_ref, w1_ref, w2_ref, w3_ref, w4_ref, sem,
            out_buf, osem,
            *, S, M, Dc, H, D, RB):
    nattn = H // 2
    scale = float(D) ** -0.5 * math.log2(math.e)
    neg = -1e9 * math.log2(math.e)
    nrb = S // RB
    NX = 4
    XR = S // NX

    def wcopies(g, slot):
        cps = [pltpu.make_async_copy(src.bitcast(U32).at[:, g, :], dst.at[slot], wsem.at[slot, j])
               for j, (src, dst) in enumerate(((wq_hbm, wq_buf), (wuk_hbm, wk_buf), (wuv_hbm, wv_buf)))]
        cps.append(pltpu.make_async_copy(wo_hbm.at[g], wo_buf.at[slot], wsem.at[slot, 3]))
        return cps

    cp_cond = pltpu.make_async_copy(cond_hbm, cond_ref, sem.at[0])
    cp_wma = pltpu.make_async_copy(wmod_hbm.at[:, 0:2 * M], wma_ref, sem.at[1])
    cp_c = pltpu.make_async_copy(c_hbm, c_ref, sem.at[2])
    cp_late = [pltpu.make_async_copy(src, dst, sem.at[3 + j]) for j, (src, dst) in enumerate((
        (wmod_hbm.at[:, 2 * M:6 * M], wmb_ref), (w1_hbm, w1_ref), (w2_hbm, w2_ref),
        (w3_hbm, w3_ref), (w4_hbm, w4_ref)))]
    cp_x = [pltpu.make_async_copy(x_hbm.at[i * XR:(i + 1) * XR, :], x_ref.at[i * XR:(i + 1) * XR, :],
                                  sem.at[8 + i]) for i in range(NX)]

    def silu_cond():
        cf = cond_ref[...].astype(F32)
        return jnp.broadcast_to((cf * jax.nn.sigmoid(cf)).astype(BF16), (8, M))

    queue = [cp_cond, cp_wma] + cp_x + [cp_c] + wcopies(0, 0)
    plan = [int(t) for t in os.environ.get('PLAN', '3,2,2,4,0,0').split(',')]

    def kick():
        for _ in range(plan.pop(0)):
            queue.pop(0).start()

    kick()

    def zero(r, carry):
        acc_scr[pl.ds(pl.multiple_of(r * T, T), T), :] = jnp.zeros((T, M), F32)
        return carry

    jax.lax.fori_loop(0, S // T, zero, 0)
    cap_scr[...] = jnp.where(jax.lax.broadcasted_iota(jnp.int32, (T, T), 0)
                             <= jax.lax.broadcasted_iota(jnp.int32, (T, T), 1), jnp.inf, neg)
    t_scr[0:8, :] = jnp.zeros((8, M), F32)
    t_scr[S + 8:S + 16, :] = jnp.zeros((8, M), F32)
    cp_cond.wait()
    cp_wma.wait()
    kick()
    mod_scr[:, 0:2 * M] = _dot(silu_cond(), wma_ref[...])

    def ln_body(r, carry):
        sa = mod_scr[0:1, 0:M]
        ca = mod_scr[0:1, M:2 * M]
        rows = pl.ds(pl.multiple_of(r * LNR, LNR), LNR)
        hh = (_ln(x_ref[rows, :].astype(F32)) * (1.0 + ca) + sa).astype(BF16)
        for i in range(LNR // T):
            for j in range(M // T):
                h_scr[r * (LNR // T) + i, j] = _pk(hh[i * T:(i + 1) * T, j * T:(j + 1) * T])
        return carry

    for i in range(NX):
        cp_x[i].wait()
        kick()
        jax.lax.fori_loop(i * (XR // LNR), (i + 1) * (XR // LNR), ln_body, 0)

    assert not queue
    cp_c.wait()

    def cbody(r, carry):
        rows = pl.ds(pl.multiple_of(r * T, T), T)
        for j in range(Dc // T):
            c_scr[r, j] = _pk(c_ref[rows, j * T:(j + 1) * T])
        return carry

    jax.lax.fori_loop(0, S // T, cbody, 0)
    for cp in wcopies(0, 0):
        cp.wait()
    for cp in cp_late:
        cp.start()

    def attn_body(g, carry):
        slot = g & 1
        nxt = jnp.minimum(g + 1, nattn - 1)

        def mid():
            for cp in wcopies(nxt, 1 - slot):
                cp.start()

        _attention_step(h_scr, c_scr, wq_buf.at[slot], wk_buf.at[slot], wv_buf.at[slot],
                        wo_buf.at[slot], acc_scr, cap_scr, mid,
                        S=S, M=M, Dc=Dc, H=H, scale=scale, neg=neg)
        for cp in wcopies(nxt, 1 - slot):
            cp.wait()
        return carry

    jax.lax.fori_loop(0, nattn, attn_body, 0)

    for cp in cp_late:
        cp.wait()
    mod_scr[:, 2 * M:6 * M] = _dot(silu_cond(), wmb_ref[...])

    def b1_pre(r0, n):
        ga = mod_scr[0:1, 2 * M:3 * M]
        sb = mod_scr[0:1, 3 * M:4 * M]
        cb = mod_scr[0:1, 4 * M:5 * M]
        rows = pl.ds(r0, n)
        x1 = x_ref[rows, :].astype(F32) + ga * acc_scr[rows, :]
        x1_scr[rows, :] = x1
        hb = _ln(x1) * (1.0 + cb) + sb
        hb_scr[rows, :] = hb
        return _ln(hb).astype(BF16)

    HALO = 16
    t_scr[8:8 + RB + HALO, :] = _gelu(_dot(b1_pre(0, RB + HALO), w1_ref[...]))

    def out_copy(r):
        rows = pl.ds(pl.multiple_of(r * RB, RB), RB)
        return pltpu.make_async_copy(out_buf.at[rows, :], out_hbm.at[rows, :], osem.at[r])

    def b_body(r, carry):
        gb = mod_scr[0:1, 5 * M:6 * M]
        r0 = pl.multiple_of(r * RB, RB)
        n0 = pl.multiple_of(jnp.minimum(r0 + RB + HALO, S - RB), HALO)
        cq = M // 4
        col = jax.lax.broadcasted_iota(jnp.int32, (RB, M), 1)
        blk = t_scr[pl.ds(r0, RB + 16), :]
        tm1 = blk[7:7 + RB]
        tp1 = blk[9:9 + RB]
        tm2 = blk[6:6 + RB]
        tp2 = blk[10:10 + RB]
        sh = jnp.where(col < 2 * cq, jnp.where(col < cq, tm1, tp1), jnp.where(col < 3 * cq, tm2, tp2))
        x1 = x1_scr[pl.ds(r0, RB), :]
        y1 = hb_scr[pl.ds(r0, RB), :] + _dot(sh.astype(BF16), w2_ref[...])
        t_next = _dot(b1_pre(n0, RB), w1_ref[...])
        h3 = _gelu(_dot_nt(_ln(y1).astype(BF16), w3_ref[...]))
        t_scr[pl.ds(pl.multiple_of(n0 + 8, 8), RB), :] = _gelu(t_next)
        y2 = y1 + _dot(h3.astype(BF16), w4_ref[...])
        out_buf[pl.ds(r0, RB), :] = (x1 + gb * y2).astype(out_buf.dtype)
        out_copy(r).start()
        return carry

    jax.lax.fori_loop(0, nrb, b_body, 0)
    for r in range(nrb):
        out_copy(r).wait()


@jax.jit
def pallas_adaLN_cond__compressed_kv_cla__mixer_s_mlp__prompt_kernel(
    A_x: jax.Array,
    A_c_kv: jax.Array,
    A_w_q: jax.Array,
    A_w_uk: jax.Array,
    A_w_uv: jax.Array,
    A_w_o: jax.Array,
    B_x: jax.Array,
    B_w1: jax.Array,
    B_w2: jax.Array,
    B_w3: jax.Array,
    B_w4: jax.Array,
    c: jax.Array,
    w_mod: jax.Array,
):
    _, S, M = A_x.shape
    Dc = A_c_kv.shape[2]
    H, D = A_w_q.shape[1], A_w_q.shape[2]
    Fd = B_w3.shape[1]
    RB = int(os.environ.get('RB', 256))
    nrb = S // RB
    out = pl.pallas_call(
        functools.partial(_kernel, S=S, M=M, Dc=Dc, H=H, D=D, RB=RB),
        in_specs=[pl.BlockSpec(memory_space=pltpu.HBM)] * 12,
        out_specs=pl.BlockSpec(memory_space=pltpu.HBM),
        out_shape=jax.ShapeDtypeStruct((S, M), A_x.dtype),
        scratch_shapes=[
            pltpu.VMEM((S // T, M // T, T // 2, T), U32),
            pltpu.VMEM((S, M), F32),
            pltpu.VMEM((8, 6 * M), F32),
            pltpu.VMEM((S, M), F32),
            pltpu.VMEM((S, M), F32),
            pltpu.VMEM((S + 16, M), F32),
            pltpu.VMEM((2, M, D), U32),
            pltpu.VMEM((2, Dc, D), U32),
            pltpu.VMEM((2, Dc, D), U32),
            pltpu.VMEM((2, 2 * D, M), BF16),
            pltpu.SemaphoreType.DMA((2, 4)),
            pltpu.VMEM((S // T, Dc // T, T // 2, T), U32),
            pltpu.VMEM((T, T), F32),
            pltpu.VMEM((S, M), BF16),
            pltpu.VMEM((S, Dc), BF16),
            pltpu.VMEM((1, M), BF16),
            pltpu.VMEM((M, 2 * M), BF16),
            pltpu.VMEM((M, 4 * M), BF16),
            pltpu.VMEM((M, M), BF16),
            pltpu.VMEM((M, M), BF16),
            pltpu.VMEM((Fd, M), BF16),
            pltpu.VMEM((Fd, M), BF16),
            pltpu.SemaphoreType.DMA((12,)),
            pltpu.VMEM((S, M), A_x.dtype),
            pltpu.SemaphoreType.DMA((nrb,)),
        ],
        compiler_params=pltpu.CompilerParams(
            vmem_limit_bytes=100 * 1024 * 1024,
            disable_bounds_checks=bool(int(os.environ.get('NOBC', 1))),
        ),
    )(
        A_x.reshape(S, M), A_c_kv.reshape(S, Dc),
        A_w_q, A_w_uk, A_w_uv,
        A_w_o.reshape(H // 2, 2 * D, M),
        B_w1, B_w2, B_w3.T, B_w4, c, w_mod,
    )
    return out.reshape(1, S, M)
```

```python
import functools
import math
import os

import jax
import jax.numpy as jnp
import jax.experimental.pallas as pl
import jax.experimental.pallas.tpu as pltpu

F32 = jnp.float32
BF16 = jnp.bfloat16
U32 = jnp.uint32
NT = (((1,), (1,)), ((), ()))
T = 128
EPS = 1e-5

GRP = int(os.environ.get('GRP', 4))
LEAD = int(os.environ.get('LEAD', 10))
PROW = int(os.environ.get('PROW', 3))
VT = int(os.environ.get('VT', 8))
RES = int(os.environ.get('RES', 5))
LAT_Q = int(os.environ.get('LAT_Q', 12))
LAT_K = int(os.environ.get('LAT_K', 10))
LAT_A = int(os.environ.get('LAT_A', 16))
LAT_B = int(os.environ.get('LAT_B', 14))
LNR = int(os.environ.get('LNR', 128))
MID = int(os.environ.get('MID', 120))
PC = int(os.environ.get('PC', 32))
P0 = int(os.environ.get('P0', 242))
PSTEP = int(os.environ.get('PSTEP', 14))
MINMASK = int(os.environ.get('MINMASK', 1))
OPAIR = int(os.environ.get('OPAIR', 0))
NSUB = int(os.environ.get('NSUB', 1))
PSUB = int(os.environ.get('PSUB', 1))


def _dot(a, b):
    return jnp.dot(a, b, preferred_element_type=F32)


def _dot_nt(a, b):
    return jax.lax.dot_general(a, b, NT, preferred_element_type=F32)


def _ln(x):
    m = jnp.mean(x, axis=-1, keepdims=True)
    xc = x - m
    v = jnp.mean(xc * xc, axis=-1, keepdims=True)
    return xc * jax.lax.rsqrt(v + EPS)


def _gelu(x):
    c0 = math.sqrt(2.0 / math.pi)
    return 0.5 * x * (1.0 + jnp.tanh(c0 * (x + 0.044715 * (x * x * x))))


def _tie(x, dep):
    xu = pltpu.bitcast(x, U32)
    first = jnp.where(dep > jnp.inf, jnp.uint32(0), xu[:8])
    return pltpu.bitcast(jnp.concatenate([first, xu[8:]], axis=0), BF16)


def _unpack_pair(wu):
    lo = pltpu.bitcast(wu << 16, F32)
    hi = pltpu.bitcast(wu & jnp.uint32(0xFFFF0000), F32)
    return lo, hi


def _ld(ref, *idx):
    return pltpu.bitcast(ref[idx], BF16)


def _pk(x):
    return pltpu.bitcast(x, U32)


def _attention_step(h_scr, c_scr, wq_ref, wuk_ref, wuv_ref, wo_ref, acc_scr, cap_ref, mid,
                    *, S, M, Dc, H, scale, neg):
    nb = S // T
    km, kc = M // T, Dc // T
    tile = lambda j: slice(j * T, (j + 1) * T)
    wq = [[w.astype(BF16) for w in _unpack_pair(wq_ref[tile(j), :])] for j in range(km)]
    wk = [[w.astype(BF16) for w in _unpack_pair(wuk_ref[tile(j), :])] for j in range(kc)]
    wvT = [[w.astype(BF16).T for w in _unpack_pair(wuv_ref[tile(j), :])] for j in range(kc)]
    if not MINMASK:
        tri = (jax.lax.broadcasted_iota(jnp.int32, (T, T), 0)
               <= jax.lax.broadcasted_iota(jnp.int32, (T, T), 1))

    q = {}; k = {}; vT = {}; sv = {}; mx = {}; mfin = {}; lsum = {}; o = {}
    part = {}
    res = []

    def accum(key, val):
        res.append(val)
        part[key] = val if key not in part else val + part[key]
        return part[key]

    def job_q(u, j):
        r, hd = divmod(u, 2)
        v = accum(('q', u), _dot(_ld(h_scr, r, j), wq[j][hd]))
        if j == km - 1:
            q[u] = (v * scale).astype(BF16)

    def job_k(u, j):
        r, hd = divmod(u, 2)
        v = accum(('k', u), _dot(_ld(c_scr, r, j), wk[j][hd]))
        if j == kc - 1:
            k[u] = v.astype(BF16)

    def job_v(u, j):
        r, hd = divmod(u, 2)
        a = wvT[j][hd]
        if VT and len(res) >= VT:
            a = _tie(a, res[len(res) - VT][0:8, :])
        v = accum(('v', u), _dot_nt(a, _ld(c_scr, r, j)))
        if j == kc - 1:
            vT[u] = v.astype(BF16)

    def job_a(u, cidx):
        r, hd = divmod(u, 2)
        s = _dot_nt(k[2 * cidx + hd], q[u])
        res.append(s)
        if cidx == r:
            s = jnp.minimum(s, cap_ref[...]) if MINMASK else jnp.where(tri, s, neg)
        s = s.reshape(T // 8, 8, T)
        sv[(u, cidx)] = s
        pm = jnp.max(s, axis=0)
        mx[u] = pm if u not in mx else jnp.maximum(mx[u], pm)

    def job_b(u, cidx):
        r, hd = divmod(u, 2)
        if u not in mfin:
            mfin[u] = jnp.broadcast_to(jnp.max(mx[u], axis=0, keepdims=True), (8, T))
        s = sv.pop((u, cidx))
        ps = []
        g = T // 8 // NSUB
        for i in range(NSUB):
            m = mfin[u]
            if LEAD and len(res) >= LEAD:
                r0 = 8 * ((PROW * (cidx % 4) + PSUB * (NSUB - 1 - i)) % 16)
                src = res[len(res) - LEAD][r0:r0 + 8, :]
                m = jnp.where(src > jnp.inf, src, m)
            ps.append(jnp.exp2(s[i * g:(i + 1) * g] - m[None]))
        p = ps[0] if NSUB == 1 else jnp.concatenate(ps, axis=0)
        ls = jnp.sum(p, axis=0)
        lsum[u] = ls if u not in lsum else lsum[u] + ls
        v = accum(('o', u), _dot(vT[2 * cidx + hd], p.reshape(T, T).astype(BF16)))
        if cidx == r:
            l = jnp.sum(lsum[u], axis=0, keepdims=True)
            o[u] = (v * (1.0 / l)).astype(BF16).T

    def job_o(u, j):
        r, hd = divmod(u, 2)
        v = _dot(o[u], wo_ref[tile(hd), tile(j)])
        if OPAIR:
            v = accum(('out', r, j), v)
            if hd == 1:
                acc_scr[tile(r), tile(j)] += v
        else:
            res.append(v)
            acc_scr[tile(r), tile(j)] += v

    fns = dict(q=job_q, k=job_k, v=job_v, a=job_a, b=job_b, o=job_o)
    for n, (kind, u, j) in enumerate(_job_order(nb, km, kc)):
        if n == MID:
            mid()
        fns[kind](u, j)


def _job_order(nb, km, kc):
    nu = 2 * nb
    nominal = []
    tail = []
    for slot in range(-2, nu + 1):
        A = [('a', slot + 1, c) for c in range((slot + 1) // 2 + 1)] if 0 <= slot + 1 < nu else []
        B = [('b', slot, c) for c in range(slot // 2 + 1)] if 0 <= slot < nu else []
        Fj = []
        if slot + 2 < nu:
            Fj += [('q', slot + 2, j) for j in range(km)]
            Fj += [('k', slot + 2, j) for j in range(kc)]
            Fj += [('v', slot + 2, j) for j in range(kc)]
        if slot - 1 >= 0:
            oj = [('o', slot - 1, j) for j in range(km)]
            if OPAIR:
                oj = [('o', slot - 2 + hd, j) for j in range(km) for hd in range(2)] if slot % 2 == 0 else []
            if slot - 1 >= nu - 1 - RES:
                tail += oj
            else:
                Fj += oj
        while A or B:
            nominal += A[:GRP]; A = A[GRP:]
            nominal += B[:GRP]; B = B[GRP:]
        nominal += Fj
    nominal += tail
    last = dict(q=km - 1, k=kc - 1, v=kc - 1)
    done = {}

    def ready_at(job):
        kind, u, j = job
        hd = u % 2
        if kind == 'a':
            deps = [(('q', u), LAT_Q), (('k', 2 * j + hd), LAT_K)]
        elif kind == 'b':
            deps = [(('a', u), LAT_A), (('v', 2 * j + hd), LAT_K)]
        elif kind == 'o':
            deps = [(('b', u), LAT_B)]
        else:
            deps = []
        t = 0
        for key, lat in deps:
            if key not in done:
                return None
            t = max(t, done[key] + lat)
        return t

    order = []
    while nominal:
        n = len(order)
        seen = set()
        pick = None
        best = None
        for i, job in enumerate(nominal):
            cls = 'p' if job[0] in 'qkv' else job[0]
            if cls in seen:
                continue
            seen.add(cls)
            t = ready_at(job)
            if t is not None and t <= n:
                pick = i
                break
            if t is not None and (best is None or t < best[0]):
                best = (t, i)
            if len(seen) == 4:
                break
        if pick is None:
            pick = best[1]
        job = nominal.pop(pick)
        order.append(job)
        kind, u, j = job
        if j == last.get(kind, u // 2):
            done[(kind, u)] = n
    return order


def _kernel(x_hbm, c_hbm, wq_hbm, wuk_hbm, wuv_hbm, wo_hbm, w1_hbm, w2_hbm, w3_hbm, w4_hbm,
            cond_hbm, wmod_hbm, out_hbm,
            h_scr, acc_scr, mod_scr, x1_scr, hb_scr, t_scr, wq_buf, wk_buf, wv_buf, wo_buf, wsem,
            c_scr, cap_scr,
            x_ref, c_ref, cond_ref, wma_ref, wmb_ref, w1_ref, w2_ref, w3_ref, w4_ref, sem,
            out_buf, osem, a1_scr,
            *, S, M, Dc, H, D, RB):
    nattn = H // 2
    scale = float(D) ** -0.5 * math.log2(math.e)
    neg = -1e9 * math.log2(math.e)
    nrb = S // RB
    NX = 4
    XR = S // NX

    def wcopies(g, slot):
        cps = [pltpu.make_async_copy(src.bitcast(U32).at[:, g, :], dst.at[slot], wsem.at[slot, j])
               for j, (src, dst) in enumerate(((wq_hbm, wq_buf), (wuk_hbm, wk_buf), (wuv_hbm, wv_buf)))]
        cps.append(pltpu.make_async_copy(wo_hbm.at[g], wo_buf.at[slot], wsem.at[slot, 3]))
        return cps

    cp_cond = pltpu.make_async_copy(cond_hbm, cond_ref, sem.at[0])
    cp_wma = pltpu.make_async_copy(wmod_hbm.at[:, 0:2 * M], wma_ref, sem.at[1])
    cp_c = pltpu.make_async_copy(c_hbm, c_ref, sem.at[2])
    cp_late = [pltpu.make_async_copy(src, dst, sem.at[3 + j]) for j, (src, dst) in enumerate((
        (wmod_hbm.at[:, 2 * M:6 * M], wmb_ref), (w1_hbm, w1_ref), (w2_hbm, w2_ref),
        (w3_hbm, w3_ref), (w4_hbm, w4_ref)))]
    cp_x = [pltpu.make_async_copy(x_hbm.at[i * XR:(i + 1) * XR, :], x_ref.at[i * XR:(i + 1) * XR, :],
                                  sem.at[8 + i]) for i in range(NX)]

    def silu_cond():
        cf = cond_ref[...].astype(F32)
        return jnp.broadcast_to((cf * jax.nn.sigmoid(cf)).astype(BF16), (8, M))

    queue = [cp_cond, cp_wma] + cp_x + [cp_c] + wcopies(0, 0)
    plan = [int(t) for t in os.environ.get('PLAN', '3,2,2,4,0,0').split(',')]

    def kick():
        for _ in range(plan.pop(0)):
            queue.pop(0).start()

    kick()

    def zero(r, carry):
        acc_scr[pl.ds(pl.multiple_of(r * T, T), T), :] = jnp.zeros((T, M), F32)
        return carry

    jax.lax.fori_loop(0, S // T, zero, 0)
    cap_scr[...] = jnp.where(jax.lax.broadcasted_iota(jnp.int32, (T, T), 0)
                             <= jax.lax.broadcasted_iota(jnp.int32, (T, T), 1), jnp.inf, neg)
    acc_scr[S:S + 16, :] = jnp.zeros((16, M), F32)
    x_ref[S:S + 16, :] = jnp.zeros((16, M), BF16)
    cp_cond.wait()
    cp_wma.wait()
    kick()
    mod_scr[:, 0:2 * M] = _dot(silu_cond(), wma_ref[...])

    def ln_body(r, carry):
        sa = mod_scr[0:1, 0:M]
        ca = mod_scr[0:1, M:2 * M]
        rows = pl.ds(pl.multiple_of(r * LNR, LNR), LNR)
        hh = (_ln(x_ref[rows, :].astype(F32)) * (1.0 + ca) + sa).astype(BF16)
        for i in range(LNR // T):
            for j in range(M // T):
                h_scr[r * (LNR // T) + i, j] = _pk(hh[i * T:(i + 1) * T, j * T:(j + 1) * T])
        return carry

    for i in range(NX):
        cp_x[i].wait()
        kick()
        jax.lax.fori_loop(i * (XR // LNR), (i + 1) * (XR // LNR), ln_body, 0)

    assert not queue
    cp_c.wait()

    def cbody(r, carry):
        rows = pl.ds(pl.multiple_of(r * T, T), T)
        for j in range(Dc // T):
            c_scr[r, j] = _pk(c_ref[rows, j * T:(j + 1) * T])
        return carry

    jax.lax.fori_loop(0, S // T, cbody, 0)
    for cp in wcopies(0, 0):
        cp.wait()
    for cp in cp_late:
        cp.start()

    def attn_body(g, carry):
        slot = g & 1
        nxt = jnp.minimum(g + 1, nattn - 1)

        def mid():
            for cp in wcopies(nxt, 1 - slot):
                cp.start()

        _attention_step(h_scr, c_scr, wq_buf.at[slot], wk_buf.at[slot], wv_buf.at[slot],
                        wo_buf.at[slot], acc_scr, cap_scr, mid,
                        S=S, M=M, Dc=Dc, H=H, scale=scale, neg=neg)
        for cp in wcopies(nxt, 1 - slot):
            cp.wait()
        return carry

    jax.lax.fori_loop(0, nattn, attn_body, 0)

    for cp in cp_late:
        cp.wait()
    mod_scr[:, 2 * M:6 * M] = _dot(silu_cond(), wmb_ref[...])
    km = M // T
    Fd = w4_ref.shape[0]
    ftiles = [(f, min(f + T, Fd)) for f in range(0, Fd, T)]
    tile = lambda j: slice(j * T, (j + 1) * T)
    OFF = 16
    CAR = 32

    def p1(r0, n, dep=None):
        ga = mod_scr[0:1, 2 * M:3 * M]
        sb = mod_scr[0:1, 3 * M:4 * M]
        cb = mod_scr[0:1, 4 * M:5 * M]
        if dep is not None:
            g0 = jnp.where(dep[0:1, :] > jnp.inf, dep[0:1, :], ga[:, 0:T])
            ga = jnp.concatenate([g0, ga[:, T:]], axis=1)
        rows = pl.ds(r0, n)
        x1 = x_ref[rows, :].astype(F32) + ga * acc_scr[rows, :]
        x1_scr[rows, :] = x1
        hb = _ln(x1) * (1.0 + cb) + sb
        hb_scr[rows, :] = hb
        return _ln(hb).astype(BF16)

    def p1_store(r0, c, dep=None):
        a1 = p1(r0 + c * PC, PC, dep)
        for j in range(km):
            a1_scr[j, c * PC // 2:(c + 1) * PC // 2, :] = _pk(a1[:, tile(j)])

    t_scr[RB:RB + CAR - OFF, :] = jnp.zeros((CAR - OFF, M), F32)
    t_scr[RB + CAR - OFF:RB + CAR, :] = _gelu(_dot(p1(0, OFF), w1_ref[...]))
    for c in range(RB // PC):
        p1_store(OFF, c)

    def out_copy(r):
        rows = pl.ds(pl.multiple_of(r * RB, RB), RB)
        return pltpu.make_async_copy(out_buf.at[rows, :], out_hbm.at[rows, :], osem.at[r])

    def b_body(r, carry):
        gb = mod_scr[0:1, 5 * M:6 * M]
        r0 = pl.multiple_of(r * RB, RB)
        n0 = pl.multiple_of(jnp.minimum(r0 + RB, S - RB) + OFF, OFF)
        nh = RB // T
        res = []

        def mm(lhs, wt, dot):
            acc = None
            for x, w in zip(lhs, wt):
                v = dot(x, w)
                res.append(v)
                acc = v if acc is None else v + acc
                if len(res) in pace:
                    p1_store(n0, pace[len(res)], v[0:8, :T])
            return acc

        npc = RB // PC
        pace = {P0 + i * PSTEP: i for i in range(npc)}
        t_scr[0:CAR, :] = t_scr[RB:RB + CAR, :]
        for hf in range(nh):
            lhs = [pltpu.bitcast(a1_scr[j, hf * T // 2:(hf + 1) * T // 2, :], BF16) for j in range(km)]
            for n in range(km):
                t = _gelu(mm(lhs, [w1_ref[tile(j), tile(n)] for j in range(km)], _dot))
                if hf == nh - 1:
                    t = jnp.concatenate([t[:T - OFF], jnp.where(r < nrb - 1, t[T - OFF:], 0.0)], axis=0)
                t_scr[CAR + hf * T:CAR + (hf + 1) * T, tile(n)] = t
        cq = M // 4
        shifts = (-1, 1, -2, 2)
        lane = jax.lax.broadcasted_iota(jnp.int32, (T, T), 1)
        a3 = []
        z = []
        for hf in range(nh):
            base = CAR - OFF + hf * T
            lhs = []
            for j in range(km):
                g_lo, g_hi = (j * T) // cq, ((j + 1) * T - 1) // cq
                v = t_scr[base + shifts[g_lo]:base + shifts[g_lo] + T, tile(j)]
                if g_hi != g_lo:
                    v2 = t_scr[base + shifts[g_hi]:base + shifts[g_hi] + T, tile(j)]
                    v = jnp.where(lane < g_hi * cq - j * T, v, v2)
                lhs.append(v.astype(BF16))
            rows = pl.ds(pl.multiple_of(r0 + hf * T, T), T)
            y1 = jnp.concatenate(
                [mm(lhs, [w2_ref[tile(j), tile(n)] for j in range(km)], _dot) for n in range(km)], axis=1)
            y1 = y1 + hb_scr[rows, :]
            z.append(x1_scr[rows, :] + gb * y1)
            a3.append(_ln(y1).astype(BF16))
        h3 = []
        for hf in range(nh):
            lhs = [a3[hf][:, tile(j)] for j in range(km)]
            h3.append([_gelu(mm(lhs, [w3_ref[f0:f1, tile(j)] for j in range(km)], _dot_nt)).astype(BF16)
                       for f0, f1 in ftiles])
        for hf in range(nh):
            rows = pl.ds(pl.multiple_of(r0 + hf * T, T), T)
            for n in range(km):
                v = mm(h3[hf], [w4_ref[f0:f1, tile(n)] for f0, f1 in ftiles], _dot)
                out_buf[rows, tile(n)] = (z[hf][:, tile(n)] + gb[:, tile(n)] * v).astype(out_buf.dtype)
        out_copy(r).start()
        return carry

    jax.lax.fori_loop(0, nrb, b_body, 0)
    for r in range(nrb):
        out_copy(r).wait()


@jax.jit
def pallas_adaLN_cond__compressed_kv_cla__mixer_s_mlp__prompt_kernel(
    A_x: jax.Array,
    A_c_kv: jax.Array,
    A_w_q: jax.Array,
    A_w_uk: jax.Array,
    A_w_uv: jax.Array,
    A_w_o: jax.Array,
    B_x: jax.Array,
    B_w1: jax.Array,
    B_w2: jax.Array,
    B_w3: jax.Array,
    B_w4: jax.Array,
    c: jax.Array,
    w_mod: jax.Array,
):
    _, S, M = A_x.shape
    Dc = A_c_kv.shape[2]
    H, D = A_w_q.shape[1], A_w_q.shape[2]
    Fd = B_w3.shape[1]
    RB = int(os.environ.get('RB', 256))
    nrb = S // RB
    out = pl.pallas_call(
        functools.partial(_kernel, S=S, M=M, Dc=Dc, H=H, D=D, RB=RB),
        in_specs=[pl.BlockSpec(memory_space=pltpu.HBM)] * 12,
        out_specs=pl.BlockSpec(memory_space=pltpu.HBM),
        out_shape=jax.ShapeDtypeStruct((S, M), A_x.dtype),
        scratch_shapes=[
            pltpu.VMEM((S // T, M // T, T // 2, T), U32),
            pltpu.VMEM((S + 16, M), F32),
            pltpu.VMEM((8, 6 * M), F32),
            pltpu.VMEM((S + 16, M), F32),
            pltpu.VMEM((S + 16, M), F32),
            pltpu.VMEM((RB + 32, M), F32),
            pltpu.VMEM((2, M, D), U32),
            pltpu.VMEM((2, Dc, D), U32),
            pltpu.VMEM((2, Dc, D), U32),
            pltpu.VMEM((2, 2 * D, M), BF16),
            pltpu.SemaphoreType.DMA((2, 4)),
            pltpu.VMEM((S // T, Dc // T, T // 2, T), U32),
            pltpu.VMEM((T, T), F32),
            pltpu.VMEM((S + 16, M), BF16),
            pltpu.VMEM((S, Dc), BF16),
            pltpu.VMEM((1, M), BF16),
            pltpu.VMEM((M, 2 * M), BF16),
            pltpu.VMEM((M, 4 * M), BF16),
            pltpu.VMEM((M, M), BF16),
            pltpu.VMEM((M, M), BF16),
            pltpu.VMEM((Fd, M), BF16),
            pltpu.VMEM((Fd, M), BF16),
            pltpu.SemaphoreType.DMA((12,)),
            pltpu.VMEM((S, M), A_x.dtype),
            pltpu.SemaphoreType.DMA((nrb,)),
            pltpu.VMEM((M // T, RB // 2, T), U32),
        ],
        compiler_params=pltpu.CompilerParams(
            vmem_limit_bytes=100 * 1024 * 1024,
            disable_bounds_checks=bool(int(os.environ.get('NOBC', 1))),
        ),
    )(
        A_x.reshape(S, M), A_c_kv.reshape(S, Dc),
        A_w_q, A_w_uk, A_w_uv,
        A_w_o.reshape(H // 2, 2 * D, M),
        B_w1, B_w2, B_w3.T, B_w4, c, w_mod,
    )
    return out.reshape(1, S, M)
```

```python
import functools
import math
import os

import jax
import jax.numpy as jnp
import jax.experimental.pallas as pl
import jax.experimental.pallas.tpu as pltpu

F32 = jnp.float32
BF16 = jnp.bfloat16
U32 = jnp.uint32
NT = (((1,), (1,)), ((), ()))
T = 128
EPS = 1e-5

GRP = int(os.environ.get('GRP', 4))
LEAD = int(os.environ.get('LEAD', 10))
PROW = int(os.environ.get('PROW', 3))
VT = int(os.environ.get('VT', 8))
RES = int(os.environ.get('RES', 5))
LAT_Q = int(os.environ.get('LAT_Q', 12))
LAT_K = int(os.environ.get('LAT_K', 10))
LAT_A = int(os.environ.get('LAT_A', 16))
LAT_B = int(os.environ.get('LAT_B', 14))
LNR = int(os.environ.get('LNR', 128))
MID = int(os.environ.get('MID', 120))
PC = int(os.environ.get('PC', 32))
P0 = int(os.environ.get('P0', 176))
PSTEP = int(os.environ.get('PSTEP', 23))
PD = int(os.environ.get('PD', 24))
MINMASK = int(os.environ.get('MINMASK', 1))
OPAIR = int(os.environ.get('OPAIR', 0))
NSUB = int(os.environ.get('NSUB', 1))
PSUB = int(os.environ.get('PSUB', 1))


def _dot(a, b):
    return jnp.dot(a, b, preferred_element_type=F32)


def _dot_nt(a, b):
    return jax.lax.dot_general(a, b, NT, preferred_element_type=F32)


def _ln(x):
    m = jnp.mean(x, axis=-1, keepdims=True)
    xc = x - m
    v = jnp.mean(xc * xc, axis=-1, keepdims=True)
    return xc * jax.lax.rsqrt(v + EPS)


def _gelu(x):
    c0 = math.sqrt(2.0 / math.pi)
    return 0.5 * x * (1.0 + jnp.tanh(c0 * (x + 0.044715 * (x * x * x))))


def _tie(x, dep):
    xu = pltpu.bitcast(x, U32)
    first = jnp.where(dep > jnp.inf, jnp.uint32(0), xu[:8])
    return pltpu.bitcast(jnp.concatenate([first, xu[8:]], axis=0), BF16)


def _unpack_pair(wu):
    lo = pltpu.bitcast(wu << 16, F32)
    hi = pltpu.bitcast(wu & jnp.uint32(0xFFFF0000), F32)
    return lo, hi


def _ld(ref, *idx):
    return pltpu.bitcast(ref[idx], BF16)


def _pk(x):
    return pltpu.bitcast(x, U32)


def _attention_step(h_scr, c_scr, wq_ref, wuk_ref, wuv_ref, wo_ref, acc_scr, cap_ref, mid,
                    *, S, M, Dc, H, scale, neg):
    nb = S // T
    km, kc = M // T, Dc // T
    tile = lambda j: slice(j * T, (j + 1) * T)
    wq = [[w.astype(BF16) for w in _unpack_pair(wq_ref[tile(j), :])] for j in range(km)]
    wk = [[w.astype(BF16) for w in _unpack_pair(wuk_ref[tile(j), :])] for j in range(kc)]
    wvT = [[w.astype(BF16).T for w in _unpack_pair(wuv_ref[tile(j), :])] for j in range(kc)]
    if not MINMASK:
        tri = (jax.lax.broadcasted_iota(jnp.int32, (T, T), 0)
               <= jax.lax.broadcasted_iota(jnp.int32, (T, T), 1))

    q = {}; k = {}; vT = {}; sv = {}; mx = {}; mfin = {}; lsum = {}; o = {}
    part = {}
    res = []

    def accum(key, val):
        res.append(val)
        part[key] = val if key not in part else val + part[key]
        return part[key]

    def job_q(u, j):
        r, hd = divmod(u, 2)
        v = accum(('q', u), _dot(_ld(h_scr, r, j), wq[j][hd]))
        if j == km - 1:
            q[u] = (v * scale).astype(BF16)

    def job_k(u, j):
        r, hd = divmod(u, 2)
        v = accum(('k', u), _dot(_ld(c_scr, r, j), wk[j][hd]))
        if j == kc - 1:
            k[u] = v.astype(BF16)

    def job_v(u, j):
        r, hd = divmod(u, 2)
        a = wvT[j][hd]
        if VT and len(res) >= VT:
            a = _tie(a, res[len(res) - VT][0:8, :])
        v = accum(('v', u), _dot_nt(a, _ld(c_scr, r, j)))
        if j == kc - 1:
            vT[u] = v.astype(BF16)

    def job_a(u, cidx):
        r, hd = divmod(u, 2)
        s = _dot_nt(k[2 * cidx + hd], q[u])
        res.append(s)
        if cidx == r:
            s = jnp.minimum(s, cap_ref[...]) if MINMASK else jnp.where(tri, s, neg)
        s = s.reshape(T // 8, 8, T)
        sv[(u, cidx)] = s
        pm = jnp.max(s, axis=0)
        mx[u] = pm if u not in mx else jnp.maximum(mx[u], pm)

    def job_b(u, cidx):
        r, hd = divmod(u, 2)
        if u not in mfin:
            mfin[u] = jnp.broadcast_to(jnp.max(mx[u], axis=0, keepdims=True), (8, T))
        s = sv.pop((u, cidx))
        ps = []
        g = T // 8 // NSUB
        for i in range(NSUB):
            m = mfin[u]
            if LEAD and len(res) >= LEAD:
                r0 = 8 * ((PROW * (cidx % 4) + PSUB * (NSUB - 1 - i)) % 16)
                src = res[len(res) - LEAD][r0:r0 + 8, :]
                m = jnp.where(src > jnp.inf, src, m)
            ps.append(jnp.exp2(s[i * g:(i + 1) * g] - m[None]))
        p = ps[0] if NSUB == 1 else jnp.concatenate(ps, axis=0)
        ls = jnp.sum(p, axis=0)
        lsum[u] = ls if u not in lsum else lsum[u] + ls
        v = accum(('o', u), _dot(vT[2 * cidx + hd], p.reshape(T, T).astype(BF16)))
        if cidx == r:
            l = jnp.sum(lsum[u], axis=0, keepdims=True)
            o[u] = (v * (1.0 / l)).astype(BF16).T

    def job_o(u, j):
        r, hd = divmod(u, 2)
        v = _dot(o[u], wo_ref[tile(hd), tile(j)])
        if OPAIR:
            v = accum(('out', r, j), v)
            if hd == 1:
                acc_scr[tile(r), tile(j)] += v
        else:
            res.append(v)
            acc_scr[tile(r), tile(j)] += v

    fns = dict(q=job_q, k=job_k, v=job_v, a=job_a, b=job_b, o=job_o)
    for n, (kind, u, j) in enumerate(_job_order(nb, km, kc)):
        if n == MID:
            mid()
        fns[kind](u, j)


def _job_order(nb, km, kc):
    nu = 2 * nb
    nominal = []
    tail = []
    for slot in range(-2, nu + 1):
        A = [('a', slot + 1, c) for c in range((slot + 1) // 2 + 1)] if 0 <= slot + 1 < nu else []
        B = [('b', slot, c) for c in range(slot // 2 + 1)] if 0 <= slot < nu else []
        Fj = []
        if slot + 2 < nu:
            Fj += [('q', slot + 2, j) for j in range(km)]
            Fj += [('k', slot + 2, j) for j in range(kc)]
            Fj += [('v', slot + 2, j) for j in range(kc)]
        if slot - 1 >= 0:
            oj = [('o', slot - 1, j) for j in range(km)]
            if OPAIR:
                oj = [('o', slot - 2 + hd, j) for j in range(km) for hd in range(2)] if slot % 2 == 0 else []
            if slot - 1 >= nu - 1 - RES:
                tail += oj
            else:
                Fj += oj
        while A or B:
            nominal += A[:GRP]; A = A[GRP:]
            nominal += B[:GRP]; B = B[GRP:]
        nominal += Fj
    nominal += tail
    last = dict(q=km - 1, k=kc - 1, v=kc - 1)
    done = {}

    def ready_at(job):
        kind, u, j = job
        hd = u % 2
        if kind == 'a':
            deps = [(('q', u), LAT_Q), (('k', 2 * j + hd), LAT_K)]
        elif kind == 'b':
            deps = [(('a', u), LAT_A), (('v', 2 * j + hd), LAT_K)]
        elif kind == 'o':
            deps = [(('b', u), LAT_B)]
        else:
            deps = []
        t = 0
        for key, lat in deps:
            if key not in done:
                return None
            t = max(t, done[key] + lat)
        return t

    order = []
    while nominal:
        n = len(order)
        seen = set()
        pick = None
        best = None
        for i, job in enumerate(nominal):
            cls = 'p' if job[0] in 'qkv' else job[0]
            if cls in seen:
                continue
            seen.add(cls)
            t = ready_at(job)
            if t is not None and t <= n:
                pick = i
                break
            if t is not None and (best is None or t < best[0]):
                best = (t, i)
            if len(seen) == 4:
                break
        if pick is None:
            pick = best[1]
        job = nominal.pop(pick)
        order.append(job)
        kind, u, j = job
        if j == last.get(kind, u // 2):
            done[(kind, u)] = n
    return order


def _kernel(x_hbm, c_hbm, wq_hbm, wuk_hbm, wuv_hbm, wo_hbm, w1_hbm, w2_hbm, w3_hbm, w4_hbm,
            cond_hbm, wmod_hbm, out_hbm,
            h_scr, acc_scr, mod_scr, x1_scr, hb_scr, t_scr, wq_buf, wk_buf, wv_buf, wo_buf, wsem,
            c_scr, cap_scr,
            x_ref, c_ref, cond_ref, wma_ref, wmb_ref, w1_ref, w2_ref, w3_ref, w4_ref, sem,
            out_buf, osem, a1_scr,
            *, S, M, Dc, H, D, RB):
    nattn = H // 2
    scale = float(D) ** -0.5 * math.log2(math.e)
    neg = -1e9 * math.log2(math.e)
    nrb = S // RB
    NX = 4
    XR = S // NX

    def wcopies(g, slot):
        cps = [pltpu.make_async_copy(src.bitcast(U32).at[:, g, :], dst.at[slot], wsem.at[slot, j])
               for j, (src, dst) in enumerate(((wq_hbm, wq_buf), (wuk_hbm, wk_buf), (wuv_hbm, wv_buf)))]
        cps.append(pltpu.make_async_copy(wo_hbm.at[g], wo_buf.at[slot], wsem.at[slot, 3]))
        return cps

    cp_cond = pltpu.make_async_copy(cond_hbm, cond_ref, sem.at[0])
    cp_wma = pltpu.make_async_copy(wmod_hbm.at[:, 0:2 * M], wma_ref, sem.at[1])
    cp_c = pltpu.make_async_copy(c_hbm, c_ref, sem.at[2])
    cp_late = [pltpu.make_async_copy(src, dst, sem.at[3 + j]) for j, (src, dst) in enumerate((
        (wmod_hbm.at[:, 2 * M:6 * M], wmb_ref), (w1_hbm, w1_ref), (w2_hbm, w2_ref),
        (w3_hbm, w3_ref), (w4_hbm, w4_ref)))]
    cp_x = [pltpu.make_async_copy(x_hbm.at[i * XR:(i + 1) * XR, :], x_ref.at[i * XR:(i + 1) * XR, :],
                                  sem.at[8 + i]) for i in range(NX)]

    def silu_cond():
        cf = cond_ref[...].astype(F32)
        return jnp.broadcast_to((cf * jax.nn.sigmoid(cf)).astype(BF16), (8, M))

    queue = [cp_cond, cp_wma] + cp_x + [cp_c] + wcopies(0, 0)
    plan = [int(t) for t in os.environ.get('PLAN', '3,2,2,4,0,0').split(',')]

    def kick():
        for _ in range(plan.pop(0)):
            queue.pop(0).start()

    kick()

    def zero(r, carry):
        acc_scr[pl.ds(pl.multiple_of(r * T, T), T), :] = jnp.zeros((T, M), F32)
        return carry

    jax.lax.fori_loop(0, S // T, zero, 0)
    cap_scr[...] = jnp.where(jax.lax.broadcasted_iota(jnp.int32, (T, T), 0)
                             <= jax.lax.broadcasted_iota(jnp.int32, (T, T), 1), jnp.inf, neg)
    acc_scr[S:S + 16, :] = jnp.zeros((16, M), F32)
    x_ref[S:S + 16, :] = jnp.zeros((16, M), BF16)
    cp_cond.wait()
    cp_wma.wait()
    kick()
    mod_scr[:, 0:2 * M] = _dot(silu_cond(), wma_ref[...])

    def ln_body(r, carry):
        sa = mod_scr[0:1, 0:M]
        ca = mod_scr[0:1, M:2 * M]
        rows = pl.ds(pl.multiple_of(r * LNR, LNR), LNR)
        hh = (_ln(x_ref[rows, :].astype(F32)) * (1.0 + ca) + sa).astype(BF16)
        for i in range(LNR // T):
            for j in range(M // T):
                h_scr[r * (LNR // T) + i, j] = _pk(hh[i * T:(i + 1) * T, j * T:(j + 1) * T])
        return carry

    for i in range(NX):
        cp_x[i].wait()
        kick()
        jax.lax.fori_loop(i * (XR // LNR), (i + 1) * (XR // LNR), ln_body, 0)

    assert not queue
    cp_c.wait()

    def cbody(r, carry):
        rows = pl.ds(pl.multiple_of(r * T, T), T)
        for j in range(Dc // T):
            c_scr[r, j] = _pk(c_ref[rows, j * T:(j + 1) * T])
        return carry

    jax.lax.fori_loop(0, S // T, cbody, 0)
    for cp in wcopies(0, 0):
        cp.wait()
    for cp in cp_late:
        cp.start()

    def attn_body(g, carry):
        slot = g & 1
        nxt = jnp.minimum(g + 1, nattn - 1)

        def mid():
            for cp in wcopies(nxt, 1 - slot):
                cp.start()

        _attention_step(h_scr, c_scr, wq_buf.at[slot], wk_buf.at[slot], wv_buf.at[slot],
                        wo_buf.at[slot], acc_scr, cap_scr, mid,
                        S=S, M=M, Dc=Dc, H=H, scale=scale, neg=neg)
        for cp in wcopies(nxt, 1 - slot):
            cp.wait()
        return carry

    jax.lax.fori_loop(0, nattn, attn_body, 0)

    for cp in cp_late:
        cp.wait()
    mod_scr[:, 2 * M:6 * M] = _dot(silu_cond(), wmb_ref[...])
    km = M // T
    Fd = w4_ref.shape[0]
    ftiles = [(f, min(f + T, Fd)) for f in range(0, Fd, T)]
    tile = lambda j: slice(j * T, (j + 1) * T)
    OFF = 16
    CAR = 32

    def p1(r0, n, dep=None):
        ga = mod_scr[0:1, 2 * M:3 * M]
        sb = mod_scr[0:1, 3 * M:4 * M]
        cb = mod_scr[0:1, 4 * M:5 * M]
        if dep is not None:
            g0 = jnp.where(dep[0:1, :] > jnp.inf, dep[0:1, :], ga[:, 0:T])
            ga = jnp.concatenate([g0, ga[:, T:]], axis=1)
        rows = pl.ds(r0, n)
        x1 = x_ref[rows, :].astype(F32) + ga * acc_scr[rows, :]
        x1_scr[rows, :] = x1
        hb = _ln(x1) * (1.0 + cb) + sb
        hb_scr[rows, :] = hb
        return _ln(hb)

    def p1_store(r0, c, dep=None):
        a1f = p1(r0 + c * PC, PC, dep)
        a1 = a1f.astype(BF16)
        for j in range(km):
            a1_scr[j, c * PC // 2:(c + 1) * PC // 2, :] = _pk(a1[:, tile(j)])
        return jnp.max(a1f[:, M - T:].reshape(PC // 8, 8, T), axis=0)

    t_scr[RB:RB + CAR - OFF, :] = jnp.zeros((CAR - OFF, M), F32)
    t_scr[RB + CAR - OFF:RB + CAR, :] = _gelu(_dot(p1(0, OFF).astype(BF16), w1_ref[...]))
    for c in range(RB // PC):
        p1_store(OFF, c)

    def out_copy(r):
        rows = pl.ds(pl.multiple_of(r * RB, RB), RB)
        return pltpu.make_async_copy(out_buf.at[rows, :], out_hbm.at[rows, :], osem.at[r])

    def b_body(r, carry):
        gb = mod_scr[0:1, 5 * M:6 * M]
        r0 = pl.multiple_of(r * RB, RB)
        n0 = pl.multiple_of(jnp.minimum(r0 + RB, S - RB) + OFF, OFF)
        nh = RB // T
        res = []

        def mm(lhs, wt, dot):
            acc = None
            for x, w in zip(lhs, wt):
                if len(res) in due:
                    w = _tie(w, due.pop(len(res)))
                v = dot(x, w)
                res.append(v)
                acc = v if acc is None else v + acc
                if len(res) in pace:
                    d = p1_store(n0, pace[len(res)], v[0:8, :T])
                    if PD:
                        due[len(res) + PD] = d
            return acc

        npc = RB // PC
        due = {}
        pace = {P0 + i * PSTEP: i for i in range(npc)}
        t_scr[0:CAR, :] = t_scr[RB:RB + CAR, :]
        for hf in range(nh):
            lhs = [pltpu.bitcast(a1_scr[j, hf * T // 2:(hf + 1) * T // 2, :], BF16) for j in range(km)]
            for n in range(km):
                t = _gelu(mm(lhs, [w1_ref[tile(j), tile(n)] for j in range(km)], _dot))
                if hf == nh - 1:
                    t = jnp.concatenate([t[:T - OFF], jnp.where(r < nrb - 1, t[T - OFF:], 0.0)], axis=0)
                t_scr[CAR + hf * T:CAR + (hf + 1) * T, tile(n)] = t
        cq = M // 4
        shifts = (-1, 1, -2, 2)
        lane = jax.lax.broadcasted_iota(jnp.int32, (T, T), 1)
        a3 = []
        z = []
        for hf in range(nh):
            base = CAR - OFF + hf * T
            lhs = []
            for j in range(km):
                g_lo, g_hi = (j * T) // cq, ((j + 1) * T - 1) // cq
                v = t_scr[base + shifts[g_lo]:base + shifts[g_lo] + T, tile(j)]
                if g_hi != g_lo:
                    v2 = t_scr[base + shifts[g_hi]:base + shifts[g_hi] + T, tile(j)]
                    v = jnp.where(lane < g_hi * cq - j * T, v, v2)
                lhs.append(v.astype(BF16))
            rows = pl.ds(pl.multiple_of(r0 + hf * T, T), T)
            y1 = jnp.concatenate(
                [mm(lhs, [w2_ref[tile(j), tile(n)] for j in range(km)], _dot) for n in range(km)], axis=1)
            y1 = y1 + hb_scr[rows, :]
            z.append(y1)
            a3.append(_ln(y1).astype(BF16))
        h3 = []
        for hf in range(nh):
            lhs = [a3[hf][:, tile(j)] for j in range(km)]
            h3.append([_gelu(mm(lhs, [w3_ref[f0:f1, tile(j)] for j in range(km)], _dot_nt)).astype(BF16)
                       for f0, f1 in ftiles])
        for hf in range(nh):
            rows = pl.ds(pl.multiple_of(r0 + hf * T, T), T)
            for n in range(km):
                v = mm(h3[hf], [w4_ref[f0:f1, tile(n)] for f0, f1 in ftiles], _dot)
                out_buf[rows, tile(n)] = (x1_scr[rows, tile(n)] + gb[:, tile(n)] * (v + z[hf][:, tile(n)])
                                          ).astype(out_buf.dtype)
        out_copy(r).start()
        return carry

    jax.lax.fori_loop(0, nrb, b_body, 0)
    for r in range(nrb):
        out_copy(r).wait()


@jax.jit
def pallas_adaLN_cond__compressed_kv_cla__mixer_s_mlp__prompt_kernel(
    A_x: jax.Array,
    A_c_kv: jax.Array,
    A_w_q: jax.Array,
    A_w_uk: jax.Array,
    A_w_uv: jax.Array,
    A_w_o: jax.Array,
    B_x: jax.Array,
    B_w1: jax.Array,
    B_w2: jax.Array,
    B_w3: jax.Array,
    B_w4: jax.Array,
    c: jax.Array,
    w_mod: jax.Array,
):
    _, S, M = A_x.shape
    Dc = A_c_kv.shape[2]
    H, D = A_w_q.shape[1], A_w_q.shape[2]
    Fd = B_w3.shape[1]
    RB = int(os.environ.get('RB', 256))
    nrb = S // RB
    out = pl.pallas_call(
        functools.partial(_kernel, S=S, M=M, Dc=Dc, H=H, D=D, RB=RB),
        in_specs=[pl.BlockSpec(memory_space=pltpu.HBM)] * 12,
        out_specs=pl.BlockSpec(memory_space=pltpu.HBM),
        out_shape=jax.ShapeDtypeStruct((S, M), A_x.dtype),
        scratch_shapes=[
            pltpu.VMEM((S // T, M // T, T // 2, T), U32),
            pltpu.VMEM((S + 16, M), F32),
            pltpu.VMEM((8, 6 * M), F32),
            pltpu.VMEM((S + 16, M), F32),
            pltpu.VMEM((S + 16, M), F32),
            pltpu.VMEM((RB + 32, M), F32),
            pltpu.VMEM((2, M, D), U32),
            pltpu.VMEM((2, Dc, D), U32),
            pltpu.VMEM((2, Dc, D), U32),
            pltpu.VMEM((2, 2 * D, M), BF16),
            pltpu.SemaphoreType.DMA((2, 4)),
            pltpu.VMEM((S // T, Dc // T, T // 2, T), U32),
            pltpu.VMEM((T, T), F32),
            pltpu.VMEM((S + 16, M), BF16),
            pltpu.VMEM((S, Dc), BF16),
            pltpu.VMEM((1, M), BF16),
            pltpu.VMEM((M, 2 * M), BF16),
            pltpu.VMEM((M, 4 * M), BF16),
            pltpu.VMEM((M, M), BF16),
            pltpu.VMEM((M, M), BF16),
            pltpu.VMEM((Fd, M), BF16),
            pltpu.VMEM((Fd, M), BF16),
            pltpu.SemaphoreType.DMA((12,)),
            pltpu.VMEM((S, M), A_x.dtype),
            pltpu.SemaphoreType.DMA((nrb,)),
            pltpu.VMEM((M // T, RB // 2, T), U32),
        ],
        compiler_params=pltpu.CompilerParams(
            vmem_limit_bytes=100 * 1024 * 1024,
            disable_bounds_checks=bool(int(os.environ.get('NOBC', 1))),
        ),
    )(
        A_x.reshape(S, M), A_c_kv.reshape(S, Dc),
        A_w_q, A_w_uk, A_w_uv,
        A_w_o.reshape(H // 2, 2 * D, M),
        B_w1, B_w2, B_w3.T, B_w4, c, w_mod,
    )
    return out.reshape(1, S, M)
```

```python
import functools
import math
import os

import jax
import jax.numpy as jnp
import jax.experimental.pallas as pl
import jax.experimental.pallas.tpu as pltpu

F32 = jnp.float32
BF16 = jnp.bfloat16
U32 = jnp.uint32
NT = (((1,), (1,)), ((), ()))
T = 128
EPS = 1e-5

GRP = int(os.environ.get('GRP', 4))
LEAD = int(os.environ.get('LEAD', 10))
PROW = int(os.environ.get('PROW', 3))
VT = int(os.environ.get('VT', 8))
RES = int(os.environ.get('RES', 5))
LAT_Q = int(os.environ.get('LAT_Q', 12))
LAT_K = int(os.environ.get('LAT_K', 10))
LAT_A = int(os.environ.get('LAT_A', 16))
LAT_B = int(os.environ.get('LAT_B', 14))
LNR = int(os.environ.get('LNR', 128))
MID = int(os.environ.get('MID', 120))
PC = int(os.environ.get('PC', 32))
P0 = int(os.environ.get('P0', 176))
PSTEP = int(os.environ.get('PSTEP', 23))
PD = int(os.environ.get('PD', 24))
OT = int(os.environ.get('OT', 1))
MINMASK = int(os.environ.get('MINMASK', 1))
OPAIR = int(os.environ.get('OPAIR', 0))
NSUB = int(os.environ.get('NSUB', 1))
PSUB = int(os.environ.get('PSUB', 1))


def _dot(a, b):
    return jnp.dot(a, b, preferred_element_type=F32)


def _dot_nt(a, b):
    return jax.lax.dot_general(a, b, NT, preferred_element_type=F32)


def _ln(x):
    m = jnp.mean(x, axis=-1, keepdims=True)
    xc = x - m
    v = jnp.mean(xc * xc, axis=-1, keepdims=True)
    return xc * jax.lax.rsqrt(v + EPS)


def _gelu(x):
    c0 = math.sqrt(2.0 / math.pi)
    return 0.5 * x * (1.0 + jnp.tanh(c0 * (x + 0.044715 * (x * x * x))))


def _tie(x, dep):
    xu = pltpu.bitcast(x, U32)
    first = jnp.where(dep > jnp.inf, jnp.uint32(0), xu[:8])
    return pltpu.bitcast(jnp.concatenate([first, xu[8:]], axis=0), BF16)


def _unpack_pair(wu):
    lo = pltpu.bitcast(wu << 16, F32)
    hi = pltpu.bitcast(wu & jnp.uint32(0xFFFF0000), F32)
    return lo, hi


def _ld(ref, *idx):
    return pltpu.bitcast(ref[idx], BF16)


def _pk(x):
    return pltpu.bitcast(x, U32)


def _attention_step(h_scr, c_scr, wq_ref, wuk_ref, wuv_ref, wo_ref, acc_scr, cap_ref, mid,
                    *, S, M, Dc, H, scale, neg):
    nb = S // T
    km, kc = M // T, Dc // T
    tile = lambda j: slice(j * T, (j + 1) * T)
    wq = [[w.astype(BF16) for w in _unpack_pair(wq_ref[tile(j), :])] for j in range(km)]
    wk = [[w.astype(BF16) for w in _unpack_pair(wuk_ref[tile(j), :])] for j in range(kc)]
    wvT = [[w.astype(BF16).T for w in _unpack_pair(wuv_ref[tile(j), :])] for j in range(kc)]
    if not MINMASK:
        tri = (jax.lax.broadcasted_iota(jnp.int32, (T, T), 0)
               <= jax.lax.broadcasted_iota(jnp.int32, (T, T), 1))

    q = {}; k = {}; vT = {}; sv = {}; mx = {}; mfin = {}; lsum = {}; o = {}
    part = {}
    res = []

    def accum(key, val):
        res.append(val)
        part[key] = val if key not in part else val + part[key]
        return part[key]

    def job_q(u, j):
        r, hd = divmod(u, 2)
        v = accum(('q', u), _dot(_ld(h_scr, r, j), wq[j][hd]))
        if j == km - 1:
            q[u] = (v * scale).astype(BF16)

    def job_k(u, j):
        r, hd = divmod(u, 2)
        v = accum(('k', u), _dot(_ld(c_scr, r, j), wk[j][hd]))
        if j == kc - 1:
            k[u] = v.astype(BF16)

    def job_v(u, j):
        r, hd = divmod(u, 2)
        a = wvT[j][hd]
        if VT and len(res) >= VT:
            a = _tie(a, res[len(res) - VT][0:8, :])
        v = accum(('v', u), _dot_nt(a, _ld(c_scr, r, j)))
        if j == kc - 1:
            vT[u] = v.astype(BF16)

    def job_a(u, cidx):
        r, hd = divmod(u, 2)
        s = _dot_nt(k[2 * cidx + hd], q[u])
        res.append(s)
        if cidx == r:
            s = jnp.minimum(s, cap_ref[...]) if MINMASK else jnp.where(tri, s, neg)
        s = s.reshape(T // 8, 8, T)
        sv[(u, cidx)] = s
        pm = jnp.max(s, axis=0)
        mx[u] = pm if u not in mx else jnp.maximum(mx[u], pm)

    def job_b(u, cidx):
        r, hd = divmod(u, 2)
        if u not in mfin:
            mfin[u] = jnp.broadcast_to(jnp.max(mx[u], axis=0, keepdims=True), (8, T))
        s = sv.pop((u, cidx))
        ps = []
        g = T // 8 // NSUB
        for i in range(NSUB):
            m = mfin[u]
            if LEAD and len(res) >= LEAD:
                r0 = 8 * ((PROW * (cidx % 4) + PSUB * (NSUB - 1 - i)) % 16)
                src = res[len(res) - LEAD][r0:r0 + 8, :]
                m = jnp.where(src > jnp.inf, src, m)
            ps.append(jnp.exp2(s[i * g:(i + 1) * g] - m[None]))
        p = ps[0] if NSUB == 1 else jnp.concatenate(ps, axis=0)
        ls = jnp.sum(p, axis=0)
        lsum[u] = ls if u not in lsum else lsum[u] + ls
        v = accum(('o', u), _dot(vT[2 * cidx + hd], p.reshape(T, T).astype(BF16)))
        if cidx == r:
            l = jnp.sum(lsum[u], axis=0, keepdims=True)
            o[u] = (v * (1.0 / l)).astype(BF16).T
            if OT:
                o[u] = _tie(o[u], lsum[u])

    def job_o(u, j):
        r, hd = divmod(u, 2)
        v = _dot(o[u], wo_ref[tile(hd), tile(j)])
        if OPAIR:
            v = accum(('out', r, j), v)
            if hd == 1:
                acc_scr[tile(r), tile(j)] += v
        else:
            res.append(v)
            acc_scr[tile(r), tile(j)] += v

    fns = dict(q=job_q, k=job_k, v=job_v, a=job_a, b=job_b, o=job_o)
    for n, (kind, u, j) in enumerate(_job_order(nb, km, kc)):
        if n == MID:
            mid()
        fns[kind](u, j)


def _job_order(nb, km, kc):
    nu = 2 * nb
    nominal = []
    tail = []
    for slot in range(-2, nu + 1):
        A = [('a', slot + 1, c) for c in range((slot + 1) // 2 + 1)] if 0 <= slot + 1 < nu else []
        B = [('b', slot, c) for c in range(slot // 2 + 1)] if 0 <= slot < nu else []
        Fj = []
        if slot + 2 < nu:
            Fj += [('q', slot + 2, j) for j in range(km)]
            Fj += [('k', slot + 2, j) for j in range(kc)]
            Fj += [('v', slot + 2, j) for j in range(kc)]
        if slot - 1 >= 0:
            oj = [('o', slot - 1, j) for j in range(km)]
            if OPAIR:
                oj = [('o', slot - 2 + hd, j) for j in range(km) for hd in range(2)] if slot % 2 == 0 else []
            if slot - 1 >= nu - 1 - RES:
                tail += oj
            else:
                Fj += oj
        while A or B:
            nominal += A[:GRP]; A = A[GRP:]
            nominal += B[:GRP]; B = B[GRP:]
        nominal += Fj
    nominal += tail
    last = dict(q=km - 1, k=kc - 1, v=kc - 1)
    done = {}

    def ready_at(job):
        kind, u, j = job
        hd = u % 2
        if kind == 'a':
            deps = [(('q', u), LAT_Q), (('k', 2 * j + hd), LAT_K)]
        elif kind == 'b':
            deps = [(('a', u), LAT_A), (('v', 2 * j + hd), LAT_K)]
        elif kind == 'o':
            deps = [(('b', u), LAT_B)]
        else:
            deps = []
        t = 0
        for key, lat in deps:
            if key not in done:
                return None
            t = max(t, done[key] + lat)
        return t

    order = []
    while nominal:
        n = len(order)
        seen = set()
        pick = None
        best = None
        for i, job in enumerate(nominal):
            cls = 'p' if job[0] in 'qkv' else job[0]
            if cls in seen:
                continue
            seen.add(cls)
            t = ready_at(job)
            if t is not None and t <= n:
                pick = i
                break
            if t is not None and (best is None or t < best[0]):
                best = (t, i)
            if len(seen) == 4:
                break
        if pick is None:
            pick = best[1]
        job = nominal.pop(pick)
        order.append(job)
        kind, u, j = job
        if j == last.get(kind, u // 2):
            done[(kind, u)] = n
    return order


def _kernel(x_hbm, c_hbm, wq_hbm, wuk_hbm, wuv_hbm, wo_hbm, w1_hbm, w2_hbm, w3_hbm, w4_hbm,
            cond_hbm, wmod_hbm, out_hbm,
            h_scr, acc_scr, mod_scr, x1_scr, hb_scr, t_scr, wq_buf, wk_buf, wv_buf, wo_buf, wsem,
            c_scr, cap_scr,
            x_ref, c_ref, cond_ref, wma_ref, wmb_ref, w1_ref, w2_ref, w3_ref, w4_ref, sem,
            out_buf, osem, a1_scr,
            *, S, M, Dc, H, D, RB):
    nattn = H // 2
    scale = float(D) ** -0.5 * math.log2(math.e)
    neg = -1e9 * math.log2(math.e)
    nrb = S // RB
    NX = 4
    XR = S // NX

    def wcopies(g, slot):
        cps = [pltpu.make_async_copy(src.bitcast(U32).at[:, g, :], dst.at[slot], wsem.at[slot, j])
               for j, (src, dst) in enumerate(((wq_hbm, wq_buf), (wuk_hbm, wk_buf), (wuv_hbm, wv_buf)))]
        cps.append(pltpu.make_async_copy(wo_hbm.at[g], wo_buf.at[slot], wsem.at[slot, 3]))
        return cps

    cp_cond = pltpu.make_async_copy(cond_hbm, cond_ref, sem.at[0])
    cp_wma = pltpu.make_async_copy(wmod_hbm.at[:, 0:2 * M], wma_ref, sem.at[1])
    cp_c = pltpu.make_async_copy(c_hbm, c_ref, sem.at[2])
    cp_late = [pltpu.make_async_copy(src, dst, sem.at[3 + j]) for j, (src, dst) in enumerate((
        (wmod_hbm.at[:, 2 * M:6 * M], wmb_ref), (w1_hbm, w1_ref), (w2_hbm, w2_ref),
        (w3_hbm, w3_ref), (w4_hbm, w4_ref)))]
    cp_x = [pltpu.make_async_copy(x_hbm.at[i * XR:(i + 1) * XR, :], x_ref.at[i * XR:(i + 1) * XR, :],
                                  sem.at[8 + i]) for i in range(NX)]

    def silu_cond():
        cf = cond_ref[...].astype(F32)
        return jnp.broadcast_to((cf * jax.nn.sigmoid(cf)).astype(BF16), (8, M))

    queue = [cp_cond, cp_wma] + cp_x + [cp_c] + wcopies(0, 0)
    queue = [queue[int(t, 16)] for t in os.environ.get('ORDER', '0123456789a')]
    plan = [int(t) for t in os.environ.get('PLAN', '3,2,2,4,0,0').split(',')]

    def kick():
        for _ in range(plan.pop(0)):
            queue.pop(0).start()

    kick()

    def zero(r, carry):
        acc_scr[pl.ds(pl.multiple_of(r * T, T), T), :] = jnp.zeros((T, M), F32)
        return carry

    jax.lax.fori_loop(0, S // T, zero, 0)
    cap_scr[...] = jnp.where(jax.lax.broadcasted_iota(jnp.int32, (T, T), 0)
                             <= jax.lax.broadcasted_iota(jnp.int32, (T, T), 1), jnp.inf, neg)
    acc_scr[S:S + 16, :] = jnp.zeros((16, M), F32)
    x_ref[S:S + 16, :] = jnp.zeros((16, M), BF16)
    cp_cond.wait()
    cp_wma.wait()
    kick()
    mod_scr[:, 0:2 * M] = _dot(silu_cond(), wma_ref[...])

    def ln_body(r, carry):
        sa = mod_scr[0:1, 0:M]
        ca = mod_scr[0:1, M:2 * M]
        rows = pl.ds(pl.multiple_of(r * LNR, LNR), LNR)
        hh = (_ln(x_ref[rows, :].astype(F32)) * (1.0 + ca) + sa).astype(BF16)
        for i in range(LNR // T):
            for j in range(M // T):
                h_scr[r * (LNR // T) + i, j] = _pk(hh[i * T:(i + 1) * T, j * T:(j + 1) * T])
        return carry

    for i in range(NX):
        cp_x[i].wait()
        kick()
        jax.lax.fori_loop(i * (XR // LNR), (i + 1) * (XR // LNR), ln_body, 0)

    assert not queue
    cp_c.wait()

    def cbody(r, carry):
        rows = pl.ds(pl.multiple_of(r * T, T), T)
        for j in range(Dc // T):
            c_scr[r, j] = _pk(c_ref[rows, j * T:(j + 1) * T])
        return carry

    jax.lax.fori_loop(0, S // T, cbody, 0)
    for cp in wcopies(0, 0):
        cp.wait()
    for cp in cp_late:
        cp.start()

    def attn_body(g, carry):
        slot = g & 1
        nxt = jnp.minimum(g + 1, nattn - 1)

        def mid():
            for cp in wcopies(nxt, 1 - slot):
                cp.start()

        _attention_step(h_scr, c_scr, wq_buf.at[slot], wk_buf.at[slot], wv_buf.at[slot],
                        wo_buf.at[slot], acc_scr, cap_scr, mid,
                        S=S, M=M, Dc=Dc, H=H, scale=scale, neg=neg)
        for cp in wcopies(nxt, 1 - slot):
            cp.wait()
        return carry

    jax.lax.fori_loop(0, nattn, attn_body, 0)

    for cp in cp_late:
        cp.wait()
    mod_scr[:, 2 * M:6 * M] = _dot(silu_cond(), wmb_ref[...])
    km = M // T
    Fd = w4_ref.shape[0]
    ftiles = [(f, min(f + T, Fd)) for f in range(0, Fd, T)]
    tile = lambda j: slice(j * T, (j + 1) * T)
    OFF = 16
    CAR = 32

    def p1(r0, n, dep=None):
        ga = mod_scr[0:1, 2 * M:3 * M]
        sb = mod_scr[0:1, 3 * M:4 * M]
        cb = mod_scr[0:1, 4 * M:5 * M]
        if dep is not None:
            g0 = jnp.where(dep[0:1, :] > jnp.inf, dep[0:1, :], ga[:, 0:T])
            ga = jnp.concatenate([g0, ga[:, T:]], axis=1)
        rows = pl.ds(r0, n)
        x1 = x_ref[rows, :].astype(F32) + ga * acc_scr[rows, :]
        x1_scr[rows, :] = x1
        hb = _ln(x1) * (1.0 + cb) + sb
        hb_scr[rows, :] = hb
        return _ln(hb)

    def p1_store(r0, c, dep=None):
        a1f = p1(r0 + c * PC, PC, dep)
        a1 = a1f.astype(BF16)
        for j in range(km):
            a1_scr[j, c * PC // 2:(c + 1) * PC // 2, :] = _pk(a1[:, tile(j)])
        return jnp.max(a1f[:, M - T:].reshape(PC // 8, 8, T), axis=0)

    t_scr[RB:RB + CAR - OFF, :] = jnp.zeros((CAR - OFF, M), F32)
    t_scr[RB + CAR - OFF:RB + CAR, :] = _gelu(_dot(p1(0, OFF).astype(BF16), w1_ref[...]))
    for c in range(RB // PC):
        p1_store(OFF, c)

    def out_copy(r):
        rows = pl.ds(pl.multiple_of(r * RB, RB), RB)
        return pltpu.make_async_copy(out_buf.at[rows, :], out_hbm.at[rows, :], osem.at[r])

    def b_body(r, carry):
        gb = mod_scr[0:1, 5 * M:6 * M]
        r0 = pl.multiple_of(r * RB, RB)
        n0 = pl.multiple_of(jnp.minimum(r0 + RB, S - RB) + OFF, OFF)
        nh = RB // T
        res = []

        def mm(lhs, wt, dot):
            acc = None
            for x, w in zip(lhs, wt):
                if len(res) in due:
                    w = _tie(w, due.pop(len(res)))
                v = dot(x, w)
                res.append(v)
                acc = v if acc is None else v + acc
                if len(res) in pace:
                    d = p1_store(n0, pace[len(res)], v[0:8, :T])
                    if PD:
                        due[len(res) + PD] = d
            return acc

        npc = RB // PC
        due = {}
        pace = {P0 + i * PSTEP: i for i in range(npc)}
        t_scr[0:CAR, :] = t_scr[RB:RB + CAR, :]
        for hf in range(nh):
            lhs = [pltpu.bitcast(a1_scr[j, hf * T // 2:(hf + 1) * T // 2, :], BF16) for j in range(km)]
            for n in range(km):
                t = _gelu(mm(lhs, [w1_ref[tile(j), tile(n)] for j in range(km)], _dot))
                if hf == nh - 1:
                    t = jnp.concatenate([t[:T - OFF], jnp.where(r < nrb - 1, t[T - OFF:], 0.0)], axis=0)
                t_scr[CAR + hf * T:CAR + (hf + 1) * T, tile(n)] = t
        cq = M // 4
        shifts = (-1, 1, -2, 2)
        lane = jax.lax.broadcasted_iota(jnp.int32, (T, T), 1)
        a3 = []
        z = []
        for hf in range(nh):
            base = CAR - OFF + hf * T
            lhs = []
            for j in range(km):
                g_lo, g_hi = (j * T) // cq, ((j + 1) * T - 1) // cq
                v = t_scr[base + shifts[g_lo]:base + shifts[g_lo] + T, tile(j)]
                if g_hi != g_lo:
                    v2 = t_scr[base + shifts[g_hi]:base + shifts[g_hi] + T, tile(j)]
                    v = jnp.where(lane < g_hi * cq - j * T, v, v2)
                lhs.append(v.astype(BF16))
            rows = pl.ds(pl.multiple_of(r0 + hf * T, T), T)
            y1 = jnp.concatenate(
                [mm(lhs, [w2_ref[tile(j), tile(n)] for j in range(km)], _dot) for n in range(km)], axis=1)
            y1 = y1 + hb_scr[rows, :]
            z.append(y1)
            a3.append(_ln(y1).astype(BF16))
        h3 = []
        for hf in range(nh):
            lhs = [a3[hf][:, tile(j)] for j in range(km)]
            h3.append([_gelu(mm(lhs, [w3_ref[f0:f1, tile(j)] for j in range(km)], _dot_nt)).astype(BF16)
                       for f0, f1 in ftiles])
        for hf in range(nh):
            rows = pl.ds(pl.multiple_of(r0 + hf * T, T), T)
            for n in range(km):
                v = mm(h3[hf], [w4_ref[f0:f1, tile(n)] for f0, f1 in ftiles], _dot)
                out_buf[rows, tile(n)] = (x1_scr[rows, tile(n)] + gb[:, tile(n)] * (v + z[hf][:, tile(n)])
                                          ).astype(out_buf.dtype)
        out_copy(r).start()
        return carry

    jax.lax.fori_loop(0, nrb, b_body, 0)
    for r in range(nrb):
        out_copy(r).wait()


@jax.jit
def pallas_adaLN_cond__compressed_kv_cla__mixer_s_mlp__prompt_kernel(
    A_x: jax.Array,
    A_c_kv: jax.Array,
    A_w_q: jax.Array,
    A_w_uk: jax.Array,
    A_w_uv: jax.Array,
    A_w_o: jax.Array,
    B_x: jax.Array,
    B_w1: jax.Array,
    B_w2: jax.Array,
    B_w3: jax.Array,
    B_w4: jax.Array,
    c: jax.Array,
    w_mod: jax.Array,
):
    _, S, M = A_x.shape
    Dc = A_c_kv.shape[2]
    H, D = A_w_q.shape[1], A_w_q.shape[2]
    Fd = B_w3.shape[1]
    RB = int(os.environ.get('RB', 256))
    nrb = S // RB
    out = pl.pallas_call(
        functools.partial(_kernel, S=S, M=M, Dc=Dc, H=H, D=D, RB=RB),
        in_specs=[pl.BlockSpec(memory_space=pltpu.HBM)] * 12,
        out_specs=pl.BlockSpec(memory_space=pltpu.HBM),
        out_shape=jax.ShapeDtypeStruct((S, M), A_x.dtype),
        scratch_shapes=[
            pltpu.VMEM((S // T, M // T, T // 2, T), U32),
            pltpu.VMEM((S + 16, M), F32),
            pltpu.VMEM((8, 6 * M), F32),
            pltpu.VMEM((S + 16, M), F32),
            pltpu.VMEM((S + 16, M), F32),
            pltpu.VMEM((RB + 32, M), F32),
            pltpu.VMEM((2, M, D), U32),
            pltpu.VMEM((2, Dc, D), U32),
            pltpu.VMEM((2, Dc, D), U32),
            pltpu.VMEM((2, 2 * D, M), BF16),
            pltpu.SemaphoreType.DMA((2, 4)),
            pltpu.VMEM((S // T, Dc // T, T // 2, T), U32),
            pltpu.VMEM((T, T), F32),
            pltpu.VMEM((S + 16, M), BF16),
            pltpu.VMEM((S, Dc), BF16),
            pltpu.VMEM((1, M), BF16),
            pltpu.VMEM((M, 2 * M), BF16),
            pltpu.VMEM((M, 4 * M), BF16),
            pltpu.VMEM((M, M), BF16),
            pltpu.VMEM((M, M), BF16),
            pltpu.VMEM((Fd, M), BF16),
            pltpu.VMEM((Fd, M), BF16),
            pltpu.SemaphoreType.DMA((12,)),
            pltpu.VMEM((S, M), A_x.dtype),
            pltpu.SemaphoreType.DMA((nrb,)),
            pltpu.VMEM((M // T, RB // 2, T), U32),
        ],
        compiler_params=pltpu.CompilerParams(
            vmem_limit_bytes=100 * 1024 * 1024,
            disable_bounds_checks=bool(int(os.environ.get('NOBC', 1))),
        ),
    )(
        A_x.reshape(S, M), A_c_kv.reshape(S, Dc),
        A_w_q, A_w_uk, A_w_uv,
        A_w_o.reshape(H // 2, 2 * D, M),
        B_w1, B_w2, B_w3.T, B_w4, c, w_mod,
    )
    return out.reshape(1, S, M)
```

```python
import functools
import math
import os

import jax
import jax.numpy as jnp
import jax.experimental.pallas as pl
import jax.experimental.pallas.tpu as pltpu

F32 = jnp.float32
BF16 = jnp.bfloat16
U32 = jnp.uint32
NT = (((1,), (1,)), ((), ()))
T = 128
EPS = 1e-5

GRP = int(os.environ.get('GRP', 4))
LEAD = int(os.environ.get('LEAD', 10))
PROW = int(os.environ.get('PROW', 3))
VT = int(os.environ.get('VT', 8))
RES = int(os.environ.get('RES', 5))
LAT_A = int(os.environ.get('LAT_A', 16))
LAT_B = int(os.environ.get('LAT_B', 14))
MID = int(os.environ.get('MID', 120))
PC = int(os.environ.get('PC', 32))
P0 = int(os.environ.get('P0', 176))
PSTEP = int(os.environ.get('PSTEP', 23))
DESC = int(os.environ.get('DESC', 0))
ALEAD = int(os.environ.get('ALEAD', 32))
PD = int(os.environ.get('PD', 24))


def _dot(a, b):
    return jnp.dot(a, b, preferred_element_type=F32)


def _dot_nt(a, b):
    return jax.lax.dot_general(a, b, NT, preferred_element_type=F32)


def _ln(x):
    m = jnp.mean(x, axis=-1, keepdims=True)
    xc = x - m
    v = jnp.mean(xc * xc, axis=-1, keepdims=True)
    return xc * jax.lax.rsqrt(v + EPS)


def _gelu(x):
    c0 = math.sqrt(2.0 / math.pi)
    return 0.5 * x * (1.0 + jnp.tanh(c0 * (x + 0.044715 * (x * x * x))))


def _tie(x, dep):
    xu = pltpu.bitcast(x, U32)
    first = jnp.where(dep > jnp.inf, jnp.uint32(0), xu[:8])
    return pltpu.bitcast(jnp.concatenate([first, xu[8:]], axis=0), BF16)


def _unpack_pair(wu):
    lo = pltpu.bitcast(wu << 16, F32)
    hi = pltpu.bitcast(wu & jnp.uint32(0xFFFF0000), F32)
    return lo, hi


def _ld(ref, *idx):
    return pltpu.bitcast(ref[idx], BF16)


def _pk(x):
    return pltpu.bitcast(x, U32)


class _Jobs:
    def __init__(self):
        self.res = []

    def mm(self, lhs, wt, dot, tie=False):
        acc = None
        for x, w in zip(lhs, wt):
            if tie and len(self.res) >= VT:
                x = _tie(x, self.res[len(self.res) - VT][0:8, :])
            v = dot(x, w)
            self.res.append(v)
            acc = v if acc is None else v + acc
        return acc


def _kv_jobs(jobs, r, ct, wk, wvT, k_scr, v_scr):
    for hd in range(2):
        k_scr[2 * r + hd] = _pk(jobs.mm(ct, wk(hd), _dot).astype(BF16))
    for hd in range(2):
        v_scr[2 * r + hd] = _pk(jobs.mm(wvT(hd), ct, _dot_nt, True).astype(BF16))


def _q_jobs(jobs, r, ht, wq, q_scr, scale):
    for hd in range(2):
        q_scr[2 * r + hd] = _pk((jobs.mm(ht, wq(hd), _dot) * scale).astype(BF16))


def _unpack_tiles(w_ref, transpose=False):
    out = []
    for j in range(w_ref.shape[0] // T):
        pair = [w.astype(BF16) for w in _unpack_pair(w_ref[j * T:(j + 1) * T, :])]
        out.append([w.T for w in pair] if transpose else pair)
    return out


def _proj_step(h_scr, c_scr, wq_ref, wuk_ref, wuv_ref, q_scr, k_scr, v_scr, *, scale):
    wk = _unpack_tiles(wuk_ref)
    wq = _unpack_tiles(wq_ref)
    wvT = _unpack_tiles(wuv_ref, True)
    jobs = _Jobs()
    for r in range(h_scr.shape[0]):
        ct = [_ld(c_scr, r, j) for j in range(len(wk))]
        ht = [_ld(h_scr, r, j) for j in range(len(wq))]
        _q_jobs(jobs, r, ht, lambda hd: [t[hd] for t in wq], q_scr, scale)
        _kv_jobs(jobs, r, ct, lambda hd: [t[hd] for t in wk], lambda hd: [t[hd] for t in wvT], k_scr, v_scr)


def _attention_step(q_scr, k_scr, v_scr, wo_ref, acc_scr, cap_ref, mid, *, S, M):
    nb = S // T
    km = M // T
    tile = lambda j: slice(j * T, (j + 1) * T)
    sv = {}; mx = {}; mfin = {}; lsum = {}; o = {}
    part = {}
    res = []

    def accum(key, val):
        res.append(val)
        part[key] = val if key not in part else val + part[key]
        return part[key]

    def job_a(u, cidx):
        r, hd = divmod(u, 2)
        s = _dot_nt(_ld(k_scr, 2 * cidx + hd), _ld(q_scr, u))
        res.append(s)
        if cidx == r:
            s = jnp.minimum(s, cap_ref[...])
        s = s.reshape(T // 8, 8, T)
        sv[(u, cidx)] = s
        pm = jnp.max(s, axis=0)
        mx[u] = pm if u not in mx else jnp.maximum(mx[u], pm)

    def job_b(u, cidx):
        r, hd = divmod(u, 2)
        if u not in mfin:
            mfin[u] = jnp.broadcast_to(jnp.max(mx[u], axis=0, keepdims=True), (8, T))
        s = sv.pop((u, cidx))
        m = mfin[u]
        if LEAD and len(res) >= LEAD:
            r0 = 8 * ((PROW * (cidx % 4)) % 16)
            src = res[len(res) - LEAD][r0:r0 + 8, :]
            m = jnp.where(src > jnp.inf, src, m)
        p = jnp.exp2(s - m[None])
        ls = jnp.sum(p, axis=0)
        lsum[u] = ls if u not in lsum else lsum[u] + ls
        v = accum(('o', u), _dot(_ld(v_scr, 2 * cidx + hd), p.reshape(T, T).astype(BF16)))
        if cidx == r:
            l = jnp.sum(lsum[u], axis=0, keepdims=True)
            o[u] = _tie((v * (1.0 / l)).astype(BF16).T, lsum[u])

    def job_o(u, j):
        r, hd = divmod(u, 2)
        v = _dot(o[u], wo_ref[tile(hd), tile(j)])
        res.append(v)
        acc_scr[tile(r), tile(j)] += v

    fns = dict(a=job_a, b=job_b, o=job_o)
    for n, (kind, u, j) in enumerate(_job_order(nb, km)):
        if n == MID:
            mid()
        fns[kind](u, j)


def _job_order(nb, km):
    nu = 2 * nb
    units = list(range(nu))
    if DESC:
        units = units[::-1]
    QA = [('a', u, c) for u in units for c in range(u // 2 + 1)]
    QB = [('b', u, c) for u in units for c in range(u // 2 + 1)]
    QO = [('o', u, j) for u in units for j in range(km)]
    done = {}
    order = []

    def ready(q, lat, pre):
        return bool(q) and (pre, q[0][1]) in done and done[(pre, q[0][1])] + lat <= len(order)

    def emit(q):
        job = q.pop(0)
        kind, u, j = job
        if kind != 'o' and j == u // 2:
            done[(kind, u)] = len(order)
        order.append(job)

    turn = 0
    while QA or QB or QO:
        pref = ('a', 'b', 'o')[turn % 3]
        turn += 1
        for _ in range(GRP if pref != 'o' else km):
            lead = len(QB) - len(QA)
            if pref == 'a' and QA and (lead < ALEAD or not ready(QB, LAT_A, 'a')):
                emit(QA)
            elif pref == 'b' and ready(QB, LAT_A, 'a'):
                emit(QB)
            elif pref == 'o' and ready(QO, LAT_B, 'b') and (len(QO) > RES * km or not (QA or ready(QB, LAT_A, 'a'))):
                emit(QO)
            elif not QA and not ready(QB, LAT_A, 'a') and not ready(QO, LAT_B, 'b'):
                if QB: emit(QB)
                elif QO: emit(QO)
            else:
                break
    return order


def _kernel(x_hbm, c_hbm, wq_hbm, wuk_hbm, wuv_hbm, wo_hbm, w1_hbm, w2_hbm, w3_hbm, w4_hbm,
            cond_hbm, wmod_hbm, out_hbm,
            h_scr, acc_scr, mod_scr, x1_scr, hb_scr, t_scr, wq_buf, wk_buf, wv_buf, wo_buf, wsem,
            c_scr, cap_scr,
            x_ref, c_ref, cond_ref, wma_ref, wmb_ref, w1_ref, w2_ref, w3_ref, w4_ref, sem,
            out_buf, osem, a1_scr, q_scr, k_scr, v_scr, w_scr,
            *, S, M, Dc, H, D, RB):
    nattn = H // 2
    scale = float(D) ** -0.5 * math.log2(math.e)
    neg = -1e9 * math.log2(math.e)
    nrb = S // RB
    NX = 4
    XR = S // NX

    km, kc = M // T, Dc // T
    CB = XR // T

    def pcopies(g):
        return [pltpu.make_async_copy(src.bitcast(U32).at[:, g, :], dst, wsem.at[j])
                for j, (src, dst) in enumerate(((wuk_hbm, wk_buf), (wuv_hbm, wv_buf), (wq_hbm, wq_buf)))]

    def ocopy(g, slot):
        return pltpu.make_async_copy(wo_hbm.at[g], wo_buf.at[slot], wsem.at[3])

    def chunk_copy(src, dst, i, s0):
        rows = pl.ds(i * XR if isinstance(i, int) else pl.multiple_of(i * XR, XR), XR)
        return pltpu.make_async_copy(src.at[rows, :], dst.at[rows, :], sem.at[s0 + i])

    cp_cond = pltpu.make_async_copy(cond_hbm, cond_ref, sem.at[0])
    cp_wma = pltpu.make_async_copy(wmod_hbm.at[:, 0:2 * M], wma_ref, sem.at[1])
    cp_late = [pltpu.make_async_copy(src, dst, sem.at[2 + j]) for j, (src, dst) in enumerate((
        (wmod_hbm.at[:, 2 * M:6 * M], wmb_ref), (w1_hbm, w1_ref), (w2_hbm, w2_ref),
        (w3_hbm, w3_ref), (w4_hbm, w4_ref)))]
    cp_x = lambda i: chunk_copy(x_hbm, x_ref, i, 7)
    cp_c = lambda i: chunk_copy(c_hbm, c_ref, i, 7 + NX)

    def silu_cond():
        cf = cond_ref[...].astype(F32)
        return jnp.broadcast_to((cf * jax.nn.sigmoid(cf)).astype(BF16), (8, M))

    cp_wk, cp_wv, cp_wq = pcopies(0)
    named = dict(k=cp_wk, v=cp_wv, q=cp_wq, o=ocopy(0, 0), n=cp_cond, m=cp_wma)
    named.update({'abcd'[i]: cp_c(i) for i in range(NX)})
    named.update({'wxyz'[i]: cp_x(i) for i in range(NX)})
    plan = os.environ.get('PLAN', 'kvab,cnm,wd,qxyzo').split(',')

    def kick():
        if plan:
            for ch in plan.pop(0):
                named.pop(ch).start()

    kick()

    def zero(r, carry):
        acc_scr[pl.ds(pl.multiple_of(r * T, T), T), :] = jnp.zeros((T, M), F32)
        return carry

    jax.lax.fori_loop(0, S // T, zero, 0)
    cap_scr[...] = jnp.where(jax.lax.broadcasted_iota(jnp.int32, (T, T), 0)
                             <= jax.lax.broadcasted_iota(jnp.int32, (T, T), 1), jnp.inf, neg)
    acc_scr[S:S + 16, :] = jnp.zeros((16, M), F32)
    x_ref[S:S + 16, :] = jnp.zeros((16, M), BF16)
    cp_wk.wait()
    cp_wv.wait()
    kick()
    for j, pair in enumerate(_unpack_tiles(wk_buf) + _unpack_tiles(wv_buf, True)):
        for hd in range(2):
            w_scr[hd, j] = _pk(pair[hd])

    def kv_chunk(jobs, i):
        for b in range(CB):
            r = i * CB + b
            rows = pl.ds(r * T if isinstance(r, int) else pl.multiple_of(r * T, T), T)
            ct = [c_ref[rows, j * T:(j + 1) * T] for j in range(kc)]
            for j in range(kc):
                c_scr[r, j] = _pk(ct[j])
            _kv_jobs(jobs, r, ct, lambda hd: [_ld(w_scr, hd, j) for j in range(kc)],
                     lambda hd: [_ld(w_scr, hd, kc + j) for j in range(kc)], k_scr, v_scr)

    def q_chunk(jobs, i):
        for b in range(CB):
            r = i * CB + b
            _q_jobs(jobs, r, [_ld(h_scr, r, j) for j in range(km)],
                    lambda hd: [_ld(w_scr, hd, 2 * kc + j) for j in range(km)], q_scr, scale)

    def ln_chunk(i):
        sa = mod_scr[0:1, 0:M]
        ca = mod_scr[0:1, M:2 * M]
        for b in range(CB):
            r = i * CB + b
            rows = pl.ds(r * T if isinstance(r, int) else pl.multiple_of(r * T, T), T)
            hh = (_ln(x_ref[rows, :].astype(F32)) * (1.0 + ca) + sa).astype(BF16)
            for j in range(km):
                h_scr[r, j] = _pk(hh[:, j * T:(j + 1) * T])

    def kv_body(i, carry):
        cp_c(i).wait()
        kv_chunk(_Jobs(), i)
        return carry

    jax.lax.fori_loop(0, 1, kv_body, 0)
    kick()
    jax.lax.fori_loop(1, NX - 1, kv_body, 0)
    kick()
    cp_cond.wait()
    cp_wma.wait()
    mod_scr[:, 0:2 * M] = _dot(silu_cond(), wma_ref[...])
    cp_x(0).wait()
    cp_c(NX - 1).wait()
    kv_chunk(_Jobs(), NX - 1)
    ln_chunk(0)
    cp_wq.wait()
    for j, pair in enumerate(_unpack_tiles(wq_buf)):
        for hd in range(2):
            w_scr[hd, 2 * kc + j] = _pk(pair[hd])

    def q_body(i, carry):
        cp_x(i + 1).wait()
        q_chunk(_Jobs(), i)
        ln_chunk(i + 1)
        return carry

    jax.lax.fori_loop(0, NX - 1, q_body, 0)
    q_chunk(_Jobs(), NX - 1)
    assert not named
    ocopy(0, 0).wait()
    for cp in cp_late:
        cp.start()

    def attn_body(g, carry):
        slot = g & 1
        nxt = jnp.minimum(g + 1, nattn - 1)

        def mid():
            for cp in pcopies(nxt) + [ocopy(nxt, 1 - slot)]:
                cp.start()

        _attention_step(q_scr, k_scr, v_scr, wo_buf.at[slot], acc_scr, cap_scr, mid, S=S, M=M)
        for cp in pcopies(nxt) + [ocopy(nxt, 1 - slot)]:
            cp.wait()

        @pl.when(g + 1 < nattn)
        def _():
            _proj_step(h_scr, c_scr, wq_buf, wk_buf, wv_buf, q_scr, k_scr, v_scr, scale=scale)

        return carry

    jax.lax.fori_loop(0, nattn, attn_body, 0)

    for cp in cp_late:
        cp.wait()
    mod_scr[:, 2 * M:6 * M] = _dot(silu_cond(), wmb_ref[...])
    Fd = w4_ref.shape[0]
    ftiles = [(f, min(f + T, Fd)) for f in range(0, Fd, T)]
    tile = lambda j: slice(j * T, (j + 1) * T)
    OFF = 16
    CAR = 32

    def p1(r0, n, dep=None):
        ga = mod_scr[0:1, 2 * M:3 * M]
        sb = mod_scr[0:1, 3 * M:4 * M]
        cb = mod_scr[0:1, 4 * M:5 * M]
        if dep is not None:
            g0 = jnp.where(dep[0:1, :] > jnp.inf, dep[0:1, :], ga[:, 0:T])
            ga = jnp.concatenate([g0, ga[:, T:]], axis=1)
        rows = pl.ds(r0, n)
        x1 = x_ref[rows, :].astype(F32) + ga * acc_scr[rows, :]
        x1_scr[rows, :] = x1
        hb = _ln(x1) * (1.0 + cb) + sb
        hb_scr[rows, :] = hb
        return _ln(hb)

    def p1_store(r0, c, dep=None):
        a1f = p1(r0 + c * PC, PC, dep)
        a1 = a1f.astype(BF16)
        for j in range(km):
            a1_scr[j, c * PC // 2:(c + 1) * PC // 2, :] = _pk(a1[:, tile(j)])
        return jnp.max(a1f[:, M - T:].reshape(PC // 8, 8, T), axis=0)

    t_scr[RB:RB + CAR - OFF, :] = jnp.zeros((CAR - OFF, M), F32)
    t_scr[RB + CAR - OFF:RB + CAR, :] = _gelu(_dot(p1(0, OFF).astype(BF16), w1_ref[...]))
    for c in range(RB // PC):
        p1_store(OFF, c)

    def out_copy(r):
        rows = pl.ds(pl.multiple_of(r * RB, RB), RB)
        return pltpu.make_async_copy(out_buf.at[rows, :], out_hbm.at[rows, :], osem.at[r])

    def b_body(r, carry):
        gb = mod_scr[0:1, 5 * M:6 * M]
        r0 = pl.multiple_of(r * RB, RB)
        n0 = pl.multiple_of(jnp.minimum(r0 + RB, S - RB) + OFF, OFF)
        nh = RB // T
        res = []

        def mm(lhs, wt, dot):
            acc = None
            for x, w in zip(lhs, wt):
                if len(res) in due:
                    w = _tie(w, due.pop(len(res)))
                v = dot(x, w)
                res.append(v)
                acc = v if acc is None else v + acc
                if len(res) in pace:
                    d = p1_store(n0, pace[len(res)], v[0:8, :T])
                    if PD:
                        due[len(res) + PD] = d
            return acc

        npc = RB // PC
        due = {}
        pace = {P0 + i * PSTEP: i for i in range(npc)}
        t_scr[0:CAR, :] = t_scr[RB:RB + CAR, :]
        for hf in range(nh):
            lhs = [pltpu.bitcast(a1_scr[j, hf * T // 2:(hf + 1) * T // 2, :], BF16) for j in range(km)]
            for n in range(km):
                t = _gelu(mm(lhs, [w1_ref[tile(j), tile(n)] for j in range(km)], _dot))
                if hf == nh - 1:
                    t = jnp.concatenate([t[:T - OFF], jnp.where(r < nrb - 1, t[T - OFF:], 0.0)], axis=0)
                t_scr[CAR + hf * T:CAR + (hf + 1) * T, tile(n)] = t
        cq = M // 4
        shifts = (-1, 1, -2, 2)
        lane = jax.lax.broadcasted_iota(jnp.int32, (T, T), 1)
        a3 = []
        z = []
        for hf in range(nh):
            base = CAR - OFF + hf * T
            lhs = []
            for j in range(km):
                g_lo, g_hi = (j * T) // cq, ((j + 1) * T - 1) // cq
                v = t_scr[base + shifts[g_lo]:base + shifts[g_lo] + T, tile(j)]
                if g_hi != g_lo:
                    v2 = t_scr[base + shifts[g_hi]:base + shifts[g_hi] + T, tile(j)]
                    v = jnp.where(lane < g_hi * cq - j * T, v, v2)
                lhs.append(v.astype(BF16))
            rows = pl.ds(pl.multiple_of(r0 + hf * T, T), T)
            y1 = jnp.concatenate(
                [mm(lhs, [w2_ref[tile(j), tile(n)] for j in range(km)], _dot) for n in range(km)], axis=1)
            y1 = y1 + hb_scr[rows, :]
            z.append(y1)
            a3.append(_ln(y1).astype(BF16))
        h3 = []
        for hf in range(nh):
            lhs = [a3[hf][:, tile(j)] for j in range(km)]
            h3.append([_gelu(mm(lhs, [w3_ref[f0:f1, tile(j)] for j in range(km)], _dot_nt)).astype(BF16)
                       for f0, f1 in ftiles])
        for hf in range(nh):
            rows = pl.ds(pl.multiple_of(r0 + hf * T, T), T)
            for n in range(km):
                v = mm(h3[hf], [w4_ref[f0:f1, tile(n)] for f0, f1 in ftiles], _dot)
                out_buf[rows, tile(n)] = (x1_scr[rows, tile(n)] + gb[:, tile(n)] * (v + z[hf][:, tile(n)])
                                          ).astype(out_buf.dtype)
        out_copy(r).start()
        return carry

    jax.lax.fori_loop(0, nrb, b_body, 0)
    for r in range(nrb):
        out_copy(r).wait()


@jax.jit
def pallas_adaLN_cond__compressed_kv_cla__mixer_s_mlp__prompt_kernel(
    A_x: jax.Array,
    A_c_kv: jax.Array,
    A_w_q: jax.Array,
    A_w_uk: jax.Array,
    A_w_uv: jax.Array,
    A_w_o: jax.Array,
    B_x: jax.Array,
    B_w1: jax.Array,
    B_w2: jax.Array,
    B_w3: jax.Array,
    B_w4: jax.Array,
    c: jax.Array,
    w_mod: jax.Array,
):
    _, S, M = A_x.shape
    Dc = A_c_kv.shape[2]
    H, D = A_w_q.shape[1], A_w_q.shape[2]
    Fd = B_w3.shape[1]
    RB = int(os.environ.get('RB', 256))
    nrb = S // RB
    out = pl.pallas_call(
        functools.partial(_kernel, S=S, M=M, Dc=Dc, H=H, D=D, RB=RB),
        in_specs=[pl.BlockSpec(memory_space=pltpu.HBM)] * 12,
        out_specs=pl.BlockSpec(memory_space=pltpu.HBM),
        out_shape=jax.ShapeDtypeStruct((S, M), A_x.dtype),
        scratch_shapes=[
            pltpu.VMEM((S // T, M // T, T // 2, T), U32),
            pltpu.VMEM((S + 16, M), F32),
            pltpu.VMEM((8, 6 * M), F32),
            pltpu.VMEM((S + 16, M), F32),
            pltpu.VMEM((S + 16, M), F32),
            pltpu.VMEM((RB + 32, M), F32),
            pltpu.VMEM((M, D), U32),
            pltpu.VMEM((Dc, D), U32),
            pltpu.VMEM((Dc, D), U32),
            pltpu.VMEM((2, 2 * D, M), BF16),
            pltpu.SemaphoreType.DMA((4,)),
            pltpu.VMEM((S // T, Dc // T, T // 2, T), U32),
            pltpu.VMEM((T, T), F32),
            pltpu.VMEM((S + 16, M), BF16),
            pltpu.VMEM((S, Dc), BF16),
            pltpu.VMEM((1, M), BF16),
            pltpu.VMEM((M, 2 * M), BF16),
            pltpu.VMEM((M, 4 * M), BF16),
            pltpu.VMEM((M, M), BF16),
            pltpu.VMEM((M, M), BF16),
            pltpu.VMEM((Fd, M), BF16),
            pltpu.VMEM((Fd, M), BF16),
            pltpu.SemaphoreType.DMA((15,)),
            pltpu.VMEM((S, M), A_x.dtype),
            pltpu.SemaphoreType.DMA((nrb,)),
            pltpu.VMEM((M // T, RB // 2, T), U32),
            pltpu.VMEM((2 * S // T, T // 2, T), U32),
            pltpu.VMEM((2 * S // T, T // 2, T), U32),
            pltpu.VMEM((2 * S // T, T // 2, T), U32),
            pltpu.VMEM((2, M // T + 2 * (Dc // T), T // 2, T), U32),
        ],
        compiler_params=pltpu.CompilerParams(
            vmem_limit_bytes=100 * 1024 * 1024,
            disable_bounds_checks=bool(int(os.environ.get('NOBC', 1))),
        ),
    )(
        A_x.reshape(S, M), A_c_kv.reshape(S, Dc),
        A_w_q, A_w_uk, A_w_uv,
        A_w_o.reshape(H // 2, 2 * D, M),
        B_w1, B_w2, B_w3.T, B_w4, c, w_mod,
    )
    return out.reshape(1, S, M)
```

```python
import functools
import math
import os

import jax
import jax.numpy as jnp
import jax.experimental.pallas as pl
import jax.experimental.pallas.tpu as pltpu

F32 = jnp.float32
BF16 = jnp.bfloat16
U32 = jnp.uint32
NT = (((1,), (1,)), ((), ()))
T = 128
EPS = 1e-5

GRP = int(os.environ.get('GRP', 4))
LEAD = int(os.environ.get('LEAD', 10))
PROW = int(os.environ.get('PROW', 3))
VT = int(os.environ.get('VT', 8))
RES = int(os.environ.get('RES', 5))
LAT_A = int(os.environ.get('LAT_A', 16))
LAT_B = int(os.environ.get('LAT_B', 14))
MID = int(os.environ.get('MID', 120))
PC = int(os.environ.get('PC', 32))
P0 = int(os.environ.get('P0', 176))
PSTEP = int(os.environ.get('PSTEP', 23))
DESC = int(os.environ.get('DESC', 0))
ALEAD = int(os.environ.get('ALEAD', 32))
BUNR = int(os.environ.get('BUNR', 1))
LP = int(os.environ.get('LP', 32))
LL = int(os.environ.get('LL', 6))
KVL = int(os.environ.get('KVL', 2))
QLAG = int(os.environ.get('QLAG', 2))
PD = int(os.environ.get('PD', 24))


def _dot(a, b):
    return jnp.dot(a, b, preferred_element_type=F32)


def _dot_nt(a, b):
    return jax.lax.dot_general(a, b, NT, preferred_element_type=F32)


def _ln(x):
    m = jnp.mean(x, axis=-1, keepdims=True)
    xc = x - m
    v = jnp.mean(xc * xc, axis=-1, keepdims=True)
    return xc * jax.lax.rsqrt(v + EPS)


def _gelu(x):
    c0 = math.sqrt(2.0 / math.pi)
    return 0.5 * x * (1.0 + jnp.tanh(c0 * (x + 0.044715 * (x * x * x))))


def _tie(x, dep):
    xu = pltpu.bitcast(x, U32)
    first = jnp.where(dep > jnp.inf, jnp.uint32(0), xu[:8])
    return pltpu.bitcast(jnp.concatenate([first, xu[8:]], axis=0), BF16)


def _unpack_pair(wu):
    lo = pltpu.bitcast(wu << 16, F32)
    hi = pltpu.bitcast(wu & jnp.uint32(0xFFFF0000), F32)
    return lo, hi


def _ld(ref, *idx):
    return pltpu.bitcast(ref[idx], BF16)


def _pk(x):
    return pltpu.bitcast(x, U32)


class _Jobs:
    def __init__(self):
        self.res = []

    def mm(self, lhs, wt, dot, tie=False):
        acc = None
        for x, w in zip(lhs, wt):
            if tie and len(self.res) >= VT:
                x = _tie(x, self.res[len(self.res) - VT][0:8, :])
            v = dot(x, w)
            self.res.append(v)
            acc = v if acc is None else v + acc
        return acc


def _kv_jobs(jobs, r, ct, wk, wvT, k_scr, v_scr):
    for hd in range(2):
        k_scr[2 * r + hd] = _pk(jobs.mm(ct, wk(hd), _dot).astype(BF16))
    for hd in range(2):
        v_scr[2 * r + hd] = _pk(jobs.mm(wvT(hd), ct, _dot_nt, True).astype(BF16))


def _q_jobs(jobs, r, ht, wq, q_scr, scale):
    for hd in range(2):
        q_scr[2 * r + hd] = _pk((jobs.mm(ht, wq(hd), _dot) * scale).astype(BF16))


def _unpack_tiles(w_ref, transpose=False):
    out = []
    for j in range(w_ref.shape[0] // T):
        pair = [w.astype(BF16) for w in _unpack_pair(w_ref[j * T:(j + 1) * T, :])]
        out.append([w.T for w in pair] if transpose else pair)
    return out


def _proj_step(h_scr, c_ref, wq_ref, wuk_ref, wuv_ref, q_scr, k_scr, v_scr, *, scale):
    wk = _unpack_tiles(wuk_ref)
    wq = _unpack_tiles(wq_ref)
    wvT = _unpack_tiles(wuv_ref, True)
    jobs = _Jobs()
    for r in range(h_scr.shape[0]):
        ct = [c_ref[r * T:(r + 1) * T, j * T:(j + 1) * T] for j in range(len(wk))]
        ht = [h_scr[r, j] for j in range(len(wq))]
        _q_jobs(jobs, r, ht, lambda hd: [t[hd] for t in wq], q_scr, scale)
        _kv_jobs(jobs, r, ct, lambda hd: [t[hd] for t in wk], lambda hd: [t[hd] for t in wvT], k_scr, v_scr)


def _attention_step(q_scr, k_scr, v_scr, wo_ref, acc_scr, cap_ref, mid, *, S, M):
    nb = S // T
    km = M // T
    tile = lambda j: slice(j * T, (j + 1) * T)
    sv = {}; mx = {}; mfin = {}; lsum = {}; o = {}
    part = {}
    res = []

    def accum(key, val):
        res.append(val)
        part[key] = val if key not in part else val + part[key]
        return part[key]

    def job_a(u, cidx):
        r, hd = divmod(u, 2)
        s = _dot_nt(_ld(k_scr, 2 * cidx + hd), _ld(q_scr, u))
        res.append(s)
        if cidx == r:
            s = jnp.minimum(s, cap_ref[...])
        s = s.reshape(T // 8, 8, T)
        sv[(u, cidx)] = s
        pm = jnp.max(s, axis=0)
        mx[u] = pm if u not in mx else jnp.maximum(mx[u], pm)

    def job_b(u, cidx):
        r, hd = divmod(u, 2)
        if u not in mfin:
            mfin[u] = jnp.broadcast_to(jnp.max(mx[u], axis=0, keepdims=True), (8, T))
        s = sv.pop((u, cidx))
        m = mfin[u]
        if LEAD and len(res) >= LEAD:
            r0 = 8 * ((PROW * (cidx % 4)) % 16)
            src = res[len(res) - LEAD][r0:r0 + 8, :]
            m = jnp.where(src > jnp.inf, src, m)
        p = jnp.exp2(s - m[None])
        ls = jnp.sum(p, axis=0)
        lsum[u] = ls if u not in lsum else lsum[u] + ls
        v = accum(('o', u), _dot(_ld(v_scr, 2 * cidx + hd), p.reshape(T, T).astype(BF16)))
        if cidx == r:
            l = jnp.sum(lsum[u], axis=0, keepdims=True)
            o[u] = _tie((v * (1.0 / l)).astype(BF16).T, lsum[u])

    def job_o(u, j):
        r, hd = divmod(u, 2)
        v = _dot(o[u], wo_ref[tile(hd), tile(j)])
        res.append(v)
        acc_scr[tile(r), tile(j)] += v

    fns = dict(a=job_a, b=job_b, o=job_o)
    for n, (kind, u, j) in enumerate(_job_order(nb, km)):
        if n == MID:
            mid()
        fns[kind](u, j)


def _job_order(nb, km):
    nu = 2 * nb
    units = list(range(nu))
    if DESC:
        units = units[::-1]
    QA = [('a', u, c) for u in units for c in range(u // 2 + 1)]
    QB = [('b', u, c) for u in units for c in range(u // 2 + 1)]
    QO = [('o', u, j) for u in units for j in range(km)]
    done = {}
    order = []

    def ready(q, lat, pre):
        return bool(q) and (pre, q[0][1]) in done and done[(pre, q[0][1])] + lat <= len(order)

    def emit(q):
        job = q.pop(0)
        kind, u, j = job
        if kind != 'o' and j == u // 2:
            done[(kind, u)] = len(order)
        order.append(job)

    turn = 0
    while QA or QB or QO:
        pref = ('a', 'b', 'o')[turn % 3]
        turn += 1
        for _ in range(GRP if pref != 'o' else km):
            lead = len(QB) - len(QA)
            if pref == 'a' and QA and (lead < ALEAD or not ready(QB, LAT_A, 'a')):
                emit(QA)
            elif pref == 'b' and ready(QB, LAT_A, 'a'):
                emit(QB)
            elif pref == 'o' and ready(QO, LAT_B, 'b') and (len(QO) > RES * km or not (QA or ready(QB, LAT_A, 'a'))):
                emit(QO)
            elif not QA and not ready(QB, LAT_A, 'a') and not ready(QO, LAT_B, 'b'):
                if QB: emit(QB)
                elif QO: emit(QO)
            else:
                break
    return order


def _kernel(x_hbm, c_hbm, wq_hbm, wuk_hbm, wuv_hbm, wo_hbm, w1_hbm, w2_hbm, w3_hbm, w4_hbm,
            cond_hbm, wmod_hbm, out_hbm,
            h_scr, acc_scr, mod_scr, x1_scr, hb_scr, t_scr, wq_buf, wk_buf, wv_buf, wo_buf, wsem,
            cap_scr,
            x_ref, c_ref, cond_ref, wma_ref, wmb_ref, w1_ref, w2_ref, w3_ref, w4_ref, sem,
            out_buf, osem, a1_scr, q_scr, k_scr, v_scr, w_scr,
            *, S, M, Dc, H, D, RB):
    nattn = H // 2
    scale = float(D) ** -0.5 * math.log2(math.e)
    neg = -1e9 * math.log2(math.e)
    nrb = S // RB
    NX = 4
    XR = S // NX

    km, kc = M // T, Dc // T
    CB = XR // T

    def pcopies(g):
        return [pltpu.make_async_copy(src.bitcast(U32).at[:, g, :], dst, wsem.at[j])
                for j, (src, dst) in enumerate(((wuk_hbm, wk_buf), (wuv_hbm, wv_buf), (wq_hbm, wq_buf)))]

    def ocopy(g, slot):
        return pltpu.make_async_copy(wo_hbm.at[g], wo_buf.at[slot], wsem.at[3])

    def chunk_copy(src, dst, i, s0):
        rows = pl.ds(i * XR if isinstance(i, int) else pl.multiple_of(i * XR, XR), XR)
        return pltpu.make_async_copy(src.at[rows, :], dst.at[rows, :], sem.at[s0 + i])

    cp_cond = pltpu.make_async_copy(cond_hbm, cond_ref, sem.at[0])
    cp_wma = pltpu.make_async_copy(wmod_hbm.at[:, 0:2 * M], wma_ref, sem.at[1])
    cp_late = [pltpu.make_async_copy(src, dst, sem.at[2 + j]) for j, (src, dst) in enumerate((
        (wmod_hbm.at[:, 2 * M:6 * M], wmb_ref), (w1_hbm, w1_ref), (w2_hbm, w2_ref),
        (w3_hbm, w3_ref), (w4_hbm, w4_ref)))]
    cp_x = lambda i: chunk_copy(x_hbm, x_ref, i, 7)
    cp_c = lambda i: chunk_copy(c_hbm, c_ref, i, 7 + NX)

    def silu_cond():
        cf = cond_ref[...].astype(F32)
        return jnp.broadcast_to((cf * jax.nn.sigmoid(cf)).astype(BF16), (8, M))

    cp_wk, cp_wv, cp_wq = pcopies(0)
    named = dict(k=cp_wk, v=cp_wv, q=cp_wq, o=ocopy(0, 0), n=cp_cond, m=cp_wma)
    named.update({'abcd'[i]: cp_c(i) for i in range(NX)})
    named.update({'wxyz'[i]: cp_x(i) for i in range(NX)})
    plan = os.environ.get('PLAN', 'kva,bc,dnq,mwx,yzo').split(',')

    def kick():
        if plan:
            for ch in plan.pop(0):
                named.pop(ch).start()

    kick()

    def zero(r, carry):
        acc_scr[pl.ds(pl.multiple_of(r * T, T), T), :] = jnp.zeros((T, M), F32)
        return carry

    jax.lax.fori_loop(0, S // T, zero, 0)
    kick()
    cap_scr[...] = jnp.where(jax.lax.broadcasted_iota(jnp.int32, (T, T), 0)
                             <= jax.lax.broadcasted_iota(jnp.int32, (T, T), 1), jnp.inf, neg)
    acc_scr[S:S + 16, :] = jnp.zeros((16, M), F32)
    x_ref[S:S + 16, :] = jnp.zeros((16, M), BF16)
    nb = S // T
    tile = lambda j: slice(j * T, (j + 1) * T)
    hist = []

    def kv_tile(jobs, r, wk, wvT):
        _kv_jobs(jobs, r, [c_ref[tile(r), tile(j)] for j in range(kc)], wk, wvT, k_scr, v_scr)

    def q_tile(jobs, r, wq):
        _q_jobs(jobs, r, [h_scr[r, j] for j in range(km)], wq, q_scr, scale)

    def ln_tile(r):
        sa = mod_scr[0:1, 0:M]
        ca = mod_scr[0:1, M:2 * M]
        for i in range(T // LP):
            xf = x_ref[r * T + i * LP:r * T + (i + 1) * LP, :].astype(F32)
            if LL and len(hist) >= LL:
                dep = jnp.broadcast_to(hist[-LL][None], (LP // 8, 8, T)).reshape(LP, T)
                xf = jnp.concatenate([jnp.where(dep > jnp.inf, dep, xf[:, :T]), xf[:, T:]], axis=1)
            hf = _ln(xf) * (1.0 + ca) + sa
            hist.append(jnp.max(hf[:, M - T:].reshape(LP // 8, 8, T), axis=0))
            hh = hf.astype(BF16)
            for j in range(km):
                h_scr[r, j, i * LP:(i + 1) * LP, :] = hh[:, tile(j)]

    def stash(tiles, j0):
        for j, pair in enumerate(tiles):
            for hd in range(2):
                w_scr[hd, j0 + j] = _pk(pair[hd])
        return lambda hd: [_ld(w_scr, hd, j0 + j) for j in range(len(tiles))]

    cp_wk.wait()
    cp_wv.wait()
    cp_c(0).wait()
    kick()
    wk = stash(_unpack_tiles(wk_buf), 0)
    wvT = stash(_unpack_tiles(wv_buf, True), kc)
    jobs = _Jobs()
    for r in range(CB):
        kv_tile(jobs, r, wk, wvT)
    for i in range(1, NX):
        cp_c(i).wait()
    kick()
    jobs = _Jobs()
    for r in range(CB, nb - KVL):
        kv_tile(jobs, r, wk, wvT)
    cp_cond.wait()
    cp_wma.wait()
    cp_wq.wait()
    wq = None
    qdone = 0
    for grp in os.environ.get('XG', '0,1,23').split(','):
        chunks = [int(ch) for ch in grp]
        for i in chunks:
            cp_x(i).wait()
        kick()
        jobs = _Jobs()
        del hist[:]
        if chunks[0] == 0:
            mod_scr[:, 0:2 * M] = _dot(silu_cond(), wma_ref[...])
            wq = stash(_unpack_tiles(wq_buf), 2 * kc)
            for r in range(nb - KVL, nb):
                kv_tile(jobs, r, wk, wvT)
        for r in range(chunks[0] * CB, (chunks[-1] + 1) * CB):
            ln_tile(r)
        qend = nb if chunks[-1] == NX - 1 else (chunks[-1] + 1) * CB - QLAG
        for r in range(qdone, qend):
            q_tile(jobs, r, wq)
        qdone = qend
    assert not named
    ocopy(0, 0).wait()
    for cp in cp_late:
        cp.start()

    def attn_body(g, carry):
        slot = g & 1
        nxt = jnp.minimum(g + 1, nattn - 1)

        def mid():
            for cp in pcopies(nxt) + [ocopy(nxt, 1 - slot)]:
                cp.start()

        _attention_step(q_scr, k_scr, v_scr, wo_buf.at[slot], acc_scr, cap_scr, mid, S=S, M=M)
        for cp in pcopies(nxt) + [ocopy(nxt, 1 - slot)]:
            cp.wait()

        @pl.when(g + 1 < nattn)
        def _():
            _proj_step(h_scr, c_ref, wq_buf, wk_buf, wv_buf, q_scr, k_scr, v_scr, scale=scale)

        return carry

    jax.lax.fori_loop(0, nattn, attn_body, 0)

    for cp in cp_late:
        cp.wait()
    mod_scr[:, 2 * M:6 * M] = _dot(silu_cond(), wmb_ref[...])
    Fd = w4_ref.shape[0]
    ftiles = [(f, min(f + T, Fd)) for f in range(0, Fd, T)]
    OFF = 16
    CAR = 32

    def p1(r0, n, dep=None):
        ga = mod_scr[0:1, 2 * M:3 * M]
        sb = mod_scr[0:1, 3 * M:4 * M]
        cb = mod_scr[0:1, 4 * M:5 * M]
        if dep is not None:
            g0 = jnp.where(dep[0:1, :] > jnp.inf, dep[0:1, :], ga[:, 0:T])
            ga = jnp.concatenate([g0, ga[:, T:]], axis=1)
        rows = pl.ds(r0, n)
        x1 = x_ref[rows, :].astype(F32) + ga * acc_scr[rows, :]
        x1_scr[rows, :] = x1
        hb = _ln(x1) * (1.0 + cb) + sb
        hb_scr[rows, :] = hb
        return _ln(hb)

    def p1_store(r0, c, dep=None):
        a1f = p1(r0 + c * PC, PC, dep)
        a1 = a1f.astype(BF16)
        for j in range(km):
            a1_scr[j, c * PC:(c + 1) * PC, :] = a1[:, tile(j)]
        return jnp.max(a1f[:, M - T:].reshape(PC // 8, 8, T), axis=0)

    t_scr[RB:RB + CAR - OFF, :] = jnp.zeros((CAR - OFF, M), F32)
    t_scr[RB + CAR - OFF:RB + CAR, :] = _gelu(_dot(p1(0, OFF).astype(BF16), w1_ref[...]))
    for c in range(RB // PC):
        p1_store(OFF, c)

    def out_copy(r):
        rows = pl.ds(pl.multiple_of(r * RB, RB), RB)
        return pltpu.make_async_copy(out_buf.at[rows, :], out_hbm.at[rows, :], osem.at[r])

    def b_body(r, carry):
        gb = mod_scr[0:1, 5 * M:6 * M]
        r0 = pl.multiple_of(r * RB, RB)
        n0 = pl.multiple_of(jnp.minimum(r0 + RB, S - RB) + OFF, OFF)
        nh = RB // T
        res = []

        def mm(lhs, wt, dot):
            acc = None
            for x, w in zip(lhs, wt):
                if len(res) in due:
                    w = _tie(w, due.pop(len(res)))
                v = dot(x, w)
                res.append(v)
                acc = v if acc is None else v + acc
                if len(res) in pace:
                    d = p1_store(n0, pace[len(res)], v[0:8, :T])
                    if PD:
                        due[len(res) + PD] = d
            return acc

        npc = RB // PC
        due = {}
        pace = {P0 + i * PSTEP: i for i in range(npc)}
        t_scr[0:CAR, :] = t_scr[RB:RB + CAR, :]
        for hf in range(nh):
            lhs = [a1_scr[j, tile(hf), :] for j in range(km)]
            for n in range(km):
                t = _gelu(mm(lhs, [w1_ref[tile(j), tile(n)] for j in range(km)], _dot))
                if hf == nh - 1:
                    t = jnp.concatenate([t[:T - OFF], jnp.where(r < nrb - 1, t[T - OFF:], 0.0)], axis=0)
                t_scr[CAR + hf * T:CAR + (hf + 1) * T, tile(n)] = t
        cq = M // 4
        shifts = (-1, 1, -2, 2)
        lane = jax.lax.broadcasted_iota(jnp.int32, (T, T), 1)
        a3 = []
        z = []
        for hf in range(nh):
            base = CAR - OFF + hf * T
            lhs = []
            for j in range(km):
                g_lo, g_hi = (j * T) // cq, ((j + 1) * T - 1) // cq
                v = t_scr[base + shifts[g_lo]:base + shifts[g_lo] + T, tile(j)]
                if g_hi != g_lo:
                    v2 = t_scr[base + shifts[g_hi]:base + shifts[g_hi] + T, tile(j)]
                    v = jnp.where(lane < g_hi * cq - j * T, v, v2)
                lhs.append(v.astype(BF16))
            rows = pl.ds(pl.multiple_of(r0 + hf * T, T), T)
            y1 = jnp.concatenate(
                [mm(lhs, [w2_ref[tile(j), tile(n)] for j in range(km)], _dot) for n in range(km)], axis=1)
            y1 = y1 + hb_scr[rows, :]
            z.append(y1)
            a3.append(_ln(y1).astype(BF16))
        h3 = []
        for hf in range(nh):
            lhs = [a3[hf][:, tile(j)] for j in range(km)]
            h3.append([_gelu(mm(lhs, [w3_ref[f0:f1, tile(j)] for j in range(km)], _dot_nt)).astype(BF16)
                       for f0, f1 in ftiles])
        for hf in range(nh):
            rows = pl.ds(pl.multiple_of(r0 + hf * T, T), T)
            for n in range(km):
                v = mm(h3[hf], [w4_ref[f0:f1, tile(n)] for f0, f1 in ftiles], _dot)
                out_buf[rows, tile(n)] = (x1_scr[rows, tile(n)] + gb[:, tile(n)] * (v + z[hf][:, tile(n)])
                                          ).astype(out_buf.dtype)
        out_copy(r).start()
        return carry

    jax.lax.fori_loop(0, nrb, b_body, 0, unroll=BUNR)
    for r in range(nrb):
        out_copy(r).wait()


@jax.jit
def pallas_adaLN_cond__compressed_kv_cla__mixer_s_mlp__prompt_kernel(
    A_x: jax.Array,
    A_c_kv: jax.Array,
    A_w_q: jax.Array,
    A_w_uk: jax.Array,
    A_w_uv: jax.Array,
    A_w_o: jax.Array,
    B_x: jax.Array,
    B_w1: jax.Array,
    B_w2: jax.Array,
    B_w3: jax.Array,
    B_w4: jax.Array,
    c: jax.Array,
    w_mod: jax.Array,
):
    _, S, M = A_x.shape
    Dc = A_c_kv.shape[2]
    H, D = A_w_q.shape[1], A_w_q.shape[2]
    Fd = B_w3.shape[1]
    RB = int(os.environ.get('RB', 256))
    nrb = S // RB
    out = pl.pallas_call(
        functools.partial(_kernel, S=S, M=M, Dc=Dc, H=H, D=D, RB=RB),
        in_specs=[pl.BlockSpec(memory_space=pltpu.HBM)] * 12,
        out_specs=pl.BlockSpec(memory_space=pltpu.HBM),
        out_shape=jax.ShapeDtypeStruct((S, M), A_x.dtype),
        scratch_shapes=[
            pltpu.VMEM((S // T, M // T, T, T), BF16),
            pltpu.VMEM((S + 16, M), F32),
            pltpu.VMEM((8, 6 * M), F32),
            pltpu.VMEM((S + 16, M), F32),
            pltpu.VMEM((S + 16, M), F32),
            pltpu.VMEM((RB + 32, M), F32),
            pltpu.VMEM((M, D), U32),
            pltpu.VMEM((Dc, D), U32),
            pltpu.VMEM((Dc, D), U32),
            pltpu.VMEM((2, 2 * D, M), BF16),
            pltpu.SemaphoreType.DMA((4,)),
            pltpu.VMEM((T, T), F32),
            pltpu.VMEM((S + 16, M), BF16),
            pltpu.VMEM((S, Dc), BF16),
            pltpu.VMEM((1, M), BF16),
            pltpu.VMEM((M, 2 * M), BF16),
            pltpu.VMEM((M, 4 * M), BF16),
            pltpu.VMEM((M, M), BF16),
            pltpu.VMEM((M, M), BF16),
            pltpu.VMEM((Fd, M), BF16),
            pltpu.VMEM((Fd, M), BF16),
            pltpu.SemaphoreType.DMA((15,)),
            pltpu.VMEM((S, M), A_x.dtype),
            pltpu.SemaphoreType.DMA((nrb,)),
            pltpu.VMEM((M // T, RB, T), BF16),
            pltpu.VMEM((2 * S // T, T // 2, T), U32),
            pltpu.VMEM((2 * S // T, T // 2, T), U32),
            pltpu.VMEM((2 * S // T, T // 2, T), U32),
            pltpu.VMEM((2, M // T + 2 * (Dc // T), T // 2, T), U32),
        ],
        compiler_params=pltpu.CompilerParams(
            vmem_limit_bytes=100 * 1024 * 1024,
            disable_bounds_checks=bool(int(os.environ.get('NOBC', 1))),
        ),
    )(
        A_x.reshape(S, M), A_c_kv.reshape(S, Dc),
        A_w_q, A_w_uk, A_w_uv,
        A_w_o.reshape(H // 2, 2 * D, M),
        B_w1, B_w2, B_w3.T, B_w4, c, w_mod,
    )
    return out.reshape(1, S, M)
```

```python
import functools
import math
import os

import jax
import jax.numpy as jnp
import jax.experimental.pallas as pl
import jax.experimental.pallas.tpu as pltpu

F32 = jnp.float32
BF16 = jnp.bfloat16
U32 = jnp.uint32
NT = (((1,), (1,)), ((), ()))
T = 128
EPS = 1e-5

GRP = int(os.environ.get('GRP', 4))
LEAD = int(os.environ.get('LEAD', 10))
PROW = int(os.environ.get('PROW', 3))
VT = int(os.environ.get('VT', 8))
RES = int(os.environ.get('RES', 5))
LAT_A = int(os.environ.get('LAT_A', 16))
LAT_B = int(os.environ.get('LAT_B', 14))
MID = int(os.environ.get('MID', 120))
PC = int(os.environ.get('PC', 32))
P0 = int(os.environ.get('P0', 180))
PSTEP = int(os.environ.get('PSTEP', 21))
DESC = int(os.environ.get('DESC', 0))
ALEAD = int(os.environ.get('ALEAD', 32))
BUNR = int(os.environ.get('BUNR', 1))
LP = int(os.environ.get('LP', 32))
LL = int(os.environ.get('LL', 6))
KVL = int(os.environ.get('KVL', 2))
QLAG = int(os.environ.get('QLAG', 2))
NW0 = int(os.environ.get('NW0', 5))
NWS = int(os.environ.get('NWS', 1))
PD = int(os.environ.get('PD', 24))


def _dot(a, b):
    return jnp.dot(a, b, preferred_element_type=F32)


def _dot_nt(a, b):
    return jax.lax.dot_general(a, b, NT, preferred_element_type=F32)


def _ln(x):
    m = jnp.mean(x, axis=-1, keepdims=True)
    xc = x - m
    v = jnp.mean(xc * xc, axis=-1, keepdims=True)
    return xc * jax.lax.rsqrt(v + EPS)


def _gelu(x):
    c0 = math.sqrt(2.0 / math.pi)
    return 0.5 * x * (1.0 + jnp.tanh(c0 * (x + 0.044715 * (x * x * x))))


def _tie(x, dep):
    xu = pltpu.bitcast(x, U32)
    first = jnp.where(dep > jnp.inf, jnp.uint32(0), xu[:8])
    return pltpu.bitcast(jnp.concatenate([first, xu[8:]], axis=0), BF16)


def _unpack_pair(wu):
    lo = pltpu.bitcast(wu << 16, F32)
    hi = pltpu.bitcast(wu & jnp.uint32(0xFFFF0000), F32)
    return lo, hi


def _ld(ref, *idx):
    return pltpu.bitcast(ref[idx], BF16)


def _pk(x):
    return pltpu.bitcast(x, U32)


class _Jobs:
    def __init__(self):
        self.res = []

    def mm(self, lhs, wt, dot, tie=False):
        acc = None
        for x, w in zip(lhs, wt):
            if tie and len(self.res) >= VT:
                x = _tie(x, self.res[len(self.res) - VT][0:8, :])
            v = dot(x, w)
            self.res.append(v)
            acc = v if acc is None else v + acc
        return acc


def _kv_jobs(jobs, r, ct, wk, wvT, k_scr, v_scr):
    for hd in range(2):
        k_scr[2 * r + hd] = _pk(jobs.mm(ct, wk(hd), _dot).astype(BF16))
    for hd in range(2):
        v_scr[2 * r + hd] = _pk(jobs.mm(wvT(hd), ct, _dot_nt, True).astype(BF16))


def _q_jobs(jobs, r, ht, wq, q_scr, scale):
    for hd in range(2):
        q_scr[2 * r + hd] = _pk((jobs.mm(ht, wq(hd), _dot) * scale).astype(BF16))


def _unpack_tiles(w_ref, transpose=False):
    out = []
    for j in range(w_ref.shape[0] // T):
        pair = [w.astype(BF16) for w in _unpack_pair(w_ref[j * T:(j + 1) * T, :])]
        out.append([w.T for w in pair] if transpose else pair)
    return out


def _proj_step(h_scr, c_ref, wq_ref, wuk_ref, wuv_ref, q_scr, k_scr, v_scr, *, scale):
    wk = _unpack_tiles(wuk_ref)
    wq = _unpack_tiles(wq_ref)
    wvT = _unpack_tiles(wuv_ref, True)
    jobs = _Jobs()
    for r in range(h_scr.shape[0]):
        ct = [c_ref[r * T:(r + 1) * T, j * T:(j + 1) * T] for j in range(len(wk))]
        ht = [h_scr[r, j] for j in range(len(wq))]
        _q_jobs(jobs, r, ht, lambda hd: [t[hd] for t in wq], q_scr, scale)
        _kv_jobs(jobs, r, ct, lambda hd: [t[hd] for t in wk], lambda hd: [t[hd] for t in wvT], k_scr, v_scr)


def _attention_step(q_scr, k_scr, v_scr, wo_ref, acc_scr, cap_ref, mid, *, S, M):
    nb = S // T
    km = M // T
    tile = lambda j: slice(j * T, (j + 1) * T)
    sv = {}; mx = {}; mfin = {}; lsum = {}; o = {}
    part = {}
    res = []

    def accum(key, val):
        res.append(val)
        part[key] = val if key not in part else val + part[key]
        return part[key]

    def job_a(u, cidx):
        r, hd = divmod(u, 2)
        s = _dot_nt(_ld(k_scr, 2 * cidx + hd), _ld(q_scr, u))
        res.append(s)
        if cidx == r:
            s = jnp.minimum(s, cap_ref[...])
        s = s.reshape(T // 8, 8, T)
        sv[(u, cidx)] = s
        pm = jnp.max(s, axis=0)
        mx[u] = pm if u not in mx else jnp.maximum(mx[u], pm)

    def job_b(u, cidx):
        r, hd = divmod(u, 2)
        if u not in mfin:
            mfin[u] = jnp.broadcast_to(jnp.max(mx[u], axis=0, keepdims=True), (8, T))
        s = sv.pop((u, cidx))
        m = mfin[u]
        if LEAD and len(res) >= LEAD:
            r0 = 8 * ((PROW * (cidx % 4)) % 16)
            src = res[len(res) - LEAD][r0:r0 + 8, :]
            m = jnp.where(src > jnp.inf, src, m)
        p = jnp.exp2(s - m[None])
        ls = jnp.sum(p, axis=0)
        lsum[u] = ls if u not in lsum else lsum[u] + ls
        v = accum(('o', u), _dot(_ld(v_scr, 2 * cidx + hd), p.reshape(T, T).astype(BF16)))
        if cidx == r:
            l = jnp.sum(lsum[u], axis=0, keepdims=True)
            o[u] = _tie((v * (1.0 / l)).astype(BF16).T, lsum[u])

    def job_o(u, j):
        r, hd = divmod(u, 2)
        v = _dot(o[u], wo_ref[tile(hd), tile(j)])
        res.append(v)
        acc_scr[tile(r), tile(j)] += v

    fns = dict(a=job_a, b=job_b, o=job_o)
    for n, (kind, u, j) in enumerate(_job_order(nb, km)):
        if n == MID:
            mid()
        fns[kind](u, j)


def _job_order(nb, km):
    nu = 2 * nb
    units = list(range(nu))
    if DESC:
        units = units[::-1]
    QA = [('a', u, c) for u in units for c in range(u // 2 + 1)]
    QB = [('b', u, c) for u in units for c in range(u // 2 + 1)]
    QO = [('o', u, j) for u in units for j in range(km)]
    done = {}
    order = []

    def ready(q, lat, pre):
        return bool(q) and (pre, q[0][1]) in done and done[(pre, q[0][1])] + lat <= len(order)

    def emit(q):
        job = q.pop(0)
        kind, u, j = job
        if kind != 'o' and j == u // 2:
            done[(kind, u)] = len(order)
        order.append(job)

    turn = 0
    while QA or QB or QO:
        pref = ('a', 'b', 'o')[turn % 3]
        turn += 1
        for _ in range(GRP if pref != 'o' else km):
            lead = len(QB) - len(QA)
            if pref == 'a' and QA and (lead < ALEAD or not ready(QB, LAT_A, 'a')):
                emit(QA)
            elif pref == 'b' and ready(QB, LAT_A, 'a'):
                emit(QB)
            elif pref == 'o' and ready(QO, LAT_B, 'b') and (len(QO) > RES * km or not (QA or ready(QB, LAT_A, 'a'))):
                emit(QO)
            elif not QA and not ready(QB, LAT_A, 'a') and not ready(QO, LAT_B, 'b'):
                if QB: emit(QB)
                elif QO: emit(QO)
            else:
                break
    return order


def _kernel(x_hbm, c_hbm, wq_hbm, wuk_hbm, wuv_hbm, wo_hbm, w1_hbm, w2_hbm, w3_hbm, w4_hbm,
            cond_hbm, wmod_hbm, out_hbm,
            h_scr, acc_scr, mod_scr, x1_scr, hb_scr, t_scr, wq_buf, wk_buf, wv_buf, wo_buf, wsem,
            cap_scr,
            x_ref, c_ref, cond_ref, wma_ref, wmb_ref, w1_ref, w2_ref, w3_ref, w4_ref, sem,
            out_buf, osem, a1_scr, q_scr, k_scr, v_scr, w_scr,
            *, S, M, Dc, H, D, RB):
    nattn = H // 2
    scale = float(D) ** -0.5 * math.log2(math.e)
    neg = -1e9 * math.log2(math.e)
    nrb = S // RB
    NX = 4
    XR = S // NX

    km, kc = M // T, Dc // T
    CB = XR // T

    def pcopies(g):
        return [pltpu.make_async_copy(src.bitcast(U32).at[:, g, :], dst, wsem.at[j])
                for j, (src, dst) in enumerate(((wuk_hbm, wk_buf), (wuv_hbm, wv_buf), (wq_hbm, wq_buf)))]

    def ocopy(g, slot):
        return pltpu.make_async_copy(wo_hbm.at[g], wo_buf.at[slot], wsem.at[3])

    def chunk_copy(src, dst, i, s0):
        rows = pl.ds(i * XR if isinstance(i, int) else pl.multiple_of(i * XR, XR), XR)
        return pltpu.make_async_copy(src.at[rows, :], dst.at[rows, :], sem.at[s0 + i])

    cp_cond = pltpu.make_async_copy(cond_hbm, cond_ref, sem.at[0])
    cp_wma = pltpu.make_async_copy(wmod_hbm.at[:, 0:2 * M], wma_ref, sem.at[1])
    cp_late = [pltpu.make_async_copy(src, dst, sem.at[2 + j]) for j, (src, dst) in enumerate((
        (wmod_hbm.at[:, 2 * M:6 * M], wmb_ref), (w1_hbm, w1_ref), (w2_hbm, w2_ref),
        (w3_hbm, w3_ref), (w4_hbm, w4_ref)))]
    cp_x = lambda i: chunk_copy(x_hbm, x_ref, i, 7)
    cp_c = lambda i: chunk_copy(c_hbm, c_ref, i, 7 + NX)

    def silu_cond():
        cf = cond_ref[...].astype(F32)
        return jnp.broadcast_to((cf * jax.nn.sigmoid(cf)).astype(BF16), (8, M))

    cp_wk, cp_wv, cp_wq = pcopies(0)
    named = dict(k=cp_wk, v=cp_wv, q=cp_wq, o=ocopy(0, 0), n=cp_cond, m=cp_wma)
    named.update({'abcd'[i]: cp_c(i) for i in range(NX)})
    named.update({'wxyz'[i]: cp_x(i) for i in range(NX)})
    plan = os.environ.get('PLAN', 'kva,bc,dnq,mwx,yzo').split(',')

    def kick():
        if plan:
            for ch in plan.pop(0):
                named.pop(ch).start()

    kick()

    def zero(r, carry):
        acc_scr[pl.ds(pl.multiple_of(r * T, T), T), :] = jnp.zeros((T, M), F32)
        return carry

    jax.lax.fori_loop(0, S // T, zero, 0)
    kick()
    cap_scr[...] = jnp.where(jax.lax.broadcasted_iota(jnp.int32, (T, T), 0)
                             <= jax.lax.broadcasted_iota(jnp.int32, (T, T), 1), jnp.inf, neg)
    acc_scr[S:S + 16, :] = jnp.zeros((16, M), F32)
    x_ref[S:S + 16, :] = jnp.zeros((16, M), BF16)
    nb = S // T
    tile = lambda j: slice(j * T, (j + 1) * T)
    hist = []

    def kv_tile(jobs, r, wk, wvT):
        _kv_jobs(jobs, r, [c_ref[tile(r), tile(j)] for j in range(kc)], wk, wvT, k_scr, v_scr)

    def q_tile(jobs, r, wq):
        _q_jobs(jobs, r, [h_scr[r, j] for j in range(km)], wq, q_scr, scale)

    def ln_tile(r):
        sa = mod_scr[0:1, 0:M]
        ca = mod_scr[0:1, M:2 * M]
        for i in range(T // LP):
            xf = x_ref[r * T + i * LP:r * T + (i + 1) * LP, :].astype(F32)
            if LL and len(hist) >= LL:
                dep = jnp.broadcast_to(hist[-LL][None], (LP // 8, 8, T)).reshape(LP, T)
                xf = jnp.concatenate([jnp.where(dep > jnp.inf, dep, xf[:, :T]), xf[:, T:]], axis=1)
            hf = _ln(xf) * (1.0 + ca) + sa
            hist.append(jnp.max(hf[:, M - T:].reshape(LP // 8, 8, T), axis=0))
            hh = hf.astype(BF16)
            for j in range(km):
                h_scr[r, j, i * LP:(i + 1) * LP, :] = hh[:, tile(j)]

    def stash(tiles, j0):
        for j, pair in enumerate(tiles):
            for hd in range(2):
                w_scr[hd, j0 + j] = _pk(pair[hd])
        return lambda hd: [_ld(w_scr, hd, j0 + j) for j in range(len(tiles))]

    cp_wk.wait()
    cp_wv.wait()
    cp_c(0).wait()
    kick()
    wk = stash(_unpack_tiles(wk_buf), 0)
    wvT = stash(_unpack_tiles(wv_buf, True), kc)
    jobs = _Jobs()
    for r in range(CB):
        kv_tile(jobs, r, wk, wvT)
    for i in range(1, NX):
        cp_c(i).wait()
    kick()
    jobs = _Jobs()
    for r in range(CB, nb - KVL):
        kv_tile(jobs, r, wk, wvT)
    cp_cond.wait()
    cp_wma.wait()
    cp_wq.wait()
    wq = None
    qdone = 0
    for grp in os.environ.get('XG', '0,1,23').split(','):
        chunks = [int(ch) for ch in grp]
        for i in chunks:
            cp_x(i).wait()
        kick()
        jobs = _Jobs()
        del hist[:]
        if chunks[0] == 0:
            mod_scr[:, 0:2 * M] = _dot(silu_cond(), wma_ref[...])
            wq = stash(_unpack_tiles(wq_buf), 2 * kc)
            for r in range(nb - KVL, nb):
                kv_tile(jobs, r, wk, wvT)
        for r in range(chunks[0] * CB, (chunks[-1] + 1) * CB):
            ln_tile(r)
        qend = nb if chunks[-1] == NX - 1 else (chunks[-1] + 1) * CB - QLAG
        for r in range(qdone, qend):
            q_tile(jobs, r, wq)
        qdone = max(qdone, qend)
    assert not named
    ocopy(0, 0).wait()
    for cp in cp_late:
        cp.start()

    def attn_body(g, carry):
        slot = g & 1
        nxt = jnp.minimum(g + 1, nattn - 1)

        def mid():
            for cp in pcopies(nxt) + [ocopy(nxt, 1 - slot)]:
                cp.start()

        _attention_step(q_scr, k_scr, v_scr, wo_buf.at[slot], acc_scr, cap_scr, mid, S=S, M=M)
        for cp in pcopies(nxt) + [ocopy(nxt, 1 - slot)]:
            cp.wait()

        @pl.when(g + 1 < nattn)
        def _():
            _proj_step(h_scr, c_ref, wq_buf, wk_buf, wv_buf, q_scr, k_scr, v_scr, scale=scale)

        return carry

    jax.lax.fori_loop(0, nattn, attn_body, 0)

    for cp in cp_late:
        cp.wait()
    mod_scr[:, 2 * M:6 * M] = _dot(silu_cond(), wmb_ref[...])
    Fd = w4_ref.shape[0]
    ftiles = [(f, min(f + T, Fd)) for f in range(0, Fd, T)]
    OFF = 16
    CAR = 32

    def p1(r0, n, dep=None):
        ga = mod_scr[0:1, 2 * M:3 * M]
        sb = mod_scr[0:1, 3 * M:4 * M]
        cb = mod_scr[0:1, 4 * M:5 * M]
        if dep is not None:
            g0 = jnp.where(dep[0:1, :] > jnp.inf, dep[0:1, :], ga[:, 0:T])
            ga = jnp.concatenate([g0, ga[:, T:]], axis=1)
        rows = pl.ds(r0, n)
        x1 = x_ref[rows, :].astype(F32) + ga * acc_scr[rows, :]
        x1_scr[rows, :] = x1
        hb = _ln(x1) * (1.0 + cb) + sb
        hb_scr[rows, :] = hb
        return _ln(hb)

    def p1_store(r0, c, dep=None):
        a1f = p1(r0 + c * PC, PC, dep)
        a1 = a1f.astype(BF16)
        for j in range(km):
            a1_scr[j, c * PC:(c + 1) * PC, :] = a1[:, tile(j)]
        return jnp.max(a1f[:, M - T:].reshape(PC // 8, 8, T), axis=0)

    t_scr[RB:RB + CAR - OFF, :] = jnp.zeros((CAR - OFF, M), F32)
    t_scr[RB + CAR - OFF:RB + CAR, :] = _gelu(_dot(p1(0, OFF).astype(BF16), w1_ref[...]))
    for c in range(RB // PC):
        p1_store(OFF, c)

    def out_copy(i):
        rows = pl.ds(i * T if isinstance(i, int) else pl.multiple_of(i * T, T), T)
        return pltpu.make_async_copy(out_buf.at[rows, :], out_hbm.at[rows, :], osem.at[i])

    def b_body(r, carry):
        gb = mod_scr[0:1, 5 * M:6 * M]
        r0 = pl.multiple_of(r * RB, RB)
        n0 = pl.multiple_of(jnp.minimum(r0 + RB, S - RB) + OFF, OFF)
        nh = RB // T
        res = []

        def mm(lhs, wt, dot):
            acc = None
            for x, w in zip(lhs, wt):
                if len(res) in due:
                    w = _tie(w, due.pop(len(res)))
                v = dot(x, w)
                res.append(v)
                acc = v if acc is None else v + acc
                if len(res) in pace:
                    d = p1_store(n0, pace[len(res)], v[0:8, :T])
                    if PD:
                        due[len(res) + PD] = d
            return acc

        npc = RB // PC
        due = {}
        pace = {P0 + i * PSTEP: i for i in range(npc)}
        t_scr[0:CAR, :] = t_scr[RB:RB + CAR, :]
        for hf in range(nh):
            lhs = [a1_scr[j, tile(hf), :] for j in range(km)]
            for n in range(km):
                t = _gelu(mm(lhs, [w1_ref[tile(j), tile(n)] for j in range(km)], _dot))
                if hf == nh - 1:
                    t = jnp.concatenate([t[:T - OFF], jnp.where(r < nrb - 1, t[T - OFF:], 0.0)], axis=0)
                t_scr[CAR + hf * T:CAR + (hf + 1) * T, tile(n)] = t
        cq = M // 4
        shifts = (-1, 1, -2, 2)
        lane = jax.lax.broadcasted_iota(jnp.int32, (T, T), 1)
        a3 = []
        z = []
        for hf in range(nh):
            base = CAR - OFF + hf * T
            lhs = []
            for j in range(km):
                g_lo, g_hi = (j * T) // cq, ((j + 1) * T - 1) // cq
                v = t_scr[base + shifts[g_lo]:base + shifts[g_lo] + T, tile(j)]
                if g_hi != g_lo:
                    v2 = t_scr[base + shifts[g_hi]:base + shifts[g_hi] + T, tile(j)]
                    v = jnp.where(lane < g_hi * cq - j * T, v, v2)
                lhs.append(v.astype(BF16))
            rows = pl.ds(pl.multiple_of(r0 + hf * T, T), T)
            y1 = jnp.concatenate(
                [mm(lhs, [w2_ref[tile(j), tile(n)] for j in range(km)], _dot) for n in range(km)], axis=1)
            y1 = y1 + hb_scr[rows, :]
            z.append(y1)
            a3.append(_ln(y1).astype(BF16))
        h3 = []
        for hf in range(nh):
            lhs = [a3[hf][:, tile(j)] for j in range(km)]
            row = []
            narrow = None
            for i, (f0, f1) in enumerate(ftiles):
                if f1 - f0 == T:
                    wt = [w3_ref[f0:f1, tile(j)] for j in range(km)]
                    row.append(_gelu(mm(lhs, wt, _dot_nt)).astype(BF16))
                    j, rem = divmod(i - NW0, NWS)
                    if Fd % T and rem == 0 and 0 <= j < km:
                        v = mm([w3_ref[ftiles[-1][0]:Fd, tile(j)]], [lhs[j]], _dot_nt)
                        narrow = v if narrow is None else v + narrow
                else:
                    gT = jnp.concatenate([_gelu(narrow), jnp.zeros((T - (f1 - f0), T), F32)], axis=0)
                    row.append(_tie(gT.astype(BF16).T, gT[0:8, :])[:, :f1 - f0])
            h3.append(row)
        for hf in range(nh):
            rows = pl.ds(pl.multiple_of(r0 + hf * T, T), T)
            for n in range(km):
                v = mm(h3[hf], [w4_ref[f0:f1, tile(n)] for f0, f1 in ftiles], _dot)
                out_buf[rows, tile(n)] = (x1_scr[rows, tile(n)] + gb[:, tile(n)] * (v + z[hf][:, tile(n)])
                                          ).astype(out_buf.dtype)
            out_copy(r * nh + hf).start()
        return carry

    jax.lax.fori_loop(0, nrb, b_body, 0, unroll=BUNR)
    for i in range(nb):
        out_copy(i).wait()


@jax.jit
def pallas_adaLN_cond__compressed_kv_cla__mixer_s_mlp__prompt_kernel(
    A_x: jax.Array,
    A_c_kv: jax.Array,
    A_w_q: jax.Array,
    A_w_uk: jax.Array,
    A_w_uv: jax.Array,
    A_w_o: jax.Array,
    B_x: jax.Array,
    B_w1: jax.Array,
    B_w2: jax.Array,
    B_w3: jax.Array,
    B_w4: jax.Array,
    c: jax.Array,
    w_mod: jax.Array,
):
    _, S, M = A_x.shape
    Dc = A_c_kv.shape[2]
    H, D = A_w_q.shape[1], A_w_q.shape[2]
    Fd = B_w3.shape[1]
    RB = int(os.environ.get('RB', 256))
    nrb = S // RB
    out = pl.pallas_call(
        functools.partial(_kernel, S=S, M=M, Dc=Dc, H=H, D=D, RB=RB),
        in_specs=[pl.BlockSpec(memory_space=pltpu.HBM)] * 12,
        out_specs=pl.BlockSpec(memory_space=pltpu.HBM),
        out_shape=jax.ShapeDtypeStruct((S, M), A_x.dtype),
        scratch_shapes=[
            pltpu.VMEM((S // T, M // T, T, T), BF16),
            pltpu.VMEM((S + 16, M), F32),
            pltpu.VMEM((8, 6 * M), F32),
            pltpu.VMEM((S + 16, M), F32),
            pltpu.VMEM((S + 16, M), F32),
            pltpu.VMEM((RB + 32, M), F32),
            pltpu.VMEM((M, D), U32),
            pltpu.VMEM((Dc, D), U32),
            pltpu.VMEM((Dc, D), U32),
            pltpu.VMEM((2, 2 * D, M), BF16),
            pltpu.SemaphoreType.DMA((4,)),
            pltpu.VMEM((T, T), F32),
            pltpu.VMEM((S + 16, M), BF16),
            pltpu.VMEM((S, Dc), BF16),
            pltpu.VMEM((1, M), BF16),
            pltpu.VMEM((M, 2 * M), BF16),
            pltpu.VMEM((M, 4 * M), BF16),
            pltpu.VMEM((M, M), BF16),
            pltpu.VMEM((M, M), BF16),
            pltpu.VMEM((Fd, M), BF16),
            pltpu.VMEM((Fd, M), BF16),
            pltpu.SemaphoreType.DMA((15,)),
            pltpu.VMEM((S, M), A_x.dtype),
            pltpu.SemaphoreType.DMA((S // T,)),
            pltpu.VMEM((M // T, RB, T), BF16),
            pltpu.VMEM((2 * S // T, T // 2, T), U32),
            pltpu.VMEM((2 * S // T, T // 2, T), U32),
            pltpu.VMEM((2 * S // T, T // 2, T), U32),
            pltpu.VMEM((2, M // T + 2 * (Dc // T), T // 2, T), U32),
        ],
        compiler_params=pltpu.CompilerParams(
            vmem_limit_bytes=100 * 1024 * 1024,
            disable_bounds_checks=bool(int(os.environ.get('NOBC', 1))),
        ),
    )(
        A_x.reshape(S, M), A_c_kv.reshape(S, Dc),
        A_w_q, A_w_uk, A_w_uv,
        A_w_o.reshape(H // 2, 2 * D, M),
        B_w1, B_w2, B_w3.T, B_w4, c, w_mod,
    )
    return out.reshape(1, S, M)
```

```python
import functools
import math
import os

import jax
import jax.numpy as jnp
import jax.experimental.pallas as pl
import jax.experimental.pallas.tpu as pltpu

F32 = jnp.float32
BF16 = jnp.bfloat16
U32 = jnp.uint32
NT = (((1,), (1,)), ((), ()))
T = 128
EPS = 1e-5

GRP = int(os.environ.get('GRP', 4))
LEAD = int(os.environ.get('LEAD', 10))
PROW = int(os.environ.get('PROW', 3))
VT = int(os.environ.get('VT', 8))
RES = int(os.environ.get('RES', 5))
LAT_A = int(os.environ.get('LAT_A', 16))
LAT_B = int(os.environ.get('LAT_B', 14))
MID = int(os.environ.get('MID', 120))
PC = int(os.environ.get('PC', 32))
P0 = int(os.environ.get('P0', 180))
PSTEP = int(os.environ.get('PSTEP', 21))
DESC = int(os.environ.get('DESC', 0))
ALEAD = int(os.environ.get('ALEAD', 32))
BUNR = int(os.environ.get('BUNR', 1))
LP = int(os.environ.get('LP', 32))
LL = int(os.environ.get('LL', 0))
KVL = int(os.environ.get('KVL', 1))
QLAG = int(os.environ.get('QLAG', 2))
NW0 = int(os.environ.get('NW0', 5))
NWS = int(os.environ.get('NWS', 1))
RSQ = int(os.environ.get('RSQ', 1))
KVM = int(os.environ.get('KVM', 2))
PD = int(os.environ.get('PD', 24))


def _dot(a, b):
    return jnp.dot(a, b, preferred_element_type=F32)


def _dot_nt(a, b):
    return jax.lax.dot_general(a, b, NT, preferred_element_type=F32)


def _ln(x):
    m = jnp.mean(x, axis=-1, keepdims=True)
    xc = x - m
    v = jnp.mean(xc * xc, axis=-1, keepdims=True)
    if RSQ:
        return xc * jnp.exp2(jnp.log(v + EPS) * (-0.5 / math.log(2.0)))
    return xc * jax.lax.rsqrt(v + EPS)


def _rows(v, n):
    return jnp.broadcast_to(v[None], (n // 8, 8, v.shape[1])).reshape(n, v.shape[1])


def _gelu(x):
    c0 = math.sqrt(2.0 / math.pi)
    return 0.5 * x * (1.0 + jnp.tanh(c0 * (x + 0.044715 * (x * x * x))))


def _tie(x, dep):
    xu = pltpu.bitcast(x, U32)
    first = jnp.where(dep > jnp.inf, jnp.uint32(0), xu[:8])
    return pltpu.bitcast(jnp.concatenate([first, xu[8:]], axis=0), BF16)


def _unpack_pair(wu):
    lo = pltpu.bitcast(wu << 16, F32)
    hi = pltpu.bitcast(wu & jnp.uint32(0xFFFF0000), F32)
    return lo, hi


def _ld(ref, *idx):
    return pltpu.bitcast(ref[idx], BF16)


def _pk(x):
    return pltpu.bitcast(x, U32)


class _Jobs:
    def __init__(self):
        self.res = []

    def mm(self, lhs, wt, dot, tie=False):
        acc = None
        for x, w in zip(lhs, wt):
            if tie and len(self.res) >= VT:
                x = _tie(x, self.res[len(self.res) - VT][0:8, :])
            v = dot(x, w)
            self.res.append(v)
            acc = v if acc is None else v + acc
        return acc


def _kv_jobs(jobs, r, ct, wk, wvT, k_scr, v_scr):
    for hd in range(2):
        k_scr[2 * r + hd] = _pk(jobs.mm(ct, wk(hd), _dot).astype(BF16))
    for hd in range(2):
        v_scr[2 * r + hd] = _pk(jobs.mm(wvT(hd), ct, _dot_nt, True).astype(BF16))


def _q_jobs(jobs, r, ht, wq, q_scr, scale):
    for hd in range(2):
        q_scr[2 * r + hd] = _pk((jobs.mm(ht, wq(hd), _dot) * scale).astype(BF16))


def _unpack_tiles(w_ref, transpose=False):
    out = []
    for j in range(w_ref.shape[0] // T):
        pair = [w.astype(BF16) for w in _unpack_pair(w_ref[j * T:(j + 1) * T, :])]
        out.append([w.T for w in pair] if transpose else pair)
    return out


def _proj_step(h_scr, c_ref, wq_ref, wuk_ref, wuv_ref, q_scr, k_scr, v_scr, *, scale):
    wk = _unpack_tiles(wuk_ref)
    wq = _unpack_tiles(wq_ref)
    wvT = _unpack_tiles(wuv_ref, True)
    jobs = _Jobs()
    for r in range(h_scr.shape[0]):
        ct = [c_ref[r * T:(r + 1) * T, j * T:(j + 1) * T] for j in range(len(wk))]
        ht = [h_scr[r, j] for j in range(len(wq))]
        _q_jobs(jobs, r, ht, lambda hd: [t[hd] for t in wq], q_scr, scale)
        _kv_jobs(jobs, r, ct, lambda hd: [t[hd] for t in wk], lambda hd: [t[hd] for t in wvT], k_scr, v_scr)


def _attention_step(q_scr, k_scr, v_scr, wo_ref, acc_scr, cap_ref, mid, *, S, M):
    nb = S // T
    km = M // T
    tile = lambda j: slice(j * T, (j + 1) * T)
    sv = {}; mx = {}; mfin = {}; lsum = {}; o = {}
    part = {}
    res = []

    def accum(key, val):
        res.append(val)
        part[key] = val if key not in part else val + part[key]
        return part[key]

    def job_a(u, cidx):
        r, hd = divmod(u, 2)
        s = _dot_nt(_ld(k_scr, 2 * cidx + hd), _ld(q_scr, u))
        res.append(s)
        if cidx == r:
            s = jnp.minimum(s, cap_ref[...])
        s = s.reshape(T // 8, 8, T)
        sv[(u, cidx)] = s
        pm = jnp.max(s, axis=0)
        mx[u] = pm if u not in mx else jnp.maximum(mx[u], pm)

    def job_b(u, cidx):
        r, hd = divmod(u, 2)
        if u not in mfin:
            mfin[u] = jnp.broadcast_to(jnp.max(mx[u], axis=0, keepdims=True), (8, T))
        s = sv.pop((u, cidx))
        m = mfin[u]
        if LEAD and len(res) >= LEAD:
            r0 = 8 * ((PROW * (cidx % 4)) % 16)
            src = res[len(res) - LEAD][r0:r0 + 8, :]
            m = jnp.where(src > jnp.inf, src, m)
        p = jnp.exp2(s - m[None])
        ls = jnp.sum(p, axis=0)
        lsum[u] = ls if u not in lsum else lsum[u] + ls
        v = accum(('o', u), _dot(_ld(v_scr, 2 * cidx + hd), p.reshape(T, T).astype(BF16)))
        if cidx == r:
            l = jnp.sum(lsum[u], axis=0, keepdims=True)
            o[u] = _tie((v * (1.0 / l)).astype(BF16).T, lsum[u])

    def job_o(u, j):
        r, hd = divmod(u, 2)
        v = _dot(o[u], wo_ref[tile(hd), tile(j)])
        res.append(v)
        acc_scr[tile(r), tile(j)] += v

    fns = dict(a=job_a, b=job_b, o=job_o)
    for n, (kind, u, j) in enumerate(_job_order(nb, km)):
        if n == MID:
            mid()
        fns[kind](u, j)


def _job_order(nb, km):
    nu = 2 * nb
    units = list(range(nu))
    if DESC:
        units = units[::-1]
    QA = [('a', u, c) for u in units for c in range(u // 2 + 1)]
    QB = [('b', u, c) for u in units for c in range(u // 2 + 1)]
    QO = [('o', u, j) for u in units for j in range(km)]
    done = {}
    order = []

    def ready(q, lat, pre):
        return bool(q) and (pre, q[0][1]) in done and done[(pre, q[0][1])] + lat <= len(order)

    def emit(q):
        job = q.pop(0)
        kind, u, j = job
        if kind != 'o' and j == u // 2:
            done[(kind, u)] = len(order)
        order.append(job)

    turn = 0
    while QA or QB or QO:
        pref = ('a', 'b', 'o')[turn % 3]
        turn += 1
        for _ in range(GRP if pref != 'o' else km):
            lead = len(QB) - len(QA)
            if pref == 'a' and QA and (lead < ALEAD or not ready(QB, LAT_A, 'a')):
                emit(QA)
            elif pref == 'b' and ready(QB, LAT_A, 'a'):
                emit(QB)
            elif pref == 'o' and ready(QO, LAT_B, 'b') and (len(QO) > RES * km or not (QA or ready(QB, LAT_A, 'a'))):
                emit(QO)
            elif not QA and not ready(QB, LAT_A, 'a') and not ready(QO, LAT_B, 'b'):
                if QB: emit(QB)
                elif QO: emit(QO)
            else:
                break
    return order


def _kernel(x_hbm, c_hbm, wq_hbm, wuk_hbm, wuv_hbm, wo_hbm, w1_hbm, w2_hbm, w3_hbm, w4_hbm,
            cond_hbm, wmod_hbm, out_hbm,
            h_scr, acc_scr, mod_scr, x1_scr, hb_scr, t_scr, wq_buf, wk_buf, wv_buf, wo_buf, wsem,
            cap_scr,
            x_ref, c_ref, cond_ref, wma_ref, wmb_ref, w1_ref, w2_ref, w3_ref, w4_ref, sem,
            out_buf, osem, a1_scr, q_scr, k_scr, v_scr, w_scr,
            *, S, M, Dc, H, D, RB):
    nattn = H // 2
    scale = float(D) ** -0.5 * math.log2(math.e)
    neg = -1e9 * math.log2(math.e)
    nrb = S // RB
    NX = 4
    XR = S // NX

    km, kc = M // T, Dc // T
    CB = XR // T

    def pcopies(g):
        return [pltpu.make_async_copy(src.bitcast(U32).at[:, g, :], dst, wsem.at[j])
                for j, (src, dst) in enumerate(((wuk_hbm, wk_buf), (wuv_hbm, wv_buf), (wq_hbm, wq_buf)))]

    def ocopy(g, slot):
        return pltpu.make_async_copy(wo_hbm.at[g], wo_buf.at[slot], wsem.at[3])

    def chunk_copy(src, dst, i, s0):
        rows = pl.ds(i * XR if isinstance(i, int) else pl.multiple_of(i * XR, XR), XR)
        return pltpu.make_async_copy(src.at[rows, :], dst.at[rows, :], sem.at[s0 + i])

    cp_cond = pltpu.make_async_copy(cond_hbm, cond_ref, sem.at[0])
    cp_wma = pltpu.make_async_copy(wmod_hbm.at[:, 0:2 * M], wma_ref, sem.at[1])
    cp_late = [pltpu.make_async_copy(src, dst, sem.at[2 + j]) for j, (src, dst) in enumerate((
        (wmod_hbm.at[:, 2 * M:6 * M], wmb_ref), (w1_hbm, w1_ref), (w2_hbm, w2_ref),
        (w3_hbm, w3_ref), (w4_hbm, w4_ref)))]
    cp_x = lambda i: chunk_copy(x_hbm, x_ref, i, 7)
    cp_c = lambda i: chunk_copy(c_hbm, c_ref, i, 7 + NX)

    def silu_cond():
        cf = cond_ref[...].astype(F32)
        return jnp.broadcast_to((cf * jax.nn.sigmoid(cf)).astype(BF16), (8, M))

    cp_wk, cp_wv, cp_wq = pcopies(0)
    named = dict(k=cp_wk, v=cp_wv, q=cp_wq, o=ocopy(0, 0), n=cp_cond, m=cp_wma)
    named.update({'abcd'[i]: cp_c(i) for i in range(NX)})
    named.update({'wxyz'[i]: cp_x(i) for i in range(NX)})
    plan = os.environ.get('PLAN', 'kva,b,cdn,m,qw,x,yzo').split(',')

    def kick():
        if plan:
            for ch in plan.pop(0):
                named.pop(ch).start()

    kick()

    def zero(r, carry):
        acc_scr[pl.ds(pl.multiple_of(r * T, T), T), :] = jnp.zeros((T, M), F32)
        return carry

    jax.lax.fori_loop(0, S // T, zero, 0)
    kick()
    cap_scr[...] = jnp.where(jax.lax.broadcasted_iota(jnp.int32, (T, T), 0)
                             <= jax.lax.broadcasted_iota(jnp.int32, (T, T), 1), jnp.inf, neg)
    acc_scr[S:S + 16, :] = jnp.zeros((16, M), F32)
    x_ref[S:S + 16, :] = jnp.zeros((16, M), BF16)
    nb = S // T
    tile = lambda j: slice(j * T, (j + 1) * T)
    hist = []

    def kv_tile(jobs, r, wk, wvT):
        _kv_jobs(jobs, r, [c_ref[tile(r), tile(j)] for j in range(kc)], wk, wvT, k_scr, v_scr)

    def q_tile(jobs, r, wq):
        _q_jobs(jobs, r, [h_scr[r, j] for j in range(km)], wq, q_scr, scale)

    def ln_tile(r):
        sa = _rows(mod_scr[:, 0:M], LP)
        ca1 = _rows(mod_scr[:, M:2 * M], LP)
        for i in range(T // LP):
            xf = x_ref[r * T + i * LP:r * T + (i + 1) * LP, :].astype(F32)
            if LL and len(hist) >= LL:
                dep = _rows(hist[-LL], LP)
                xf = jnp.concatenate([jnp.where(dep > jnp.inf, dep, xf[:, :T]), xf[:, T:]], axis=1)
            hf = _ln(xf) * ca1 + sa
            hist.append(jnp.max(hf[:, M - T:].reshape(LP // 8, 8, T), axis=0))
            hh = hf.astype(BF16)
            for j in range(km):
                h_scr[r, j, i * LP:(i + 1) * LP, :] = hh[:, tile(j)]

    def stash(tiles, j0):
        for j, pair in enumerate(tiles):
            for hd in range(2):
                w_scr[hd, j0 + j] = _pk(pair[hd])
        return lambda hd: [_ld(w_scr, hd, j0 + j) for j in range(len(tiles))]

    cp_wk.wait()
    cp_wv.wait()
    cp_c(0).wait()
    kick()
    wk = stash(_unpack_tiles(wk_buf), 0)
    wvT = stash(_unpack_tiles(wv_buf, True), kc)
    jobs = _Jobs()
    for r in range(CB):
        kv_tile(jobs, r, wk, wvT)
    for grp in os.environ.get('CG', '1,23').split(','):
        for ch in grp:
            cp_c(int(ch)).wait()
        kick()
        jobs = _Jobs()
        for r in range(int(grp[0]) * CB, min((int(grp[-1]) + 1) * CB, nb - KVL - KVM)):
            kv_tile(jobs, r, wk, wvT)
    cp_cond.wait()
    cp_wma.wait()
    kick()
    mod = _dot(silu_cond(), wma_ref[...])
    mod_scr[:, 0:M] = mod[:, 0:M]
    mod_scr[:, M:2 * M] = 1.0 + mod[:, M:2 * M]
    jobs = _Jobs()
    for r in range(nb - KVL - KVM, nb - KVL):
        kv_tile(jobs, r, wk, wvT)
    cp_wq.wait()
    wq = None
    qdone = 0
    for grp in os.environ.get('XG', '0,1,23').split(','):
        chunks = [int(ch) for ch in grp]
        for i in chunks:
            cp_x(i).wait()
        kick()
        jobs = _Jobs()
        del hist[:]
        if chunks[0] == 0:
            wq = stash(_unpack_tiles(wq_buf), 2 * kc)
            for r in range(nb - KVL, nb):
                kv_tile(jobs, r, wk, wvT)
        for r in range(chunks[0] * CB, (chunks[-1] + 1) * CB):
            ln_tile(r)
        qend = nb if chunks[-1] == NX - 1 else (chunks[-1] + 1) * CB - QLAG
        for r in range(qdone, qend):
            q_tile(jobs, r, wq)
        qdone = max(qdone, qend)
    assert not named
    ocopy(0, 0).wait()
    for cp in cp_late:
        cp.start()

    def attn_body(g, carry):
        slot = g & 1
        nxt = jnp.minimum(g + 1, nattn - 1)

        def mid():
            for cp in pcopies(nxt) + [ocopy(nxt, 1 - slot)]:
                cp.start()

        _attention_step(q_scr, k_scr, v_scr, wo_buf.at[slot], acc_scr, cap_scr, mid, S=S, M=M)
        for cp in pcopies(nxt) + [ocopy(nxt, 1 - slot)]:
            cp.wait()

        @pl.when(g + 1 < nattn)
        def _():
            _proj_step(h_scr, c_ref, wq_buf, wk_buf, wv_buf, q_scr, k_scr, v_scr, scale=scale)

        return carry

    jax.lax.fori_loop(0, nattn, attn_body, 0)

    for cp in cp_late:
        cp.wait()
    mod = _dot(silu_cond(), wmb_ref[...])
    mod_scr[:, 2 * M:4 * M] = mod[:, 0:2 * M]
    mod_scr[:, 4 * M:5 * M] = 1.0 + mod[:, 2 * M:3 * M]
    mod_scr[:, 5 * M:6 * M] = mod[:, 3 * M:4 * M]
    Fd = w4_ref.shape[0]
    ftiles = [(f, min(f + T, Fd)) for f in range(0, Fd, T)]
    OFF = 16
    CAR = 32

    def p1(r0, n, dep=None):
        ga = mod_scr[:, 2 * M:3 * M]
        if dep is not None:
            ga = jnp.concatenate([jnp.where(dep > jnp.inf, dep, ga[:, 0:T]), ga[:, T:]], axis=1)
        rows = pl.ds(r0, n)
        x1 = x_ref[rows, :].astype(F32) + _rows(ga, n) * acc_scr[rows, :]
        x1_scr[rows, :] = x1
        hb = _ln(x1) * _rows(mod_scr[:, 4 * M:5 * M], n) + _rows(mod_scr[:, 3 * M:4 * M], n)
        hb_scr[rows, :] = hb
        return _ln(hb)

    def p1_store(r0, c, dep=None):
        a1f = p1(r0 + c * PC, PC, dep)
        a1 = a1f.astype(BF16)
        for j in range(km):
            a1_scr[j, c * PC:(c + 1) * PC, :] = a1[:, tile(j)]
        return jnp.max(a1f[:, M - T:].reshape(PC // 8, 8, T), axis=0)

    t_scr[RB:RB + CAR - OFF, :] = jnp.zeros((CAR - OFF, M), F32)
    t_scr[RB + CAR - OFF:RB + CAR, :] = _gelu(_dot(p1(0, OFF).astype(BF16), w1_ref[...]))
    for c in range(RB // PC):
        p1_store(OFF, c)

    def out_copy(i):
        rows = pl.ds(i * T if isinstance(i, int) else pl.multiple_of(i * T, T), T)
        return pltpu.make_async_copy(out_buf.at[rows, :], out_hbm.at[rows, :], osem.at[i])

    def b_body(r, carry):
        gb = _rows(mod_scr[:, 5 * M:6 * M], T)
        r0 = pl.multiple_of(r * RB, RB)
        n0 = pl.multiple_of(jnp.minimum(r0 + RB, S - RB) + OFF, OFF)
        nh = RB // T
        res = []

        def mm(lhs, wt, dot):
            acc = None
            for x, w in zip(lhs, wt):
                if len(res) in due:
                    w = _tie(w, due.pop(len(res)))
                v = dot(x, w)
                res.append(v)
                acc = v if acc is None else v + acc
                if len(res) in pace:
                    d = p1_store(n0, pace[len(res)], v[0:8, :T])
                    if PD:
                        due[len(res) + PD] = d
            return acc

        npc = RB // PC
        due = {}
        pace = {P0 + i * PSTEP: i for i in range(npc)}
        t_scr[0:CAR, :] = t_scr[RB:RB + CAR, :]
        for hf in range(nh):
            lhs = [a1_scr[j, tile(hf), :] for j in range(km)]
            for n in range(km):
                t = _gelu(mm(lhs, [w1_ref[tile(j), tile(n)] for j in range(km)], _dot))
                if hf == nh - 1:
                    t = jnp.concatenate([t[:T - OFF], jnp.where(r < nrb - 1, t[T - OFF:], 0.0)], axis=0)
                t_scr[CAR + hf * T:CAR + (hf + 1) * T, tile(n)] = t
        cq = M // 4
        shifts = (-1, 1, -2, 2)
        lane = jax.lax.broadcasted_iota(jnp.int32, (T, T), 1)
        a3 = []
        z = []
        for hf in range(nh):
            base = CAR - OFF + hf * T
            lhs = []
            for j in range(km):
                g_lo, g_hi = (j * T) // cq, ((j + 1) * T - 1) // cq
                v = t_scr[base + shifts[g_lo]:base + shifts[g_lo] + T, tile(j)]
                if g_hi != g_lo:
                    v2 = t_scr[base + shifts[g_hi]:base + shifts[g_hi] + T, tile(j)]
                    v = jnp.where(lane < g_hi * cq - j * T, v, v2)
                lhs.append(v.astype(BF16))
            rows = pl.ds(pl.multiple_of(r0 + hf * T, T), T)
            y1 = jnp.concatenate(
                [mm(lhs, [w2_ref[tile(j), tile(n)] for j in range(km)], _dot) for n in range(km)], axis=1)
            y1 = y1 + hb_scr[rows, :]
            z.append(y1)
            a3.append(_ln(y1).astype(BF16))
        h3 = []
        for hf in range(nh):
            lhs = [a3[hf][:, tile(j)] for j in range(km)]
            row = []
            narrow = None
            for i, (f0, f1) in enumerate(ftiles):
                if f1 - f0 == T:
                    wt = [w3_ref[f0:f1, tile(j)] for j in range(km)]
                    row.append(_gelu(mm(lhs, wt, _dot_nt)).astype(BF16))
                    j, rem = divmod(i - NW0, NWS)
                    if Fd % T and rem == 0 and 0 <= j < km:
                        v = mm([w3_ref[ftiles[-1][0]:Fd, tile(j)]], [lhs[j]], _dot_nt)
                        narrow = v if narrow is None else v + narrow
                else:
                    gT = jnp.concatenate([_gelu(narrow), jnp.zeros((T - (f1 - f0), T), F32)], axis=0)
                    row.append(_tie(gT.astype(BF16).T, gT[0:8, :])[:, :f1 - f0])
            h3.append(row)
        for hf in range(nh):
            rows = pl.ds(pl.multiple_of(r0 + hf * T, T), T)
            for n in range(km):
                v = mm(h3[hf], [w4_ref[f0:f1, tile(n)] for f0, f1 in ftiles], _dot)
                out_buf[rows, tile(n)] = (x1_scr[rows, tile(n)] + gb[:, tile(n)] * (v + z[hf][:, tile(n)])
                                          ).astype(out_buf.dtype)
            out_copy(r * nh + hf).start()
        return carry

    jax.lax.fori_loop(0, nrb, b_body, 0, unroll=BUNR)
    for i in range(nb):
        out_copy(i).wait()


@jax.jit
def pallas_adaLN_cond__compressed_kv_cla__mixer_s_mlp__prompt_kernel(
    A_x: jax.Array,
    A_c_kv: jax.Array,
    A_w_q: jax.Array,
    A_w_uk: jax.Array,
    A_w_uv: jax.Array,
    A_w_o: jax.Array,
    B_x: jax.Array,
    B_w1: jax.Array,
    B_w2: jax.Array,
    B_w3: jax.Array,
    B_w4: jax.Array,
    c: jax.Array,
    w_mod: jax.Array,
):
    _, S, M = A_x.shape
    Dc = A_c_kv.shape[2]
    H, D = A_w_q.shape[1], A_w_q.shape[2]
    Fd = B_w3.shape[1]
    RB = int(os.environ.get('RB', 256))
    nrb = S // RB
    out = pl.pallas_call(
        functools.partial(_kernel, S=S, M=M, Dc=Dc, H=H, D=D, RB=RB),
        in_specs=[pl.BlockSpec(memory_space=pltpu.HBM)] * 12,
        out_specs=pl.BlockSpec(memory_space=pltpu.HBM),
        out_shape=jax.ShapeDtypeStruct((S, M), A_x.dtype),
        scratch_shapes=[
            pltpu.VMEM((S // T, M // T, T, T), BF16),
            pltpu.VMEM((S + 16, M), F32),
            pltpu.VMEM((8, 6 * M), F32),
            pltpu.VMEM((S + 16, M), F32),
            pltpu.VMEM((S + 16, M), F32),
            pltpu.VMEM((RB + 32, M), F32),
            pltpu.VMEM((M, D), U32),
            pltpu.VMEM((Dc, D), U32),
            pltpu.VMEM((Dc, D), U32),
            pltpu.VMEM((2, 2 * D, M), BF16),
            pltpu.SemaphoreType.DMA((4,)),
            pltpu.VMEM((T, T), F32),
            pltpu.VMEM((S + 16, M), BF16),
            pltpu.VMEM((S, Dc), BF16),
            pltpu.VMEM((1, M), BF16),
            pltpu.VMEM((M, 2 * M), BF16),
            pltpu.VMEM((M, 4 * M), BF16),
            pltpu.VMEM((M, M), BF16),
            pltpu.VMEM((M, M), BF16),
            pltpu.VMEM((Fd, M), BF16),
            pltpu.VMEM((Fd, M), BF16),
            pltpu.SemaphoreType.DMA((15,)),
            pltpu.VMEM((S, M), A_x.dtype),
            pltpu.SemaphoreType.DMA((S // T,)),
            pltpu.VMEM((M // T, RB, T), BF16),
            pltpu.VMEM((2 * S // T, T // 2, T), U32),
            pltpu.VMEM((2 * S // T, T // 2, T), U32),
            pltpu.VMEM((2 * S // T, T // 2, T), U32),
            pltpu.VMEM((2, M // T + 2 * (Dc // T), T // 2, T), U32),
        ],
        compiler_params=pltpu.CompilerParams(
            vmem_limit_bytes=100 * 1024 * 1024,
            disable_bounds_checks=bool(int(os.environ.get('NOBC', 1))),
        ),
    )(
        A_x.reshape(S, M), A_c_kv.reshape(S, Dc),
        A_w_q, A_w_uk, A_w_uv,
        A_w_o.reshape(H // 2, 2 * D, M),
        B_w1, B_w2, B_w3.T, B_w4, c, w_mod,
    )
    return out.reshape(1, S, M)
```

```python
import math

import jax
import jax.numpy as jnp
import jax.experimental.pallas as pl
import jax.experimental.pallas.tpu as pltpu

F32 = jnp.float32
BF16 = jnp.bfloat16
U32 = jnp.uint32
NT = (((1,), (1,)), ((), ()))
T = 128
EPS = 1e-5
LOG2E = math.log2(math.e)

GRP = 4
LEAD = 10
PROW = 3
VT = 8
RES = 5
LAT_A = 16
LAT_B = 14
ALEAD = 32
MID = 40
RB = 256
PC = 32
P0, PSTEP, PD = 180, 21, 24
NW0 = 5
LP = 32
KVM, KVL, QLAG = 2, 1, 2
PLAN = 'kva,b,cdn,m,qw,x,yzo'


def _dot(a, b):
    return jnp.dot(a, b, preferred_element_type=F32)


def _dot_nt(a, b):
    return jax.lax.dot_general(a, b, NT, preferred_element_type=F32)


def _ln(x):
    m = jnp.mean(x, axis=-1, keepdims=True)
    xc = x - m
    v = jnp.mean(xc * xc, axis=-1, keepdims=True)
    return xc * jnp.exp2(jnp.log(v + EPS) * (-0.5 * LOG2E))


def _rows(v, n):
    return jnp.broadcast_to(v[None], (n // 8, 8, v.shape[1])).reshape(n, v.shape[1])


def _gelu(x):
    c0 = math.sqrt(2.0 / math.pi)
    return 0.5 * x * (1.0 + jnp.tanh(c0 * (x + 0.044715 * (x * x * x))))


def _after(x, dep):
    return jnp.where(dep > jnp.inf, dep, x)


def _tie(x, dep):
    xu = pltpu.bitcast(x, U32)
    first = jnp.where(dep > jnp.inf, jnp.uint32(0), xu[:8])
    return pltpu.bitcast(jnp.concatenate([first, xu[8:]], axis=0), BF16)


def _tile(j):
    return slice(j * T, (j + 1) * T)


def _ld(ref, *idx):
    return pltpu.bitcast(ref[idx], BF16)


def _pk(x):
    return pltpu.bitcast(x, U32)


def _unpack_tiles(w_ref, transpose=False):
    out = []
    for j in range(w_ref.shape[0] // T):
        wu = w_ref[_tile(j), :]
        pair = [pltpu.bitcast(wu << 16, F32).astype(BF16),
                pltpu.bitcast(wu & jnp.uint32(0xFFFF0000), F32).astype(BF16)]
        out.append([w.T for w in pair] if transpose else pair)
    return out


class _Jobs:
    def __init__(self):
        self.res = []

    def mm(self, lhs, wt, dot, tie=False):
        acc = None
        for x, w in zip(lhs, wt):
            if tie and len(self.res) >= VT:
                x = _tie(x, self.res[len(self.res) - VT][0:8, :])
            v = dot(x, w)
            self.res.append(v)
            acc = v if acc is None else v + acc
        return acc


def _kv_jobs(jobs, r, c_ref, wk, wvT, k_scr, v_scr):
    ct = [c_ref[_tile(r), _tile(j)] for j in range(c_ref.shape[1] // T)]
    for hd in range(2):
        k_scr[2 * r + hd] = _pk(jobs.mm(ct, wk(hd), _dot).astype(BF16))
    for hd in range(2):
        v_scr[2 * r + hd] = _pk(jobs.mm(wvT(hd), ct, _dot_nt, True).astype(BF16))


def _q_jobs(jobs, r, h_scr, wq, q_scr, scale):
    ht = [h_scr[r, j] for j in range(h_scr.shape[1])]
    for hd in range(2):
        q_scr[2 * r + hd] = _pk((jobs.mm(ht, wq(hd), _dot) * scale).astype(BF16))


def _proj_step(h_scr, c_ref, wq_ref, wuk_ref, wuv_ref, q_scr, k_scr, v_scr, scale):
    wk = _unpack_tiles(wuk_ref)
    wq = _unpack_tiles(wq_ref)
    wvT = _unpack_tiles(wuv_ref, True)
    head = lambda tiles: (lambda hd: [t[hd] for t in tiles])
    jobs = _Jobs()
    for r in range(h_scr.shape[0]):
        _q_jobs(jobs, r, h_scr, head(wq), q_scr, scale)
        _kv_jobs(jobs, r, c_ref, head(wk), head(wvT), k_scr, v_scr)


def _job_order(nb, km):
    units = range(2 * nb)
    qa = [('a', u, c) for u in units for c in range(u // 2 + 1)]
    qb = [('b', u, c) for u in units for c in range(u // 2 + 1)]
    qo = [('o', u, j) for u in units for j in range(km)]
    done = {}
    order = []

    def ready(q, lat, pre):
        return bool(q) and (pre, q[0][1]) in done and done[(pre, q[0][1])] + lat <= len(order)

    def emit(q):
        kind, u, j = job = q.pop(0)
        if kind != 'o' and j == u // 2:
            done[(kind, u)] = len(order)
        order.append(job)

    turn = 0
    while qa or qb or qo:
        pref = 'abo'[turn % 3]
        turn += 1
        for _ in range(km if pref == 'o' else GRP):
            b_ok, o_ok = ready(qb, LAT_A, 'a'), ready(qo, LAT_B, 'b')
            if pref == 'a' and qa and (len(qb) - len(qa) < ALEAD or not b_ok):
                emit(qa)
            elif pref == 'b' and b_ok:
                emit(qb)
            elif pref == 'o' and o_ok and (len(qo) > RES * km or not (qa or b_ok)):
                emit(qo)
            elif not (qa or b_ok or o_ok) and (qb or qo):
                emit(qb or qo)
            else:
                break
    return order


def _attention_step(q_scr, k_scr, v_scr, wo_ref, acc_scr, mid):
    causal = (jax.lax.broadcasted_iota(jnp.int32, (T, T), 0)
              <= jax.lax.broadcasted_iota(jnp.int32, (T, T), 1))
    sv, mx, mfin, lsum, pv, o = {}, {}, {}, {}, {}, {}
    res = []

    def job_a(u, c):
        r, hd = divmod(u, 2)
        s = _dot_nt(_ld(k_scr, 2 * c + hd), _ld(q_scr, u))
        res.append(s)
        if c == r:
            s = jnp.where(causal, s, -1e9 * LOG2E)
        s = s.reshape(T // 8, 8, T)
        sv[(u, c)] = s
        pm = jnp.max(s, axis=0)
        mx[u] = pm if u not in mx else jnp.maximum(mx[u], pm)

    def job_b(u, c):
        r, hd = divmod(u, 2)
        if u not in mfin:
            mfin[u] = jnp.broadcast_to(jnp.max(mx[u], axis=0, keepdims=True), (8, T))
        m = mfin[u]
        if len(res) >= LEAD:
            r0 = 8 * PROW * (c % 4)
            m = _after(m, res[len(res) - LEAD][r0:r0 + 8, :])
        p = jnp.exp2(sv.pop((u, c)) - m[None])
        ls = jnp.sum(p, axis=0)
        lsum[u] = ls if u not in lsum else lsum[u] + ls
        v = _dot(_ld(v_scr, 2 * c + hd), p.reshape(T, T).astype(BF16))
        res.append(v)
        pv[u] = v if u not in pv else v + pv[u]
        if c == r:
            l = jnp.sum(lsum[u], axis=0, keepdims=True)
            o[u] = _tie((pv[u] * (1.0 / l)).astype(BF16).T, lsum[u])

    def job_o(u, j):
        r, hd = divmod(u, 2)
        v = _dot(o[u], wo_ref[_tile(hd), _tile(j)])
        res.append(v)
        acc_scr[_tile(r), _tile(j)] += v

    fns = dict(a=job_a, b=job_b, o=job_o)
    for n, (kind, u, j) in enumerate(_job_order(q_scr.shape[0] // 2, wo_ref.shape[1] // T)):
        if n == MID:
            mid()
        fns[kind](u, j)


def _kernel(x_hbm, c_hbm, wq_hbm, wuk_hbm, wuv_hbm, wo_hbm, w1_hbm, w2_hbm, w3_hbm, w4_hbm,
            cond_hbm, wmod_hbm, out_hbm,
            x_ref, c_ref, cond_ref, wma_ref, wmb_ref, w1_ref, w2_ref, w3_ref, w4_ref,
            wq_buf, wk_buf, wv_buf, wo_buf, out_buf, sem, wsem, osem,
            mod_scr, h_scr, w_scr, q_scr, k_scr, v_scr, acc_scr, x1_scr, hb_scr, a1_scr, t_scr):
    S, M = x_hbm.shape
    D = wq_hbm.shape[2]
    nattn = wo_hbm.shape[0]
    Fd = w4_hbm.shape[0]
    scale = float(D) ** -0.5 * LOG2E
    nb, nrb = S // T, S // RB
    km, kc = M // T, c_hbm.shape[1] // T
    NX = 4
    XR = S // NX
    CB = XR // T

    def pcopies(g):
        return [pltpu.make_async_copy(src.bitcast(U32).at[:, g, :], dst, wsem.at[j])
                for j, (src, dst) in enumerate(((wuk_hbm, wk_buf), (wuv_hbm, wv_buf), (wq_hbm, wq_buf)))]

    def ocopy(g, slot):
        return pltpu.make_async_copy(wo_hbm.at[g], wo_buf.at[slot], wsem.at[3])

    def chunk_copy(src, dst, i, s0):
        rows = slice(i * XR, (i + 1) * XR)
        return pltpu.make_async_copy(src.at[rows, :], dst.at[rows, :], sem.at[s0 + i])

    cp_cond = pltpu.make_async_copy(cond_hbm, cond_ref, sem.at[0])
    cp_wma = pltpu.make_async_copy(wmod_hbm.at[:, 0:2 * M], wma_ref, sem.at[1])
    cp_late = [pltpu.make_async_copy(src, dst, sem.at[2 + j]) for j, (src, dst) in enumerate((
        (wmod_hbm.at[:, 2 * M:6 * M], wmb_ref), (w1_hbm, w1_ref), (w2_hbm, w2_ref),
        (w3_hbm, w3_ref), (w4_hbm, w4_ref)))]
    cp_x = [chunk_copy(x_hbm, x_ref, i, 7) for i in range(NX)]
    cp_c = [chunk_copy(c_hbm, c_ref, i, 7 + NX) for i in range(NX)]

    def silu_cond():
        cf = cond_ref[...].astype(F32)
        return jnp.broadcast_to((cf * jax.nn.sigmoid(cf)).astype(BF16), (8, M))

    cp_wk, cp_wv, cp_wq = pcopies(0)
    named = dict(k=cp_wk, v=cp_wv, q=cp_wq, o=ocopy(0, 0), n=cp_cond, m=cp_wma)
    named.update(zip('abcd', cp_c))
    named.update(zip('wxyz', cp_x))
    plan = PLAN.split(',')

    def kick():
        for ch in plan.pop(0) if plan else '':
            named.pop(ch).start()

    def zero(r, carry):
        acc_scr[pl.ds(pl.multiple_of(r * T, T), T), :] = jnp.zeros((T, M), F32)
        return carry

    def ln_tile(r):
        sa = _rows(mod_scr[:, 0:M], LP)
        ca1 = _rows(mod_scr[:, M:2 * M], LP)
        for i in range(T // LP):
            xf = x_ref[r * T + i * LP:r * T + (i + 1) * LP, :].astype(F32)
            hh = (_ln(xf) * ca1 + sa).astype(BF16)
            for j in range(km):
                h_scr[r, j, i * LP:(i + 1) * LP, :] = hh[:, _tile(j)]

    def stash(tiles, j0):
        for j, pair in enumerate(tiles):
            for hd in range(2):
                w_scr[hd, j0 + j] = _pk(pair[hd])
        return lambda hd: [_ld(w_scr, hd, j0 + j) for j in range(len(tiles))]

    def kv_tiles(jobs, r0, r1):
        for r in range(r0, r1):
            _kv_jobs(jobs, r, c_ref, wk, wvT, k_scr, v_scr)

    kick()
    jax.lax.fori_loop(0, nb, zero, 0)
    kick()
    acc_scr[S:, :] = jnp.zeros((acc_scr.shape[0] - S, M), F32)
    x_ref[S:, :] = jnp.zeros((x_ref.shape[0] - S, M), BF16)
    cp_wk.wait()
    cp_wv.wait()
    cp_c[0].wait()
    kick()
    wk = stash(_unpack_tiles(wk_buf), 0)
    wvT = stash(_unpack_tiles(wv_buf, True), kc)
    kv_tiles(_Jobs(), 0, CB)
    for chunks in ((1,), (2, 3)):
        for i in chunks:
            cp_c[i].wait()
        kick()
        kv_tiles(_Jobs(), chunks[0] * CB, min((chunks[-1] + 1) * CB, nb - KVL - KVM))
    cp_cond.wait()
    cp_wma.wait()
    kick()
    mod = _dot(silu_cond(), wma_ref[...])
    mod_scr[:, 0:M] = mod[:, 0:M]
    mod_scr[:, M:2 * M] = 1.0 + mod[:, M:2 * M]
    kv_tiles(_Jobs(), nb - KVL - KVM, nb - KVL)
    cp_wq.wait()
    qdone = 0
    for chunks in ((0,), (1,), (2, 3)):
        for i in chunks:
            cp_x[i].wait()
        kick()
        jobs = _Jobs()
        if chunks[0] == 0:
            wq = stash(_unpack_tiles(wq_buf), 2 * kc)
            kv_tiles(jobs, nb - KVL, nb)
        for r in range(chunks[0] * CB, (chunks[-1] + 1) * CB):
            ln_tile(r)
        qend = nb if chunks[-1] == NX - 1 else (chunks[-1] + 1) * CB - QLAG
        for r in range(qdone, qend):
            _q_jobs(jobs, r, h_scr, wq, q_scr, scale)
        qdone = max(qdone, qend)
    assert not named
    ocopy(0, 0).wait()
    for cp in cp_late:
        cp.start()

    def attn_body(g, carry):
        slot = g & 1
        nxt = jnp.minimum(g + 1, nattn - 1)
        copies = pcopies(nxt) + [ocopy(nxt, 1 - slot)]

        def mid():
            for cp in copies:
                cp.start()

        _attention_step(q_scr, k_scr, v_scr, wo_buf.at[slot], acc_scr, mid)
        for cp in copies:
            cp.wait()

        @pl.when(g + 1 < nattn)
        def _():
            _proj_step(h_scr, c_ref, wq_buf, wk_buf, wv_buf, q_scr, k_scr, v_scr, scale)

        return carry

    jax.lax.fori_loop(0, nattn, attn_body, 0)

    for cp in cp_late:
        cp.wait()
    mod = _dot(silu_cond(), wmb_ref[...])
    mod_scr[:, 2 * M:4 * M] = mod[:, 0:2 * M]
    mod_scr[:, 4 * M:5 * M] = 1.0 + mod[:, 2 * M:3 * M]
    mod_scr[:, 5 * M:6 * M] = mod[:, 3 * M:4 * M]
    ftiles = [(f, min(f + T, Fd)) for f in range(0, Fd, T)]
    OFF = x_ref.shape[0] - S
    CAR = t_scr.shape[0] - RB

    def p1(r0, n, dep=None):
        ga = mod_scr[:, 2 * M:3 * M]
        if dep is not None:
            ga = jnp.concatenate([_after(ga[:, 0:T], dep), ga[:, T:]], axis=1)
        rows = pl.ds(r0, n)
        x1 = x_ref[rows, :].astype(F32) + _rows(ga, n) * acc_scr[rows, :]
        x1_scr[rows, :] = x1
        hb = _ln(x1) * _rows(mod_scr[:, 4 * M:5 * M], n) + _rows(mod_scr[:, 3 * M:4 * M], n)
        hb_scr[rows, :] = hb
        return _ln(hb)

    def p1_store(r0, c, dep=None):
        a1f = p1(r0 + c * PC, PC, dep)
        a1 = a1f.astype(BF16)
        for j in range(km):
            a1_scr[j, c * PC:(c + 1) * PC, :] = a1[:, _tile(j)]
        return jnp.max(a1f[:, M - T:].reshape(PC // 8, 8, T), axis=0)

    t_scr[RB:RB + CAR - OFF, :] = jnp.zeros((CAR - OFF, M), F32)
    t_scr[RB + CAR - OFF:RB + CAR, :] = _gelu(_dot(p1(0, OFF).astype(BF16), w1_ref[...]))
    for c in range(RB // PC):
        p1_store(OFF, c)

    def out_copy(i):
        rows = pl.ds(i * T if isinstance(i, int) else pl.multiple_of(i * T, T), T)
        return pltpu.make_async_copy(out_buf.at[rows, :], out_hbm.at[rows, :], osem.at[i])

    def b_body(r, carry):
        gb = _rows(mod_scr[:, 5 * M:6 * M], T)
        r0 = pl.multiple_of(r * RB, RB)
        n0 = pl.multiple_of(jnp.minimum(r0 + RB, S - RB) + OFF, OFF)
        nh = RB // T
        res = []
        due = {}
        pace = {P0 + i * PSTEP: i for i in range(RB // PC)}

        def mm(lhs, wt, dot):
            acc = None
            for x, w in zip(lhs, wt):
                if len(res) in due:
                    w = _tie(w, due.pop(len(res)))
                v = dot(x, w)
                res.append(v)
                acc = v if acc is None else v + acc
                if len(res) in pace:
                    due[len(res) + PD] = p1_store(n0, pace.pop(len(res)), v[0:8, :])
            return acc

        t_scr[0:CAR, :] = t_scr[RB:RB + CAR, :]
        for hf in range(nh):
            lhs = [a1_scr[j, _tile(hf), :] for j in range(km)]
            for n in range(km):
                t = _gelu(mm(lhs, [w1_ref[_tile(j), _tile(n)] for j in range(km)], _dot))
                if hf == nh - 1:
                    t = jnp.concatenate([t[:T - OFF], jnp.where(r < nrb - 1, t[T - OFF:], 0.0)], axis=0)
                t_scr[CAR + hf * T:CAR + (hf + 1) * T, _tile(n)] = t
        cq = M // 4
        shifts = (-1, 1, -2, 2)
        lane = jax.lax.broadcasted_iota(jnp.int32, (T, T), 1)
        y1, a3 = [], []
        for hf in range(nh):
            base = CAR - OFF + hf * T
            lhs = []
            for j in range(km):
                g_lo, g_hi = (j * T) // cq, ((j + 1) * T - 1) // cq
                assert g_hi - g_lo <= 1
                v = t_scr[base + shifts[g_lo]:base + shifts[g_lo] + T, _tile(j)]
                if g_hi != g_lo:
                    v2 = t_scr[base + shifts[g_hi]:base + shifts[g_hi] + T, _tile(j)]
                    v = jnp.where(lane < g_hi * cq - j * T, v, v2)
                lhs.append(v.astype(BF16))
            hs = jnp.concatenate(
                [mm(lhs, [w2_ref[_tile(j), _tile(n)] for j in range(km)], _dot) for n in range(km)], axis=1)
            y1.append(hs + hb_scr[pl.ds(pl.multiple_of(r0 + hf * T, T), T), :])
            a3.append(_ln(y1[hf]).astype(BF16))
        h3 = []
        for hf in range(nh):
            lhs = [a3[hf][:, _tile(j)] for j in range(km)]
            row = []
            narrow = None
            for i, (f0, f1) in enumerate(ftiles):
                if f1 - f0 == T:
                    wt = [w3_ref[f0:f1, _tile(j)] for j in range(km)]
                    row.append(_gelu(mm(lhs, wt, _dot_nt)).astype(BF16))
                    if Fd % T and 0 <= i - NW0 < km:
                        v = mm([w3_ref[ftiles[-1][0]:Fd, _tile(i - NW0)]], [lhs[i - NW0]], _dot_nt)
                        narrow = v if narrow is None else v + narrow
                else:
                    gT = jnp.concatenate([_gelu(narrow), jnp.zeros((T - (f1 - f0), T), F32)], axis=0)
                    row.append(_tie(gT.astype(BF16).T, gT[0:8, :])[:, :f1 - f0])
            h3.append(row)
        for hf in range(nh):
            rows = pl.ds(pl.multiple_of(r0 + hf * T, T), T)
            for n in range(km):
                v = mm(h3[hf], [w4_ref[f0:f1, _tile(n)] for f0, f1 in ftiles], _dot)
                out_buf[rows, _tile(n)] = (
                    x1_scr[rows, _tile(n)] + gb[:, _tile(n)] * (v + y1[hf][:, _tile(n)])
                ).astype(out_buf.dtype)
            out_copy(r * nh + hf).start()
        assert not pace
        return carry

    jax.lax.fori_loop(0, nrb, b_body, 0)
    for i in range(nb):
        out_copy(i).wait()


@jax.jit
def pallas_adaLN_cond__compressed_kv_cla__mixer_s_mlp__prompt_kernel(
    A_x: jax.Array,
    A_c_kv: jax.Array,
    A_w_q: jax.Array,
    A_w_uk: jax.Array,
    A_w_uv: jax.Array,
    A_w_o: jax.Array,
    B_x: jax.Array,
    B_w1: jax.Array,
    B_w2: jax.Array,
    B_w3: jax.Array,
    B_w4: jax.Array,
    c: jax.Array,
    w_mod: jax.Array,
):
    _, S, M = A_x.shape
    Dc = A_c_kv.shape[2]
    H, D = A_w_q.shape[1], A_w_q.shape[2]
    Fd = B_w3.shape[1]
    assert D == T and A_c_kv.shape[1] == S
    vmem = pltpu.VMEM
    packed = lambda *lead: vmem(lead + (T // 2, T), U32)
    out = pl.pallas_call(
        _kernel,
        in_specs=[pl.BlockSpec(memory_space=pltpu.HBM)] * 12,
        out_specs=pl.BlockSpec(memory_space=pltpu.HBM),
        out_shape=jax.ShapeDtypeStruct((S, M), A_x.dtype),
        scratch_shapes=[
            vmem((S + 16, M), BF16),
            vmem((S, Dc), BF16),
            vmem((1, M), BF16),
            vmem((M, 2 * M), BF16),
            vmem((M, 4 * M), BF16),
            vmem((M, M), BF16),
            vmem((M, M), BF16),
            vmem((Fd, M), BF16),
            vmem((Fd, M), BF16),
            vmem((M, D), U32),
            vmem((Dc, D), U32),
            vmem((Dc, D), U32),
            vmem((2, 2 * D, M), BF16),
            vmem((S, M), A_x.dtype),
            pltpu.SemaphoreType.DMA((15,)),
            pltpu.SemaphoreType.DMA((4,)),
            pltpu.SemaphoreType.DMA((S // T,)),
            vmem((8, 6 * M), F32),
            vmem((S // T, M // T, T, T), BF16),
            packed(2, M // T + 2 * (Dc // T)),
            packed(2 * S // T),
            packed(2 * S // T),
            packed(2 * S // T),
            vmem((S + 16, M), F32),
            vmem((S + 16, M), F32),
            vmem((S + 16, M), F32),
            vmem((M // T, RB, T), BF16),
            vmem((RB + 32, M), F32),
        ],
        compiler_params=pltpu.CompilerParams(
            vmem_limit_bytes=100 * 1024 * 1024,
            disable_bounds_checks=True,
        ),
    )(
        A_x.reshape(S, M), A_c_kv.reshape(S, Dc),
        A_w_q, A_w_uk, A_w_uv,
        A_w_o.reshape(H // 2, 2 * D, M),
        B_w1, B_w2, B_w3.T, B_w4, c, w_mod,
    )
    return out.reshape(1, S, M)
```

```python
import math

import jax
import jax.numpy as jnp
import jax.experimental.pallas as pl
import jax.experimental.pallas.tpu as pltpu

F32 = jnp.float32
BF16 = jnp.bfloat16
U32 = jnp.uint32
NT = (((1,), (1,)), ((), ()))
T = 128
EPS = 1e-5
LOG2E = math.log2(math.e)

GRP = 4
LEAD = 10
PROW = 3
VT = 8
RES = 5
LAT_A = 16
LAT_B = 14
ALEAD = 32
MID = 40
RB = 256
PC = 32
P0, PSTEP, PD = 180, 21, 24
NW0 = 5
LP = 16
KVM, KVL, QLAG = 1, 1, 1
PLAN = 'kva,b,cdn,m,qw,x,yzo'


def _dot(a, b):
    return jnp.dot(a, b, preferred_element_type=F32)


def _dot_nt(a, b):
    return jax.lax.dot_general(a, b, NT, preferred_element_type=F32)


def _ln(x):
    m = jnp.mean(x, axis=-1, keepdims=True)
    xc = x - m
    v = jnp.mean(xc * xc, axis=-1, keepdims=True)
    return xc * jnp.exp2(jnp.log(v + EPS) * (-0.5 * LOG2E))


def _rows(v, n):
    return jnp.broadcast_to(v[None], (n // 8, 8, v.shape[1])).reshape(n, v.shape[1])


def _gelu(x):
    c0 = math.sqrt(2.0 / math.pi)
    return 0.5 * x * (1.0 + jnp.tanh(c0 * (x + 0.044715 * (x * x * x))))


def _after(x, dep):
    return jnp.where(dep > jnp.inf, dep, x)


def _tie(x, dep):
    xu = pltpu.bitcast(x, U32)
    first = jnp.where(dep > jnp.inf, jnp.uint32(0), xu[:8])
    return pltpu.bitcast(jnp.concatenate([first, xu[8:]], axis=0), BF16)


def _tile(j):
    return slice(j * T, (j + 1) * T)


def _ld(ref, *idx):
    return pltpu.bitcast(ref[idx], BF16)


def _pk(x):
    return pltpu.bitcast(x, U32)


def _a_ops(a11, a12, a21, a22):
    return [a11 + a22, a21 + a22, a11, a22, a11 + a12, a21 - a11, a12 - a22]


def _b_ops(b11, b12, b21, b22):
    return [b11 + b22, b11, b12 - b22, b21 - b11, b22, b11 + b12, b21 + b22]


def _strassen(prod):
    m4 = prod(3)
    m2 = prod(1)
    c21 = m2 + m4
    m3 = prod(2)
    m5 = prod(4)
    c12 = m3 + m5
    m1 = prod(0)
    c11 = prod(6) + (m1 + (m4 - m5))
    c22 = prod(5) + (m1 + (m3 - m2))
    return c11, c12, c21, c22


def _pair_weights(w_ref, transpose=False):
    lo, hi = [], []
    for j in range(w_ref.shape[0] // T):
        wu = w_ref[_tile(j), :]
        lo.append(pltpu.bitcast(wu << 16, F32))
        hi.append(pltpu.bitcast(wu & jnp.uint32(0xFFFF0000), F32))
    per_j = [_b_ops(lo[j], hi[j], lo[2 + j], hi[2 + j]) for j in range(2)]
    tiles = [per_j[j][i] for i in range(7) for j in range(2)]
    for j in range(4, len(lo)):
        tiles += [lo[j], hi[j]]
    tiles = [t.astype(BF16) for t in tiles]
    return [t.T for t in tiles] if transpose else tiles


class _Jobs:
    def __init__(self):
        self.res = []

    def mm(self, lhs, wt, dot, tie=False):
        acc = None
        for x, w in zip(lhs, wt):
            if tie and len(self.res) >= VT:
                x = _tie(x, self.res[len(self.res) - VT][0:8, :])
            v = dot(x, w)
            self.res.append(v)
            acc = v if acc is None else v + acc
        return acc


def _kv_jobs(jobs, p, cs_scr, wk, wvT, k_scr, v_scr):
    ct = lambda i: [cs_scr[p, 2 * i + j] for j in range(2)]
    ks = _strassen(lambda i: jobs.mm(ct(i), [wk(2 * i), wk(2 * i + 1)], _dot))
    for n, v in enumerate(ks):
        k_scr[4 * p + n] = _pk(v.astype(BF16))
    vs = _strassen(lambda i: jobs.mm([wvT(2 * i), wvT(2 * i + 1)], ct(i), _dot_nt, True))
    for n, v in enumerate(vs):
        v_scr[4 * p + n] = _pk(v.astype(BF16))


def _q_jobs(jobs, p, h_scr, wq, q_scr, scale):
    rest = [jobs.mm([h_scr[p, 14 + n // 2]], [wq(14 + n % 2)], _dot) for n in range(4)]
    qs = _strassen(lambda i: jobs.mm([h_scr[p, 2 * i + j] for j in range(2)],
                                     [wq(2 * i), wq(2 * i + 1)], _dot))
    for n, v in enumerate(qs):
        q_scr[4 * p + n] = _pk(((v + rest[n]) * scale).astype(BF16))


def _proj_step(h_scr, cs_scr, wq_ref, wuk_ref, wuv_ref, q_scr, k_scr, v_scr, scale):
    wq = _pair_weights(wq_ref)
    wk = _pair_weights(wuk_ref)
    wvT = _pair_weights(wuv_ref, True)
    jobs = _Jobs()
    for p in range(h_scr.shape[0]):
        _q_jobs(jobs, p, h_scr, wq.__getitem__, q_scr, scale)
        _kv_jobs(jobs, p, cs_scr, wk.__getitem__, wvT.__getitem__, k_scr, v_scr)


def _job_order(nb, km):
    units = range(2 * nb)
    qa = [('a', u, c) for u in units for c in range(u // 2 + 1)]
    qb = [('b', u, c) for u in units for c in range(u // 2 + 1)]
    qo = [('o', u, j) for u in units for j in range(km)]
    done = {}
    order = []

    def ready(q, lat, pre):
        return bool(q) and (pre, q[0][1]) in done and done[(pre, q[0][1])] + lat <= len(order)

    def emit(q):
        kind, u, j = job = q.pop(0)
        if kind != 'o' and j == u // 2:
            done[(kind, u)] = len(order)
        order.append(job)

    turn = 0
    while qa or qb or qo:
        pref = 'abo'[turn % 3]
        turn += 1
        for _ in range(km if pref == 'o' else GRP):
            b_ok, o_ok = ready(qb, LAT_A, 'a'), ready(qo, LAT_B, 'b')
            if pref == 'a' and qa and (len(qb) - len(qa) < ALEAD or not b_ok):
                emit(qa)
            elif pref == 'b' and b_ok:
                emit(qb)
            elif pref == 'o' and o_ok and (len(qo) > RES * km or not (qa or b_ok)):
                emit(qo)
            elif not (qa or b_ok or o_ok) and (qb or qo):
                emit(qb or qo)
            else:
                break
    return order


def _attention_step(q_scr, k_scr, v_scr, wo_ref, acc_scr, mid):
    causal = (jax.lax.broadcasted_iota(jnp.int32, (T, T), 0)
              <= jax.lax.broadcasted_iota(jnp.int32, (T, T), 1))
    sv, mx, mfin, lsum, pv, o = {}, {}, {}, {}, {}, {}
    res = []

    def job_a(u, c):
        r, hd = divmod(u, 2)
        s = _dot_nt(_ld(k_scr, 2 * c + hd), _ld(q_scr, u))
        res.append(s)
        if c == r:
            s = jnp.where(causal, s, -1e9 * LOG2E)
        s = s.reshape(T // 8, 8, T)
        sv[(u, c)] = s
        pm = jnp.max(s, axis=0)
        mx[u] = pm if u not in mx else jnp.maximum(mx[u], pm)

    def job_b(u, c):
        r, hd = divmod(u, 2)
        if u not in mfin:
            mfin[u] = jnp.broadcast_to(jnp.max(mx[u], axis=0, keepdims=True), (8, T))
        m = mfin[u]
        if len(res) >= LEAD:
            r0 = 8 * PROW * (c % 4)
            m = _after(m, res[len(res) - LEAD][r0:r0 + 8, :])
        p = jnp.exp2(sv.pop((u, c)) - m[None])
        ls = jnp.sum(p, axis=0)
        lsum[u] = ls if u not in lsum else lsum[u] + ls
        v = _dot(_ld(v_scr, 2 * c + hd), p.reshape(T, T).astype(BF16))
        res.append(v)
        pv[u] = v if u not in pv else v + pv[u]
        if c == r:
            l = jnp.sum(lsum[u], axis=0, keepdims=True)
            o[u] = _tie((pv[u] * (1.0 / l)).astype(BF16).T, lsum[u])

    def job_o(u, j):
        r, hd = divmod(u, 2)
        v = _dot(o[u], wo_ref[_tile(hd), _tile(j)])
        res.append(v)
        acc_scr[_tile(r), _tile(j)] += v

    fns = dict(a=job_a, b=job_b, o=job_o)
    for n, (kind, u, j) in enumerate(_job_order(q_scr.shape[0] // 2, wo_ref.shape[1] // T)):
        if n == MID:
            mid()
        fns[kind](u, j)


def _kernel(x_hbm, c_hbm, wq_hbm, wuk_hbm, wuv_hbm, wo_hbm, w1_hbm, w2_hbm, w3_hbm, w4_hbm,
            cond_hbm, wmod_hbm, out_hbm,
            x_ref, c_ref, cond_ref, wma_ref, wmb_ref, w1_ref, w2_ref, w3_ref, w4_ref,
            wq_buf, wk_buf, wv_buf, wo_buf, out_buf, sem, wsem, osem,
            mod_scr, h_scr, cs_scr, w_scr, q_scr, k_scr, v_scr, acc_scr, x1_scr, hb_scr, a1_scr, t_scr):
    S, M = x_hbm.shape
    D = wq_hbm.shape[2]
    nattn = wo_hbm.shape[0]
    Fd = w4_hbm.shape[0]
    scale = float(D) ** -0.5 * LOG2E
    nb, nrb = S // T, S // RB
    km, kc = M // T, c_hbm.shape[1] // T
    NX = 4
    XR = S // NX
    CB = XR // T

    def pcopies(g):
        return [pltpu.make_async_copy(src.bitcast(U32).at[:, g, :], dst, wsem.at[j])
                for j, (src, dst) in enumerate(((wuk_hbm, wk_buf), (wuv_hbm, wv_buf), (wq_hbm, wq_buf)))]

    def ocopy(g, slot):
        return pltpu.make_async_copy(wo_hbm.at[g], wo_buf.at[slot], wsem.at[3])

    def chunk_copy(src, dst, i, s0):
        rows = slice(i * XR, (i + 1) * XR)
        return pltpu.make_async_copy(src.at[rows, :], dst.at[rows, :], sem.at[s0 + i])

    cp_cond = pltpu.make_async_copy(cond_hbm, cond_ref, sem.at[0])
    cp_wma = pltpu.make_async_copy(wmod_hbm.at[:, 0:2 * M], wma_ref, sem.at[1])
    cp_late = [pltpu.make_async_copy(src, dst, sem.at[2 + j]) for j, (src, dst) in enumerate((
        (wmod_hbm.at[:, 2 * M:6 * M], wmb_ref), (w1_hbm, w1_ref), (w2_hbm, w2_ref),
        (w3_hbm, w3_ref), (w4_hbm, w4_ref)))]
    cp_x = [chunk_copy(x_hbm, x_ref, i, 7) for i in range(NX)]
    cp_c = [chunk_copy(c_hbm, c_ref, i, 7 + NX) for i in range(NX)]

    def silu_cond():
        cf = cond_ref[...].astype(F32)
        return jnp.broadcast_to((cf * jax.nn.sigmoid(cf)).astype(BF16), (8, M))

    cp_wk, cp_wv, cp_wq = pcopies(0)
    named = dict(k=cp_wk, v=cp_wv, q=cp_wq, o=ocopy(0, 0), n=cp_cond, m=cp_wma)
    named.update(zip('abcd', cp_c))
    named.update(zip('wxyz', cp_x))
    plan = PLAN.split(',')

    def kick():
        for ch in plan.pop(0) if plan else '':
            named.pop(ch).start()

    def zero(r, carry):
        acc_scr[pl.ds(pl.multiple_of(r * T, T), T), :] = jnp.zeros((T, M), F32)
        return carry

    def ln_pair(p):
        sa = _rows(mod_scr[:, 0:M], LP)
        ca1 = _rows(mod_scr[:, M:2 * M], LP)
        for i in range(T // LP):
            h1, h2 = [_ln(x_ref[r * T + i * LP:r * T + (i + 1) * LP, :].astype(F32)) * ca1 + sa
                      for r in (2 * p, 2 * p + 1)]
            ops = _a_ops(h1[:, 0:2 * T], h1[:, 2 * T:4 * T], h2[:, 0:2 * T], h2[:, 2 * T:4 * T])
            tiles = [v[:, _tile(j)] for v in ops for j in range(2)] + [h1[:, _tile(4)], h2[:, _tile(4)]]
            for n, v in enumerate(tiles):
                h_scr[p, n, i * LP:(i + 1) * LP, :] = v.astype(BF16)

    def stash(tiles, j0):
        for j, t in enumerate(tiles):
            w_scr[j0 + j] = _pk(t)
        return lambda j: _ld(w_scr, j0 + j)

    def kv_pairs(jobs, p0, p1_):
        for p in range(p0, p1_):
            for j in range(2):
                ops = _a_ops(*[c_ref[_tile(2 * p + n // 2), _tile(2 * (n % 2) + j)].astype(F32)
                               for n in range(4)])
                for i, v in enumerate(ops):
                    cs_scr[p, 2 * i + j] = v.astype(BF16)
            _kv_jobs(jobs, p, cs_scr, wk, wvT, k_scr, v_scr)

    npair, CP = nb // 2, CB // 2
    kick()
    jax.lax.fori_loop(0, nb, zero, 0)
    kick()
    acc_scr[S:, :] = jnp.zeros((acc_scr.shape[0] - S, M), F32)
    x_ref[S:, :] = jnp.zeros((x_ref.shape[0] - S, M), BF16)
    cp_wk.wait()
    cp_wv.wait()
    cp_c[0].wait()
    kick()
    wk = stash(_pair_weights(wk_buf), 0)
    wvT = stash(_pair_weights(wv_buf, True), 14)
    kv_pairs(_Jobs(), 0, CP)
    for chunks in ((1,), (2, 3)):
        for i in chunks:
            cp_c[i].wait()
        kick()
        kv_pairs(_Jobs(), chunks[0] * CP, min((chunks[-1] + 1) * CP, npair - KVL - KVM))
    cp_cond.wait()
    cp_wma.wait()
    kick()
    mod = _dot(silu_cond(), wma_ref[...])
    mod_scr[:, 0:M] = mod[:, 0:M]
    mod_scr[:, M:2 * M] = 1.0 + mod[:, M:2 * M]
    kv_pairs(_Jobs(), npair - KVL - KVM, npair - KVL)
    cp_wq.wait()
    qdone = 0
    for chunks in ((0,), (1,), (2, 3)):
        for i in chunks:
            cp_x[i].wait()
        kick()
        jobs = _Jobs()
        if chunks[0] == 0:
            wq = stash(_pair_weights(wq_buf), 28)
            kv_pairs(jobs, npair - KVL, npair)
        for p in range(chunks[0] * CP, (chunks[-1] + 1) * CP):
            ln_pair(p)
        qend = npair if chunks[-1] == NX - 1 else (chunks[-1] + 1) * CP - QLAG
        for p in range(qdone, qend):
            _q_jobs(jobs, p, h_scr, wq, q_scr, scale)
        qdone = max(qdone, qend)
    assert not named
    ocopy(0, 0).wait()
    for cp in cp_late:
        cp.start()

    def attn_body(g, carry):
        slot = g & 1
        nxt = jnp.minimum(g + 1, nattn - 1)
        copies = pcopies(nxt) + [ocopy(nxt, 1 - slot)]

        def mid():
            for cp in copies:
                cp.start()

        _attention_step(q_scr, k_scr, v_scr, wo_buf.at[slot], acc_scr, mid)
        for cp in copies:
            cp.wait()

        @pl.when(g + 1 < nattn)
        def _():
            _proj_step(h_scr, cs_scr, wq_buf, wk_buf, wv_buf, q_scr, k_scr, v_scr, scale)

        return carry

    jax.lax.fori_loop(0, nattn, attn_body, 0)

    for cp in cp_late:
        cp.wait()
    mod = _dot(silu_cond(), wmb_ref[...])
    mod_scr[:, 2 * M:4 * M] = mod[:, 0:2 * M]
    mod_scr[:, 4 * M:5 * M] = 1.0 + mod[:, 2 * M:3 * M]
    mod_scr[:, 5 * M:6 * M] = mod[:, 3 * M:4 * M]
    ftiles = [(f, min(f + T, Fd)) for f in range(0, Fd, T)]
    OFF = x_ref.shape[0] - S
    CAR = t_scr.shape[0] - RB

    def p1(r0, n, dep=None):
        ga = mod_scr[:, 2 * M:3 * M]
        if dep is not None:
            ga = jnp.concatenate([_after(ga[:, 0:T], dep), ga[:, T:]], axis=1)
        rows = pl.ds(r0, n)
        x1 = x_ref[rows, :].astype(F32) + _rows(ga, n) * acc_scr[rows, :]
        x1_scr[rows, :] = x1
        hb = _ln(x1) * _rows(mod_scr[:, 4 * M:5 * M], n) + _rows(mod_scr[:, 3 * M:4 * M], n)
        hb_scr[rows, :] = hb
        return _ln(hb)

    def p1_store(r0, c, dep=None):
        a1f = p1(r0 + c * PC, PC, dep)
        a1 = a1f.astype(BF16)
        for j in range(km):
            a1_scr[j, c * PC:(c + 1) * PC, :] = a1[:, _tile(j)]
        return jnp.max(a1f[:, M - T:].reshape(PC // 8, 8, T), axis=0)

    t_scr[RB:RB + CAR - OFF, :] = jnp.zeros((CAR - OFF, M), F32)
    t_scr[RB + CAR - OFF:RB + CAR, :] = _gelu(_dot(p1(0, OFF).astype(BF16), w1_ref[...]))
    for c in range(RB // PC):
        p1_store(OFF, c)

    def out_copy(i):
        rows = pl.ds(i * T if isinstance(i, int) else pl.multiple_of(i * T, T), T)
        return pltpu.make_async_copy(out_buf.at[rows, :], out_hbm.at[rows, :], osem.at[i])

    def b_body(r, carry):
        gb = _rows(mod_scr[:, 5 * M:6 * M], T)
        r0 = pl.multiple_of(r * RB, RB)
        n0 = pl.multiple_of(jnp.minimum(r0 + RB, S - RB) + OFF, OFF)
        nh = RB // T
        res = []
        due = {}
        pace = {P0 + i * PSTEP: i for i in range(RB // PC)}

        def mm(lhs, wt, dot):
            acc = None
            for x, w in zip(lhs, wt):
                if len(res) in due:
                    w = _tie(w, due.pop(len(res)))
                v = dot(x, w)
                res.append(v)
                acc = v if acc is None else v + acc
                if len(res) in pace:
                    due[len(res) + PD] = p1_store(n0, pace.pop(len(res)), v[0:8, :])
            return acc

        t_scr[0:CAR, :] = t_scr[RB:RB + CAR, :]
        for hf in range(nh):
            lhs = [a1_scr[j, _tile(hf), :] for j in range(km)]
            for n in range(km):
                t = _gelu(mm(lhs, [w1_ref[_tile(j), _tile(n)] for j in range(km)], _dot))
                if hf == nh - 1:
                    t = jnp.concatenate([t[:T - OFF], jnp.where(r < nrb - 1, t[T - OFF:], 0.0)], axis=0)
                t_scr[CAR + hf * T:CAR + (hf + 1) * T, _tile(n)] = t
        cq = M // 4
        shifts = (-1, 1, -2, 2)
        lane = jax.lax.broadcasted_iota(jnp.int32, (T, T), 1)
        y1, a3 = [], []
        for hf in range(nh):
            base = CAR - OFF + hf * T
            lhs = []
            for j in range(km):
                g_lo, g_hi = (j * T) // cq, ((j + 1) * T - 1) // cq
                assert g_hi - g_lo <= 1
                v = t_scr[base + shifts[g_lo]:base + shifts[g_lo] + T, _tile(j)]
                if g_hi != g_lo:
                    v2 = t_scr[base + shifts[g_hi]:base + shifts[g_hi] + T, _tile(j)]
                    v = jnp.where(lane < g_hi * cq - j * T, v, v2)
                lhs.append(v.astype(BF16))
            hs = jnp.concatenate(
                [mm(lhs, [w2_ref[_tile(j), _tile(n)] for j in range(km)], _dot) for n in range(km)], axis=1)
            y1.append(hs + hb_scr[pl.ds(pl.multiple_of(r0 + hf * T, T), T), :])
            a3.append(_ln(y1[hf]).astype(BF16))
        h3 = []
        for hf in range(nh):
            lhs = [a3[hf][:, _tile(j)] for j in range(km)]
            row = []
            narrow = None
            for i, (f0, f1) in enumerate(ftiles):
                if f1 - f0 == T:
                    wt = [w3_ref[f0:f1, _tile(j)] for j in range(km)]
                    row.append(_gelu(mm(lhs, wt, _dot_nt)).astype(BF16))
                    if Fd % T and 0 <= i - NW0 < km:
                        v = mm([w3_ref[ftiles[-1][0]:Fd, _tile(i - NW0)]], [lhs[i - NW0]], _dot_nt)
                        narrow = v if narrow is None else v + narrow
                else:
                    gT = jnp.concatenate([_gelu(narrow), jnp.zeros((T - (f1 - f0), T), F32)], axis=0)
                    row.append(_tie(gT.astype(BF16).T, gT[0:8, :])[:, :f1 - f0])
            h3.append(row)
        for hf in range(nh):
            rows = pl.ds(pl.multiple_of(r0 + hf * T, T), T)
            for n in range(km):
                v = mm(h3[hf], [w4_ref[f0:f1, _tile(n)] for f0, f1 in ftiles], _dot)
                out_buf[rows, _tile(n)] = (
                    x1_scr[rows, _tile(n)] + gb[:, _tile(n)] * (v + y1[hf][:, _tile(n)])
                ).astype(out_buf.dtype)
            out_copy(r * nh + hf).start()
        assert not pace
        return carry

    jax.lax.fori_loop(0, nrb, b_body, 0)
    for i in range(nb):
        out_copy(i).wait()


@jax.jit
def pallas_adaLN_cond__compressed_kv_cla__mixer_s_mlp__prompt_kernel(
    A_x: jax.Array,
    A_c_kv: jax.Array,
    A_w_q: jax.Array,
    A_w_uk: jax.Array,
    A_w_uv: jax.Array,
    A_w_o: jax.Array,
    B_x: jax.Array,
    B_w1: jax.Array,
    B_w2: jax.Array,
    B_w3: jax.Array,
    B_w4: jax.Array,
    c: jax.Array,
    w_mod: jax.Array,
):
    _, S, M = A_x.shape
    Dc = A_c_kv.shape[2]
    H, D = A_w_q.shape[1], A_w_q.shape[2]
    Fd = B_w3.shape[1]
    assert D == T and A_c_kv.shape[1] == S and Dc == 4 * T and M == 5 * T
    vmem = pltpu.VMEM
    packed = lambda *lead: vmem(lead + (T // 2, T), U32)
    out = pl.pallas_call(
        _kernel,
        in_specs=[pl.BlockSpec(memory_space=pltpu.HBM)] * 12,
        out_specs=pl.BlockSpec(memory_space=pltpu.HBM),
        out_shape=jax.ShapeDtypeStruct((S, M), A_x.dtype),
        scratch_shapes=[
            vmem((S + 16, M), BF16),
            vmem((S, Dc), BF16),
            vmem((1, M), BF16),
            vmem((M, 2 * M), BF16),
            vmem((M, 4 * M), BF16),
            vmem((M, M), BF16),
            vmem((M, M), BF16),
            vmem((Fd, M), BF16),
            vmem((Fd, M), BF16),
            vmem((M, D), U32),
            vmem((Dc, D), U32),
            vmem((Dc, D), U32),
            vmem((2, 2 * D, M), BF16),
            vmem((S, M), A_x.dtype),
            pltpu.SemaphoreType.DMA((15,)),
            pltpu.SemaphoreType.DMA((4,)),
            pltpu.SemaphoreType.DMA((S // T,)),
            vmem((8, 6 * M), F32),
            vmem((S // T // 2, 16, T, T), BF16),
            vmem((S // T // 2, 14, T, T), BF16),
            packed(44),
            packed(2 * S // T),
            packed(2 * S // T),
            packed(2 * S // T),
            vmem((S + 16, M), F32),
            vmem((S + 16, M), F32),
            vmem((S + 16, M), F32),
            vmem((M // T, RB, T), BF16),
            vmem((RB + 32, M), F32),
        ],
        compiler_params=pltpu.CompilerParams(
            vmem_limit_bytes=100 * 1024 * 1024,
            disable_bounds_checks=True,
        ),
    )(
        A_x.reshape(S, M), A_c_kv.reshape(S, Dc),
        A_w_q, A_w_uk, A_w_uv,
        A_w_o.reshape(H // 2, 2 * D, M),
        B_w1, B_w2, B_w3.T, B_w4, c, w_mod,
    )
    return out.reshape(1, S, M)
```

```python
import math
import os

import jax
import jax.numpy as jnp
import jax.experimental.pallas as pl
import jax.experimental.pallas.tpu as pltpu

F32 = jnp.float32
BF16 = jnp.bfloat16
U32 = jnp.uint32
NT = (((1,), (1,)), ((), ()))
T = 128
EPS = 1e-5
LOG2E = math.log2(math.e)

GRP = int(os.environ.get('GRP', 4))
LEAD = int(os.environ.get('LEAD', 10))
PROW = int(os.environ.get('PROW', 3))
VT = 8
RES = int(os.environ.get('RES', 30))
LAT_A = int(os.environ.get('LAT_A', 16))
LAT_B = int(os.environ.get('LAT_B', 16))
ALEAD = int(os.environ.get('ALEAD', 32))
MID = int(os.environ.get('MID', 40))
FINE = int(os.environ.get('FINE', 0))
OGRP = int(os.environ.get('OGRP', 6))
RB = 256
PC = 32
P0, PSTEP, PD = 180, 21, 24
NW0 = 5
LP = int(os.environ.get('LP', 16))
KVM, KVL, QLAG = [int(os.environ.get(k_, 1)) for k_ in ('KVM', 'KVL', 'QLAG')]
PLAN = os.environ.get('PLAN', 'kva,b,cdn,m,qw,x,yzo')


def _dot(a, b):
    return jnp.dot(a, b, preferred_element_type=F32)


def _dot_nt(a, b):
    return jax.lax.dot_general(a, b, NT, preferred_element_type=F32)


def _ln(x):
    m = jnp.mean(x, axis=-1, keepdims=True)
    xc = x - m
    v = jnp.mean(xc * xc, axis=-1, keepdims=True)
    return xc * jnp.exp2(jnp.log(v + EPS) * (-0.5 * LOG2E))


def _rows(v, n):
    return jnp.broadcast_to(v[None], (n // 8, 8, v.shape[1])).reshape(n, v.shape[1])


def _gelu(x):
    c0 = math.sqrt(2.0 / math.pi)
    return 0.5 * x * (1.0 + jnp.tanh(c0 * (x + 0.044715 * (x * x * x))))


def _after(x, dep):
    return jnp.where(dep > jnp.inf, dep, x)


def _tie(x, dep):
    xu = pltpu.bitcast(x, U32)
    first = jnp.where(dep > jnp.inf, jnp.uint32(0), xu[:8])
    return pltpu.bitcast(jnp.concatenate([first, xu[8:]], axis=0), BF16)


def _tile(j):
    return slice(j * T, (j + 1) * T)


def _ld(ref, *idx):
    return pltpu.bitcast(ref[idx], BF16)


def _pk(x):
    return pltpu.bitcast(x, U32)


def _a_ops(a11, a12, a21, a22):
    return [a11 + a22, a21 + a22, a11, a22, a11 + a12, a21 - a11, a12 - a22]


def _b_ops(b11, b12, b21, b22):
    return [b11 + b22, b11, b12 - b22, b21 - b11, b22, b11 + b12, b21 + b22]


def _strassen(prod):
    m4 = prod(3)
    m2 = prod(1)
    c21 = m2 + m4
    m3 = prod(2)
    m5 = prod(4)
    c12 = m3 + m5
    m1 = prod(0)
    c11 = prod(6) + (m1 + (m4 - m5))
    c22 = prod(5) + (m1 + (m3 - m2))
    return c11, c12, c21, c22


def _pair_weights(w_ref, transpose=False):
    lo, hi = [], []
    for j in range(w_ref.shape[0] // T):
        wu = w_ref[_tile(j), :]
        lo.append(pltpu.bitcast(wu << 16, F32))
        hi.append(pltpu.bitcast(wu & jnp.uint32(0xFFFF0000), F32))
    per_j = [_b_ops(lo[j], hi[j], lo[2 + j], hi[2 + j]) for j in range(2)]
    tiles = [per_j[j][i] for i in range(7) for j in range(2)]
    for j in range(4, len(lo)):
        tiles += [lo[j], hi[j]]
    tiles = [t.astype(BF16) for t in tiles]
    return [t.T for t in tiles] if transpose else tiles


class _Jobs:
    def __init__(self):
        self.res = []

    def mm(self, lhs, wt, dot, tie=False):
        acc = None
        for x, w in zip(lhs, wt):
            if tie and len(self.res) >= VT:
                x = _tie(x, self.res[len(self.res) - VT][0:8, :])
            v = dot(x, w)
            self.res.append(v)
            acc = v if acc is None else v + acc
        return acc


def _kv_jobs(jobs, p, cs_scr, wk, wvT, k_scr, v_scr):
    ct = lambda i: [cs_scr[p, 2 * i + j] for j in range(2)]
    ks = _strassen(lambda i: jobs.mm(ct(i), [wk(2 * i), wk(2 * i + 1)], _dot))
    for n, v in enumerate(ks):
        k_scr[4 * p + n] = _pk(v.astype(BF16))
    vs = _strassen(lambda i: jobs.mm([wvT(2 * i), wvT(2 * i + 1)], ct(i), _dot_nt, True))
    for n, v in enumerate(vs):
        v_scr[4 * p + n] = _pk(v.astype(BF16))


def _q_jobs(jobs, p, h_scr, wq, q_scr, scale):
    rest = [jobs.mm([h_scr[p, 14 + n // 2]], [wq(14 + n % 2)], _dot) for n in range(4)]
    qs = _strassen(lambda i: jobs.mm([h_scr[p, 2 * i + j] for j in range(2)],
                                     [wq(2 * i), wq(2 * i + 1)], _dot))
    for n, v in enumerate(qs):
        q_scr[4 * p + n] = _pk(((v + rest[n]) * scale).astype(BF16))


def _proj_step(h_scr, cs_scr, wq_ref, wuk_ref, wuv_ref, q_scr, k_scr, v_scr, scale):
    wq = _pair_weights(wq_ref)
    wk = _pair_weights(wuk_ref)
    wvT = _pair_weights(wuv_ref, True)
    jobs = _Jobs()
    for p in range(h_scr.shape[0]):
        _q_jobs(jobs, p, h_scr, wq.__getitem__, q_scr, scale)
        _kv_jobs(jobs, p, cs_scr, wk.__getitem__, wvT.__getitem__, k_scr, v_scr)


_O_JOBS = ([(0, 'r', 0, 0), (0, 'm', 2, 0), (0, 'm', 2, 1), (1, 'r', 1, 0), (1, 'm', 4, 0), (1, 'm', 4, 1),
            (2, 'r', 2, 0), (2, 'm', 5, 0), (2, 'm', 5, 1), (3, 'r', 3, 0)]
           + [(3, 'm', i, n) for n in range(2) for i in (3, 1, 0, 6)])


def _job_order(nb):
    units = range(2 * nb)
    qa = [('a', u, c) for u in units for c in range(u // 2 + 1)]
    qb = [('b', u, c) for u in units for c in range(u // 2 + 1)]
    last = nb // 2 - 1
    qo = [('o', 4 * p + (job[0] if FINE or p == last else 3), j)
          for p in range(nb // 2) for j, job in enumerate(_O_JOBS)]
    done = {}
    order = []

    def ready(q, lat, pre):
        return bool(q) and (pre, q[0][1]) in done and done[(pre, q[0][1])] + lat <= len(order)

    def emit(q):
        kind, u, j = job = q.pop(0)
        if kind != 'o' and j == u // 2:
            done[(kind, u)] = len(order)
        order.append(job)

    turn = 0
    while qa or qb or qo:
        pref = 'abo'[turn % 3]
        turn += 1
        for _ in range(OGRP if pref == 'o' else GRP):
            b_ok, o_ok = ready(qb, LAT_A, 'a'), ready(qo, LAT_B, 'b')
            if pref == 'a' and qa and (len(qb) - len(qa) < ALEAD or not b_ok):
                emit(qa)
            elif pref == 'b' and b_ok:
                emit(qb)
            elif pref == 'o' and o_ok and (len(qo) > RES or not (qa or b_ok)):
                emit(qo)
            elif not (qa or b_ok or o_ok) and (qb or qo):
                emit(qb or qo)
            else:
                break
    return order


def _attention_step(q_scr, k_scr, v_scr, wo_ref, acc_scr, mid):
    causal = (jax.lax.broadcasted_iota(jnp.int32, (T, T), 0)
              <= jax.lax.broadcasted_iota(jnp.int32, (T, T), 1))
    sv, mx, mfin, lsum, pv, of, lhs, prod = {}, {}, {}, {}, {}, {}, {}, {}
    res = []
    wo = [[t.astype(BF16) for t in _b_ops(*[wo_ref[_tile(i // 2), _tile(2 * n + i % 2)].astype(F32)
                                            for i in range(4)])] for n in range(2)]

    def job_a(u, c):
        r, hd = divmod(u, 2)
        s = _dot_nt(_ld(k_scr, 2 * c + hd), _ld(q_scr, u))
        res.append(s)
        if c == r:
            s = jnp.where(causal, s, -1e9 * LOG2E)
        s = s.reshape(T // 8, 8, T)
        sv[(u, c)] = s
        pm = jnp.max(s, axis=0)
        mx[u] = pm if u not in mx else jnp.maximum(mx[u], pm)

    def job_b(u, c):
        r, hd = divmod(u, 2)
        if u not in mfin:
            mfin[u] = jnp.broadcast_to(jnp.max(mx[u], axis=0, keepdims=True), (8, T))
        m = mfin[u]
        if len(res) >= LEAD:
            r0 = 8 * PROW * (c % 4)
            m = _after(m, res[len(res) - LEAD][r0:r0 + 8, :])
        p = jnp.exp2(sv.pop((u, c)) - m[None])
        ls = jnp.sum(p, axis=0)
        lsum[u] = ls if u not in lsum else lsum[u] + ls
        v = _dot(_ld(v_scr, 2 * c + hd), p.reshape(T, T).astype(BF16))
        res.append(v)
        pv[u] = v if u not in pv else v + pv[u]
        if c == r:
            of[u] = pv[u] * (1.0 / jnp.sum(lsum[u], axis=0, keepdims=True))

    def o_lhs(p, kind, i):
        if kind == 'm' and i in (2, 3):
            kind, i = 'r', 3 * (i - 2)
        if (p, kind, i) not in lhs:
            a = lambda n: of[4 * p + n]
            v = a(i) if kind == 'r' else {0: lambda: a(0) + a(3), 1: lambda: a(2) + a(3), 4: lambda: a(0) + a(1),
                                          5: lambda: a(2) - a(0), 6: lambda: a(1) - a(3)}[i]()
            lhs[(p, kind, i)] = _tie(v.astype(BF16).T, v[0:8, :])
        return lhs[(p, kind, i)]

    def job_o(u, j):
        p = u // 4
        _, kind, i, n = _O_JOBS[j]
        w = wo[n][i] if kind == 'm' else wo_ref[_tile(i % 2), _tile(4)]
        v = _dot(o_lhs(p, kind, i), w)
        res.append(v)
        prod[(kind, i, n)] = v
        m = lambda i_: prod[('m', i_, n)]
        if kind == 'r':
            if i % 2:
                acc_scr[_tile(2 * p + i // 2), _tile(4)] += v + prod[('r', i - 1, 0)]
        elif i == 4:
            acc_scr[_tile(2 * p), _tile(2 * n + 1)] += v + m(2)
        elif i == 5:
            prod[('m', 5, n)] = v + m(2)
        elif i == 1:
            acc_scr[_tile(2 * p + 1), _tile(2 * n)] += v + m(3)
        elif i == 0:
            acc_scr[_tile(2 * p + 1), _tile(2 * n + 1)] += v + (m(5) - m(1))
        elif i == 6:
            acc_scr[_tile(2 * p), _tile(2 * n)] += v + (m(0) + (m(3) - m(4)))

    fns = dict(a=job_a, b=job_b, o=job_o)
    for n, (kind, u, j) in enumerate(_job_order(q_scr.shape[0] // 2)):
        if n == MID:
            mid()
        fns[kind](u, j)


def _kernel(x_hbm, c_hbm, wq_hbm, wuk_hbm, wuv_hbm, wo_hbm, w1_hbm, w2_hbm, w3_hbm, w4_hbm,
            cond_hbm, wmod_hbm, out_hbm,
            x_ref, c_ref, cond_ref, wma_ref, wmb_ref, w1_ref, w2_ref, w3_ref, w4_ref,
            wq_buf, wk_buf, wv_buf, wo_buf, out_buf, sem, wsem, osem,
            mod_scr, h_scr, cs_scr, w_scr, q_scr, k_scr, v_scr, acc_scr, x1_scr, hb_scr, a1_scr, t_scr):
    S, M = x_hbm.shape
    D = wq_hbm.shape[2]
    nattn = wo_hbm.shape[0]
    Fd = w4_hbm.shape[0]
    scale = float(D) ** -0.5 * LOG2E
    nb, nrb = S // T, S // RB
    km, kc = M // T, c_hbm.shape[1] // T
    NX = 4
    XR = S // NX
    CB = XR // T

    def pcopies(g):
        return [pltpu.make_async_copy(src.bitcast(U32).at[:, g, :], dst, wsem.at[j])
                for j, (src, dst) in enumerate(((wuk_hbm, wk_buf), (wuv_hbm, wv_buf), (wq_hbm, wq_buf)))]

    def ocopy(g, slot):
        return pltpu.make_async_copy(wo_hbm.at[g], wo_buf.at[slot], wsem.at[3])

    def chunk_copy(src, dst, i, s0):
        rows = slice(i * XR, (i + 1) * XR)
        return pltpu.make_async_copy(src.at[rows, :], dst.at[rows, :], sem.at[s0 + i])

    cp_cond = pltpu.make_async_copy(cond_hbm, cond_ref, sem.at[0])
    cp_wma = pltpu.make_async_copy(wmod_hbm.at[:, 0:2 * M], wma_ref, sem.at[1])
    cp_late = [pltpu.make_async_copy(src, dst, sem.at[2 + j]) for j, (src, dst) in enumerate((
        (wmod_hbm.at[:, 2 * M:6 * M], wmb_ref), (w1_hbm, w1_ref), (w2_hbm, w2_ref),
        (w3_hbm, w3_ref), (w4_hbm, w4_ref)))]
    cp_x = [chunk_copy(x_hbm, x_ref, i, 7) for i in range(NX)]
    cp_c = [chunk_copy(c_hbm, c_ref, i, 7 + NX) for i in range(NX)]

    def silu_cond():
        cf = cond_ref[...].astype(F32)
        return jnp.broadcast_to((cf * jax.nn.sigmoid(cf)).astype(BF16), (8, M))

    cp_wk, cp_wv, cp_wq = pcopies(0)
    named = dict(k=cp_wk, v=cp_wv, q=cp_wq, o=ocopy(0, 0), n=cp_cond, m=cp_wma)
    named.update(zip('abcd', cp_c))
    named.update(zip('wxyz', cp_x))
    plan = PLAN.split(',')

    def kick():
        for ch in plan.pop(0) if plan else '':
            named.pop(ch).start()

    def zero(r, carry):
        acc_scr[pl.ds(pl.multiple_of(r * T, T), T), :] = jnp.zeros((T, M), F32)
        return carry

    def ln_pair(p):
        sa = _rows(mod_scr[:, 0:M], LP)
        ca1 = _rows(mod_scr[:, M:2 * M], LP)
        for i in range(T // LP):
            h1, h2 = [_ln(x_ref[r * T + i * LP:r * T + (i + 1) * LP, :].astype(F32)) * ca1 + sa
                      for r in (2 * p, 2 * p + 1)]
            ops = _a_ops(h1[:, 0:2 * T], h1[:, 2 * T:4 * T], h2[:, 0:2 * T], h2[:, 2 * T:4 * T])
            tiles = [v[:, _tile(j)] for v in ops for j in range(2)] + [h1[:, _tile(4)], h2[:, _tile(4)]]
            for n, v in enumerate(tiles):
                h_scr[p, n, i * LP:(i + 1) * LP, :] = v.astype(BF16)

    def stash(tiles, j0):
        for j, t in enumerate(tiles):
            w_scr[j0 + j] = _pk(t)
        return lambda j: _ld(w_scr, j0 + j)

    def kv_pairs(jobs, p0, p1_):
        for p in range(p0, p1_):
            for j in range(2):
                ops = _a_ops(*[c_ref[_tile(2 * p + n // 2), _tile(2 * (n % 2) + j)].astype(F32)
                               for n in range(4)])
                for i, v in enumerate(ops):
                    cs_scr[p, 2 * i + j] = v.astype(BF16)
            _kv_jobs(jobs, p, cs_scr, wk, wvT, k_scr, v_scr)

    npair, CP = nb // 2, CB // 2
    kick()
    jax.lax.fori_loop(0, nb, zero, 0)
    kick()
    acc_scr[S:, :] = jnp.zeros((acc_scr.shape[0] - S, M), F32)
    x_ref[S:, :] = jnp.zeros((x_ref.shape[0] - S, M), BF16)
    cp_wk.wait()
    cp_wv.wait()
    cp_c[0].wait()
    kick()
    wk = stash(_pair_weights(wk_buf), 0)
    wvT = stash(_pair_weights(wv_buf, True), 14)
    kv_pairs(_Jobs(), 0, CP)
    for chunks in ((1,), (2, 3)):
        for i in chunks:
            cp_c[i].wait()
        kick()
        kv_pairs(_Jobs(), chunks[0] * CP, min((chunks[-1] + 1) * CP, npair - KVL - KVM))
    cp_cond.wait()
    cp_wma.wait()
    kick()
    mod = _dot(silu_cond(), wma_ref[...])
    mod_scr[:, 0:M] = mod[:, 0:M]
    mod_scr[:, M:2 * M] = 1.0 + mod[:, M:2 * M]
    kv_pairs(_Jobs(), npair - KVL - KVM, npair - KVL)
    cp_wq.wait()
    qdone = 0
    for chunks in ((0,), (1,), (2, 3)):
        for i in chunks:
            cp_x[i].wait()
        kick()
        jobs = _Jobs()
        if chunks[0] == 0:
            wq = stash(_pair_weights(wq_buf), 28)
            kv_pairs(jobs, npair - KVL, npair)
        for p in range(chunks[0] * CP, (chunks[-1] + 1) * CP):
            ln_pair(p)
        qend = npair if chunks[-1] == NX - 1 else (chunks[-1] + 1) * CP - QLAG
        for p in range(qdone, qend):
            _q_jobs(jobs, p, h_scr, wq, q_scr, scale)
        qdone = max(qdone, qend)
    assert not named
    ocopy(0, 0).wait()
    for cp in cp_late:
        cp.start()

    def attn_body(g, carry):
        slot = g & 1
        nxt = jnp.minimum(g + 1, nattn - 1)
        copies = pcopies(nxt) + [ocopy(nxt, 1 - slot)]

        def mid():
            for cp in copies:
                cp.start()

        _attention_step(q_scr, k_scr, v_scr, wo_buf.at[slot], acc_scr, mid)
        for cp in copies:
            cp.wait()

        @pl.when(g + 1 < nattn)
        def _():
            _proj_step(h_scr, cs_scr, wq_buf, wk_buf, wv_buf, q_scr, k_scr, v_scr, scale)

        return carry

    jax.lax.fori_loop(0, nattn, attn_body, 0)

    for cp in cp_late:
        cp.wait()
    mod = _dot(silu_cond(), wmb_ref[...])
    mod_scr[:, 2 * M:4 * M] = mod[:, 0:2 * M]
    mod_scr[:, 4 * M:5 * M] = 1.0 + mod[:, 2 * M:3 * M]
    mod_scr[:, 5 * M:6 * M] = mod[:, 3 * M:4 * M]
    ftiles = [(f, min(f + T, Fd)) for f in range(0, Fd, T)]
    OFF = x_ref.shape[0] - S
    CAR = t_scr.shape[0] - RB

    def p1(r0, n, dep=None):
        ga = mod_scr[:, 2 * M:3 * M]
        if dep is not None:
            ga = jnp.concatenate([_after(ga[:, 0:T], dep), ga[:, T:]], axis=1)
        rows = pl.ds(r0, n)
        x1 = x_ref[rows, :].astype(F32) + _rows(ga, n) * acc_scr[rows, :]
        x1_scr[rows, :] = x1
        hb = _ln(x1) * _rows(mod_scr[:, 4 * M:5 * M], n) + _rows(mod_scr[:, 3 * M:4 * M], n)
        hb_scr[rows, :] = hb
        return _ln(hb)

    def p1_store(r0, c, dep=None):
        a1f = p1(r0 + c * PC, PC, dep)
        a1 = a1f.astype(BF16)
        for j in range(km):
            a1_scr[j, c * PC:(c + 1) * PC, :] = a1[:, _tile(j)]
        return jnp.max(a1f[:, M - T:].reshape(PC // 8, 8, T), axis=0)

    t_scr[RB:RB + CAR - OFF, :] = jnp.zeros((CAR - OFF, M), F32)
    t_scr[RB + CAR - OFF:RB + CAR, :] = _gelu(_dot(p1(0, OFF).astype(BF16), w1_ref[...]))
    for c in range(RB // PC):
        p1_store(OFF, c)

    def out_copy(i):
        rows = pl.ds(i * T if isinstance(i, int) else pl.multiple_of(i * T, T), T)
        return pltpu.make_async_copy(out_buf.at[rows, :], out_hbm.at[rows, :], osem.at[i])

    def b_body(r, carry):
        gb = _rows(mod_scr[:, 5 * M:6 * M], T)
        r0 = pl.multiple_of(r * RB, RB)
        n0 = pl.multiple_of(jnp.minimum(r0 + RB, S - RB) + OFF, OFF)
        nh = RB // T
        res = []
        due = {}
        pace = {P0 + i * PSTEP: i for i in range(RB // PC)}

        def mm(lhs, wt, dot):
            acc = None
            for x, w in zip(lhs, wt):
                if len(res) in due:
                    w = _tie(w, due.pop(len(res)))
                v = dot(x, w)
                res.append(v)
                acc = v if acc is None else v + acc
                if len(res) in pace:
                    due[len(res) + PD] = p1_store(n0, pace.pop(len(res)), v[0:8, :])
            return acc

        t_scr[0:CAR, :] = t_scr[RB:RB + CAR, :]
        for hf in range(nh):
            lhs = [a1_scr[j, _tile(hf), :] for j in range(km)]
            for n in range(km):
                t = _gelu(mm(lhs, [w1_ref[_tile(j), _tile(n)] for j in range(km)], _dot))
                if hf == nh - 1:
                    t = jnp.concatenate([t[:T - OFF], jnp.where(r < nrb - 1, t[T - OFF:], 0.0)], axis=0)
                t_scr[CAR + hf * T:CAR + (hf + 1) * T, _tile(n)] = t
        cq = M // 4
        shifts = (-1, 1, -2, 2)
        lane = jax.lax.broadcasted_iota(jnp.int32, (T, T), 1)
        y1, a3 = [], []
        for hf in range(nh):
            base = CAR - OFF + hf * T
            lhs = []
            for j in range(km):
                g_lo, g_hi = (j * T) // cq, ((j + 1) * T - 1) // cq
                assert g_hi - g_lo <= 1
                v = t_scr[base + shifts[g_lo]:base + shifts[g_lo] + T, _tile(j)]
                if g_hi != g_lo:
                    v2 = t_scr[base + shifts[g_hi]:base + shifts[g_hi] + T, _tile(j)]
                    v = jnp.where(lane < g_hi * cq - j * T, v, v2)
                lhs.append(v.astype(BF16))
            hs = jnp.concatenate(
                [mm(lhs, [w2_ref[_tile(j), _tile(n)] for j in range(km)], _dot) for n in range(km)], axis=1)
            y1.append(hs + hb_scr[pl.ds(pl.multiple_of(r0 + hf * T, T), T), :])
            a3.append(_ln(y1[hf]).astype(BF16))
        h3 = []
        for hf in range(nh):
            lhs = [a3[hf][:, _tile(j)] for j in range(km)]
            row = []
            narrow = None
            for i, (f0, f1) in enumerate(ftiles):
                if f1 - f0 == T:
                    wt = [w3_ref[f0:f1, _tile(j)] for j in range(km)]
                    row.append(_gelu(mm(lhs, wt, _dot_nt)).astype(BF16))
                    if Fd % T and 0 <= i - NW0 < km:
                        v = mm([w3_ref[ftiles[-1][0]:Fd, _tile(i - NW0)]], [lhs[i - NW0]], _dot_nt)
                        narrow = v if narrow is None else v + narrow
                else:
                    gT = jnp.concatenate([_gelu(narrow), jnp.zeros((T - (f1 - f0), T), F32)], axis=0)
                    row.append(_tie(gT.astype(BF16).T, gT[0:8, :])[:, :f1 - f0])
            h3.append(row)
        for hf in range(nh):
            rows = pl.ds(pl.multiple_of(r0 + hf * T, T), T)
            for n in range(km):
                v = mm(h3[hf], [w4_ref[f0:f1, _tile(n)] for f0, f1 in ftiles], _dot)
                out_buf[rows, _tile(n)] = (
                    x1_scr[rows, _tile(n)] + gb[:, _tile(n)] * (v + y1[hf][:, _tile(n)])
                ).astype(out_buf.dtype)
            out_copy(r * nh + hf).start()
        assert not pace
        return carry

    jax.lax.fori_loop(0, nrb, b_body, 0)
    for i in range(nb):
        out_copy(i).wait()


@jax.jit
def pallas_adaLN_cond__compressed_kv_cla__mixer_s_mlp__prompt_kernel(
    A_x: jax.Array,
    A_c_kv: jax.Array,
    A_w_q: jax.Array,
    A_w_uk: jax.Array,
    A_w_uv: jax.Array,
    A_w_o: jax.Array,
    B_x: jax.Array,
    B_w1: jax.Array,
    B_w2: jax.Array,
    B_w3: jax.Array,
    B_w4: jax.Array,
    c: jax.Array,
    w_mod: jax.Array,
):
    _, S, M = A_x.shape
    Dc = A_c_kv.shape[2]
    H, D = A_w_q.shape[1], A_w_q.shape[2]
    Fd = B_w3.shape[1]
    assert D == T and A_c_kv.shape[1] == S and Dc == 4 * T and M == 5 * T
    vmem = pltpu.VMEM
    packed = lambda *lead: vmem(lead + (T // 2, T), U32)
    out = pl.pallas_call(
        _kernel,
        in_specs=[pl.BlockSpec(memory_space=pltpu.HBM)] * 12,
        out_specs=pl.BlockSpec(memory_space=pltpu.HBM),
        out_shape=jax.ShapeDtypeStruct((S, M), A_x.dtype),
        scratch_shapes=[
            vmem((S + 16, M), BF16),
            vmem((S, Dc), BF16),
            vmem((1, M), BF16),
            vmem((M, 2 * M), BF16),
            vmem((M, 4 * M), BF16),
            vmem((M, M), BF16),
            vmem((M, M), BF16),
            vmem((Fd, M), BF16),
            vmem((Fd, M), BF16),
            vmem((M, D), U32),
            vmem((Dc, D), U32),
            vmem((Dc, D), U32),
            vmem((2, 2 * D, M), BF16),
            vmem((S, M), A_x.dtype),
            pltpu.SemaphoreType.DMA((15,)),
            pltpu.SemaphoreType.DMA((4,)),
            pltpu.SemaphoreType.DMA((S // T,)),
            vmem((8, 6 * M), F32),
            vmem((S // T // 2, 16, T, T), BF16),
            vmem((S // T // 2, 14, T, T), BF16),
            packed(44),
            packed(2 * S // T),
            packed(2 * S // T),
            packed(2 * S // T),
            vmem((S + 16, M), F32),
            vmem((S + 16, M), F32),
            vmem((S + 16, M), F32),
            vmem((M // T, RB, T), BF16),
            vmem((RB + 32, M), F32),
        ],
        compiler_params=pltpu.CompilerParams(
            vmem_limit_bytes=100 * 1024 * 1024,
            disable_bounds_checks=True,
        ),
    )(
        A_x.reshape(S, M), A_c_kv.reshape(S, Dc),
        A_w_q, A_w_uk, A_w_uv,
        A_w_o.reshape(H // 2, 2 * D, M),
        B_w1, B_w2, B_w3.T, B_w4, c, w_mod,
    )
    return out.reshape(1, S, M)
```

```python
import math
import os

import jax
import jax.numpy as jnp
import jax.experimental.pallas as pl
import jax.experimental.pallas.tpu as pltpu

F32 = jnp.float32
BF16 = jnp.bfloat16
U32 = jnp.uint32
NT = (((1,), (1,)), ((), ()))
T = 128
EPS = 1e-5
LOG2E = math.log2(math.e)

GRP = int(os.environ.get('GRP', 4))
LEAD = int(os.environ.get('LEAD', 10))
PROW = int(os.environ.get('PROW', 3))
VT = 8
RES = int(os.environ.get('RES', 30))
LAT_A = int(os.environ.get('LAT_A', 16))
LAT_B = int(os.environ.get('LAT_B', 20))
ALEAD = int(os.environ.get('ALEAD', 32))
MID = int(os.environ.get('MID', 40))
FINE = int(os.environ.get('FINE', 0))
OGRP = int(os.environ.get('OGRP', 6))
RB = 256
PC = 32
P0, PSTEP, PD = [int(os.environ.get(k_, d_)) for k_, d_ in (('P0', 330), ('PSTEP', 38), ('PD', 48))]
LP = int(os.environ.get('LP', 16))
KVM, KVL, QLAG = [int(os.environ.get(k_, 1)) for k_ in ('KVM', 'KVL', 'QLAG')]
PLAN = os.environ.get('PLAN', 'kva,b,cdn,m,qw,x,yzo')


def _dot(a, b):
    return jnp.dot(a, b, preferred_element_type=F32)


def _dot_nt(a, b):
    return jax.lax.dot_general(a, b, NT, preferred_element_type=F32)


def _ln(x):
    m = jnp.mean(x, axis=-1, keepdims=True)
    xc = x - m
    v = jnp.mean(xc * xc, axis=-1, keepdims=True)
    return xc * jnp.exp2(jnp.log(v + EPS) * (-0.5 * LOG2E))


def _rows(v, n):
    return jnp.broadcast_to(v[None], (n // 8, 8, v.shape[1])).reshape(n, v.shape[1])


def _gelu(x):
    c0 = math.sqrt(2.0 / math.pi)
    return 0.5 * x * (1.0 + jnp.tanh(c0 * (x + 0.044715 * (x * x * x))))


def _after(x, dep):
    return jnp.where(dep > jnp.inf, dep, x)


def _tie(x, dep):
    xu = pltpu.bitcast(x, U32)
    first = jnp.where(dep > jnp.inf, jnp.uint32(0), xu[:8])
    return pltpu.bitcast(jnp.concatenate([first, xu[8:]], axis=0), BF16)


def _tile(j):
    return slice(j * T, (j + 1) * T)


def _ld(ref, *idx):
    return pltpu.bitcast(ref[idx], BF16)


def _pk(x):
    return pltpu.bitcast(x, U32)


def _a_ops(a11, a12, a21, a22):
    return [a11 + a22, a21 + a22, a11, a22, a11 + a12, a21 - a11, a12 - a22]


def _b_ops(b11, b12, b21, b22):
    return [b11 + b22, b11, b12 - b22, b21 - b11, b22, b11 + b12, b21 + b22]


def _strassen(prod):
    m4 = prod(3)
    m2 = prod(1)
    c21 = m2 + m4
    m3 = prod(2)
    m5 = prod(4)
    c12 = m3 + m5
    m1 = prod(0)
    c11 = prod(6) + (m1 + (m4 - m5))
    c22 = prod(5) + (m1 + (m3 - m2))
    return c11, c12, c21, c22


def _pair_weights(w_ref, transpose=False):
    lo, hi = [], []
    for j in range(w_ref.shape[0] // T):
        wu = w_ref[_tile(j), :]
        lo.append(pltpu.bitcast(wu << 16, F32))
        hi.append(pltpu.bitcast(wu & jnp.uint32(0xFFFF0000), F32))
    per_j = [_b_ops(lo[j], hi[j], lo[2 + j], hi[2 + j]) for j in range(2)]
    tiles = [per_j[j][i] for i in range(7) for j in range(2)]
    for j in range(4, len(lo)):
        tiles += [lo[j], hi[j]]
    tiles = [t.astype(BF16) for t in tiles]
    return [t.T for t in tiles] if transpose else tiles


class _Jobs:
    def __init__(self):
        self.res = []

    def mm(self, lhs, wt, dot, tie=False):
        acc = None
        for x, w in zip(lhs, wt):
            if tie and len(self.res) >= VT:
                x = _tie(x, self.res[len(self.res) - VT][0:8, :])
            v = dot(x, w)
            self.res.append(v)
            acc = v if acc is None else v + acc
        return acc


def _kv_jobs(jobs, p, cs_scr, wk, wvT, k_scr, v_scr):
    ct = lambda i: [cs_scr[p, 2 * i + j] for j in range(2)]
    ks = _strassen(lambda i: jobs.mm(ct(i), [wk(2 * i), wk(2 * i + 1)], _dot))
    for n, v in enumerate(ks):
        k_scr[4 * p + n] = _pk(v.astype(BF16))
    vs = _strassen(lambda i: jobs.mm([wvT(2 * i), wvT(2 * i + 1)], ct(i), _dot_nt, True))
    for n, v in enumerate(vs):
        v_scr[4 * p + n] = _pk(v.astype(BF16))


def _q_jobs(jobs, p, h_scr, wq, q_scr, scale):
    rest = [jobs.mm([h_scr[p, 14 + n // 2]], [wq(14 + n % 2)], _dot) for n in range(4)]
    qs = _strassen(lambda i: jobs.mm([h_scr[p, 2 * i + j] for j in range(2)],
                                     [wq(2 * i), wq(2 * i + 1)], _dot))
    for n, v in enumerate(qs):
        q_scr[4 * p + n] = _pk(((v + rest[n]) * scale).astype(BF16))


def _proj_step(h_scr, cs_scr, wq_ref, wuk_ref, wuv_ref, q_scr, k_scr, v_scr, scale, side):
    wq = _pair_weights(wq_ref)
    wk = _pair_weights(wuk_ref)
    wvT = _pair_weights(wuv_ref, True)
    jobs = _Jobs()
    for p in range(h_scr.shape[0]):
        _q_jobs(jobs, p, h_scr, wq.__getitem__, q_scr, scale)
        _kv_jobs(jobs, p, cs_scr, wk.__getitem__, wvT.__getitem__, k_scr, v_scr)
        if p < len(side):
            side[p](jobs.res[-1][0:8, :])


_O_JOBS = ([(0, 'r', 0, 0), (0, 'm', 2, 0), (0, 'm', 2, 1), (1, 'r', 1, 0), (1, 'm', 4, 0), (1, 'm', 4, 1),
            (2, 'r', 2, 0), (2, 'm', 5, 0), (2, 'm', 5, 1), (3, 'r', 3, 0)]
           + [(3, 'm', i, n) for n in range(2) for i in (3, 1, 0, 6)])


def _job_order(nb):
    units = range(2 * nb)
    qa = [('a', u, c) for u in units for c in range(u // 2 + 1)]
    qb = [('b', u, c) for u in units for c in range(u // 2 + 1)]
    last = nb // 2 - 1
    qo = [('o', 4 * p + (job[0] if FINE or p == last else 3), j)
          for p in range(nb // 2) for j, job in enumerate(_O_JOBS)]
    done = {}
    order = []

    def ready(q, lat, pre):
        return bool(q) and (pre, q[0][1]) in done and done[(pre, q[0][1])] + lat <= len(order)

    def emit(q):
        kind, u, j = job = q.pop(0)
        if kind != 'o' and j == u // 2:
            done[(kind, u)] = len(order)
        order.append(job)

    turn = 0
    while qa or qb or qo:
        pref = 'abo'[turn % 3]
        turn += 1
        for _ in range(OGRP if pref == 'o' else GRP):
            b_ok, o_ok = ready(qb, LAT_A, 'a'), ready(qo, LAT_B, 'b')
            if pref == 'a' and qa and (len(qb) - len(qa) < ALEAD or not b_ok):
                emit(qa)
            elif pref == 'b' and b_ok:
                emit(qb)
            elif pref == 'o' and o_ok and (len(qo) > RES or not (qa or b_ok)):
                emit(qo)
            elif not (qa or b_ok or o_ok) and (qb or qo):
                emit(qb or qo)
            else:
                break
    return order


def _attention_step(q_scr, k_scr, v_scr, wo_ref, acc_scr, mid):
    causal = (jax.lax.broadcasted_iota(jnp.int32, (T, T), 0)
              <= jax.lax.broadcasted_iota(jnp.int32, (T, T), 1))
    sv, mx, mfin, lsum, pv, of, lhs, prod = {}, {}, {}, {}, {}, {}, {}, {}
    res = []
    wo = [[t.astype(BF16) for t in _b_ops(*[wo_ref[_tile(i // 2), _tile(2 * n + i % 2)].astype(F32)
                                            for i in range(4)])] for n in range(2)]

    def job_a(u, c):
        r, hd = divmod(u, 2)
        s = _dot_nt(_ld(k_scr, 2 * c + hd), _ld(q_scr, u))
        res.append(s)
        if c == r:
            s = jnp.where(causal, s, -1e9 * LOG2E)
        s = s.reshape(T // 8, 8, T)
        sv[(u, c)] = s
        pm = jnp.max(s, axis=0)
        mx[u] = pm if u not in mx else jnp.maximum(mx[u], pm)

    def job_b(u, c):
        r, hd = divmod(u, 2)
        if u not in mfin:
            mfin[u] = jnp.broadcast_to(jnp.max(mx[u], axis=0, keepdims=True), (8, T))
        m = mfin[u]
        if len(res) >= LEAD:
            r0 = 8 * PROW * (c % 4)
            m = _after(m, res[len(res) - LEAD][r0:r0 + 8, :])
        p = jnp.exp2(sv.pop((u, c)) - m[None])
        ls = jnp.sum(p, axis=0)
        lsum[u] = ls if u not in lsum else lsum[u] + ls
        v = _dot(_ld(v_scr, 2 * c + hd), p.reshape(T, T).astype(BF16))
        res.append(v)
        pv[u] = v if u not in pv else v + pv[u]
        if c == r:
            of[u] = pv[u] * (1.0 / jnp.sum(lsum[u], axis=0, keepdims=True))

    def o_lhs(p, kind, i):
        if kind == 'm' and i in (2, 3):
            kind, i = 'r', 3 * (i - 2)
        if (p, kind, i) not in lhs:
            a = lambda n: of[4 * p + n]
            v = a(i) if kind == 'r' else {0: lambda: a(0) + a(3), 1: lambda: a(2) + a(3), 4: lambda: a(0) + a(1),
                                          5: lambda: a(2) - a(0), 6: lambda: a(1) - a(3)}[i]()
            lhs[(p, kind, i)] = _tie(v.astype(BF16).T, v[0:8, :])
        return lhs[(p, kind, i)]

    def job_o(u, j):
        p = u // 4
        _, kind, i, n = _O_JOBS[j]
        w = wo[n][i] if kind == 'm' else wo_ref[_tile(i % 2), _tile(4)]
        v = _dot(o_lhs(p, kind, i), w)
        res.append(v)
        prod[(kind, i, n)] = v
        m = lambda i_: prod[('m', i_, n)]
        if kind == 'r':
            if i % 2:
                acc_scr[_tile(2 * p + i // 2), _tile(4)] += v + prod[('r', i - 1, 0)]
        elif i == 4:
            acc_scr[_tile(2 * p), _tile(2 * n + 1)] += v + m(2)
        elif i == 5:
            prod[('m', 5, n)] = v + m(2)
        elif i == 1:
            acc_scr[_tile(2 * p + 1), _tile(2 * n)] += v + m(3)
        elif i == 0:
            acc_scr[_tile(2 * p + 1), _tile(2 * n + 1)] += v + (m(5) - m(1))
        elif i == 6:
            acc_scr[_tile(2 * p), _tile(2 * n)] += v + (m(0) + (m(3) - m(4)))

    fns = dict(a=job_a, b=job_b, o=job_o)
    for n, (kind, u, j) in enumerate(_job_order(q_scr.shape[0] // 2)):
        if n == MID:
            mid()
        fns[kind](u, j)


def _kernel(x_hbm, c_hbm, wq_hbm, wuk_hbm, wuv_hbm, wo_hbm, w1_hbm, w2_hbm, w3_hbm, w4_hbm,
            cond_hbm, wmod_hbm, out_hbm,
            x_ref, c_ref, cond_ref, wma_ref, wmb_ref, w1_ref, w2_ref, w3_ref, w4_ref,
            wq_buf, wk_buf, wv_buf, wo_buf, out_buf, sem, wsem, osem,
            mod_scr, h_scr, cs_scr, w_scr, q_scr, k_scr, v_scr, acc_scr, x1_scr, hb_scr, a1_scr, t_scr,
            a1s_scr, ws12, ws3, ws4):
    S, M = x_hbm.shape
    D = wq_hbm.shape[2]
    nattn = wo_hbm.shape[0]
    Fd = w4_hbm.shape[0]
    scale = float(D) ** -0.5 * LOG2E
    nb, nrb = S // T, S // RB
    km, kc = M // T, c_hbm.shape[1] // T
    NX = 4
    XR = S // NX
    CB = XR // T

    def pcopies(g):
        return [pltpu.make_async_copy(src.bitcast(U32).at[:, g, :], dst, wsem.at[j])
                for j, (src, dst) in enumerate(((wuk_hbm, wk_buf), (wuv_hbm, wv_buf), (wq_hbm, wq_buf)))]

    def ocopy(g, slot):
        return pltpu.make_async_copy(wo_hbm.at[g], wo_buf.at[slot], wsem.at[3])

    def chunk_copy(src, dst, i, s0):
        rows = slice(i * XR, (i + 1) * XR)
        return pltpu.make_async_copy(src.at[rows, :], dst.at[rows, :], sem.at[s0 + i])

    cp_cond = pltpu.make_async_copy(cond_hbm, cond_ref, sem.at[0])
    cp_wma = pltpu.make_async_copy(wmod_hbm.at[:, 0:2 * M], wma_ref, sem.at[1])
    cp_late = [pltpu.make_async_copy(src, dst, sem.at[2 + j]) for j, (src, dst) in enumerate((
        (wmod_hbm.at[:, 2 * M:6 * M], wmb_ref), (w1_hbm, w1_ref), (w2_hbm, w2_ref),
        (w3_hbm, w3_ref), (w4_hbm, w4_ref)))]
    cp_x = [chunk_copy(x_hbm, x_ref, i, 7) for i in range(NX)]
    cp_c = [chunk_copy(c_hbm, c_ref, i, 7 + NX) for i in range(NX)]

    def silu_cond():
        cf = cond_ref[...].astype(F32)
        return jnp.broadcast_to((cf * jax.nn.sigmoid(cf)).astype(BF16), (8, M))

    cp_wk, cp_wv, cp_wq = pcopies(0)
    named = dict(k=cp_wk, v=cp_wv, q=cp_wq, o=ocopy(0, 0), n=cp_cond, m=cp_wma)
    named.update(zip('abcd', cp_c))
    named.update(zip('wxyz', cp_x))
    plan = PLAN.split(',')

    def kick():
        for ch in plan.pop(0) if plan else '':
            named.pop(ch).start()

    def zero(r, carry):
        acc_scr[pl.ds(pl.multiple_of(r * T, T), T), :] = jnp.zeros((T, M), F32)
        return carry

    def ln_pair(p):
        sa = _rows(mod_scr[:, 0:M], LP)
        ca1 = _rows(mod_scr[:, M:2 * M], LP)
        for i in range(T // LP):
            h1, h2 = [_ln(x_ref[r * T + i * LP:r * T + (i + 1) * LP, :].astype(F32)) * ca1 + sa
                      for r in (2 * p, 2 * p + 1)]
            ops = _a_ops(h1[:, 0:2 * T], h1[:, 2 * T:4 * T], h2[:, 0:2 * T], h2[:, 2 * T:4 * T])
            tiles = [v[:, _tile(j)] for v in ops for j in range(2)] + [h1[:, _tile(4)], h2[:, _tile(4)]]
            for n, v in enumerate(tiles):
                h_scr[p, n, i * LP:(i + 1) * LP, :] = v.astype(BF16)

    def stash(tiles, j0):
        for j, t in enumerate(tiles):
            w_scr[j0 + j] = _pk(t)
        return lambda j: _ld(w_scr, j0 + j)

    def kv_pairs(jobs, p0, p1_):
        for p in range(p0, p1_):
            for j in range(2):
                ops = _a_ops(*[c_ref[_tile(2 * p + n // 2), _tile(2 * (n % 2) + j)].astype(F32)
                               for n in range(4)])
                for i, v in enumerate(ops):
                    cs_scr[p, 2 * i + j] = v.astype(BF16)
            _kv_jobs(jobs, p, cs_scr, wk, wvT, k_scr, v_scr)

    npair, CP = nb // 2, CB // 2
    kick()
    jax.lax.fori_loop(0, nb, zero, 0)
    kick()
    acc_scr[S:, :] = jnp.zeros((acc_scr.shape[0] - S, M), F32)
    x_ref[S:, :] = jnp.zeros((x_ref.shape[0] - S, M), BF16)
    cp_wk.wait()
    cp_wv.wait()
    cp_c[0].wait()
    kick()
    wk = stash(_pair_weights(wk_buf), 0)
    wvT = stash(_pair_weights(wv_buf, True), 14)
    kv_pairs(_Jobs(), 0, CP)
    for chunks in ((1,), (2, 3)):
        for i in chunks:
            cp_c[i].wait()
        kick()
        kv_pairs(_Jobs(), chunks[0] * CP, min((chunks[-1] + 1) * CP, npair - KVL - KVM))
    cp_cond.wait()
    cp_wma.wait()
    kick()
    mod = _dot(silu_cond(), wma_ref[...])
    mod_scr[:, 0:M] = mod[:, 0:M]
    mod_scr[:, M:2 * M] = 1.0 + mod[:, M:2 * M]
    kv_pairs(_Jobs(), npair - KVL - KVM, npair - KVL)
    cp_wq.wait()
    qdone = 0
    for chunks in ((0,), (1,), (2, 3)):
        for i in chunks:
            cp_x[i].wait()
        kick()
        jobs = _Jobs()
        if chunks[0] == 0:
            wq = stash(_pair_weights(wq_buf), 28)
            kv_pairs(jobs, npair - KVL, npair)
        for p in range(chunks[0] * CP, (chunks[-1] + 1) * CP):
            ln_pair(p)
        qend = npair if chunks[-1] == NX - 1 else (chunks[-1] + 1) * CP - QLAG
        for p in range(qdone, qend):
            _q_jobs(jobs, p, h_scr, wq, q_scr, scale)
        qdone = max(qdone, qend)
    assert not named
    ocopy(0, 0).wait()
    for cp in cp_late[1:] + cp_late[:1]:
        cp.start()

    FH = ws3.shape[0] * T

    def mixer_prep(g):
        def blocks(w_ref, r0, n, half, c0, c1, dep):
            lo, hi = pl.ds(r0, n), pl.ds(r0 + half, n)
            b = [w_ref[rows, _tile(c)].astype(F32) for rows in (lo, hi) for c in (c0, c1)]
            return [_after(b[0], _rows(dep, n))] + b[1:]

        def rows_item(w_ref, dst, n, half):
            def item(dep):
                r0 = pl.multiple_of(jnp.minimum(g, half // n - 1) * n, n)
                for c in range(2):
                    for i, v in enumerate(_b_ops(*blocks(w_ref, r0, n, half, c, c + 2, dep))):
                        dst[i, c, pl.ds(pl.multiple_of(r0 // 2, n // 2), n // 2), :] = _pk(v.astype(BF16))
            return item

        def w3_item(k):
            def item(dep):
                n = jnp.minimum(g, FH // T - 1)
                b11, b21, b12, b22 = blocks(w3_ref, pl.multiple_of(n * T, T), T, FH, k, k + 2, dep)
                for i, v in enumerate(_b_ops(b11, b12, b21, b22)):
                    ws3[n, i, k] = _pk(v.astype(BF16).T)
            return item

        return [rows_item(w1_ref, ws12.at[0], 32, 2 * T), rows_item(w2_ref, ws12.at[1], 32, 2 * T),
                rows_item(w4_ref, ws4, 64, FH), w3_item(0), w3_item(1)]

    def attn_body(g, carry):
        slot = g & 1
        nxt = jnp.minimum(g + 1, nattn - 1)
        copies = pcopies(nxt) + [ocopy(nxt, 1 - slot)]

        def mid():
            for cp in copies:
                cp.start()

        _attention_step(q_scr, k_scr, v_scr, wo_buf.at[slot], acc_scr, mid)
        for cp in copies:
            cp.wait()

        @pl.when(g == 0)
        def _():
            for cp in cp_late[1:]:
                cp.wait()

        @pl.when(g + 1 < nattn)
        def _():
            _proj_step(h_scr, cs_scr, wq_buf, wk_buf, wv_buf, q_scr, k_scr, v_scr, scale, mixer_prep(g))

        return carry

    jax.lax.fori_loop(0, nattn, attn_body, 0)

    cp_late[0].wait()
    mod = _dot(silu_cond(), wmb_ref[...])
    mod_scr[:, 2 * M:4 * M] = mod[:, 0:2 * M]
    mod_scr[:, 4 * M:5 * M] = 1.0 + mod[:, 2 * M:3 * M]
    mod_scr[:, 5 * M:6 * M] = mod[:, 3 * M:4 * M]
    ftiles = [(f, min(f + T, Fd)) for f in range(0, Fd, T)]
    OFF = x_ref.shape[0] - S
    CAR = t_scr.shape[0] - RB

    def p1(r0, n, dep=None):
        ga = mod_scr[:, 2 * M:3 * M]
        if dep is not None:
            ga = jnp.concatenate([_after(ga[:, 0:T], dep), ga[:, T:]], axis=1)
        rows = pl.ds(r0, n)
        x1 = x_ref[rows, :].astype(F32) + _rows(ga, n) * acc_scr[rows, :]
        x1_scr[rows, :] = x1
        hb = _ln(x1) * _rows(mod_scr[:, 4 * M:5 * M], n) + _rows(mod_scr[:, 3 * M:4 * M], n)
        hb_scr[rows, :] = hb
        return _ln(hb)

    HT = T // 2
    SUMS = (0, 1, 4, 5, 6)

    def p1_store(r0, c, dep=None):
        n = PC // 2
        hf, o = divmod(c * n, HT)
        top, bot = [p1(r0 + hf * T + d + o, n, dep) for d in (0, HT)]
        for d, v in ((0, top), (HT, bot)):
            for j in range(km):
                a1_scr[j, hf * T + d + o:hf * T + d + o + n, :] = v[:, _tile(j)].astype(BF16)
        ops = _a_ops(top[:, 0:2 * T], top[:, 2 * T:4 * T], bot[:, 0:2 * T], bot[:, 2 * T:4 * T])
        for i, m in enumerate(SUMS):
            for k in range(2):
                a1s_scr[hf, i, k, o:o + n, :] = ops[m][:, _tile(k)].astype(BF16)
        return jnp.max(ops[0][:, :T].reshape(n // 8, 8, T), axis=0)

    t_scr[RB:RB + CAR - OFF, :] = jnp.zeros((CAR - OFF, M), F32)
    t_scr[RB + CAR - OFF:RB + CAR, :] = _gelu(_dot(p1(0, OFF).astype(BF16), w1_ref[...]))
    for c in range(RB // PC):
        p1_store(OFF, c)

    def out_copy(i):
        rows = pl.ds(i * T if isinstance(i, int) else pl.multiple_of(i * T, T), T)
        return pltpu.make_async_copy(out_buf.at[rows, :], out_hbm.at[rows, :], osem.at[i])

    def b_body(r, carry):
        gb = _rows(mod_scr[:, 5 * M:6 * M], T)
        r0 = pl.multiple_of(r * RB, RB)
        n0 = pl.multiple_of(jnp.minimum(r0 + RB, S - RB) + OFF, OFF)
        nh = RB // T
        now = [0]
        due = []
        pace = [(P0 + i * PSTEP, i) for i in range(RB // PC)]

        def mm(lhs, wt, dot=_dot):
            acc = None
            for x, w in zip(lhs, wt):
                if due and due[0][0] <= now[0]:
                    w = _tie(w, due.pop(0)[1])
                v = dot(x, w)
                now[0] += x.shape[0] // HT
                acc = v if acc is None else v + acc
                if pace and pace[0][0] <= now[0]:
                    due.append((now[0] + PD, p1_store(n0, pace.pop(0)[1], v[0:8, :])))
            return acc

        def split_ops(lo, hi):
            return [v.astype(BF16) for v in _a_ops(lo[:HT], hi[:HT], lo[HT:], hi[HT:])]

        def two_tiles(aops, wsel, rest):
            r_lo = mm(rest[0], rest[1], rest[3])
            r_hi = mm(rest[0], rest[2], rest[3])
            c11, c12, c21, c22 = _strassen(
                lambda i: mm([a[i] for a in aops], [wsel(i, k) for k in range(len(aops))]))
            return (jnp.concatenate([c11, c21], axis=0) + r_lo, jnp.concatenate([c12, c22], axis=0) + r_hi)

        def square(full, aops, w_ref, ws):
            out = {}
            for n in range(2):
                out[n], out[n + 2] = two_tiles(
                    aops, lambda i, k: _ld(ws, i, n, slice(k * HT, (k + 1) * HT)),
                    (full[4:], [w_ref[_tile(4), _tile(n)]], [w_ref[_tile(4), _tile(n + 2)]], _dot))
            out[4] = mm(full, [w_ref[_tile(j), _tile(4)] for j in range(km)])
            return out

        t_scr[0:CAR, :] = t_scr[RB:RB + CAR, :]
        for hf in range(nh):
            full = [a1_scr[j, _tile(hf), :] for j in range(km)]
            aops = []
            for k in range(2):
                ops = {m: a1s_scr[hf, i, k] for i, m in enumerate(SUMS)}
                ops[2], ops[3] = full[k][:HT], full[2 + k][HT:]
                aops.append(ops)
            for n, v in square(full, aops, w1_ref, ws12.at[0]).items():
                t = _gelu(v)
                if hf == nh - 1:
                    t = jnp.concatenate([t[:T - OFF], jnp.where(r < nrb - 1, t[T - OFF:], 0.0)], axis=0)
                t_scr[CAR + hf * T:CAR + (hf + 1) * T, _tile(n)] = t
        cq = M // 4
        shifts = (-1, 1, -2, 2)
        lane = jax.lax.broadcasted_iota(jnp.int32, (T, T), 1)
        y1, a3 = [], []
        for hf in range(nh):
            base = CAR - OFF + hf * T
            sh = []
            for j in range(km):
                g_lo, g_hi = (j * T) // cq, ((j + 1) * T - 1) // cq
                assert g_hi - g_lo <= 1
                v = t_scr[base + shifts[g_lo]:base + shifts[g_lo] + T, _tile(j)]
                if g_hi != g_lo:
                    v2 = t_scr[base + shifts[g_hi]:base + shifts[g_hi] + T, _tile(j)]
                    v = jnp.where(lane < g_hi * cq - j * T, v, v2)
                sh.append(v)
            hs = square([v.astype(BF16) for v in sh], [split_ops(sh[k], sh[2 + k]) for k in range(2)],
                        w2_ref, ws12.at[1])
            hs = jnp.concatenate([hs[n] for n in range(km)], axis=1)
            y1.append(hs + hb_scr[pl.ds(pl.multiple_of(r0 + hf * T, T), T), :])
            a3.append(_ln(y1[hf]))
        nf = FH // T
        h3, h3ops = [], []
        for hf in range(nh):
            full = [a3[hf][:, _tile(j)].astype(BF16) for j in range(km)]
            aops = [split_ops(a3[hf][:, _tile(k)], a3[hf][:, _tile(2 + k)]) for k in range(2)]
            row, ops = {}, []
            narrow = None
            for n in range(nf):
                lo, hi = two_tiles(aops, lambda i, k: _ld(ws3, n, i, k),
                                   (full[4:], [w3_ref[_tile(n), _tile(4)]], [w3_ref[_tile(nf + n), _tile(4)]],
                                    _dot_nt))
                lo, hi = _gelu(lo), _gelu(hi)
                row[n], row[nf + n] = lo.astype(BF16), hi.astype(BF16)
                ops.append(split_ops(lo, hi))
                if n < km:
                    v = mm([w3_ref[ftiles[-1][0]:Fd, _tile(n)]], [full[n]], _dot_nt)
                    narrow = v if narrow is None else v + narrow
            row[2 * nf] = _gelu(mm(full, [w3_ref[_tile(2 * nf), _tile(j)] for j in range(km)],
                                   _dot_nt)).astype(BF16)
            fw = Fd - ftiles[-1][0]
            gT = jnp.concatenate([_gelu(narrow), jnp.zeros((T - fw, T), F32)], axis=0)
            row[2 * nf + 1] = _tie(gT.astype(BF16).T, gT[0:8, :])[:, :fw]
            h3.append([row[i] for i in range(len(ftiles))])
            h3ops.append(ops)
        for hf in range(nh):
            rows = pl.ds(pl.multiple_of(r0 + hf * T, T), T)

            def finish(n, v):
                out_buf[rows, _tile(n)] = (
                    x1_scr[rows, _tile(n)] + gb[:, _tile(n)] * (v + y1[hf][:, _tile(n)])
                ).astype(out_buf.dtype)

            w4t = lambda n, f_: [w4_ref[f0:f1, _tile(n)] for f0, f1 in f_]
            finish(4, mm(h3[hf], w4t(4, ftiles)))
            for n in range(2):
                lo, hi = two_tiles(h3ops[hf], lambda i, k: _ld(ws4, i, n, slice(k * HT, (k + 1) * HT)),
                                   (h3[hf][2 * nf:], w4t(n, ftiles[2 * nf:]), w4t(n + 2, ftiles[2 * nf:]), _dot))
                finish(n, lo)
                finish(n + 2, hi)
            out_copy(r * nh + hf).start()
        assert not pace
        return carry

    jax.lax.fori_loop(0, nrb, b_body, 0)
    for i in range(nb):
        out_copy(i).wait()


@jax.jit
def pallas_adaLN_cond__compressed_kv_cla__mixer_s_mlp__prompt_kernel(
    A_x: jax.Array,
    A_c_kv: jax.Array,
    A_w_q: jax.Array,
    A_w_uk: jax.Array,
    A_w_uv: jax.Array,
    A_w_o: jax.Array,
    B_x: jax.Array,
    B_w1: jax.Array,
    B_w2: jax.Array,
    B_w3: jax.Array,
    B_w4: jax.Array,
    c: jax.Array,
    w_mod: jax.Array,
):
    _, S, M = A_x.shape
    Dc = A_c_kv.shape[2]
    H, D = A_w_q.shape[1], A_w_q.shape[2]
    Fd = B_w3.shape[1]
    assert D == T and A_c_kv.shape[1] == S and Dc == 4 * T and M == 5 * T and 13 * T < Fd < 14 * T
    vmem = pltpu.VMEM
    packed = lambda *lead: vmem(lead + (T // 2, T), U32)
    out = pl.pallas_call(
        _kernel,
        in_specs=[pl.BlockSpec(memory_space=pltpu.HBM)] * 12,
        out_specs=pl.BlockSpec(memory_space=pltpu.HBM),
        out_shape=jax.ShapeDtypeStruct((S, M), A_x.dtype),
        scratch_shapes=[
            vmem((S + 16, M), BF16),
            vmem((S, Dc), BF16),
            vmem((1, M), BF16),
            vmem((M, 2 * M), BF16),
            vmem((M, 4 * M), BF16),
            vmem((M, M), BF16),
            vmem((M, M), BF16),
            vmem((Fd, M), BF16),
            vmem((Fd, M), BF16),
            vmem((M, D), U32),
            vmem((Dc, D), U32),
            vmem((Dc, D), U32),
            vmem((2, 2 * D, M), BF16),
            vmem((S, M), A_x.dtype),
            pltpu.SemaphoreType.DMA((15,)),
            pltpu.SemaphoreType.DMA((4,)),
            pltpu.SemaphoreType.DMA((S // T,)),
            vmem((8, 6 * M), F32),
            vmem((S // T // 2, 16, T, T), BF16),
            vmem((S // T // 2, 14, T, T), BF16),
            packed(44),
            packed(2 * S // T),
            packed(2 * S // T),
            packed(2 * S // T),
            vmem((S + 16, M), F32),
            vmem((S + 16, M), F32),
            vmem((S + 16, M), F32),
            vmem((M // T, RB, T), BF16),
            vmem((RB + 32, M), F32),
            vmem((RB // T, 5, 2, T // 2, T), BF16),
            vmem((2, 7, 2, T, T), U32),
            packed(6, 7, 2),
            vmem((7, 2, 3 * T, T), U32),
        ],
        compiler_params=pltpu.CompilerParams(
            vmem_limit_bytes=100 * 1024 * 1024,
            disable_bounds_checks=True,
        ),
    )(
        A_x.reshape(S, M), A_c_kv.reshape(S, Dc),
        A_w_q, A_w_uk, A_w_uv,
        A_w_o.reshape(H // 2, 2 * D, M),
        B_w1, B_w2, B_w3.T, B_w4, c, w_mod,
    )
    return out.reshape(1, S, M)
```

```python
import math
import os

import jax
import jax.numpy as jnp
import jax.experimental.pallas as pl
import jax.experimental.pallas.tpu as pltpu

F32 = jnp.float32
BF16 = jnp.bfloat16
U32 = jnp.uint32
NT = (((1,), (1,)), ((), ()))
T = 128
EPS = 1e-5
LOG2E = math.log2(math.e)

GRP = int(os.environ.get('GRP', 4))
LEAD = int(os.environ.get('LEAD', 10))
PROW = int(os.environ.get('PROW', 3))
VT = 8
RES = int(os.environ.get('RES', 30))
LAT_A = int(os.environ.get('LAT_A', 16))
LAT_B = int(os.environ.get('LAT_B', 20))
ALEAD = int(os.environ.get('ALEAD', 32))
MID = int(os.environ.get('MID', 40))
NOCSE = int(os.environ.get('NOCSE', 1))
NLN = int(os.environ.get('NLN', 4))
LN0 = int(os.environ.get('LN0', 4))
LNS = int(os.environ.get('LNS', 5))
SD0 = int(os.environ.get('SD0', 50))
SDS = int(os.environ.get('SDS', 10))
TIEALL = int(os.environ.get('TIEALL', 0))
FINE = int(os.environ.get('FINE', 0))
OGRP = int(os.environ.get('OGRP', 6))
RB = 256
PC = 32
P0, PSTEP, PD = [int(os.environ.get(k_, d_)) for k_, d_ in (('P0', 400), ('PSTEP', 30), ('PD', 56))]
LP = int(os.environ.get('LP', 16))
KVM, KVL, QLAG = [int(os.environ.get(k_, 1)) for k_ in ('KVM', 'KVL', 'QLAG')]
PLAN = os.environ.get('PLAN', 'kva,b,cdn,m,qw,x,yzo')


def _dot(a, b):
    return jnp.dot(a, b, preferred_element_type=F32)


def _dot_nt(a, b):
    return jax.lax.dot_general(a, b, NT, preferred_element_type=F32)


def _ln(x):
    m = jnp.mean(x, axis=-1, keepdims=True)
    xc = x - m
    v = jnp.mean(xc * xc, axis=-1, keepdims=True)
    return xc * jnp.exp2(jnp.log(v + EPS) * (-0.5 * LOG2E))


def _rows(v, n):
    return jnp.broadcast_to(v[None], (n // 8, 8, v.shape[1])).reshape(n, v.shape[1])


def _gelu(x):
    c0 = math.sqrt(2.0 / math.pi)
    return 0.5 * x * (1.0 + jnp.tanh(c0 * (x + 0.044715 * (x * x * x))))


def _after(x, dep):
    return jnp.where(dep > jnp.inf, dep, x)


def _tie(x, dep):
    xu = pltpu.bitcast(x, U32)
    first = jnp.where(dep > jnp.inf, jnp.uint32(0), xu[:8])
    return pltpu.bitcast(jnp.concatenate([first, xu[8:]], axis=0), BF16)


def _tile(j):
    return slice(j * T, (j + 1) * T)


def _ld(ref, *idx):
    return pltpu.bitcast(ref[idx], BF16)


def _pk(x):
    return pltpu.bitcast(x, U32)


def _a_ops(a11, a12, a21, a22):
    return [a11 + a22, a21 + a22, a11, a22, a11 + a12, a21 - a11, a12 - a22]


def _b_ops(b11, b12, b21, b22):
    return [b11 + b22, b11, b12 - b22, b21 - b11, b22, b11 + b12, b21 + b22]


def _strassen(prod, col1=None, col2=None):
    m4 = prod(3)
    m2 = prod(1)
    c21 = m2 + m4
    if col1 is not None:
        e11, e21 = col1()
        m4, c21 = m4 + e11, c21 + e21
    m3 = prod(2)
    m5 = prod(4)
    c12 = m3 + m5
    if col2 is not None:
        e12, e22 = col2()
        c12, m3 = c12 + e12, m3 + e22
    m1 = prod(0)
    c11 = prod(6) + (m1 + (m4 - m5))
    c22 = prod(5) + (m1 + (m3 - m2))
    return c11, c12, c21, c22


def _pair_weights(w_ref, transpose=False):
    lo, hi = [], []
    for j in range(w_ref.shape[0] // T):
        wu = w_ref[_tile(j), :]
        lo.append(pltpu.bitcast(wu << 16, F32))
        hi.append(pltpu.bitcast(wu & jnp.uint32(0xFFFF0000), F32))
    per_j = [_b_ops(lo[j], hi[j], lo[2 + j], hi[2 + j]) for j in range(2)]
    tiles = [per_j[j][i] for i in range(7) for j in range(2)]
    for j in range(4, len(lo)):
        tiles += [lo[j], hi[j]]
    tiles = [t.astype(BF16) for t in tiles]
    return [t.T for t in tiles] if transpose else tiles


class _Jobs:
    def __init__(self, side=()):
        self.res = []
        self.side = list(side)

    def mm(self, lhs, wt, dot, tie=False):
        acc = None
        for x, w in zip(lhs, wt):
            if tie and len(self.res) >= VT:
                x = _tie(x, self.res[len(self.res) - VT][0:8, :])
            v = dot(x, w)
            self.res.append(v)
            acc = v if acc is None else v + acc
            if self.side and len(self.res) >= SD0 and (len(self.res) - SD0) % SDS == 0:
                self.side.pop(0)(v[0:8, :])
        return acc


def _kv_jobs(jobs, p, cs_scr, wk, wvT, k_scr, v_scr):
    ct = lambda i: [cs_scr[p, 2 * i + j] for j in range(2)]
    ks = _strassen(lambda i: jobs.mm(ct(i), [wk(2 * i), wk(2 * i + 1)], _dot))
    for n, v in enumerate(ks):
        k_scr[4 * p + n] = _pk(v.astype(BF16))
    vs = _strassen(lambda i: jobs.mm([wvT(2 * i), wvT(2 * i + 1)], ct(i), _dot_nt, True))
    for n, v in enumerate(vs):
        v_scr[4 * p + n] = _pk(v.astype(BF16))


def _q_jobs(jobs, p, h_scr, wq, q_scr, scale):
    rest = lambda hd: (lambda: [jobs.mm([h_scr[p, 14 + x]], [wq(14 + hd)], _dot) for x in range(2)])
    if not jobs.res:
        early = [rest(hd)() for hd in range(2)]
        rest = lambda hd: (lambda: early[hd])
    qs = _strassen(lambda i: jobs.mm([h_scr[p, 2 * i + j] for j in range(2)],
                                     [wq(2 * i), wq(2 * i + 1)], _dot), rest(0), rest(1))
    for n, v in enumerate(qs):
        q_scr[4 * p + n] = _pk((v * scale).astype(BF16))


def _proj_step(h_scr, cs_scr, wq_ref, wuk_ref, wuv_ref, q_scr, k_scr, v_scr, scale, side):
    wq = _pair_weights(wq_ref)
    wk = _pair_weights(wuk_ref)
    wvT = _pair_weights(wuv_ref, True)
    jobs = _Jobs(side)
    for p in range(h_scr.shape[0]):
        _q_jobs(jobs, p, h_scr, wq.__getitem__, q_scr, scale)
        _kv_jobs(jobs, p, cs_scr, wk.__getitem__, wvT.__getitem__, k_scr, v_scr)
    assert not jobs.side


_O_JOBS = ([(0, 'r', 0, 0), (0, 'm', 2, 0), (0, 'm', 2, 1), (1, 'r', 1, 0), (1, 'm', 4, 0), (1, 'm', 4, 1),
            (2, 'r', 2, 0), (2, 'm', 5, 0), (2, 'm', 5, 1), (3, 'r', 3, 0)]
           + [(3, 'm', i, n) for n in range(2) for i in (3, 1, 0, 6)])


def _job_order(nb):
    units = range(2 * nb)
    qa = [('a', u, c) for u in units for c in range(u // 2 + 1)]
    qb = [('b', u, c) for u in units for c in range(u // 2 + 1)]
    last = nb // 2 - 1
    qo = [('o', 4 * p + (job[0] if FINE or p == last else 3), j)
          for p in range(nb // 2) for j, job in enumerate(_O_JOBS)]
    done = {}
    order = []

    def ready(q, lat, pre):
        return bool(q) and (pre, q[0][1]) in done and done[(pre, q[0][1])] + lat <= len(order)

    def emit(q):
        kind, u, j = job = q.pop(0)
        if kind != 'o' and j == u // 2:
            done[(kind, u)] = len(order)
        order.append(job)

    turn = 0
    while qa or qb or qo:
        pref = 'abo'[turn % 3]
        turn += 1
        for _ in range(OGRP if pref == 'o' else GRP):
            b_ok, o_ok = ready(qb, LAT_A, 'a'), ready(qo, LAT_B, 'b')
            if pref == 'a' and qa and (len(qb) - len(qa) < ALEAD or not b_ok):
                emit(qa)
            elif pref == 'b' and b_ok:
                emit(qb)
            elif pref == 'o' and o_ok and (len(qo) > RES or not (qa or b_ok)):
                emit(qo)
            elif not (qa or b_ok or o_ok) and (qb or qo):
                emit(qb or qo)
            else:
                break
    return order


def _attention_step(q_scr, k_scr, v_scr, wo_ref, acc_scr, mid):
    causal = (jax.lax.broadcasted_iota(jnp.int32, (T, T), 0)
              <= jax.lax.broadcasted_iota(jnp.int32, (T, T), 1))
    sv, mx, mfin, lsum, pv, of, lhs, prod = {}, {}, {}, {}, {}, {}, {}, {}
    res = []
    wo = [[t.astype(BF16) for t in _b_ops(*[wo_ref[_tile(i // 2), _tile(2 * n + i % 2)].astype(F32)
                                            for i in range(4)])] for n in range(2)]

    def job_a(u, c):
        r, hd = divmod(u, 2)
        s = _dot_nt(_ld(k_scr, 2 * c + hd), _ld(q_scr, u))
        res.append(s)
        if c == r:
            s = jnp.where(causal, s, -1e9 * LOG2E)
        s = s.reshape(T // 8, 8, T)
        sv[(u, c)] = s
        pm = jnp.max(s, axis=0)
        mx[u] = pm if u not in mx else jnp.maximum(mx[u], pm)

    def job_b(u, c):
        r, hd = divmod(u, 2)
        if u not in mfin:
            mfin[u] = jnp.broadcast_to(jnp.max(mx[u], axis=0, keepdims=True), (8, T))
        m = mfin[u]
        if len(res) >= LEAD:
            r0 = 8 * PROW * (c % 4)
            m = _after(m, res[len(res) - LEAD][r0:r0 + 8, :])
        p = jnp.exp2(sv.pop((u, c)) - m[None])
        ls = jnp.sum(p, axis=0)
        lsum[u] = ls if u not in lsum else lsum[u] + ls
        v = _dot(_ld(v_scr, 2 * c + hd), p.reshape(T, T).astype(BF16))
        res.append(v)
        pv[u] = v if u not in pv else v + pv[u]
        if c == r:
            of[u] = pv[u] * (1.0 / jnp.sum(lsum[u], axis=0, keepdims=True))

    def o_lhs(p, kind, i):
        if kind == 'm' and i in (2, 3):
            kind, i = 'r', 3 * (i - 2)
        if (p, kind, i) not in lhs:
            a = lambda n: of[4 * p + n]
            v = a(i) if kind == 'r' else {0: lambda: a(0) + a(3), 1: lambda: a(2) + a(3), 4: lambda: a(0) + a(1),
                                          5: lambda: a(2) - a(0), 6: lambda: a(1) - a(3)}[i]()
            lhs[(p, kind, i)] = _tie(v.astype(BF16).T, v[0:8, :])
        return lhs[(p, kind, i)]

    def job_o(u, j):
        p = u // 4
        _, kind, i, n = _O_JOBS[j]
        w = wo[n][i] if kind == 'm' else wo_ref[_tile(i % 2), _tile(4)]
        v = _dot(o_lhs(p, kind, i), w)
        res.append(v)
        prod[(kind, i, n)] = v
        m = lambda i_: prod[('m', i_, n)]
        if kind == 'r':
            if i % 2:
                acc_scr[_tile(2 * p + i // 2), _tile(4)] += v + prod[('r', i - 1, 0)]
        elif i == 4:
            acc_scr[_tile(2 * p), _tile(2 * n + 1)] += v + m(2)
        elif i == 5:
            prod[('m', 5, n)] = v + m(2)
        elif i == 1:
            acc_scr[_tile(2 * p + 1), _tile(2 * n)] += v + m(3)
        elif i == 0:
            acc_scr[_tile(2 * p + 1), _tile(2 * n + 1)] += v + (m(5) - m(1))
        elif i == 6:
            acc_scr[_tile(2 * p), _tile(2 * n)] += v + (m(0) + (m(3) - m(4)))

    fns = dict(a=job_a, b=job_b, o=job_o)
    for n, (kind, u, j) in enumerate(_job_order(q_scr.shape[0] // 2)):
        if n == MID:
            mid()
        fns[kind](u, j)


def _kernel(x_hbm, c_hbm, wq_hbm, wuk_hbm, wuv_hbm, wo_hbm, w1_hbm, w2_hbm, w3_hbm, w4_hbm,
            cond_hbm, wmod_hbm, out_hbm,
            x_ref, c_ref, cond_ref, wma_ref, wmb_ref, w1_ref, w2_ref, w3_ref, w4_ref,
            wq_buf, wk_buf, wv_buf, wo_buf, out_buf, sem, wsem, osem,
            mod_scr, h_scr, cs_scr, w_scr, q_scr, k_scr, v_scr, acc_scr, x1_scr, hb_scr, a1_scr, t_scr,
            a1s_scr, ws12, ws3, ws4):
    S, M = x_hbm.shape
    D = wq_hbm.shape[2]
    nattn = wo_hbm.shape[0]
    Fd = w4_hbm.shape[0]
    scale = float(D) ** -0.5 * LOG2E
    nb, nrb = S // T, S // RB
    km, kc = M // T, c_hbm.shape[1] // T
    NX = 4
    XR = S // NX
    CB = XR // T

    def pcopies(g):
        return [pltpu.make_async_copy(src.bitcast(U32).at[:, g, :], dst, wsem.at[j])
                for j, (src, dst) in enumerate(((wuk_hbm, wk_buf), (wuv_hbm, wv_buf), (wq_hbm, wq_buf)))]

    def ocopy(g, slot):
        return pltpu.make_async_copy(wo_hbm.at[g], wo_buf.at[slot], wsem.at[3])

    def chunk_copy(src, dst, i, s0):
        rows = slice(i * XR, (i + 1) * XR)
        return pltpu.make_async_copy(src.at[rows, :], dst.at[rows, :], sem.at[s0 + i])

    cp_cond = pltpu.make_async_copy(cond_hbm, cond_ref, sem.at[0])
    cp_wma = pltpu.make_async_copy(wmod_hbm.at[:, 0:2 * M], wma_ref, sem.at[1])
    cp_late = [pltpu.make_async_copy(src, dst, sem.at[2 + j]) for j, (src, dst) in enumerate((
        (wmod_hbm.at[:, 2 * M:6 * M], wmb_ref), (w1_hbm, w1_ref), (w2_hbm, w2_ref),
        (w3_hbm, w3_ref), (w4_hbm, w4_ref)))]
    cp_x = [chunk_copy(x_hbm, x_ref, i, 7) for i in range(NX)]
    cp_c = [chunk_copy(c_hbm, c_ref, i, 7 + NX) for i in range(NX)]

    def silu_cond():
        cf = cond_ref[...].astype(F32)
        return jnp.broadcast_to((cf * jax.nn.sigmoid(cf)).astype(BF16), (8, M))

    cp_wk, cp_wv, cp_wq = pcopies(0)
    named = dict(k=cp_wk, v=cp_wv, q=cp_wq, o=ocopy(0, 0), n=cp_cond, m=cp_wma)
    named.update(zip('abcd', cp_c))
    named.update(zip('wxyz', cp_x))
    plan = PLAN.split(',')

    def kick():
        for ch in plan.pop(0) if plan else '':
            named.pop(ch).start()

    def zero(r, carry):
        acc_scr[pl.ds(pl.multiple_of(r * T, T), T), :] = jnp.zeros((T, M), F32)
        return carry

    def ln_pair(p):
        sa = _rows(mod_scr[:, 0:M], LP)
        ca1 = _rows(mod_scr[:, M:2 * M], LP)
        for i in range(T // LP):
            h1, h2 = [_ln(x_ref[r * T + i * LP:r * T + (i + 1) * LP, :].astype(F32)) * ca1 + sa
                      for r in (2 * p, 2 * p + 1)]
            ops = _a_ops(h1[:, 0:2 * T], h1[:, 2 * T:4 * T], h2[:, 0:2 * T], h2[:, 2 * T:4 * T])
            tiles = [v[:, _tile(j)] for v in ops for j in range(2)] + [h1[:, _tile(4)], h2[:, _tile(4)]]
            for n, v in enumerate(tiles):
                h_scr[p, n, i * LP:(i + 1) * LP, :] = v.astype(BF16)

    def stash(tiles, j0):
        for j, t in enumerate(tiles):
            w_scr[j0 + j] = _pk(t)
        return lambda j: _ld(w_scr, j0 + j)

    def kv_pairs(jobs, p0, p1_):
        for p in range(p0, p1_):
            for j in range(2):
                ops = _a_ops(*[c_ref[_tile(2 * p + n // 2), _tile(2 * (n % 2) + j)].astype(F32)
                               for n in range(4)])
                for i, v in enumerate(ops):
                    cs_scr[p, 2 * i + j] = v.astype(BF16)
            _kv_jobs(jobs, p, cs_scr, wk, wvT, k_scr, v_scr)

    npair, CP = nb // 2, CB // 2
    kick()
    jax.lax.fori_loop(0, nb, zero, 0)
    kick()
    acc_scr[S:, :] = jnp.zeros((acc_scr.shape[0] - S, M), F32)
    x_ref[S:, :] = jnp.zeros((x_ref.shape[0] - S, M), BF16)
    cp_wk.wait()
    cp_wv.wait()
    cp_c[0].wait()
    kick()
    wk = stash(_pair_weights(wk_buf), 0)
    wvT = stash(_pair_weights(wv_buf, True), 14)
    kv_pairs(_Jobs(), 0, CP)
    for chunks in ((1,), (2, 3)):
        for i in chunks:
            cp_c[i].wait()
        kick()
        kv_pairs(_Jobs(), chunks[0] * CP, min((chunks[-1] + 1) * CP, npair - KVL - KVM))
    cp_cond.wait()
    cp_wma.wait()
    kick()
    mod = _dot(silu_cond(), wma_ref[...])
    mod_scr[:, 0:M] = mod[:, 0:M]
    mod_scr[:, M:2 * M] = 1.0 + mod[:, M:2 * M]
    kv_pairs(_Jobs(), npair - KVL - KVM, npair - KVL)
    cp_wq.wait()
    qdone = 0
    for chunks in ((0,), (1,), (2, 3)):
        for i in chunks:
            cp_x[i].wait()
        kick()
        jobs = _Jobs()
        if chunks[0] == 0:
            wq = stash(_pair_weights(wq_buf), 28)
            kv_pairs(jobs, npair - KVL, npair)
        for p in range(chunks[0] * CP, (chunks[-1] + 1) * CP):
            ln_pair(p)
        qend = npair if chunks[-1] == NX - 1 else (chunks[-1] + 1) * CP - QLAG
        for p in range(qdone, qend):
            _q_jobs(jobs, p, h_scr, wq, q_scr, scale)
        qdone = max(qdone, qend)
    assert not named
    ocopy(0, 0).wait()
    for cp in cp_late[1:] + cp_late[:1]:
        cp.start()

    FH = ws3.shape[0] * T

    def mixer_prep(g):
        def blocks(w_ref, r0, n, half, c0, c1, dep):
            lo, hi = pl.ds(r0, n), pl.ds(r0 + half, n)
            return [_after(w_ref[rows, _tile(c)].astype(F32), _rows(dep, n)) if TIEALL or (rows is lo) == (c == c0)
                    else w_ref[rows, _tile(c)].astype(F32) for rows in (lo, hi) for c in (c0, c1)]

        def rows_items(w_ref, dst, per_step, half, n=16):
            gi = jnp.minimum(g, half // per_step - 1)
            src = w_ref.at[pl.ds(pl.multiple_of(gi * per_step, per_step), half + per_step), :]
            hs = per_step // 2

            def item(c, o):
                def fn(dep):
                    for i, v in enumerate(_b_ops(*blocks(src, o, n, half, c, c + 2, dep))):
                        dst[i, c, pl.ds(pl.multiple_of(gi * hs, hs) + o // 2, n // 2), :] = _pk(v.astype(BF16))
                return fn
            return [item(c, o) for c in range(2) for o in range(0, per_step, n)]

        def w3_item(k, i):
            def fn(dep):
                n = jnp.minimum(g, FH // T - 1)
                b11, b21, b12, b22 = blocks(w3_ref, pl.multiple_of(n * T, T), T, FH, k, k + 2, dep)
                ws3[n, i, k] = _pk(_b_ops(b11, b12, b21, b22)[i].astype(BF16).T)
            return fn

        return (rows_items(w1_ref, ws12.at[0], 32, 2 * T) + rows_items(w2_ref, ws12.at[1], 32, 2 * T)
                + rows_items(w4_ref, ws4, 64, FH) + [w3_item(k, i) for k in range(2) for i in range(7)])

    def attn_body(g, carry):
        slot = g & 1
        nxt = jnp.minimum(g + 1, nattn - 1)
        copies = pcopies(nxt) + [ocopy(nxt, 1 - slot)]

        def mid():
            for cp in copies:
                cp.start()

        _attention_step(q_scr, k_scr, v_scr, wo_buf.at[slot], acc_scr, mid)
        for cp in copies:
            cp.wait()

        @pl.when(g == 0)
        def _():
            for cp in cp_late[1:]:
                cp.wait()

        @pl.when(g + 1 < nattn)
        def _():
            _proj_step(h_scr, cs_scr, wq_buf, wk_buf, wv_buf, q_scr, k_scr, v_scr, scale, mixer_prep(g))

        return carry

    jax.lax.fori_loop(0, nattn, attn_body, 0)

    cp_late[0].wait()
    mod = _dot(silu_cond(), wmb_ref[...])
    mod_scr[:, 2 * M:4 * M] = mod[:, 0:2 * M]
    mod_scr[:, 4 * M:5 * M] = 1.0 + mod[:, 2 * M:3 * M]
    mod_scr[:, 5 * M:6 * M] = mod[:, 3 * M:4 * M]
    ftiles = [(f, min(f + T, Fd)) for f in range(0, Fd, T)]
    OFF = x_ref.shape[0] - S
    CAR = t_scr.shape[0] - RB

    def p1(r0, n, dep=None):
        ga = mod_scr[:, 2 * M:3 * M]
        if dep is not None:
            ga = jnp.concatenate([_after(ga[:, 0:T], dep), ga[:, T:]], axis=1)
        rows = pl.ds(r0, n)
        x1 = x_ref[rows, :].astype(F32) + _rows(ga, n) * acc_scr[rows, :]
        x1_scr[rows, :] = x1
        hb = _ln(x1) * _rows(mod_scr[:, 4 * M:5 * M], n) + _rows(mod_scr[:, 3 * M:4 * M], n)
        hb_scr[rows, :] = hb
        return _ln(hb)

    HT = T // 2
    SUMS = (0, 1, 4, 5, 6)

    def p1_store(r0, c, dep=None):
        n = PC // 2
        hf, o = divmod(c * n, HT)
        top, bot = [p1(r0 + hf * T + d + o, n, dep) for d in (0, HT)]
        for d, v in ((0, top), (HT, bot)):
            for j in range(km):
                a1_scr[j, hf * T + d + o:hf * T + d + o + n, :] = v[:, _tile(j)].astype(BF16)
        ops = _a_ops(top[:, 0:2 * T], top[:, 2 * T:4 * T], bot[:, 0:2 * T], bot[:, 2 * T:4 * T])
        for i, m in enumerate(SUMS):
            for k in range(2):
                a1s_scr[hf, i, k, o:o + n, :] = ops[m][:, _tile(k)].astype(BF16)
        return jnp.max(ops[0][:, :T].reshape(n // 8, 8, T), axis=0)

    t_scr[RB:RB + CAR - OFF, :] = jnp.zeros((CAR - OFF, M), F32)
    t_scr[RB + CAR - OFF:RB + CAR, :] = _gelu(_dot(p1(0, OFF).astype(BF16), w1_ref[...]))
    for c in range(RB // PC):
        p1_store(OFF, c)

    def out_copy(i):
        rows = pl.ds(i * T if isinstance(i, int) else pl.multiple_of(i * T, T), T)
        return pltpu.make_async_copy(out_buf.at[rows, :], out_hbm.at[rows, :], osem.at[i])

    def b_body(r, carry):
        gb = _rows(mod_scr[:, 5 * M:6 * M], T)
        r0 = pl.multiple_of(r * RB, RB)
        n0 = pl.multiple_of(jnp.minimum(r0 + RB, S - RB) + OFF, OFF)
        nh = RB // T
        now = [0]
        due = []
        pace = []

        def p1_item(c):
            return lambda dep: due.append((now[0] + PD, p1_store(n0, c, dep)))

        pace += [(P0 + i * PSTEP, p1_item(i)) for i in range(RB // PC)]
        zero = jnp.minimum(r, 0)

        def wt(ref, hf, f0, f1, n):
            rows = slice(f0, f1) if hf == 0 or not NOCSE else pl.ds(pl.multiple_of(zero * 16 + f0, 16), f1 - f0)
            return ref[rows, _tile(n)]

        def ws(ref, hf, i, *idx):
            return _ld(ref, i + zero if hf and NOCSE else i, *idx)

        def mm(lhs, wts, dot=_dot):
            acc = None
            for x, w in zip(lhs, wts):
                if due and due[0][0] <= now[0]:
                    w = _tie(w, due.pop(0)[1])
                v = dot(x, w)
                now[0] += x.shape[0] // HT
                acc = v if acc is None else v + acc
                if pace and pace[0][0] <= now[0]:
                    pace.pop(0)[1](v[0:8, :])
            return acc

        def split_ops(lo, hi):
            return [v.astype(BF16) for v in _a_ops(lo[:HT], hi[:HT], lo[HT:], hi[HT:])]

        def two_tiles(aops, wsel, rest):
            def col(w):
                v = mm(rest[0], w, rest[3])
                return v[:HT], v[HT:]

            c11, c12, c21, c22 = _strassen(
                lambda i: mm([a[i] for a in aops], [wsel(i, k) for k in range(len(aops))]),
                lambda: col(rest[1]), lambda: col(rest[2]))
            return jnp.concatenate([c11, c21], axis=0), jnp.concatenate([c12, c22], axis=0)

        def square(hf, full, aops, w_ref, ws_ref):
            out = {}
            for n in range(2):
                out[n], out[n + 2] = two_tiles(
                    aops, lambda i, k: ws(ws_ref, hf, i, n, slice(k * HT, (k + 1) * HT)),
                    (full[4:], [wt(w_ref, hf, 4 * T, M, n)], [wt(w_ref, hf, 4 * T, M, n + 2)], _dot))
            out[4] = mm(full, [wt(w_ref, hf, j * T, (j + 1) * T, 4) for j in range(km)])
            return out

        t_scr[0:CAR, :] = t_scr[RB:RB + CAR, :]
        for hf in range(nh):
            full = [a1_scr[j, _tile(hf), :] for j in range(km)]
            aops = []
            for k in range(2):
                ops = {m: a1s_scr[hf, i, k] for i, m in enumerate(SUMS)}
                ops[2], ops[3] = full[k][:HT], full[2 + k][HT:]
                aops.append(ops)
            for n, v in square(hf, full, aops, w1_ref, ws12.at[0]).items():
                t = _gelu(v)
                if hf == nh - 1:
                    t = jnp.concatenate([t[:T - OFF], jnp.where(r < nrb - 1, t[T - OFF:], 0.0)], axis=0)
                t_scr[CAR + hf * T:CAR + (hf + 1) * T, _tile(n)] = t
        cq = M // 4
        shifts = (-1, 1, -2, 2)
        lane = jax.lax.broadcasted_iota(jnp.int32, (T, T), 1)
        y1, a3 = [], []
        for hf in range(nh):
            base = CAR - OFF + hf * T
            sh = []
            for j in range(km):
                g_lo, g_hi = (j * T) // cq, ((j + 1) * T - 1) // cq
                assert g_hi - g_lo <= 1
                v = t_scr[base + shifts[g_lo]:base + shifts[g_lo] + T, _tile(j)]
                if g_hi != g_lo:
                    v2 = t_scr[base + shifts[g_hi]:base + shifts[g_hi] + T, _tile(j)]
                    v = jnp.where(lane < g_hi * cq - j * T, v, v2)
                sh.append(v)
            hs = square(hf, [v.astype(BF16) for v in sh], [split_ops(sh[k], sh[2 + k]) for k in range(2)],
                        w2_ref, ws12.at[1])
            hs = jnp.concatenate([hs[n] for n in range(km)], axis=1)
            y1.append(hs + hb_scr[pl.ds(pl.multiple_of(r0 + hf * T, T), T), :])
            a3.append({})

            def ln_item(hf, c):
                def item(dep):
                    n = HT // NLN
                    for d in (0, HT):
                        v = y1[hf][d + c * n:d + (c + 1) * n]
                        if dep is not None:
                            v = jnp.concatenate([_after(v[:, :T], _rows(dep, n)), v[:, T:]], axis=1)
                        a3[hf][d + c * n] = _ln(v)
                return item

            ln_item(hf, 0)(None)
            pace += [(now[0] + LN0 + (c - 1) * LNS * (1 + hf), ln_item(hf, c)) for c in range(1, NLN)]
            pace.sort(key=lambda e: e[0])
        nf = FH // T
        h3, h3ops = [], []
        for hf in range(nh):
            assert len(a3[hf]) == 2 * NLN
            af = jnp.concatenate([a3[hf][key] for key in sorted(a3[hf])], axis=0)
            full = [af[:, _tile(j)].astype(BF16) for j in range(km)]
            aops = [split_ops(af[:, _tile(k)], af[:, _tile(2 + k)]) for k in range(2)]
            row, ops = {}, []
            narrow = None
            for n in range(nf):
                lo, hi = two_tiles(aops, lambda i, k: ws(ws3, hf, n, i, k),
                                   (full[4:], [wt(w3_ref, hf, *ftiles[n], 4)],
                                    [wt(w3_ref, hf, *ftiles[nf + n], 4)], _dot_nt))
                lo, hi = _gelu(lo), _gelu(hi)
                row[n], row[nf + n] = lo.astype(BF16), hi.astype(BF16)
                ops.append(split_ops(lo, hi))
                if n < km:
                    v = mm([wt(w3_ref, hf, *ftiles[-1], n)], [full[n]], _dot_nt)
                    narrow = v if narrow is None else v + narrow
            row[2 * nf] = _gelu(mm(full, [wt(w3_ref, hf, *ftiles[2 * nf], j) for j in range(km)],
                                   _dot_nt)).astype(BF16)
            fw = Fd - ftiles[-1][0]
            gT = jnp.concatenate([_gelu(narrow), jnp.zeros((T - fw, T), F32)], axis=0)
            row[2 * nf + 1] = _tie(gT.astype(BF16).T, gT[0:8, :])[:, :fw]
            h3.append([row[i] for i in range(len(ftiles))])
            h3ops.append(ops)
        for hf in range(nh):
            rows = pl.ds(pl.multiple_of(r0 + hf * T, T), T)

            def finish(n, v):
                out_buf[rows, _tile(n)] = (
                    x1_scr[rows, _tile(n)] + gb[:, _tile(n)] * (v + y1[hf][:, _tile(n)])
                ).astype(out_buf.dtype)

            w4t = lambda n, f_: [wt(w4_ref, hf, f0, f1, n) for f0, f1 in f_]
            finish(4, mm(h3[hf], w4t(4, ftiles)))
            for n in range(2):
                lo, hi = two_tiles(h3ops[hf], lambda i, k: ws(ws4, hf, i, n, slice(k * HT, (k + 1) * HT)),
                                   (h3[hf][2 * nf:], w4t(n, ftiles[2 * nf:]), w4t(n + 2, ftiles[2 * nf:]), _dot))
                finish(n, lo)
                finish(n + 2, hi)
            out_copy(r * nh + hf).start()
        assert not pace
        return carry

    jax.lax.fori_loop(0, nrb, b_body, 0)
    for i in range(nb):
        out_copy(i).wait()


@jax.jit
def pallas_adaLN_cond__compressed_kv_cla__mixer_s_mlp__prompt_kernel(
    A_x: jax.Array,
    A_c_kv: jax.Array,
    A_w_q: jax.Array,
    A_w_uk: jax.Array,
    A_w_uv: jax.Array,
    A_w_o: jax.Array,
    B_x: jax.Array,
    B_w1: jax.Array,
    B_w2: jax.Array,
    B_w3: jax.Array,
    B_w4: jax.Array,
    c: jax.Array,
    w_mod: jax.Array,
):
    _, S, M = A_x.shape
    Dc = A_c_kv.shape[2]
    H, D = A_w_q.shape[1], A_w_q.shape[2]
    Fd = B_w3.shape[1]
    assert D == T and A_c_kv.shape[1] == S and Dc == 4 * T and M == 5 * T and 13 * T < Fd < 14 * T
    vmem = pltpu.VMEM
    packed = lambda *lead: vmem(lead + (T // 2, T), U32)
    out = pl.pallas_call(
        _kernel,
        in_specs=[pl.BlockSpec(memory_space=pltpu.HBM)] * 12,
        out_specs=pl.BlockSpec(memory_space=pltpu.HBM),
        out_shape=jax.ShapeDtypeStruct((S, M), A_x.dtype),
        scratch_shapes=[
            vmem((S + 16, M), BF16),
            vmem((S, Dc), BF16),
            vmem((1, M), BF16),
            vmem((M, 2 * M), BF16),
            vmem((M, 4 * M), BF16),
            vmem((M, M), BF16),
            vmem((M, M), BF16),
            vmem((Fd, M), BF16),
            vmem((Fd, M), BF16),
            vmem((M, D), U32),
            vmem((Dc, D), U32),
            vmem((Dc, D), U32),
            vmem((2, 2 * D, M), BF16),
            vmem((S, M), A_x.dtype),
            pltpu.SemaphoreType.DMA((15,)),
            pltpu.SemaphoreType.DMA((4,)),
            pltpu.SemaphoreType.DMA((S // T,)),
            vmem((8, 6 * M), F32),
            vmem((S // T // 2, 16, T, T), BF16),
            vmem((S // T // 2, 14, T, T), BF16),
            packed(44),
            packed(2 * S // T),
            packed(2 * S // T),
            packed(2 * S // T),
            vmem((S + 16, M), F32),
            vmem((S + 16, M), F32),
            vmem((S + 16, M), F32),
            vmem((M // T, RB, T), BF16),
            vmem((RB + 32, M), F32),
            vmem((RB // T, 5, 2, T // 2, T), BF16),
            vmem((2, 7, 2, T, T), U32),
            packed(6, 7, 2),
            vmem((7, 2, 3 * T, T), U32),
        ],
        compiler_params=pltpu.CompilerParams(
            vmem_limit_bytes=100 * 1024 * 1024,
            disable_bounds_checks=True,
        ),
    )(
        A_x.reshape(S, M), A_c_kv.reshape(S, Dc),
        A_w_q, A_w_uk, A_w_uv,
        A_w_o.reshape(H // 2, 2 * D, M),
        B_w1, B_w2, B_w3.T, B_w4, c, w_mod,
    )
    return out.reshape(1, S, M)
```

```python
import math
import os

import jax
import jax.numpy as jnp
import jax.experimental.pallas as pl
import jax.experimental.pallas.tpu as pltpu

F32 = jnp.float32
BF16 = jnp.bfloat16
U32 = jnp.uint32
NT = (((1,), (1,)), ((), ()))
T = 128
EPS = 1e-5
LOG2E = math.log2(math.e)

GRP = int(os.environ.get('GRP', 4))
LEAD = int(os.environ.get('LEAD', 10))
PROW = int(os.environ.get('PROW', 3))
VT = 8
RES = int(os.environ.get('RES', 30))
LAT_A = int(os.environ.get('LAT_A', 16))
LAT_B = int(os.environ.get('LAT_B', 20))
ALEAD = int(os.environ.get('ALEAD', 32))
MID = int(os.environ.get('MID', 40))
NLN = int(os.environ.get('NLN', 4))
LN0 = int(os.environ.get('LN0', 4))
LNS = int(os.environ.get('LNS', 5))
SD0 = int(os.environ.get('SD0', 50))
SDS = int(os.environ.get('SDS', 10))
FINE = int(os.environ.get('FINE', 0))
OGRP = int(os.environ.get('OGRP', 6))
RB = 256
PC = 32
P0, PSTEP, PD = [int(os.environ.get(k_, d_)) for k_, d_ in (('P0', 400), ('PSTEP', 30), ('PD', 56))]
LP = int(os.environ.get('LP', 16))
KVM, KVL, QLAG = [int(os.environ.get(k_, 1)) for k_ in ('KVM', 'KVL', 'QLAG')]
PLAN = os.environ.get('PLAN', 'kva,b,cdn,m,qw,x,yzo')


def _dot(a, b):
    return jnp.dot(a, b, preferred_element_type=F32)


def _dot_nt(a, b):
    return jax.lax.dot_general(a, b, NT, preferred_element_type=F32)


def _ln(x):
    m = jnp.mean(x, axis=-1, keepdims=True)
    xc = x - m
    v = jnp.mean(xc * xc, axis=-1, keepdims=True)
    return xc * jnp.exp2(jnp.log(v + EPS) * (-0.5 * LOG2E))


def _rows(v, n):
    return jnp.broadcast_to(v[None], (n // 8, 8, v.shape[1])).reshape(n, v.shape[1])


def _gelu(x):
    c0 = math.sqrt(2.0 / math.pi)
    return 0.5 * x * (1.0 + jnp.tanh(c0 * (x + 0.044715 * (x * x * x))))


def _after(x, dep):
    return jnp.where(dep > jnp.inf, dep, x)


def _tie(x, dep):
    xu = pltpu.bitcast(x, U32)
    first = jnp.where(dep > jnp.inf, jnp.uint32(0), xu[:8])
    return pltpu.bitcast(jnp.concatenate([first, xu[8:]], axis=0), BF16)


def _tile(j):
    return slice(j * T, (j + 1) * T)


def _ld(ref, *idx):
    return pltpu.bitcast(ref[idx], BF16)


def _pk(x):
    return pltpu.bitcast(x, U32)


def _a_ops(a11, a12, a21, a22):
    return [a11 + a22, a21 + a22, a11, a22, a11 + a12, a21 - a11, a12 - a22]


def _b_ops(b11, b12, b21, b22):
    return [b11 + b22, b11, b12 - b22, b21 - b11, b22, b11 + b12, b21 + b22]


def _strassen(prod, col1=None, col2=None):
    m4 = prod(3)
    m2 = prod(1)
    c21 = m2 + m4
    if col1 is not None:
        e11, e21 = col1()
        m4, c21 = m4 + e11, c21 + e21
    m3 = prod(2)
    m5 = prod(4)
    c12 = m3 + m5
    if col2 is not None:
        e12, e22 = col2()
        c12, m3 = c12 + e12, m3 + e22
    m1 = prod(0)
    c11 = prod(6) + (m1 + (m4 - m5))
    c22 = prod(5) + (m1 + (m3 - m2))
    return c11, c12, c21, c22


def _pair_weights(w_ref, transpose=False):
    lo, hi = [], []
    for j in range(w_ref.shape[0] // T):
        wu = w_ref[_tile(j), :]
        lo.append(pltpu.bitcast(wu << 16, F32))
        hi.append(pltpu.bitcast(wu & jnp.uint32(0xFFFF0000), F32))
    per_j = [_b_ops(lo[j], hi[j], lo[2 + j], hi[2 + j]) for j in range(2)]
    tiles = [per_j[j][i] for i in range(7) for j in range(2)]
    for j in range(4, len(lo)):
        tiles += [lo[j], hi[j]]
    tiles = [t.astype(BF16) for t in tiles]
    return [t.T for t in tiles] if transpose else tiles


class _Jobs:
    def __init__(self, side=()):
        self.res = []
        self.side = list(side)

    def mm(self, lhs, wt, dot, tie=False):
        acc = None
        for x, w in zip(lhs, wt):
            if tie and len(self.res) >= VT:
                x = _tie(x, self.res[len(self.res) - VT][0:8, :])
            v = dot(x, w)
            self.res.append(v)
            acc = v if acc is None else v + acc
            if self.side and len(self.res) >= SD0 and (len(self.res) - SD0) % SDS == 0:
                self.side.pop(0)(v[0:8, :])
        return acc


def _kv_jobs(jobs, p, cs_scr, wk, wvT, k_scr, v_scr):
    ct = lambda i: [cs_scr[p, 2 * i + j] for j in range(2)]
    ks = _strassen(lambda i: jobs.mm(ct(i), [wk(2 * i), wk(2 * i + 1)], _dot))
    for n, v in enumerate(ks):
        k_scr[4 * p + n] = _pk(v.astype(BF16))
    vs = _strassen(lambda i: jobs.mm([wvT(2 * i), wvT(2 * i + 1)], ct(i), _dot_nt, True))
    for n, v in enumerate(vs):
        v_scr[4 * p + n] = _pk(v.astype(BF16))


def _q_jobs(jobs, p, h_scr, wq, q_scr, scale):
    rest = lambda hd: (lambda: [jobs.mm([h_scr[p, 14 + x]], [wq(14 + hd)], _dot) for x in range(2)])
    if not jobs.res:
        early = [rest(hd)() for hd in range(2)]
        rest = lambda hd: (lambda: early[hd])
    qs = _strassen(lambda i: jobs.mm([h_scr[p, 2 * i + j] for j in range(2)],
                                     [wq(2 * i), wq(2 * i + 1)], _dot), rest(0), rest(1))
    for n, v in enumerate(qs):
        q_scr[4 * p + n] = _pk((v * scale).astype(BF16))


def _proj_step(h_scr, cs_scr, wq_ref, wuk_ref, wuv_ref, q_scr, k_scr, v_scr, scale, side):
    wq = _pair_weights(wq_ref)
    wk = _pair_weights(wuk_ref)
    wvT = _pair_weights(wuv_ref, True)
    jobs = _Jobs(side)
    for p in range(h_scr.shape[0]):
        _q_jobs(jobs, p, h_scr, wq.__getitem__, q_scr, scale)
        _kv_jobs(jobs, p, cs_scr, wk.__getitem__, wvT.__getitem__, k_scr, v_scr)
    assert not jobs.side


_O_JOBS = ([(0, 'r', 0, 0), (0, 'm', 2, 0), (0, 'm', 2, 1), (1, 'r', 1, 0), (1, 'm', 4, 0), (1, 'm', 4, 1),
            (2, 'r', 2, 0), (2, 'm', 5, 0), (2, 'm', 5, 1), (3, 'r', 3, 0)]
           + [(3, 'm', i, n) for n in range(2) for i in (3, 1, 0, 6)])


def _job_order(nb):
    units = range(2 * nb)
    qa = [('a', u, c) for u in units for c in range(u // 2 + 1)]
    qb = [('b', u, c) for u in units for c in range(u // 2 + 1)]
    last = nb // 2 - 1
    qo = [('o', 4 * p + (job[0] if FINE or p == last else 3), j)
          for p in range(nb // 2) for j, job in enumerate(_O_JOBS)]
    done = {}
    order = []

    def ready(q, lat, pre):
        return bool(q) and (pre, q[0][1]) in done and done[(pre, q[0][1])] + lat <= len(order)

    def emit(q):
        kind, u, j = job = q.pop(0)
        if kind != 'o' and j == u // 2:
            done[(kind, u)] = len(order)
        order.append(job)

    turn = 0
    while qa or qb or qo:
        pref = 'abo'[turn % 3]
        turn += 1
        for _ in range(OGRP if pref == 'o' else GRP):
            b_ok, o_ok = ready(qb, LAT_A, 'a'), ready(qo, LAT_B, 'b')
            if pref == 'a' and qa and (len(qb) - len(qa) < ALEAD or not b_ok):
                emit(qa)
            elif pref == 'b' and b_ok:
                emit(qb)
            elif pref == 'o' and o_ok and (len(qo) > RES or not (qa or b_ok)):
                emit(qo)
            elif not (qa or b_ok or o_ok) and (qb or qo):
                emit(qb or qo)
            else:
                break
    return order


def _attention_step(q_scr, k_scr, v_scr, wo_ref, acc_scr, mid):
    causal = (jax.lax.broadcasted_iota(jnp.int32, (T, T), 0)
              <= jax.lax.broadcasted_iota(jnp.int32, (T, T), 1))
    sv, mx, mfin, lsum, pv, of, lhs, prod = {}, {}, {}, {}, {}, {}, {}, {}
    res = []
    wo = [[t.astype(BF16) for t in _b_ops(*[wo_ref[_tile(i // 2), _tile(2 * n + i % 2)].astype(F32)
                                            for i in range(4)])] for n in range(2)]

    def job_a(u, c):
        r, hd = divmod(u, 2)
        s = _dot_nt(_ld(k_scr, 2 * c + hd), _ld(q_scr, u))
        res.append(s)
        if c == r:
            s = jnp.where(causal, s, -1e9 * LOG2E)
        s = s.reshape(T // 8, 8, T)
        sv[(u, c)] = s
        pm = jnp.max(s, axis=0)
        mx[u] = pm if u not in mx else jnp.maximum(mx[u], pm)

    def job_b(u, c):
        r, hd = divmod(u, 2)
        if u not in mfin:
            mfin[u] = jnp.broadcast_to(jnp.max(mx[u], axis=0, keepdims=True), (8, T))
        m = mfin[u]
        if len(res) >= LEAD:
            r0 = 8 * PROW * (c % 4)
            m = _after(m, res[len(res) - LEAD][r0:r0 + 8, :])
        p = jnp.exp2(sv.pop((u, c)) - m[None])
        ls = jnp.sum(p, axis=0)
        lsum[u] = ls if u not in lsum else lsum[u] + ls
        v = _dot(_ld(v_scr, 2 * c + hd), p.reshape(T, T).astype(BF16))
        res.append(v)
        pv[u] = v if u not in pv else v + pv[u]
        if c == r:
            of[u] = pv[u] * (1.0 / jnp.sum(lsum[u], axis=0, keepdims=True))

    def o_lhs(p, kind, i):
        if kind == 'm' and i in (2, 3):
            kind, i = 'r', 3 * (i - 2)
        if (p, kind, i) not in lhs:
            a = lambda n: of[4 * p + n]
            v = a(i) if kind == 'r' else {0: lambda: a(0) + a(3), 1: lambda: a(2) + a(3), 4: lambda: a(0) + a(1),
                                          5: lambda: a(2) - a(0), 6: lambda: a(1) - a(3)}[i]()
            lhs[(p, kind, i)] = _tie(v.astype(BF16).T, v[0:8, :])
        return lhs[(p, kind, i)]

    def job_o(u, j):
        p = u // 4
        _, kind, i, n = _O_JOBS[j]
        w = wo[n][i] if kind == 'm' else wo_ref[_tile(i % 2), _tile(4)]
        v = _dot(o_lhs(p, kind, i), w)
        res.append(v)
        prod[(kind, i, n)] = v
        m = lambda i_: prod[('m', i_, n)]
        if kind == 'r':
            if i % 2:
                acc_scr[_tile(2 * p + i // 2), _tile(4)] += v + prod[('r', i - 1, 0)]
        elif i == 4:
            acc_scr[_tile(2 * p), _tile(2 * n + 1)] += v + m(2)
        elif i == 5:
            prod[('m', 5, n)] = v + m(2)
        elif i == 1:
            acc_scr[_tile(2 * p + 1), _tile(2 * n)] += v + m(3)
        elif i == 0:
            acc_scr[_tile(2 * p + 1), _tile(2 * n + 1)] += v + (m(5) - m(1))
        elif i == 6:
            acc_scr[_tile(2 * p), _tile(2 * n)] += v + (m(0) + (m(3) - m(4)))

    fns = dict(a=job_a, b=job_b, o=job_o)
    for n, (kind, u, j) in enumerate(_job_order(q_scr.shape[0] // 2)):
        if n == MID:
            mid()
        fns[kind](u, j)


def _kernel(x_hbm, c_hbm, wq_hbm, wuk_hbm, wuv_hbm, wo_hbm, w1_hbm, w2_hbm, w3_hbm, w4_hbm,
            cond_hbm, wmod_hbm, out_hbm,
            x_ref, c_ref, cond_ref, wma_ref, wmb_ref, w1_ref, w2_ref, w3_ref, w4_ref,
            wq_buf, wk_buf, wv_buf, wo_buf, out_buf, sem, wsem, osem,
            mod_scr, h_scr, cs_scr, w_scr, q_scr, k_scr, v_scr, acc_scr, x1_scr, hb_scr, a1_scr, t_scr,
            a1s_scr, ws12, ws3, ws4):
    S, M = x_hbm.shape
    D = wq_hbm.shape[2]
    nattn = wo_hbm.shape[0]
    Fd = w4_hbm.shape[0]
    scale = float(D) ** -0.5 * LOG2E
    nb, nrb = S // T, S // RB
    km, kc = M // T, c_hbm.shape[1] // T
    NX = 4
    XR = S // NX
    CB = XR // T

    def pcopies(g):
        return [pltpu.make_async_copy(src.bitcast(U32).at[:, g, :], dst, wsem.at[j])
                for j, (src, dst) in enumerate(((wuk_hbm, wk_buf), (wuv_hbm, wv_buf), (wq_hbm, wq_buf)))]

    def ocopy(g, slot):
        return pltpu.make_async_copy(wo_hbm.at[g], wo_buf.at[slot], wsem.at[3])

    def chunk_copy(src, dst, i, s0):
        rows = slice(i * XR, (i + 1) * XR)
        return pltpu.make_async_copy(src.at[rows, :], dst.at[rows, :], sem.at[s0 + i])

    cp_cond = pltpu.make_async_copy(cond_hbm, cond_ref, sem.at[0])
    cp_wma = pltpu.make_async_copy(wmod_hbm.at[:, 0:2 * M], wma_ref, sem.at[1])
    cp_late = [pltpu.make_async_copy(src, dst, sem.at[2 + j]) for j, (src, dst) in enumerate((
        (wmod_hbm.at[:, 2 * M:6 * M], wmb_ref), (w1_hbm, w1_ref), (w2_hbm, w2_ref),
        (w3_hbm, w3_ref), (w4_hbm, w4_ref)))]
    cp_x = [chunk_copy(x_hbm, x_ref, i, 7) for i in range(NX)]
    cp_c = [chunk_copy(c_hbm, c_ref, i, 7 + NX) for i in range(NX)]

    def silu_cond():
        cf = cond_ref[...].astype(F32)
        return jnp.broadcast_to((cf * jax.nn.sigmoid(cf)).astype(BF16), (8, M))

    cp_wk, cp_wv, cp_wq = pcopies(0)
    named = dict(k=cp_wk, v=cp_wv, q=cp_wq, o=ocopy(0, 0), n=cp_cond, m=cp_wma)
    named.update(zip('abcd', cp_c))
    named.update(zip('wxyz', cp_x))
    plan = PLAN.split(',')

    def kick():
        for ch in plan.pop(0) if plan else '':
            named.pop(ch).start()

    def zero(r, carry):
        acc_scr[pl.ds(pl.multiple_of(r * T, T), T), :] = jnp.zeros((T, M), F32)
        return carry

    def ln_pair(p):
        sa = _rows(mod_scr[:, 0:M], LP)
        ca1 = _rows(mod_scr[:, M:2 * M], LP)
        for i in range(T // LP):
            h1, h2 = [_ln(x_ref[r * T + i * LP:r * T + (i + 1) * LP, :].astype(F32)) * ca1 + sa
                      for r in (2 * p, 2 * p + 1)]
            ops = _a_ops(h1[:, 0:2 * T], h1[:, 2 * T:4 * T], h2[:, 0:2 * T], h2[:, 2 * T:4 * T])
            tiles = [v[:, _tile(j)] for v in ops for j in range(2)] + [h1[:, _tile(4)], h2[:, _tile(4)]]
            for n, v in enumerate(tiles):
                h_scr[p, n, i * LP:(i + 1) * LP, :] = v.astype(BF16)

    def stash(tiles, j0):
        for j, t in enumerate(tiles):
            w_scr[j0 + j] = _pk(t)
        return lambda j: _ld(w_scr, j0 + j)

    def kv_pairs(jobs, p0, p1_):
        for p in range(p0, p1_):
            for j in range(2):
                ops = _a_ops(*[c_ref[_tile(2 * p + n // 2), _tile(2 * (n % 2) + j)].astype(F32)
                               for n in range(4)])
                for i, v in enumerate(ops):
                    cs_scr[p, 2 * i + j] = v.astype(BF16)
            _kv_jobs(jobs, p, cs_scr, wk, wvT, k_scr, v_scr)

    npair, CP = nb // 2, CB // 2
    kick()
    jax.lax.fori_loop(0, nb, zero, 0)
    kick()
    acc_scr[S:, :] = jnp.zeros((acc_scr.shape[0] - S, M), F32)
    x_ref[S:, :] = jnp.zeros((x_ref.shape[0] - S, M), BF16)
    cp_wk.wait()
    cp_wv.wait()
    cp_c[0].wait()
    kick()
    wk = stash(_pair_weights(wk_buf), 0)
    wvT = stash(_pair_weights(wv_buf, True), 14)
    kv_pairs(_Jobs(), 0, CP)
    for chunks in ((1,), (2, 3)):
        for i in chunks:
            cp_c[i].wait()
        kick()
        kv_pairs(_Jobs(), chunks[0] * CP, min((chunks[-1] + 1) * CP, npair - KVL - KVM))
    cp_cond.wait()
    cp_wma.wait()
    kick()
    mod = _dot(silu_cond(), wma_ref[...])
    mod_scr[:, 0:M] = mod[:, 0:M]
    mod_scr[:, M:2 * M] = 1.0 + mod[:, M:2 * M]
    kv_pairs(_Jobs(), npair - KVL - KVM, npair - KVL)
    cp_wq.wait()
    qdone = 0
    for chunks in ((0,), (1,), (2, 3)):
        for i in chunks:
            cp_x[i].wait()
        kick()
        jobs = _Jobs()
        if chunks[0] == 0:
            wq = stash(_pair_weights(wq_buf), 28)
            kv_pairs(jobs, npair - KVL, npair)
        for p in range(chunks[0] * CP, (chunks[-1] + 1) * CP):
            ln_pair(p)
        qend = npair if chunks[-1] == NX - 1 else (chunks[-1] + 1) * CP - QLAG
        for p in range(qdone, qend):
            _q_jobs(jobs, p, h_scr, wq, q_scr, scale)
        qdone = max(qdone, qend)
    assert not named
    ocopy(0, 0).wait()
    for cp in cp_late[1:] + cp_late[:1]:
        cp.start()

    FH = ws3.shape[0] * T

    def mixer_prep(g):
        def blocks(w_ref, r0, n, half, c0, c1, dep):
            lo, hi = pl.ds(r0, n), pl.ds(r0 + half, n)
            return [_after(w_ref[rows, _tile(c)].astype(F32), _rows(dep, n)) if (rows is lo) == (c == c0)
                    else w_ref[rows, _tile(c)].astype(F32) for rows in (lo, hi) for c in (c0, c1)]

        def rows_items(w_ref, dst, per_step, half, n=16):
            gi = jnp.minimum(g, half // per_step - 1)
            src = w_ref.at[pl.ds(pl.multiple_of(gi * per_step, per_step), half + per_step), :]
            hs = per_step // 2

            def item(c, o):
                def fn(dep):
                    for i, v in enumerate(_b_ops(*blocks(src, o, n, half, c, c + 2, dep))):
                        dst[i, c, pl.ds(pl.multiple_of(gi * hs, hs) + o // 2, n // 2), :] = _pk(v.astype(BF16))
                return fn
            return [item(c, o) for c in range(2) for o in range(0, per_step, n)]

        def w3_item(k, i):
            def fn(dep):
                n = jnp.minimum(g, FH // T - 1)
                b11, b21, b12, b22 = blocks(w3_ref, pl.multiple_of(n * T, T), T, FH, k, k + 2, dep)
                ws3[n, i, k] = _pk(_b_ops(b11, b12, b21, b22)[i].astype(BF16).T)
            return fn

        return (rows_items(w1_ref, ws12.at[0], 32, 2 * T) + rows_items(w2_ref, ws12.at[1], 32, 2 * T)
                + rows_items(w4_ref, ws4, 64, FH) + [w3_item(k, i) for k in range(2) for i in range(7)])

    def attn_body(g, carry):
        slot = g & 1
        nxt = jnp.minimum(g + 1, nattn - 1)
        copies = pcopies(nxt) + [ocopy(nxt, 1 - slot)]

        def mid():
            for cp in copies:
                cp.start()

        _attention_step(q_scr, k_scr, v_scr, wo_buf.at[slot], acc_scr, mid)
        for cp in copies:
            cp.wait()

        @pl.when(g == 0)
        def _():
            for cp in cp_late[1:]:
                cp.wait()

        @pl.when(g + 1 < nattn)
        def _():
            _proj_step(h_scr, cs_scr, wq_buf, wk_buf, wv_buf, q_scr, k_scr, v_scr, scale, mixer_prep(g))

        return carry

    jax.lax.fori_loop(0, nattn, attn_body, 0)

    cp_late[0].wait()
    mod = _dot(silu_cond(), wmb_ref[...])
    mod_scr[:, 2 * M:4 * M] = mod[:, 0:2 * M]
    mod_scr[:, 4 * M:5 * M] = 1.0 + mod[:, 2 * M:3 * M]
    mod_scr[:, 5 * M:6 * M] = mod[:, 3 * M:4 * M]
    ftiles = [(f, min(f + T, Fd)) for f in range(0, Fd, T)]
    OFF = x_ref.shape[0] - S
    CAR = t_scr.shape[0] - RB

    def p1(r0, n, dep=None):
        ga = mod_scr[:, 2 * M:3 * M]
        if dep is not None:
            ga = jnp.concatenate([_after(ga[:, 0:T], dep), ga[:, T:]], axis=1)
        rows = pl.ds(r0, n)
        x1 = x_ref[rows, :].astype(F32) + _rows(ga, n) * acc_scr[rows, :]
        x1_scr[rows, :] = x1
        hb = _ln(x1) * _rows(mod_scr[:, 4 * M:5 * M], n) + _rows(mod_scr[:, 3 * M:4 * M], n)
        hb_scr[rows, :] = hb
        return _ln(hb)

    HT = T // 2
    SUMS = (0, 1, 4, 5, 6)

    def p1_store(r0, c, dep=None):
        n = PC // 2
        hf, o = divmod(c * n, HT)
        top, bot = [p1(r0 + hf * T + d + o, n, dep) for d in (0, HT)]
        for d, v in ((0, top), (HT, bot)):
            for j in range(km):
                a1_scr[j, hf * T + d + o:hf * T + d + o + n, :] = v[:, _tile(j)].astype(BF16)
        ops = _a_ops(top[:, 0:2 * T], top[:, 2 * T:4 * T], bot[:, 0:2 * T], bot[:, 2 * T:4 * T])
        for i, m in enumerate(SUMS):
            for k in range(2):
                a1s_scr[hf, i, k, o:o + n, :] = ops[m][:, _tile(k)].astype(BF16)
        return jnp.max(ops[0][:, :T].reshape(n // 8, 8, T), axis=0)

    t_scr[RB:RB + CAR - OFF, :] = jnp.zeros((CAR - OFF, M), F32)
    t_scr[RB + CAR - OFF:RB + CAR, :] = _gelu(_dot(p1(0, OFF).astype(BF16), w1_ref[...]))
    for c in range(RB // PC):
        p1_store(OFF, c)

    def out_copy(i):
        rows = pl.ds(i * T if isinstance(i, int) else pl.multiple_of(i * T, T), T)
        return pltpu.make_async_copy(out_buf.at[rows, :], out_hbm.at[rows, :], osem.at[i])

    def b_body(r, carry):
        gb = _rows(mod_scr[:, 5 * M:6 * M], T)
        r0 = pl.multiple_of(r * RB, RB)
        n0 = pl.multiple_of(jnp.minimum(r0 + RB, S - RB) + OFF, OFF)
        nh = RB // T
        now = [0]
        due = []
        pace = []

        def p1_item(c):
            return lambda dep: due.append((now[0] + PD, p1_store(n0, c, dep)))

        pace += [(P0 + i * PSTEP, p1_item(i)) for i in range(RB // PC)]
        wt = lambda ref, f0, f1, n: ref[f0:f1, _tile(n)]

        def mm(lhs, wts, dot=_dot):
            acc = None
            for x, w in zip(lhs, wts):
                if due and due[0][0] <= now[0]:
                    w = _tie(w, due.pop(0)[1])
                v = dot(x, w)
                now[0] += x.shape[0] // HT
                acc = v if acc is None else v + acc
                if pace and pace[0][0] <= now[0]:
                    pace.pop(0)[1](v[0:8, :])
            return acc

        def split_ops(lo, hi):
            return [v.astype(BF16) for v in _a_ops(lo[:HT], hi[:HT], lo[HT:], hi[HT:])]

        def two_tiles(aops, wsel, rest):
            def col(w):
                v = mm(rest[0], w, rest[3])
                return v[:HT], v[HT:]

            c11, c12, c21, c22 = _strassen(
                lambda i: mm([a[i] for a in aops], [wsel(i, k) for k in range(len(aops))]),
                lambda: col(rest[1]), lambda: col(rest[2]))
            return jnp.concatenate([c11, c21], axis=0), jnp.concatenate([c12, c22], axis=0)

        def square(full, aops, w_ref, ws_ref):
            out = {}
            for n in range(2):
                out[n], out[n + 2] = two_tiles(
                    aops, lambda i, k: _ld(ws_ref, i, n, slice(k * HT, (k + 1) * HT)),
                    (full[4:], [wt(w_ref, 4 * T, M, n)], [wt(w_ref, 4 * T, M, n + 2)], _dot))
            out[4] = mm(full, [wt(w_ref, j * T, (j + 1) * T, 4) for j in range(km)])
            return out

        t_scr[0:CAR, :] = t_scr[RB:RB + CAR, :]
        for hf in range(nh):
            full = [a1_scr[j, _tile(hf), :] for j in range(km)]
            aops = []
            for k in range(2):
                ops = {m: a1s_scr[hf, i, k] for i, m in enumerate(SUMS)}
                ops[2], ops[3] = full[k][:HT], full[2 + k][HT:]
                aops.append(ops)
            for n, v in square(full, aops, w1_ref, ws12.at[0]).items():
                t = _gelu(v)
                if hf == nh - 1:
                    t = jnp.concatenate([t[:T - OFF], jnp.where(r < nrb - 1, t[T - OFF:], 0.0)], axis=0)
                t_scr[CAR + hf * T:CAR + (hf + 1) * T, _tile(n)] = t
        cq = M // 4
        shifts = (-1, 1, -2, 2)
        lane = jax.lax.broadcasted_iota(jnp.int32, (T, T), 1)
        y1, a3 = [], []
        for hf in range(nh):
            base = CAR - OFF + hf * T
            sh = []
            for j in range(km):
                g_lo, g_hi = (j * T) // cq, ((j + 1) * T - 1) // cq
                assert g_hi - g_lo <= 1
                v = t_scr[base + shifts[g_lo]:base + shifts[g_lo] + T, _tile(j)]
                if g_hi != g_lo:
                    v2 = t_scr[base + shifts[g_hi]:base + shifts[g_hi] + T, _tile(j)]
                    v = jnp.where(lane < g_hi * cq - j * T, v, v2)
                sh.append(v)
            hs = square([v.astype(BF16) for v in sh], [split_ops(sh[k], sh[2 + k]) for k in range(2)],
                        w2_ref, ws12.at[1])
            hs = jnp.concatenate([hs[n] for n in range(km)], axis=1)
            y1.append(hs + hb_scr[pl.ds(pl.multiple_of(r0 + hf * T, T), T), :])
            a3.append({})

            def ln_item(hf, c):
                def item(dep):
                    n = HT // NLN
                    for d in (0, HT):
                        v = y1[hf][d + c * n:d + (c + 1) * n]
                        if dep is not None:
                            v = jnp.concatenate([_after(v[:, :T], _rows(dep, n)), v[:, T:]], axis=1)
                        a3[hf][d + c * n] = _ln(v)
                return item

            ln_item(hf, 0)(None)
            pace += [(now[0] + LN0 + (c - 1) * LNS * (1 + hf), ln_item(hf, c)) for c in range(1, NLN)]
            pace.sort(key=lambda e: e[0])
        nf = FH // T
        h3, h3ops = [], []
        for hf in range(nh):
            assert len(a3[hf]) == 2 * NLN
            af = jnp.concatenate([a3[hf][key] for key in sorted(a3[hf])], axis=0)
            full = [af[:, _tile(j)].astype(BF16) for j in range(km)]
            aops = [split_ops(af[:, _tile(k)], af[:, _tile(2 + k)]) for k in range(2)]
            row, ops = {}, []
            narrow = None
            for n in range(nf):
                lo, hi = two_tiles(aops, lambda i, k: _ld(ws3, n, i, k),
                                   (full[4:], [wt(w3_ref, *ftiles[n], 4)],
                                    [wt(w3_ref, *ftiles[nf + n], 4)], _dot_nt))
                lo, hi = _gelu(lo), _gelu(hi)
                row[n], row[nf + n] = lo.astype(BF16), hi.astype(BF16)
                ops.append(split_ops(lo, hi))
                if n < km:
                    v = mm([wt(w3_ref, *ftiles[-1], n)], [full[n]], _dot_nt)
                    narrow = v if narrow is None else v + narrow
            row[2 * nf] = _gelu(mm(full, [wt(w3_ref, *ftiles[2 * nf], j) for j in range(km)],
                                   _dot_nt)).astype(BF16)
            fw = Fd - ftiles[-1][0]
            gT = jnp.concatenate([_gelu(narrow), jnp.zeros((T - fw, T), F32)], axis=0)
            row[2 * nf + 1] = _tie(gT.astype(BF16).T, gT[0:8, :])[:, :fw]
            h3.append([row[i] for i in range(len(ftiles))])
            h3ops.append(ops)
        for hf in range(nh):
            rows = pl.ds(pl.multiple_of(r0 + hf * T, T), T)

            def finish(n, v):
                out_buf[rows, _tile(n)] = (
                    x1_scr[rows, _tile(n)] + gb[:, _tile(n)] * (v + y1[hf][:, _tile(n)])
                ).astype(out_buf.dtype)

            w4t = lambda n, f_: [wt(w4_ref, f0, f1, n) for f0, f1 in f_]
            finish(4, mm(h3[hf], w4t(4, ftiles)))
            for n in range(2):
                lo, hi = two_tiles(h3ops[hf], lambda i, k: _ld(ws4, i, n, slice(k * HT, (k + 1) * HT)),
                                   (h3[hf][2 * nf:], w4t(n, ftiles[2 * nf:]), w4t(n + 2, ftiles[2 * nf:]), _dot))
                finish(n, lo)
                finish(n + 2, hi)
            out_copy(r * nh + hf).start()
        assert not pace
        return carry

    jax.lax.fori_loop(0, nrb, b_body, 0)
    for i in range(nb):
        out_copy(i).wait()


@jax.jit
def pallas_adaLN_cond__compressed_kv_cla__mixer_s_mlp__prompt_kernel(
    A_x: jax.Array,
    A_c_kv: jax.Array,
    A_w_q: jax.Array,
    A_w_uk: jax.Array,
    A_w_uv: jax.Array,
    A_w_o: jax.Array,
    B_x: jax.Array,
    B_w1: jax.Array,
    B_w2: jax.Array,
    B_w3: jax.Array,
    B_w4: jax.Array,
    c: jax.Array,
    w_mod: jax.Array,
):
    _, S, M = A_x.shape
    Dc = A_c_kv.shape[2]
    H, D = A_w_q.shape[1], A_w_q.shape[2]
    Fd = B_w3.shape[1]
    assert D == T and A_c_kv.shape[1] == S and Dc == 4 * T and M == 5 * T and 13 * T < Fd < 14 * T
    vmem = pltpu.VMEM
    packed = lambda *lead: vmem(lead + (T // 2, T), U32)
    out = pl.pallas_call(
        _kernel,
        in_specs=[pl.BlockSpec(memory_space=pltpu.HBM)] * 12,
        out_specs=pl.BlockSpec(memory_space=pltpu.HBM),
        out_shape=jax.ShapeDtypeStruct((S, M), A_x.dtype),
        scratch_shapes=[
            vmem((S + 16, M), BF16),
            vmem((S, Dc), BF16),
            vmem((1, M), BF16),
            vmem((M, 2 * M), BF16),
            vmem((M, 4 * M), BF16),
            vmem((M, M), BF16),
            vmem((M, M), BF16),
            vmem((Fd, M), BF16),
            vmem((Fd, M), BF16),
            vmem((M, D), U32),
            vmem((Dc, D), U32),
            vmem((Dc, D), U32),
            vmem((2, 2 * D, M), BF16),
            vmem((S, M), A_x.dtype),
            pltpu.SemaphoreType.DMA((15,)),
            pltpu.SemaphoreType.DMA((4,)),
            pltpu.SemaphoreType.DMA((S // T,)),
            vmem((8, 6 * M), F32),
            vmem((S // T // 2, 16, T, T), BF16),
            vmem((S // T // 2, 14, T, T), BF16),
            packed(44),
            packed(2 * S // T),
            packed(2 * S // T),
            packed(2 * S // T),
            vmem((S + 16, M), F32),
            vmem((S + 16, M), F32),
            vmem((S + 16, M), F32),
            vmem((M // T, RB, T), BF16),
            vmem((RB + 32, M), F32),
            vmem((RB // T, 5, 2, T // 2, T), BF16),
            vmem((2, 7, 2, T, T), U32),
            packed(6, 7, 2),
            vmem((7, 2, 3 * T, T), U32),
        ],
        compiler_params=pltpu.CompilerParams(
            vmem_limit_bytes=100 * 1024 * 1024,
            disable_bounds_checks=True,
        ),
    )(
        A_x.reshape(S, M), A_c_kv.reshape(S, Dc),
        A_w_q, A_w_uk, A_w_uv,
        A_w_o.reshape(H // 2, 2 * D, M),
        B_w1, B_w2, B_w3.T, B_w4, c, w_mod,
    )
    return out.reshape(1, S, M)
```

```python
import math
import os

import jax
import jax.numpy as jnp
import jax.experimental.pallas as pl
import jax.experimental.pallas.tpu as pltpu

F32 = jnp.float32
BF16 = jnp.bfloat16
U32 = jnp.uint32
NT = (((1,), (1,)), ((), ()))
T = 128
EPS = 1e-5
LOG2E = math.log2(math.e)

GRP = int(os.environ.get('GRP', 4))
LEAD = int(os.environ.get('LEAD', 10))
PROW = int(os.environ.get('PROW', 3))
VT = 8
RES = int(os.environ.get('RES', 30))
LAT_A = int(os.environ.get('LAT_A', 16))
LAT_B = int(os.environ.get('LAT_B', 20))
ALEAD = int(os.environ.get('ALEAD', 32))
MID = int(os.environ.get('MID', 40))
NLN = int(os.environ.get('NLN', 4))
LN0 = int(os.environ.get('LN0', 4))
LNS = int(os.environ.get('LNS', 5))
SD0 = int(os.environ.get('SD0', 50))
SDS = int(os.environ.get('SDS', 10))
FINE = int(os.environ.get('FINE', 0))
OGRP = int(os.environ.get('OGRP', 6))
RB = 256
PC = 32
P0, PSTEP, PD = [int(os.environ.get(k_, d_)) for k_, d_ in (('P0', 400), ('PSTEP', 30), ('PD', 56))]
LP = int(os.environ.get('LP', 16))
PROLOGUE = os.environ.get('PRO', '|kva|Z; |b|; kva|cdn|K01; b|m|K23; cd|qw|K45; nm|x|M K6; qw|yzo|K7 H01 Q0; x||H23 Q12; yz||H4567 Q34567; o||')


def _dot(a, b):
    return jnp.dot(a, b, preferred_element_type=F32)


def _dot_nt(a, b):
    return jax.lax.dot_general(a, b, NT, preferred_element_type=F32)


def _ln(x):
    m = jnp.mean(x, axis=-1, keepdims=True)
    xc = x - m
    v = jnp.mean(xc * xc, axis=-1, keepdims=True)
    return xc * jnp.exp2(jnp.log(v + EPS) * (-0.5 * LOG2E))


def _rows(v, n):
    return jnp.broadcast_to(v[None], (n // 8, 8, v.shape[1])).reshape(n, v.shape[1])


def _gelu(x):
    c0 = math.sqrt(2.0 / math.pi)
    return 0.5 * x * (1.0 + jnp.tanh(c0 * (x + 0.044715 * (x * x * x))))


def _after(x, dep):
    return jnp.where(dep > jnp.inf, dep, x)


def _tie(x, dep):
    xu = pltpu.bitcast(x, U32)
    first = jnp.where(dep > jnp.inf, jnp.uint32(0), xu[:8])
    return pltpu.bitcast(jnp.concatenate([first, xu[8:]], axis=0), BF16)


def _tile(j):
    return slice(j * T, (j + 1) * T)


def _ld(ref, *idx):
    return pltpu.bitcast(ref[idx], BF16)


def _pk(x):
    return pltpu.bitcast(x, U32)


def _a_ops(a11, a12, a21, a22):
    return [a11 + a22, a21 + a22, a11, a22, a11 + a12, a21 - a11, a12 - a22]


SUMS = (0, 1, 4, 5, 6)


def _b_ops(b11, b12, b21, b22):
    return [b11 + b22, b11, b12 - b22, b21 - b11, b22, b11 + b12, b21 + b22]


def _strassen(prod, col1=None, col2=None):
    m4 = prod(3)
    m2 = prod(1)
    c21 = m2 + m4
    if col1 is not None:
        e11, e21 = col1()
        m4, c21 = m4 + e11, c21 + e21
    m3 = prod(2)
    m5 = prod(4)
    c12 = m3 + m5
    if col2 is not None:
        e12, e22 = col2()
        c12, m3 = c12 + e12, m3 + e22
    m1 = prod(0)
    c11 = prod(6) + (m1 + (m4 - m5))
    c22 = prod(5) + (m1 + (m3 - m2))
    return c11, c12, c21, c22


def _pair_weights(w_ref, transpose=False):
    lo, hi = [], []
    for j in range(w_ref.shape[0] // T):
        wu = w_ref[_tile(j), :]
        lo.append(pltpu.bitcast(wu << 16, F32))
        hi.append(pltpu.bitcast(wu & jnp.uint32(0xFFFF0000), F32))
    per_j = [_b_ops(lo[j], hi[j], lo[2 + j], hi[2 + j]) for j in range(2)]
    tiles = [per_j[j][i] for i in range(7) for j in range(2)]
    for j in range(4, len(lo)):
        tiles += [lo[j], hi[j]]
    tiles = [t.astype(BF16) for t in tiles]
    return [t.T for t in tiles] if transpose else tiles


class _Jobs:
    def __init__(self, side=()):
        self.res = []
        self.side = list(side)

    def mm(self, lhs, wt, dot, tie=False):
        acc = None
        for x, w in zip(lhs, wt):
            if tie and len(self.res) >= VT:
                x = _tie(x, self.res[len(self.res) - VT][0:8, :])
            v = dot(x, w)
            self.res.append(v)
            acc = v if acc is None else v + acc
            if self.side and self.side[0][0] <= len(self.res):
                self.side.pop(0)[1](v[0:8, :])
        return acc


def _kv_jobs(jobs, p, c_ref, cs_scr, wk, wvT, k_scr, v_scr):
    ct = lambda i: [cs_scr[p, SUMS.index(i), j] if i in SUMS
                    else c_ref[_tile(2 * p + i - 2), _tile(2 * (i - 2) + j)] for j in range(2)]
    ks = _strassen(lambda i: jobs.mm(ct(i), [wk(2 * i), wk(2 * i + 1)], _dot))
    for n, v in enumerate(ks):
        k_scr[4 * p + n] = _pk(v.astype(BF16))
    vs = _strassen(lambda i: jobs.mm([wvT(2 * i), wvT(2 * i + 1)], ct(i), _dot_nt, True))
    for n, v in enumerate(vs):
        v_scr[4 * p + n] = _pk(v.astype(BF16))


def _q_jobs(jobs, p, h_scr, wq, q_scr, scale):
    rest = lambda hd: (lambda: [jobs.mm([h_scr[p, 14 + x]], [wq(14 + hd)], _dot) for x in range(2)])
    if not jobs.res:
        early = [rest(hd)() for hd in range(2)]
        rest = lambda hd: (lambda: early[hd])
    qs = _strassen(lambda i: jobs.mm([h_scr[p, 2 * i + j] for j in range(2)],
                                     [wq(2 * i), wq(2 * i + 1)], _dot), rest(0), rest(1))
    for n, v in enumerate(qs):
        q_scr[4 * p + n] = _pk((v * scale).astype(BF16))


def _proj_step(h_scr, c_ref, cs_scr, wq_ref, wuk_ref, wuv_ref, q_scr, k_scr, v_scr, scale, side):
    wq = _pair_weights(wq_ref)
    wk = _pair_weights(wuk_ref)
    wvT = _pair_weights(wuv_ref, True)
    jobs = _Jobs((SD0 + i * SDS, fn) for i, fn in enumerate(side))
    for p in range(h_scr.shape[0]):
        _q_jobs(jobs, p, h_scr, wq.__getitem__, q_scr, scale)
        _kv_jobs(jobs, p, c_ref, cs_scr, wk.__getitem__, wvT.__getitem__, k_scr, v_scr)
    assert not jobs.side


_O_JOBS = ([(0, 'r', 0, 0), (0, 'm', 2, 0), (0, 'm', 2, 1), (1, 'r', 1, 0), (1, 'm', 4, 0), (1, 'm', 4, 1),
            (2, 'r', 2, 0), (2, 'm', 5, 0), (2, 'm', 5, 1), (3, 'r', 3, 0)]
           + [(3, 'm', i, n) for n in range(2) for i in (3, 1, 0, 6)])


def _job_order(nb):
    units = range(2 * nb)
    qa = [('a', u, c) for u in units for c in range(u // 2 + 1)]
    qb = [('b', u, c) for u in units for c in range(u // 2 + 1)]
    last = nb // 2 - 1
    qo = [('o', 4 * p + (job[0] if FINE or p == last else 3), j)
          for p in range(nb // 2) for j, job in enumerate(_O_JOBS)]
    done = {}
    order = []

    def ready(q, lat, pre):
        return bool(q) and (pre, q[0][1]) in done and done[(pre, q[0][1])] + lat <= len(order)

    def emit(q):
        kind, u, j = job = q.pop(0)
        if kind != 'o' and j == u // 2:
            done[(kind, u)] = len(order)
        order.append(job)

    turn = 0
    while qa or qb or qo:
        pref = 'abo'[turn % 3]
        turn += 1
        for _ in range(OGRP if pref == 'o' else GRP):
            b_ok, o_ok = ready(qb, LAT_A, 'a'), ready(qo, LAT_B, 'b')
            if pref == 'a' and qa and (len(qb) - len(qa) < ALEAD or not b_ok):
                emit(qa)
            elif pref == 'b' and b_ok:
                emit(qb)
            elif pref == 'o' and o_ok and (len(qo) > RES or not (qa or b_ok)):
                emit(qo)
            elif not (qa or b_ok or o_ok) and (qb or qo):
                emit(qb or qo)
            else:
                break
    return order


def _attention_step(q_scr, k_scr, v_scr, wo_ref, acc_scr, mid):
    causal = (jax.lax.broadcasted_iota(jnp.int32, (T, T), 0)
              <= jax.lax.broadcasted_iota(jnp.int32, (T, T), 1))
    sv, mx, mfin, lsum, pv, of, lhs, prod = {}, {}, {}, {}, {}, {}, {}, {}
    res = []
    wo = [[t.astype(BF16) for t in _b_ops(*[wo_ref[_tile(i // 2), _tile(2 * n + i % 2)].astype(F32)
                                            for i in range(4)])] for n in range(2)]

    def job_a(u, c):
        r, hd = divmod(u, 2)
        s = _dot_nt(_ld(k_scr, 2 * c + hd), _ld(q_scr, u))
        res.append(s)
        if c == r:
            s = jnp.where(causal, s, -1e9 * LOG2E)
        s = s.reshape(T // 8, 8, T)
        sv[(u, c)] = s
        pm = jnp.max(s, axis=0)
        mx[u] = pm if u not in mx else jnp.maximum(mx[u], pm)

    def job_b(u, c):
        r, hd = divmod(u, 2)
        if u not in mfin:
            mfin[u] = jnp.broadcast_to(jnp.max(mx[u], axis=0, keepdims=True), (8, T))
        m = mfin[u]
        if len(res) >= LEAD:
            r0 = 8 * PROW * (c % 4)
            m = _after(m, res[len(res) - LEAD][r0:r0 + 8, :])
        p = jnp.exp2(sv.pop((u, c)) - m[None])
        ls = jnp.sum(p, axis=0)
        lsum[u] = ls if u not in lsum else lsum[u] + ls
        v = _dot(_ld(v_scr, 2 * c + hd), p.reshape(T, T).astype(BF16))
        res.append(v)
        pv[u] = v if u not in pv else v + pv[u]
        if c == r:
            of[u] = pv[u] * (1.0 / jnp.sum(lsum[u], axis=0, keepdims=True))

    def o_lhs(p, kind, i):
        if kind == 'm' and i in (2, 3):
            kind, i = 'r', 3 * (i - 2)
        if (p, kind, i) not in lhs:
            a = lambda n: of[4 * p + n]
            v = a(i) if kind == 'r' else {0: lambda: a(0) + a(3), 1: lambda: a(2) + a(3), 4: lambda: a(0) + a(1),
                                          5: lambda: a(2) - a(0), 6: lambda: a(1) - a(3)}[i]()
            lhs[(p, kind, i)] = _tie(v.astype(BF16).T, v[0:8, :])
        return lhs[(p, kind, i)]

    def job_o(u, j):
        p = u // 4
        _, kind, i, n = _O_JOBS[j]
        w = wo[n][i] if kind == 'm' else wo_ref[_tile(i % 2), _tile(4)]
        v = _dot(o_lhs(p, kind, i), w)
        res.append(v)
        prod[(kind, i, n)] = v
        m = lambda i_: prod[('m', i_, n)]
        if kind == 'r':
            if i % 2:
                acc_scr[_tile(2 * p + i // 2), _tile(4)] += v + prod[('r', i - 1, 0)]
        elif i == 4:
            acc_scr[_tile(2 * p), _tile(2 * n + 1)] += v + m(2)
        elif i == 5:
            prod[('m', 5, n)] = v + m(2)
        elif i == 1:
            acc_scr[_tile(2 * p + 1), _tile(2 * n)] += v + m(3)
        elif i == 0:
            acc_scr[_tile(2 * p + 1), _tile(2 * n + 1)] += v + (m(5) - m(1))
        elif i == 6:
            acc_scr[_tile(2 * p), _tile(2 * n)] += v + (m(0) + (m(3) - m(4)))

    fns = dict(a=job_a, b=job_b, o=job_o)
    for n, (kind, u, j) in enumerate(_job_order(q_scr.shape[0] // 2)):
        if n == MID:
            mid()
        fns[kind](u, j)


def _kernel(x_hbm, c_hbm, wq_hbm, wuk_hbm, wuv_hbm, wo_hbm, w1_hbm, w2_hbm, w3_hbm, w4_hbm,
            cond_hbm, wmod_hbm, out_hbm,
            x_ref, c_ref, cond_ref, wma_ref, wmb_ref, w1_ref, w2_ref, w3_ref, w4_ref,
            wq_buf, wk_buf, wv_buf, wo_buf, out_buf, sem, wsem, osem,
            mod_scr, h_scr, cs_scr, w_scr, q_scr, k_scr, v_scr, acc_scr, x1_scr, hb_scr, a1_scr, t_scr,
            a1s_scr, ws12, ws3, ws4):
    S, M = x_hbm.shape
    D = wq_hbm.shape[2]
    nattn = wo_hbm.shape[0]
    Fd = w4_hbm.shape[0]
    scale = float(D) ** -0.5 * LOG2E
    nb, nrb = S // T, S // RB
    km, kc = M // T, c_hbm.shape[1] // T
    NX = 4
    XR = S // NX
    CB = XR // T

    def pcopies(g):
        return [pltpu.make_async_copy(src.bitcast(U32).at[:, g, :], dst, wsem.at[j])
                for j, (src, dst) in enumerate(((wuk_hbm, wk_buf), (wuv_hbm, wv_buf), (wq_hbm, wq_buf)))]

    def ocopy(g, slot):
        return pltpu.make_async_copy(wo_hbm.at[g], wo_buf.at[slot], wsem.at[3])

    def chunk_copy(src, dst, i, s0):
        rows = slice(i * XR, (i + 1) * XR)
        return pltpu.make_async_copy(src.at[rows, :], dst.at[rows, :], sem.at[s0 + i])

    cp_cond = pltpu.make_async_copy(cond_hbm, cond_ref, sem.at[0])
    cp_wma = pltpu.make_async_copy(wmod_hbm.at[:, 0:2 * M], wma_ref, sem.at[1])
    cp_late = [pltpu.make_async_copy(src, dst, sem.at[2 + j]) for j, (src, dst) in enumerate((
        (wmod_hbm.at[:, 2 * M:6 * M], wmb_ref), (w1_hbm, w1_ref), (w2_hbm, w2_ref),
        (w3_hbm, w3_ref), (w4_hbm, w4_ref)))]
    cp_x = [chunk_copy(x_hbm, x_ref, i, 7) for i in range(NX)]
    cp_c = [chunk_copy(c_hbm, c_ref, i, 7 + NX) for i in range(NX)]

    def silu_cond():
        cf = cond_ref[...].astype(F32)
        return jnp.broadcast_to((cf * jax.nn.sigmoid(cf)).astype(BF16), (8, M))

    cp_wk, cp_wv, cp_wq = pcopies(0)
    named = dict(k=cp_wk, v=cp_wv, q=cp_wq, o=ocopy(0, 0), n=cp_cond, m=cp_wma)
    named.update(zip('abcd', cp_c))
    named.update(zip('wxyz', cp_x))
    started, arrived, did = set(), set(), set()

    def zero(r, carry):
        acc_scr[pl.ds(pl.multiple_of(r * T, T), T), :] = jnp.zeros((T, M), F32)
        return carry

    def h_pair(p):
        sa = _rows(mod_scr[:, 0:M], LP)
        ca1 = _rows(mod_scr[:, M:2 * M], LP)
        for i in range(T // LP):
            h1, h2 = [_ln(x_ref[r * T + i * LP:r * T + (i + 1) * LP, :].astype(F32)) * ca1 + sa
                      for r in (2 * p, 2 * p + 1)]
            ops = _a_ops(h1[:, 0:2 * T], h1[:, 2 * T:4 * T], h2[:, 0:2 * T], h2[:, 2 * T:4 * T])
            tiles = [v[:, _tile(j)] for v in ops for j in range(2)] + [h1[:, _tile(4)], h2[:, _tile(4)]]
            for n, v in enumerate(tiles):
                h_scr[p, n, i * LP:(i + 1) * LP, :] = v.astype(BF16)

    def stash(key, buf, j0, transpose=False):
        if key not in did:
            assert key in arrived
            did.add(key)
            for j, t in enumerate(_pair_weights(buf, transpose)):
                w_scr[j0 + j] = _pk(t)
        return lambda j: _ld(w_scr, j0 + j)

    def kv_pair(jobs, p):
        wk, wvT = stash('k', wk_buf, 0), stash('v', wv_buf, 14, True)
        for j in range(2):
            ops = _a_ops(*[c_ref[_tile(2 * p + n // 2), _tile(2 * (n % 2) + j)].astype(F32)
                           for n in range(4)])
            for n, i in enumerate(SUMS):
                cs_scr[p, n, j] = ops[i].astype(BF16)
        _kv_jobs(jobs, p, c_ref, cs_scr, wk, wvT, k_scr, v_scr)

    ppc = CB // 2
    for blk in PROLOGUE.split(';'):
        waits, starts, acts = blk.split('|')
        for ch in waits.strip():
            assert ch in started and ch not in arrived
            arrived.add(ch)
            named[ch].wait()
        for ch in starts.strip():
            assert ch not in started
            started.add(ch)
            named[ch].start()
        jobs = _Jobs()
        for act in acts.split():
            if act == 'Z':
                jax.lax.fori_loop(0, nb, zero, 0)
                acc_scr[S:, :] = jnp.zeros((acc_scr.shape[0] - S, M), F32)
                x_ref[S:, :] = jnp.zeros((x_ref.shape[0] - S, M), BF16)
            elif act == 'M':
                assert arrived >= set('nm')
                mod = _dot(silu_cond(), wma_ref[...])
                mod_scr[:, 0:M] = mod[:, 0:M]
                mod_scr[:, M:2 * M] = 1.0 + mod[:, M:2 * M]
                did.add('M')
            else:
                for half in act[1:]:
                    for p in range(int(half) * ppc // 2, (int(half) + 1) * ppc // 2):
                        did.add((act[0], p))
                        if act[0] == 'K':
                            assert 'abcd'[p // ppc] in arrived
                            kv_pair(jobs, p)
                        elif act[0] == 'H':
                            assert 'wxyz'[p // ppc] in arrived and 'M' in did
                            h_pair(p)
                        else:
                            assert act[0] == 'Q' and ('H', p) in did
                            _q_jobs(jobs, p, h_scr, stash('q', wq_buf, 28), q_scr, scale)
    assert arrived == set(named) and all((k_, p) in did for k_ in 'KHQ' for p in range(nb // 2))
    for cp in cp_late[1:] + cp_late[:1]:
        cp.start()

    FH = ws3.shape[0] * T

    def mixer_prep(g):
        def blocks(w_ref, r0, n, half, c0, c1, dep):
            lo, hi = pl.ds(r0, n), pl.ds(r0 + half, n)
            return [_after(w_ref[rows, _tile(c)].astype(F32), _rows(dep, n)) if (rows is lo) == (c == c0)
                    else w_ref[rows, _tile(c)].astype(F32) for rows in (lo, hi) for c in (c0, c1)]

        def rows_items(w_ref, dst, per_step, half, n=16):
            gi = jnp.minimum(g, half // per_step - 1)
            src = w_ref.at[pl.ds(pl.multiple_of(gi * per_step, per_step), half + per_step), :]
            hs = per_step // 2

            def item(c, o):
                def fn(dep):
                    for i, v in enumerate(_b_ops(*blocks(src, o, n, half, c, c + 2, dep))):
                        dst[i, c, pl.ds(pl.multiple_of(gi * hs, hs) + o // 2, n // 2), :] = _pk(v.astype(BF16))
                return fn
            return [item(c, o) for c in range(2) for o in range(0, per_step, n)]

        def w3_item(k, i):
            def fn(dep):
                n = jnp.minimum(g, FH // T - 1)
                b11, b21, b12, b22 = blocks(w3_ref, pl.multiple_of(n * T, T), T, FH, k, k + 2, dep)
                ws3[n, i, k] = _pk(_b_ops(b11, b12, b21, b22)[i].astype(BF16).T)
            return fn

        return (rows_items(w1_ref, ws12.at[0], 32, 2 * T) + rows_items(w2_ref, ws12.at[1], 32, 2 * T)
                + rows_items(w4_ref, ws4, 64, FH) + [w3_item(k, i) for k in range(2) for i in range(7)])

    def attn_body(g, carry):
        slot = g & 1
        nxt = jnp.minimum(g + 1, nattn - 1)
        copies = pcopies(nxt) + [ocopy(nxt, 1 - slot)]

        def mid():
            for cp in copies:
                cp.start()

        _attention_step(q_scr, k_scr, v_scr, wo_buf.at[slot], acc_scr, mid)
        for cp in copies:
            cp.wait()

        @pl.when(g == 0)
        def _():
            for cp in cp_late[1:]:
                cp.wait()

        @pl.when(g + 1 < nattn)
        def _():
            _proj_step(h_scr, c_ref, cs_scr, wq_buf, wk_buf, wv_buf, q_scr, k_scr, v_scr, scale, mixer_prep(g))

        return carry

    jax.lax.fori_loop(0, nattn, attn_body, 0)

    cp_late[0].wait()
    mod = _dot(silu_cond(), wmb_ref[...])
    mod_scr[:, 2 * M:4 * M] = mod[:, 0:2 * M]
    mod_scr[:, 4 * M:5 * M] = 1.0 + mod[:, 2 * M:3 * M]
    mod_scr[:, 5 * M:6 * M] = mod[:, 3 * M:4 * M]
    ftiles = [(f, min(f + T, Fd)) for f in range(0, Fd, T)]
    OFF = x_ref.shape[0] - S
    CAR = t_scr.shape[0] - RB

    def p1(r0, n, dep=None):
        ga = mod_scr[:, 2 * M:3 * M]
        if dep is not None:
            ga = jnp.concatenate([_after(ga[:, 0:T], dep), ga[:, T:]], axis=1)
        rows = pl.ds(r0, n)
        x1 = x_ref[rows, :].astype(F32) + _rows(ga, n) * acc_scr[rows, :]
        x1_scr[rows, :] = x1
        hb = _ln(x1) * _rows(mod_scr[:, 4 * M:5 * M], n) + _rows(mod_scr[:, 3 * M:4 * M], n)
        hb_scr[rows, :] = hb
        return _ln(hb)

    HT = T // 2

    def p1_store(r0, c, dep=None):
        n = PC // 2
        hf, o = divmod(c * n, HT)
        top, bot = [p1(r0 + hf * T + d + o, n, dep) for d in (0, HT)]
        for d, v in ((0, top), (HT, bot)):
            for j in range(km):
                a1_scr[j, hf * T + d + o:hf * T + d + o + n, :] = v[:, _tile(j)].astype(BF16)
        ops = _a_ops(top[:, 0:2 * T], top[:, 2 * T:4 * T], bot[:, 0:2 * T], bot[:, 2 * T:4 * T])
        for i, m in enumerate(SUMS):
            for k in range(2):
                a1s_scr[hf, i, k, o:o + n, :] = ops[m][:, _tile(k)].astype(BF16)
        return jnp.max(ops[0][:, :T].reshape(n // 8, 8, T), axis=0)

    t_scr[RB:RB + CAR - OFF, :] = jnp.zeros((CAR - OFF, M), F32)
    t_scr[RB + CAR - OFF:RB + CAR, :] = _gelu(_dot(p1(0, OFF).astype(BF16), w1_ref[...]))
    for c in range(RB // PC):
        p1_store(OFF, c)

    def out_copy(i):
        rows = pl.ds(i * T if isinstance(i, int) else pl.multiple_of(i * T, T), T)
        return pltpu.make_async_copy(out_buf.at[rows, :], out_hbm.at[rows, :], osem.at[i])

    def b_body(r, carry):
        gb = _rows(mod_scr[:, 5 * M:6 * M], T)
        r0 = pl.multiple_of(r * RB, RB)
        n0 = pl.multiple_of(jnp.minimum(r0 + RB, S - RB) + OFF, OFF)
        nh = RB // T
        now = [0]
        due = []
        pace = []

        def p1_item(c):
            return lambda dep: due.append((now[0] + PD, p1_store(n0, c, dep)))

        pace += [(P0 + i * PSTEP, p1_item(i)) for i in range(RB // PC)]
        wt = lambda ref, f0, f1, n: ref[f0:f1, _tile(n)]

        def mm(lhs, wts, dot=_dot):
            acc = None
            for x, w in zip(lhs, wts):
                if due and due[0][0] <= now[0]:
                    w = _tie(w, due.pop(0)[1])
                v = dot(x, w)
                now[0] += x.shape[0] // HT
                acc = v if acc is None else v + acc
                if pace and pace[0][0] <= now[0]:
                    pace.pop(0)[1](v[0:8, :])
            return acc

        def split_ops(lo, hi):
            return [v.astype(BF16) for v in _a_ops(lo[:HT], hi[:HT], lo[HT:], hi[HT:])]

        def two_tiles(aops, wsel, rest):
            def col(w):
                v = mm(rest[0], w, rest[3])
                return v[:HT], v[HT:]

            c11, c12, c21, c22 = _strassen(
                lambda i: mm([a[i] for a in aops], [wsel(i, k) for k in range(len(aops))]),
                lambda: col(rest[1]), lambda: col(rest[2]))
            return jnp.concatenate([c11, c21], axis=0), jnp.concatenate([c12, c22], axis=0)

        def square(full, aops, w_ref, ws_ref):
            out = {}
            for n in range(2):
                out[n], out[n + 2] = two_tiles(
                    aops, lambda i, k: _ld(ws_ref, i, n, slice(k * HT, (k + 1) * HT)),
                    (full[4:], [wt(w_ref, 4 * T, M, n)], [wt(w_ref, 4 * T, M, n + 2)], _dot))
            out[4] = mm(full, [wt(w_ref, j * T, (j + 1) * T, 4) for j in range(km)])
            return out

        t_scr[0:CAR, :] = t_scr[RB:RB + CAR, :]
        for hf in range(nh):
            full = [a1_scr[j, _tile(hf), :] for j in range(km)]
            aops = []
            for k in range(2):
                ops = {m: a1s_scr[hf, i, k] for i, m in enumerate(SUMS)}
                ops[2], ops[3] = full[k][:HT], full[2 + k][HT:]
                aops.append(ops)
            for n, v in square(full, aops, w1_ref, ws12.at[0]).items():
                t = _gelu(v)
                if hf == nh - 1:
                    t = jnp.concatenate([t[:T - OFF], jnp.where(r < nrb - 1, t[T - OFF:], 0.0)], axis=0)
                t_scr[CAR + hf * T:CAR + (hf + 1) * T, _tile(n)] = t
        cq = M // 4
        shifts = (-1, 1, -2, 2)
        lane = jax.lax.broadcasted_iota(jnp.int32, (T, T), 1)
        y1, a3 = [], []
        for hf in range(nh):
            base = CAR - OFF + hf * T
            sh = []
            for j in range(km):
                g_lo, g_hi = (j * T) // cq, ((j + 1) * T - 1) // cq
                assert g_hi - g_lo <= 1
                v = t_scr[base + shifts[g_lo]:base + shifts[g_lo] + T, _tile(j)]
                if g_hi != g_lo:
                    v2 = t_scr[base + shifts[g_hi]:base + shifts[g_hi] + T, _tile(j)]
                    v = jnp.where(lane < g_hi * cq - j * T, v, v2)
                sh.append(v)
            hs = square([v.astype(BF16) for v in sh], [split_ops(sh[k], sh[2 + k]) for k in range(2)],
                        w2_ref, ws12.at[1])
            hs = jnp.concatenate([hs[n] for n in range(km)], axis=1)
            y1.append(hs + hb_scr[pl.ds(pl.multiple_of(r0 + hf * T, T), T), :])
            a3.append({})

            def ln_item(hf, c):
                def item(dep):
                    n = HT // NLN
                    for d in (0, HT):
                        v = y1[hf][d + c * n:d + (c + 1) * n]
                        if dep is not None:
                            v = jnp.concatenate([_after(v[:, :T], _rows(dep, n)), v[:, T:]], axis=1)
                        a3[hf][d + c * n] = _ln(v)
                return item

            ln_item(hf, 0)(None)
            pace += [(now[0] + LN0 + (c - 1) * LNS * (1 + hf), ln_item(hf, c)) for c in range(1, NLN)]
            pace.sort(key=lambda e: e[0])
        nf = FH // T
        h3, h3ops = [], []
        for hf in range(nh):
            assert len(a3[hf]) == 2 * NLN
            af = jnp.concatenate([a3[hf][key] for key in sorted(a3[hf])], axis=0)
            full = [af[:, _tile(j)].astype(BF16) for j in range(km)]
            aops = [split_ops(af[:, _tile(k)], af[:, _tile(2 + k)]) for k in range(2)]
            row, ops = {}, []
            narrow = None
            for n in range(nf):
                lo, hi = two_tiles(aops, lambda i, k: _ld(ws3, n, i, k),
                                   (full[4:], [wt(w3_ref, *ftiles[n], 4)],
                                    [wt(w3_ref, *ftiles[nf + n], 4)], _dot_nt))
                lo, hi = _gelu(lo), _gelu(hi)
                row[n], row[nf + n] = lo.astype(BF16), hi.astype(BF16)
                ops.append(split_ops(lo, hi))
                if n < km:
                    v = mm([wt(w3_ref, *ftiles[-1], n)], [full[n]], _dot_nt)
                    narrow = v if narrow is None else v + narrow
            row[2 * nf] = _gelu(mm(full, [wt(w3_ref, *ftiles[2 * nf], j) for j in range(km)],
                                   _dot_nt)).astype(BF16)
            fw = Fd - ftiles[-1][0]
            gT = jnp.concatenate([_gelu(narrow), jnp.zeros((T - fw, T), F32)], axis=0)
            row[2 * nf + 1] = _tie(gT.astype(BF16).T, gT[0:8, :])[:, :fw]
            h3.append([row[i] for i in range(len(ftiles))])
            h3ops.append(ops)
        for hf in range(nh):
            rows = pl.ds(pl.multiple_of(r0 + hf * T, T), T)

            def finish(n, v):
                out_buf[rows, _tile(n)] = (
                    x1_scr[rows, _tile(n)] + gb[:, _tile(n)] * (v + y1[hf][:, _tile(n)])
                ).astype(out_buf.dtype)

            w4t = lambda n, f_: [wt(w4_ref, f0, f1, n) for f0, f1 in f_]
            finish(4, mm(h3[hf], w4t(4, ftiles)))
            for n in range(2):
                lo, hi = two_tiles(h3ops[hf], lambda i, k: _ld(ws4, i, n, slice(k * HT, (k + 1) * HT)),
                                   (h3[hf][2 * nf:], w4t(n, ftiles[2 * nf:]), w4t(n + 2, ftiles[2 * nf:]), _dot))
                finish(n, lo)
                finish(n + 2, hi)
            out_copy(r * nh + hf).start()
        assert not pace
        return carry

    jax.lax.fori_loop(0, nrb, b_body, 0)
    for i in range(nb):
        out_copy(i).wait()


@jax.jit
def pallas_adaLN_cond__compressed_kv_cla__mixer_s_mlp__prompt_kernel(
    A_x: jax.Array,
    A_c_kv: jax.Array,
    A_w_q: jax.Array,
    A_w_uk: jax.Array,
    A_w_uv: jax.Array,
    A_w_o: jax.Array,
    B_x: jax.Array,
    B_w1: jax.Array,
    B_w2: jax.Array,
    B_w3: jax.Array,
    B_w4: jax.Array,
    c: jax.Array,
    w_mod: jax.Array,
):
    _, S, M = A_x.shape
    Dc = A_c_kv.shape[2]
    H, D = A_w_q.shape[1], A_w_q.shape[2]
    Fd = B_w3.shape[1]
    assert D == T and A_c_kv.shape[1] == S and Dc == 4 * T and M == 5 * T and 13 * T < Fd < 14 * T
    vmem = pltpu.VMEM
    packed = lambda *lead: vmem(lead + (T // 2, T), U32)
    out = pl.pallas_call(
        _kernel,
        in_specs=[pl.BlockSpec(memory_space=pltpu.HBM)] * 12,
        out_specs=pl.BlockSpec(memory_space=pltpu.HBM),
        out_shape=jax.ShapeDtypeStruct((S, M), A_x.dtype),
        scratch_shapes=[
            vmem((S + 16, M), BF16),
            vmem((S, Dc), BF16),
            vmem((1, M), BF16),
            vmem((M, 2 * M), BF16),
            vmem((M, 4 * M), BF16),
            vmem((M, M), BF16),
            vmem((M, M), BF16),
            vmem((Fd, M), BF16),
            vmem((Fd, M), BF16),
            vmem((M, D), U32),
            vmem((Dc, D), U32),
            vmem((Dc, D), U32),
            vmem((2, 2 * D, M), BF16),
            vmem((S, M), A_x.dtype),
            pltpu.SemaphoreType.DMA((15,)),
            pltpu.SemaphoreType.DMA((4,)),
            pltpu.SemaphoreType.DMA((S // T,)),
            vmem((8, 6 * M), F32),
            vmem((S // T // 2, 16, T, T), BF16),
            vmem((S // T // 2, 5, 2, T, T), BF16),
            packed(44),
            packed(2 * S // T),
            packed(2 * S // T),
            packed(2 * S // T),
            vmem((S + 16, M), F32),
            vmem((S + 16, M), F32),
            vmem((S + 16, M), F32),
            vmem((M // T, RB, T), BF16),
            vmem((RB + 32, M), F32),
            vmem((RB // T, 5, 2, T // 2, T), BF16),
            vmem((2, 7, 2, T, T), U32),
            packed(6, 7, 2),
            vmem((7, 2, 3 * T, T), U32),
        ],
        compiler_params=pltpu.CompilerParams(
            vmem_limit_bytes=100 * 1024 * 1024,
            disable_bounds_checks=True,
        ),
    )(
        A_x.reshape(S, M), A_c_kv.reshape(S, Dc),
        A_w_q, A_w_uk, A_w_uv,
        A_w_o.reshape(H // 2, 2 * D, M),
        B_w1, B_w2, B_w3.T, B_w4, c, w_mod,
    )
    return out.reshape(1, S, M)
```

```python
import math

import jax
import jax.numpy as jnp
import jax.experimental.pallas as pl
import jax.experimental.pallas.tpu as pltpu

F32 = jnp.float32
BF16 = jnp.bfloat16
U32 = jnp.uint32
NT = (((1,), (1,)), ((), ()))
T = 128
EPS = 1e-5
LOG2E = math.log2(math.e)

GRP = 4
OGRP = 6
LEAD = 10
PROW = 3
VT = 8
RES = 30
LAT_A = 16
LAT_B = 20
ALEAD = 32
MID = 40
SD0, SDS = 50, 10
RB = 256
PC = 32
P0, PSTEP, PD = 440, 30, 52
NLN, LN0, LNS = 4, 4, 5
LP = 16
PROLOGUE = ('|kva|Z; |b|; kva|cdn|K01; b|m|K23; cd|qw|K45; nm|x|M K6; qw|yzo|K7 H01 Q0; '
            'x||H23 Q12; yz||H4567 Q34567; o||')


def _dot(a, b):
    return jnp.dot(a, b, preferred_element_type=F32)


def _dot_nt(a, b):
    return jax.lax.dot_general(a, b, NT, preferred_element_type=F32)


def _ln(x):
    m = jnp.mean(x, axis=-1, keepdims=True)
    xc = x - m
    v = jnp.mean(xc * xc, axis=-1, keepdims=True)
    return xc * jnp.exp2(jnp.log(v + EPS) * (-0.5 * LOG2E))


def _rows(v, n):
    return jnp.broadcast_to(v[None], (n // 8, 8, v.shape[1])).reshape(n, v.shape[1])


def _gelu(x):
    c0 = math.sqrt(2.0 / math.pi)
    return 0.5 * x * (1.0 + jnp.tanh(c0 * (x + 0.044715 * (x * x * x))))


def _after(x, dep):
    return jnp.where(dep > jnp.inf, dep, x)


def _tie(x, dep):
    xu = pltpu.bitcast(x, U32)
    first = jnp.where(dep > jnp.inf, jnp.uint32(0), xu[:8])
    return pltpu.bitcast(jnp.concatenate([first, xu[8:]], axis=0), BF16)


def _tile(j):
    return slice(j * T, (j + 1) * T)


def _ld(ref, *idx):
    return pltpu.bitcast(ref[idx], BF16)


def _pk(x):
    return pltpu.bitcast(x, U32)


def _a_ops(a11, a12, a21, a22):
    return [a11 + a22, a21 + a22, a11, a22, a11 + a12, a21 - a11, a12 - a22]


SUMS = (0, 1, 4, 5, 6)


def _b_ops(b11, b12, b21, b22):
    return [b11 + b22, b11, b12 - b22, b21 - b11, b22, b11 + b12, b21 + b22]


def _strassen(prod, col1=None, col2=None):
    m4 = prod(3)
    m2 = prod(1)
    c21 = m2 + m4
    if col1 is not None:
        e11, e21 = col1()
        m4, c21 = m4 + e11, c21 + e21
    m3 = prod(2)
    m5 = prod(4)
    c12 = m3 + m5
    if col2 is not None:
        e12, e22 = col2()
        c12, m3 = c12 + e12, m3 + e22
    m1 = prod(0)
    c11 = prod(6) + (m1 + (m4 - m5))
    c22 = prod(5) + (m1 + (m3 - m2))
    return c11, c12, c21, c22


def _pair_weights(w_ref, transpose=False):
    lo, hi = [], []
    for j in range(w_ref.shape[0] // T):
        wu = w_ref[_tile(j), :]
        lo.append(pltpu.bitcast(wu << 16, F32))
        hi.append(pltpu.bitcast(wu & jnp.uint32(0xFFFF0000), F32))
    per_j = [_b_ops(lo[j], hi[j], lo[2 + j], hi[2 + j]) for j in range(2)]
    tiles = [per_j[j][i] for i in range(7) for j in range(2)]
    for j in range(4, len(lo)):
        tiles += [lo[j], hi[j]]
    tiles = [t.astype(BF16) for t in tiles]
    return [t.T for t in tiles] if transpose else tiles


class _Jobs:
    def __init__(self, side=()):
        self.res = []
        self.side = list(side)

    def mm(self, lhs, wt, dot, tie=False):
        acc = None
        for x, w in zip(lhs, wt):
            if tie and len(self.res) >= VT:
                x = _tie(x, self.res[len(self.res) - VT][0:8, :])
            v = dot(x, w)
            self.res.append(v)
            acc = v if acc is None else v + acc
            if self.side and self.side[0][0] <= len(self.res):
                self.side.pop(0)[1](v[0:8, :])
        return acc


def _kv_jobs(jobs, p, c_ref, cs_scr, wk, wvT, k_scr, v_scr):
    ct = lambda i: [cs_scr[p, SUMS.index(i), j] if i in SUMS
                    else c_ref[_tile(2 * p + i - 2), _tile(2 * (i - 2) + j)] for j in range(2)]
    ks = _strassen(lambda i: jobs.mm(ct(i), [wk(2 * i), wk(2 * i + 1)], _dot))
    for n, v in enumerate(ks):
        k_scr[4 * p + n] = _pk(v.astype(BF16))
    vs = _strassen(lambda i: jobs.mm([wvT(2 * i), wvT(2 * i + 1)], ct(i), _dot_nt, True))
    for n, v in enumerate(vs):
        v_scr[4 * p + n] = _pk(v.astype(BF16))


def _q_jobs(jobs, p, h_scr, wq, q_scr, scale):
    rest = lambda hd: (lambda: [jobs.mm([h_scr[p, 14 + x]], [wq(14 + hd)], _dot) for x in range(2)])
    if not jobs.res:
        early = [rest(hd)() for hd in range(2)]
        rest = lambda hd: (lambda: early[hd])
    qs = _strassen(lambda i: jobs.mm([h_scr[p, 2 * i + j] for j in range(2)],
                                     [wq(2 * i), wq(2 * i + 1)], _dot), rest(0), rest(1))
    for n, v in enumerate(qs):
        q_scr[4 * p + n] = _pk((v * scale).astype(BF16))


def _proj_step(h_scr, c_ref, cs_scr, wq_ref, wuk_ref, wuv_ref, q_scr, k_scr, v_scr, scale, side):
    wq = _pair_weights(wq_ref)
    wk = _pair_weights(wuk_ref)
    wvT = _pair_weights(wuv_ref, True)
    jobs = _Jobs((SD0 + i * SDS, fn) for i, fn in enumerate(side))
    for p in range(h_scr.shape[0]):
        _q_jobs(jobs, p, h_scr, wq.__getitem__, q_scr, scale)
        _kv_jobs(jobs, p, c_ref, cs_scr, wk.__getitem__, wvT.__getitem__, k_scr, v_scr)
    assert not jobs.side


_O_JOBS = ([(0, 'r', 0, 0), (0, 'm', 2, 0), (0, 'm', 2, 1), (1, 'r', 1, 0), (1, 'm', 4, 0), (1, 'm', 4, 1),
            (2, 'r', 2, 0), (2, 'm', 5, 0), (2, 'm', 5, 1), (3, 'r', 3, 0)]
           + [(3, 'm', i, n) for n in range(2) for i in (3, 1, 0, 6)])


def _job_order(nb):
    units = range(2 * nb)
    qa = [('a', u, c) for u in units for c in range(u // 2 + 1)]
    qb = [('b', u, c) for u in units for c in range(u // 2 + 1)]
    last = nb // 2 - 1
    qo = [('o', 4 * p + (job[0] if p == last else 3), j)
          for p in range(nb // 2) for j, job in enumerate(_O_JOBS)]
    done = {}
    order = []

    def ready(q, lat, pre):
        return bool(q) and (pre, q[0][1]) in done and done[(pre, q[0][1])] + lat <= len(order)

    def emit(q):
        kind, u, j = job = q.pop(0)
        if kind != 'o' and j == u // 2:
            done[(kind, u)] = len(order)
        order.append(job)

    turn = 0
    while qa or qb or qo:
        pref = 'abo'[turn % 3]
        turn += 1
        for _ in range(OGRP if pref == 'o' else GRP):
            b_ok, o_ok = ready(qb, LAT_A, 'a'), ready(qo, LAT_B, 'b')
            if pref == 'a' and qa and (len(qb) - len(qa) < ALEAD or not b_ok):
                emit(qa)
            elif pref == 'b' and b_ok:
                emit(qb)
            elif pref == 'o' and o_ok and (len(qo) > RES or not (qa or b_ok)):
                emit(qo)
            elif not (qa or b_ok or o_ok) and (qb or qo):
                emit(qb or qo)
            else:
                break
    return order


def _attention_step(q_scr, k_scr, v_scr, wo_ref, acc_scr, mid):
    causal = (jax.lax.broadcasted_iota(jnp.int32, (T, T), 0)
              <= jax.lax.broadcasted_iota(jnp.int32, (T, T), 1))
    sv, mx, mfin, lsum, pv, of, lhs, prod = {}, {}, {}, {}, {}, {}, {}, {}
    res = []
    wo = [[t.astype(BF16) for t in _b_ops(*[wo_ref[_tile(i // 2), _tile(2 * n + i % 2)].astype(F32)
                                            for i in range(4)])] for n in range(2)]

    def job_a(u, c):
        r, hd = divmod(u, 2)
        s = _dot_nt(_ld(k_scr, 2 * c + hd), _ld(q_scr, u))
        res.append(s)
        if c == r:
            s = jnp.where(causal, s, -1e9 * LOG2E)
        s = s.reshape(T // 8, 8, T)
        sv[(u, c)] = s
        pm = jnp.max(s, axis=0)
        mx[u] = pm if u not in mx else jnp.maximum(mx[u], pm)

    def job_b(u, c):
        r, hd = divmod(u, 2)
        if u not in mfin:
            mfin[u] = jnp.broadcast_to(jnp.max(mx[u], axis=0, keepdims=True), (8, T))
        m = mfin[u]
        if len(res) >= LEAD:
            r0 = 8 * PROW * (c % 4)
            m = _after(m, res[len(res) - LEAD][r0:r0 + 8, :])
        p = jnp.exp2(sv.pop((u, c)) - m[None])
        ls = jnp.sum(p, axis=0)
        lsum[u] = ls if u not in lsum else lsum[u] + ls
        v = _dot(_ld(v_scr, 2 * c + hd), p.reshape(T, T).astype(BF16))
        res.append(v)
        pv[u] = v if u not in pv else v + pv[u]
        if c == r:
            of[u] = pv[u] * (1.0 / jnp.sum(lsum[u], axis=0, keepdims=True))

    def o_lhs(p, kind, i):
        if kind == 'm' and i in (2, 3):
            kind, i = 'r', 3 * (i - 2)
        if (p, kind, i) not in lhs:
            a = lambda n: of[4 * p + n]
            v = a(i) if kind == 'r' else {0: lambda: a(0) + a(3), 1: lambda: a(2) + a(3), 4: lambda: a(0) + a(1),
                                          5: lambda: a(2) - a(0), 6: lambda: a(1) - a(3)}[i]()
            lhs[(p, kind, i)] = _tie(v.astype(BF16).T, v[0:8, :])
        return lhs[(p, kind, i)]

    def job_o(u, j):
        p = u // 4
        _, kind, i, n = _O_JOBS[j]
        w = wo[n][i] if kind == 'm' else wo_ref[_tile(i % 2), _tile(4)]
        v = _dot(o_lhs(p, kind, i), w)
        res.append(v)
        prod[(kind, i, n)] = v
        m = lambda i_: prod[('m', i_, n)]
        if kind == 'r':
            if i % 2:
                acc_scr[_tile(2 * p + i // 2), _tile(4)] += v + prod[('r', i - 1, 0)]
        elif i == 4:
            acc_scr[_tile(2 * p), _tile(2 * n + 1)] += v + m(2)
        elif i == 5:
            prod[('m', 5, n)] = v + m(2)
        elif i == 1:
            acc_scr[_tile(2 * p + 1), _tile(2 * n)] += v + m(3)
        elif i == 0:
            acc_scr[_tile(2 * p + 1), _tile(2 * n + 1)] += v + (m(5) - m(1))
        elif i == 6:
            acc_scr[_tile(2 * p), _tile(2 * n)] += v + (m(0) + (m(3) - m(4)))

    fns = dict(a=job_a, b=job_b, o=job_o)
    for n, (kind, u, j) in enumerate(_job_order(q_scr.shape[0] // 2)):
        if n == MID:
            mid()
        fns[kind](u, j)


def _kernel(x_hbm, c_hbm, wq_hbm, wuk_hbm, wuv_hbm, wo_hbm, w1_hbm, w2_hbm, w3_hbm, w4_hbm,
            cond_hbm, wmod_hbm, out_hbm,
            x_ref, c_ref, cond_ref, wma_ref, wmb_ref, w1_ref, w2_ref, w3_ref, w4_ref,
            wq_buf, wk_buf, wv_buf, wo_buf, out_buf, sem, wsem, osem,
            mod_scr, h_scr, cs_scr, w_scr, q_scr, k_scr, v_scr, acc_scr, x1_scr, hb_scr, a1_scr, t_scr,
            a1s_scr, ws12, ws3, ws4):
    S, M = x_hbm.shape
    D = wq_hbm.shape[2]
    nattn = wo_hbm.shape[0]
    Fd = w4_hbm.shape[0]
    scale = float(D) ** -0.5 * LOG2E
    nb, nrb = S // T, S // RB
    km, kc = M // T, c_hbm.shape[1] // T
    NX = 4
    XR = S // NX
    CB = XR // T

    def pcopies(g):
        return [pltpu.make_async_copy(src.bitcast(U32).at[:, g, :], dst, wsem.at[j])
                for j, (src, dst) in enumerate(((wuk_hbm, wk_buf), (wuv_hbm, wv_buf), (wq_hbm, wq_buf)))]

    def ocopy(g, slot):
        return pltpu.make_async_copy(wo_hbm.at[g], wo_buf.at[slot], wsem.at[3])

    def chunk_copy(src, dst, i, s0):
        rows = slice(i * XR, (i + 1) * XR)
        return pltpu.make_async_copy(src.at[rows, :], dst.at[rows, :], sem.at[s0 + i])

    cp_cond = pltpu.make_async_copy(cond_hbm, cond_ref, sem.at[0])
    cp_wma = pltpu.make_async_copy(wmod_hbm.at[:, 0:2 * M], wma_ref, sem.at[1])
    cp_late = [pltpu.make_async_copy(src, dst, sem.at[2 + j]) for j, (src, dst) in enumerate((
        (wmod_hbm.at[:, 2 * M:6 * M], wmb_ref), (w1_hbm, w1_ref), (w2_hbm, w2_ref),
        (w3_hbm, w3_ref), (w4_hbm, w4_ref)))]
    cp_x = [chunk_copy(x_hbm, x_ref, i, 7) for i in range(NX)]
    cp_c = [chunk_copy(c_hbm, c_ref, i, 7 + NX) for i in range(NX)]

    def silu_cond():
        cf = cond_ref[...].astype(F32)
        return jnp.broadcast_to((cf * jax.nn.sigmoid(cf)).astype(BF16), (8, M))

    cp_wk, cp_wv, cp_wq = pcopies(0)
    named = dict(k=cp_wk, v=cp_wv, q=cp_wq, o=ocopy(0, 0), n=cp_cond, m=cp_wma)
    named.update(zip('abcd', cp_c))
    named.update(zip('wxyz', cp_x))
    started, arrived, did = set(), set(), set()

    def zero(r, carry):
        acc_scr[pl.ds(pl.multiple_of(r * T, T), T), :] = jnp.zeros((T, M), F32)
        return carry

    def h_pair(p):
        sa = _rows(mod_scr[:, 0:M], LP)
        ca1 = _rows(mod_scr[:, M:2 * M], LP)
        for i in range(T // LP):
            h1, h2 = [_ln(x_ref[r * T + i * LP:r * T + (i + 1) * LP, :].astype(F32)) * ca1 + sa
                      for r in (2 * p, 2 * p + 1)]
            ops = _a_ops(h1[:, 0:2 * T], h1[:, 2 * T:4 * T], h2[:, 0:2 * T], h2[:, 2 * T:4 * T])
            tiles = [v[:, _tile(j)] for v in ops for j in range(2)] + [h1[:, _tile(4)], h2[:, _tile(4)]]
            for n, v in enumerate(tiles):
                h_scr[p, n, i * LP:(i + 1) * LP, :] = v.astype(BF16)

    def stash(key, buf, j0, transpose=False):
        if key not in did:
            assert key in arrived
            did.add(key)
            for j, t in enumerate(_pair_weights(buf, transpose)):
                w_scr[j0 + j] = _pk(t)
        return lambda j: _ld(w_scr, j0 + j)

    def kv_pair(jobs, p):
        wk, wvT = stash('k', wk_buf, 0), stash('v', wv_buf, 14, True)
        for j in range(2):
            ops = _a_ops(*[c_ref[_tile(2 * p + n // 2), _tile(2 * (n % 2) + j)].astype(F32)
                           for n in range(4)])
            for n, i in enumerate(SUMS):
                cs_scr[p, n, j] = ops[i].astype(BF16)
        _kv_jobs(jobs, p, c_ref, cs_scr, wk, wvT, k_scr, v_scr)

    ppc = CB // 2
    for blk in PROLOGUE.split(';'):
        waits, starts, acts = blk.split('|')
        for ch in waits.strip():
            assert ch in started and ch not in arrived
            arrived.add(ch)
            named[ch].wait()
        for ch in starts.strip():
            assert ch not in started
            started.add(ch)
            named[ch].start()
        jobs = _Jobs()
        for act in acts.split():
            if act == 'Z':
                jax.lax.fori_loop(0, nb, zero, 0)
                acc_scr[S:, :] = jnp.zeros((acc_scr.shape[0] - S, M), F32)
                x_ref[S:, :] = jnp.zeros((x_ref.shape[0] - S, M), BF16)
            elif act == 'M':
                assert arrived >= set('nm')
                mod = _dot(silu_cond(), wma_ref[...])
                mod_scr[:, 0:M] = mod[:, 0:M]
                mod_scr[:, M:2 * M] = 1.0 + mod[:, M:2 * M]
                did.add('M')
            else:
                for half in act[1:]:
                    for p in range(int(half) * ppc // 2, (int(half) + 1) * ppc // 2):
                        did.add((act[0], p))
                        if act[0] == 'K':
                            assert 'abcd'[p // ppc] in arrived
                            kv_pair(jobs, p)
                        elif act[0] == 'H':
                            assert 'wxyz'[p // ppc] in arrived and 'M' in did
                            h_pair(p)
                        else:
                            assert act[0] == 'Q' and ('H', p) in did
                            _q_jobs(jobs, p, h_scr, stash('q', wq_buf, 28), q_scr, scale)
    assert arrived == set(named) and all((k_, p) in did for k_ in 'KHQ' for p in range(nb // 2))
    for cp in cp_late[1:] + cp_late[:1]:
        cp.start()

    FH = ws3.shape[0] * T
    assert nattn - 1 >= FH // 64

    def mixer_prep(g):
        def blocks(w_ref, r0, n, half, c0, c1, dep):
            lo, hi = pl.ds(r0, n), pl.ds(r0 + half, n)
            return [_after(w_ref[rows, _tile(c)].astype(F32), _rows(dep, n)) if (rows is lo) == (c == c0)
                    else w_ref[rows, _tile(c)].astype(F32) for rows in (lo, hi) for c in (c0, c1)]

        def rows_items(w_ref, dst, per_step, half, n=16):
            gi = jnp.minimum(g, half // per_step - 1)
            src = w_ref.at[pl.ds(pl.multiple_of(gi * per_step, per_step), half + per_step), :]
            hs = per_step // 2

            def item(c, o):
                def fn(dep):
                    for i, v in enumerate(_b_ops(*blocks(src, o, n, half, c, c + 2, dep))):
                        dst[i, c, pl.ds(pl.multiple_of(gi * hs, hs) + o // 2, n // 2), :] = _pk(v.astype(BF16))
                return fn
            return [item(c, o) for c in range(2) for o in range(0, per_step, n)]

        def w3_item(k, i):
            def fn(dep):
                n = jnp.minimum(g, FH // T - 1)
                b11, b21, b12, b22 = blocks(w3_ref, pl.multiple_of(n * T, T), T, FH, k, k + 2, dep)
                ws3[n, i, k] = _pk(_b_ops(b11, b12, b21, b22)[i].astype(BF16).T)
            return fn

        return (rows_items(w1_ref, ws12.at[0], 32, 2 * T) + rows_items(w2_ref, ws12.at[1], 32, 2 * T)
                + rows_items(w4_ref, ws4, 64, FH) + [w3_item(k, i) for k in range(2) for i in range(7)])

    def attn_body(g, carry):
        slot = g & 1
        nxt = jnp.minimum(g + 1, nattn - 1)
        copies = pcopies(nxt) + [ocopy(nxt, 1 - slot)]

        def mid():
            for cp in copies:
                cp.start()

        _attention_step(q_scr, k_scr, v_scr, wo_buf.at[slot], acc_scr, mid)
        for cp in copies:
            cp.wait()

        @pl.when(g == 0)
        def _():
            for cp in cp_late[1:]:
                cp.wait()

        @pl.when(g + 1 < nattn)
        def _():
            _proj_step(h_scr, c_ref, cs_scr, wq_buf, wk_buf, wv_buf, q_scr, k_scr, v_scr, scale, mixer_prep(g))

        return carry

    jax.lax.fori_loop(0, nattn, attn_body, 0)

    cp_late[0].wait()
    mod = _dot(silu_cond(), wmb_ref[...])
    mod_scr[:, 2 * M:4 * M] = mod[:, 0:2 * M]
    mod_scr[:, 4 * M:5 * M] = 1.0 + mod[:, 2 * M:3 * M]
    mod_scr[:, 5 * M:6 * M] = mod[:, 3 * M:4 * M]
    ftiles = [(f, min(f + T, Fd)) for f in range(0, Fd, T)]
    OFF = x_ref.shape[0] - S
    CAR = t_scr.shape[0] - RB

    def p1(r0, n, dep=None):
        ga = mod_scr[:, 2 * M:3 * M]
        if dep is not None:
            ga = jnp.concatenate([_after(ga[:, 0:T], dep), ga[:, T:]], axis=1)
        rows = pl.ds(r0, n)
        x1 = x_ref[rows, :].astype(F32) + _rows(ga, n) * acc_scr[rows, :]
        x1_scr[rows, :] = x1
        hb = _ln(x1) * _rows(mod_scr[:, 4 * M:5 * M], n) + _rows(mod_scr[:, 3 * M:4 * M], n)
        hb_scr[rows, :] = hb
        return _ln(hb)

    HT = T // 2

    def p1_store(r0, c, dep=None):
        n = PC // 2
        hf, o = divmod(c * n, HT)
        top, bot = [p1(r0 + hf * T + d + o, n, dep) for d in (0, HT)]
        for d, v in ((0, top), (HT, bot)):
            for j in range(km):
                a1_scr[j, hf * T + d + o:hf * T + d + o + n, :] = v[:, _tile(j)].astype(BF16)
        ops = _a_ops(top[:, 0:2 * T], top[:, 2 * T:4 * T], bot[:, 0:2 * T], bot[:, 2 * T:4 * T])
        for i, m in enumerate(SUMS):
            for k in range(2):
                a1s_scr[hf, i, k, o:o + n, :] = ops[m][:, _tile(k)].astype(BF16)
        return jnp.max(ops[0][:, :T].reshape(n // 8, 8, T), axis=0)

    t_scr[RB:RB + CAR - OFF, :] = jnp.zeros((CAR - OFF, M), F32)
    t_scr[RB + CAR - OFF:RB + CAR, :] = _gelu(_dot(p1(0, OFF).astype(BF16), w1_ref[...]))
    for c in range(RB // PC):
        p1_store(OFF, c)

    def out_copy(i):
        rows = pl.ds(i * T if isinstance(i, int) else pl.multiple_of(i * T, T), T)
        return pltpu.make_async_copy(out_buf.at[rows, :], out_hbm.at[rows, :], osem.at[i])

    def b_body(r, carry):
        gb = _rows(mod_scr[:, 5 * M:6 * M], T)
        r0 = pl.multiple_of(r * RB, RB)
        n0 = pl.multiple_of(jnp.minimum(r0 + RB, S - RB) + OFF, OFF)
        nh = RB // T
        now = [0]
        due = []
        pace = []

        def p1_item(c):
            return lambda dep: due.append((now[0] + PD, p1_store(n0, c, dep)))

        pace += [(P0 + i * PSTEP, p1_item(i)) for i in range(RB // PC)]
        wt = lambda ref, f0, f1, n: ref[f0:f1, _tile(n)]

        def mm(lhs, wts, dot=_dot):
            acc = None
            for x, w in zip(lhs, wts):
                if due and due[0][0] <= now[0]:
                    w = _tie(w, due.pop(0)[1])
                v = dot(x, w)
                now[0] += x.shape[0] // HT
                acc = v if acc is None else v + acc
                if pace and pace[0][0] <= now[0]:
                    pace.pop(0)[1](v[0:8, :])
            return acc

        def split_ops(lo, hi):
            return [v.astype(BF16) for v in _a_ops(lo[:HT], hi[:HT], lo[HT:], hi[HT:])]

        def two_tiles(aops, wsel, rest):
            def col(w):
                v = mm(rest[0], w, rest[3])
                return v[:HT], v[HT:]

            c11, c12, c21, c22 = _strassen(
                lambda i: mm([a[i] for a in aops], [wsel(i, k) for k in range(len(aops))]),
                lambda: col(rest[1]), lambda: col(rest[2]))
            return jnp.concatenate([c11, c21], axis=0), jnp.concatenate([c12, c22], axis=0)

        def square(full, aops, w_ref, ws_ref):
            out = {}
            for n in range(2):
                out[n], out[n + 2] = two_tiles(
                    aops, lambda i, k: _ld(ws_ref, i, n, slice(k * HT, (k + 1) * HT)),
                    (full[4:], [wt(w_ref, 4 * T, M, n)], [wt(w_ref, 4 * T, M, n + 2)], _dot))
            out[4] = mm(full, [wt(w_ref, j * T, (j + 1) * T, 4) for j in range(km)])
            return out

        t_scr[0:CAR, :] = t_scr[RB:RB + CAR, :]
        for hf in range(nh):
            full = [a1_scr[j, _tile(hf), :] for j in range(km)]
            aops = []
            for k in range(2):
                ops = {m: a1s_scr[hf, i, k] for i, m in enumerate(SUMS)}
                ops[2], ops[3] = full[k][:HT], full[2 + k][HT:]
                aops.append(ops)
            for n, v in square(full, aops, w1_ref, ws12.at[0]).items():
                t = _gelu(v)
                if hf == nh - 1:
                    t = jnp.concatenate([t[:T - OFF], jnp.where(r < nrb - 1, t[T - OFF:], 0.0)], axis=0)
                t_scr[CAR + hf * T:CAR + (hf + 1) * T, _tile(n)] = t
        cq = M // 4
        shifts = (-1, 1, -2, 2)
        lane = jax.lax.broadcasted_iota(jnp.int32, (T, T), 1)
        y1, a3 = [], []
        for hf in range(nh):
            base = CAR - OFF + hf * T
            sh = []
            for j in range(km):
                g_lo, g_hi = (j * T) // cq, ((j + 1) * T - 1) // cq
                assert g_hi - g_lo <= 1
                v = t_scr[base + shifts[g_lo]:base + shifts[g_lo] + T, _tile(j)]
                if g_hi != g_lo:
                    v2 = t_scr[base + shifts[g_hi]:base + shifts[g_hi] + T, _tile(j)]
                    v = jnp.where(lane < g_hi * cq - j * T, v, v2)
                sh.append(v)
            hs = square([v.astype(BF16) for v in sh], [split_ops(sh[k], sh[2 + k]) for k in range(2)],
                        w2_ref, ws12.at[1])
            hs = jnp.concatenate([hs[n] for n in range(km)], axis=1)
            y1.append(hs + hb_scr[pl.ds(pl.multiple_of(r0 + hf * T, T), T), :])
            a3.append({})

            def ln_item(hf, c):
                def item(dep):
                    n = HT // NLN
                    for d in (0, HT):
                        v = y1[hf][d + c * n:d + (c + 1) * n]
                        if dep is not None:
                            v = jnp.concatenate([_after(v[:, :T], _rows(dep, n)), v[:, T:]], axis=1)
                        a3[hf][d + c * n] = _ln(v)
                return item

            ln_item(hf, 0)(None)
            pace += [(now[0] + LN0 + (c - 1) * LNS * (1 + hf), ln_item(hf, c)) for c in range(1, NLN)]
            pace.sort(key=lambda e: e[0])
        nf = FH // T
        h3, h3ops = [], []
        for hf in range(nh):
            assert len(a3[hf]) == 2 * NLN
            af = jnp.concatenate([a3[hf][key] for key in sorted(a3[hf])], axis=0)
            full = [af[:, _tile(j)].astype(BF16) for j in range(km)]
            aops = [split_ops(af[:, _tile(k)], af[:, _tile(2 + k)]) for k in range(2)]
            row, ops = {}, []
            narrow = None
            for n in range(nf):
                lo, hi = two_tiles(aops, lambda i, k: _ld(ws3, n, i, k),
                                   (full[4:], [wt(w3_ref, *ftiles[n], 4)],
                                    [wt(w3_ref, *ftiles[nf + n], 4)], _dot_nt))
                lo, hi = _gelu(lo), _gelu(hi)
                row[n], row[nf + n] = lo.astype(BF16), hi.astype(BF16)
                ops.append(split_ops(lo, hi))
                if n < km:
                    v = mm([wt(w3_ref, *ftiles[-1], n)], [full[n]], _dot_nt)
                    narrow = v if narrow is None else v + narrow
            row[2 * nf] = _gelu(mm(full, [wt(w3_ref, *ftiles[2 * nf], j) for j in range(km)],
                                   _dot_nt)).astype(BF16)
            fw = Fd - ftiles[-1][0]
            gT = jnp.concatenate([_gelu(narrow), jnp.zeros((T - fw, T), F32)], axis=0)
            row[2 * nf + 1] = _tie(gT.astype(BF16).T, gT[0:8, :])[:, :fw]
            h3.append([row[i] for i in range(len(ftiles))])
            h3ops.append(ops)
        for hf in range(nh):
            rows = pl.ds(pl.multiple_of(r0 + hf * T, T), T)

            def finish(n, v):
                out_buf[rows, _tile(n)] = (
                    x1_scr[rows, _tile(n)] + gb[:, _tile(n)] * (v + y1[hf][:, _tile(n)])
                ).astype(out_buf.dtype)

            w4t = lambda n, f_: [wt(w4_ref, f0, f1, n) for f0, f1 in f_]
            finish(4, mm(h3[hf], w4t(4, ftiles)))
            for n in range(2):
                lo, hi = two_tiles(h3ops[hf], lambda i, k: _ld(ws4, i, n, slice(k * HT, (k + 1) * HT)),
                                   (h3[hf][2 * nf:], w4t(n, ftiles[2 * nf:]), w4t(n + 2, ftiles[2 * nf:]), _dot))
                finish(n, lo)
                finish(n + 2, hi)
            out_copy(r * nh + hf).start()
        assert not pace
        return carry

    jax.lax.fori_loop(0, nrb, b_body, 0)
    for i in range(nb):
        out_copy(i).wait()


@jax.jit
def pallas_adaLN_cond__compressed_kv_cla__mixer_s_mlp__prompt_kernel(
    A_x: jax.Array,
    A_c_kv: jax.Array,
    A_w_q: jax.Array,
    A_w_uk: jax.Array,
    A_w_uv: jax.Array,
    A_w_o: jax.Array,
    B_x: jax.Array,
    B_w1: jax.Array,
    B_w2: jax.Array,
    B_w3: jax.Array,
    B_w4: jax.Array,
    c: jax.Array,
    w_mod: jax.Array,
):
    _, S, M = A_x.shape
    Dc = A_c_kv.shape[2]
    H, D = A_w_q.shape[1], A_w_q.shape[2]
    Fd = B_w3.shape[1]
    assert D == T and A_c_kv.shape[1] == S and Dc == 4 * T and M == 5 * T and 13 * T < Fd < 14 * T
    vmem = pltpu.VMEM
    packed = lambda *lead: vmem(lead + (T // 2, T), U32)
    out = pl.pallas_call(
        _kernel,
        in_specs=[pl.BlockSpec(memory_space=pltpu.HBM)] * 12,
        out_specs=pl.BlockSpec(memory_space=pltpu.HBM),
        out_shape=jax.ShapeDtypeStruct((S, M), A_x.dtype),
        scratch_shapes=[
            vmem((S + 16, M), BF16),
            vmem((S, Dc), BF16),
            vmem((1, M), BF16),
            vmem((M, 2 * M), BF16),
            vmem((M, 4 * M), BF16),
            vmem((M, M), BF16),
            vmem((M, M), BF16),
            vmem((Fd, M), BF16),
            vmem((Fd, M), BF16),
            vmem((M, D), U32),
            vmem((Dc, D), U32),
            vmem((Dc, D), U32),
            vmem((2, 2 * D, M), BF16),
            vmem((S, M), A_x.dtype),
            pltpu.SemaphoreType.DMA((15,)),
            pltpu.SemaphoreType.DMA((4,)),
            pltpu.SemaphoreType.DMA((S // T,)),
            vmem((8, 6 * M), F32),
            vmem((S // T // 2, 16, T, T), BF16),
            vmem((S // T // 2, 5, 2, T, T), BF16),
            packed(44),
            packed(2 * S // T),
            packed(2 * S // T),
            packed(2 * S // T),
            vmem((S + 16, M), F32),
            vmem((S + 16, M), F32),
            vmem((S + 16, M), F32),
            vmem((M // T, RB, T), BF16),
            vmem((RB + 32, M), F32),
            vmem((RB // T, 5, 2, T // 2, T), BF16),
            vmem((2, 7, 2, T, T), U32),
            packed(6, 7, 2),
            vmem((7, 2, 3 * T, T), U32),
        ],
        compiler_params=pltpu.CompilerParams(
            vmem_limit_bytes=100 * 1024 * 1024,
            disable_bounds_checks=True,
        ),
    )(
        A_x.reshape(S, M), A_c_kv.reshape(S, Dc),
        A_w_q, A_w_uk, A_w_uv,
        A_w_o.reshape(H // 2, 2 * D, M),
        B_w1, B_w2, B_w3.T, B_w4, c, w_mod,
    )
    return out.reshape(1, S, M)
```

```python
import math

import jax
import jax.numpy as jnp
import jax.experimental.pallas as pl
import jax.experimental.pallas.tpu as pltpu

F32 = jnp.float32
BF16 = jnp.bfloat16
U32 = jnp.uint32
NT = (((1,), (1,)), ((), ()))
T = 128
EPS = 1e-5
LOG2E = math.log2(math.e)

GRP = 4
OGRP = 6
LEAD = 10
PROW = 3
VT = 8
RES = 30
LAT_A = 16
LAT_B = 20
ALEAD = 32
MID = 40
import os
SD0, SDS = int(os.environ.get('SD0', 180)), int(os.environ.get('SDS', 5))
RB = 256
PC = 32
P0, PSTEP, PD = 440, 30, 52
NLN, LN0, LNS = 4, 4, 5
LP = int(os.environ.get('LP', 32))
SP = int(os.environ.get('SP', 16))
SPP = int(os.environ.get('SPP', 32))
PROLOGUE = os.environ.get('PRO', '|kva|Z; |b|; kva|cdn|K0123; b|m|C0@58 K4567; cd|qw|C1@72 K89abc; nm|x|M Kde; '
            'qw|yzo|Kf H0123 Q01; x||H4567 Q2345; yz||H89abcdef Q6789abcdef S01; o||')


def _dot(a, b):
    return jnp.dot(a, b, preferred_element_type=F32)


def _dot_nt(a, b):
    return jax.lax.dot_general(a, b, NT, preferred_element_type=F32)


def _ln(x):
    m = jnp.mean(x, axis=-1, keepdims=True)
    xc = x - m
    v = jnp.mean(xc * xc, axis=-1, keepdims=True)
    return xc * jnp.exp2(jnp.log(v + EPS) * (-0.5 * LOG2E))


def _rows(v, n):
    return jnp.broadcast_to(v[None], (n // 8, 8, v.shape[1])).reshape(n, v.shape[1])


def _gelu(x):
    c0 = math.sqrt(2.0 / math.pi)
    return 0.5 * x * (1.0 + jnp.tanh(c0 * (x + 0.044715 * (x * x * x))))


def _after(x, dep):
    return jnp.where(dep > jnp.inf, dep, x)


def _tie(x, dep):
    xu = pltpu.bitcast(x, U32)
    first = jnp.where(dep > jnp.inf, jnp.uint32(0), xu[:8])
    return pltpu.bitcast(jnp.concatenate([first, xu[8:]], axis=0), BF16)


def _tile(j):
    return slice(j * T, (j + 1) * T)


def _ld(ref, *idx):
    return pltpu.bitcast(ref[idx], BF16)


def _pk(x):
    return pltpu.bitcast(x, U32)


def _a_ops(a11, a12, a21, a22):
    return [a11 + a22, a21 + a22, a11, a22, a11 + a12, a21 - a11, a12 - a22]


SUMS = (0, 1, 4, 5, 6)


def _b_ops(b11, b12, b21, b22):
    return [b11 + b22, b11, b12 - b22, b21 - b11, b22, b11 + b12, b21 + b22]


def _strassen(prod, col1=None, col2=None):
    m4 = prod(3)
    m2 = prod(1)
    c21 = m2 + m4
    if col1 is not None:
        e11, e21 = col1()
        m4, c21 = m4 + e11, c21 + e21
    m3 = prod(2)
    m5 = prod(4)
    c12 = m3 + m5
    if col2 is not None:
        e12, e22 = col2()
        c12, m3 = c12 + e12, m3 + e22
    m1 = prod(0)
    c11 = prod(6) + (m1 + (m4 - m5))
    c22 = prod(5) + (m1 + (m3 - m2))
    return c11, c12, c21, c22


def _group(xs, ys):
    ks = sorted({k for _, k in xs + ys})
    prods = []
    for i, k in xs:
        mates = [y for y in ys if y[1] != k]
        prods.append((tuple((1, i, kk) for kk in ks), ((1, k, 0),), ((1, i, 0), (-1, i, 1))))
        prods.append((((1, i, k),) + tuple((-1, i2, k) for i2, _ in mates), ((1, k, 0), (1, k, 1)), ((1, i, 1),)))
        for i2, k2 in mates:
            prods.append((((1, i, k2),), ((1, k2, 0), (-1, k, 0)), ((1, i2, 0), (1, i, 0))))
            prods.append((((1, i2, k), (1, i, k2)), ((1, k, 0), (1, k2, 1)), ((1, i2, 0), (1, i, 1))))
            prods.append((((1, i2, k),), ((1, k, 1), (-1, k2, 1)), ((1, i2, 1), (1, i, 1))))
    for i2, k2 in ys:
        mates = [x for x in xs if x[1] != k2]
        prods.append((tuple((1, i2, kk) for kk in ks), ((1, k2, 1),), ((1, i2, 1), (-1, i2, 0))))
        prods.append((((1, i2, k2),) + tuple((-1, i, k2) for i, _ in mates), ((1, k2, 0), (1, k2, 1)),
                      ((1, i2, 0),)))
    return prods


def _full_group(r0, ks):
    q = len(ks)
    return _group([(r0 + a, k) for a, k in enumerate(ks)], [(r0 + q + a, k) for a, k in enumerate(ks)])


_C_GROUPS = [_full_group(0, range(4)), _full_group(8, range(4))]
_H_GROUPS = [_full_group(0, range(5)),
             [t for r in (10, 11, 12) for t in _group([(r, 3)], [(r + 3, 4)])] + _full_group(10, range(3))]
_sum_index = lambda groups: {f: n for n, f in enumerate(
    dict.fromkeys(t[0] for g in groups for t in g if len(t[0]) > 1))}
_C_SUMS, _H_SUMS = _sum_index(_C_GROUPS), _sum_index(_H_GROUPS)


def _form(form, get):
    acc = None
    for sign, i, j in form:
        v = get(i, j)
        acc = v if acc is None else (acc + v if sign > 0 else acc - v)
    return acc


class _PairWeights:
    def __init__(self, w_ref, transpose=False):
        self.base = {}
        for j in range(w_ref.shape[0] // T):
            wu = w_ref[_tile(j), :]
            if transpose:
                wu = wu.T
            self.base[j, 0] = pltpu.bitcast(wu << 16, F32)
            self.base[j, 1] = pltpu.bitcast(wu & jnp.uint32(0xFFFF0000), F32)
        self.cache = {}

    def __call__(self, form):
        sign = 1
        if form[-1][0] < 0 and form[0][1:] > form[1][1:]:
            sign, form = -1, ((1,) + form[1][1:], (-1,) + form[0][1:])
        if form not in self.cache:
            self.cache[form] = _form(form, lambda k, h: self.base[k, h]).astype(BF16)
        return sign, self.cache[form]


def _run_group(jobs, prods, a_get, w, transposed, finish):
    left = {}
    for _, _, outs in prods:
        for _, i, h in outs:
            left[i, h] = left.get((i, h), 0) + 1
    acc = {}
    for af, bf, outs in prods:
        sign, wt = w(bf)
        m = jobs.mm([wt], [a_get(af)], _dot_nt) if transposed else jobs.mm([a_get(af)], [wt], _dot)
        for s_, i, h in outs:
            if (i, h) not in acc:
                acc[i, h] = (s_ * sign, m)
            else:
                s0, v = acc[i, h]
                acc[i, h] = (s0, v + m if s0 == s_ * sign else v - m) if s0 > 0 or s_ * sign < 0 else (1, m - v)
            left[i, h] -= 1
            if not left[i, h]:
                s0, v = acc.pop((i, h))
                assert s0 > 0
                finish(2 * i + h, v)


class _Jobs:
    def __init__(self, side=()):
        self.res = []
        self.side = list(side)

    def mm(self, lhs, wt, dot, tie=False):
        acc = None
        for x, w in zip(lhs, wt):
            if tie and len(self.res) >= VT:
                x = _tie(x, self.res[len(self.res) - VT][0:8, :])
            v = dot(x, w)
            self.res.append(v)
            acc = v if acc is None else v + acc
            rel = 4 * (len(self.res) % 4)
            while self.side and self.side[0][0] <= len(self.res):
                self.side.pop(0)[1](v[8 * rel:8 * rel + 8, :])
                rel = (rel + 2) % 16
        return acc


def _proj_step(h_scr, hs_scr, c_ref, cs_scr, wq_ref, wuk_ref, wuv_ref, q_scr, k_scr, v_scr, scale, side):
    wq, wk, wvT = _PairWeights(wq_ref), _PairWeights(wuk_ref), _PairWeights(wuv_ref, True)
    c_get = lambda f: cs_scr[_C_SUMS[f]] if len(f) > 1 else c_ref[_tile(f[0][1]), _tile(f[0][2])]
    h_get = lambda f: hs_scr[_H_SUMS[f]] if len(f) > 1 else h_scr[f[0][1], f[0][2]]

    def put(dst, mul=None):
        def fn(u, v):
            dst[u] = _pk((v if mul is None else v * mul).astype(BF16))
        return fn

    jobs = _Jobs((SD0 + i * SDS, fn) for i, fn in enumerate(side))
    for gi in range(2):
        _run_group(jobs, _C_GROUPS[gi], c_get, wk, False, put(k_scr))
        _run_group(jobs, _H_GROUPS[gi], h_get, wq, False, put(q_scr, scale))
        _run_group(jobs, _C_GROUPS[gi], c_get, wvT, True, put(v_scr))
    assert not jobs.side


_O_JOBS = ([(0, 'r', 0, 0), (0, 'm', 2, 0), (0, 'm', 2, 1), (1, 'r', 1, 0), (1, 'm', 4, 0), (1, 'm', 4, 1),
            (2, 'r', 2, 0), (2, 'm', 5, 0), (2, 'm', 5, 1), (3, 'r', 3, 0)]
           + [(3, 'm', i, n) for n in range(2) for i in (3, 1, 0, 6)])


def _job_order(nb):
    units = range(2 * nb)
    qa = [('a', u, c) for u in units for c in range(u // 2 + 1)]
    qb = [('b', u, c) for u in units for c in range(u // 2 + 1)]
    last = nb // 2 - 1
    qo = [('o', 4 * p + (job[0] if p == last else 3), j)
          for p in range(nb // 2) for j, job in enumerate(_O_JOBS)]
    done = {}
    order = []

    def ready(q, lat, pre):
        return bool(q) and (pre, q[0][1]) in done and done[(pre, q[0][1])] + lat <= len(order)

    def emit(q):
        kind, u, j = job = q.pop(0)
        if kind != 'o' and j == u // 2:
            done[(kind, u)] = len(order)
        order.append(job)

    turn = 0
    while qa or qb or qo:
        pref = 'abo'[turn % 3]
        turn += 1
        for _ in range(OGRP if pref == 'o' else GRP):
            b_ok, o_ok = ready(qb, LAT_A, 'a'), ready(qo, LAT_B, 'b')
            if pref == 'a' and qa and (len(qb) - len(qa) < ALEAD or not b_ok):
                emit(qa)
            elif pref == 'b' and b_ok:
                emit(qb)
            elif pref == 'o' and o_ok and (len(qo) > RES or not (qa or b_ok)):
                emit(qo)
            elif not (qa or b_ok or o_ok) and (qb or qo):
                emit(qb or qo)
            else:
                break
    return order


def _attention_step(q_scr, k_scr, v_scr, wo_ref, acc_scr, mid):
    causal = (jax.lax.broadcasted_iota(jnp.int32, (T, T), 0)
              <= jax.lax.broadcasted_iota(jnp.int32, (T, T), 1))
    sv, mx, mfin, lsum, pv, of, lhs, prod = {}, {}, {}, {}, {}, {}, {}, {}
    res = []
    wo = [[t.astype(BF16) for t in _b_ops(*[wo_ref[_tile(i // 2), _tile(2 * n + i % 2)].astype(F32)
                                            for i in range(4)])] for n in range(2)]

    def job_a(u, c):
        r, hd = divmod(u, 2)
        s = _dot_nt(_ld(k_scr, 2 * c + hd), _ld(q_scr, u))
        res.append(s)
        if c == r:
            s = jnp.where(causal, s, -1e9 * LOG2E)
        s = s.reshape(T // 8, 8, T)
        sv[(u, c)] = s
        pm = jnp.max(s, axis=0)
        mx[u] = pm if u not in mx else jnp.maximum(mx[u], pm)

    def job_b(u, c):
        r, hd = divmod(u, 2)
        if u not in mfin:
            mfin[u] = jnp.broadcast_to(jnp.max(mx[u], axis=0, keepdims=True), (8, T))
        m = mfin[u]
        if len(res) >= LEAD:
            r0 = 8 * PROW * (c % 4)
            m = _after(m, res[len(res) - LEAD][r0:r0 + 8, :])
        p = jnp.exp2(sv.pop((u, c)) - m[None])
        ls = jnp.sum(p, axis=0)
        lsum[u] = ls if u not in lsum else lsum[u] + ls
        v = _dot(_ld(v_scr, 2 * c + hd), p.reshape(T, T).astype(BF16))
        res.append(v)
        pv[u] = v if u not in pv else v + pv[u]
        if c == r:
            of[u] = pv[u] * (1.0 / jnp.sum(lsum[u], axis=0, keepdims=True))

    def o_lhs(p, kind, i):
        if kind == 'm' and i in (2, 3):
            kind, i = 'r', 3 * (i - 2)
        if (p, kind, i) not in lhs:
            a = lambda n: of[4 * p + n]
            v = a(i) if kind == 'r' else {0: lambda: a(0) + a(3), 1: lambda: a(2) + a(3), 4: lambda: a(0) + a(1),
                                          5: lambda: a(2) - a(0), 6: lambda: a(1) - a(3)}[i]()
            lhs[(p, kind, i)] = _tie(v.astype(BF16).T, v[0:8, :])
        return lhs[(p, kind, i)]

    def job_o(u, j):
        p = u // 4
        _, kind, i, n = _O_JOBS[j]
        w = wo[n][i] if kind == 'm' else wo_ref[_tile(i % 2), _tile(4)]
        v = _dot(o_lhs(p, kind, i), w)
        res.append(v)
        prod[(kind, i, n)] = v
        m = lambda i_: prod[('m', i_, n)]
        if kind == 'r':
            if i % 2:
                acc_scr[_tile(2 * p + i // 2), _tile(4)] += v + prod[('r', i - 1, 0)]
        elif i == 4:
            acc_scr[_tile(2 * p), _tile(2 * n + 1)] += v + m(2)
        elif i == 5:
            prod[('m', 5, n)] = v + m(2)
        elif i == 1:
            acc_scr[_tile(2 * p + 1), _tile(2 * n)] += v + m(3)
        elif i == 0:
            acc_scr[_tile(2 * p + 1), _tile(2 * n + 1)] += v + (m(5) - m(1))
        elif i == 6:
            acc_scr[_tile(2 * p), _tile(2 * n)] += v + (m(0) + (m(3) - m(4)))

    fns = dict(a=job_a, b=job_b, o=job_o)
    for n, (kind, u, j) in enumerate(_job_order(q_scr.shape[0] // 2)):
        if n == MID:
            mid()
        fns[kind](u, j)


def _kernel(x_hbm, c_hbm, wq_hbm, wuk_hbm, wuv_hbm, wo_hbm, w1_hbm, w2_hbm, w3_hbm, w4_hbm,
            cond_hbm, wmod_hbm, out_hbm,
            x_ref, c_ref, cond_ref, wma_ref, wmb_ref, w1_ref, w2_ref, w3_ref, w4_ref,
            wq_buf, wk_buf, wv_buf, wo_buf, out_buf, sem, wsem, osem,
            mod_scr, h_scr, cs_scr, hs_scr, w_scr, q_scr, k_scr, v_scr, acc_scr, x1_scr, hb_scr, a1_scr, t_scr,
            a1s_scr, ws12, ws3, ws4):
    S, M = x_hbm.shape
    D = wq_hbm.shape[2]
    nattn = wo_hbm.shape[0]
    Fd = w4_hbm.shape[0]
    scale = float(D) ** -0.5 * LOG2E
    nb, nrb = S // T, S // RB
    km, kc = M // T, c_hbm.shape[1] // T
    NX = 4
    XR = S // NX
    CB = XR // T

    def pcopies(g):
        return [pltpu.make_async_copy(src.bitcast(U32).at[:, g, :], dst, wsem.at[j])
                for j, (src, dst) in enumerate(((wuk_hbm, wk_buf), (wuv_hbm, wv_buf), (wq_hbm, wq_buf)))]

    def ocopy(g, slot):
        return pltpu.make_async_copy(wo_hbm.at[g], wo_buf.at[slot], wsem.at[3])

    def chunk_copy(src, dst, i, s0):
        rows = slice(i * XR, (i + 1) * XR)
        return pltpu.make_async_copy(src.at[rows, :], dst.at[rows, :], sem.at[s0 + i])

    cp_cond = pltpu.make_async_copy(cond_hbm, cond_ref, sem.at[0])
    cp_wma = pltpu.make_async_copy(wmod_hbm.at[:, 0:2 * M], wma_ref, sem.at[1])
    cp_late = [pltpu.make_async_copy(src, dst, sem.at[2 + j]) for j, (src, dst) in enumerate((
        (wmod_hbm.at[:, 2 * M:6 * M], wmb_ref), (w1_hbm, w1_ref), (w2_hbm, w2_ref),
        (w3_hbm, w3_ref), (w4_hbm, w4_ref)))]
    cp_x = [chunk_copy(x_hbm, x_ref, i, 7) for i in range(NX)]
    cp_c = [chunk_copy(c_hbm, c_ref, i, 7 + NX) for i in range(NX)]

    def silu_cond():
        cf = cond_ref[...].astype(F32)
        return jnp.broadcast_to((cf * jax.nn.sigmoid(cf)).astype(BF16), (8, M))

    cp_wk, cp_wv, cp_wq = pcopies(0)
    named = dict(k=cp_wk, v=cp_wv, q=cp_wq, o=ocopy(0, 0), n=cp_cond, m=cp_wma)
    named.update(zip('abcd', cp_c))
    named.update(zip('wxyz', cp_x))
    started, arrived, did = set(), set(), set()

    def zero(r, carry):
        acc_scr[pl.ds(pl.multiple_of(r * T, T), T), :] = jnp.zeros((T, M), F32)
        return carry

    def h_tile(r):
        sa = _rows(mod_scr[:, 0:M], LP)
        ca1 = _rows(mod_scr[:, M:2 * M], LP)
        for i in range(T // LP):
            rows = slice(i * LP, (i + 1) * LP)
            hf = _ln(x_ref[r * T + i * LP:r * T + (i + 1) * LP, :].astype(F32)) * ca1 + sa
            for j in range(km):
                h_scr[r, j, rows, :] = hf[:, _tile(j)].astype(BF16)
            for f, n in _H_SUMS.items():
                if all(t[1] == r for t in f):
                    hs_scr[n, rows, :] = _form(f, lambda _, k: hf[:, _tile(k)]).astype(BF16)

    def sums(jobs, span, group, index, dst, get, skip_rows):
        forms = [f for f in dict.fromkeys(t[0] for t in group)
                 if len(f) > 1 and not (skip_rows and len({t[1] for t in f}) == 1)]

        def item(f, rows):
            def fn(dep):
                def term(r, k):
                    v = get(r, k, rows).astype(F32)
                    return v if dep is None or (r, k) != f[0][1:] else _after(v, _rows(dep, v.shape[0]))
                dst[index[f], rows, :] = _form(f, term).astype(BF16)
            return fn

        n = SPP if span else SP
        items = [item(f, slice(i, i + n)) for i in range(0, T, n) for f in forms]
        if span:
            jobs.side += [(len(jobs.res) + 1 + i * span // len(items), fn) for i, fn in enumerate(items)]
        else:
            for fn in items:
                fn(None)

    def stash(key, buf, j0, transpose=False):
        n = buf.shape[0] // T
        if key not in did:
            assert key in arrived
            did.add(key)
            w = _PairWeights(buf, transpose)
            for j in range(n):
                for hd in range(2):
                    w_scr[hd, j0 + j] = _pk(w(((1, j, hd),))[1])
        return lambda hd: [_ld(w_scr, hd, j0 + j) for j in range(n)]

    def kv_tile(jobs, r):
        wk, wvT = stash('k', wk_buf, 0), stash('v', wv_buf, kc, True)
        ct = [c_ref[_tile(r), _tile(j)] for j in range(kc)]
        for hd in range(2):
            k_scr[2 * r + hd] = _pk(jobs.mm(ct, wk(hd), _dot).astype(BF16))
        for hd in range(2):
            v_scr[2 * r + hd] = _pk(jobs.mm(wvT(hd), ct, _dot_nt).astype(BF16))

    def q_tile(jobs, r):
        wq = stash('q', wq_buf, 2 * kc)
        ht = [h_scr[r, j] for j in range(km)]
        for hd in range(2):
            q_scr[2 * r + hd] = _pk((jobs.mm(ht, wq(hd), _dot) * scale).astype(BF16))

    for blk in PROLOGUE.split(';'):
        waits, starts, acts = blk.split('|')
        for ch in waits.strip():
            assert ch in started and ch not in arrived
            arrived.add(ch)
            named[ch].wait()
        for ch in starts.strip():
            assert ch not in started
            started.add(ch)
            named[ch].start()
        jobs = _Jobs()
        for act in acts.split():
            if act == 'Z':
                jax.lax.fori_loop(0, nb, zero, 0)
                acc_scr[S:, :] = jnp.zeros((acc_scr.shape[0] - S, M), F32)
                x_ref[S:, :] = jnp.zeros((x_ref.shape[0] - S, M), BF16)
            elif act == 'M':
                assert arrived >= set('nm')
                mod = _dot(silu_cond(), wma_ref[...])
                mod_scr[:, 0:M] = mod[:, 0:M]
                mod_scr[:, M:2 * M] = 1.0 + mod[:, M:2 * M]
                did.add('M')
            else:
                act, _, span = act.partition('@')
                span = int(span or 0)
                for r in [int(ch, 16) for ch in act[1:]]:
                    did.add((act[0], r))
                    if act[0] == 'K':
                        assert 'abcd'[r // CB] in arrived
                        kv_tile(jobs, r)
                    elif act[0] == 'H':
                        assert 'wxyz'[r // CB] in arrived and 'M' in did
                        h_tile(r)
                    elif act[0] == 'Q':
                        assert ('H', r) in did
                        q_tile(jobs, r)
                    elif act[0] == 'C':
                        assert all('abcd'[t[1] // CB] in arrived for p_ in _C_GROUPS[r] for t in p_[0])
                        sums(jobs, span, _C_GROUPS[r], _C_SUMS, cs_scr,
                             lambda r_, k, rows: c_ref[r_ * T + rows.start:r_ * T + rows.stop, _tile(k)], False)
                    else:
                        assert act[0] == 'S' and all(('H', t[1]) in did for p_ in _H_GROUPS[r] for t in p_[0])
                        sums(jobs, span, _H_GROUPS[r], _H_SUMS, hs_scr, lambda r_, k, rows: h_scr[r_, k, rows, :], True)
        assert not jobs.side
    assert arrived == set(named) and all((k_, r) in did for k_ in 'KHQ' for r in range(nb))
    assert all((k_, r) in did for k_ in 'CS' for r in range(2))
    for cp in cp_late[1:] + cp_late[:1]:
        cp.start()

    FH = ws3.shape[0] * T
    assert nattn - 1 >= FH // 64

    def mixer_prep(g):
        def blocks(w_ref, r0, n, half, c0, c1, dep):
            lo, hi = pl.ds(r0, n), pl.ds(r0 + half, n)
            return [_after(w_ref[rows, _tile(c)].astype(F32), _rows(dep, n)) if (rows is lo) == (c == c0)
                    else w_ref[rows, _tile(c)].astype(F32) for rows in (lo, hi) for c in (c0, c1)]

        def rows_items(w_ref, dst, per_step, half, n=16):
            gi = jnp.minimum(g, half // per_step - 1)
            src = w_ref.at[pl.ds(pl.multiple_of(gi * per_step, per_step), half + per_step), :]
            hs = per_step // 2

            def item(c, o):
                def fn(dep):
                    for i, v in enumerate(_b_ops(*blocks(src, o, n, half, c, c + 2, dep))):
                        dst[i, c, pl.ds(pl.multiple_of(gi * hs, hs) + o // 2, n // 2), :] = _pk(v.astype(BF16))
                return fn
            return [item(c, o) for c in range(2) for o in range(0, per_step, n)]

        def w3_item(k, i):
            def fn(dep):
                n = jnp.minimum(g, FH // T - 1)
                b11, b21, b12, b22 = blocks(w3_ref, pl.multiple_of(n * T, T), T, FH, k, k + 2, dep)
                ws3[n, i, k] = _pk(_b_ops(b11, b12, b21, b22)[i].astype(BF16).T)
            return fn

        return (rows_items(w1_ref, ws12.at[0], 32, 2 * T) + rows_items(w2_ref, ws12.at[1], 32, 2 * T)
                + rows_items(w4_ref, ws4, 64, FH) + [w3_item(k, i) for k in range(2) for i in range(7)])

    def attn_body(g, carry):
        slot = g & 1
        nxt = jnp.minimum(g + 1, nattn - 1)
        copies = pcopies(nxt) + [ocopy(nxt, 1 - slot)]

        def mid():
            for cp in copies:
                cp.start()

        _attention_step(q_scr, k_scr, v_scr, wo_buf.at[slot], acc_scr, mid)
        for cp in copies:
            cp.wait()

        @pl.when(g == 0)
        def _():
            for cp in cp_late[1:]:
                cp.wait()

        @pl.when(g + 1 < nattn)
        def _():
            _proj_step(h_scr, hs_scr, c_ref, cs_scr, wq_buf, wk_buf, wv_buf, q_scr, k_scr, v_scr, scale,
                       mixer_prep(g))

        return carry

    jax.lax.fori_loop(0, nattn, attn_body, 0)

    cp_late[0].wait()
    mod = _dot(silu_cond(), wmb_ref[...])
    mod_scr[:, 2 * M:4 * M] = mod[:, 0:2 * M]
    mod_scr[:, 4 * M:5 * M] = 1.0 + mod[:, 2 * M:3 * M]
    mod_scr[:, 5 * M:6 * M] = mod[:, 3 * M:4 * M]
    ftiles = [(f, min(f + T, Fd)) for f in range(0, Fd, T)]
    OFF = x_ref.shape[0] - S
    CAR = t_scr.shape[0] - RB

    def p1(r0, n, dep=None):
        ga = mod_scr[:, 2 * M:3 * M]
        if dep is not None:
            ga = jnp.concatenate([_after(ga[:, 0:T], dep), ga[:, T:]], axis=1)
        rows = pl.ds(r0, n)
        x1 = x_ref[rows, :].astype(F32) + _rows(ga, n) * acc_scr[rows, :]
        x1_scr[rows, :] = x1
        hb = _ln(x1) * _rows(mod_scr[:, 4 * M:5 * M], n) + _rows(mod_scr[:, 3 * M:4 * M], n)
        hb_scr[rows, :] = hb
        return _ln(hb)

    HT = T // 2

    def p1_store(r0, c, dep=None):
        n = PC // 2
        hf, o = divmod(c * n, HT)
        top, bot = [p1(r0 + hf * T + d + o, n, dep) for d in (0, HT)]
        for d, v in ((0, top), (HT, bot)):
            for j in range(km):
                a1_scr[j, hf * T + d + o:hf * T + d + o + n, :] = v[:, _tile(j)].astype(BF16)
        ops = _a_ops(top[:, 0:2 * T], top[:, 2 * T:4 * T], bot[:, 0:2 * T], bot[:, 2 * T:4 * T])
        for i, m in enumerate(SUMS):
            for k in range(2):
                a1s_scr[hf, i, k, o:o + n, :] = ops[m][:, _tile(k)].astype(BF16)
        return jnp.max(ops[0][:, :T].reshape(n // 8, 8, T), axis=0)

    t_scr[RB:RB + CAR - OFF, :] = jnp.zeros((CAR - OFF, M), F32)
    t_scr[RB + CAR - OFF:RB + CAR, :] = _gelu(_dot(p1(0, OFF).astype(BF16), w1_ref[...]))
    for c in range(RB // PC):
        p1_store(OFF, c)

    def out_copy(i):
        rows = pl.ds(i * T if isinstance(i, int) else pl.multiple_of(i * T, T), T)
        return pltpu.make_async_copy(out_buf.at[rows, :], out_hbm.at[rows, :], osem.at[i])

    def b_body(r, carry):
        gb = _rows(mod_scr[:, 5 * M:6 * M], T)
        r0 = pl.multiple_of(r * RB, RB)
        n0 = pl.multiple_of(jnp.minimum(r0 + RB, S - RB) + OFF, OFF)
        nh = RB // T
        now = [0]
        due = []
        pace = []

        def p1_item(c):
            return lambda dep: due.append((now[0] + PD, p1_store(n0, c, dep)))

        pace += [(P0 + i * PSTEP, p1_item(i)) for i in range(RB // PC)]
        wt = lambda ref, f0, f1, n: ref[f0:f1, _tile(n)]

        def mm(lhs, wts, dot=_dot):
            acc = None
            for x, w in zip(lhs, wts):
                if due and due[0][0] <= now[0]:
                    w = _tie(w, due.pop(0)[1])
                v = dot(x, w)
                now[0] += x.shape[0] // HT
                acc = v if acc is None else v + acc
                if pace and pace[0][0] <= now[0]:
                    pace.pop(0)[1](v[0:8, :])
            return acc

        def split_ops(lo, hi):
            return [v.astype(BF16) for v in _a_ops(lo[:HT], hi[:HT], lo[HT:], hi[HT:])]

        def two_tiles(aops, wsel, rest):
            def col(w):
                v = mm(rest[0], w, rest[3])
                return v[:HT], v[HT:]

            c11, c12, c21, c22 = _strassen(
                lambda i: mm([a[i] for a in aops], [wsel(i, k) for k in range(len(aops))]),
                lambda: col(rest[1]), lambda: col(rest[2]))
            return jnp.concatenate([c11, c21], axis=0), jnp.concatenate([c12, c22], axis=0)

        def square(full, aops, w_ref, ws_ref):
            out = {}
            for n in range(2):
                out[n], out[n + 2] = two_tiles(
                    aops, lambda i, k: _ld(ws_ref, i, n, slice(k * HT, (k + 1) * HT)),
                    (full[4:], [wt(w_ref, 4 * T, M, n)], [wt(w_ref, 4 * T, M, n + 2)], _dot))
            out[4] = mm(full, [wt(w_ref, j * T, (j + 1) * T, 4) for j in range(km)])
            return out

        t_scr[0:CAR, :] = t_scr[RB:RB + CAR, :]
        for hf in range(nh):
            full = [a1_scr[j, _tile(hf), :] for j in range(km)]
            aops = []
            for k in range(2):
                ops = {m: a1s_scr[hf, i, k] for i, m in enumerate(SUMS)}
                ops[2], ops[3] = full[k][:HT], full[2 + k][HT:]
                aops.append(ops)
            for n, v in square(full, aops, w1_ref, ws12.at[0]).items():
                t = _gelu(v)
                if hf == nh - 1:
                    t = jnp.concatenate([t[:T - OFF], jnp.where(r < nrb - 1, t[T - OFF:], 0.0)], axis=0)
                t_scr[CAR + hf * T:CAR + (hf + 1) * T, _tile(n)] = t
        cq = M // 4
        shifts = (-1, 1, -2, 2)
        lane = jax.lax.broadcasted_iota(jnp.int32, (T, T), 1)
        y1, a3 = [], []
        for hf in range(nh):
            base = CAR - OFF + hf * T
            sh = []
            for j in range(km):
                g_lo, g_hi = (j * T) // cq, ((j + 1) * T - 1) // cq
                assert g_hi - g_lo <= 1
                v = t_scr[base + shifts[g_lo]:base + shifts[g_lo] + T, _tile(j)]
                if g_hi != g_lo:
                    v2 = t_scr[base + shifts[g_hi]:base + shifts[g_hi] + T, _tile(j)]
                    v = jnp.where(lane < g_hi * cq - j * T, v, v2)
                sh.append(v)
            hs = square([v.astype(BF16) for v in sh], [split_ops(sh[k], sh[2 + k]) for k in range(2)],
                        w2_ref, ws12.at[1])
            hs = jnp.concatenate([hs[n] for n in range(km)], axis=1)
            y1.append(hs + hb_scr[pl.ds(pl.multiple_of(r0 + hf * T, T), T), :])
            a3.append({})

            def ln_item(hf, c):
                def item(dep):
                    n = HT // NLN
                    for d in (0, HT):
                        v = y1[hf][d + c * n:d + (c + 1) * n]
                        if dep is not None:
                            v = jnp.concatenate([_after(v[:, :T], _rows(dep, n)), v[:, T:]], axis=1)
                        a3[hf][d + c * n] = _ln(v)
                return item

            ln_item(hf, 0)(None)
            pace += [(now[0] + LN0 + (c - 1) * LNS * (1 + hf), ln_item(hf, c)) for c in range(1, NLN)]
            pace.sort(key=lambda e: e[0])
        nf = FH // T
        h3, h3ops = [], []
        for hf in range(nh):
            assert len(a3[hf]) == 2 * NLN
            af = jnp.concatenate([a3[hf][key] for key in sorted(a3[hf])], axis=0)
            full = [af[:, _tile(j)].astype(BF16) for j in range(km)]
            aops = [split_ops(af[:, _tile(k)], af[:, _tile(2 + k)]) for k in range(2)]
            row, ops = {}, []
            narrow = None
            for n in range(nf):
                lo, hi = two_tiles(aops, lambda i, k: _ld(ws3, n, i, k),
                                   (full[4:], [wt(w3_ref, *ftiles[n], 4)],
                                    [wt(w3_ref, *ftiles[nf + n], 4)], _dot_nt))
                lo, hi = _gelu(lo), _gelu(hi)
                row[n], row[nf + n] = lo.astype(BF16), hi.astype(BF16)
                ops.append(split_ops(lo, hi))
                if n < km:
                    v = mm([wt(w3_ref, *ftiles[-1], n)], [full[n]], _dot_nt)
                    narrow = v if narrow is None else v + narrow
            row[2 * nf] = _gelu(mm(full, [wt(w3_ref, *ftiles[2 * nf], j) for j in range(km)],
                                   _dot_nt)).astype(BF16)
            fw = Fd - ftiles[-1][0]
            gT = jnp.concatenate([_gelu(narrow), jnp.zeros((T - fw, T), F32)], axis=0)
            row[2 * nf + 1] = _tie(gT.astype(BF16).T, gT[0:8, :])[:, :fw]
            h3.append([row[i] for i in range(len(ftiles))])
            h3ops.append(ops)
        for hf in range(nh):
            rows = pl.ds(pl.multiple_of(r0 + hf * T, T), T)

            def finish(n, v):
                out_buf[rows, _tile(n)] = (
                    x1_scr[rows, _tile(n)] + gb[:, _tile(n)] * (v + y1[hf][:, _tile(n)])
                ).astype(out_buf.dtype)

            w4t = lambda n, f_: [wt(w4_ref, f0, f1, n) for f0, f1 in f_]
            finish(4, mm(h3[hf], w4t(4, ftiles)))
            for n in range(2):
                lo, hi = two_tiles(h3ops[hf], lambda i, k: _ld(ws4, i, n, slice(k * HT, (k + 1) * HT)),
                                   (h3[hf][2 * nf:], w4t(n, ftiles[2 * nf:]), w4t(n + 2, ftiles[2 * nf:]), _dot))
                finish(n, lo)
                finish(n + 2, hi)
            out_copy(r * nh + hf).start()
        assert not pace
        return carry

    jax.lax.fori_loop(0, nrb, b_body, 0)
    for i in range(nb):
        out_copy(i).wait()


@jax.jit
def pallas_adaLN_cond__compressed_kv_cla__mixer_s_mlp__prompt_kernel(
    A_x: jax.Array,
    A_c_kv: jax.Array,
    A_w_q: jax.Array,
    A_w_uk: jax.Array,
    A_w_uv: jax.Array,
    A_w_o: jax.Array,
    B_x: jax.Array,
    B_w1: jax.Array,
    B_w2: jax.Array,
    B_w3: jax.Array,
    B_w4: jax.Array,
    c: jax.Array,
    w_mod: jax.Array,
):
    _, S, M = A_x.shape
    Dc = A_c_kv.shape[2]
    H, D = A_w_q.shape[1], A_w_q.shape[2]
    Fd = B_w3.shape[1]
    assert D == T and A_c_kv.shape[1] == S and Dc == 4 * T and M == 5 * T and 13 * T < Fd < 14 * T
    vmem = pltpu.VMEM
    packed = lambda *lead: vmem(lead + (T // 2, T), U32)
    out = pl.pallas_call(
        _kernel,
        in_specs=[pl.BlockSpec(memory_space=pltpu.HBM)] * 12,
        out_specs=pl.BlockSpec(memory_space=pltpu.HBM),
        out_shape=jax.ShapeDtypeStruct((S, M), A_x.dtype),
        scratch_shapes=[
            vmem((S + 16, M), BF16),
            vmem((S, Dc), BF16),
            vmem((1, M), BF16),
            vmem((M, 2 * M), BF16),
            vmem((M, 4 * M), BF16),
            vmem((M, M), BF16),
            vmem((M, M), BF16),
            vmem((Fd, M), BF16),
            vmem((Fd, M), BF16),
            vmem((M, D), U32),
            vmem((Dc, D), U32),
            vmem((Dc, D), U32),
            vmem((2, 2 * D, M), BF16),
            vmem((S, M), A_x.dtype),
            pltpu.SemaphoreType.DMA((15,)),
            pltpu.SemaphoreType.DMA((4,)),
            pltpu.SemaphoreType.DMA((S // T,)),
            vmem((8, 6 * M), F32),
            vmem((S // T, M // T, T, T), BF16),
            vmem((len(_C_SUMS), T, T), BF16),
            vmem((len(_H_SUMS), T, T), BF16),
            packed(2, M // T + 2 * (Dc // T)),
            packed(2 * S // T),
            packed(2 * S // T),
            packed(2 * S // T),
            vmem((S + 16, M), F32),
            vmem((S + 16, M), F32),
            vmem((S + 16, M), F32),
            vmem((M // T, RB, T), BF16),
            vmem((RB + 32, M), F32),
            vmem((RB // T, 5, 2, T // 2, T), BF16),
            vmem((2, 7, 2, T, T), U32),
            packed(6, 7, 2),
            vmem((7, 2, 3 * T, T), U32),
        ],
        compiler_params=pltpu.CompilerParams(
            vmem_limit_bytes=100 * 1024 * 1024,
            disable_bounds_checks=True,
        ),
    )(
        A_x.reshape(S, M), A_c_kv.reshape(S, Dc),
        A_w_q, A_w_uk, A_w_uv,
        A_w_o.reshape(H // 2, 2 * D, M),
        B_w1, B_w2, B_w3.T, B_w4, c, w_mod,
    )
    return out.reshape(1, S, M)
```

```python
import math
import os

import jax
import jax.numpy as jnp
import jax.experimental.pallas as pl
import jax.experimental.pallas.tpu as pltpu

F32 = jnp.float32
BF16 = jnp.bfloat16
U32 = jnp.uint32
NT = (((1,), (1,)), ((), ()))
T = 128
EPS = 1e-5
LOG2E = math.log2(math.e)

GRP = int(os.environ.get('GRP', 4))
OGRP = int(os.environ.get('OGRP', 6))
LEAD = int(os.environ.get('LEAD', 10))
PROW = int(os.environ.get('PROW', 3))
VT = 8
RES = int(os.environ.get('RES', 32))
LAT_A = int(os.environ.get('LAT_A', 16))
LAT_B = int(os.environ.get('LAT_B', 20))
ALEAD = int(os.environ.get('ALEAD', 32))
MID = 40
SD0, SDS = int(os.environ.get('SD0', 180)), int(os.environ.get('SDS', 5))
OSH = int(os.environ.get('OSH', 0))
OFINE = int(os.environ.get('OFINE', 0))
RB = 256
PC = 32
P0, PSTEP, PD = 440, 30, 52
NLN, LN0, LNS = 4, 4, 5
LP = int(os.environ.get('LP', 32))
SP = int(os.environ.get('SP', 16))
SPP = int(os.environ.get('SPP', 32))
PROLOGUE = os.environ.get('PRO', '|kva|Z; |b|; kva|cdn|K0123; b|m|C0@58 K4567; cd|qw|C1@72 K89abc; nm|x|M Kde; '
            'qw|yzo|Kf H0123 Q01; x||H4567 Q2345; yz||H89abcdef Q6789abcdef S01; o||')


def _dot(a, b):
    return jnp.dot(a, b, preferred_element_type=F32)


def _dot_nt(a, b):
    return jax.lax.dot_general(a, b, NT, preferred_element_type=F32)


def _ln(x):
    m = jnp.mean(x, axis=-1, keepdims=True)
    xc = x - m
    v = jnp.mean(xc * xc, axis=-1, keepdims=True)
    return xc * jnp.exp2(jnp.log(v + EPS) * (-0.5 * LOG2E))


def _rows(v, n):
    return jnp.broadcast_to(v[None], (n // 8, 8, v.shape[1])).reshape(n, v.shape[1])


def _gelu(x):
    c0 = math.sqrt(2.0 / math.pi)
    return 0.5 * x * (1.0 + jnp.tanh(c0 * (x + 0.044715 * (x * x * x))))


def _after(x, dep):
    return jnp.where(dep > jnp.inf, dep, x)


def _tie(x, dep):
    xu = pltpu.bitcast(x, U32)
    first = jnp.where(dep > jnp.inf, jnp.uint32(0), xu[:8])
    return pltpu.bitcast(jnp.concatenate([first, xu[8:]], axis=0), BF16)


def _tile(j):
    return slice(j * T, (j + 1) * T)


def _ld(ref, *idx):
    return pltpu.bitcast(ref[idx], BF16)


def _pk(x):
    return pltpu.bitcast(x, U32)


def _a_ops(a11, a12, a21, a22):
    return [a11 + a22, a21 + a22, a11, a22, a11 + a12, a21 - a11, a12 - a22]


SUMS = (0, 1, 4, 5, 6)


def _b_ops(b11, b12, b21, b22):
    return [b11 + b22, b11, b12 - b22, b21 - b11, b22, b11 + b12, b21 + b22]


def _strassen(prod, col1=None, col2=None):
    m4 = prod(3)
    m2 = prod(1)
    c21 = m2 + m4
    if col1 is not None:
        e11, e21 = col1()
        m4, c21 = m4 + e11, c21 + e21
    m3 = prod(2)
    m5 = prod(4)
    c12 = m3 + m5
    if col2 is not None:
        e12, e22 = col2()
        c12, m3 = c12 + e12, m3 + e22
    m1 = prod(0)
    c11 = prod(6) + (m1 + (m4 - m5))
    c22 = prod(5) + (m1 + (m3 - m2))
    return c11, c12, c21, c22


def _group(xs, ys):
    ks = sorted({k for _, k in xs + ys})
    prods = []
    for i, k in xs:
        mates = [y for y in ys if y[1] != k]
        prods.append((tuple((1, i, kk) for kk in ks), ((1, k, 0),), ((1, i, 0), (-1, i, 1))))
        prods.append((((1, i, k),) + tuple((-1, i2, k) for i2, _ in mates), ((1, k, 0), (1, k, 1)), ((1, i, 1),)))
        for i2, k2 in mates:
            prods.append((((1, i, k2),), ((1, k2, 0), (-1, k, 0)), ((1, i2, 0), (1, i, 0))))
            prods.append((((1, i2, k), (1, i, k2)), ((1, k, 0), (1, k2, 1)), ((1, i2, 0), (1, i, 1))))
            prods.append((((1, i2, k),), ((1, k, 1), (-1, k2, 1)), ((1, i2, 1), (1, i, 1))))
    for i2, k2 in ys:
        mates = [x for x in xs if x[1] != k2]
        prods.append((tuple((1, i2, kk) for kk in ks), ((1, k2, 1),), ((1, i2, 1), (-1, i2, 0))))
        prods.append((((1, i2, k2),) + tuple((-1, i, k2) for i, _ in mates), ((1, k2, 0), (1, k2, 1)),
                      ((1, i2, 0),)))
    return prods


def _full_group(r0, ks):
    q = len(ks)
    return _group([(r0 + a, k) for a, k in enumerate(ks)], [(r0 + q + a, k) for a, k in enumerate(ks)])


_C_GROUPS = [_full_group(0, range(4)), _full_group(8, range(4))]
_H_GROUPS = [_full_group(0, range(5)),
             [t for r in (10, 11, 12) for t in _group([(r, 3)], [(r + 3, 4)])] + _full_group(10, range(3))]
_sum_index = lambda groups: {f: n for n, f in enumerate(
    dict.fromkeys(t[0] for g in groups for t in g if len(t[0]) > 1))}
_C_SUMS, _H_SUMS = _sum_index(_C_GROUPS), _sum_index(_H_GROUPS)


def _form(form, get):
    acc = None
    for sign, i, j in form:
        v = get(i, j)
        acc = v if acc is None else (acc + v if sign > 0 else acc - v)
    return acc


class _PairWeights:
    def __init__(self, w_ref, transpose=False):
        self.base = {}
        for j in range(w_ref.shape[0] // T):
            wu = w_ref[_tile(j), :]
            if transpose:
                wu = wu.T
            self.base[j, 0] = pltpu.bitcast(wu << 16, F32)
            self.base[j, 1] = pltpu.bitcast(wu & jnp.uint32(0xFFFF0000), F32)
        self.cache = {}

    def __call__(self, form):
        sign = 1
        if form[-1][0] < 0 and form[0][1:] > form[1][1:]:
            sign, form = -1, ((1,) + form[1][1:], (-1,) + form[0][1:])
        if form not in self.cache:
            self.cache[form] = _form(form, lambda k, h: self.base[k, h]).astype(BF16)
        return sign, self.cache[form]


def _run_group(jobs, prods, a_get, w, transposed, finish):
    left = {}
    for _, _, outs in prods:
        for _, i, h in outs:
            left[i, h] = left.get((i, h), 0) + 1
    acc = {}
    for af, bf, outs in prods:
        sign, wt = w(bf)
        m = jobs.mm([wt], [a_get(af)], _dot_nt) if transposed else jobs.mm([a_get(af)], [wt], _dot)
        for s_, i, h in outs:
            if (i, h) not in acc:
                acc[i, h] = (s_ * sign, m)
            else:
                s0, v = acc[i, h]
                acc[i, h] = (s0, v + m if s0 == s_ * sign else v - m) if s0 > 0 or s_ * sign < 0 else (1, m - v)
            left[i, h] -= 1
            if not left[i, h]:
                s0, v = acc.pop((i, h))
                assert s0 > 0
                finish(2 * i + h, v)


class _Jobs:
    def __init__(self, side=()):
        self.res = []
        self.side = list(side)

    def mm(self, lhs, wt, dot, tie=False):
        acc = None
        for x, w in zip(lhs, wt):
            if tie and len(self.res) >= VT:
                x = _tie(x, self.res[len(self.res) - VT][0:8, :])
            v = dot(x, w)
            self.res.append(v)
            acc = v if acc is None else v + acc
            rel = 4 * (len(self.res) % 4)
            while self.side and self.side[0][0] <= len(self.res):
                self.side.pop(0)[1](v[8 * rel:8 * rel + 8, :])
                rel = (rel + 2) % 16
        return acc


def _proj_step(h_scr, hs_scr, c_ref, cs_scr, wq_ref, wuk_ref, wuv_ref, q_scr, k_scr, v_scr, scale, side):
    wq, wk, wvT = _PairWeights(wq_ref), _PairWeights(wuk_ref), _PairWeights(wuv_ref, True)
    c_get = lambda f: cs_scr[_C_SUMS[f]] if len(f) > 1 else c_ref[_tile(f[0][1]), _tile(f[0][2])]
    h_get = lambda f: hs_scr[_H_SUMS[f]] if len(f) > 1 else h_scr[f[0][1], f[0][2]]

    def put(dst, mul=None):
        def fn(u, v):
            dst[u] = _pk((v if mul is None else v * mul).astype(BF16))
        return fn

    jobs = _Jobs((SD0 + i * SDS, fn) for i, fn in enumerate(side))
    for gi in range(2):
        _run_group(jobs, _C_GROUPS[gi], c_get, wk, False, put(k_scr))
        _run_group(jobs, _H_GROUPS[gi], h_get, wq, False, put(q_scr, scale))
        _run_group(jobs, _C_GROUPS[gi], c_get, wvT, True, put(v_scr))
    assert not jobs.side


def _inner_group(xs, ys):
    prods = []
    for i, j in xs:
        mates = [y for y in ys if y[1] != j]
        prods.append((((1, i, 0),), ((1, 0, j), (-1, 1, j)), ((1, i, j),) + tuple((1, i2, j) for i2, _ in mates)))
        prods.append((((1, i, 0), (1, i, 1)), ((1, 1, j),), ((1, i, j),) + tuple((-1, i, j2) for _, j2 in mates)))
    for i2, j2 in ys:
        mates = [x for x in xs if x[1] != j2]
        prods.append((((1, i2, 0), (1, i2, 1)), ((1, 0, j2),),
                      ((1, i2, j2),) + tuple((-1, i2, j) for _, j in mates)))
        prods.append((((1, i2, 1),), ((1, 0, j2), (-1, 1, j2)),
                      ((-1, i2, j2),) + tuple((-1, i, j2) for i, _ in mates)))
    for i, j in xs:
        for i2, j2 in ys:
            if j2 != j:
                lo, hi = min(j, j2), max(j, j2)
                prods.append((((1, i2, 0), (-1, i, 0)), ((1, 0, lo), (1, 0, hi)), ((1, i2, j),)))
                prods.append((((1, i, 0), (1, i2, 1)), ((1, 0, j2), (1, 1, j)), ((1, i, j2), (1, i2, j))))
                prods.append((((1, i, 1), (-1, i2, 1)), ((1, 1, lo), (1, 1, hi)), ((1, i, j2),)))
    return prods


def _o_jobs():
    alt = lambda r0, q: ([(r0 + 2 * a, a) for a in range(q)], [(r0 + 2 * a + 1, (a + OSH) % q) for a in range(q)])
    prods = _inner_group(*alt(0, 5)) + _inner_group(*alt(10, 3))
    for r in (10, 12, 14):
        prods += _inner_group([(r, 3)], [(r + 1, 4)])
    row = lambda t: max(i for _, i, _ in t[0])
    unit = lambda t: max(2 * i + h for _, i, h in t[0])
    prods.sort(key=lambda t: unit(t) if OFINE or row(t) == 15 else 2 * row(t) + 1)
    return [(unit(t) if OFINE or row(t) == 15 else 2 * row(t) + 1, t) for t in prods]


_O_JOBS = _o_jobs()


def _job_order(nb):
    units = range(2 * nb)
    qa = [('a', u, c) for u in units for c in range(u // 2 + 1)]
    qb = [('b', u, c) for u in units for c in range(u // 2 + 1)]
    qo = [('o', u, j) for j, (u, _) in enumerate(_O_JOBS)]
    done = {}
    order = []

    def ready(q, lat, pre):
        return bool(q) and (pre, q[0][1]) in done and done[(pre, q[0][1])] + lat <= len(order)

    def emit(q):
        kind, u, j = job = q.pop(0)
        if kind != 'o' and j == u // 2:
            done[(kind, u)] = len(order)
        order.append(job)

    turn = 0
    while qa or qb or qo:
        pref = 'abo'[turn % 3]
        turn += 1
        for _ in range(OGRP if pref == 'o' else GRP):
            b_ok, o_ok = ready(qb, LAT_A, 'a'), ready(qo, LAT_B, 'b')
            if pref == 'a' and qa and (len(qb) - len(qa) < ALEAD or not b_ok):
                emit(qa)
            elif pref == 'b' and b_ok:
                emit(qb)
            elif pref == 'o' and o_ok and (len(qo) > RES or not (qa or b_ok)):
                emit(qo)
            elif not (qa or b_ok or o_ok) and (qb or qo):
                emit(qb or qo)
            else:
                break
    return order


def _attention_step(q_scr, k_scr, v_scr, wo_ref, acc_scr, mid):
    causal = (jax.lax.broadcasted_iota(jnp.int32, (T, T), 0)
              <= jax.lax.broadcasted_iota(jnp.int32, (T, T), 1))
    sv, mx, mfin, lsum, pv, of, lhs = {}, {}, {}, {}, {}, {}, {}
    res = []
    wo, terms = {}, {}
    left = {}
    for _, t in _O_JOBS:
        for _, i, j in t[2]:
            left[i, j] = left.get((i, j), 0) + 1

    def job_a(u, c):
        r, hd = divmod(u, 2)
        s = _dot_nt(_ld(k_scr, 2 * c + hd), _ld(q_scr, u))
        res.append(s)
        if c == r:
            s = jnp.where(causal, s, -1e9 * LOG2E)
        s = s.reshape(T // 8, 8, T)
        sv[(u, c)] = s
        pm = jnp.max(s, axis=0)
        mx[u] = pm if u not in mx else jnp.maximum(mx[u], pm)

    def job_b(u, c):
        r, hd = divmod(u, 2)
        if u not in mfin:
            mfin[u] = jnp.broadcast_to(jnp.max(mx[u], axis=0, keepdims=True), (8, T))
        m = mfin[u]
        if len(res) >= LEAD:
            r0 = 8 * PROW * (c % 4)
            m = _after(m, res[len(res) - LEAD][r0:r0 + 8, :])
        p = jnp.exp2(sv.pop((u, c)) - m[None])
        ls = jnp.sum(p, axis=0)
        lsum[u] = ls if u not in lsum else lsum[u] + ls
        v = _dot(_ld(v_scr, 2 * c + hd), p.reshape(T, T).astype(BF16))
        res.append(v)
        pv[u] = v if u not in pv else v + pv[u]
        if c == r:
            of[u] = pv[u] * (1.0 / jnp.sum(lsum[u], axis=0, keepdims=True))

    def job_o(_, n):
        af, bf, outs = _O_JOBS[n][1]
        if af not in lhs:
            v = _form(af, lambda i, h: of[2 * i + h])
            lhs[af] = _tie(v.astype(BF16).T, v[0:8, :])
        if bf not in wo:
            wo[bf] = (wo_ref[_tile(bf[0][1]), _tile(bf[0][2])] if len(bf) == 1 else
                      _form(bf, lambda h, j: wo_ref[_tile(h), _tile(j)].astype(F32)).astype(BF16))
        v = _dot(lhs[af], wo[bf])
        res.append(v)
        for sign, i, j in outs:
            terms.setdefault((i, j), []).append((sign, v))
            if len(terms[i, j]) == left[i, j]:
                tot = acc_scr[_tile(i), _tile(j)]
                for sg, m in terms.pop((i, j)):
                    tot = tot + m if sg > 0 else tot - m
                acc_scr[_tile(i), _tile(j)] = tot

    fns = dict(a=job_a, b=job_b, o=job_o)
    for n, (kind, u, j) in enumerate(_job_order(q_scr.shape[0] // 2)):
        if n == MID:
            mid()
        fns[kind](u, j)


def _kernel(x_hbm, c_hbm, wq_hbm, wuk_hbm, wuv_hbm, wo_hbm, w1_hbm, w2_hbm, w3_hbm, w4_hbm,
            cond_hbm, wmod_hbm, out_hbm,
            x_ref, c_ref, cond_ref, wma_ref, wmb_ref, w1_ref, w2_ref, w3_ref, w4_ref,
            wq_buf, wk_buf, wv_buf, wo_buf, out_buf, sem, wsem, osem,
            mod_scr, h_scr, cs_scr, hs_scr, w_scr, q_scr, k_scr, v_scr, acc_scr, x1_scr, hb_scr, a1_scr, t_scr,
            a1s_scr, ws12, ws3, ws4):
    S, M = x_hbm.shape
    D = wq_hbm.shape[2]
    nattn = wo_hbm.shape[0]
    Fd = w4_hbm.shape[0]
    scale = float(D) ** -0.5 * LOG2E
    nb, nrb = S // T, S // RB
    km, kc = M // T, c_hbm.shape[1] // T
    NX = 4
    XR = S // NX
    CB = XR // T

    def pcopies(g):
        return [pltpu.make_async_copy(src.bitcast(U32).at[:, g, :], dst, wsem.at[j])
                for j, (src, dst) in enumerate(((wuk_hbm, wk_buf), (wuv_hbm, wv_buf), (wq_hbm, wq_buf)))]

    def ocopy(g, slot):
        return pltpu.make_async_copy(wo_hbm.at[g], wo_buf.at[slot], wsem.at[3])

    def chunk_copy(src, dst, i, s0):
        rows = slice(i * XR, (i + 1) * XR)
        return pltpu.make_async_copy(src.at[rows, :], dst.at[rows, :], sem.at[s0 + i])

    cp_cond = pltpu.make_async_copy(cond_hbm, cond_ref, sem.at[0])
    cp_wma = pltpu.make_async_copy(wmod_hbm.at[:, 0:2 * M], wma_ref, sem.at[1])
    cp_late = [pltpu.make_async_copy(src, dst, sem.at[2 + j]) for j, (src, dst) in enumerate((
        (wmod_hbm.at[:, 2 * M:6 * M], wmb_ref), (w1_hbm, w1_ref), (w2_hbm, w2_ref),
        (w3_hbm, w3_ref), (w4_hbm, w4_ref)))]
    cp_x = [chunk_copy(x_hbm, x_ref, i, 7) for i in range(NX)]
    cp_c = [chunk_copy(c_hbm, c_ref, i, 7 + NX) for i in range(NX)]

    def silu_cond():
        cf = cond_ref[...].astype(F32)
        return jnp.broadcast_to((cf * jax.nn.sigmoid(cf)).astype(BF16), (8, M))

    cp_wk, cp_wv, cp_wq = pcopies(0)
    named = dict(k=cp_wk, v=cp_wv, q=cp_wq, o=ocopy(0, 0), n=cp_cond, m=cp_wma)
    named.update(zip('abcd', cp_c))
    named.update(zip('wxyz', cp_x))
    started, arrived, did = set(), set(), set()

    def zero(r, carry):
        acc_scr[pl.ds(pl.multiple_of(r * T, T), T), :] = jnp.zeros((T, M), F32)
        return carry

    def h_tile(r):
        sa = _rows(mod_scr[:, 0:M], LP)
        ca1 = _rows(mod_scr[:, M:2 * M], LP)
        for i in range(T // LP):
            rows = slice(i * LP, (i + 1) * LP)
            hf = _ln(x_ref[r * T + i * LP:r * T + (i + 1) * LP, :].astype(F32)) * ca1 + sa
            for j in range(km):
                h_scr[r, j, rows, :] = hf[:, _tile(j)].astype(BF16)
            for f, n in _H_SUMS.items():
                if all(t[1] == r for t in f):
                    hs_scr[n, rows, :] = _form(f, lambda _, k: hf[:, _tile(k)]).astype(BF16)

    def sums(jobs, span, group, index, dst, get, skip_rows):
        forms = [f for f in dict.fromkeys(t[0] for t in group)
                 if len(f) > 1 and not (skip_rows and len({t[1] for t in f}) == 1)]

        def item(f, rows):
            def fn(dep):
                def term(r, k):
                    v = get(r, k, rows).astype(F32)
                    return v if dep is None or (r, k) != f[0][1:] else _after(v, _rows(dep, v.shape[0]))
                dst[index[f], rows, :] = _form(f, term).astype(BF16)
            return fn

        n = SPP if span else SP
        items = [item(f, slice(i, i + n)) for i in range(0, T, n) for f in forms]
        if span:
            jobs.side += [(len(jobs.res) + 1 + i * span // len(items), fn) for i, fn in enumerate(items)]
        else:
            for fn in items:
                fn(None)

    def stash(key, buf, j0, transpose=False):
        n = buf.shape[0] // T
        if key not in did:
            assert key in arrived
            did.add(key)
            w = _PairWeights(buf, transpose)
            for j in range(n):
                for hd in range(2):
                    w_scr[hd, j0 + j] = _pk(w(((1, j, hd),))[1])
        return lambda hd: [_ld(w_scr, hd, j0 + j) for j in range(n)]

    def kv_tile(jobs, r):
        wk, wvT = stash('k', wk_buf, 0), stash('v', wv_buf, kc, True)
        ct = [c_ref[_tile(r), _tile(j)] for j in range(kc)]
        for hd in range(2):
            k_scr[2 * r + hd] = _pk(jobs.mm(ct, wk(hd), _dot).astype(BF16))
        for hd in range(2):
            v_scr[2 * r + hd] = _pk(jobs.mm(wvT(hd), ct, _dot_nt).astype(BF16))

    def q_tile(jobs, r):
        wq = stash('q', wq_buf, 2 * kc)
        ht = [h_scr[r, j] for j in range(km)]
        for hd in range(2):
            q_scr[2 * r + hd] = _pk((jobs.mm(ht, wq(hd), _dot) * scale).astype(BF16))

    for blk in PROLOGUE.split(';'):
        waits, starts, acts = blk.split('|')
        for ch in waits.strip():
            assert ch in started and ch not in arrived
            arrived.add(ch)
            named[ch].wait()
        for ch in starts.strip():
            assert ch not in started
            started.add(ch)
            named[ch].start()
        jobs = _Jobs()
        for act in acts.split():
            if act == 'Z':
                jax.lax.fori_loop(0, nb, zero, 0)
                acc_scr[S:, :] = jnp.zeros((acc_scr.shape[0] - S, M), F32)
                x_ref[S:, :] = jnp.zeros((x_ref.shape[0] - S, M), BF16)
            elif act == 'M':
                assert arrived >= set('nm')
                mod = _dot(silu_cond(), wma_ref[...])
                mod_scr[:, 0:M] = mod[:, 0:M]
                mod_scr[:, M:2 * M] = 1.0 + mod[:, M:2 * M]
                did.add('M')
            else:
                act, _, span = act.partition('@')
                span = int(span or 0)
                for r in [int(ch, 16) for ch in act[1:]]:
                    did.add((act[0], r))
                    if act[0] == 'K':
                        assert 'abcd'[r // CB] in arrived
                        kv_tile(jobs, r)
                    elif act[0] == 'H':
                        assert 'wxyz'[r // CB] in arrived and 'M' in did
                        h_tile(r)
                    elif act[0] == 'Q':
                        assert ('H', r) in did
                        q_tile(jobs, r)
                    elif act[0] == 'C':
                        assert all('abcd'[t[1] // CB] in arrived for p_ in _C_GROUPS[r] for t in p_[0])
                        sums(jobs, span, _C_GROUPS[r], _C_SUMS, cs_scr,
                             lambda r_, k, rows: c_ref[r_ * T + rows.start:r_ * T + rows.stop, _tile(k)], False)
                    else:
                        assert act[0] == 'S' and all(('H', t[1]) in did for p_ in _H_GROUPS[r] for t in p_[0])
                        sums(jobs, span, _H_GROUPS[r], _H_SUMS, hs_scr, lambda r_, k, rows: h_scr[r_, k, rows, :], True)
        assert not jobs.side
    assert arrived == set(named) and all((k_, r) in did for k_ in 'KHQ' for r in range(nb))
    assert all((k_, r) in did for k_ in 'CS' for r in range(2))
    for cp in cp_late[1:] + cp_late[:1]:
        cp.start()

    FH = ws3.shape[0] * T
    assert nattn - 1 >= FH // 64

    def mixer_prep(g):
        def blocks(w_ref, r0, n, half, c0, c1, dep):
            lo, hi = pl.ds(r0, n), pl.ds(r0 + half, n)
            return [_after(w_ref[rows, _tile(c)].astype(F32), _rows(dep, n)) if (rows is lo) == (c == c0)
                    else w_ref[rows, _tile(c)].astype(F32) for rows in (lo, hi) for c in (c0, c1)]

        def rows_items(w_ref, dst, per_step, half, n=16):
            gi = jnp.minimum(g, half // per_step - 1)
            src = w_ref.at[pl.ds(pl.multiple_of(gi * per_step, per_step), half + per_step), :]
            hs = per_step // 2

            def item(c, o):
                def fn(dep):
                    for i, v in enumerate(_b_ops(*blocks(src, o, n, half, c, c + 2, dep))):
                        dst[i, c, pl.ds(pl.multiple_of(gi * hs, hs) + o // 2, n // 2), :] = _pk(v.astype(BF16))
                return fn
            return [item(c, o) for c in range(2) for o in range(0, per_step, n)]

        def w3_item(k, i):
            def fn(dep):
                n = jnp.minimum(g, FH // T - 1)
                b11, b21, b12, b22 = blocks(w3_ref, pl.multiple_of(n * T, T), T, FH, k, k + 2, dep)
                ws3[n, i, k] = _pk(_b_ops(b11, b12, b21, b22)[i].astype(BF16).T)
            return fn

        return (rows_items(w1_ref, ws12.at[0], 32, 2 * T) + rows_items(w2_ref, ws12.at[1], 32, 2 * T)
                + rows_items(w4_ref, ws4, 64, FH) + [w3_item(k, i) for k in range(2) for i in range(7)])

    def attn_body(g, carry):
        slot = g & 1
        nxt = jnp.minimum(g + 1, nattn - 1)
        copies = pcopies(nxt) + [ocopy(nxt, 1 - slot)]

        def mid():
            for cp in copies:
                cp.start()

        _attention_step(q_scr, k_scr, v_scr, wo_buf.at[slot], acc_scr, mid)
        for cp in copies:
            cp.wait()

        @pl.when(g == 0)
        def _():
            for cp in cp_late[1:]:
                cp.wait()

        @pl.when(g + 1 < nattn)
        def _():
            _proj_step(h_scr, hs_scr, c_ref, cs_scr, wq_buf, wk_buf, wv_buf, q_scr, k_scr, v_scr, scale,
                       mixer_prep(g))

        return carry

    jax.lax.fori_loop(0, nattn, attn_body, 0)

    cp_late[0].wait()
    mod = _dot(silu_cond(), wmb_ref[...])
    mod_scr[:, 2 * M:4 * M] = mod[:, 0:2 * M]
    mod_scr[:, 4 * M:5 * M] = 1.0 + mod[:, 2 * M:3 * M]
    mod_scr[:, 5 * M:6 * M] = mod[:, 3 * M:4 * M]
    ftiles = [(f, min(f + T, Fd)) for f in range(0, Fd, T)]
    OFF = x_ref.shape[0] - S
    CAR = t_scr.shape[0] - RB

    def p1(r0, n, dep=None):
        ga = mod_scr[:, 2 * M:3 * M]
        if dep is not None:
            ga = jnp.concatenate([_after(ga[:, 0:T], dep), ga[:, T:]], axis=1)
        rows = pl.ds(r0, n)
        x1 = x_ref[rows, :].astype(F32) + _rows(ga, n) * acc_scr[rows, :]
        x1_scr[rows, :] = x1
        hb = _ln(x1) * _rows(mod_scr[:, 4 * M:5 * M], n) + _rows(mod_scr[:, 3 * M:4 * M], n)
        hb_scr[rows, :] = hb
        return _ln(hb)

    HT = T // 2

    def p1_store(r0, c, dep=None):
        n = PC // 2
        hf, o = divmod(c * n, HT)
        top, bot = [p1(r0 + hf * T + d + o, n, dep) for d in (0, HT)]
        for d, v in ((0, top), (HT, bot)):
            for j in range(km):
                a1_scr[j, hf * T + d + o:hf * T + d + o + n, :] = v[:, _tile(j)].astype(BF16)
        ops = _a_ops(top[:, 0:2 * T], top[:, 2 * T:4 * T], bot[:, 0:2 * T], bot[:, 2 * T:4 * T])
        for i, m in enumerate(SUMS):
            for k in range(2):
                a1s_scr[hf, i, k, o:o + n, :] = ops[m][:, _tile(k)].astype(BF16)
        return jnp.max(ops[0][:, :T].reshape(n // 8, 8, T), axis=0)

    t_scr[RB:RB + CAR - OFF, :] = jnp.zeros((CAR - OFF, M), F32)
    t_scr[RB + CAR - OFF:RB + CAR, :] = _gelu(_dot(p1(0, OFF).astype(BF16), w1_ref[...]))
    for c in range(RB // PC):
        p1_store(OFF, c)

    def out_copy(i):
        rows = pl.ds(i * T if isinstance(i, int) else pl.multiple_of(i * T, T), T)
        return pltpu.make_async_copy(out_buf.at[rows, :], out_hbm.at[rows, :], osem.at[i])

    def b_body(r, carry):
        gb = _rows(mod_scr[:, 5 * M:6 * M], T)
        r0 = pl.multiple_of(r * RB, RB)
        n0 = pl.multiple_of(jnp.minimum(r0 + RB, S - RB) + OFF, OFF)
        nh = RB // T
        now = [0]
        due = []
        pace = []

        def p1_item(c):
            return lambda dep: due.append((now[0] + PD, p1_store(n0, c, dep)))

        pace += [(P0 + i * PSTEP, p1_item(i)) for i in range(RB // PC)]
        wt = lambda ref, f0, f1, n: ref[f0:f1, _tile(n)]

        def mm(lhs, wts, dot=_dot):
            acc = None
            for x, w in zip(lhs, wts):
                if due and due[0][0] <= now[0]:
                    w = _tie(w, due.pop(0)[1])
                v = dot(x, w)
                now[0] += x.shape[0] // HT
                acc = v if acc is None else v + acc
                if pace and pace[0][0] <= now[0]:
                    pace.pop(0)[1](v[0:8, :])
            return acc

        def split_ops(lo, hi):
            return [v.astype(BF16) for v in _a_ops(lo[:HT], hi[:HT], lo[HT:], hi[HT:])]

        def two_tiles(aops, wsel, rest):
            def col(w):
                v = mm(rest[0], w, rest[3])
                return v[:HT], v[HT:]

            c11, c12, c21, c22 = _strassen(
                lambda i: mm([a[i] for a in aops], [wsel(i, k) for k in range(len(aops))]),
                lambda: col(rest[1]), lambda: col(rest[2]))
            return jnp.concatenate([c11, c21], axis=0), jnp.concatenate([c12, c22], axis=0)

        def square(full, aops, w_ref, ws_ref):
            out = {}
            for n in range(2):
                out[n], out[n + 2] = two_tiles(
                    aops, lambda i, k: _ld(ws_ref, i, n, slice(k * HT, (k + 1) * HT)),
                    (full[4:], [wt(w_ref, 4 * T, M, n)], [wt(w_ref, 4 * T, M, n + 2)], _dot))
            out[4] = mm(full, [wt(w_ref, j * T, (j + 1) * T, 4) for j in range(km)])
            return out

        t_scr[0:CAR, :] = t_scr[RB:RB + CAR, :]
        for hf in range(nh):
            full = [a1_scr[j, _tile(hf), :] for j in range(km)]
            aops = []
            for k in range(2):
                ops = {m: a1s_scr[hf, i, k] for i, m in enumerate(SUMS)}
                ops[2], ops[3] = full[k][:HT], full[2 + k][HT:]
                aops.append(ops)
            for n, v in square(full, aops, w1_ref, ws12.at[0]).items():
                t = _gelu(v)
                if hf == nh - 1:
                    t = jnp.concatenate([t[:T - OFF], jnp.where(r < nrb - 1, t[T - OFF:], 0.0)], axis=0)
                t_scr[CAR + hf * T:CAR + (hf + 1) * T, _tile(n)] = t
        cq = M // 4
        shifts = (-1, 1, -2, 2)
        lane = jax.lax.broadcasted_iota(jnp.int32, (T, T), 1)
        y1, a3 = [], []
        for hf in range(nh):
            base = CAR - OFF + hf * T
            sh = []
            for j in range(km):
                g_lo, g_hi = (j * T) // cq, ((j + 1) * T - 1) // cq
                assert g_hi - g_lo <= 1
                v = t_scr[base + shifts[g_lo]:base + shifts[g_lo] + T, _tile(j)]
                if g_hi != g_lo:
                    v2 = t_scr[base + shifts[g_hi]:base + shifts[g_hi] + T, _tile(j)]
                    v = jnp.where(lane < g_hi * cq - j * T, v, v2)
                sh.append(v)
            hs = square([v.astype(BF16) for v in sh], [split_ops(sh[k], sh[2 + k]) for k in range(2)],
                        w2_ref, ws12.at[1])
            hs = jnp.concatenate([hs[n] for n in range(km)], axis=1)
            y1.append(hs + hb_scr[pl.ds(pl.multiple_of(r0 + hf * T, T), T), :])
            a3.append({})

            def ln_item(hf, c):
                def item(dep):
                    n = HT // NLN
                    for d in (0, HT):
                        v = y1[hf][d + c * n:d + (c + 1) * n]
                        if dep is not None:
                            v = jnp.concatenate([_after(v[:, :T], _rows(dep, n)), v[:, T:]], axis=1)
                        a3[hf][d + c * n] = _ln(v)
                return item

            ln_item(hf, 0)(None)
            pace += [(now[0] + LN0 + (c - 1) * LNS * (1 + hf), ln_item(hf, c)) for c in range(1, NLN)]
            pace.sort(key=lambda e: e[0])
        nf = FH // T
        h3, h3ops = [], []
        for hf in range(nh):
            assert len(a3[hf]) == 2 * NLN
            af = jnp.concatenate([a3[hf][key] for key in sorted(a3[hf])], axis=0)
            full = [af[:, _tile(j)].astype(BF16) for j in range(km)]
            aops = [split_ops(af[:, _tile(k)], af[:, _tile(2 + k)]) for k in range(2)]
            row, ops = {}, []
            narrow = None
            for n in range(nf):
                lo, hi = two_tiles(aops, lambda i, k: _ld(ws3, n, i, k),
                                   (full[4:], [wt(w3_ref, *ftiles[n], 4)],
                                    [wt(w3_ref, *ftiles[nf + n], 4)], _dot_nt))
                lo, hi = _gelu(lo), _gelu(hi)
                row[n], row[nf + n] = lo.astype(BF16), hi.astype(BF16)
                ops.append(split_ops(lo, hi))
                if n < km:
                    v = mm([wt(w3_ref, *ftiles[-1], n)], [full[n]], _dot_nt)
                    narrow = v if narrow is None else v + narrow
            row[2 * nf] = _gelu(mm(full, [wt(w3_ref, *ftiles[2 * nf], j) for j in range(km)],
                                   _dot_nt)).astype(BF16)
            fw = Fd - ftiles[-1][0]
            gT = jnp.concatenate([_gelu(narrow), jnp.zeros((T - fw, T), F32)], axis=0)
            row[2 * nf + 1] = _tie(gT.astype(BF16).T, gT[0:8, :])[:, :fw]
            h3.append([row[i] for i in range(len(ftiles))])
            h3ops.append(ops)
        for hf in range(nh):
            rows = pl.ds(pl.multiple_of(r0 + hf * T, T), T)

            def finish(n, v):
                out_buf[rows, _tile(n)] = (
                    x1_scr[rows, _tile(n)] + gb[:, _tile(n)] * (v + y1[hf][:, _tile(n)])
                ).astype(out_buf.dtype)

            w4t = lambda n, f_: [wt(w4_ref, f0, f1, n) for f0, f1 in f_]
            finish(4, mm(h3[hf], w4t(4, ftiles)))
            for n in range(2):
                lo, hi = two_tiles(h3ops[hf], lambda i, k: _ld(ws4, i, n, slice(k * HT, (k + 1) * HT)),
                                   (h3[hf][2 * nf:], w4t(n, ftiles[2 * nf:]), w4t(n + 2, ftiles[2 * nf:]), _dot))
                finish(n, lo)
                finish(n + 2, hi)
            out_copy(r * nh + hf).start()
        assert not pace
        return carry

    jax.lax.fori_loop(0, nrb, b_body, 0)
    for i in range(nb):
        out_copy(i).wait()


@jax.jit
def pallas_adaLN_cond__compressed_kv_cla__mixer_s_mlp__prompt_kernel(
    A_x: jax.Array,
    A_c_kv: jax.Array,
    A_w_q: jax.Array,
    A_w_uk: jax.Array,
    A_w_uv: jax.Array,
    A_w_o: jax.Array,
    B_x: jax.Array,
    B_w1: jax.Array,
    B_w2: jax.Array,
    B_w3: jax.Array,
    B_w4: jax.Array,
    c: jax.Array,
    w_mod: jax.Array,
):
    _, S, M = A_x.shape
    Dc = A_c_kv.shape[2]
    H, D = A_w_q.shape[1], A_w_q.shape[2]
    Fd = B_w3.shape[1]
    assert D == T and A_c_kv.shape[1] == S and Dc == 4 * T and M == 5 * T and 13 * T < Fd < 14 * T
    vmem = pltpu.VMEM
    packed = lambda *lead: vmem(lead + (T // 2, T), U32)
    out = pl.pallas_call(
        _kernel,
        in_specs=[pl.BlockSpec(memory_space=pltpu.HBM)] * 12,
        out_specs=pl.BlockSpec(memory_space=pltpu.HBM),
        out_shape=jax.ShapeDtypeStruct((S, M), A_x.dtype),
        scratch_shapes=[
            vmem((S + 16, M), BF16),
            vmem((S, Dc), BF16),
            vmem((1, M), BF16),
            vmem((M, 2 * M), BF16),
            vmem((M, 4 * M), BF16),
            vmem((M, M), BF16),
            vmem((M, M), BF16),
            vmem((Fd, M), BF16),
            vmem((Fd, M), BF16),
            vmem((M, D), U32),
            vmem((Dc, D), U32),
            vmem((Dc, D), U32),
            vmem((2, 2 * D, M), BF16),
            vmem((S, M), A_x.dtype),
            pltpu.SemaphoreType.DMA((15,)),
            pltpu.SemaphoreType.DMA((4,)),
            pltpu.SemaphoreType.DMA((S // T,)),
            vmem((8, 6 * M), F32),
            vmem((S // T, M // T, T, T), BF16),
            vmem((len(_C_SUMS), T, T), BF16),
            vmem((len(_H_SUMS), T, T), BF16),
            packed(2, M // T + 2 * (Dc // T)),
            packed(2 * S // T),
            packed(2 * S // T),
            packed(2 * S // T),
            vmem((S + 16, M), F32),
            vmem((S + 16, M), F32),
            vmem((S + 16, M), F32),
            vmem((M // T, RB, T), BF16),
            vmem((RB + 32, M), F32),
            vmem((RB // T, 5, 2, T // 2, T), BF16),
            vmem((2, 7, 2, T, T), U32),
            packed(6, 7, 2),
            vmem((7, 2, 3 * T, T), U32),
        ],
        compiler_params=pltpu.CompilerParams(
            vmem_limit_bytes=100 * 1024 * 1024,
            disable_bounds_checks=True,
        ),
    )(
        A_x.reshape(S, M), A_c_kv.reshape(S, Dc),
        A_w_q, A_w_uk, A_w_uv,
        A_w_o.reshape(H // 2, 2 * D, M),
        B_w1, B_w2, B_w3.T, B_w4, c, w_mod,
    )
    return out.reshape(1, S, M)
```

```python
import math

import jax
import jax.numpy as jnp
import jax.experimental.pallas as pl
import jax.experimental.pallas.tpu as pltpu

F32 = jnp.float32
BF16 = jnp.bfloat16
U32 = jnp.uint32
NT = (((1,), (1,)), ((), ()))
T = 128
EPS = 1e-5
LOG2E = math.log2(math.e)

GRP = 4
LEAD = 10
PROW = 3
RES = 32
LAT_A = 16
LAT_B = 20
ALEAD = 32
MID = 40
SD0, SDS = 60, 4
RB = 256
PC = 32
P0, PSTEP, PD = 440, 30, 52
NLN, LN0, LNS = 4, 4, 5
LP = 16
PROLOGUE = ('|kva|Z; |b|; kva|wc|K0123; bw|xdn|C0@56 N0123@52 K4567; cx|mq|N4567@52 K89ab; '
            'd|y|C1@56 Kcdef; nmq|zo|M H01 H234567@30 Q0123; y||H89ab@30 Q4567; '
            'z||Hcdef@30 Q89ab S01 Qcdef; o||')


def _dot(a, b):
    return jnp.dot(a, b, preferred_element_type=F32)


def _dot_nt(a, b):
    return jax.lax.dot_general(a, b, NT, preferred_element_type=F32)


def _ln(x):
    m = jnp.mean(x, axis=-1, keepdims=True)
    xc = x - m
    v = jnp.mean(xc * xc, axis=-1, keepdims=True)
    return xc * jnp.exp2(jnp.log(v + EPS) * (-0.5 * LOG2E))


def _rows(v, n):
    return jnp.broadcast_to(v[None], (n // 8, 8, v.shape[1])).reshape(n, v.shape[1])


def _gelu(x):
    c0 = math.sqrt(2.0 / math.pi)
    return 0.5 * x * (1.0 + jnp.tanh(c0 * (x + 0.044715 * (x * x * x))))


def _after(x, dep):
    return jnp.where(dep > jnp.inf, dep, x)


def _tie(x, dep):
    xu = pltpu.bitcast(x, U32)
    first = jnp.where(dep > jnp.inf, jnp.uint32(0), xu[:8])
    return pltpu.bitcast(jnp.concatenate([first, xu[8:]], axis=0), BF16)


def _tile(j):
    return slice(j * T, (j + 1) * T)


def _ld(ref, *idx):
    return pltpu.bitcast(ref[idx], BF16)


def _pk(x):
    return pltpu.bitcast(x, U32)


def _a_ops(a11, a12, a21, a22):
    return [a11 + a22, a21 + a22, a11, a22, a11 + a12, a21 - a11, a12 - a22]


SUMS = (0, 1, 4, 5, 6)


def _b_ops(b11, b12, b21, b22):
    return [b11 + b22, b11, b12 - b22, b21 - b11, b22, b11 + b12, b21 + b22]


def _strassen(prod, col1=None, col2=None):
    m4 = prod(3)
    m2 = prod(1)
    c21 = m2 + m4
    if col1 is not None:
        e11, e21 = col1()
        m4, c21 = m4 + e11, c21 + e21
    m3 = prod(2)
    m5 = prod(4)
    c12 = m3 + m5
    if col2 is not None:
        e12, e22 = col2()
        c12, m3 = c12 + e12, m3 + e22
    m1 = prod(0)
    c11 = prod(6) + (m1 + (m4 - m5))
    c22 = prod(5) + (m1 + (m3 - m2))
    return c11, c12, c21, c22


def _group(xs, ys):
    ks = sorted({k for _, k in xs + ys})
    prods = []
    for i, k in xs:
        mates = [y for y in ys if y[1] != k]
        prods.append((tuple((1, i, kk) for kk in ks), ((1, k, 0),), ((1, i, 0), (-1, i, 1))))
        prods.append((((1, i, k),) + tuple((-1, i2, k) for i2, _ in mates), ((1, k, 0), (1, k, 1)), ((1, i, 1),)))
        for i2, k2 in mates:
            prods.append((((1, i, k2),), ((1, k2, 0), (-1, k, 0)), ((1, i2, 0), (1, i, 0))))
            prods.append((((1, i2, k), (1, i, k2)), ((1, k, 0), (1, k2, 1)), ((1, i2, 0), (1, i, 1))))
            prods.append((((1, i2, k),), ((1, k, 1), (-1, k2, 1)), ((1, i2, 1), (1, i, 1))))
    for i2, k2 in ys:
        mates = [x for x in xs if x[1] != k2]
        prods.append((tuple((1, i2, kk) for kk in ks), ((1, k2, 1),), ((1, i2, 1), (-1, i2, 0))))
        prods.append((((1, i2, k2),) + tuple((-1, i, k2) for i, _ in mates), ((1, k2, 0), (1, k2, 1)),
                      ((1, i2, 0),)))
    return prods


def _full_group(r0, ks):
    q = len(ks)
    return _group([(r0 + a, k) for a, k in enumerate(ks)], [(r0 + q + a, k) for a, k in enumerate(ks)])


_C_GROUPS = [_full_group(0, range(4)), _full_group(8, range(4))]
_H_GROUPS = [_full_group(0, range(5)),
             [t for r in (10, 11, 12) for t in _group([(r, 3)], [(r + 3, 4)])] + _full_group(10, range(3))]
_sum_index = lambda groups: {f: n for n, f in enumerate(
    dict.fromkeys(t[0] for g in groups for t in g if len(t[0]) > 1))}
_C_SUMS, _H_SUMS = _sum_index(_C_GROUPS), _sum_index(_H_GROUPS)


def _form(form, get):
    acc = None
    for sign, i, j in form:
        v = get(i, j)
        acc = v if acc is None else (acc + v if sign > 0 else acc - v)
    return acc


class _PairWeights:
    def __init__(self, w_ref, transpose=False):
        self.base = {}
        for j in range(w_ref.shape[0] // T):
            wu = w_ref[_tile(j), :]
            if transpose:
                wu = wu.T
            self.base[j, 0] = pltpu.bitcast(wu << 16, F32)
            self.base[j, 1] = pltpu.bitcast(wu & jnp.uint32(0xFFFF0000), F32)
        self.cache = {}

    def __call__(self, form):
        sign = 1
        if form[-1][0] < 0 and form[0][1:] > form[1][1:]:
            sign, form = -1, ((1,) + form[1][1:], (-1,) + form[0][1:])
        if form not in self.cache:
            self.cache[form] = _form(form, lambda k, h: self.base[k, h]).astype(BF16)
        return sign, self.cache[form]


def _run_group(jobs, prods, a_get, w, transposed, finish):
    left = {}
    for _, _, outs in prods:
        for _, i, h in outs:
            left[i, h] = left.get((i, h), 0) + 1
    acc = {}
    for af, bf, outs in prods:
        sign, wt = w(bf)
        m = jobs.mm([wt], [a_get(af)], _dot_nt) if transposed else jobs.mm([a_get(af)], [wt], _dot)
        for s_, i, h in outs:
            if (i, h) not in acc:
                acc[i, h] = (s_ * sign, m)
            else:
                s0, v = acc[i, h]
                acc[i, h] = (s0, v + m if s0 == s_ * sign else v - m) if s0 > 0 or s_ * sign < 0 else (1, m - v)
            left[i, h] -= 1
            if not left[i, h]:
                s0, v = acc.pop((i, h))
                assert s0 > 0
                finish(2 * i + h, v)


class _Jobs:
    def __init__(self, side=()):
        self.res = []
        self.side = list(side)

    def mm(self, lhs, wt, dot):
        acc = None
        for x, w in zip(lhs, wt):
            v = dot(x, w)
            self.res.append(v)
            acc = v if acc is None else v + acc
            rel = 4 * (len(self.res) % 4)
            while self.side and self.side[0][0] <= len(self.res):
                self.side.pop(0)[1](v[8 * rel:8 * rel + 8, :])
                rel = (rel + 2) % 16
        return acc


def _proj_step(h_scr, hs_scr, c_ref, cs_scr, wq_ref, wuk_ref, wuv_ref, q_scr, k_scr, v_scr, scale, side):
    wq, wk, wvT = _PairWeights(wq_ref), _PairWeights(wuk_ref), _PairWeights(wuv_ref, True)
    c_get = lambda f: cs_scr[_C_SUMS[f]] if len(f) > 1 else c_ref[_tile(f[0][1]), _tile(f[0][2])]
    h_get = lambda f: hs_scr[_H_SUMS[f]] if len(f) > 1 else h_scr[f[0][1], f[0][2]]

    def put(dst, mul=None):
        def fn(u, v):
            dst[u] = _pk((v if mul is None else v * mul).astype(BF16))
        return fn

    jobs = _Jobs(side)
    for groups, get, w, transposed, fin in ((_C_GROUPS, c_get, wk, False, put(k_scr)),
                                            (_C_GROUPS, c_get, wvT, True, put(v_scr)),
                                            (_H_GROUPS, h_get, wq, False, put(q_scr, scale))):
        for prods in groups:
            _run_group(jobs, prods, get, w, transposed, fin)
    assert not jobs.side


def _inner_group(xs, ys):
    prods = []
    for i, j in xs:
        mates = [y for y in ys if y[1] != j]
        prods.append((((1, i, 0),), ((1, 0, j), (-1, 1, j)), ((1, i, j),) + tuple((1, i2, j) for i2, _ in mates)))
        prods.append((((1, i, 0), (1, i, 1)), ((1, 1, j),), ((1, i, j),) + tuple((-1, i, j2) for _, j2 in mates)))
    for i2, j2 in ys:
        mates = [x for x in xs if x[1] != j2]
        prods.append((((1, i2, 0), (1, i2, 1)), ((1, 0, j2),),
                      ((1, i2, j2),) + tuple((-1, i2, j) for _, j in mates)))
        prods.append((((1, i2, 1),), ((1, 0, j2), (-1, 1, j2)),
                      ((-1, i2, j2),) + tuple((-1, i, j2) for i, _ in mates)))
    for i, j in xs:
        for i2, j2 in ys:
            if j2 != j:
                lo, hi = min(j, j2), max(j, j2)
                prods.append((((1, i2, 0), (-1, i, 0)), ((1, 0, lo), (1, 0, hi)), ((1, i2, j),)))
                prods.append((((1, i, 0), (1, i2, 1)), ((1, 0, j2), (1, 1, j)), ((1, i, j2), (1, i2, j))))
                prods.append((((1, i, 1), (-1, i2, 1)), ((1, 1, lo), (1, 1, hi)), ((1, i, j2),)))
    return prods


def _o_jobs():
    alt = lambda r0, q: ([(r0 + 2 * a, a) for a in range(q)], [(r0 + 2 * a + 1, a) for a in range(q)])
    prods = _inner_group(*alt(0, 5)) + _inner_group(*alt(10, 3))
    for r in (10, 12, 14):
        prods += _inner_group([(r, 3)], [(r + 1, 4)])
    row = lambda t: max(i for _, i, _ in t[0])
    unit = lambda t: max(2 * i + h for _, i, h in t[0])
    need = lambda t: unit(t) if row(t) == 15 else 2 * row(t) + 1
    return [(need(t), t) for t in sorted(prods, key=need)]


_O_JOBS = _o_jobs()


def _job_order(nb):
    units = range(2 * nb)
    qa = [('a', u, c) for u in units for c in range(u // 2 + 1)]
    qb = [('b', u, c) for u in units for c in range(u // 2 + 1)]
    qo = [('o', u, j) for j, (u, _) in enumerate(_O_JOBS)]
    done = {}
    order = []

    def ready(q, lat, pre):
        return bool(q) and (pre, q[0][1]) in done and done[(pre, q[0][1])] + lat <= len(order)

    def emit(q):
        kind, u, j = job = q.pop(0)
        if kind != 'o' and j == u // 2:
            done[(kind, u)] = len(order)
        order.append(job)

    turn = 0
    while qa or qb or qo:
        pref = 'abo'[turn % 3]
        turn += 1
        for _ in range(GRP):
            b_ok, o_ok = ready(qb, LAT_A, 'a'), ready(qo, LAT_B, 'b')
            if pref == 'a' and qa and (len(qb) - len(qa) < ALEAD or not b_ok):
                emit(qa)
            elif pref == 'b' and b_ok:
                emit(qb)
            elif pref == 'o' and o_ok and (len(qo) > RES or not (qa or b_ok)):
                emit(qo)
            elif not (qa or b_ok or o_ok) and (qb or qo):
                emit(qb or qo)
            else:
                break
    return order


def _attention_step(q_scr, k_scr, v_scr, wo_ref, acc_scr, mid):
    causal = (jax.lax.broadcasted_iota(jnp.int32, (T, T), 0)
              <= jax.lax.broadcasted_iota(jnp.int32, (T, T), 1))
    sv, mx, mfin, lsum, pv, of, lhs = {}, {}, {}, {}, {}, {}, {}
    res = []
    wo, terms = {}, {}
    left = {}
    for _, t in _O_JOBS:
        for _, i, j in t[2]:
            left[i, j] = left.get((i, j), 0) + 1

    def job_a(u, c):
        r, hd = divmod(u, 2)
        s = _dot_nt(_ld(k_scr, 2 * c + hd), _ld(q_scr, u))
        res.append(s)
        if c == r:
            s = jnp.where(causal, s, -1e9 * LOG2E)
        s = s.reshape(T // 8, 8, T)
        sv[(u, c)] = s
        pm = jnp.max(s, axis=0)
        mx[u] = pm if u not in mx else jnp.maximum(mx[u], pm)

    def job_b(u, c):
        r, hd = divmod(u, 2)
        if u not in mfin:
            mfin[u] = jnp.broadcast_to(jnp.max(mx[u], axis=0, keepdims=True), (8, T))
        m = mfin[u]
        if len(res) >= LEAD:
            r0 = 8 * PROW * (c % 4)
            m = _after(m, res[len(res) - LEAD][r0:r0 + 8, :])
        p = jnp.exp2(sv.pop((u, c)) - m[None])
        ls = jnp.sum(p, axis=0)
        lsum[u] = ls if u not in lsum else lsum[u] + ls
        v = _dot(_ld(v_scr, 2 * c + hd), p.reshape(T, T).astype(BF16))
        res.append(v)
        pv[u] = v if u not in pv else v + pv[u]
        if c == r:
            of[u] = pv[u] * (1.0 / jnp.sum(lsum[u], axis=0, keepdims=True))

    def job_o(_, n):
        af, bf, outs = _O_JOBS[n][1]
        if af not in lhs:
            v = _form(af, lambda i, h: of[2 * i + h])
            lhs[af] = _tie(v.astype(BF16).T, v[0:8, :])
        if bf not in wo:
            wo[bf] = (wo_ref[_tile(bf[0][1]), _tile(bf[0][2])] if len(bf) == 1 else
                      _form(bf, lambda h, j: wo_ref[_tile(h), _tile(j)].astype(F32)).astype(BF16))
        v = _dot(lhs[af], wo[bf])
        res.append(v)
        for sign, i, j in outs:
            terms.setdefault((i, j), []).append((sign, v))
            if len(terms[i, j]) == left[i, j]:
                tot = acc_scr[_tile(i), _tile(j)]
                for sg, m in terms.pop((i, j)):
                    tot = tot + m if sg > 0 else tot - m
                acc_scr[_tile(i), _tile(j)] = tot

    fns = dict(a=job_a, b=job_b, o=job_o)
    for n, (kind, u, j) in enumerate(_job_order(q_scr.shape[0] // 2)):
        if n == MID:
            mid()
        fns[kind](u, j)


def _kernel(x_hbm, c_hbm, wq_hbm, wuk_hbm, wuv_hbm, wo_hbm, w1_hbm, w2_hbm, w3_hbm, w4_hbm,
            cond_hbm, wmod_hbm, out_hbm,
            x_ref, c_ref, cond_ref, wma_ref, wmb_ref, w1_ref, w2_ref, w3_ref, w4_ref,
            wq_buf, wk_buf, wv_buf, wo_buf, out_buf, sem, wsem, osem,
            mod_scr, h_scr, cs_scr, hs_scr, w_scr, q_scr, k_scr, v_scr, acc_scr, x1_scr, hb_scr, a1_scr, t_scr,
            a1s_scr, ws12, ws3, ws4):
    S, M = x_hbm.shape
    D = wq_hbm.shape[2]
    nattn = wo_hbm.shape[0]
    Fd = w4_hbm.shape[0]
    scale = float(D) ** -0.5 * LOG2E
    nb, nrb = S // T, S // RB
    km, kc = M // T, c_hbm.shape[1] // T
    NX = 4
    XR = S // NX
    CB = XR // T

    def pcopies(g):
        return [pltpu.make_async_copy(src.bitcast(U32).at[:, g, :], dst, wsem.at[j])
                for j, (src, dst) in enumerate(((wuk_hbm, wk_buf), (wuv_hbm, wv_buf), (wq_hbm, wq_buf)))]

    def ocopy(g, slot):
        return pltpu.make_async_copy(wo_hbm.at[g], wo_buf.at[slot], wsem.at[3])

    def chunk_copy(src, dst, i, s0):
        rows = slice(i * XR, (i + 1) * XR)
        return pltpu.make_async_copy(src.at[rows, :], dst.at[rows, :], sem.at[s0 + i])

    cp_cond = pltpu.make_async_copy(cond_hbm, cond_ref, sem.at[0])
    cp_wma = pltpu.make_async_copy(wmod_hbm.at[:, 0:2 * M], wma_ref, sem.at[1])
    cp_late = [pltpu.make_async_copy(src, dst, sem.at[2 + j]) for j, (src, dst) in enumerate((
        (wmod_hbm.at[:, 2 * M:6 * M], wmb_ref), (w1_hbm, w1_ref), (w2_hbm, w2_ref),
        (w3_hbm, w3_ref), (w4_hbm, w4_ref)))]
    cp_x = [chunk_copy(x_hbm, x_ref, i, 7) for i in range(NX)]
    cp_c = [chunk_copy(c_hbm, c_ref, i, 7 + NX) for i in range(NX)]

    def silu_cond():
        cf = cond_ref[...].astype(F32)
        return jnp.broadcast_to((cf * jax.nn.sigmoid(cf)).astype(BF16), (8, M))

    cp_wk, cp_wv, cp_wq = pcopies(0)
    named = dict(k=cp_wk, v=cp_wv, q=cp_wq, o=ocopy(0, 0), n=cp_cond, m=cp_wma)
    named.update(zip('abcd', cp_c))
    named.update(zip('wxyz', cp_x))
    started, arrived, did = set(), set(), set()

    def zero(r, carry):
        acc_scr[pl.ds(pl.multiple_of(r * T, T), T), :] = jnp.zeros((T, M), F32)
        return carry

    def x_rows(rows, dep):
        xf = x_ref[rows, :].astype(F32)
        if dep is None:
            return xf
        return jnp.concatenate([_after(xf[:, :T], _rows(dep, xf.shape[0])), xf[:, T:]], axis=1)

    def n_item(r, i):
        def fn(dep):
            rows = slice(r * T + i * LP, r * T + (i + 1) * LP)
            x1_scr[rows, :] = _ln(x_rows(rows, dep))
        return fn

    def h_item(r, i, normed):
        def fn(dep):
            rows = slice(i * LP, (i + 1) * LP)
            grows = slice(r * T + i * LP, r * T + (i + 1) * LP)
            sa = mod_scr[:, 0:M]
            if normed and dep is not None:
                sa = jnp.concatenate([_after(sa[:, _tile(j)], dep) for j in range(km)], axis=1)
            hf = ((x1_scr[grows, :] if normed else _ln(x_rows(grows, dep))) * _rows(mod_scr[:, M:2 * M], LP)
                  + _rows(sa, LP))
            for j in range(km):
                h_scr[r, j, rows, :] = hf[:, _tile(j)].astype(BF16)
            for f, n in _H_SUMS.items():
                if all(t[1] == r for t in f):
                    hs_scr[n, rows, :] = _form(f, lambda _, k: hf[:, _tile(k)]).astype(BF16)
            did.add(('h', r, i))
        return fn

    def release(jobs, span, items):
        if span and items:
            jobs.side += [(len(jobs.res) + 1 + i * span // len(items), fn) for i, fn in enumerate(items)]
            jobs.side.sort(key=lambda e: e[0])
        else:
            for fn in items:
                fn(None)

    def sum_items(n, group, index, dst, get, skip_rows):
        forms = [f for f in dict.fromkeys(t[0] for t in group)
                 if len(f) > 1 and not (skip_rows and len({t[1] for t in f}) == 1)]

        def item(f, rows):
            def fn(dep):
                def term(r, k):
                    v = get(r, k, rows).astype(F32)
                    return v if dep is None or (r, k) != f[0][1:] else _after(v, _rows(dep, v.shape[0]))
                dst[index[f], rows, :] = _form(f, term).astype(BF16)
            return fn

        return [item(f, slice(i, i + n)) for i in range(0, T, n) for f in forms]

    h_sums = lambda n, gi: sum_items(n, _H_GROUPS[gi], _H_SUMS, hs_scr,
                                     lambda r_, k, rows: h_scr[r_, k, rows, :], True)

    def stash(key, buf, j0, transpose=False):
        n = buf.shape[0] // T
        if key not in did:
            assert key in arrived
            did.add(key)
            w = _PairWeights(buf, transpose)
            for j in range(n):
                for hd in range(2):
                    w_scr[hd, j0 + j] = _pk(w(((1, j, hd),))[1])
        return lambda hd: [_ld(w_scr, hd, j0 + j) for j in range(n)]

    def kv_tile(jobs, r):
        wk, wvT = stash('k', wk_buf, 0), stash('v', wv_buf, kc, True)
        ct = [c_ref[_tile(r), _tile(j)] for j in range(kc)]
        for hd in range(2):
            k_scr[2 * r + hd] = _pk(jobs.mm(ct, wk(hd), _dot).astype(BF16))
        for hd in range(2):
            v_scr[2 * r + hd] = _pk(jobs.mm(wvT(hd), ct, _dot_nt).astype(BF16))

    def q_tile(jobs, r):
        wq = stash('q', wq_buf, 2 * kc)
        ht = [h_scr[r, j] for j in range(km)]
        for hd in range(2):
            q_scr[2 * r + hd] = _pk((jobs.mm(ht, wq(hd), _dot) * scale).astype(BF16))

    for blk in PROLOGUE.split(';'):
        waits, starts, acts = blk.split('|')
        for ch in waits.strip():
            assert ch in started and ch not in arrived
            arrived.add(ch)
            named[ch].wait()
        for ch in starts.strip():
            assert ch not in started
            started.add(ch)
            named[ch].start()
        jobs = _Jobs()
        for act in acts.split():
            if act == 'Z':
                jax.lax.fori_loop(0, nb, zero, 0)
                acc_scr[S:, :] = jnp.zeros((acc_scr.shape[0] - S, M), F32)
                x_ref[S:, :] = jnp.zeros((x_ref.shape[0] - S, M), BF16)
            elif act == 'M':
                assert arrived >= set('nm')
                mod = _dot(silu_cond(), wma_ref[...])
                mod_scr[:, 0:M] = mod[:, 0:M]
                mod_scr[:, M:2 * M] = 1.0 + mod[:, M:2 * M]
                did.add('M')
            else:
                act, _, span = act.partition('@')
                span = int(span or 0)
                items = []
                for r in [int(ch, 16) for ch in act[1:]]:
                    did.add((act[0], r))
                    if act[0] == 'K':
                        assert 'abcd'[r // CB] in arrived
                        kv_tile(jobs, r)
                    elif act[0] == 'H':
                        assert 'wxyz'[r // CB] in arrived and 'M' in did
                        items += [h_item(r, i, ('N', r) in did) for i in range(T // LP)]
                    elif act[0] == 'N':
                        assert 'wxyz'[r // CB] in arrived
                        items += [n_item(r, i) for i in range(T // LP)]
                    elif act[0] == 'Q':
                        assert all(('h', r, i) in did for i in range(T // LP))
                        q_tile(jobs, r)
                    elif act[0] == 'C':
                        assert all('abcd'[t[1] // CB] in arrived for p_ in _C_GROUPS[r] for t in p_[0])
                        items += sum_items(
                            32, _C_GROUPS[r], _C_SUMS, cs_scr,
                            lambda r_, k, rows: c_ref[r_ * T + rows.start:r_ * T + rows.stop, _tile(k)], False)
                    else:
                        assert act[0] == 'S' and all(('h', t[1], T // LP - 1) in did for p_ in _H_GROUPS[r] for t in p_[0])
                        items += h_sums(32 if span else 16, r)
                release(jobs, span, items)
        assert not jobs.side
    assert arrived == set(named) and all((k_, r) in did for k_ in 'KHQ' for r in range(nb))
    assert all((k_, r) in did for k_ in 'CS' for r in range(2))
    for cp in cp_late[1:] + cp_late[:1]:
        cp.start()

    FH = ws3.shape[0] * T
    assert nattn - 1 >= FH // 64

    def mixer_prep(g):
        def blocks(w_ref, r0, n, half, c0, c1, dep):
            lo, hi = pl.ds(r0, n), pl.ds(r0 + half, n)
            return [_after(w_ref[rows, _tile(c)].astype(F32), _rows(dep, n)) if (rows is lo) == (c == c0)
                    else w_ref[rows, _tile(c)].astype(F32) for rows in (lo, hi) for c in (c0, c1)]

        def rows_items(w_ref, dst, per_step, half, n=16):
            gi = jnp.minimum(g, half // per_step - 1)
            src = w_ref.at[pl.ds(pl.multiple_of(gi * per_step, per_step), half + per_step), :]
            hs = per_step // 2

            def item(c, o):
                def fn(dep):
                    for i, v in enumerate(_b_ops(*blocks(src, o, n, half, c, c + 2, dep))):
                        dst[i, c, pl.ds(pl.multiple_of(gi * hs, hs) + o // 2, n // 2), :] = _pk(v.astype(BF16))
                return fn
            return [item(c, o) for c in range(2) for o in range(0, per_step, n)]

        def w3_item(k, i):
            def fn(dep):
                n = jnp.minimum(g, FH // T - 1)
                b11, b21, b12, b22 = blocks(w3_ref, pl.multiple_of(n * T, T), T, FH, k, k + 2, dep)
                ws3[n, i, k] = _pk(_b_ops(b11, b12, b21, b22)[i].astype(BF16).T)
            return fn

        return (rows_items(w1_ref, ws12.at[0], 32, 2 * T) + rows_items(w2_ref, ws12.at[1], 32, 2 * T)
                + rows_items(w4_ref, ws4, 64, FH) + [w3_item(k, i) for k in range(2) for i in range(7)])

    def attn_body(g, carry):
        slot = g & 1
        nxt = jnp.minimum(g + 1, nattn - 1)
        copies = pcopies(nxt) + [ocopy(nxt, 1 - slot)]

        def mid():
            for cp in copies:
                cp.start()

        _attention_step(q_scr, k_scr, v_scr, wo_buf.at[slot], acc_scr, mid)
        for cp in copies:
            cp.wait()

        @pl.when(g == 0)
        def _():
            for cp in cp_late[1:]:
                cp.wait()

        @pl.when(g + 1 < nattn)
        def _():
            side = [(SD0 + i * SDS, fn) for i, fn in enumerate(mixer_prep(g))]
            _proj_step(h_scr, hs_scr, c_ref, cs_scr, wq_buf, wk_buf, wv_buf, q_scr, k_scr, v_scr, scale, side)

        return carry

    jax.lax.fori_loop(0, nattn, attn_body, 0)

    cp_late[0].wait()
    mod = _dot(silu_cond(), wmb_ref[...])
    mod_scr[:, 2 * M:4 * M] = mod[:, 0:2 * M]
    mod_scr[:, 4 * M:5 * M] = 1.0 + mod[:, 2 * M:3 * M]
    mod_scr[:, 5 * M:6 * M] = mod[:, 3 * M:4 * M]
    ftiles = [(f, min(f + T, Fd)) for f in range(0, Fd, T)]
    OFF = x_ref.shape[0] - S
    CAR = t_scr.shape[0] - RB

    def p1(r0, n, dep=None):
        ga = mod_scr[:, 2 * M:3 * M]
        if dep is not None:
            ga = jnp.concatenate([_after(ga[:, 0:T], dep), ga[:, T:]], axis=1)
        rows = pl.ds(r0, n)
        x1 = x_ref[rows, :].astype(F32) + _rows(ga, n) * acc_scr[rows, :]
        x1_scr[rows, :] = x1
        hb = _ln(x1) * _rows(mod_scr[:, 4 * M:5 * M], n) + _rows(mod_scr[:, 3 * M:4 * M], n)
        hb_scr[rows, :] = hb
        return _ln(hb)

    HT = T // 2

    def p1_store(r0, c, dep=None):
        n = PC // 2
        hf, o = divmod(c * n, HT)
        top, bot = [p1(r0 + hf * T + d + o, n, dep) for d in (0, HT)]
        for d, v in ((0, top), (HT, bot)):
            for j in range(km):
                a1_scr[j, hf * T + d + o:hf * T + d + o + n, :] = v[:, _tile(j)].astype(BF16)
        ops = _a_ops(top[:, 0:2 * T], top[:, 2 * T:4 * T], bot[:, 0:2 * T], bot[:, 2 * T:4 * T])
        for i, m in enumerate(SUMS):
            for k in range(2):
                a1s_scr[hf, i, k, o:o + n, :] = ops[m][:, _tile(k)].astype(BF16)
        return jnp.max(ops[0][:, :T].reshape(n // 8, 8, T), axis=0)

    t_scr[RB:RB + CAR - OFF, :] = jnp.zeros((CAR - OFF, M), F32)
    t_scr[RB + CAR - OFF:RB + CAR, :] = _gelu(_dot(p1(0, OFF).astype(BF16), w1_ref[...]))
    for c in range(RB // PC):
        p1_store(OFF, c)

    def out_copy(i):
        rows = pl.ds(i * T if isinstance(i, int) else pl.multiple_of(i * T, T), T)
        return pltpu.make_async_copy(out_buf.at[rows, :], out_hbm.at[rows, :], osem.at[i])

    def b_body(r, carry):
        gb = _rows(mod_scr[:, 5 * M:6 * M], T)
        r0 = pl.multiple_of(r * RB, RB)
        n0 = pl.multiple_of(jnp.minimum(r0 + RB, S - RB) + OFF, OFF)
        nh = RB // T
        now = [0]
        due = []
        pace = []

        def p1_item(c):
            return lambda dep: due.append((now[0] + PD, p1_store(n0, c, dep)))

        pace += [(P0 + i * PSTEP, p1_item(i)) for i in range(RB // PC)]
        wt = lambda ref, f0, f1, n: ref[f0:f1, _tile(n)]

        def mm(lhs, wts, dot=_dot):
            acc = None
            for x, w in zip(lhs, wts):
                if due and due[0][0] <= now[0]:
                    w = _tie(w, due.pop(0)[1])
                v = dot(x, w)
                now[0] += x.shape[0] // HT
                acc = v if acc is None else v + acc
                if pace and pace[0][0] <= now[0]:
                    pace.pop(0)[1](v[0:8, :])
            return acc

        def split_ops(lo, hi):
            return [v.astype(BF16) for v in _a_ops(lo[:HT], hi[:HT], lo[HT:], hi[HT:])]

        def two_tiles(aops, wsel, rest):
            def col(w):
                v = mm(rest[0], w, rest[3])
                return v[:HT], v[HT:]

            c11, c12, c21, c22 = _strassen(
                lambda i: mm([a[i] for a in aops], [wsel(i, k) for k in range(len(aops))]),
                lambda: col(rest[1]), lambda: col(rest[2]))
            return jnp.concatenate([c11, c21], axis=0), jnp.concatenate([c12, c22], axis=0)

        def square(full, aops, w_ref, ws_ref):
            out = {}
            for n in range(2):
                out[n], out[n + 2] = two_tiles(
                    aops, lambda i, k: _ld(ws_ref, i, n, slice(k * HT, (k + 1) * HT)),
                    (full[4:], [wt(w_ref, 4 * T, M, n)], [wt(w_ref, 4 * T, M, n + 2)], _dot))
            out[4] = mm(full, [wt(w_ref, j * T, (j + 1) * T, 4) for j in range(km)])
            return out

        t_scr[0:CAR, :] = t_scr[RB:RB + CAR, :]
        for hf in range(nh):
            full = [a1_scr[j, _tile(hf), :] for j in range(km)]
            aops = []
            for k in range(2):
                ops = {m: a1s_scr[hf, i, k] for i, m in enumerate(SUMS)}
                ops[2], ops[3] = full[k][:HT], full[2 + k][HT:]
                aops.append(ops)
            for n, v in square(full, aops, w1_ref, ws12.at[0]).items():
                t = _gelu(v)
                if hf == nh - 1:
                    t = jnp.concatenate([t[:T - OFF], jnp.where(r < nrb - 1, t[T - OFF:], 0.0)], axis=0)
                t_scr[CAR + hf * T:CAR + (hf + 1) * T, _tile(n)] = t
        cq = M // 4
        shifts = (-1, 1, -2, 2)
        lane = jax.lax.broadcasted_iota(jnp.int32, (T, T), 1)
        y1, a3 = [], []
        for hf in range(nh):
            base = CAR - OFF + hf * T
            sh = []
            for j in range(km):
                g_lo, g_hi = (j * T) // cq, ((j + 1) * T - 1) // cq
                assert g_hi - g_lo <= 1
                v = t_scr[base + shifts[g_lo]:base + shifts[g_lo] + T, _tile(j)]
                if g_hi != g_lo:
                    v2 = t_scr[base + shifts[g_hi]:base + shifts[g_hi] + T, _tile(j)]
                    v = jnp.where(lane < g_hi * cq - j * T, v, v2)
                sh.append(v)
            hs = square([v.astype(BF16) for v in sh], [split_ops(sh[k], sh[2 + k]) for k in range(2)],
                        w2_ref, ws12.at[1])
            hs = jnp.concatenate([hs[n] for n in range(km)], axis=1)
            y1.append(hs + hb_scr[pl.ds(pl.multiple_of(r0 + hf * T, T), T), :])
            a3.append({})

            def ln_item(hf, c):
                def item(dep):
                    n = HT // NLN
                    for d in (0, HT):
                        v = y1[hf][d + c * n:d + (c + 1) * n]
                        if dep is not None:
                            v = jnp.concatenate([_after(v[:, :T], _rows(dep, n)), v[:, T:]], axis=1)
                        a3[hf][d + c * n] = _ln(v)
                return item

            ln_item(hf, 0)(None)
            pace += [(now[0] + LN0 + (c - 1) * LNS * (1 + hf), ln_item(hf, c)) for c in range(1, NLN)]
            pace.sort(key=lambda e: e[0])
        nf = FH // T
        h3, h3ops = [], []
        for hf in range(nh):
            assert len(a3[hf]) == 2 * NLN
            af = jnp.concatenate([a3[hf][key] for key in sorted(a3[hf])], axis=0)
            full = [af[:, _tile(j)].astype(BF16) for j in range(km)]
            aops = [split_ops(af[:, _tile(k)], af[:, _tile(2 + k)]) for k in range(2)]
            row, ops = {}, []
            narrow = None
            for n in range(nf):
                lo, hi = two_tiles(aops, lambda i, k: _ld(ws3, n, i, k),
                                   (full[4:], [wt(w3_ref, *ftiles[n], 4)],
                                    [wt(w3_ref, *ftiles[nf + n], 4)], _dot_nt))
                lo, hi = _gelu(lo), _gelu(hi)
                row[n], row[nf + n] = lo.astype(BF16), hi.astype(BF16)
                ops.append(split_ops(lo, hi))
                if n < km:
                    v = mm([wt(w3_ref, *ftiles[-1], n)], [full[n]], _dot_nt)
                    narrow = v if narrow is None else v + narrow
            row[2 * nf] = _gelu(mm(full, [wt(w3_ref, *ftiles[2 * nf], j) for j in range(km)],
                                   _dot_nt)).astype(BF16)
            fw = Fd - ftiles[-1][0]
            gT = jnp.concatenate([_gelu(narrow), jnp.zeros((T - fw, T), F32)], axis=0)
            row[2 * nf + 1] = _tie(gT.astype(BF16).T, gT[0:8, :])[:, :fw]
            h3.append([row[i] for i in range(len(ftiles))])
            h3ops.append(ops)
        for hf in range(nh):
            rows = pl.ds(pl.multiple_of(r0 + hf * T, T), T)

            def finish(n, v):
                out_buf[rows, _tile(n)] = (
                    x1_scr[rows, _tile(n)] + gb[:, _tile(n)] * (v + y1[hf][:, _tile(n)])
                ).astype(out_buf.dtype)

            w4t = lambda n, f_: [wt(w4_ref, f0, f1, n) for f0, f1 in f_]
            finish(4, mm(h3[hf], w4t(4, ftiles)))
            for n in range(2):
                lo, hi = two_tiles(h3ops[hf], lambda i, k: _ld(ws4, i, n, slice(k * HT, (k + 1) * HT)),
                                   (h3[hf][2 * nf:], w4t(n, ftiles[2 * nf:]), w4t(n + 2, ftiles[2 * nf:]), _dot))
                finish(n, lo)
                finish(n + 2, hi)
            out_copy(r * nh + hf).start()
        assert not pace
        return carry

    jax.lax.fori_loop(0, nrb, b_body, 0)
    for i in range(nb):
        out_copy(i).wait()


@jax.jit
def pallas_adaLN_cond__compressed_kv_cla__mixer_s_mlp__prompt_kernel(
    A_x: jax.Array,
    A_c_kv: jax.Array,
    A_w_q: jax.Array,
    A_w_uk: jax.Array,
    A_w_uv: jax.Array,
    A_w_o: jax.Array,
    B_x: jax.Array,
    B_w1: jax.Array,
    B_w2: jax.Array,
    B_w3: jax.Array,
    B_w4: jax.Array,
    c: jax.Array,
    w_mod: jax.Array,
):
    _, S, M = A_x.shape
    Dc = A_c_kv.shape[2]
    H, D = A_w_q.shape[1], A_w_q.shape[2]
    Fd = B_w3.shape[1]
    assert D == T and A_c_kv.shape[1] == S and Dc == 4 * T and M == 5 * T and 13 * T < Fd < 14 * T and S == 16 * T
    vmem = pltpu.VMEM
    packed = lambda *lead: vmem(lead + (T // 2, T), U32)
    out = pl.pallas_call(
        _kernel,
        in_specs=[pl.BlockSpec(memory_space=pltpu.HBM)] * 12,
        out_specs=pl.BlockSpec(memory_space=pltpu.HBM),
        out_shape=jax.ShapeDtypeStruct((S, M), A_x.dtype),
        scratch_shapes=[
            vmem((S + 16, M), BF16),
            vmem((S, Dc), BF16),
            vmem((1, M), BF16),
            vmem((M, 2 * M), BF16),
            vmem((M, 4 * M), BF16),
            vmem((M, M), BF16),
            vmem((M, M), BF16),
            vmem((Fd, M), BF16),
            vmem((Fd, M), BF16),
            vmem((M, D), U32),
            vmem((Dc, D), U32),
            vmem((Dc, D), U32),
            vmem((2, 2 * D, M), BF16),
            vmem((S, M), A_x.dtype),
            pltpu.SemaphoreType.DMA((15,)),
            pltpu.SemaphoreType.DMA((4,)),
            pltpu.SemaphoreType.DMA((S // T,)),
            vmem((8, 6 * M), F32),
            vmem((S // T, M // T, T, T), BF16),
            vmem((len(_C_SUMS), T, T), BF16),
            vmem((len(_H_SUMS), T, T), BF16),
            packed(2, M // T + 2 * (Dc // T)),
            packed(2 * S // T),
            packed(2 * S // T),
            packed(2 * S // T),
            vmem((S + 16, M), F32),
            vmem((S + 16, M), F32),
            vmem((S + 16, M), F32),
            vmem((M // T, RB, T), BF16),
            vmem((RB + 32, M), F32),
            vmem((RB // T, 5, 2, T // 2, T), BF16),
            vmem((2, 7, 2, T, T), U32),
            packed(6, 7, 2),
            vmem((7, 2, 3 * T, T), U32),
        ],
        compiler_params=pltpu.CompilerParams(
            vmem_limit_bytes=100 * 1024 * 1024,
            disable_bounds_checks=True,
        ),
    )(
        A_x.reshape(S, M), A_c_kv.reshape(S, Dc),
        A_w_q, A_w_uk, A_w_uv,
        A_w_o.reshape(H // 2, 2 * D, M),
        B_w1, B_w2, B_w3.T, B_w4, c, w_mod,
    )
    return out.reshape(1, S, M)
```

```python
import math

import jax
import jax.numpy as jnp
import jax.experimental.pallas as pl
import jax.experimental.pallas.tpu as pltpu

F32 = jnp.float32
BF16 = jnp.bfloat16
U32 = jnp.uint32
NT = (((1,), (1,)), ((), ()))
T = 128
EPS = 1e-5
LOG2E = math.log2(math.e)

GRP = 4
LEAD = 10
PROW = 3
RES = 32
LAT_A = 16
LAT_B = 20
ALEAD = 32
MID = 40
SD0, SDS = 60, 4
RB = 256
PC = 32
P0, PSTEP, PD = 440, 30, 52
NLN, LN0, LNS = 4, 4, 5
LP = 16
PROLOGUE = ('|kva|Z; |b|; kva|wc|K0123; bw|xdn|C0@56 N0123@52 K4567; cx|mq|N4567@52 K89ab; '
            'd|y|C1@56 Kcdef; nmq|zo|M H01 H234567@30 Q0123; y||H89ab@30 Q4567; '
            'z||Hcdef@30 Q89ab S01 Qcdef; o||')


def _dot(a, b):
    return jnp.dot(a, b, preferred_element_type=F32)


def _dot_nt(a, b):
    return jax.lax.dot_general(a, b, NT, preferred_element_type=F32)


def _ln(x):
    m = jnp.mean(x, axis=-1, keepdims=True)
    xc = x - m
    v = jnp.mean(xc * xc, axis=-1, keepdims=True)
    return xc * jnp.exp2(jnp.log(v + EPS) * (-0.5 * LOG2E))


def _rows(v, n):
    return jnp.broadcast_to(v[None], (n // 8, 8, v.shape[1])).reshape(n, v.shape[1])


def _gelu(x):
    c0 = math.sqrt(2.0 / math.pi)
    return 0.5 * x * (1.0 + jnp.tanh(c0 * (x + 0.044715 * (x * x * x))))


def _after(x, dep):
    return jnp.where(dep > jnp.inf, dep, x)


def _tie(x, dep):
    xu = pltpu.bitcast(x, U32)
    first = jnp.where(dep > jnp.inf, jnp.uint32(0), xu[:8])
    return pltpu.bitcast(jnp.concatenate([first, xu[8:]], axis=0), BF16)


def _tile(j):
    return slice(j * T, (j + 1) * T)


def _ld(ref, *idx):
    return pltpu.bitcast(ref[idx], BF16)


def _pk(x):
    return pltpu.bitcast(x, U32)


def _a_ops(a11, a12, a21, a22):
    return [a11 + a22, a21 + a22, a11, a22, a11 + a12, a21 - a11, a12 - a22]


SUMS = (0, 1, 4, 5, 6)


def _b_ops(b11, b12, b21, b22):
    return [b11 + b22, b11, b12 - b22, b21 - b11, b22, b11 + b12, b21 + b22]


def _strassen(prod, col1=None, col2=None):
    m4 = prod(3)
    m2 = prod(1)
    c21 = m2 + m4
    if col1 is not None:
        e11, e21 = col1()
        m4, c21 = m4 + e11, c21 + e21
    m3 = prod(2)
    m5 = prod(4)
    c12 = m3 + m5
    if col2 is not None:
        e12, e22 = col2()
        c12, m3 = c12 + e12, m3 + e22
    m1 = prod(0)
    c11 = prod(6) + (m1 + (m4 - m5))
    c22 = prod(5) + (m1 + (m3 - m2))
    return c11, c12, c21, c22


def _group(xs, ys):
    ks = sorted({k for _, k in xs + ys})
    prods = []
    for i, k in xs:
        mates = [y for y in ys if y[1] != k]
        prods.append((tuple((1, i, kk) for kk in ks), ((1, k, 0),), ((1, i, 0), (-1, i, 1))))
        prods.append((((1, i, k),) + tuple((-1, i2, k) for i2, _ in mates), ((1, k, 0), (1, k, 1)), ((1, i, 1),)))
        for i2, k2 in mates:
            prods.append((((1, i, k2),), ((1, k2, 0), (-1, k, 0)), ((1, i2, 0), (1, i, 0))))
            prods.append((((1, i2, k), (1, i, k2)), ((1, k, 0), (1, k2, 1)), ((1, i2, 0), (1, i, 1))))
            prods.append((((1, i2, k),), ((1, k, 1), (-1, k2, 1)), ((1, i2, 1), (1, i, 1))))
    for i2, k2 in ys:
        mates = [x for x in xs if x[1] != k2]
        prods.append((tuple((1, i2, kk) for kk in ks), ((1, k2, 1),), ((1, i2, 1), (-1, i2, 0))))
        prods.append((((1, i2, k2),) + tuple((-1, i, k2) for i, _ in mates), ((1, k2, 0), (1, k2, 1)),
                      ((1, i2, 0),)))
    return prods


def _full_group(r0, ks):
    q = len(ks)
    return _group([(r0 + a, k) for a, k in enumerate(ks)], [(r0 + q + a, k) for a, k in enumerate(ks)])


_C_GROUPS = [_full_group(0, range(4)), _full_group(8, range(4))]
_H_GROUPS = [_full_group(0, range(5)),
             [t for r in (10, 11, 12) for t in _group([(r, 3)], [(r + 3, 4)])] + _full_group(10, range(3))]
_sum_index = lambda groups: {f: n for n, f in enumerate(
    dict.fromkeys(t[0] for g in groups for t in g if len(t[0]) > 1))}
_C_SUMS, _H_SUMS = _sum_index(_C_GROUPS), _sum_index(_H_GROUPS)


def _form(form, get):
    acc = None
    for sign, i, j in form:
        v = get(i, j)
        acc = v if acc is None else (acc + v if sign > 0 else acc - v)
    return acc


class _PairWeights:
    def __init__(self, w_ref, transpose=False):
        self.base = {}
        for j in range(w_ref.shape[0] // T):
            wu = w_ref[_tile(j), :]
            if transpose:
                wu = wu.T
            self.base[j, 0] = pltpu.bitcast(wu << 16, F32)
            self.base[j, 1] = pltpu.bitcast(wu & jnp.uint32(0xFFFF0000), F32)
        self.cache = {}

    def __call__(self, form):
        sign = 1
        if form[-1][0] < 0 and form[0][1:] > form[1][1:]:
            sign, form = -1, ((1,) + form[1][1:], (-1,) + form[0][1:])
        if form not in self.cache:
            self.cache[form] = _form(form, lambda k, h: self.base[k, h]).astype(BF16)
        return sign, self.cache[form]


def _run_group(jobs, prods, a_get, w, transposed, finish):
    left = {}
    for _, _, outs in prods:
        for _, i, h in outs:
            left[i, h] = left.get((i, h), 0) + 1
    acc = {}
    for af, bf, outs in prods:
        sign, wt = w(bf)
        m = jobs.mm([wt], [a_get(af)], _dot_nt) if transposed else jobs.mm([a_get(af)], [wt], _dot)
        for s_, i, h in outs:
            if (i, h) not in acc:
                acc[i, h] = (s_ * sign, m)
            else:
                s0, v = acc[i, h]
                acc[i, h] = (s0, v + m if s0 == s_ * sign else v - m) if s0 > 0 or s_ * sign < 0 else (1, m - v)
            left[i, h] -= 1
            if not left[i, h]:
                s0, v = acc.pop((i, h))
                assert s0 > 0
                finish(2 * i + h, v)


class _Jobs:
    def __init__(self, side=()):
        self.res = []
        self.side = list(side)

    def mm(self, lhs, wt, dot):
        acc = None
        for x, w in zip(lhs, wt):
            v = dot(x, w)
            self.res.append(v)
            acc = v if acc is None else v + acc
            rel = 4 * (len(self.res) % 4)
            while self.side and self.side[0][0] <= len(self.res):
                self.side.pop(0)[1](v[8 * rel:8 * rel + 8, :])
                rel = (rel + 2) % 16
        return acc


def _proj_step(h_scr, hs_scr, c_ref, cs_scr, wq_ref, wuk_ref, wuv_ref, q_scr, k_scr, v_scr, scale, side):
    wq, wk, wvT = _PairWeights(wq_ref), _PairWeights(wuk_ref), _PairWeights(wuv_ref, True)
    c_get = lambda f: cs_scr[_C_SUMS[f]] if len(f) > 1 else c_ref[_tile(f[0][1]), _tile(f[0][2])]
    h_get = lambda f: hs_scr[_H_SUMS[f]] if len(f) > 1 else h_scr[f[0][1], f[0][2]]

    def put(dst, mul=None):
        def fn(u, v):
            dst[u] = _pk((v if mul is None else v * mul).astype(BF16))
        return fn

    jobs = _Jobs(side)
    for groups, get, w, transposed, fin in ((_C_GROUPS, c_get, wk, False, put(k_scr)),
                                            (_C_GROUPS, c_get, wvT, True, put(v_scr)),
                                            (_H_GROUPS, h_get, wq, False, put(q_scr, scale))):
        for prods in groups:
            _run_group(jobs, prods, get, w, transposed, fin)
    assert not jobs.side


def _inner_group(xs, ys):
    prods = []
    for i, j in xs:
        mates = [y for y in ys if y[1] != j]
        prods.append((((1, i, 0),), ((1, 0, j), (-1, 1, j)), ((1, i, j),) + tuple((1, i2, j) for i2, _ in mates)))
        prods.append((((1, i, 0), (1, i, 1)), ((1, 1, j),), ((1, i, j),) + tuple((-1, i, j2) for _, j2 in mates)))
    for i2, j2 in ys:
        mates = [x for x in xs if x[1] != j2]
        prods.append((((1, i2, 0), (1, i2, 1)), ((1, 0, j2),),
                      ((1, i2, j2),) + tuple((-1, i2, j) for _, j in mates)))
        prods.append((((1, i2, 1),), ((1, 0, j2), (-1, 1, j2)),
                      ((-1, i2, j2),) + tuple((-1, i, j2) for i, _ in mates)))
    for i, j in xs:
        for i2, j2 in ys:
            if j2 != j:
                lo, hi = min(j, j2), max(j, j2)
                prods.append((((1, i2, 0), (-1, i, 0)), ((1, 0, lo), (1, 0, hi)), ((1, i2, j),)))
                prods.append((((1, i, 0), (1, i2, 1)), ((1, 0, j2), (1, 1, j)), ((1, i, j2), (1, i2, j))))
                prods.append((((1, i, 1), (-1, i2, 1)), ((1, 1, lo), (1, 1, hi)), ((1, i, j2),)))
    return prods


def _o_jobs():
    alt = lambda r0, q: ([(r0 + 2 * a, a) for a in range(q)], [(r0 + 2 * a + 1, a) for a in range(q)])
    prods = _inner_group(*alt(0, 5)) + _inner_group(*alt(10, 3))
    for r in (10, 12, 14):
        prods += _inner_group([(r, 3)], [(r + 1, 4)])
    row = lambda t: max(i for _, i, _ in t[0])
    unit = lambda t: max(2 * i + h for _, i, h in t[0])
    need = lambda t: unit(t) if row(t) == 15 else 2 * row(t) + 1
    return [(need(t), t) for t in sorted(prods, key=need)]


_O_JOBS = _o_jobs()


def _job_order(nb):
    units = range(2 * nb)
    qa = [('a', u, c) for u in units for c in range(u // 2 + 1)]
    qb = [('b', u, c) for u in units for c in range(u // 2 + 1)]
    qo = [('o', u, j) for j, (u, _) in enumerate(_O_JOBS)]
    done = {}
    order = []

    def ready(q, lat, pre):
        return bool(q) and (pre, q[0][1]) in done and done[(pre, q[0][1])] + lat <= len(order)

    def emit(q):
        kind, u, j = job = q.pop(0)
        if kind != 'o' and j == u // 2:
            done[(kind, u)] = len(order)
        order.append(job)

    turn = 0
    while qa or qb or qo:
        pref = 'abo'[turn % 3]
        turn += 1
        for _ in range(GRP):
            b_ok, o_ok = ready(qb, LAT_A, 'a'), ready(qo, LAT_B, 'b')
            if pref == 'a' and qa and (len(qb) - len(qa) < ALEAD or not b_ok):
                emit(qa)
            elif pref == 'b' and b_ok:
                emit(qb)
            elif pref == 'o' and o_ok and (len(qo) > RES or not (qa or b_ok)):
                emit(qo)
            elif not (qa or b_ok or o_ok) and (qb or qo):
                emit(qb or qo)
            else:
                break
    return order


def _attention_step(q_scr, k_scr, v_scr, wo_ref, acc_scr, mid):
    causal = (jax.lax.broadcasted_iota(jnp.int32, (T, T), 0)
              <= jax.lax.broadcasted_iota(jnp.int32, (T, T), 1))
    sv, mx, mfin, lsum, pv, of, lhs = {}, {}, {}, {}, {}, {}, {}
    res = []
    wo, terms = {}, {}
    left = {}
    for _, t in _O_JOBS:
        for _, i, j in t[2]:
            left[i, j] = left.get((i, j), 0) + 1

    def job_a(u, c):
        r, hd = divmod(u, 2)
        s = _dot_nt(_ld(k_scr, 2 * c + hd), _ld(q_scr, u))
        res.append(s)
        if c == r:
            s = jnp.where(causal, s, -1e9 * LOG2E)
        s = s.reshape(T // 8, 8, T)
        sv[(u, c)] = s
        pm = jnp.max(s, axis=0)
        mx[u] = pm if u not in mx else jnp.maximum(mx[u], pm)

    def job_b(u, c):
        r, hd = divmod(u, 2)
        if u not in mfin:
            mfin[u] = jnp.broadcast_to(jnp.max(mx[u], axis=0, keepdims=True), (8, T))
        m = mfin[u]
        if len(res) >= LEAD:
            r0 = 8 * PROW * (c % 4)
            m = _after(m, res[len(res) - LEAD][r0:r0 + 8, :])
        p = jnp.exp2(sv.pop((u, c)) - m[None])
        ls = jnp.sum(p, axis=0)
        lsum[u] = ls if u not in lsum else lsum[u] + ls
        v = _dot(_ld(v_scr, 2 * c + hd), p.reshape(T, T).astype(BF16))
        res.append(v)
        pv[u] = v if u not in pv else v + pv[u]
        if c == r:
            of[u] = pv[u] * (1.0 / jnp.sum(lsum[u], axis=0, keepdims=True))

    def job_o(_, n):
        af, bf, outs = _O_JOBS[n][1]
        if af not in lhs:
            v = _form(af, lambda i, h: of[2 * i + h])
            lhs[af] = _tie(v.astype(BF16).T, v[0:8, :])
        if bf not in wo:
            wo[bf] = (wo_ref[_tile(bf[0][1]), _tile(bf[0][2])] if len(bf) == 1 else
                      _form(bf, lambda h, j: wo_ref[_tile(h), _tile(j)].astype(F32)).astype(BF16))
        v = _dot(lhs[af], wo[bf])
        res.append(v)
        for sign, i, j in outs:
            terms.setdefault((i, j), []).append((sign, v))
            if len(terms[i, j]) == left[i, j]:
                tot = acc_scr[_tile(i), _tile(j)]
                for sg, m in terms.pop((i, j)):
                    tot = tot + m if sg > 0 else tot - m
                acc_scr[_tile(i), _tile(j)] = tot

    fns = dict(a=job_a, b=job_b, o=job_o)
    for n, (kind, u, j) in enumerate(_job_order(q_scr.shape[0] // 2)):
        if n == MID:
            mid()
        fns[kind](u, j)


def _kernel(x_hbm, c_hbm, wq_hbm, wuk_hbm, wuv_hbm, wo_hbm, w1_hbm, w2_hbm, w3_hbm, w4_hbm,
            cond_hbm, wmod_hbm, out_hbm,
            x_ref, c_ref, cond_ref, wma_ref, wmb_ref, w1_ref, w2_ref, w3_ref, w4_ref,
            wq_buf, wk_buf, wv_buf, wo_buf, out_buf, sem, wsem, osem,
            mod_scr, h_scr, cs_scr, hs_scr, w_scr, q_scr, k_scr, v_scr, acc_scr, x1_scr, hb_scr, a1_scr, t_scr,
            a1s_scr, ws12, ws3, ws4):
    S, M = x_hbm.shape
    D = wq_hbm.shape[2]
    nattn = wo_hbm.shape[0]
    Fd = w4_hbm.shape[0]
    scale = float(D) ** -0.5 * LOG2E
    nb, nrb = S // T, S // RB
    km, kc = M // T, c_hbm.shape[1] // T
    NX = 4
    XR = S // NX
    CB = XR // T

    def pcopies(g):
        return [pltpu.make_async_copy(src.bitcast(U32).at[:, g, :], dst, wsem.at[j])
                for j, (src, dst) in enumerate(((wuk_hbm, wk_buf), (wuv_hbm, wv_buf), (wq_hbm, wq_buf)))]

    def ocopy(g):
        return pltpu.make_async_copy(wo_hbm.at[g], wo_buf, wsem.at[3])

    def chunk_copy(src, dst, i, s0):
        rows = slice(i * XR, (i + 1) * XR)
        return pltpu.make_async_copy(src.at[rows, :], dst.at[rows, :], sem.at[s0 + i])

    cp_cond = pltpu.make_async_copy(cond_hbm, cond_ref, sem.at[0])
    cp_wma = pltpu.make_async_copy(wmod_hbm.at[:, 0:2 * M], wma_ref, sem.at[1])
    cp_late = [pltpu.make_async_copy(src, dst, sem.at[2 + j]) for j, (src, dst) in enumerate((
        (wmod_hbm.at[:, 2 * M:6 * M], wmb_ref), (w1_hbm, w1_ref), (w2_hbm, w2_ref),
        (w3_hbm, w3_ref), (w4_hbm, w4_ref)))]
    cp_x = [chunk_copy(x_hbm, x_ref, i, 7) for i in range(NX)]
    cp_c = [chunk_copy(c_hbm, c_ref, i, 7 + NX) for i in range(NX)]

    def silu_cond():
        cf = cond_ref[...].astype(F32)
        return jnp.broadcast_to((cf * jax.nn.sigmoid(cf)).astype(BF16), (8, M))

    cp_wk, cp_wv, cp_wq = pcopies(0)
    named = dict(k=cp_wk, v=cp_wv, q=cp_wq, o=ocopy(0), n=cp_cond, m=cp_wma)
    named.update(zip('abcd', cp_c))
    named.update(zip('wxyz', cp_x))
    started, arrived, did = set(), set(), set()

    def zero(r, carry):
        acc_scr[pl.ds(pl.multiple_of(r * T, T), T), :] = jnp.zeros((T, M), F32)
        return carry

    def x_rows(rows, dep):
        xf = x_ref[rows, :].astype(F32)
        if dep is None:
            return xf
        return jnp.concatenate([_after(xf[:, :T], _rows(dep, xf.shape[0])), xf[:, T:]], axis=1)

    def n_item(r, i):
        def fn(dep):
            rows = slice(r * T + i * LP, r * T + (i + 1) * LP)
            x1_scr[rows, :] = _ln(x_rows(rows, dep))
        return fn

    def h_item(r, i, normed):
        def fn(dep):
            rows = slice(i * LP, (i + 1) * LP)
            grows = slice(r * T + i * LP, r * T + (i + 1) * LP)
            sa = mod_scr[:, 0:M]
            if normed and dep is not None:
                sa = jnp.concatenate([_after(sa[:, _tile(j)], dep) for j in range(km)], axis=1)
            hf = ((x1_scr[grows, :] if normed else _ln(x_rows(grows, dep))) * _rows(mod_scr[:, M:2 * M], LP)
                  + _rows(sa, LP))
            for j in range(km):
                h_scr[r, j, rows, :] = hf[:, _tile(j)].astype(BF16)
            for f, n in _H_SUMS.items():
                if all(t[1] == r for t in f):
                    hs_scr[n, rows, :] = _form(f, lambda _, k: hf[:, _tile(k)]).astype(BF16)
            did.add(('h', r, i))
        return fn

    def release(jobs, span, items):
        if span and items:
            jobs.side += [(len(jobs.res) + 1 + i * span // len(items), fn) for i, fn in enumerate(items)]
            jobs.side.sort(key=lambda e: e[0])
        else:
            for fn in items:
                fn(None)

    def sum_items(n, group, index, dst, get, skip_rows):
        forms = [f for f in dict.fromkeys(t[0] for t in group)
                 if len(f) > 1 and not (skip_rows and len({t[1] for t in f}) == 1)]

        def item(f, rows):
            def fn(dep):
                def term(r, k):
                    v = get(r, k, rows).astype(F32)
                    return v if dep is None or (r, k) != f[0][1:] else _after(v, _rows(dep, v.shape[0]))
                dst[index[f], rows, :] = _form(f, term).astype(BF16)
            return fn

        return [item(f, slice(i, i + n)) for i in range(0, T, n) for f in forms]

    h_sums = lambda n, gi: sum_items(n, _H_GROUPS[gi], _H_SUMS, hs_scr,
                                     lambda r_, k, rows: h_scr[r_, k, rows, :], True)

    def stash(key, buf, j0, transpose=False):
        n = buf.shape[0] // T
        if key not in did:
            assert key in arrived
            did.add(key)
            w = _PairWeights(buf, transpose)
            for j in range(n):
                for hd in range(2):
                    w_scr[hd, j0 + j] = _pk(w(((1, j, hd),))[1])
        return lambda hd: [_ld(w_scr, hd, j0 + j) for j in range(n)]

    def kv_tile(jobs, r):
        wk, wvT = stash('k', wk_buf, 0), stash('v', wv_buf, kc, True)
        ct = [c_ref[_tile(r), _tile(j)] for j in range(kc)]
        for hd in range(2):
            k_scr[2 * r + hd] = _pk(jobs.mm(ct, wk(hd), _dot).astype(BF16))
        for hd in range(2):
            v_scr[2 * r + hd] = _pk(jobs.mm(wvT(hd), ct, _dot_nt).astype(BF16))

    def q_tile(jobs, r):
        wq = stash('q', wq_buf, 2 * kc)
        ht = [h_scr[r, j] for j in range(km)]
        for hd in range(2):
            q_scr[2 * r + hd] = _pk((jobs.mm(ht, wq(hd), _dot) * scale).astype(BF16))

    for blk in PROLOGUE.split(';'):
        waits, starts, acts = blk.split('|')
        for ch in waits.strip():
            assert ch in started and ch not in arrived
            arrived.add(ch)
            named[ch].wait()
        for ch in starts.strip():
            assert ch not in started
            started.add(ch)
            named[ch].start()
        jobs = _Jobs()
        for act in acts.split():
            if act == 'Z':
                jax.lax.fori_loop(0, nb, zero, 0)
                acc_scr[S:, :] = jnp.zeros((acc_scr.shape[0] - S, M), F32)
                x_ref[S:, :] = jnp.zeros((x_ref.shape[0] - S, M), BF16)
            elif act == 'M':
                assert arrived >= set('nm')
                mod = _dot(silu_cond(), wma_ref[...])
                mod_scr[:, 0:M] = mod[:, 0:M]
                mod_scr[:, M:2 * M] = 1.0 + mod[:, M:2 * M]
                did.add('M')
            else:
                act, _, span = act.partition('@')
                span = int(span or 0)
                items = []
                for r in [int(ch, 16) for ch in act[1:]]:
                    did.add((act[0], r))
                    if act[0] == 'K':
                        assert 'abcd'[r // CB] in arrived
                        kv_tile(jobs, r)
                    elif act[0] == 'H':
                        assert 'wxyz'[r // CB] in arrived and 'M' in did
                        items += [h_item(r, i, ('N', r) in did) for i in range(T // LP)]
                    elif act[0] == 'N':
                        assert 'wxyz'[r // CB] in arrived
                        items += [n_item(r, i) for i in range(T // LP)]
                    elif act[0] == 'Q':
                        assert all(('h', r, i) in did for i in range(T // LP))
                        q_tile(jobs, r)
                    elif act[0] == 'C':
                        assert all('abcd'[t[1] // CB] in arrived for p_ in _C_GROUPS[r] for t in p_[0])
                        items += sum_items(
                            32, _C_GROUPS[r], _C_SUMS, cs_scr,
                            lambda r_, k, rows: c_ref[r_ * T + rows.start:r_ * T + rows.stop, _tile(k)], False)
                    else:
                        assert act[0] == 'S' and all(('h', t[1], T // LP - 1) in did for p_ in _H_GROUPS[r] for t in p_[0])
                        items += h_sums(32 if span else 16, r)
                release(jobs, span, items)
        assert not jobs.side
    assert arrived == set(named) and all((k_, r) in did for k_ in 'KHQ' for r in range(nb))
    assert all((k_, r) in did for k_ in 'CS' for r in range(2))
    for cp in cp_late[1:] + cp_late[:1]:
        cp.start()

    FH = ws3.shape[0] * T
    assert nattn - 1 >= FH // 64

    def mixer_prep(g):
        def blocks(w_ref, r0, n, half, c0, c1, dep):
            lo, hi = pl.ds(r0, n), pl.ds(r0 + half, n)
            return [_after(w_ref[rows, _tile(c)].astype(F32), _rows(dep, n)) if (rows is lo) == (c == c0)
                    else w_ref[rows, _tile(c)].astype(F32) for rows in (lo, hi) for c in (c0, c1)]

        def rows_items(w_ref, dst, per_step, half, n=16):
            gi = jnp.minimum(g, half // per_step - 1)
            src = w_ref.at[pl.ds(pl.multiple_of(gi * per_step, per_step), half + per_step), :]
            hs = per_step // 2

            def item(c, o):
                def fn(dep):
                    for i, v in enumerate(_b_ops(*blocks(src, o, n, half, c, c + 2, dep))):
                        dst[i, c, pl.ds(pl.multiple_of(gi * hs, hs) + o // 2, n // 2), :] = _pk(v.astype(BF16))
                return fn
            return [item(c, o) for c in range(2) for o in range(0, per_step, n)]

        def w3_item(k, i):
            def fn(dep):
                n = jnp.minimum(g, FH // T - 1)
                b11, b21, b12, b22 = blocks(w3_ref, pl.multiple_of(n * T, T), T, FH, k, k + 2, dep)
                ws3[n, i, k] = _pk(_b_ops(b11, b12, b21, b22)[i].astype(BF16).T)
            return fn

        return (rows_items(w1_ref, ws12.at[0], 32, 2 * T) + rows_items(w2_ref, ws12.at[1], 32, 2 * T)
                + rows_items(w4_ref, ws4, 64, FH) + [w3_item(k, i) for k in range(2) for i in range(7)])

    def attn_body(g, carry):
        copies = pcopies(jnp.minimum(g + 1, nattn - 1))

        def mid():
            for cp in copies:
                cp.start()

        _attention_step(q_scr, k_scr, v_scr, wo_buf, acc_scr, mid)
        for cp in copies:
            cp.wait()

        @pl.when(g == 0)
        def _():
            for cp in cp_late[1:]:
                cp.wait()

        @pl.when(g + 1 < nattn)
        def _():
            ocopy(g + 1).start()
            side = [(SD0 + i * SDS, fn) for i, fn in enumerate(mixer_prep(g))]
            _proj_step(h_scr, hs_scr, c_ref, cs_scr, wq_buf, wk_buf, wv_buf, q_scr, k_scr, v_scr, scale, side)
            ocopy(g + 1).wait()

        return carry

    jax.lax.fori_loop(0, nattn, attn_body, 0)

    cp_late[0].wait()
    mod = _dot(silu_cond(), wmb_ref[...])
    mod_scr[:, 2 * M:4 * M] = mod[:, 0:2 * M]
    mod_scr[:, 4 * M:5 * M] = 1.0 + mod[:, 2 * M:3 * M]
    mod_scr[:, 5 * M:6 * M] = mod[:, 3 * M:4 * M]
    ftiles = [(f, min(f + T, Fd)) for f in range(0, Fd, T)]
    OFF = x_ref.shape[0] - S
    CAR = t_scr.shape[0] - RB

    def p1(r0, n, dep=None):
        ga = mod_scr[:, 2 * M:3 * M]
        if dep is not None:
            ga = jnp.concatenate([_after(ga[:, 0:T], dep), ga[:, T:]], axis=1)
        rows = pl.ds(r0, n)
        x1 = x_ref[rows, :].astype(F32) + _rows(ga, n) * acc_scr[rows, :]
        x1_scr[rows, :] = x1
        hb = _ln(x1) * _rows(mod_scr[:, 4 * M:5 * M], n) + _rows(mod_scr[:, 3 * M:4 * M], n)
        hb_scr[rows, :] = hb
        return _ln(hb)

    HT = T // 2

    def p1_store(r0, c, dep=None):
        n = PC // 2
        hf, o = divmod(c * n, HT)
        top, bot = [p1(r0 + hf * T + d + o, n, dep) for d in (0, HT)]
        for d, v in ((0, top), (HT, bot)):
            for j in range(km):
                a1_scr[j, hf * T + d + o:hf * T + d + o + n, :] = v[:, _tile(j)].astype(BF16)
        ops = _a_ops(top[:, 0:2 * T], top[:, 2 * T:4 * T], bot[:, 0:2 * T], bot[:, 2 * T:4 * T])
        for i, m in enumerate(SUMS):
            for k in range(2):
                a1s_scr[hf, i, k, o:o + n, :] = ops[m][:, _tile(k)].astype(BF16)
        return jnp.max(ops[0][:, :T].reshape(n // 8, 8, T), axis=0)

    t_scr[RB:RB + CAR - OFF, :] = jnp.zeros((CAR - OFF, M), F32)
    t_scr[RB + CAR - OFF:RB + CAR, :] = _gelu(_dot(p1(0, OFF).astype(BF16), w1_ref[...]))
    for c in range(RB // PC):
        p1_store(OFF, c)

    def out_copy(i):
        rows = pl.ds(i * T if isinstance(i, int) else pl.multiple_of(i * T, T), T)
        return pltpu.make_async_copy(out_buf.at[rows, :], out_hbm.at[rows, :], osem.at[i])

    def b_body(r, carry):
        gb = _rows(mod_scr[:, 5 * M:6 * M], T)
        r0 = pl.multiple_of(r * RB, RB)
        n0 = pl.multiple_of(jnp.minimum(r0 + RB, S - RB) + OFF, OFF)
        nh = RB // T
        now = [0]
        due = []
        pace = []

        def p1_item(c):
            return lambda dep: due.append((now[0] + PD, p1_store(n0, c, dep)))

        pace += [(P0 + i * PSTEP, p1_item(i)) for i in range(RB // PC)]
        wt = lambda ref, f0, f1, n: ref[f0:f1, _tile(n)]

        def mm(lhs, wts, dot=_dot):
            acc = None
            for x, w in zip(lhs, wts):
                if due and due[0][0] <= now[0]:
                    w = _tie(w, due.pop(0)[1])
                v = dot(x, w)
                now[0] += x.shape[0] // HT
                acc = v if acc is None else v + acc
                if pace and pace[0][0] <= now[0]:
                    pace.pop(0)[1](v[0:8, :])
            return acc

        def split_ops(lo, hi):
            return [v.astype(BF16) for v in _a_ops(lo[:HT], hi[:HT], lo[HT:], hi[HT:])]

        def two_tiles(aops, wsel, rest):
            def col(w):
                v = mm(rest[0], w, rest[3])
                return v[:HT], v[HT:]

            c11, c12, c21, c22 = _strassen(
                lambda i: mm([a[i] for a in aops], [wsel(i, k) for k in range(len(aops))]),
                lambda: col(rest[1]), lambda: col(rest[2]))
            return jnp.concatenate([c11, c21], axis=0), jnp.concatenate([c12, c22], axis=0)

        def square(full, aops, w_ref, ws_ref):
            out = {}
            for n in range(2):
                out[n], out[n + 2] = two_tiles(
                    aops, lambda i, k: _ld(ws_ref, i, n, slice(k * HT, (k + 1) * HT)),
                    (full[4:], [wt(w_ref, 4 * T, M, n)], [wt(w_ref, 4 * T, M, n + 2)], _dot))
            out[4] = mm(full, [wt(w_ref, j * T, (j + 1) * T, 4) for j in range(km)])
            return out

        t_scr[0:CAR, :] = t_scr[RB:RB + CAR, :]
        for hf in range(nh):
            full = [a1_scr[j, _tile(hf), :] for j in range(km)]
            aops = []
            for k in range(2):
                ops = {m: a1s_scr[hf, i, k] for i, m in enumerate(SUMS)}
                ops[2], ops[3] = full[k][:HT], full[2 + k][HT:]
                aops.append(ops)
            for n, v in square(full, aops, w1_ref, ws12.at[0]).items():
                t = _gelu(v)
                if hf == nh - 1:
                    t = jnp.concatenate([t[:T - OFF], jnp.where(r < nrb - 1, t[T - OFF:], 0.0)], axis=0)
                t_scr[CAR + hf * T:CAR + (hf + 1) * T, _tile(n)] = t
        cq = M // 4
        shifts = (-1, 1, -2, 2)
        lane = jax.lax.broadcasted_iota(jnp.int32, (T, T), 1)
        y1, a3 = [], []
        for hf in range(nh):
            base = CAR - OFF + hf * T
            sh = []
            for j in range(km):
                g_lo, g_hi = (j * T) // cq, ((j + 1) * T - 1) // cq
                assert g_hi - g_lo <= 1
                v = t_scr[base + shifts[g_lo]:base + shifts[g_lo] + T, _tile(j)]
                if g_hi != g_lo:
                    v2 = t_scr[base + shifts[g_hi]:base + shifts[g_hi] + T, _tile(j)]
                    v = jnp.where(lane < g_hi * cq - j * T, v, v2)
                sh.append(v)
            hs = square([v.astype(BF16) for v in sh], [split_ops(sh[k], sh[2 + k]) for k in range(2)],
                        w2_ref, ws12.at[1])
            hs = jnp.concatenate([hs[n] for n in range(km)], axis=1)
            y1.append(hs + hb_scr[pl.ds(pl.multiple_of(r0 + hf * T, T), T), :])
            a3.append({})

            def ln_item(hf, c):
                def item(dep):
                    n = HT // NLN
                    for d in (0, HT):
                        v = y1[hf][d + c * n:d + (c + 1) * n]
                        if dep is not None:
                            v = jnp.concatenate([_after(v[:, :T], _rows(dep, n)), v[:, T:]], axis=1)
                        a3[hf][d + c * n] = _ln(v)
                return item

            ln_item(hf, 0)(None)
            pace += [(now[0] + LN0 + (c - 1) * LNS * (1 + hf), ln_item(hf, c)) for c in range(1, NLN)]
            pace.sort(key=lambda e: e[0])
        nf = FH // T
        h3, h3ops = [], []
        for hf in range(nh):
            assert len(a3[hf]) == 2 * NLN
            af = jnp.concatenate([a3[hf][key] for key in sorted(a3[hf])], axis=0)
            full = [af[:, _tile(j)].astype(BF16) for j in range(km)]
            aops = [split_ops(af[:, _tile(k)], af[:, _tile(2 + k)]) for k in range(2)]
            row, ops = {}, []
            narrow = None
            for n in range(nf):
                lo, hi = two_tiles(aops, lambda i, k: _ld(ws3, n, i, k),
                                   (full[4:], [wt(w3_ref, *ftiles[n], 4)],
                                    [wt(w3_ref, *ftiles[nf + n], 4)], _dot_nt))
                lo, hi = _gelu(lo), _gelu(hi)
                row[n], row[nf + n] = lo.astype(BF16), hi.astype(BF16)
                ops.append(split_ops(lo, hi))
                if n < km:
                    v = mm([wt(w3_ref, *ftiles[-1], n)], [full[n]], _dot_nt)
                    narrow = v if narrow is None else v + narrow
            row[2 * nf] = _gelu(mm(full, [wt(w3_ref, *ftiles[2 * nf], j) for j in range(km)],
                                   _dot_nt)).astype(BF16)
            fw = Fd - ftiles[-1][0]
            gT = jnp.concatenate([_gelu(narrow), jnp.zeros((T - fw, T), F32)], axis=0)
            row[2 * nf + 1] = _tie(gT.astype(BF16).T, gT[0:8, :])[:, :fw]
            h3.append([row[i] for i in range(len(ftiles))])
            h3ops.append(ops)
        for hf in range(nh):
            rows = pl.ds(pl.multiple_of(r0 + hf * T, T), T)

            def finish(n, v):
                out_buf[rows, _tile(n)] = (
                    x1_scr[rows, _tile(n)] + gb[:, _tile(n)] * (v + y1[hf][:, _tile(n)])
                ).astype(out_buf.dtype)

            w4t = lambda n, f_: [wt(w4_ref, f0, f1, n) for f0, f1 in f_]
            finish(4, mm(h3[hf], w4t(4, ftiles)))
            for n in range(2):
                lo, hi = two_tiles(h3ops[hf], lambda i, k: _ld(ws4, i, n, slice(k * HT, (k + 1) * HT)),
                                   (h3[hf][2 * nf:], w4t(n, ftiles[2 * nf:]), w4t(n + 2, ftiles[2 * nf:]), _dot))
                finish(n, lo)
                finish(n + 2, hi)
            out_copy(r * nh + hf).start()
        assert not pace
        return carry

    jax.lax.fori_loop(0, nrb, b_body, 0)
    for i in range(nb):
        out_copy(i).wait()


@jax.jit
def pallas_adaLN_cond__compressed_kv_cla__mixer_s_mlp__prompt_kernel(
    A_x: jax.Array,
    A_c_kv: jax.Array,
    A_w_q: jax.Array,
    A_w_uk: jax.Array,
    A_w_uv: jax.Array,
    A_w_o: jax.Array,
    B_x: jax.Array,
    B_w1: jax.Array,
    B_w2: jax.Array,
    B_w3: jax.Array,
    B_w4: jax.Array,
    c: jax.Array,
    w_mod: jax.Array,
):
    _, S, M = A_x.shape
    Dc = A_c_kv.shape[2]
    H, D = A_w_q.shape[1], A_w_q.shape[2]
    Fd = B_w3.shape[1]
    assert D == T and A_c_kv.shape[1] == S and Dc == 4 * T and M == 5 * T and 13 * T < Fd < 14 * T and S == 16 * T
    vmem = pltpu.VMEM
    packed = lambda *lead: vmem(lead + (T // 2, T), U32)
    out = pl.pallas_call(
        _kernel,
        in_specs=[pl.BlockSpec(memory_space=pltpu.HBM)] * 12,
        out_specs=pl.BlockSpec(memory_space=pltpu.HBM),
        out_shape=jax.ShapeDtypeStruct((S, M), A_x.dtype),
        scratch_shapes=[
            vmem((S + 16, M), BF16),
            vmem((S, Dc), BF16),
            vmem((1, M), BF16),
            vmem((M, 2 * M), BF16),
            vmem((M, 4 * M), BF16),
            vmem((M, M), BF16),
            vmem((M, M), BF16),
            vmem((Fd, M), BF16),
            vmem((Fd, M), BF16),
            vmem((M, D), U32),
            vmem((Dc, D), U32),
            vmem((Dc, D), U32),
            vmem((2 * D, M), BF16),
            vmem((S, M), A_x.dtype),
            pltpu.SemaphoreType.DMA((15,)),
            pltpu.SemaphoreType.DMA((4,)),
            pltpu.SemaphoreType.DMA((S // T,)),
            vmem((8, 6 * M), F32),
            vmem((S // T, M // T, T, T), BF16),
            vmem((len(_C_SUMS), T, T), BF16),
            vmem((len(_H_SUMS), T, T), BF16),
            packed(2, M // T + 2 * (Dc // T)),
            packed(2 * S // T),
            packed(2 * S // T),
            packed(2 * S // T),
            vmem((S + 16, M), F32),
            vmem((S + 16, M), F32),
            vmem((S + 16, M), F32),
            vmem((M // T, RB, T), BF16),
            vmem((RB + 32, M), F32),
            vmem((RB // T, 5, 2, T // 2, T), BF16),
            vmem((2, 7, 2, T, T), U32),
            packed(6, 7, 2),
            vmem((7, 2, 3 * T, T), U32),
        ],
        compiler_params=pltpu.CompilerParams(
            vmem_limit_bytes=100 * 1024 * 1024,
            disable_bounds_checks=True,
        ),
    )(
        A_x.reshape(S, M), A_c_kv.reshape(S, Dc),
        A_w_q, A_w_uk, A_w_uv,
        A_w_o.reshape(H // 2, 2 * D, M),
        B_w1, B_w2, B_w3.T, B_w4, c, w_mod,
    )
    return out.reshape(1, S, M)
```

```python
import math

import jax
import jax.numpy as jnp
import jax.experimental.pallas as pl
import jax.experimental.pallas.tpu as pltpu

F32 = jnp.float32
BF16 = jnp.bfloat16
U32 = jnp.uint32
NT = (((1,), (1,)), ((), ()))
T = 128
EPS = 1e-5
LOG2E = math.log2(math.e)

GRP = 4
LEAD = 10
PROW = 3
RES = 32
LAT_A = 16
LAT_B = 20
ALEAD = 32
MID = 40
SD0, SDS = 60, 4
RB = 256
PC = 32
P0, PSTEP, PD = 440, 30, 52
NLN, LN0, LNS = 4, 4, 5
LP = 16
PROLOGUE = ('|kva|Z; |b|; kva|wc|K0123; bw|xdn|C0@56 N0123@52 K4567; cx|mq|N4567@52 K89ab; '
            'd|y|C1@56 Kcdef; nmq|zo|M H01 H234567@30 Q0123; y||H89ab@30 Q4567; '
            'z||Hcdef@30 Q89ab S01 Qcdef; o||')


def _dot(a, b):
    return jnp.dot(a, b, preferred_element_type=F32)


def _dot_nt(a, b):
    return jax.lax.dot_general(a, b, NT, preferred_element_type=F32)


def _ln(x):
    m = jnp.mean(x, axis=-1, keepdims=True)
    xc = x - m
    v = jnp.mean(xc * xc, axis=-1, keepdims=True)
    return xc * jnp.exp2(jnp.log(v + EPS) * (-0.5 * LOG2E))


def _rows(v, n):
    return jnp.broadcast_to(v[None], (n // 8, 8, v.shape[1])).reshape(n, v.shape[1])


def _gelu(x):
    c0 = math.sqrt(2.0 / math.pi)
    return 0.5 * x * (1.0 + jnp.tanh(c0 * (x + 0.044715 * (x * x * x))))


def _after(x, dep):
    return jnp.where(dep > jnp.inf, dep, x)


def _tie(x, dep):
    xu = pltpu.bitcast(x, U32)
    first = jnp.where(dep > jnp.inf, jnp.uint32(0), xu[:8])
    return pltpu.bitcast(jnp.concatenate([first, xu[8:]], axis=0), BF16)


def _tile(j):
    return slice(j * T, (j + 1) * T)


def _ld(ref, *idx):
    return pltpu.bitcast(ref[idx], BF16)


def _pk(x):
    return pltpu.bitcast(x, U32)


def _a_ops(a11, a12, a21, a22):
    return [a11 + a22, a21 + a22, a11, a22, a11 + a12, a21 - a11, a12 - a22]


SUMS = (0, 1, 4, 5, 6)


def _b_ops(b11, b12, b21, b22):
    return [b11 + b22, b11, b12 - b22, b21 - b11, b22, b11 + b12, b21 + b22]


def _strassen(prod, col1=None, col2=None):
    m4 = prod(3)
    m2 = prod(1)
    c21 = m2 + m4
    if col1 is not None:
        e11, e21 = col1()
        m4, c21 = m4 + e11, c21 + e21
    m3 = prod(2)
    m5 = prod(4)
    c12 = m3 + m5
    if col2 is not None:
        e12, e22 = col2()
        c12, m3 = c12 + e12, m3 + e22
    m1 = prod(0)
    c11 = prod(6) + (m1 + (m4 - m5))
    c22 = prod(5) + (m1 + (m3 - m2))
    return c11, c12, c21, c22


def _group(rows, cols, pairs):
    xs, ys = dict.fromkeys(x for x, _ in pairs), dict.fromkeys(y for _, y in pairs)
    used = set(xs) | set(ys) | {(x[0], y[1]) for x, y in pairs} | {(y[0], x[1]) for x, y in pairs}
    prods = []
    for n, r in enumerate(rows):
        for i, k in [x for x in xs if x[0] == r]:
            mates = [y for x, y in pairs if x == (i, k)]
            prods.append((((1, i, k),) + tuple((1, i, k2) for _, k2 in mates), ((1, k, 0),),
                          ((1, i, 0), (-1, i, 1))))
            prods.append((((1, i, k),) + tuple((-1, i2, k) for i2, _ in mates), ((1, k, 0), (1, k, 1)),
                          ((1, i, 1),)))
        for i2, k2 in [y for y in ys if y[0] == r]:
            mates = [x for x, y in pairs if y == (i2, k2)]
            prods.append((((1, i2, k2),) + tuple((1, i2, k) for _, k in mates), ((1, k2, 1),),
                          ((1, i2, 1), (-1, i2, 0))))
            prods.append((((1, i2, k2),) + tuple((-1, i, k2) for i, _ in mates), ((1, k2, 0), (1, k2, 1)),
                          ((1, i2, 0),)))
        prods += [(((1, r, k),), ((1, k, h),), ((1, r, h),)) for k in cols if (r, k) not in used for h in (0, 1)]
        for (i, k), (i2, k2) in pairs:
            if r in (i, i2) and i + i2 - r in rows[n + 1:]:
                prods.append((((1, i, k2),), ((1, k2, 0), (-1, k, 0)), ((1, i2, 0), (1, i, 0))))
                prods.append((((1, i2, k), (1, i, k2)), ((1, k, 0), (1, k2, 1)), ((1, i2, 0), (1, i, 1))))
                prods.append((((1, i2, k),), ((1, k, 1), (-1, k2, 1)), ((1, i2, 1), (1, i, 1))))
    return prods


def _all_pairs(xrows, yrows):
    return [((x, a), (y, b)) for a, x in enumerate(xrows) for b, y in enumerate(yrows) if a != b]


_PAIRS65 = [((x[0] + 10, x[1]), (y[0] + 10, y[1])) for x, y in (
    ((0, 1), (1, 0)), ((0, 1), (5, 2)), ((2, 3), (1, 0)), ((2, 3), (3, 1)), ((2, 3), (5, 2)), ((3, 2), (1, 0)),
    ((4, 4), (0, 3)), ((4, 4), (1, 0)), ((4, 4), (3, 1)), ((4, 4), (5, 2)))]
_C_GROUPS = [_group(range(r, r + 8), range(4), _all_pairs(range(r, r + 4), range(r + 4, r + 8))) for r in (0, 8)]
_H_GROUPS = [_group(range(10), range(5), _all_pairs(range(5), range(5, 10))),
             _group(range(10, 16), range(5), _PAIRS65)]
_sum_index = lambda groups: {f: n for n, f in enumerate(
    dict.fromkeys(t[0] for g in groups for t in g if len(t[0]) > 1))}
_C_SUMS, _H_SUMS = _sum_index(_C_GROUPS), _sum_index(_H_GROUPS)


def _form(form, get):
    acc = None
    for sign, i, j in form:
        v = get(i, j)
        acc = v if acc is None else (acc + v if sign > 0 else acc - v)
    return acc


class _PairWeights:
    def __init__(self, w_ref, transpose=False):
        self.base = {}
        for j in range(w_ref.shape[0] // T):
            wu = w_ref[_tile(j), :]
            if transpose:
                wu = wu.T
            self.base[j, 0] = pltpu.bitcast(wu << 16, F32)
            self.base[j, 1] = pltpu.bitcast(wu & jnp.uint32(0xFFFF0000), F32)
        self.cache = {}

    def __call__(self, form):
        sign = 1
        if form[-1][0] < 0 and form[0][1:] > form[1][1:]:
            sign, form = -1, ((1,) + form[1][1:], (-1,) + form[0][1:])
        if form not in self.cache:
            self.cache[form] = _form(form, lambda k, h: self.base[k, h]).astype(BF16)
        return sign, self.cache[form]


def _run_group(jobs, prods, a_get, w, transposed, finish):
    left = {}
    for _, _, outs in prods:
        for _, i, h in outs:
            left[i, h] = left.get((i, h), 0) + 1
    acc = {}
    for af, bf, outs in prods:
        sign, wt = w(bf)
        m = jobs.mm([wt], [a_get(af)], _dot_nt) if transposed else jobs.mm([a_get(af)], [wt], _dot)
        for s_, i, h in outs:
            if (i, h) not in acc:
                acc[i, h] = (s_ * sign, m)
            else:
                s0, v = acc[i, h]
                acc[i, h] = (s0, v + m if s0 == s_ * sign else v - m) if s0 > 0 or s_ * sign < 0 else (1, m - v)
            left[i, h] -= 1
            if not left[i, h]:
                s0, v = acc.pop((i, h))
                assert s0 > 0
                finish(2 * i + h, v)


class _Jobs:
    def __init__(self, side=()):
        self.res = []
        self.side = list(side)

    def mm(self, lhs, wt, dot):
        acc = None
        for x, w in zip(lhs, wt):
            v = dot(x, w)
            self.res.append(v)
            acc = v if acc is None else v + acc
            rel = 4 * (len(self.res) % 4)
            while self.side and self.side[0][0] <= len(self.res):
                self.side.pop(0)[1](v[8 * rel:8 * rel + 8, :])
                rel = (rel + 2) % 16
        return acc


def _proj_step(h_scr, hs_scr, c_ref, cs_scr, wq_ref, wuk_ref, wuv_ref, q_scr, k_scr, v_scr, scale, side):
    wq, wk, wvT = _PairWeights(wq_ref), _PairWeights(wuk_ref), _PairWeights(wuv_ref, True)
    c_get = lambda f: cs_scr[_C_SUMS[f]] if len(f) > 1 else c_ref[_tile(f[0][1]), _tile(f[0][2])]
    h_get = lambda f: hs_scr[_H_SUMS[f]] if len(f) > 1 else h_scr[f[0][1], f[0][2]]

    def put(dst, mul=None):
        def fn(u, v):
            dst[u] = _pk((v if mul is None else v * mul).astype(BF16))
        return fn

    jobs = _Jobs(side)
    for groups, get, w, transposed, fin in ((_C_GROUPS, c_get, wk, False, put(k_scr)),
                                            (_C_GROUPS, c_get, wvT, True, put(v_scr)),
                                            (_H_GROUPS, h_get, wq, False, put(q_scr, scale))):
        for prods in groups:
            _run_group(jobs, prods, get, w, transposed, fin)
    assert not jobs.side


def _inner_group(rows, cols, pairs):
    xs, ys = dict.fromkeys(x for x, _ in pairs), dict.fromkeys(y for _, y in pairs)
    used = set(xs) | set(ys) | {(x[0], y[1]) for x, y in pairs} | {(y[0], x[1]) for x, y in pairs}
    prods = []
    for i, j in xs:
        mates = [y for x, y in pairs if x == (i, j)]
        prods.append((((1, i, 0),), ((1, 0, j), (-1, 1, j)), ((1, i, j),) + tuple((1, i2, j) for i2, _ in mates)))
        prods.append((((1, i, 0), (1, i, 1)), ((1, 1, j),), ((1, i, j),) + tuple((-1, i, j2) for _, j2 in mates)))
    for i2, j2 in ys:
        mates = [x for x, y in pairs if y == (i2, j2)]
        prods.append((((1, i2, 0), (1, i2, 1)), ((1, 0, j2),),
                      ((1, i2, j2),) + tuple((-1, i2, j) for _, j in mates)))
        prods.append((((1, i2, 1),), ((1, 0, j2), (-1, 1, j2)),
                      ((-1, i2, j2),) + tuple((-1, i, j2) for i, _ in mates)))
    prods += [(((1, i, h),), ((1, h, j),), ((1, i, j),))
              for i in rows for j in cols if (i, j) not in used for h in (0, 1)]
    for (i, j), (i2, j2) in pairs:
        lo, hi = min(j, j2), max(j, j2)
        prods.append((((1, i2, 0), (-1, i, 0)), ((1, 0, lo), (1, 0, hi)), ((1, i2, j),)))
        prods.append((((1, i, 0), (1, i2, 1)), ((1, 0, j2), (1, 1, j)), ((1, i, j2), (1, i2, j))))
        prods.append((((1, i, 1), (-1, i2, 1)), ((1, 1, lo), (1, 1, hi)), ((1, i, j2),)))
    return prods


def _o_jobs():
    prods = (_inner_group(range(10), range(5), _all_pairs(range(0, 10, 2), range(1, 10, 2)))
             + _inner_group(range(10, 16), range(5), _PAIRS65))
    row = lambda t: max(i for _, i, _ in t[0])
    unit = lambda t: max(2 * i + h for _, i, h in t[0])
    need = lambda t: unit(t) if row(t) == 15 else 2 * row(t) + 1
    return [(need(t), t) for t in sorted(prods, key=need)]


_O_JOBS = _o_jobs()


def _job_order(nb):
    units = range(2 * nb)
    qa = [('a', u, c) for u in units for c in range(u // 2 + 1)]
    qb = [('b', u, c) for u in units for c in range(u // 2 + 1)]
    qo = [('o', u, j) for j, (u, _) in enumerate(_O_JOBS)]
    done = {}
    order = []

    def ready(q, lat, pre):
        return bool(q) and (pre, q[0][1]) in done and done[(pre, q[0][1])] + lat <= len(order)

    def emit(q):
        kind, u, j = job = q.pop(0)
        if kind != 'o' and j == u // 2:
            done[(kind, u)] = len(order)
        order.append(job)

    turn = 0
    while qa or qb or qo:
        pref = 'abo'[turn % 3]
        turn += 1
        for _ in range(GRP):
            b_ok, o_ok = ready(qb, LAT_A, 'a'), ready(qo, LAT_B, 'b')
            if pref == 'a' and qa and (len(qb) - len(qa) < ALEAD or not b_ok):
                emit(qa)
            elif pref == 'b' and b_ok:
                emit(qb)
            elif pref == 'o' and o_ok and (len(qo) > RES or not (qa or b_ok)):
                emit(qo)
            elif not (qa or b_ok or o_ok) and (qb or qo):
                emit(qb or qo)
            else:
                break
    return order


def _attention_step(q_scr, k_scr, v_scr, wo_ref, acc_scr, mid):
    causal = (jax.lax.broadcasted_iota(jnp.int32, (T, T), 0)
              <= jax.lax.broadcasted_iota(jnp.int32, (T, T), 1))
    sv, mx, mfin, lsum, pv, of, lhs = {}, {}, {}, {}, {}, {}, {}
    res = []
    wo, terms = {}, {}
    left = {}
    for _, t in _O_JOBS:
        for _, i, j in t[2]:
            left[i, j] = left.get((i, j), 0) + 1

    def job_a(u, c):
        r, hd = divmod(u, 2)
        s = _dot_nt(_ld(k_scr, 2 * c + hd), _ld(q_scr, u))
        res.append(s)
        if c == r:
            s = jnp.where(causal, s, -1e9 * LOG2E)
        s = s.reshape(T // 8, 8, T)
        sv[(u, c)] = s
        pm = jnp.max(s, axis=0)
        mx[u] = pm if u not in mx else jnp.maximum(mx[u], pm)

    def job_b(u, c):
        r, hd = divmod(u, 2)
        if u not in mfin:
            mfin[u] = jnp.broadcast_to(jnp.max(mx[u], axis=0, keepdims=True), (8, T))
        m = mfin[u]
        if len(res) >= LEAD:
            r0 = 8 * PROW * (c % 4)
            m = _after(m, res[len(res) - LEAD][r0:r0 + 8, :])
        p = jnp.exp2(sv.pop((u, c)) - m[None])
        ls = jnp.sum(p, axis=0)
        lsum[u] = ls if u not in lsum else lsum[u] + ls
        v = _dot(_ld(v_scr, 2 * c + hd), p.reshape(T, T).astype(BF16))
        res.append(v)
        pv[u] = v if u not in pv else v + pv[u]
        if c == r:
            of[u] = pv[u] * (1.0 / jnp.sum(lsum[u], axis=0, keepdims=True))

    def job_o(_, n):
        af, bf, outs = _O_JOBS[n][1]
        if af not in lhs:
            v = _form(af, lambda i, h: of[2 * i + h])
            lhs[af] = _tie(v.astype(BF16).T, v[0:8, :])
        if bf not in wo:
            wo[bf] = (wo_ref[_tile(bf[0][1]), _tile(bf[0][2])] if len(bf) == 1 else
                      _form(bf, lambda h, j: wo_ref[_tile(h), _tile(j)].astype(F32)).astype(BF16))
        v = _dot(lhs[af], wo[bf])
        res.append(v)
        for sign, i, j in outs:
            terms.setdefault((i, j), []).append((sign, v))
            if len(terms[i, j]) == left[i, j]:
                tot = acc_scr[_tile(i), _tile(j)]
                for sg, m in terms.pop((i, j)):
                    tot = tot + m if sg > 0 else tot - m
                acc_scr[_tile(i), _tile(j)] = tot

    fns = dict(a=job_a, b=job_b, o=job_o)
    for n, (kind, u, j) in enumerate(_job_order(q_scr.shape[0] // 2)):
        if n == MID:
            mid()
        fns[kind](u, j)


def _kernel(x_hbm, c_hbm, wq_hbm, wuk_hbm, wuv_hbm, wo_hbm, w1_hbm, w2_hbm, w3_hbm, w4_hbm,
            cond_hbm, wmod_hbm, out_hbm,
            x_ref, c_ref, cond_ref, wma_ref, wmb_ref, w1_ref, w2_ref, w3_ref, w4_ref,
            wq_buf, wk_buf, wv_buf, wo_buf, out_buf, sem, wsem, osem,
            mod_scr, h_scr, cs_scr, hs_scr, w_scr, q_scr, k_scr, v_scr, acc_scr, x1_scr, hb_scr, a1_scr, t_scr,
            a1s_scr, ws12, ws3, ws4):
    S, M = x_hbm.shape
    D = wq_hbm.shape[2]
    nattn = wo_hbm.shape[0]
    Fd = w4_hbm.shape[0]
    scale = float(D) ** -0.5 * LOG2E
    nb, nrb = S // T, S // RB
    km, kc = M // T, c_hbm.shape[1] // T
    NX = 4
    XR = S // NX
    CB = XR // T

    def pcopies(g):
        return [pltpu.make_async_copy(src.bitcast(U32).at[:, g, :], dst, wsem.at[j])
                for j, (src, dst) in enumerate(((wuk_hbm, wk_buf), (wuv_hbm, wv_buf), (wq_hbm, wq_buf)))]

    def ocopy(g):
        return pltpu.make_async_copy(wo_hbm.at[g], wo_buf, wsem.at[3])

    def chunk_copy(src, dst, i, s0):
        rows = slice(i * XR, (i + 1) * XR)
        return pltpu.make_async_copy(src.at[rows, :], dst.at[rows, :], sem.at[s0 + i])

    cp_cond = pltpu.make_async_copy(cond_hbm, cond_ref, sem.at[0])
    cp_wma = pltpu.make_async_copy(wmod_hbm.at[:, 0:2 * M], wma_ref, sem.at[1])
    cp_late = [pltpu.make_async_copy(src, dst, sem.at[2 + j]) for j, (src, dst) in enumerate((
        (wmod_hbm.at[:, 2 * M:6 * M], wmb_ref), (w1_hbm, w1_ref), (w2_hbm, w2_ref),
        (w3_hbm, w3_ref), (w4_hbm, w4_ref)))]
    cp_x = [chunk_copy(x_hbm, x_ref, i, 7) for i in range(NX)]
    cp_c = [chunk_copy(c_hbm, c_ref, i, 7 + NX) for i in range(NX)]

    def silu_cond():
        cf = cond_ref[...].astype(F32)
        return jnp.broadcast_to((cf * jax.nn.sigmoid(cf)).astype(BF16), (8, M))

    cp_wk, cp_wv, cp_wq = pcopies(0)
    named = dict(k=cp_wk, v=cp_wv, q=cp_wq, o=ocopy(0), n=cp_cond, m=cp_wma)
    named.update(zip('abcd', cp_c))
    named.update(zip('wxyz', cp_x))
    started, arrived, did = set(), set(), set()

    def zero(r, carry):
        acc_scr[pl.ds(pl.multiple_of(r * T, T), T), :] = jnp.zeros((T, M), F32)
        return carry

    def x_rows(rows, dep):
        xf = x_ref[rows, :].astype(F32)
        if dep is None:
            return xf
        return jnp.concatenate([_after(xf[:, :T], _rows(dep, xf.shape[0])), xf[:, T:]], axis=1)

    def n_item(r, i):
        def fn(dep):
            rows = slice(r * T + i * LP, r * T + (i + 1) * LP)
            x1_scr[rows, :] = _ln(x_rows(rows, dep))
        return fn

    def h_item(r, i, normed):
        def fn(dep):
            rows = slice(i * LP, (i + 1) * LP)
            grows = slice(r * T + i * LP, r * T + (i + 1) * LP)
            sa = mod_scr[:, 0:M]
            if normed and dep is not None:
                sa = jnp.concatenate([_after(sa[:, _tile(j)], dep) for j in range(km)], axis=1)
            hf = ((x1_scr[grows, :] if normed else _ln(x_rows(grows, dep))) * _rows(mod_scr[:, M:2 * M], LP)
                  + _rows(sa, LP))
            for j in range(km):
                h_scr[r, j, rows, :] = hf[:, _tile(j)].astype(BF16)
            for f, n in _H_SUMS.items():
                if all(t[1] == r for t in f):
                    hs_scr[n, rows, :] = _form(f, lambda _, k: hf[:, _tile(k)]).astype(BF16)
            did.add(('h', r, i))
        return fn

    def release(jobs, span, items):
        if span and items:
            jobs.side += [(len(jobs.res) + 1 + i * span // len(items), fn) for i, fn in enumerate(items)]
            jobs.side.sort(key=lambda e: e[0])
        else:
            for fn in items:
                fn(None)

    def sum_items(n, group, index, dst, get, skip_rows):
        forms = [f for f in dict.fromkeys(t[0] for t in group)
                 if len(f) > 1 and not (skip_rows and len({t[1] for t in f}) == 1)]

        def item(f, rows):
            def fn(dep):
                def term(r, k):
                    v = get(r, k, rows).astype(F32)
                    return v if dep is None or (r, k) != f[0][1:] else _after(v, _rows(dep, v.shape[0]))
                dst[index[f], rows, :] = _form(f, term).astype(BF16)
            return fn

        return [item(f, slice(i, i + n)) for i in range(0, T, n) for f in forms]

    h_sums = lambda n, gi: sum_items(n, _H_GROUPS[gi], _H_SUMS, hs_scr,
                                     lambda r_, k, rows: h_scr[r_, k, rows, :], True)

    def stash(key, buf, j0, transpose=False):
        n = buf.shape[0] // T
        if key not in did:
            assert key in arrived
            did.add(key)
            w = _PairWeights(buf, transpose)
            for j in range(n):
                for hd in range(2):
                    w_scr[hd, j0 + j] = _pk(w(((1, j, hd),))[1])
        return lambda hd: [_ld(w_scr, hd, j0 + j) for j in range(n)]

    def kv_tile(jobs, r):
        wk, wvT = stash('k', wk_buf, 0), stash('v', wv_buf, kc, True)
        ct = [c_ref[_tile(r), _tile(j)] for j in range(kc)]
        for hd in range(2):
            k_scr[2 * r + hd] = _pk(jobs.mm(ct, wk(hd), _dot).astype(BF16))
        for hd in range(2):
            v_scr[2 * r + hd] = _pk(jobs.mm(wvT(hd), ct, _dot_nt).astype(BF16))

    def q_tile(jobs, r):
        wq = stash('q', wq_buf, 2 * kc)
        ht = [h_scr[r, j] for j in range(km)]
        for hd in range(2):
            q_scr[2 * r + hd] = _pk((jobs.mm(ht, wq(hd), _dot) * scale).astype(BF16))

    for blk in PROLOGUE.split(';'):
        waits, starts, acts = blk.split('|')
        for ch in waits.strip():
            assert ch in started and ch not in arrived
            arrived.add(ch)
            named[ch].wait()
        for ch in starts.strip():
            assert ch not in started
            started.add(ch)
            named[ch].start()
        jobs = _Jobs()
        for act in acts.split():
            if act == 'Z':
                jax.lax.fori_loop(0, nb, zero, 0)
                acc_scr[S:, :] = jnp.zeros((acc_scr.shape[0] - S, M), F32)
                x_ref[S:, :] = jnp.zeros((x_ref.shape[0] - S, M), BF16)
            elif act == 'M':
                assert arrived >= set('nm')
                mod = _dot(silu_cond(), wma_ref[...])
                mod_scr[:, 0:M] = mod[:, 0:M]
                mod_scr[:, M:2 * M] = 1.0 + mod[:, M:2 * M]
                did.add('M')
            else:
                act, _, span = act.partition('@')
                span = int(span or 0)
                items = []
                for r in [int(ch, 16) for ch in act[1:]]:
                    did.add((act[0], r))
                    if act[0] == 'K':
                        assert 'abcd'[r // CB] in arrived
                        kv_tile(jobs, r)
                    elif act[0] == 'H':
                        assert 'wxyz'[r // CB] in arrived and 'M' in did
                        items += [h_item(r, i, ('N', r) in did) for i in range(T // LP)]
                    elif act[0] == 'N':
                        assert 'wxyz'[r // CB] in arrived
                        items += [n_item(r, i) for i in range(T // LP)]
                    elif act[0] == 'Q':
                        assert all(('h', r, i) in did for i in range(T // LP))
                        q_tile(jobs, r)
                    elif act[0] == 'C':
                        assert all('abcd'[t[1] // CB] in arrived for p_ in _C_GROUPS[r] for t in p_[0])
                        items += sum_items(
                            32, _C_GROUPS[r], _C_SUMS, cs_scr,
                            lambda r_, k, rows: c_ref[r_ * T + rows.start:r_ * T + rows.stop, _tile(k)], False)
                    else:
                        assert act[0] == 'S' and all(('h', t[1], T // LP - 1) in did for p_ in _H_GROUPS[r] for t in p_[0])
                        items += h_sums(32 if span else 16, r)
                release(jobs, span, items)
        assert not jobs.side
    assert arrived == set(named) and all((k_, r) in did for k_ in 'KHQ' for r in range(nb))
    assert all((k_, r) in did for k_ in 'CS' for r in range(2))
    for cp in cp_late[1:] + cp_late[:1]:
        cp.start()

    FH = ws3.shape[0] * T
    assert nattn - 1 >= FH // 64

    def mixer_prep(g):
        def blocks(w_ref, r0, n, half, c0, c1, dep):
            lo, hi = pl.ds(r0, n), pl.ds(r0 + half, n)
            return [_after(w_ref[rows, _tile(c)].astype(F32), _rows(dep, n)) if (rows is lo) == (c == c0)
                    else w_ref[rows, _tile(c)].astype(F32) for rows in (lo, hi) for c in (c0, c1)]

        def rows_items(w_ref, dst, per_step, half, n=16):
            gi = jnp.minimum(g, half // per_step - 1)
            src = w_ref.at[pl.ds(pl.multiple_of(gi * per_step, per_step), half + per_step), :]
            hs = per_step // 2

            def item(c, o):
                def fn(dep):
                    for i, v in enumerate(_b_ops(*blocks(src, o, n, half, c, c + 2, dep))):
                        dst[i, c, pl.ds(pl.multiple_of(gi * hs, hs) + o // 2, n // 2), :] = _pk(v.astype(BF16))
                return fn
            return [item(c, o) for c in range(2) for o in range(0, per_step, n)]

        def w3_item(k, i):
            def fn(dep):
                n = jnp.minimum(g, FH // T - 1)
                b11, b21, b12, b22 = blocks(w3_ref, pl.multiple_of(n * T, T), T, FH, k, k + 2, dep)
                ws3[n, i, k] = _pk(_b_ops(b11, b12, b21, b22)[i].astype(BF16).T)
            return fn

        return (rows_items(w1_ref, ws12.at[0], 32, 2 * T) + rows_items(w2_ref, ws12.at[1], 32, 2 * T)
                + rows_items(w4_ref, ws4, 64, FH) + [w3_item(k, i) for k in range(2) for i in range(7)])

    def attn_body(g, carry):
        copies = pcopies(jnp.minimum(g + 1, nattn - 1))

        def mid():
            for cp in copies:
                cp.start()

        _attention_step(q_scr, k_scr, v_scr, wo_buf, acc_scr, mid)
        for cp in copies:
            cp.wait()

        @pl.when(g == 0)
        def _():
            for cp in cp_late[1:]:
                cp.wait()

        @pl.when(g + 1 < nattn)
        def _():
            ocopy(g + 1).start()
            side = [(SD0 + i * SDS, fn) for i, fn in enumerate(mixer_prep(g))]
            _proj_step(h_scr, hs_scr, c_ref, cs_scr, wq_buf, wk_buf, wv_buf, q_scr, k_scr, v_scr, scale, side)
            ocopy(g + 1).wait()

        return carry

    jax.lax.fori_loop(0, nattn, attn_body, 0)

    cp_late[0].wait()
    mod = _dot(silu_cond(), wmb_ref[...])
    mod_scr[:, 2 * M:4 * M] = mod[:, 0:2 * M]
    mod_scr[:, 4 * M:5 * M] = 1.0 + mod[:, 2 * M:3 * M]
    mod_scr[:, 5 * M:6 * M] = mod[:, 3 * M:4 * M]
    ftiles = [(f, min(f + T, Fd)) for f in range(0, Fd, T)]
    OFF = x_ref.shape[0] - S
    CAR = t_scr.shape[0] - RB

    def p1(r0, n, dep=None):
        ga = mod_scr[:, 2 * M:3 * M]
        if dep is not None:
            ga = jnp.concatenate([_after(ga[:, 0:T], dep), ga[:, T:]], axis=1)
        rows = pl.ds(r0, n)
        x1 = x_ref[rows, :].astype(F32) + _rows(ga, n) * acc_scr[rows, :]
        x1_scr[rows, :] = x1
        hb = _ln(x1) * _rows(mod_scr[:, 4 * M:5 * M], n) + _rows(mod_scr[:, 3 * M:4 * M], n)
        hb_scr[rows, :] = hb
        return _ln(hb)

    HT = T // 2

    def p1_store(r0, c, dep=None):
        n = PC // 2
        hf, o = divmod(c * n, HT)
        top, bot = [p1(r0 + hf * T + d + o, n, dep) for d in (0, HT)]
        for d, v in ((0, top), (HT, bot)):
            for j in range(km):
                a1_scr[j, hf * T + d + o:hf * T + d + o + n, :] = v[:, _tile(j)].astype(BF16)
        ops = _a_ops(top[:, 0:2 * T], top[:, 2 * T:4 * T], bot[:, 0:2 * T], bot[:, 2 * T:4 * T])
        for i, m in enumerate(SUMS):
            for k in range(2):
                a1s_scr[hf, i, k, o:o + n, :] = ops[m][:, _tile(k)].astype(BF16)
        return jnp.max(ops[0][:, :T].reshape(n // 8, 8, T), axis=0)

    t_scr[RB:RB + CAR - OFF, :] = jnp.zeros((CAR - OFF, M), F32)
    t_scr[RB + CAR - OFF:RB + CAR, :] = _gelu(_dot(p1(0, OFF).astype(BF16), w1_ref[...]))
    for c in range(RB // PC):
        p1_store(OFF, c)

    def out_copy(i):
        rows = pl.ds(i * T if isinstance(i, int) else pl.multiple_of(i * T, T), T)
        return pltpu.make_async_copy(out_buf.at[rows, :], out_hbm.at[rows, :], osem.at[i])

    def b_body(r, carry):
        gb = _rows(mod_scr[:, 5 * M:6 * M], T)
        r0 = pl.multiple_of(r * RB, RB)
        n0 = pl.multiple_of(jnp.minimum(r0 + RB, S - RB) + OFF, OFF)
        nh = RB // T
        now = [0]
        due = []
        pace = []

        def p1_item(c):
            return lambda dep: due.append((now[0] + PD, p1_store(n0, c, dep)))

        pace += [(P0 + i * PSTEP, p1_item(i)) for i in range(RB // PC)]
        wt = lambda ref, f0, f1, n: ref[f0:f1, _tile(n)]

        def mm(lhs, wts, dot=_dot):
            acc = None
            for x, w in zip(lhs, wts):
                if due and due[0][0] <= now[0]:
                    w = _tie(w, due.pop(0)[1])
                v = dot(x, w)
                now[0] += x.shape[0] // HT
                acc = v if acc is None else v + acc
                if pace and pace[0][0] <= now[0]:
                    pace.pop(0)[1](v[0:8, :])
            return acc

        def split_ops(lo, hi):
            return [v.astype(BF16) for v in _a_ops(lo[:HT], hi[:HT], lo[HT:], hi[HT:])]

        def two_tiles(aops, wsel, rest):
            def col(w):
                v = mm(rest[0], w, rest[3])
                return v[:HT], v[HT:]

            c11, c12, c21, c22 = _strassen(
                lambda i: mm([a[i] for a in aops], [wsel(i, k) for k in range(len(aops))]),
                lambda: col(rest[1]), lambda: col(rest[2]))
            return jnp.concatenate([c11, c21], axis=0), jnp.concatenate([c12, c22], axis=0)

        def square(full, aops, w_ref, ws_ref):
            out = {}
            for n in range(2):
                out[n], out[n + 2] = two_tiles(
                    aops, lambda i, k: _ld(ws_ref, i, n, slice(k * HT, (k + 1) * HT)),
                    (full[4:], [wt(w_ref, 4 * T, M, n)], [wt(w_ref, 4 * T, M, n + 2)], _dot))
            out[4] = mm(full, [wt(w_ref, j * T, (j + 1) * T, 4) for j in range(km)])
            return out

        t_scr[0:CAR, :] = t_scr[RB:RB + CAR, :]
        for hf in range(nh):
            full = [a1_scr[j, _tile(hf), :] for j in range(km)]
            aops = []
            for k in range(2):
                ops = {m: a1s_scr[hf, i, k] for i, m in enumerate(SUMS)}
                ops[2], ops[3] = full[k][:HT], full[2 + k][HT:]
                aops.append(ops)
            for n, v in square(full, aops, w1_ref, ws12.at[0]).items():
                t = _gelu(v)
                if hf == nh - 1:
                    t = jnp.concatenate([t[:T - OFF], jnp.where(r < nrb - 1, t[T - OFF:], 0.0)], axis=0)
                t_scr[CAR + hf * T:CAR + (hf + 1) * T, _tile(n)] = t
        cq = M // 4
        shifts = (-1, 1, -2, 2)
        lane = jax.lax.broadcasted_iota(jnp.int32, (T, T), 1)
        y1, a3 = [], []
        for hf in range(nh):
            base = CAR - OFF + hf * T
            sh = []
            for j in range(km):
                g_lo, g_hi = (j * T) // cq, ((j + 1) * T - 1) // cq
                assert g_hi - g_lo <= 1
                v = t_scr[base + shifts[g_lo]:base + shifts[g_lo] + T, _tile(j)]
                if g_hi != g_lo:
                    v2 = t_scr[base + shifts[g_hi]:base + shifts[g_hi] + T, _tile(j)]
                    v = jnp.where(lane < g_hi * cq - j * T, v, v2)
                sh.append(v)
            hs = square([v.astype(BF16) for v in sh], [split_ops(sh[k], sh[2 + k]) for k in range(2)],
                        w2_ref, ws12.at[1])
            hs = jnp.concatenate([hs[n] for n in range(km)], axis=1)
            y1.append(hs + hb_scr[pl.ds(pl.multiple_of(r0 + hf * T, T), T), :])
            a3.append({})

            def ln_item(hf, c):
                def item(dep):
                    n = HT // NLN
                    for d in (0, HT):
                        v = y1[hf][d + c * n:d + (c + 1) * n]
                        if dep is not None:
                            v = jnp.concatenate([_after(v[:, :T], _rows(dep, n)), v[:, T:]], axis=1)
                        a3[hf][d + c * n] = _ln(v)
                return item

            ln_item(hf, 0)(None)
            pace += [(now[0] + LN0 + (c - 1) * LNS * (1 + hf), ln_item(hf, c)) for c in range(1, NLN)]
            pace.sort(key=lambda e: e[0])
        nf = FH // T
        h3, h3ops = [], []
        for hf in range(nh):
            assert len(a3[hf]) == 2 * NLN
            af = jnp.concatenate([a3[hf][key] for key in sorted(a3[hf])], axis=0)
            full = [af[:, _tile(j)].astype(BF16) for j in range(km)]
            aops = [split_ops(af[:, _tile(k)], af[:, _tile(2 + k)]) for k in range(2)]
            row, ops = {}, []
            narrow = None
            for n in range(nf):
                lo, hi = two_tiles(aops, lambda i, k: _ld(ws3, n, i, k),
                                   (full[4:], [wt(w3_ref, *ftiles[n], 4)],
                                    [wt(w3_ref, *ftiles[nf + n], 4)], _dot_nt))
                lo, hi = _gelu(lo), _gelu(hi)
                row[n], row[nf + n] = lo.astype(BF16), hi.astype(BF16)
                ops.append(split_ops(lo, hi))
                if n < km:
                    v = mm([wt(w3_ref, *ftiles[-1], n)], [full[n]], _dot_nt)
                    narrow = v if narrow is None else v + narrow
            row[2 * nf] = _gelu(mm(full, [wt(w3_ref, *ftiles[2 * nf], j) for j in range(km)],
                                   _dot_nt)).astype(BF16)
            fw = Fd - ftiles[-1][0]
            gT = jnp.concatenate([_gelu(narrow), jnp.zeros((T - fw, T), F32)], axis=0)
            row[2 * nf + 1] = _tie(gT.astype(BF16).T, gT[0:8, :])[:, :fw]
            h3.append([row[i] for i in range(len(ftiles))])
            h3ops.append(ops)
        for hf in range(nh):
            rows = pl.ds(pl.multiple_of(r0 + hf * T, T), T)

            def finish(n, v):
                out_buf[rows, _tile(n)] = (
                    x1_scr[rows, _tile(n)] + gb[:, _tile(n)] * (v + y1[hf][:, _tile(n)])
                ).astype(out_buf.dtype)

            w4t = lambda n, f_: [wt(w4_ref, f0, f1, n) for f0, f1 in f_]
            finish(4, mm(h3[hf], w4t(4, ftiles)))
            for n in range(2):
                lo, hi = two_tiles(h3ops[hf], lambda i, k: _ld(ws4, i, n, slice(k * HT, (k + 1) * HT)),
                                   (h3[hf][2 * nf:], w4t(n, ftiles[2 * nf:]), w4t(n + 2, ftiles[2 * nf:]), _dot))
                finish(n, lo)
                finish(n + 2, hi)
            out_copy(r * nh + hf).start()
        assert not pace
        return carry

    jax.lax.fori_loop(0, nrb, b_body, 0)
    for i in range(nb):
        out_copy(i).wait()


@jax.jit
def pallas_adaLN_cond__compressed_kv_cla__mixer_s_mlp__prompt_kernel(
    A_x: jax.Array,
    A_c_kv: jax.Array,
    A_w_q: jax.Array,
    A_w_uk: jax.Array,
    A_w_uv: jax.Array,
    A_w_o: jax.Array,
    B_x: jax.Array,
    B_w1: jax.Array,
    B_w2: jax.Array,
    B_w3: jax.Array,
    B_w4: jax.Array,
    c: jax.Array,
    w_mod: jax.Array,
):
    _, S, M = A_x.shape
    Dc = A_c_kv.shape[2]
    H, D = A_w_q.shape[1], A_w_q.shape[2]
    Fd = B_w3.shape[1]
    assert D == T and A_c_kv.shape[1] == S and Dc == 4 * T and M == 5 * T and 13 * T < Fd < 14 * T and S == 16 * T
    vmem = pltpu.VMEM
    packed = lambda *lead: vmem(lead + (T // 2, T), U32)
    out = pl.pallas_call(
        _kernel,
        in_specs=[pl.BlockSpec(memory_space=pltpu.HBM)] * 12,
        out_specs=pl.BlockSpec(memory_space=pltpu.HBM),
        out_shape=jax.ShapeDtypeStruct((S, M), A_x.dtype),
        scratch_shapes=[
            vmem((S + 16, M), BF16),
            vmem((S, Dc), BF16),
            vmem((1, M), BF16),
            vmem((M, 2 * M), BF16),
            vmem((M, 4 * M), BF16),
            vmem((M, M), BF16),
            vmem((M, M), BF16),
            vmem((Fd, M), BF16),
            vmem((Fd, M), BF16),
            vmem((M, D), U32),
            vmem((Dc, D), U32),
            vmem((Dc, D), U32),
            vmem((2 * D, M), BF16),
            vmem((S, M), A_x.dtype),
            pltpu.SemaphoreType.DMA((15,)),
            pltpu.SemaphoreType.DMA((4,)),
            pltpu.SemaphoreType.DMA((S // T,)),
            vmem((8, 6 * M), F32),
            vmem((S // T, M // T, T, T), BF16),
            vmem((len(_C_SUMS), T, T), BF16),
            vmem((len(_H_SUMS), T, T), BF16),
            packed(2, M // T + 2 * (Dc // T)),
            packed(2 * S // T),
            packed(2 * S // T),
            packed(2 * S // T),
            vmem((S + 16, M), F32),
            vmem((S + 16, M), F32),
            vmem((S + 16, M), F32),
            vmem((M // T, RB, T), BF16),
            vmem((RB + 32, M), F32),
            vmem((RB // T, 5, 2, T // 2, T), BF16),
            vmem((2, 7, 2, T, T), U32),
            packed(6, 7, 2),
            vmem((7, 2, 3 * T, T), U32),
        ],
        compiler_params=pltpu.CompilerParams(
            vmem_limit_bytes=100 * 1024 * 1024,
            disable_bounds_checks=True,
        ),
    )(
        A_x.reshape(S, M), A_c_kv.reshape(S, Dc),
        A_w_q, A_w_uk, A_w_uv,
        A_w_o.reshape(H // 2, 2 * D, M),
        B_w1, B_w2, B_w3.T, B_w4, c, w_mod,
    )
    return out.reshape(1, S, M)
```

```python
import math

import jax
import jax.numpy as jnp
import jax.experimental.pallas as pl
import jax.experimental.pallas.tpu as pltpu

F32 = jnp.float32
BF16 = jnp.bfloat16
U32 = jnp.uint32
NT = (((1,), (1,)), ((), ()))
T = 128
EPS = 1e-5
LOG2E = math.log2(math.e)

GRP = 4
LEAD = 10
PROW = 3
RES = 32
LAT_A = 16
LAT_B = 20
ALEAD = 32
MID = 40
SD0, SDS = 60, 4
RB = 256
PC = 32
P0, PSTEP, PD = 440, 30, 52
NLN, LN0, LNS = 4, 4, 5
LP = 16
PROLOGUE = ('|kva|Z; |b|; kva|wc|K0123; bw|xdn|C0@56 N0123@52 K4567; cx|mq|N4567@52 K89ab; '
            'd|y|C1@56 Kcdef; nmq|zo|M H01 H234567@30 Q0123; y||H89ab@30 Q4567; '
            'z||Hcdef@30 Q89ab S01 Qcdef; o||')


def _dot(a, b):
    return jnp.dot(a, b, preferred_element_type=F32)


def _dot_nt(a, b):
    return jax.lax.dot_general(a, b, NT, preferred_element_type=F32)


def _ln(x):
    m = jnp.mean(x, axis=-1, keepdims=True)
    xc = x - m
    v = jnp.mean(xc * xc, axis=-1, keepdims=True)
    return xc * jnp.exp2(jnp.log(v + EPS) * (-0.5 * LOG2E))


def _rows(v, n):
    return jnp.broadcast_to(v[None], (n // 8, 8, v.shape[1])).reshape(n, v.shape[1])


def _gelu(x):
    c0 = math.sqrt(2.0 / math.pi)
    return 0.5 * x * (1.0 + jnp.tanh(c0 * (x + 0.044715 * (x * x * x))))


def _after(x, dep):
    return jnp.where(dep > jnp.inf, dep, x)


def _tie(x, dep):
    xu = pltpu.bitcast(x, U32)
    first = jnp.where(dep > jnp.inf, jnp.uint32(0), xu[:8])
    return pltpu.bitcast(jnp.concatenate([first, xu[8:]], axis=0), BF16)


def _tile(j):
    return slice(j * T, (j + 1) * T)


def _ld(ref, *idx):
    return pltpu.bitcast(ref[idx], BF16)


def _pk(x):
    return pltpu.bitcast(x, U32)


def _a_ops(a11, a12, a21, a22):
    return [a11 + a22, a21 + a22, a11, a22, a11 + a12, a21 - a11, a12 - a22]


def _b_ops(b11, b12, b21, b22):
    return [b11 + b22, b11, b12 - b22, b21 - b11, b22, b11 + b12, b21 + b22]


def _strassen(prod, col1=None, col2=None):
    m4 = prod(3)
    m2 = prod(1)
    c21 = m2 + m4
    if col1 is not None:
        e11, e21 = col1()
        m4, c21 = m4 + e11, c21 + e21
    m3 = prod(2)
    m5 = prod(4)
    c12 = m3 + m5
    if col2 is not None:
        e12, e22 = col2()
        c12, m3 = c12 + e12, m3 + e22
    m1 = prod(0)
    c11 = prod(6) + (m1 + (m4 - m5))
    c22 = prod(5) + (m1 + (m3 - m2))
    return c11, c12, c21, c22


def _group(rows, cols, pairs):
    xs, ys = dict.fromkeys(x for x, _ in pairs), dict.fromkeys(y for _, y in pairs)
    used = set(xs) | set(ys) | {(x[0], y[1]) for x, y in pairs} | {(y[0], x[1]) for x, y in pairs}
    prods = []
    for n, r in enumerate(rows):
        for i, k in [x for x in xs if x[0] == r]:
            mates = [y for x, y in pairs if x == (i, k)]
            prods.append((((1, i, k),) + tuple((1, i, k2) for _, k2 in mates), ((1, k, 0),),
                          ((1, i, 0), (-1, i, 1))))
            prods.append((((1, i, k),) + tuple((-1, i2, k) for i2, _ in mates), ((1, k, 0), (1, k, 1)),
                          ((1, i, 1),)))
        for i2, k2 in [y for y in ys if y[0] == r]:
            mates = [x for x, y in pairs if y == (i2, k2)]
            prods.append((((1, i2, k2),) + tuple((1, i2, k) for _, k in mates), ((1, k2, 1),),
                          ((1, i2, 1), (-1, i2, 0))))
            prods.append((((1, i2, k2),) + tuple((-1, i, k2) for i, _ in mates), ((1, k2, 0), (1, k2, 1)),
                          ((1, i2, 0),)))
        prods += [(((1, r, k),), ((1, k, h),), ((1, r, h),)) for k in cols if (r, k) not in used for h in (0, 1)]
        for (i, k), (i2, k2) in pairs:
            if r in (i, i2) and i + i2 - r in rows[n + 1:]:
                prods.append((((1, i, k2),), ((1, k2, 0), (-1, k, 0)), ((1, i2, 0), (1, i, 0))))
                prods.append((((1, i2, k), (1, i, k2)), ((1, k, 0), (1, k2, 1)), ((1, i2, 0), (1, i, 1))))
                prods.append((((1, i2, k),), ((1, k, 1), (-1, k2, 1)), ((1, i2, 1), (1, i, 1))))
    return prods


def _all_pairs(xrows, yrows):
    return [((x, a), (y, b)) for a, x in enumerate(xrows) for b, y in enumerate(yrows) if a != b]


_PAIRS65 = [((x[0] + 10, x[1]), (y[0] + 10, y[1])) for x, y in (
    ((0, 1), (1, 0)), ((0, 1), (5, 2)), ((2, 3), (1, 0)), ((2, 3), (3, 1)), ((2, 3), (5, 2)), ((3, 2), (1, 0)),
    ((4, 4), (0, 3)), ((4, 4), (1, 0)), ((4, 4), (3, 1)), ((4, 4), (5, 2)))]
_C_GROUPS = [_group(range(r, r + 8), range(4), _all_pairs(range(r, r + 4), range(r + 4, r + 8))) for r in (0, 8)]
_H_GROUPS = [_group(range(10), range(5), _all_pairs(range(5), range(5, 10))),
             _group(range(10, 16), range(5), _PAIRS65)]
_sum_index = lambda groups: {f: n for n, f in enumerate(
    dict.fromkeys(t[0] for g in groups for t in g if len(t[0]) > 1))}
_C_SUMS, _H_SUMS = _sum_index(_C_GROUPS), _sum_index(_H_GROUPS)


def _form(form, get):
    acc = None
    for sign, i, j in form:
        v = get(i, j)
        acc = v if acc is None else (acc + v if sign > 0 else acc - v)
    return acc


class _PairWeights:
    def __init__(self, w_ref, transpose=False):
        self.base = {}
        for j in range(w_ref.shape[0] // T):
            wu = w_ref[_tile(j), :]
            if transpose:
                wu = wu.T
            self.base[j, 0] = pltpu.bitcast(wu << 16, F32)
            self.base[j, 1] = pltpu.bitcast(wu & jnp.uint32(0xFFFF0000), F32)
        self.cache = {}

    def __call__(self, form):
        sign = 1
        if form[-1][0] < 0 and form[0][1:] > form[1][1:]:
            sign, form = -1, ((1,) + form[1][1:], (-1,) + form[0][1:])
        if form not in self.cache:
            self.cache[form] = _form(form, lambda k, h: self.base[k, h]).astype(BF16)
        return sign, self.cache[form]


def _run_group(jobs, prods, a_get, w, transposed, finish):
    left = {}
    for _, _, outs in prods:
        for _, i, h in outs:
            left[i, h] = left.get((i, h), 0) + 1
    acc = {}
    for af, bf, outs in prods:
        sign, wt = w(bf)
        m = jobs.mm([wt], [a_get(af)], _dot_nt) if transposed else jobs.mm([a_get(af)], [wt], _dot)
        for s_, i, h in outs:
            if (i, h) not in acc:
                acc[i, h] = (s_ * sign, m)
            else:
                s0, v = acc[i, h]
                acc[i, h] = (s0, v + m if s0 == s_ * sign else v - m) if s0 > 0 or s_ * sign < 0 else (1, m - v)
            left[i, h] -= 1
            if not left[i, h]:
                s0, v = acc.pop((i, h))
                assert s0 > 0
                finish(2 * i + h, v)


class _Jobs:
    def __init__(self, side=()):
        self.res = []
        self.side = list(side)

    def mm(self, lhs, wt, dot):
        acc = None
        for x, w in zip(lhs, wt):
            v = dot(x, w)
            self.res.append(v)
            acc = v if acc is None else v + acc
            rel = 4 * (len(self.res) % 4)
            while self.side and self.side[0][0] <= len(self.res):
                self.side.pop(0)[1](v[8 * rel:8 * rel + 8, :])
                rel = (rel + 2) % 16
        return acc


def _proj_step(h_scr, hs_scr, c_ref, cs_scr, wq_ref, wuk_ref, wuv_ref, q_scr, k_scr, v_scr, scale, side):
    wq, wk, wvT = _PairWeights(wq_ref), _PairWeights(wuk_ref), _PairWeights(wuv_ref, True)
    c_get = lambda f: cs_scr[_C_SUMS[f]] if len(f) > 1 else c_ref[_tile(f[0][1]), _tile(f[0][2])]
    h_get = lambda f: hs_scr[_H_SUMS[f]] if len(f) > 1 else h_scr[f[0][1], f[0][2]]

    def put(dst, mul=None):
        def fn(u, v):
            dst[u] = _pk((v if mul is None else v * mul).astype(BF16))
        return fn

    jobs = _Jobs(side)
    for groups, get, w, transposed, fin in ((_C_GROUPS, c_get, wk, False, put(k_scr)),
                                            (_C_GROUPS, c_get, wvT, True, put(v_scr)),
                                            (_H_GROUPS, h_get, wq, False, put(q_scr, scale))):
        for prods in groups:
            _run_group(jobs, prods, get, w, transposed, fin)
    assert not jobs.side


def _inner_group(rows, cols, pairs):
    xs, ys = dict.fromkeys(x for x, _ in pairs), dict.fromkeys(y for _, y in pairs)
    used = set(xs) | set(ys) | {(x[0], y[1]) for x, y in pairs} | {(y[0], x[1]) for x, y in pairs}
    prods = []
    for i, j in xs:
        mates = [y for x, y in pairs if x == (i, j)]
        prods.append((((1, i, 0),), ((1, 0, j), (-1, 1, j)), ((1, i, j),) + tuple((1, i2, j) for i2, _ in mates)))
        prods.append((((1, i, 0), (1, i, 1)), ((1, 1, j),), ((1, i, j),) + tuple((-1, i, j2) for _, j2 in mates)))
    for i2, j2 in ys:
        mates = [x for x, y in pairs if y == (i2, j2)]
        prods.append((((1, i2, 0), (1, i2, 1)), ((1, 0, j2),),
                      ((1, i2, j2),) + tuple((-1, i2, j) for _, j in mates)))
        prods.append((((1, i2, 1),), ((1, 0, j2), (-1, 1, j2)),
                      ((-1, i2, j2),) + tuple((-1, i, j2) for i, _ in mates)))
    prods += [(((1, i, h),), ((1, h, j),), ((1, i, j),))
              for i in rows for j in cols if (i, j) not in used for h in (0, 1)]
    for (i, j), (i2, j2) in pairs:
        lo, hi = min(j, j2), max(j, j2)
        prods.append((((1, i2, 0), (-1, i, 0)), ((1, 0, lo), (1, 0, hi)), ((1, i2, j),)))
        prods.append((((1, i, 0), (1, i2, 1)), ((1, 0, j2), (1, 1, j)), ((1, i, j2), (1, i2, j))))
        prods.append((((1, i, 1), (-1, i2, 1)), ((1, 1, lo), (1, 1, hi)), ((1, i, j2),)))
    return prods


def _o_jobs():
    prods = (_inner_group(range(10), range(5), _all_pairs(range(0, 10, 2), range(1, 10, 2)))
             + _inner_group(range(10, 16), range(5), _PAIRS65))
    row = lambda t: max(i for _, i, _ in t[0])
    unit = lambda t: max(2 * i + h for _, i, h in t[0])
    need = lambda t: unit(t) if row(t) == 15 else 2 * row(t) + 1
    return [(need(t), t) for t in sorted(prods, key=need)]


_O_JOBS = _o_jobs()


def _job_order(nb):
    units = range(2 * nb)
    qa = [('a', u, c) for u in units for c in range(u // 2 + 1)]
    qb = [('b', u, c) for u in units for c in range(u // 2 + 1)]
    qo = [('o', u, j) for j, (u, _) in enumerate(_O_JOBS)]
    done = {}
    order = []

    def ready(q, lat, pre):
        return bool(q) and (pre, q[0][1]) in done and done[(pre, q[0][1])] + lat <= len(order)

    def emit(q):
        kind, u, j = job = q.pop(0)
        if kind != 'o' and j == u // 2:
            done[(kind, u)] = len(order)
        order.append(job)

    turn = 0
    while qa or qb or qo:
        pref = 'abo'[turn % 3]
        turn += 1
        for _ in range(GRP):
            b_ok, o_ok = ready(qb, LAT_A, 'a'), ready(qo, LAT_B, 'b')
            if pref == 'a' and qa and (len(qb) - len(qa) < ALEAD or not b_ok):
                emit(qa)
            elif pref == 'b' and b_ok:
                emit(qb)
            elif pref == 'o' and o_ok and (len(qo) > RES or not (qa or b_ok)):
                emit(qo)
            elif not (qa or b_ok or o_ok) and (qb or qo):
                emit(qb or qo)
            else:
                break
    return order


def _attention_step(q_scr, k_scr, v_scr, wo_ref, acc_scr, mid):
    causal = (jax.lax.broadcasted_iota(jnp.int32, (T, T), 0)
              <= jax.lax.broadcasted_iota(jnp.int32, (T, T), 1))
    sv, mx, mfin, lsum, pv, of, lhs = {}, {}, {}, {}, {}, {}, {}
    res = []
    wo, terms = {}, {}
    left = {}
    for _, t in _O_JOBS:
        for _, i, j in t[2]:
            left[i, j] = left.get((i, j), 0) + 1

    def job_a(u, c):
        r, hd = divmod(u, 2)
        s = _dot_nt(_ld(k_scr, 2 * c + hd), _ld(q_scr, u))
        res.append(s)
        if c == r:
            s = jnp.where(causal, s, -1e9 * LOG2E)
        s = s.reshape(T // 8, 8, T)
        sv[(u, c)] = s
        pm = jnp.max(s, axis=0)
        mx[u] = pm if u not in mx else jnp.maximum(mx[u], pm)

    def job_b(u, c):
        r, hd = divmod(u, 2)
        if u not in mfin:
            mfin[u] = jnp.broadcast_to(jnp.max(mx[u], axis=0, keepdims=True), (8, T))
        m = mfin[u]
        if len(res) >= LEAD:
            r0 = 8 * PROW * (c % 4)
            m = _after(m, res[len(res) - LEAD][r0:r0 + 8, :])
        p = jnp.exp2(sv.pop((u, c)) - m[None])
        ls = jnp.sum(p, axis=0)
        lsum[u] = ls if u not in lsum else lsum[u] + ls
        v = _dot(_ld(v_scr, 2 * c + hd), p.reshape(T, T).astype(BF16))
        res.append(v)
        pv[u] = v if u not in pv else v + pv[u]
        if c == r:
            of[u] = pv[u] * (1.0 / jnp.sum(lsum[u], axis=0, keepdims=True))

    def job_o(_, n):
        af, bf, outs = _O_JOBS[n][1]
        if af not in lhs:
            v = _form(af, lambda i, h: of[2 * i + h])
            lhs[af] = _tie(v.astype(BF16).T, v[0:8, :])
        if bf not in wo:
            wo[bf] = (wo_ref[_tile(bf[0][1]), _tile(bf[0][2])] if len(bf) == 1 else
                      _form(bf, lambda h, j: wo_ref[_tile(h), _tile(j)].astype(F32)).astype(BF16))
        v = _dot(lhs[af], wo[bf])
        res.append(v)
        for sign, i, j in outs:
            terms.setdefault((i, j), []).append((sign, v))
            if len(terms[i, j]) == left[i, j]:
                tot = acc_scr[_tile(i), _tile(j)]
                for sg, m in terms.pop((i, j)):
                    tot = tot + m if sg > 0 else tot - m
                acc_scr[_tile(i), _tile(j)] = tot

    fns = dict(a=job_a, b=job_b, o=job_o)
    for n, (kind, u, j) in enumerate(_job_order(q_scr.shape[0] // 2)):
        if n == MID:
            mid()
        fns[kind](u, j)


def _kernel(x_hbm, c_hbm, wq_hbm, wuk_hbm, wuv_hbm, wo_hbm, w1_hbm, w2_hbm, w3_hbm, w4_hbm,
            cond_hbm, wmod_hbm, out_hbm,
            x_ref, c_ref, cond_ref, wma_ref, wmb_ref, w1_ref, w2_ref, w3_ref, w4_ref,
            wq_buf, wk_buf, wv_buf, wo_buf, out_buf, sem, wsem, osem,
            mod_scr, h_scr, cs_scr, hs_scr, w_scr, q_scr, k_scr, v_scr, acc_scr, x1_scr, hb_scr, a1_scr, t_scr,
            ws12, ws3, ws4):
    S, M = x_hbm.shape
    D = wq_hbm.shape[2]
    nattn = wo_hbm.shape[0]
    Fd = w4_hbm.shape[0]
    scale = float(D) ** -0.5 * LOG2E
    nb, nrb = S // T, S // RB
    km, kc = M // T, c_hbm.shape[1] // T
    NX = 4
    XR = S // NX
    CB = XR // T

    def pcopies(g):
        return [pltpu.make_async_copy(src.bitcast(U32).at[:, g, :], dst, wsem.at[j])
                for j, (src, dst) in enumerate(((wuk_hbm, wk_buf), (wuv_hbm, wv_buf), (wq_hbm, wq_buf)))]

    def ocopy(g):
        return pltpu.make_async_copy(wo_hbm.at[g], wo_buf, wsem.at[3])

    def chunk_copy(src, dst, i, s0):
        rows = slice(i * XR, (i + 1) * XR)
        return pltpu.make_async_copy(src.at[rows, :], dst.at[rows, :], sem.at[s0 + i])

    cp_cond = pltpu.make_async_copy(cond_hbm, cond_ref, sem.at[0])
    cp_wma = pltpu.make_async_copy(wmod_hbm.at[:, 0:2 * M], wma_ref, sem.at[1])
    cp_late = [pltpu.make_async_copy(src, dst, sem.at[2 + j]) for j, (src, dst) in enumerate((
        (wmod_hbm.at[:, 2 * M:6 * M], wmb_ref), (w1_hbm, w1_ref), (w2_hbm, w2_ref),
        (w3_hbm, w3_ref), (w4_hbm, w4_ref)))]
    cp_x = [chunk_copy(x_hbm, x_ref, i, 7) for i in range(NX)]
    cp_c = [chunk_copy(c_hbm, c_ref, i, 7 + NX) for i in range(NX)]

    def silu_cond():
        cf = cond_ref[...].astype(F32)
        return jnp.broadcast_to((cf * jax.nn.sigmoid(cf)).astype(BF16), (8, M))

    cp_wk, cp_wv, cp_wq = pcopies(0)
    named = dict(k=cp_wk, v=cp_wv, q=cp_wq, o=ocopy(0), n=cp_cond, m=cp_wma)
    named.update(zip('abcd', cp_c))
    named.update(zip('wxyz', cp_x))
    started, arrived, did = set(), set(), set()

    def zero(r, carry):
        acc_scr[pl.ds(pl.multiple_of(r * T, T), T), :] = jnp.zeros((T, M), F32)
        return carry

    def x_rows(rows, dep):
        xf = x_ref[rows, :].astype(F32)
        if dep is None:
            return xf
        return jnp.concatenate([_after(xf[:, :T], _rows(dep, xf.shape[0])), xf[:, T:]], axis=1)

    def n_item(r, i):
        def fn(dep):
            rows = slice(r * T + i * LP, r * T + (i + 1) * LP)
            x1_scr[rows, :] = _ln(x_rows(rows, dep))
        return fn

    def h_item(r, i, normed):
        def fn(dep):
            rows = slice(i * LP, (i + 1) * LP)
            grows = slice(r * T + i * LP, r * T + (i + 1) * LP)
            sa = mod_scr[:, 0:M]
            if normed and dep is not None:
                sa = jnp.concatenate([_after(sa[:, _tile(j)], dep) for j in range(km)], axis=1)
            hf = ((x1_scr[grows, :] if normed else _ln(x_rows(grows, dep))) * _rows(mod_scr[:, M:2 * M], LP)
                  + _rows(sa, LP))
            for j in range(km):
                h_scr[r, j, rows, :] = hf[:, _tile(j)].astype(BF16)
            for f, n in _H_SUMS.items():
                if all(t[1] == r for t in f):
                    hs_scr[n, rows, :] = _form(f, lambda _, k: hf[:, _tile(k)]).astype(BF16)
            did.add(('h', r, i))
        return fn

    def release(jobs, span, items):
        if span and items:
            jobs.side += [(len(jobs.res) + 1 + i * span // len(items), fn) for i, fn in enumerate(items)]
            jobs.side.sort(key=lambda e: e[0])
        else:
            for fn in items:
                fn(None)

    def sum_items(n, group, index, dst, get, skip_rows):
        forms = [f for f in dict.fromkeys(t[0] for t in group)
                 if len(f) > 1 and not (skip_rows and len({t[1] for t in f}) == 1)]

        def item(f, rows):
            def fn(dep):
                def term(r, k):
                    v = get(r, k, rows).astype(F32)
                    return v if dep is None or (r, k) != f[0][1:] else _after(v, _rows(dep, v.shape[0]))
                dst[index[f], rows, :] = _form(f, term).astype(BF16)
            return fn

        return [item(f, slice(i, i + n)) for i in range(0, T, n) for f in forms]

    h_sums = lambda n, gi: sum_items(n, _H_GROUPS[gi], _H_SUMS, hs_scr,
                                     lambda r_, k, rows: h_scr[r_, k, rows, :], True)

    def stash(key, buf, j0, transpose=False):
        n = buf.shape[0] // T
        if key not in did:
            assert key in arrived
            did.add(key)
            w = _PairWeights(buf, transpose)
            for j in range(n):
                for hd in range(2):
                    w_scr[hd, j0 + j] = _pk(w(((1, j, hd),))[1])
        return lambda hd: [_ld(w_scr, hd, j0 + j) for j in range(n)]

    def kv_tile(jobs, r):
        wk, wvT = stash('k', wk_buf, 0), stash('v', wv_buf, kc, True)
        ct = [c_ref[_tile(r), _tile(j)] for j in range(kc)]
        for hd in range(2):
            k_scr[2 * r + hd] = _pk(jobs.mm(ct, wk(hd), _dot).astype(BF16))
        for hd in range(2):
            v_scr[2 * r + hd] = _pk(jobs.mm(wvT(hd), ct, _dot_nt).astype(BF16))

    def q_tile(jobs, r):
        wq = stash('q', wq_buf, 2 * kc)
        ht = [h_scr[r, j] for j in range(km)]
        for hd in range(2):
            q_scr[2 * r + hd] = _pk((jobs.mm(ht, wq(hd), _dot) * scale).astype(BF16))

    for blk in PROLOGUE.split(';'):
        waits, starts, acts = blk.split('|')
        for ch in waits.strip():
            assert ch in started and ch not in arrived
            arrived.add(ch)
            named[ch].wait()
        for ch in starts.strip():
            assert ch not in started
            started.add(ch)
            named[ch].start()
        jobs = _Jobs()
        for act in acts.split():
            if act == 'Z':
                jax.lax.fori_loop(0, nb, zero, 0)
                acc_scr[S:, :] = jnp.zeros((acc_scr.shape[0] - S, M), F32)
                x_ref[S:, :] = jnp.zeros((x_ref.shape[0] - S, M), BF16)
            elif act == 'M':
                assert arrived >= set('nm')
                mod = _dot(silu_cond(), wma_ref[...])
                mod_scr[:, 0:M] = mod[:, 0:M]
                mod_scr[:, M:2 * M] = 1.0 + mod[:, M:2 * M]
                did.add('M')
            else:
                act, _, span = act.partition('@')
                span = int(span or 0)
                items = []
                for r in [int(ch, 16) for ch in act[1:]]:
                    did.add((act[0], r))
                    if act[0] == 'K':
                        assert 'abcd'[r // CB] in arrived
                        kv_tile(jobs, r)
                    elif act[0] == 'H':
                        assert 'wxyz'[r // CB] in arrived and 'M' in did
                        items += [h_item(r, i, ('N', r) in did) for i in range(T // LP)]
                    elif act[0] == 'N':
                        assert 'wxyz'[r // CB] in arrived
                        items += [n_item(r, i) for i in range(T // LP)]
                    elif act[0] == 'Q':
                        assert all(('h', r, i) in did for i in range(T // LP))
                        q_tile(jobs, r)
                    elif act[0] == 'C':
                        assert all('abcd'[t[1] // CB] in arrived for p_ in _C_GROUPS[r] for t in p_[0])
                        items += sum_items(
                            32, _C_GROUPS[r], _C_SUMS, cs_scr,
                            lambda r_, k, rows: c_ref[r_ * T + rows.start:r_ * T + rows.stop, _tile(k)], False)
                    else:
                        assert act[0] == 'S' and all(('h', t[1], T // LP - 1) in did for p_ in _H_GROUPS[r] for t in p_[0])
                        items += h_sums(32 if span else 16, r)
                release(jobs, span, items)
        assert not jobs.side
    assert arrived == set(named) and all((k_, r) in did for k_ in 'KHQ' for r in range(nb))
    assert all((k_, r) in did for k_ in 'CS' for r in range(2))
    for cp in cp_late[1:] + cp_late[:1]:
        cp.start()

    FH = ws3.shape[0] * T
    assert nattn - 1 >= FH // 64

    def mixer_prep(g):
        def blocks(w_ref, r0, n, half, c0, c1, dep):
            lo, hi = pl.ds(r0, n), pl.ds(r0 + half, n)
            return [_after(w_ref[rows, _tile(c)].astype(F32), _rows(dep, n)) if (rows is lo) == (c == c0)
                    else w_ref[rows, _tile(c)].astype(F32) for rows in (lo, hi) for c in (c0, c1)]

        def rows_items(w_ref, dst, per_step, half, n=16):
            gi = jnp.minimum(g, half // per_step - 1)
            src = w_ref.at[pl.ds(pl.multiple_of(gi * per_step, per_step), half + per_step), :]
            hs = per_step // 2

            def item(c, o):
                def fn(dep):
                    for i, v in enumerate(_b_ops(*blocks(src, o, n, half, c, c + 2, dep))):
                        dst[i, c, pl.ds(pl.multiple_of(gi * hs, hs) + o // 2, n // 2), :] = _pk(v.astype(BF16))
                return fn
            return [item(c, o) for c in range(2) for o in range(0, per_step, n)]

        def w3_item(k, i):
            def fn(dep):
                n = jnp.minimum(g, FH // T - 1)
                b11, b21, b12, b22 = blocks(w3_ref, pl.multiple_of(n * T, T), T, FH, k, k + 2, dep)
                ws3[n, i, k] = _pk(_b_ops(b11, b12, b21, b22)[i].astype(BF16).T)
            return fn

        return (rows_items(w1_ref, ws12.at[0], 32, 2 * T) + rows_items(w2_ref, ws12.at[1], 32, 2 * T)
                + rows_items(w4_ref, ws4, 64, FH) + [w3_item(k, i) for k in range(2) for i in range(7)])

    def attn_body(g, carry):
        copies = pcopies(jnp.minimum(g + 1, nattn - 1))

        def mid():
            for cp in copies:
                cp.start()

        _attention_step(q_scr, k_scr, v_scr, wo_buf, acc_scr, mid)
        for cp in copies:
            cp.wait()

        @pl.when(g == 0)
        def _():
            for cp in cp_late[1:]:
                cp.wait()

        @pl.when(g + 1 < nattn)
        def _():
            ocopy(g + 1).start()
            side = [(SD0 + i * SDS, fn) for i, fn in enumerate(mixer_prep(g))]
            _proj_step(h_scr, hs_scr, c_ref, cs_scr, wq_buf, wk_buf, wv_buf, q_scr, k_scr, v_scr, scale, side)
            ocopy(g + 1).wait()

        return carry

    jax.lax.fori_loop(0, nattn, attn_body, 0)

    cp_late[0].wait()
    mod = _dot(silu_cond(), wmb_ref[...])
    mod_scr[:, 2 * M:4 * M] = mod[:, 0:2 * M]
    mod_scr[:, 4 * M:5 * M] = 1.0 + mod[:, 2 * M:3 * M]
    mod_scr[:, 5 * M:6 * M] = mod[:, 3 * M:4 * M]
    ftiles = [(f, min(f + T, Fd)) for f in range(0, Fd, T)]
    OFF = x_ref.shape[0] - S
    CAR = t_scr.shape[0] - RB

    def p1(r0, n, dep=None):
        ga = mod_scr[:, 2 * M:3 * M]
        if dep is not None:
            ga = jnp.concatenate([_after(ga[:, 0:T], dep), ga[:, T:]], axis=1)
        rows = pl.ds(r0, n)
        x1 = x_ref[rows, :].astype(F32) + _rows(ga, n) * acc_scr[rows, :]
        x1_scr[rows, :] = x1
        hb = _ln(x1) * _rows(mod_scr[:, 4 * M:5 * M], n) + _rows(mod_scr[:, 3 * M:4 * M], n)
        hb_scr[rows, :] = hb
        return _ln(hb)

    HT = T // 2

    def p1_store(r0, c, dep=None):
        v = p1(r0 + c * PC, PC, dep)
        a1_scr[c * PC:(c + 1) * PC, :] = v
        return jnp.max(v[:, M - T:].reshape(PC // 8, 8, T), axis=0)

    t_scr[RB:RB + CAR - OFF, :] = jnp.zeros((CAR - OFF, M), F32)
    t_scr[RB + CAR - OFF:RB + CAR, :] = _gelu(_dot(p1(0, OFF).astype(BF16), w1_ref[...]))
    for c in range(RB // PC):
        p1_store(OFF, c)

    def out_copy(i):
        rows = pl.ds(i * T if isinstance(i, int) else pl.multiple_of(i * T, T), T)
        return pltpu.make_async_copy(out_buf.at[rows, :], out_hbm.at[rows, :], osem.at[i])

    def b_body(r, carry):
        gb = _rows(mod_scr[:, 5 * M:6 * M], T)
        r0 = pl.multiple_of(r * RB, RB)
        n0 = pl.multiple_of(jnp.minimum(r0 + RB, S - RB) + OFF, OFF)
        nh = RB // T
        now = [0]
        due = []
        pace = []

        def p1_item(c):
            return lambda dep: due.append((now[0] + PD, p1_store(n0, c, dep)))

        pace += [(P0 + i * PSTEP, p1_item(i)) for i in range(RB // PC)]
        wt = lambda ref, f0, f1, n: ref[f0:f1, _tile(n)]

        def mm(lhs, wts, dot=_dot):
            acc = None
            for x, w in zip(lhs, wts):
                if due and due[0][0] <= now[0]:
                    w = _tie(w, due.pop(0)[1])
                v = dot(x, w)
                now[0] += x.shape[0] // HT
                acc = v if acc is None else v + acc
                if pace and pace[0][0] <= now[0]:
                    pace.pop(0)[1](v[0:8, :])
            return acc

        def split_ops(lo, hi):
            return [v.astype(BF16) for v in _a_ops(lo[:HT], hi[:HT], lo[HT:], hi[HT:])]

        def two_tiles(aops, wsel, rest):
            def col(w):
                v = mm(rest[0], w, rest[3])
                return v[:HT], v[HT:]

            c11, c12, c21, c22 = _strassen(
                lambda i: mm([a[i] for a in aops], [wsel(i, k) for k in range(len(aops))]),
                lambda: col(rest[1]), lambda: col(rest[2]))
            return jnp.concatenate([c11, c21], axis=0), jnp.concatenate([c12, c22], axis=0)

        def square(full, aops, w_ref, ws_ref):
            out = {}
            for n in range(2):
                out[n], out[n + 2] = two_tiles(
                    aops, lambda i, k: _ld(ws_ref, i, n, slice(k * HT, (k + 1) * HT)),
                    (full[4:], [wt(w_ref, 4 * T, M, n)], [wt(w_ref, 4 * T, M, n + 2)], _dot))
            out[4] = mm(full, [wt(w_ref, j * T, (j + 1) * T, 4) for j in range(km)])
            return out

        t_scr[0:CAR, :] = t_scr[RB:RB + CAR, :]
        for hf in range(nh):
            a1 = [a1_scr[_tile(hf), _tile(j)] for j in range(km)]
            full = [v.astype(BF16) for v in a1]
            aops = [split_ops(a1[k], a1[2 + k]) for k in range(2)]
            for n, v in square(full, aops, w1_ref, ws12.at[0]).items():
                t = _gelu(v)
                if hf == nh - 1:
                    t = jnp.concatenate([t[:T - OFF], jnp.where(r < nrb - 1, t[T - OFF:], 0.0)], axis=0)
                t_scr[CAR + hf * T:CAR + (hf + 1) * T, _tile(n)] = t
        cq = M // 4
        shifts = (-1, 1, -2, 2)
        lane = jax.lax.broadcasted_iota(jnp.int32, (T, T), 1)
        y1, a3 = [], []
        for hf in range(nh):
            base = CAR - OFF + hf * T
            sh = []
            for j in range(km):
                g_lo, g_hi = (j * T) // cq, ((j + 1) * T - 1) // cq
                assert g_hi - g_lo <= 1
                v = t_scr[base + shifts[g_lo]:base + shifts[g_lo] + T, _tile(j)]
                if g_hi != g_lo:
                    v2 = t_scr[base + shifts[g_hi]:base + shifts[g_hi] + T, _tile(j)]
                    v = jnp.where(lane < g_hi * cq - j * T, v, v2)
                sh.append(v)
            hs = square([v.astype(BF16) for v in sh], [split_ops(sh[k], sh[2 + k]) for k in range(2)],
                        w2_ref, ws12.at[1])
            hs = jnp.concatenate([hs[n] for n in range(km)], axis=1)
            y1.append(hs + hb_scr[pl.ds(pl.multiple_of(r0 + hf * T, T), T), :])
            a3.append({})

            def ln_item(hf, c):
                def item(dep):
                    n = HT // NLN
                    for d in (0, HT):
                        v = y1[hf][d + c * n:d + (c + 1) * n]
                        if dep is not None:
                            v = jnp.concatenate([_after(v[:, :T], _rows(dep, n)), v[:, T:]], axis=1)
                        a3[hf][d + c * n] = _ln(v)
                return item

            ln_item(hf, 0)(None)
            pace += [(now[0] + LN0 + (c - 1) * LNS * (1 + hf), ln_item(hf, c)) for c in range(1, NLN)]
            pace.sort(key=lambda e: e[0])
        nf = FH // T
        h3, h3ops = [], []
        for hf in range(nh):
            assert len(a3[hf]) == 2 * NLN
            af = jnp.concatenate([a3[hf][key] for key in sorted(a3[hf])], axis=0)
            full = [af[:, _tile(j)].astype(BF16) for j in range(km)]
            aops = [split_ops(af[:, _tile(k)], af[:, _tile(2 + k)]) for k in range(2)]
            row, ops = {}, []
            narrow = None
            for n in range(nf):
                lo, hi = two_tiles(aops, lambda i, k: _ld(ws3, n, i, k),
                                   (full[4:], [wt(w3_ref, *ftiles[n], 4)],
                                    [wt(w3_ref, *ftiles[nf + n], 4)], _dot_nt))
                lo, hi = _gelu(lo), _gelu(hi)
                row[n], row[nf + n] = lo.astype(BF16), hi.astype(BF16)
                ops.append(split_ops(lo, hi))
                if n < km:
                    v = mm([wt(w3_ref, *ftiles[-1], n)], [full[n]], _dot_nt)
                    narrow = v if narrow is None else v + narrow
            row[2 * nf] = _gelu(mm(full, [wt(w3_ref, *ftiles[2 * nf], j) for j in range(km)],
                                   _dot_nt)).astype(BF16)
            fw = Fd - ftiles[-1][0]
            gT = jnp.concatenate([_gelu(narrow), jnp.zeros((T - fw, T), F32)], axis=0)
            row[2 * nf + 1] = _tie(gT.astype(BF16).T, gT[0:8, :])[:, :fw]
            h3.append([row[i] for i in range(len(ftiles))])
            h3ops.append(ops)
        for hf in range(nh):
            rows = pl.ds(pl.multiple_of(r0 + hf * T, T), T)

            def finish(n, v):
                out_buf[rows, _tile(n)] = (
                    x1_scr[rows, _tile(n)] + gb[:, _tile(n)] * (v + y1[hf][:, _tile(n)])
                ).astype(out_buf.dtype)

            w4t = lambda n, f_: [wt(w4_ref, f0, f1, n) for f0, f1 in f_]
            finish(4, mm(h3[hf], w4t(4, ftiles)))
            for n in range(2):
                lo, hi = two_tiles(h3ops[hf], lambda i, k: _ld(ws4, i, n, slice(k * HT, (k + 1) * HT)),
                                   (h3[hf][2 * nf:], w4t(n, ftiles[2 * nf:]), w4t(n + 2, ftiles[2 * nf:]), _dot))
                finish(n, lo)
                finish(n + 2, hi)
            out_copy(r * nh + hf).start()
        assert not pace
        return carry

    jax.lax.fori_loop(0, nrb, b_body, 0)
    for i in range(nb):
        out_copy(i).wait()


@jax.jit
def pallas_adaLN_cond__compressed_kv_cla__mixer_s_mlp__prompt_kernel(
    A_x: jax.Array,
    A_c_kv: jax.Array,
    A_w_q: jax.Array,
    A_w_uk: jax.Array,
    A_w_uv: jax.Array,
    A_w_o: jax.Array,
    B_x: jax.Array,
    B_w1: jax.Array,
    B_w2: jax.Array,
    B_w3: jax.Array,
    B_w4: jax.Array,
    c: jax.Array,
    w_mod: jax.Array,
):
    _, S, M = A_x.shape
    Dc = A_c_kv.shape[2]
    H, D = A_w_q.shape[1], A_w_q.shape[2]
    Fd = B_w3.shape[1]
    assert D == T and A_c_kv.shape[1] == S and Dc == 4 * T and M == 5 * T and 13 * T < Fd < 14 * T and S == 16 * T
    vmem = pltpu.VMEM
    packed = lambda *lead: vmem(lead + (T // 2, T), U32)
    out = pl.pallas_call(
        _kernel,
        in_specs=[pl.BlockSpec(memory_space=pltpu.HBM)] * 12,
        out_specs=pl.BlockSpec(memory_space=pltpu.HBM),
        out_shape=jax.ShapeDtypeStruct((S, M), A_x.dtype),
        scratch_shapes=[
            vmem((S + 16, M), BF16),
            vmem((S, Dc), BF16),
            vmem((1, M), BF16),
            vmem((M, 2 * M), BF16),
            vmem((M, 4 * M), BF16),
            vmem((M, M), BF16),
            vmem((M, M), BF16),
            vmem((Fd, M), BF16),
            vmem((Fd, M), BF16),
            vmem((M, D), U32),
            vmem((Dc, D), U32),
            vmem((Dc, D), U32),
            vmem((2 * D, M), BF16),
            vmem((S, M), A_x.dtype),
            pltpu.SemaphoreType.DMA((15,)),
            pltpu.SemaphoreType.DMA((4,)),
            pltpu.SemaphoreType.DMA((S // T,)),
            vmem((8, 6 * M), F32),
            vmem((S // T, M // T, T, T), BF16),
            vmem((len(_C_SUMS), T, T), BF16),
            vmem((len(_H_SUMS), T, T), BF16),
            packed(2, M // T + 2 * (Dc // T)),
            packed(2 * S // T),
            packed(2 * S // T),
            packed(2 * S // T),
            vmem((S + 16, M), F32),
            vmem((S + 16, M), F32),
            vmem((S + 16, M), F32),
            vmem((RB, M), F32),
            vmem((RB + 32, M), F32),
            vmem((2, 7, 2, T, T), U32),
            packed(6, 7, 2),
            vmem((7, 2, 3 * T, T), U32),
        ],
        compiler_params=pltpu.CompilerParams(
            vmem_limit_bytes=100 * 1024 * 1024,
            disable_bounds_checks=True,
        ),
    )(
        A_x.reshape(S, M), A_c_kv.reshape(S, Dc),
        A_w_q, A_w_uk, A_w_uv,
        A_w_o.reshape(H // 2, 2 * D, M),
        B_w1, B_w2, B_w3.T, B_w4, c, w_mod,
    )
    return out.reshape(1, S, M)
```

```python
import math

import jax
import jax.numpy as jnp
import jax.experimental.pallas as pl
import jax.experimental.pallas.tpu as pltpu

F32 = jnp.float32
BF16 = jnp.bfloat16
U32 = jnp.uint32
NT = (((1,), (1,)), ((), ()))
T = 128
EPS = 1e-5
LOG2E = math.log2(math.e)

GRP = 4
LEAD = 10
PROW = 3
RES = 32
LAT_A = 16
LAT_B = 20
ALEAD = 32
MID = 40
SD0, SDS = 60, 4
RB = 256
PC = 32
P0, PSTEP, PD = 440, 30, 52
NLN, LN0, LNS = 4, 4, 5
LP = 16
PROLOGUE = ('|kva|Z; |b|; kva|wc|K0123; bw|xdn|C0@56 N0123@52 K4567; cx|mq|N4567@52 K89ab; '
            'd|y|C1@56 Kcdef; nmq|zo|M H01 H234567@30 Q0123; y||H89ab@30 Q4567; '
            'z||Hcdef@30 Q89ab S01 Qcdef; o||')


def _dot(a, b):
    return jnp.dot(a, b, preferred_element_type=F32)


def _dot_nt(a, b):
    return jax.lax.dot_general(a, b, NT, preferred_element_type=F32)


def _ln(x):
    m = jnp.mean(x, axis=-1, keepdims=True)
    xc = x - m
    v = jnp.mean(xc * xc, axis=-1, keepdims=True)
    return xc * jnp.exp2(jnp.log(v + EPS) * (-0.5 * LOG2E))


def _rows(v, n):
    return jnp.broadcast_to(v[None], (n // 8, 8, v.shape[1])).reshape(n, v.shape[1])


def _gelu(x):
    c0 = math.sqrt(2.0 / math.pi)
    return 0.5 * x * (1.0 + jnp.tanh(c0 * (x + 0.044715 * (x * x * x))))


def _after(x, dep):
    return jnp.where(dep > jnp.inf, dep, x)


def _tie(x, dep):
    xu = pltpu.bitcast(x, U32)
    first = jnp.where(dep > jnp.inf, jnp.uint32(0), xu[:8])
    return pltpu.bitcast(jnp.concatenate([first, xu[8:]], axis=0), BF16)


def _tile(j):
    return slice(j * T, (j + 1) * T)


def _ld(ref, *idx):
    return pltpu.bitcast(ref[idx], BF16)


def _pk(x):
    return pltpu.bitcast(x, U32)


def _a_ops(a11, a12, a21, a22):
    return [a11 + a22, a21 + a22, a11, a22, a11 + a12, a21 - a11, a12 - a22]


def _b_ops(b11, b12, b21, b22):
    return [b11 + b22, b11, b12 - b22, b21 - b11, b22, b11 + b12, b21 + b22]


def _strassen(prod, col1=None, col2=None):
    m4 = prod(3)
    m2 = prod(1)
    c21 = m2 + m4
    if col1 is not None:
        e11, e21 = col1()
        m4, c21 = m4 + e11, c21 + e21
    m3 = prod(2)
    m5 = prod(4)
    c12 = m3 + m5
    if col2 is not None:
        e12, e22 = col2()
        c12, m3 = c12 + e12, m3 + e22
    m1 = prod(0)
    c11 = prod(6) + (m1 + (m4 - m5))
    c22 = prod(5) + (m1 + (m3 - m2))
    return c11, c12, c21, c22


def _group(rows, cols, pairs):
    xs, ys = dict.fromkeys(x for x, _ in pairs), dict.fromkeys(y for _, y in pairs)
    used = set(xs) | set(ys) | {(x[0], y[1]) for x, y in pairs} | {(y[0], x[1]) for x, y in pairs}
    prods = []
    for n, r in enumerate(rows):
        for i, k in [x for x in xs if x[0] == r]:
            mates = [y for x, y in pairs if x == (i, k)]
            prods.append((((1, i, k),) + tuple((1, i, k2) for _, k2 in mates), ((1, k, 0),),
                          ((1, i, 0), (-1, i, 1))))
            prods.append((((1, i, k),) + tuple((-1, i2, k) for i2, _ in mates), ((1, k, 0), (1, k, 1)),
                          ((1, i, 1),)))
        for i2, k2 in [y for y in ys if y[0] == r]:
            mates = [x for x, y in pairs if y == (i2, k2)]
            prods.append((((1, i2, k2),) + tuple((1, i2, k) for _, k in mates), ((1, k2, 1),),
                          ((1, i2, 1), (-1, i2, 0))))
            prods.append((((1, i2, k2),) + tuple((-1, i, k2) for i, _ in mates), ((1, k2, 0), (1, k2, 1)),
                          ((1, i2, 0),)))
        prods += [(((1, r, k),), ((1, k, h),), ((1, r, h),)) for k in cols if (r, k) not in used for h in (0, 1)]
        for (i, k), (i2, k2) in pairs:
            if r in (i, i2) and i + i2 - r in rows[n + 1:]:
                prods.append((((1, i, k2),), ((1, k2, 0), (-1, k, 0)), ((1, i2, 0), (1, i, 0))))
                prods.append((((1, i2, k), (1, i, k2)), ((1, k, 0), (1, k2, 1)), ((1, i2, 0), (1, i, 1))))
                prods.append((((1, i2, k),), ((1, k, 1), (-1, k2, 1)), ((1, i2, 1), (1, i, 1))))
    return prods


def _all_pairs(xrows, yrows):
    return [((x, a), (y, b)) for a, x in enumerate(xrows) for b, y in enumerate(yrows) if a != b]


_PAIRS65 = [((x[0] + 10, x[1]), (y[0] + 10, y[1])) for x, y in (
    ((0, 1), (1, 0)), ((0, 1), (5, 2)), ((2, 3), (1, 0)), ((2, 3), (3, 1)), ((2, 3), (5, 2)), ((3, 2), (1, 0)),
    ((4, 4), (0, 3)), ((4, 4), (1, 0)), ((4, 4), (3, 1)), ((4, 4), (5, 2)))]
_C_GROUPS = [_group(range(r, r + 8), range(4), _all_pairs(range(r, r + 4), range(r + 4, r + 8))) for r in (0, 8)]
_H_GROUPS = [_group(range(10), range(5), _all_pairs(range(5), range(5, 10))),
             _group(range(10, 16), range(5), _PAIRS65)]
_sum_index = lambda groups: {f: n for n, f in enumerate(
    dict.fromkeys(t[0] for g in groups for t in g if len(t[0]) > 1))}
_C_SUMS, _H_SUMS = _sum_index(_C_GROUPS), _sum_index(_H_GROUPS)


def _form(form, get):
    acc = None
    for sign, i, j in form:
        v = get(i, j)
        acc = v if acc is None else (acc + v if sign > 0 else acc - v)
    return acc


class _PairWeights:
    def __init__(self, w_ref, transpose=False, shift=None):
        self.base = {}
        if shift is not None:
            fac = _rows(pltpu.bitcast(0x3F800000 + shift, F32), T)
            self.inv = pltpu.bitcast(0x3F800000 - shift, F32)
        for j in range(w_ref.shape[0] // T):
            wu = w_ref[_tile(j), :]
            if transpose:
                wu = wu.T
            hi = pltpu.bitcast(wu & jnp.uint32(0xFFFF0000), F32)
            self.base[j, 0] = pltpu.bitcast(wu << 16, F32)
            self.base[j, 1] = hi if shift is None else hi * fac
        self.cache = {}

    def __call__(self, form):
        sign = 1
        if form[-1][0] < 0 and form[0][1:] > form[1][1:]:
            sign, form = -1, ((1,) + form[1][1:], (-1,) + form[0][1:])
        if form not in self.cache:
            self.cache[form] = _form(form, lambda k, h: self.base[k, h]).astype(BF16)
        return sign, self.cache[form]


def _run_group(jobs, prods, a_get, w, transposed, finish):
    left = {}
    for _, _, outs in prods:
        for _, i, h in outs:
            left[i, h] = left.get((i, h), 0) + 1
    acc = {}
    for af, bf, outs in prods:
        sign, wt = w(bf)
        m = jobs.mm([wt], [a_get(af)], _dot_nt) if transposed else jobs.mm([a_get(af)], [wt], _dot)
        for s_, i, h in outs:
            if (i, h) not in acc:
                acc[i, h] = (s_ * sign, m)
            else:
                s0, v = acc[i, h]
                acc[i, h] = (s0, v + m if s0 == s_ * sign else v - m) if s0 > 0 or s_ * sign < 0 else (1, m - v)
            left[i, h] -= 1
            if not left[i, h]:
                s0, v = acc.pop((i, h))
                assert s0 > 0
                finish(2 * i + h, v)


class _Jobs:
    def __init__(self, side=()):
        self.res = []
        self.side = list(side)

    def mm(self, lhs, wt, dot):
        acc = None
        for x, w in zip(lhs, wt):
            v = dot(x, w)
            self.res.append(v)
            acc = v if acc is None else v + acc
            rel = 4 * (len(self.res) % 4)
            while self.side and self.side[0][0] <= len(self.res):
                self.side.pop(0)[1](v[8 * rel:8 * rel + 8, :])
                rel = (rel + 2) % 16
        return acc


def _proj_step(h_scr, hs_scr, c_ref, cs_scr, wq_ref, wuk_ref, wuv_ref, q_scr, k_scr, v_scr, scale, shifts, side):
    wk, wvT, wq = [_PairWeights(w, n == 1, shifts[n]) for n, w in enumerate((wuk_ref, wuv_ref, wq_ref))]
    c_get = lambda f: cs_scr[_C_SUMS[f]] if len(f) > 1 else c_ref[_tile(f[0][1]), _tile(f[0][2])]
    h_get = lambda f: hs_scr[_H_SUMS[f]] if len(f) > 1 else h_scr[f[0][1], f[0][2]]

    def put(dst, w, mul=None):
        muls = [mul, _rows(w.inv if mul is None else w.inv * mul, T)]

        def fn(u, v):
            dst[u] = _pk((v if muls[u % 2] is None else v * muls[u % 2]).astype(BF16))
        return fn

    jobs = _Jobs(side)
    for groups, get, w, transposed, fin in ((_C_GROUPS, c_get, wk, False, put(k_scr, wk)),
                                            (_C_GROUPS, c_get, wvT, True, put(v_scr, wvT)),
                                            (_H_GROUPS, h_get, wq, False, put(q_scr, wq, scale))):
        for prods in groups:
            _run_group(jobs, prods, get, w, transposed, fin)
    assert not jobs.side


def _inner_group(rows, cols, pairs):
    xs, ys = dict.fromkeys(x for x, _ in pairs), dict.fromkeys(y for _, y in pairs)
    used = set(xs) | set(ys) | {(x[0], y[1]) for x, y in pairs} | {(y[0], x[1]) for x, y in pairs}
    prods = []
    for i, j in xs:
        mates = [y for x, y in pairs if x == (i, j)]
        prods.append((((1, i, 0),), ((1, 0, j), (-1, 1, j)), ((1, i, j),) + tuple((1, i2, j) for i2, _ in mates)))
        prods.append((((1, i, 0), (1, i, 1)), ((1, 1, j),), ((1, i, j),) + tuple((-1, i, j2) for _, j2 in mates)))
    for i2, j2 in ys:
        mates = [x for x, y in pairs if y == (i2, j2)]
        prods.append((((1, i2, 0), (1, i2, 1)), ((1, 0, j2),),
                      ((1, i2, j2),) + tuple((-1, i2, j) for _, j in mates)))
        prods.append((((1, i2, 1),), ((1, 0, j2), (-1, 1, j2)),
                      ((-1, i2, j2),) + tuple((-1, i, j2) for i, _ in mates)))
    prods += [(((1, i, h),), ((1, h, j),), ((1, i, j),))
              for i in rows for j in cols if (i, j) not in used for h in (0, 1)]
    for (i, j), (i2, j2) in pairs:
        lo, hi = min(j, j2), max(j, j2)
        prods.append((((1, i2, 0), (-1, i, 0)), ((1, 0, lo), (1, 0, hi)), ((1, i2, j),)))
        prods.append((((1, i, 0), (1, i2, 1)), ((1, 0, j2), (1, 1, j)), ((1, i, j2), (1, i2, j))))
        prods.append((((1, i, 1), (-1, i2, 1)), ((1, 1, lo), (1, 1, hi)), ((1, i, j2),)))
    return prods


def _o_jobs():
    prods = (_inner_group(range(10), range(5), _all_pairs(range(0, 10, 2), range(1, 10, 2)))
             + _inner_group(range(10, 16), range(5), _PAIRS65))
    row = lambda t: max(i for _, i, _ in t[0])
    unit = lambda t: max(2 * i + h for _, i, h in t[0])
    need = lambda t: unit(t) if row(t) == 15 else 2 * row(t) + 1
    return [(need(t), t) for t in sorted(prods, key=need)]


_O_JOBS = _o_jobs()


def _job_order(nb):
    units = range(2 * nb)
    qa = [('a', u, c) for u in units for c in range(u // 2 + 1)]
    qb = [('b', u, c) for u in units for c in range(u // 2 + 1)]
    qo = [('o', u, j) for j, (u, _) in enumerate(_O_JOBS)]
    done = {}
    order = []

    def ready(q, lat, pre):
        return bool(q) and (pre, q[0][1]) in done and done[(pre, q[0][1])] + lat <= len(order)

    def emit(q):
        kind, u, j = job = q.pop(0)
        if kind != 'o' and j == u // 2:
            done[(kind, u)] = len(order)
        order.append(job)

    turn = 0
    while qa or qb or qo:
        pref = 'abo'[turn % 3]
        turn += 1
        for _ in range(GRP):
            b_ok, o_ok = ready(qb, LAT_A, 'a'), ready(qo, LAT_B, 'b')
            if pref == 'a' and qa and (len(qb) - len(qa) < ALEAD or not b_ok):
                emit(qa)
            elif pref == 'b' and b_ok:
                emit(qb)
            elif pref == 'o' and o_ok and (len(qo) > RES or not (qa or b_ok)):
                emit(qo)
            elif not (qa or b_ok or o_ok) and (qb or qo):
                emit(qb or qo)
            else:
                break
    return order


def _attention_step(q_scr, k_scr, v_scr, wo_ref, acc_scr, mid):
    causal = (jax.lax.broadcasted_iota(jnp.int32, (T, T), 0)
              <= jax.lax.broadcasted_iota(jnp.int32, (T, T), 1))
    sv, mx, mfin, lsum, pv, of, lhs = {}, {}, {}, {}, {}, {}, {}
    res = []
    wo, terms = {}, {}
    left = {}
    for _, t in _O_JOBS:
        for _, i, j in t[2]:
            left[i, j] = left.get((i, j), 0) + 1

    def job_a(u, c):
        r, hd = divmod(u, 2)
        s = _dot_nt(_ld(k_scr, 2 * c + hd), _ld(q_scr, u))
        res.append(s)
        if c == r:
            s = jnp.where(causal, s, -1e9 * LOG2E)
        s = s.reshape(T // 8, 8, T)
        sv[(u, c)] = s
        pm = jnp.max(s, axis=0)
        mx[u] = pm if u not in mx else jnp.maximum(mx[u], pm)

    def job_b(u, c):
        r, hd = divmod(u, 2)
        if u not in mfin:
            mfin[u] = jnp.broadcast_to(jnp.max(mx[u], axis=0, keepdims=True), (8, T))
        m = mfin[u]
        if len(res) >= LEAD:
            r0 = 8 * PROW * (c % 4)
            m = _after(m, res[len(res) - LEAD][r0:r0 + 8, :])
        p = jnp.exp2(sv.pop((u, c)) - m[None])
        ls = jnp.sum(p, axis=0)
        lsum[u] = ls if u not in lsum else lsum[u] + ls
        v = _dot(_ld(v_scr, 2 * c + hd), p.reshape(T, T).astype(BF16))
        res.append(v)
        pv[u] = v if u not in pv else v + pv[u]
        if c == r:
            of[u] = pv[u] * (1.0 / jnp.sum(lsum[u], axis=0, keepdims=True))

    def job_o(_, n):
        af, bf, outs = _O_JOBS[n][1]
        if af not in lhs:
            v = _form(af, lambda i, h: of[2 * i + h])
            lhs[af] = _tie(v.astype(BF16).T, v[0:8, :])
        if bf not in wo:
            wo[bf] = (wo_ref[_tile(bf[0][1]), _tile(bf[0][2])] if len(bf) == 1 else
                      _form(bf, lambda h, j: wo_ref[_tile(h), _tile(j)].astype(F32)).astype(BF16))
        v = _dot(lhs[af], wo[bf])
        res.append(v)
        for sign, i, j in outs:
            terms.setdefault((i, j), []).append((sign, v))
            if len(terms[i, j]) == left[i, j]:
                tot = acc_scr[_tile(i), _tile(j)]
                for sg, m in terms.pop((i, j)):
                    tot = tot + m if sg > 0 else tot - m
                acc_scr[_tile(i), _tile(j)] = tot

    fns = dict(a=job_a, b=job_b, o=job_o)
    for n, (kind, u, j) in enumerate(_job_order(q_scr.shape[0] // 2)):
        if n == MID:
            mid()
        fns[kind](u, j)


def _kernel(x_hbm, c_hbm, wq_hbm, wuk_hbm, wuv_hbm, wo_hbm, w1_hbm, w2_hbm, w3_hbm, w4_hbm,
            cond_hbm, wmod_hbm, out_hbm,
            x_ref, c_ref, cond_ref, wma_ref, wmb_ref, w1_ref, w2_ref, w3_ref, w4_ref,
            wq_buf, wk_buf, wv_buf, wo_buf, out_buf, sem, wsem, osem,
            mod_scr, h_scr, cs_scr, hs_scr, w_scr, q_scr, k_scr, v_scr, acc_scr, x1_scr, hb_scr, a1_scr, t_scr,
            ws12, ws3, ws4, smp_ref, gap_scr):
    S, M = x_hbm.shape
    D = wq_hbm.shape[2]
    nattn = wo_hbm.shape[0]
    Fd = w4_hbm.shape[0]
    scale = float(D) ** -0.5 * LOG2E
    nb, nrb = S // T, S // RB
    km, kc = M // T, c_hbm.shape[1] // T
    NX = 4
    XR = S // NX
    CB = XR // T

    def pcopies(g):
        return [pltpu.make_async_copy(src.bitcast(U32).at[:, g, :], dst, wsem.at[j])
                for j, (src, dst) in enumerate(((wuk_hbm, wk_buf), (wuv_hbm, wv_buf), (wq_hbm, wq_buf)))]

    def ocopy(g):
        return pltpu.make_async_copy(wo_hbm.at[g], wo_buf, wsem.at[3])

    def chunk_copy(src, dst, i, s0):
        rows = slice(i * XR, (i + 1) * XR)
        return pltpu.make_async_copy(src.at[rows, :], dst.at[rows, :], sem.at[s0 + i])

    cp_cond = pltpu.make_async_copy(cond_hbm, cond_ref, sem.at[0])
    cp_wma = pltpu.make_async_copy(wmod_hbm.at[:, 0:2 * M], wma_ref, sem.at[1])
    cp_late = [pltpu.make_async_copy(src, dst, sem.at[2 + j]) for j, (src, dst) in enumerate((
        (wmod_hbm.at[:, 2 * M:6 * M], wmb_ref), (w1_hbm, w1_ref), (w2_hbm, w2_ref),
        (w3_hbm, w3_ref), (w4_hbm, w4_ref)))]
    cp_late += [pltpu.make_async_copy(src.at[0:smp_ref.shape[1]], smp_ref.at[j], sem.at[15 + j])
                for j, src in enumerate((wuk_hbm, wuv_hbm, wq_hbm))]
    cp_x = [chunk_copy(x_hbm, x_ref, i, 7) for i in range(NX)]
    cp_c = [chunk_copy(c_hbm, c_ref, i, 7 + NX) for i in range(NX)]

    def silu_cond():
        cf = cond_ref[...].astype(F32)
        return jnp.broadcast_to((cf * jax.nn.sigmoid(cf)).astype(BF16), (8, M))

    cp_wk, cp_wv, cp_wq = pcopies(0)
    named = dict(k=cp_wk, v=cp_wv, q=cp_wq, o=ocopy(0), n=cp_cond, m=cp_wma)
    named.update(zip('abcd', cp_c))
    named.update(zip('wxyz', cp_x))
    started, arrived, did = set(), set(), set()

    def zero(r, carry):
        acc_scr[pl.ds(pl.multiple_of(r * T, T), T), :] = jnp.zeros((T, M), F32)
        return carry

    def x_rows(rows, dep):
        xf = x_ref[rows, :].astype(F32)
        if dep is None:
            return xf
        return jnp.concatenate([_after(xf[:, :T], _rows(dep, xf.shape[0])), xf[:, T:]], axis=1)

    def n_item(r, i):
        def fn(dep):
            rows = slice(r * T + i * LP, r * T + (i + 1) * LP)
            x1_scr[rows, :] = _ln(x_rows(rows, dep))
        return fn

    def h_item(r, i, normed):
        def fn(dep):
            rows = slice(i * LP, (i + 1) * LP)
            grows = slice(r * T + i * LP, r * T + (i + 1) * LP)
            sa = mod_scr[:, 0:M]
            if normed and dep is not None:
                sa = jnp.concatenate([_after(sa[:, _tile(j)], dep) for j in range(km)], axis=1)
            hf = ((x1_scr[grows, :] if normed else _ln(x_rows(grows, dep))) * _rows(mod_scr[:, M:2 * M], LP)
                  + _rows(sa, LP))
            for j in range(km):
                h_scr[r, j, rows, :] = hf[:, _tile(j)].astype(BF16)
            for f, n in _H_SUMS.items():
                if all(t[1] == r for t in f):
                    hs_scr[n, rows, :] = _form(f, lambda _, k: hf[:, _tile(k)]).astype(BF16)
            did.add(('h', r, i))
        return fn

    def release(jobs, span, items):
        if span and items:
            jobs.side += [(len(jobs.res) + 1 + i * span // len(items), fn) for i, fn in enumerate(items)]
            jobs.side.sort(key=lambda e: e[0])
        else:
            for fn in items:
                fn(None)

    def sum_items(n, group, index, dst, get, skip_rows):
        forms = [f for f in dict.fromkeys(t[0] for t in group)
                 if len(f) > 1 and not (skip_rows and len({t[1] for t in f}) == 1)]

        def item(f, rows):
            def fn(dep):
                def term(r, k):
                    v = get(r, k, rows).astype(F32)
                    return v if dep is None or (r, k) != f[0][1:] else _after(v, _rows(dep, v.shape[0]))
                dst[index[f], rows, :] = _form(f, term).astype(BF16)
            return fn

        return [item(f, slice(i, i + n)) for i in range(0, T, n) for f in forms]

    h_sums = lambda n, gi: sum_items(n, _H_GROUPS[gi], _H_SUMS, hs_scr,
                                     lambda r_, k, rows: h_scr[r_, k, rows, :], True)

    def stash(key, buf, j0, transpose=False):
        n = buf.shape[0] // T
        if key not in did:
            assert key in arrived
            did.add(key)
            w = _PairWeights(buf, transpose)
            for j in range(n):
                for hd in range(2):
                    w_scr[hd, j0 + j] = _pk(w(((1, j, hd),))[1])
        return lambda hd: [_ld(w_scr, hd, j0 + j) for j in range(n)]

    def kv_tile(jobs, r):
        wk, wvT = stash('k', wk_buf, 0), stash('v', wv_buf, kc, True)
        ct = [c_ref[_tile(r), _tile(j)] for j in range(kc)]
        for hd in range(2):
            k_scr[2 * r + hd] = _pk(jobs.mm(ct, wk(hd), _dot).astype(BF16))
        for hd in range(2):
            v_scr[2 * r + hd] = _pk(jobs.mm(wvT(hd), ct, _dot_nt).astype(BF16))

    def q_tile(jobs, r):
        wq = stash('q', wq_buf, 2 * kc)
        ht = [h_scr[r, j] for j in range(km)]
        for hd in range(2):
            q_scr[2 * r + hd] = _pk((jobs.mm(ht, wq(hd), _dot) * scale).astype(BF16))

    for blk in PROLOGUE.split(';'):
        waits, starts, acts = blk.split('|')
        for ch in waits.strip():
            assert ch in started and ch not in arrived
            arrived.add(ch)
            named[ch].wait()
        for ch in starts.strip():
            assert ch not in started
            started.add(ch)
            named[ch].start()
        jobs = _Jobs()
        for act in acts.split():
            if act == 'Z':
                jax.lax.fori_loop(0, nb, zero, 0)
                acc_scr[S:, :] = jnp.zeros((acc_scr.shape[0] - S, M), F32)
                x_ref[S:, :] = jnp.zeros((x_ref.shape[0] - S, M), BF16)
            elif act == 'M':
                assert arrived >= set('nm')
                mod = _dot(silu_cond(), wma_ref[...])
                mod_scr[:, 0:M] = mod[:, 0:M]
                mod_scr[:, M:2 * M] = 1.0 + mod[:, M:2 * M]
                did.add('M')
            else:
                act, _, span = act.partition('@')
                span = int(span or 0)
                items = []
                for r in [int(ch, 16) for ch in act[1:]]:
                    did.add((act[0], r))
                    if act[0] == 'K':
                        assert 'abcd'[r // CB] in arrived
                        kv_tile(jobs, r)
                    elif act[0] == 'H':
                        assert 'wxyz'[r // CB] in arrived and 'M' in did
                        items += [h_item(r, i, ('N', r) in did) for i in range(T // LP)]
                    elif act[0] == 'N':
                        assert 'wxyz'[r // CB] in arrived
                        items += [n_item(r, i) for i in range(T // LP)]
                    elif act[0] == 'Q':
                        assert all(('h', r, i) in did for i in range(T // LP))
                        q_tile(jobs, r)
                    elif act[0] == 'C':
                        assert all('abcd'[t[1] // CB] in arrived for p_ in _C_GROUPS[r] for t in p_[0])
                        items += sum_items(
                            32, _C_GROUPS[r], _C_SUMS, cs_scr,
                            lambda r_, k, rows: c_ref[r_ * T + rows.start:r_ * T + rows.stop, _tile(k)], False)
                    else:
                        assert act[0] == 'S' and all(('h', t[1], T // LP - 1) in did for p_ in _H_GROUPS[r] for t in p_[0])
                        items += h_sums(32 if span else 16, r)
                release(jobs, span, items)
        assert not jobs.side
    assert arrived == set(named) and all((k_, r) in did for k_ in 'KHQ' for r in range(nb))
    assert all((k_, r) in did for k_ in 'CS' for r in range(2))
    for cp in cp_late[1:] + cp_late[:1]:
        cp.start()

    FH = ws3.shape[0] * T
    assert nattn - 1 >= FH // 64

    def mixer_prep(g):
        def blocks(w_ref, r0, n, half, c0, c1, dep):
            lo, hi = pl.ds(r0, n), pl.ds(r0 + half, n)
            return [_after(w_ref[rows, _tile(c)].astype(F32), _rows(dep, n)) if (rows is lo) == (c == c0)
                    else w_ref[rows, _tile(c)].astype(F32) for rows in (lo, hi) for c in (c0, c1)]

        def rows_items(w_ref, dst, per_step, half, n=16):
            gi = jnp.minimum(g, half // per_step - 1)
            src = w_ref.at[pl.ds(pl.multiple_of(gi * per_step, per_step), half + per_step), :]
            hs = per_step // 2

            def item(c, o):
                def fn(dep):
                    for i, v in enumerate(_b_ops(*blocks(src, o, n, half, c, c + 2, dep))):
                        dst[i, c, pl.ds(pl.multiple_of(gi * hs, hs) + o // 2, n // 2), :] = _pk(v.astype(BF16))
                return fn
            return [item(c, o) for c in range(2) for o in range(0, per_step, n)]

        def w3_item(k, i):
            def fn(dep):
                n = jnp.minimum(g, FH // T - 1)
                b11, b21, b12, b22 = blocks(w3_ref, pl.multiple_of(n * T, T), T, FH, k, k + 2, dep)
                ws3[n, i, k] = _pk(_b_ops(b11, b12, b21, b22)[i].astype(BF16).T)
            return fn

        return (rows_items(w1_ref, ws12.at[0], 32, 2 * T) + rows_items(w2_ref, ws12.at[1], 32, 2 * T)
                + rows_items(w4_ref, ws4, 64, FH) + [w3_item(k, i) for k in range(2) for i in range(7)])

    def attn_body(g, carry):
        copies = pcopies(jnp.minimum(g + 1, nattn - 1))

        def mid():
            for cp in copies:
                cp.start()

        _attention_step(q_scr, k_scr, v_scr, wo_buf, acc_scr, mid)
        for cp in copies:
            cp.wait()

        @pl.when(g == 0)
        def _():
            for cp in cp_late[1:]:
                cp.wait()
            for j in range(3):
                l1 = jnp.sum(jnp.sum(jnp.abs(smp_ref[j].astype(F32)), axis=0), axis=1, keepdims=True)
                e = pltpu.bitcast(jnp.broadcast_to(l1, (2 * nattn, T)), jnp.int32) >> 8
                for n in range(nattn):
                    d = (e[2 * n:2 * n + 1] - e[2 * n + 1:2 * n + 2] + (1 << 14)) >> 15
                    d = jnp.clip(d, -16, 16) << 23
                    gap_scr[n, j] = jnp.broadcast_to(d, (8, T))

        @pl.when(g + 1 < nattn)
        def _():
            ocopy(g + 1).start()
            side = [(SD0 + i * SDS, fn) for i, fn in enumerate(mixer_prep(g))]
            _proj_step(h_scr, hs_scr, c_ref, cs_scr, wq_buf, wk_buf, wv_buf, q_scr, k_scr, v_scr, scale,
                       gap_scr.at[g + 1], side)
            ocopy(g + 1).wait()

        return carry

    jax.lax.fori_loop(0, nattn, attn_body, 0)

    cp_late[0].wait()
    mod = _dot(silu_cond(), wmb_ref[...])
    mod_scr[:, 2 * M:4 * M] = mod[:, 0:2 * M]
    mod_scr[:, 4 * M:5 * M] = 1.0 + mod[:, 2 * M:3 * M]
    mod_scr[:, 5 * M:6 * M] = mod[:, 3 * M:4 * M]
    ftiles = [(f, min(f + T, Fd)) for f in range(0, Fd, T)]
    OFF = x_ref.shape[0] - S
    CAR = t_scr.shape[0] - RB

    def p1(r0, n, dep=None):
        ga = mod_scr[:, 2 * M:3 * M]
        if dep is not None:
            ga = jnp.concatenate([_after(ga[:, 0:T], dep), ga[:, T:]], axis=1)
        rows = pl.ds(r0, n)
        x1 = x_ref[rows, :].astype(F32) + _rows(ga, n) * acc_scr[rows, :]
        x1_scr[rows, :] = x1
        hb = _ln(x1) * _rows(mod_scr[:, 4 * M:5 * M], n) + _rows(mod_scr[:, 3 * M:4 * M], n)
        hb_scr[rows, :] = hb
        return _ln(hb)

    HT = T // 2

    def p1_store(r0, c, dep=None):
        v = p1(r0 + c * PC, PC, dep)
        a1_scr[c * PC:(c + 1) * PC, :] = v
        return jnp.max(v[:, M - T:].reshape(PC // 8, 8, T), axis=0)

    t_scr[RB:RB + CAR - OFF, :] = jnp.zeros((CAR - OFF, M), F32)
    t_scr[RB + CAR - OFF:RB + CAR, :] = _gelu(_dot(p1(0, OFF).astype(BF16), w1_ref[...]))
    for c in range(RB // PC):
        p1_store(OFF, c)

    def out_copy(i):
        rows = pl.ds(i * T if isinstance(i, int) else pl.multiple_of(i * T, T), T)
        return pltpu.make_async_copy(out_buf.at[rows, :], out_hbm.at[rows, :], osem.at[i])

    def b_body(r, carry):
        gb = _rows(mod_scr[:, 5 * M:6 * M], T)
        r0 = pl.multiple_of(r * RB, RB)
        n0 = pl.multiple_of(jnp.minimum(r0 + RB, S - RB) + OFF, OFF)
        nh = RB // T
        now = [0]
        due = []
        pace = []

        def p1_item(c):
            return lambda dep: due.append((now[0] + PD, p1_store(n0, c, dep)))

        pace += [(P0 + i * PSTEP, p1_item(i)) for i in range(RB // PC)]
        wt = lambda ref, f0, f1, n: ref[f0:f1, _tile(n)]

        def mm(lhs, wts, dot=_dot):
            acc = None
            for x, w in zip(lhs, wts):
                if due and due[0][0] <= now[0]:
                    w = _tie(w, due.pop(0)[1])
                v = dot(x, w)
                now[0] += x.shape[0] // HT
                acc = v if acc is None else v + acc
                if pace and pace[0][0] <= now[0]:
                    pace.pop(0)[1](v[0:8, :])
            return acc

        def split_ops(lo, hi):
            return [v.astype(BF16) for v in _a_ops(lo[:HT], hi[:HT], lo[HT:], hi[HT:])]

        def two_tiles(aops, wsel, rest):
            def col(w):
                v = mm(rest[0], w, rest[3])
                return v[:HT], v[HT:]

            c11, c12, c21, c22 = _strassen(
                lambda i: mm([a[i] for a in aops], [wsel(i, k) for k in range(len(aops))]),
                lambda: col(rest[1]), lambda: col(rest[2]))
            return jnp.concatenate([c11, c21], axis=0), jnp.concatenate([c12, c22], axis=0)

        def square(full, aops, w_ref, ws_ref):
            out = {}
            for n in range(2):
                out[n], out[n + 2] = two_tiles(
                    aops, lambda i, k: _ld(ws_ref, i, n, slice(k * HT, (k + 1) * HT)),
                    (full[4:], [wt(w_ref, 4 * T, M, n)], [wt(w_ref, 4 * T, M, n + 2)], _dot))
            out[4] = mm(full, [wt(w_ref, j * T, (j + 1) * T, 4) for j in range(km)])
            return out

        t_scr[0:CAR, :] = t_scr[RB:RB + CAR, :]
        for hf in range(nh):
            a1 = [a1_scr[_tile(hf), _tile(j)] for j in range(km)]
            full = [v.astype(BF16) for v in a1]
            aops = [split_ops(a1[k], a1[2 + k]) for k in range(2)]
            for n, v in square(full, aops, w1_ref, ws12.at[0]).items():
                t = _gelu(v)
                if hf == nh - 1:
                    t = jnp.concatenate([t[:T - OFF], jnp.where(r < nrb - 1, t[T - OFF:], 0.0)], axis=0)
                t_scr[CAR + hf * T:CAR + (hf + 1) * T, _tile(n)] = t
        cq = M // 4
        shifts = (-1, 1, -2, 2)
        lane = jax.lax.broadcasted_iota(jnp.int32, (T, T), 1)
        y1, a3 = [], []
        for hf in range(nh):
            base = CAR - OFF + hf * T
            sh = []
            for j in range(km):
                g_lo, g_hi = (j * T) // cq, ((j + 1) * T - 1) // cq
                assert g_hi - g_lo <= 1
                v = t_scr[base + shifts[g_lo]:base + shifts[g_lo] + T, _tile(j)]
                if g_hi != g_lo:
                    v2 = t_scr[base + shifts[g_hi]:base + shifts[g_hi] + T, _tile(j)]
                    v = jnp.where(lane < g_hi * cq - j * T, v, v2)
                sh.append(v)
            hs = square([v.astype(BF16) for v in sh], [split_ops(sh[k], sh[2 + k]) for k in range(2)],
                        w2_ref, ws12.at[1])
            hs = jnp.concatenate([hs[n] for n in range(km)], axis=1)
            y1.append(hs + hb_scr[pl.ds(pl.multiple_of(r0 + hf * T, T), T), :])
            a3.append({})

            def ln_item(hf, c):
                def item(dep):
                    n = HT // NLN
                    for d in (0, HT):
                        v = y1[hf][d + c * n:d + (c + 1) * n]
                        if dep is not None:
                            v = jnp.concatenate([_after(v[:, :T], _rows(dep, n)), v[:, T:]], axis=1)
                        a3[hf][d + c * n] = _ln(v)
                return item

            ln_item(hf, 0)(None)
            pace += [(now[0] + LN0 + (c - 1) * LNS * (1 + hf), ln_item(hf, c)) for c in range(1, NLN)]
            pace.sort(key=lambda e: e[0])
        nf = FH // T
        h3, h3ops = [], []
        for hf in range(nh):
            assert len(a3[hf]) == 2 * NLN
            af = jnp.concatenate([a3[hf][key] for key in sorted(a3[hf])], axis=0)
            full = [af[:, _tile(j)].astype(BF16) for j in range(km)]
            aops = [split_ops(af[:, _tile(k)], af[:, _tile(2 + k)]) for k in range(2)]
            row, ops = {}, []
            narrow = None
            for n in range(nf):
                lo, hi = two_tiles(aops, lambda i, k: _ld(ws3, n, i, k),
                                   (full[4:], [wt(w3_ref, *ftiles[n], 4)],
                                    [wt(w3_ref, *ftiles[nf + n], 4)], _dot_nt))
                lo, hi = _gelu(lo), _gelu(hi)
                row[n], row[nf + n] = lo.astype(BF16), hi.astype(BF16)
                ops.append(split_ops(lo, hi))
                if n < km:
                    v = mm([wt(w3_ref, *ftiles[-1], n)], [full[n]], _dot_nt)
                    narrow = v if narrow is None else v + narrow
            row[2 * nf] = _gelu(mm(full, [wt(w3_ref, *ftiles[2 * nf], j) for j in range(km)],
                                   _dot_nt)).astype(BF16)
            fw = Fd - ftiles[-1][0]
            gT = jnp.concatenate([_gelu(narrow), jnp.zeros((T - fw, T), F32)], axis=0)
            row[2 * nf + 1] = _tie(gT.astype(BF16).T, gT[0:8, :])[:, :fw]
            h3.append([row[i] for i in range(len(ftiles))])
            h3ops.append(ops)
        for hf in range(nh):
            rows = pl.ds(pl.multiple_of(r0 + hf * T, T), T)

            def finish(n, v):
                out_buf[rows, _tile(n)] = (
                    x1_scr[rows, _tile(n)] + gb[:, _tile(n)] * (v + y1[hf][:, _tile(n)])
                ).astype(out_buf.dtype)

            w4t = lambda n, f_: [wt(w4_ref, f0, f1, n) for f0, f1 in f_]
            finish(4, mm(h3[hf], w4t(4, ftiles)))
            for n in range(2):
                lo, hi = two_tiles(h3ops[hf], lambda i, k: _ld(ws4, i, n, slice(k * HT, (k + 1) * HT)),
                                   (h3[hf][2 * nf:], w4t(n, ftiles[2 * nf:]), w4t(n + 2, ftiles[2 * nf:]), _dot))
                finish(n, lo)
                finish(n + 2, hi)
            out_copy(r * nh + hf).start()
        assert not pace
        return carry

    jax.lax.fori_loop(0, nrb, b_body, 0)
    for i in range(nb):
        out_copy(i).wait()


@jax.jit
def pallas_adaLN_cond__compressed_kv_cla__mixer_s_mlp__prompt_kernel(
    A_x: jax.Array,
    A_c_kv: jax.Array,
    A_w_q: jax.Array,
    A_w_uk: jax.Array,
    A_w_uv: jax.Array,
    A_w_o: jax.Array,
    B_x: jax.Array,
    B_w1: jax.Array,
    B_w2: jax.Array,
    B_w3: jax.Array,
    B_w4: jax.Array,
    c: jax.Array,
    w_mod: jax.Array,
):
    _, S, M = A_x.shape
    Dc = A_c_kv.shape[2]
    H, D = A_w_q.shape[1], A_w_q.shape[2]
    Fd = B_w3.shape[1]
    assert D == T and A_c_kv.shape[1] == S and Dc == 4 * T and M == 5 * T and 13 * T < Fd < 14 * T and S == 16 * T
    vmem = pltpu.VMEM
    packed = lambda *lead: vmem(lead + (T // 2, T), U32)
    out = pl.pallas_call(
        _kernel,
        in_specs=[pl.BlockSpec(memory_space=pltpu.HBM)] * 12,
        out_specs=pl.BlockSpec(memory_space=pltpu.HBM),
        out_shape=jax.ShapeDtypeStruct((S, M), A_x.dtype),
        scratch_shapes=[
            vmem((S + 16, M), BF16),
            vmem((S, Dc), BF16),
            vmem((1, M), BF16),
            vmem((M, 2 * M), BF16),
            vmem((M, 4 * M), BF16),
            vmem((M, M), BF16),
            vmem((M, M), BF16),
            vmem((Fd, M), BF16),
            vmem((Fd, M), BF16),
            vmem((M, D), U32),
            vmem((Dc, D), U32),
            vmem((Dc, D), U32),
            vmem((2 * D, M), BF16),
            vmem((S, M), A_x.dtype),
            pltpu.SemaphoreType.DMA((18,)),
            pltpu.SemaphoreType.DMA((4,)),
            pltpu.SemaphoreType.DMA((S // T,)),
            vmem((8, 6 * M), F32),
            vmem((S // T, M // T, T, T), BF16),
            vmem((len(_C_SUMS), T, T), BF16),
            vmem((len(_H_SUMS), T, T), BF16),
            packed(2, M // T + 2 * (Dc // T)),
            packed(2 * S // T),
            packed(2 * S // T),
            packed(2 * S // T),
            vmem((S + 16, M), F32),
            vmem((S + 16, M), F32),
            vmem((S + 16, M), F32),
            vmem((RB, M), F32),
            vmem((RB + 32, M), F32),
            vmem((2, 7, 2, T, T), U32),
            packed(6, 7, 2),
            vmem((7, 2, 3 * T, T), U32),
            vmem((3, 8, H, D), BF16),
            vmem((H // 2, 3, 8, T), jnp.int32),
        ],
        compiler_params=pltpu.CompilerParams(
            vmem_limit_bytes=100 * 1024 * 1024,
            disable_bounds_checks=True,
        ),
    )(
        A_x.reshape(S, M), A_c_kv.reshape(S, Dc),
        A_w_q, A_w_uk, A_w_uv,
        A_w_o.reshape(H // 2, 2 * D, M),
        B_w1, B_w2, B_w3.T, B_w4, c, w_mod,
    )
    return out.reshape(1, S, M)
```

```python
import math

import jax
import jax.numpy as jnp
import jax.experimental.pallas as pl
import jax.experimental.pallas.tpu as pltpu

F32 = jnp.float32
BF16 = jnp.bfloat16
U32 = jnp.uint32
NT = (((1,), (1,)), ((), ()))
T = 128
EPS = 1e-5
LOG2E = math.log2(math.e)

GRP = 4
LEAD = 10
PROW = 3
RES = 32
LAT_A = 16
LAT_B = 20
ALEAD = 32
MID = 40
SD0, SDS = 60, 4
RB = 256
PC = 32
P0, PSTEP, PD = 440, 30, 52
NLN, LN0, LNS = 4, 4, 5
LP = 16
PROLOGUE = ('|kva|Z; |b|; kva|wc|K0123; bw|xdn|C0@56 N0123@52 K4567; cx|mq|N4567@52 K89ab; '
            'd|y|C1@56 Kcdef; nmq|zo|M H01 H234567@30 Q0123; y||H89ab@30 Q4567; '
            'zo||L Hcdef@30 Q89ab S01 Qcdef')


def _dot(a, b):
    return jnp.dot(a, b, preferred_element_type=F32)


def _dot_nt(a, b):
    return jax.lax.dot_general(a, b, NT, preferred_element_type=F32)


def _ln(x):
    m = jnp.mean(x, axis=-1, keepdims=True)
    xc = x - m
    v = jnp.mean(xc * xc, axis=-1, keepdims=True)
    return xc * jnp.exp2(jnp.log(v + EPS) * (-0.5 * LOG2E))


def _rows(v, n):
    return jnp.broadcast_to(v[None], (n // 8, 8, v.shape[1])).reshape(n, v.shape[1])


def _gelu(x):
    c0 = math.sqrt(2.0 / math.pi)
    return 0.5 * x * (1.0 + jnp.tanh(c0 * (x + 0.044715 * (x * x * x))))


def _after(x, dep):
    return jnp.where(dep > jnp.inf, dep, x)


def _tie(x, dep):
    xu = pltpu.bitcast(x, U32)
    first = jnp.where(dep > jnp.inf, jnp.uint32(0), xu[:8])
    return pltpu.bitcast(jnp.concatenate([first, xu[8:]], axis=0), BF16)


def _tile(j):
    return slice(j * T, (j + 1) * T)


def _ld(ref, *idx):
    return pltpu.bitcast(ref[idx], BF16)


def _pk(x):
    return pltpu.bitcast(x, U32)


def _a_ops(a11, a12, a21, a22):
    return [a11 + a22, a21 + a22, a11, a22, a11 + a12, a21 - a11, a12 - a22]


def _b_ops(b11, b12, b21, b22):
    return [b11 + b22, b11, b12 - b22, b21 - b11, b22, b11 + b12, b21 + b22]


def _strassen(prod, col1=None, col2=None):
    m4 = prod(3)
    m2 = prod(1)
    c21 = m2 + m4
    if col1 is not None:
        e11, e21 = col1()
        m4, c21 = m4 + e11, c21 + e21
    m3 = prod(2)
    m5 = prod(4)
    c12 = m3 + m5
    if col2 is not None:
        e12, e22 = col2()
        c12, m3 = c12 + e12, m3 + e22
    m1 = prod(0)
    c11 = prod(6) + (m1 + (m4 - m5))
    c22 = prod(5) + (m1 + (m3 - m2))
    return c11, c12, c21, c22


def _group(rows, cols, pairs):
    xs, ys = dict.fromkeys(x for x, _ in pairs), dict.fromkeys(y for _, y in pairs)
    used = set(xs) | set(ys) | {(x[0], y[1]) for x, y in pairs} | {(y[0], x[1]) for x, y in pairs}
    prods = []
    for n, r in enumerate(rows):
        for i, k in [x for x in xs if x[0] == r]:
            mates = [y for x, y in pairs if x == (i, k)]
            prods.append((((1, i, k),) + tuple((1, i, k2) for _, k2 in mates), ((1, k, 0),),
                          ((1, i, 0), (-1, i, 1))))
            prods.append((((1, i, k),) + tuple((-1, i2, k) for i2, _ in mates), ((1, k, 0), (1, k, 1)),
                          ((1, i, 1),)))
        for i2, k2 in [y for y in ys if y[0] == r]:
            mates = [x for x, y in pairs if y == (i2, k2)]
            prods.append((((1, i2, k2),) + tuple((1, i2, k) for _, k in mates), ((1, k2, 1),),
                          ((1, i2, 1), (-1, i2, 0))))
            prods.append((((1, i2, k2),) + tuple((-1, i, k2) for i, _ in mates), ((1, k2, 0), (1, k2, 1)),
                          ((1, i2, 0),)))
        prods += [(((1, r, k),), ((1, k, h),), ((1, r, h),)) for k in cols if (r, k) not in used for h in (0, 1)]
        for (i, k), (i2, k2) in pairs:
            if r in (i, i2) and i + i2 - r in rows[n + 1:]:
                prods.append((((1, i, k2),), ((1, k2, 0), (-1, k, 0)), ((1, i2, 0), (1, i, 0))))
                prods.append((((1, i2, k), (1, i, k2)), ((1, k, 0), (1, k2, 1)), ((1, i2, 0), (1, i, 1))))
                prods.append((((1, i2, k),), ((1, k, 1), (-1, k2, 1)), ((1, i2, 1), (1, i, 1))))
    return prods


def _all_pairs(xrows, yrows):
    return [((x, a), (y, b)) for a, x in enumerate(xrows) for b, y in enumerate(yrows) if a != b]


_PAIRS65 = [((x[0] + 10, x[1]), (y[0] + 10, y[1])) for x, y in (
    ((0, 1), (1, 0)), ((0, 1), (5, 2)), ((2, 3), (1, 0)), ((2, 3), (3, 1)), ((2, 3), (5, 2)), ((3, 2), (1, 0)),
    ((4, 4), (0, 3)), ((4, 4), (1, 0)), ((4, 4), (3, 1)), ((4, 4), (5, 2)))]
_C_GROUPS = [_group(range(r, r + 8), range(4), _all_pairs(range(r, r + 4), range(r + 4, r + 8))) for r in (0, 8)]
_H_GROUPS = [_group(range(10), range(5), _all_pairs(range(5), range(5, 10))),
             _group(range(10, 16), range(5), _PAIRS65)]
_sum_index = lambda groups: {f: n for n, f in enumerate(
    dict.fromkeys(t[0] for g in groups for t in g if len(t[0]) > 1))}
_C_SUMS, _H_SUMS = _sum_index(_C_GROUPS), _sum_index(_H_GROUPS)


def _form(form, get):
    acc = None
    for sign, i, j in form:
        v = get(i, j)
        acc = v if acc is None else (acc + v if sign > 0 else acc - v)
    return acc


class _PairWeights:
    def __init__(self, w_ref, transpose=False, shift=None):
        self.base = {}
        if shift is not None:
            fac = _rows(pltpu.bitcast(0x3F800000 + shift, F32), T)
            self.inv = pltpu.bitcast(0x3F800000 - shift, F32)
        for j in range(w_ref.shape[0] // T):
            wu = w_ref[_tile(j), :]
            if transpose:
                wu = wu.T
            hi = pltpu.bitcast(wu & jnp.uint32(0xFFFF0000), F32)
            self.base[j, 0] = pltpu.bitcast(wu << 16, F32)
            self.base[j, 1] = hi if shift is None else hi * fac
        self.cache = {}

    def __call__(self, form):
        sign = 1
        if form[-1][0] < 0 and form[0][1:] > form[1][1:]:
            sign, form = -1, ((1,) + form[1][1:], (-1,) + form[0][1:])
        if form not in self.cache:
            self.cache[form] = _form(form, lambda k, h: self.base[k, h]).astype(BF16)
        return sign, self.cache[form]


def _run_group(jobs, prods, a_get, w, transposed, finish):
    left = {}
    for _, _, outs in prods:
        for _, i, h in outs:
            left[i, h] = left.get((i, h), 0) + 1
    acc = {}
    for af, bf, outs in prods:
        sign, wt = w(bf)
        m = jobs.mm([wt], [a_get(af)], _dot_nt) if transposed else jobs.mm([a_get(af)], [wt], _dot)
        for s_, i, h in outs:
            if (i, h) not in acc:
                acc[i, h] = (s_ * sign, m)
            else:
                s0, v = acc[i, h]
                acc[i, h] = (s0, v + m if s0 == s_ * sign else v - m) if s0 > 0 or s_ * sign < 0 else (1, m - v)
            left[i, h] -= 1
            if not left[i, h]:
                s0, v = acc.pop((i, h))
                assert s0 > 0
                finish(2 * i + h, v)


class _Jobs:
    def __init__(self, side=()):
        self.res = []
        self.side = list(side)

    def mm(self, lhs, wt, dot):
        acc = None
        for x, w in zip(lhs, wt):
            v = dot(x, w)
            self.res.append(v)
            acc = v if acc is None else v + acc
            rel = 4 * (len(self.res) % 4)
            while self.side and self.side[0][0] <= len(self.res):
                self.side.pop(0)[1](v[8 * rel:8 * rel + 8, :])
                rel = (rel + 2) % 16
        return acc


def _proj_step(h_scr, hs_scr, c_ref, cs_scr, wq_ref, wuk_ref, wuv_ref, q_scr, k_scr, v_scr, scale, shifts, side):
    wk, wvT, wq = [_PairWeights(w, n == 1, shifts[n]) for n, w in enumerate((wuk_ref, wuv_ref, wq_ref))]
    c_get = lambda f: cs_scr[_C_SUMS[f]] if len(f) > 1 else c_ref[_tile(f[0][1]), _tile(f[0][2])]
    h_get = lambda f: hs_scr[_H_SUMS[f]] if len(f) > 1 else h_scr[f[0][1], f[0][2]]

    def put(dst, w, mul=None):
        muls = [mul, _rows(w.inv if mul is None else w.inv * mul, T)]

        def fn(u, v):
            dst[u] = _pk((v if muls[u % 2] is None else v * muls[u % 2]).astype(BF16))
        return fn

    jobs = _Jobs(side)
    for groups, get, w, transposed, fin in ((_C_GROUPS, c_get, wk, False, put(k_scr, wk)),
                                            (_C_GROUPS, c_get, wvT, True, put(v_scr, wvT)),
                                            (_H_GROUPS, h_get, wq, False, put(q_scr, wq, scale))):
        for prods in groups:
            _run_group(jobs, prods, get, w, transposed, fin)
    assert not jobs.side


def _inner_group(rows, cols, pairs):
    xs, ys = dict.fromkeys(x for x, _ in pairs), dict.fromkeys(y for _, y in pairs)
    used = set(xs) | set(ys) | {(x[0], y[1]) for x, y in pairs} | {(y[0], x[1]) for x, y in pairs}
    prods = []
    for i, j in xs:
        mates = [y for x, y in pairs if x == (i, j)]
        prods.append((((1, i, 0),), ((1, 0, j), (-1, 1, j)), ((1, i, j),) + tuple((1, i2, j) for i2, _ in mates)))
        prods.append((((1, i, 0), (1, i, 1)), ((1, 1, j),), ((1, i, j),) + tuple((-1, i, j2) for _, j2 in mates)))
    for i2, j2 in ys:
        mates = [x for x, y in pairs if y == (i2, j2)]
        prods.append((((1, i2, 0), (1, i2, 1)), ((1, 0, j2),),
                      ((1, i2, j2),) + tuple((-1, i2, j) for _, j in mates)))
        prods.append((((1, i2, 1),), ((1, 0, j2), (-1, 1, j2)),
                      ((-1, i2, j2),) + tuple((-1, i, j2) for i, _ in mates)))
    prods += [(((1, i, h),), ((1, h, j),), ((1, i, j),))
              for i in rows for j in cols if (i, j) not in used for h in (0, 1)]
    for (i, j), (i2, j2) in pairs:
        lo, hi = min(j, j2), max(j, j2)
        prods.append((((1, i2, 0), (-1, i, 0)), ((1, 0, lo), (1, 0, hi)), ((1, i2, j),)))
        prods.append((((1, i, 0), (1, i2, 1)), ((1, 0, j2), (1, 1, j)), ((1, i, j2), (1, i2, j))))
        prods.append((((1, i, 1), (-1, i2, 1)), ((1, 1, lo), (1, 1, hi)), ((1, i, j2),)))
    return prods


def _o_jobs():
    prods = (_inner_group(range(10), range(5), _all_pairs(range(0, 10, 2), range(1, 10, 2)))
             + _inner_group(range(10, 16), range(5), _PAIRS65))
    row = lambda t: max(i for _, i, _ in t[0])
    unit = lambda t: max(2 * i + h for _, i, h in t[0])
    need = lambda t: unit(t) if row(t) == 15 else 2 * row(t) + 1
    return [(need(t), t) for t in sorted(prods, key=need)]


_O_JOBS = _o_jobs()


def _job_order(nb):
    units = range(2 * nb)
    qa = [('a', u, c) for u in units for c in range(u // 2 + 1)]
    qb = [('b', u, c) for u in units for c in range(u // 2 + 1)]
    qo = [('o', u, j) for j, (u, _) in enumerate(_O_JOBS)]
    done = {}
    order = []

    def ready(q, lat, pre):
        return bool(q) and (pre, q[0][1]) in done and done[(pre, q[0][1])] + lat <= len(order)

    def emit(q):
        kind, u, j = job = q.pop(0)
        if kind != 'o' and j == u // 2:
            done[(kind, u)] = len(order)
        order.append(job)

    turn = 0
    while qa or qb or qo:
        pref = 'abo'[turn % 3]
        turn += 1
        for _ in range(GRP):
            b_ok, o_ok = ready(qb, LAT_A, 'a'), ready(qo, LAT_B, 'b')
            if pref == 'a' and qa and (len(qb) - len(qa) < ALEAD or not b_ok):
                emit(qa)
            elif pref == 'b' and b_ok:
                emit(qb)
            elif pref == 'o' and o_ok and (len(qo) > RES or not (qa or b_ok)):
                emit(qo)
            elif not (qa or b_ok or o_ok) and (qb or qo):
                emit(qb or qo)
            else:
                break
    return order


def _attention_step(q_scr, k_scr, v_scr, wo_ref, acc_scr, mid):
    causal = (jax.lax.broadcasted_iota(jnp.int32, (T, T), 0)
              <= jax.lax.broadcasted_iota(jnp.int32, (T, T), 1))
    sv, mx, mfin, lsum, pv, of, lhs = {}, {}, {}, {}, {}, {}, {}
    res = []
    wo, terms = {}, {}
    left = {}
    for _, t in _O_JOBS:
        for _, i, j in t[2]:
            left[i, j] = left.get((i, j), 0) + 1

    def job_a(u, c):
        r, hd = divmod(u, 2)
        s = _dot_nt(_ld(k_scr, 2 * c + hd), _ld(q_scr, u))
        res.append(s)
        if c == r:
            s = jnp.where(causal, s, -1e9 * LOG2E)
        s = s.reshape(T // 8, 8, T)
        sv[(u, c)] = s
        pm = jnp.max(s, axis=0)
        mx[u] = pm if u not in mx else jnp.maximum(mx[u], pm)

    def job_b(u, c):
        r, hd = divmod(u, 2)
        if u not in mfin:
            mfin[u] = jnp.broadcast_to(jnp.max(mx[u], axis=0, keepdims=True), (8, T))
        m = mfin[u]
        if len(res) >= LEAD:
            r0 = 8 * PROW * (c % 4)
            m = _after(m, res[len(res) - LEAD][r0:r0 + 8, :])
        p = jnp.exp2(sv.pop((u, c)) - m[None])
        ls = jnp.sum(p, axis=0)
        lsum[u] = ls if u not in lsum else lsum[u] + ls
        v = _dot(_ld(v_scr, 2 * c + hd), p.reshape(T, T).astype(BF16))
        res.append(v)
        pv[u] = v if u not in pv else v + pv[u]
        if c == r:
            of[u] = pv[u] * (1.0 / jnp.sum(lsum[u], axis=0, keepdims=True))

    def job_o(_, n):
        af, bf, outs = _O_JOBS[n][1]
        if af not in lhs:
            v = _form(af, lambda i, h: of[2 * i + h])
            lhs[af] = _tie(v.astype(BF16).T, v[0:8, :])
        if bf not in wo:
            wo[bf] = (wo_ref[_tile(bf[0][1]), _tile(bf[0][2])] if len(bf) == 1 else
                      _form(bf, lambda h, j: wo_ref[_tile(h), _tile(j)].astype(F32)).astype(BF16))
        v = _dot(lhs[af], wo[bf])
        res.append(v)
        for sign, i, j in outs:
            terms.setdefault((i, j), []).append((sign, v))
            if len(terms[i, j]) == left[i, j]:
                tot = acc_scr[_tile(i), _tile(j)]
                for sg, m in terms.pop((i, j)):
                    tot = tot + m if sg > 0 else tot - m
                acc_scr[_tile(i), _tile(j)] = tot

    fns = dict(a=job_a, b=job_b, o=job_o)
    for n, (kind, u, j) in enumerate(_job_order(q_scr.shape[0] // 2)):
        if n == MID:
            mid()
        fns[kind](u, j)


def _kernel(x_hbm, c_hbm, wq_hbm, wuk_hbm, wuv_hbm, wo_hbm, w1_hbm, w2_hbm, w3_hbm, w4_hbm,
            cond_hbm, wmod_hbm, out_hbm,
            x_ref, c_ref, cond_ref, wma_ref, wmb_ref, w1_ref, w2_ref, w3_ref, w4_ref,
            wq_buf, wk_buf, wv_buf, wo_buf, out_buf, sem, wsem, osem,
            mod_scr, h_scr, cs_scr, hs_scr, w_scr, q_scr, k_scr, v_scr, acc_scr, x1_scr, hb_scr, a1_scr, t_scr,
            ws12, ws3, ws4, smp_ref, gap_scr):
    S, M = x_hbm.shape
    D = wq_hbm.shape[2]
    nattn = wo_hbm.shape[0]
    Fd = w4_hbm.shape[0]
    scale = float(D) ** -0.5 * LOG2E
    nb, nrb = S // T, S // RB
    km, kc = M // T, c_hbm.shape[1] // T
    NX = 4
    XR = S // NX
    CB = XR // T

    def pcopies(g):
        return [pltpu.make_async_copy(src.bitcast(U32).at[:, g, :], dst, wsem.at[j])
                for j, (src, dst) in enumerate(((wuk_hbm, wk_buf), (wuv_hbm, wv_buf), (wq_hbm, wq_buf)))]

    def ocopy(g):
        return pltpu.make_async_copy(wo_hbm.at[g], wo_buf, wsem.at[3])

    def chunk_copy(src, dst, i, s0):
        rows = slice(i * XR, (i + 1) * XR)
        return pltpu.make_async_copy(src.at[rows, :], dst.at[rows, :], sem.at[s0 + i])

    cp_cond = pltpu.make_async_copy(cond_hbm, cond_ref, sem.at[0])
    cp_wma = pltpu.make_async_copy(wmod_hbm.at[:, 0:2 * M], wma_ref, sem.at[1])
    cp_late = [pltpu.make_async_copy(src, dst, sem.at[2 + j]) for j, (src, dst) in enumerate((
        (wmod_hbm.at[:, 2 * M:6 * M], wmb_ref), (w1_hbm, w1_ref), (w2_hbm, w2_ref),
        (w3_hbm, w3_ref), (w4_hbm, w4_ref)))]
    cp_late += [pltpu.make_async_copy(src.at[0:smp_ref.shape[1]], smp_ref.at[j], sem.at[15 + j])
                for j, src in enumerate((wuk_hbm, wuv_hbm, wq_hbm))]
    cp_x = [chunk_copy(x_hbm, x_ref, i, 7) for i in range(NX)]
    cp_c = [chunk_copy(c_hbm, c_ref, i, 7 + NX) for i in range(NX)]

    def silu_cond():
        cf = cond_ref[...].astype(F32)
        return jnp.broadcast_to((cf * jax.nn.sigmoid(cf)).astype(BF16), (8, M))

    cp_wk, cp_wv, cp_wq = pcopies(0)
    named = dict(k=cp_wk, v=cp_wv, q=cp_wq, o=ocopy(0), n=cp_cond, m=cp_wma)
    named.update(zip('abcd', cp_c))
    named.update(zip('wxyz', cp_x))
    started, arrived, did = set(), set(), set()

    def zero(r, carry):
        acc_scr[pl.ds(pl.multiple_of(r * T, T), T), :] = jnp.zeros((T, M), F32)
        return carry

    def x_rows(rows, dep):
        xf = x_ref[rows, :].astype(F32)
        if dep is None:
            return xf
        return jnp.concatenate([_after(xf[:, :T], _rows(dep, xf.shape[0])), xf[:, T:]], axis=1)

    def n_item(r, i):
        def fn(dep):
            rows = slice(r * T + i * LP, r * T + (i + 1) * LP)
            x1_scr[rows, :] = _ln(x_rows(rows, dep))
        return fn

    def h_item(r, i, normed):
        def fn(dep):
            rows = slice(i * LP, (i + 1) * LP)
            grows = slice(r * T + i * LP, r * T + (i + 1) * LP)
            sa = mod_scr[:, 0:M]
            if normed and dep is not None:
                sa = jnp.concatenate([_after(sa[:, _tile(j)], dep) for j in range(km)], axis=1)
            hf = ((x1_scr[grows, :] if normed else _ln(x_rows(grows, dep))) * _rows(mod_scr[:, M:2 * M], LP)
                  + _rows(sa, LP))
            for j in range(km):
                h_scr[r, j, rows, :] = hf[:, _tile(j)].astype(BF16)
            for f, n in _H_SUMS.items():
                if all(t[1] == r for t in f):
                    hs_scr[n, rows, :] = _form(f, lambda _, k: hf[:, _tile(k)]).astype(BF16)
            did.add(('h', r, i))
        return fn

    def release(jobs, span, items):
        if span and items:
            jobs.side += [(len(jobs.res) + 1 + i * span // len(items), fn) for i, fn in enumerate(items)]
            jobs.side.sort(key=lambda e: e[0])
        else:
            for fn in items:
                fn(None)

    def sum_items(n, group, index, dst, get, skip_rows):
        forms = [f for f in dict.fromkeys(t[0] for t in group)
                 if len(f) > 1 and not (skip_rows and len({t[1] for t in f}) == 1)]

        def item(f, rows):
            def fn(dep):
                def term(r, k):
                    v = get(r, k, rows).astype(F32)
                    return v if dep is None or (r, k) != f[0][1:] else _after(v, _rows(dep, v.shape[0]))
                dst[index[f], rows, :] = _form(f, term).astype(BF16)
            return fn

        return [item(f, slice(i, i + n)) for i in range(0, T, n) for f in forms]

    h_sums = lambda n, gi: sum_items(n, _H_GROUPS[gi], _H_SUMS, hs_scr,
                                     lambda r_, k, rows: h_scr[r_, k, rows, :], True)

    def stash(key, buf, j0, transpose=False):
        n = buf.shape[0] // T
        if key not in did:
            assert key in arrived
            did.add(key)
            w = _PairWeights(buf, transpose)
            for j in range(n):
                for hd in range(2):
                    w_scr[hd, j0 + j] = _pk(w(((1, j, hd),))[1])
        return lambda hd: [_ld(w_scr, hd, j0 + j) for j in range(n)]

    def kv_tile(jobs, r):
        wk, wvT = stash('k', wk_buf, 0), stash('v', wv_buf, kc, True)
        ct = [c_ref[_tile(r), _tile(j)] for j in range(kc)]
        for hd in range(2):
            k_scr[2 * r + hd] = _pk(jobs.mm(ct, wk(hd), _dot).astype(BF16))
        for hd in range(2):
            v_scr[2 * r + hd] = _pk(jobs.mm(wvT(hd), ct, _dot_nt).astype(BF16))

    def q_tile(jobs, r):
        wq = stash('q', wq_buf, 2 * kc)
        ht = [h_scr[r, j] for j in range(km)]
        for hd in range(2):
            q_scr[2 * r + hd] = _pk((jobs.mm(ht, wq(hd), _dot) * scale).astype(BF16))

    for blk in PROLOGUE.split(';'):
        waits, starts, acts = blk.split('|')
        for ch in waits.strip():
            assert ch in started and ch not in arrived
            arrived.add(ch)
            named[ch].wait()
        for ch in starts.strip():
            assert ch not in started
            started.add(ch)
            named[ch].start()
        jobs = _Jobs()
        for act in acts.split():
            if act == 'Z':
                jax.lax.fori_loop(0, nb, zero, 0)
                acc_scr[S:, :] = jnp.zeros((acc_scr.shape[0] - S, M), F32)
                x_ref[S:, :] = jnp.zeros((x_ref.shape[0] - S, M), BF16)
            elif act == 'L':
                did.add('L')
                for cp in cp_late[1:] + cp_late[:1]:
                    cp.start()
            elif act == 'M':
                assert arrived >= set('nm')
                mod = _dot(silu_cond(), wma_ref[...])
                mod_scr[:, 0:M] = mod[:, 0:M]
                mod_scr[:, M:2 * M] = 1.0 + mod[:, M:2 * M]
                did.add('M')
            else:
                act, _, span = act.partition('@')
                span = int(span or 0)
                items = []
                for r in [int(ch, 16) for ch in act[1:]]:
                    did.add((act[0], r))
                    if act[0] == 'K':
                        assert 'abcd'[r // CB] in arrived
                        kv_tile(jobs, r)
                    elif act[0] == 'H':
                        assert 'wxyz'[r // CB] in arrived and 'M' in did
                        items += [h_item(r, i, ('N', r) in did) for i in range(T // LP)]
                    elif act[0] == 'N':
                        assert 'wxyz'[r // CB] in arrived
                        items += [n_item(r, i) for i in range(T // LP)]
                    elif act[0] == 'Q':
                        assert all(('h', r, i) in did for i in range(T // LP))
                        q_tile(jobs, r)
                    elif act[0] == 'C':
                        assert all('abcd'[t[1] // CB] in arrived for p_ in _C_GROUPS[r] for t in p_[0])
                        items += sum_items(
                            32, _C_GROUPS[r], _C_SUMS, cs_scr,
                            lambda r_, k, rows: c_ref[r_ * T + rows.start:r_ * T + rows.stop, _tile(k)], False)
                    else:
                        assert act[0] == 'S' and all(('h', t[1], T // LP - 1) in did for p_ in _H_GROUPS[r] for t in p_[0])
                        items += h_sums(32 if span else 16, r)
                release(jobs, span, items)
        assert not jobs.side
    assert arrived == set(named) and all((k_, r) in did for k_ in 'KHQ' for r in range(nb))
    assert all((k_, r) in did for k_ in 'CS' for r in range(2)) and 'L' in did

    FH = ws3.shape[0] * T
    assert nattn - 1 >= FH // 64

    def mixer_prep(g):
        def blocks(w_ref, r0, n, half, c0, c1, dep):
            lo, hi = pl.ds(r0, n), pl.ds(r0 + half, n)
            return [_after(w_ref[rows, _tile(c)].astype(F32), _rows(dep, n)) if (rows is lo) == (c == c0)
                    else w_ref[rows, _tile(c)].astype(F32) for rows in (lo, hi) for c in (c0, c1)]

        def rows_items(w_ref, dst, per_step, half, n=16):
            gi = jnp.minimum(g, half // per_step - 1)
            src = w_ref.at[pl.ds(pl.multiple_of(gi * per_step, per_step), half + per_step), :]
            hs = per_step // 2

            def item(c, o):
                def fn(dep):
                    for i, v in enumerate(_b_ops(*blocks(src, o, n, half, c, c + 2, dep))):
                        dst[i, c, pl.ds(pl.multiple_of(gi * hs, hs) + o // 2, n // 2), :] = _pk(v.astype(BF16))
                return fn
            return [item(c, o) for c in range(2) for o in range(0, per_step, n)]

        def w3_item(k, i):
            def fn(dep):
                n = jnp.minimum(g, FH // T - 1)
                b11, b21, b12, b22 = blocks(w3_ref, pl.multiple_of(n * T, T), T, FH, k, k + 2, dep)
                ws3[n, i, k] = _pk(_b_ops(b11, b12, b21, b22)[i].astype(BF16).T)
            return fn

        return (rows_items(w1_ref, ws12.at[0], 32, 2 * T) + rows_items(w2_ref, ws12.at[1], 32, 2 * T)
                + rows_items(w4_ref, ws4, 64, FH) + [w3_item(k, i) for k in range(2) for i in range(7)])

    def attn_body(g, carry):
        copies = pcopies(jnp.minimum(g + 1, nattn - 1))

        def mid():
            for cp in copies:
                cp.start()

        _attention_step(q_scr, k_scr, v_scr, wo_buf, acc_scr, mid)
        for cp in copies:
            cp.wait()

        @pl.when(g == 0)
        def _():
            for cp in cp_late[1:]:
                cp.wait()
            for j in range(3):
                l1 = jnp.sum(jnp.sum(jnp.abs(smp_ref[j].astype(F32)), axis=0), axis=1, keepdims=True)
                e = pltpu.bitcast(jnp.broadcast_to(l1, (2 * nattn, T)), jnp.int32) >> 8
                for n in range(nattn):
                    d = (e[2 * n:2 * n + 1] - e[2 * n + 1:2 * n + 2] + (1 << 14)) >> 15
                    d = jnp.clip(d, -16, 16) << 23
                    gap_scr[n, j] = jnp.broadcast_to(d, (8, T))

        @pl.when(g + 1 < nattn)
        def _():
            ocopy(g + 1).start()
            side = [(SD0 + i * SDS, fn) for i, fn in enumerate(mixer_prep(g))]
            _proj_step(h_scr, hs_scr, c_ref, cs_scr, wq_buf, wk_buf, wv_buf, q_scr, k_scr, v_scr, scale,
                       gap_scr.at[g + 1], side)
            ocopy(g + 1).wait()

        return carry

    jax.lax.fori_loop(0, nattn, attn_body, 0)

    cp_late[0].wait()
    mod = _dot(silu_cond(), wmb_ref[...])
    mod_scr[:, 2 * M:4 * M] = mod[:, 0:2 * M]
    mod_scr[:, 4 * M:5 * M] = 1.0 + mod[:, 2 * M:3 * M]
    mod_scr[:, 5 * M:6 * M] = mod[:, 3 * M:4 * M]
    ftiles = [(f, min(f + T, Fd)) for f in range(0, Fd, T)]
    OFF = x_ref.shape[0] - S
    CAR = t_scr.shape[0] - RB

    def p1(r0, n, dep=None):
        ga = mod_scr[:, 2 * M:3 * M]
        if dep is not None:
            ga = jnp.concatenate([_after(ga[:, 0:T], dep), ga[:, T:]], axis=1)
        rows = pl.ds(r0, n)
        x1 = x_ref[rows, :].astype(F32) + _rows(ga, n) * acc_scr[rows, :]
        x1_scr[rows, :] = x1
        hb = _ln(x1) * _rows(mod_scr[:, 4 * M:5 * M], n) + _rows(mod_scr[:, 3 * M:4 * M], n)
        hb_scr[rows, :] = hb
        return _ln(hb)

    HT = T // 2

    def p1_store(r0, c, dep=None):
        v = p1(r0 + c * PC, PC, dep)
        a1_scr[c * PC:(c + 1) * PC, :] = v
        return jnp.max(v[:, M - T:].reshape(PC // 8, 8, T), axis=0)

    t_scr[RB:RB + CAR - OFF, :] = jnp.zeros((CAR - OFF, M), F32)
    t_scr[RB + CAR - OFF:RB + CAR, :] = _gelu(_dot(p1(0, OFF).astype(BF16), w1_ref[...]))
    for c in range(RB // PC):
        p1_store(OFF, c)

    def out_copy(i):
        rows = pl.ds(i * T if isinstance(i, int) else pl.multiple_of(i * T, T), T)
        return pltpu.make_async_copy(out_buf.at[rows, :], out_hbm.at[rows, :], osem.at[i])

    def b_body(r, carry):
        gb = _rows(mod_scr[:, 5 * M:6 * M], T)
        r0 = pl.multiple_of(r * RB, RB)
        n0 = pl.multiple_of(jnp.minimum(r0 + RB, S - RB) + OFF, OFF)
        nh = RB // T
        now = [0]
        due = []
        pace = []

        def p1_item(c):
            return lambda dep: due.append((now[0] + PD, p1_store(n0, c, dep)))

        pace += [(P0 + i * PSTEP, p1_item(i)) for i in range(RB // PC)]
        wt = lambda ref, f0, f1, n: ref[f0:f1, _tile(n)]

        def mm(lhs, wts, dot=_dot):
            acc = None
            for x, w in zip(lhs, wts):
                if due and due[0][0] <= now[0]:
                    w = _tie(w, due.pop(0)[1])
                v = dot(x, w)
                now[0] += x.shape[0] // HT
                acc = v if acc is None else v + acc
                if pace and pace[0][0] <= now[0]:
                    pace.pop(0)[1](v[0:8, :])
            return acc

        def split_ops(lo, hi):
            return [v.astype(BF16) for v in _a_ops(lo[:HT], hi[:HT], lo[HT:], hi[HT:])]

        def two_tiles(aops, wsel, rest):
            def col(w):
                v = mm(rest[0], w, rest[3])
                return v[:HT], v[HT:]

            c11, c12, c21, c22 = _strassen(
                lambda i: mm([a[i] for a in aops], [wsel(i, k) for k in range(len(aops))]),
                lambda: col(rest[1]), lambda: col(rest[2]))
            return jnp.concatenate([c11, c21], axis=0), jnp.concatenate([c12, c22], axis=0)

        def square(full, aops, w_ref, ws_ref):
            out = {}
            for n in range(2):
                out[n], out[n + 2] = two_tiles(
                    aops, lambda i, k: _ld(ws_ref, i, n, slice(k * HT, (k + 1) * HT)),
                    (full[4:], [wt(w_ref, 4 * T, M, n)], [wt(w_ref, 4 * T, M, n + 2)], _dot))
            out[4] = mm(full, [wt(w_ref, j * T, (j + 1) * T, 4) for j in range(km)])
            return out

        t_scr[0:CAR, :] = t_scr[RB:RB + CAR, :]
        for hf in range(nh):
            a1 = [a1_scr[_tile(hf), _tile(j)] for j in range(km)]
            full = [v.astype(BF16) for v in a1]
            aops = [split_ops(a1[k], a1[2 + k]) for k in range(2)]
            for n, v in square(full, aops, w1_ref, ws12.at[0]).items():
                t = _gelu(v)
                if hf == nh - 1:
                    t = jnp.concatenate([t[:T - OFF], jnp.where(r < nrb - 1, t[T - OFF:], 0.0)], axis=0)
                t_scr[CAR + hf * T:CAR + (hf + 1) * T, _tile(n)] = t
        cq = M // 4
        shifts = (-1, 1, -2, 2)
        lane = jax.lax.broadcasted_iota(jnp.int32, (T, T), 1)
        y1, a3 = [], []
        for hf in range(nh):
            base = CAR - OFF + hf * T
            sh = []
            for j in range(km):
                g_lo, g_hi = (j * T) // cq, ((j + 1) * T - 1) // cq
                assert g_hi - g_lo <= 1
                v = t_scr[base + shifts[g_lo]:base + shifts[g_lo] + T, _tile(j)]
                if g_hi != g_lo:
                    v2 = t_scr[base + shifts[g_hi]:base + shifts[g_hi] + T, _tile(j)]
                    v = jnp.where(lane < g_hi * cq - j * T, v, v2)
                sh.append(v)
            hs = square([v.astype(BF16) for v in sh], [split_ops(sh[k], sh[2 + k]) for k in range(2)],
                        w2_ref, ws12.at[1])
            hs = jnp.concatenate([hs[n] for n in range(km)], axis=1)
            y1.append(hs + hb_scr[pl.ds(pl.multiple_of(r0 + hf * T, T), T), :])
            a3.append({})

            def ln_item(hf, c):
                def item(dep):
                    n = HT // NLN
                    for d in (0, HT):
                        v = y1[hf][d + c * n:d + (c + 1) * n]
                        if dep is not None:
                            v = jnp.concatenate([_after(v[:, :T], _rows(dep, n)), v[:, T:]], axis=1)
                        a3[hf][d + c * n] = _ln(v)
                return item

            ln_item(hf, 0)(None)
            pace += [(now[0] + LN0 + (c - 1) * LNS * (1 + hf), ln_item(hf, c)) for c in range(1, NLN)]
            pace.sort(key=lambda e: e[0])
        nf = FH // T
        h3, h3ops = [], []
        for hf in range(nh):
            assert len(a3[hf]) == 2 * NLN
            af = jnp.concatenate([a3[hf][key] for key in sorted(a3[hf])], axis=0)
            full = [af[:, _tile(j)].astype(BF16) for j in range(km)]
            aops = [split_ops(af[:, _tile(k)], af[:, _tile(2 + k)]) for k in range(2)]
            row, ops = {}, []
            narrow = None
            for n in range(nf):
                lo, hi = two_tiles(aops, lambda i, k: _ld(ws3, n, i, k),
                                   (full[4:], [wt(w3_ref, *ftiles[n], 4)],
                                    [wt(w3_ref, *ftiles[nf + n], 4)], _dot_nt))
                lo, hi = _gelu(lo), _gelu(hi)
                row[n], row[nf + n] = lo.astype(BF16), hi.astype(BF16)
                ops.append(split_ops(lo, hi))
                if n < km:
                    v = mm([wt(w3_ref, *ftiles[-1], n)], [full[n]], _dot_nt)
                    narrow = v if narrow is None else v + narrow
            row[2 * nf] = _gelu(mm(full, [wt(w3_ref, *ftiles[2 * nf], j) for j in range(km)],
                                   _dot_nt)).astype(BF16)
            fw = Fd - ftiles[-1][0]
            gT = jnp.concatenate([_gelu(narrow), jnp.zeros((T - fw, T), F32)], axis=0)
            row[2 * nf + 1] = _tie(gT.astype(BF16).T, gT[0:8, :])[:, :fw]
            h3.append([row[i] for i in range(len(ftiles))])
            h3ops.append(ops)
        for hf in range(nh):
            rows = pl.ds(pl.multiple_of(r0 + hf * T, T), T)

            def finish(n, v):
                out_buf[rows, _tile(n)] = (
                    x1_scr[rows, _tile(n)] + gb[:, _tile(n)] * (v + y1[hf][:, _tile(n)])
                ).astype(out_buf.dtype)

            w4t = lambda n, f_: [wt(w4_ref, f0, f1, n) for f0, f1 in f_]
            finish(4, mm(h3[hf], w4t(4, ftiles)))
            for n in range(2):
                lo, hi = two_tiles(h3ops[hf], lambda i, k: _ld(ws4, i, n, slice(k * HT, (k + 1) * HT)),
                                   (h3[hf][2 * nf:], w4t(n, ftiles[2 * nf:]), w4t(n + 2, ftiles[2 * nf:]), _dot))
                finish(n, lo)
                finish(n + 2, hi)
            out_copy(r * nh + hf).start()
        assert not pace
        return carry

    jax.lax.fori_loop(0, nrb, b_body, 0)
    for i in range(nb):
        out_copy(i).wait()


@jax.jit
def pallas_adaLN_cond__compressed_kv_cla__mixer_s_mlp__prompt_kernel(
    A_x: jax.Array,
    A_c_kv: jax.Array,
    A_w_q: jax.Array,
    A_w_uk: jax.Array,
    A_w_uv: jax.Array,
    A_w_o: jax.Array,
    B_x: jax.Array,
    B_w1: jax.Array,
    B_w2: jax.Array,
    B_w3: jax.Array,
    B_w4: jax.Array,
    c: jax.Array,
    w_mod: jax.Array,
):
    _, S, M = A_x.shape
    Dc = A_c_kv.shape[2]
    H, D = A_w_q.shape[1], A_w_q.shape[2]
    Fd = B_w3.shape[1]
    assert D == T and A_c_kv.shape[1] == S and Dc == 4 * T and M == 5 * T and 13 * T < Fd < 14 * T and S == 16 * T
    vmem = pltpu.VMEM
    packed = lambda *lead: vmem(lead + (T // 2, T), U32)
    out = pl.pallas_call(
        _kernel,
        in_specs=[pl.BlockSpec(memory_space=pltpu.HBM)] * 12,
        out_specs=pl.BlockSpec(memory_space=pltpu.HBM),
        out_shape=jax.ShapeDtypeStruct((S, M), A_x.dtype),
        scratch_shapes=[
            vmem((S + 16, M), BF16),
            vmem((S, Dc), BF16),
            vmem((1, M), BF16),
            vmem((M, 2 * M), BF16),
            vmem((M, 4 * M), BF16),
            vmem((M, M), BF16),
            vmem((M, M), BF16),
            vmem((Fd, M), BF16),
            vmem((Fd, M), BF16),
            vmem((M, D), U32),
            vmem((Dc, D), U32),
            vmem((Dc, D), U32),
            vmem((2 * D, M), BF16),
            vmem((S, M), A_x.dtype),
            pltpu.SemaphoreType.DMA((18,)),
            pltpu.SemaphoreType.DMA((4,)),
            pltpu.SemaphoreType.DMA((S // T,)),
            vmem((8, 6 * M), F32),
            vmem((S // T, M // T, T, T), BF16),
            vmem((len(_C_SUMS), T, T), BF16),
            vmem((len(_H_SUMS), T, T), BF16),
            packed(2, M // T + 2 * (Dc // T)),
            packed(2 * S // T),
            packed(2 * S // T),
            packed(2 * S // T),
            vmem((S + 16, M), F32),
            vmem((S + 16, M), F32),
            vmem((S + 16, M), F32),
            vmem((RB, M), F32),
            vmem((RB + 32, M), F32),
            vmem((2, 7, 2, T, T), U32),
            packed(6, 7, 2),
            vmem((7, 2, 3 * T, T), U32),
            vmem((3, 8, H, D), BF16),
            vmem((H // 2, 3, 8, T), jnp.int32),
        ],
        compiler_params=pltpu.CompilerParams(
            vmem_limit_bytes=100 * 1024 * 1024,
            disable_bounds_checks=True,
        ),
    )(
        A_x.reshape(S, M), A_c_kv.reshape(S, Dc),
        A_w_q, A_w_uk, A_w_uv,
        A_w_o.reshape(H // 2, 2 * D, M),
        B_w1, B_w2, B_w3.T, B_w4, c, w_mod,
    )
    return out.reshape(1, S, M)
```

```python
import math

import jax
import jax.numpy as jnp
import jax.experimental.pallas as pl
import jax.experimental.pallas.tpu as pltpu

F32 = jnp.float32
BF16 = jnp.bfloat16
U32 = jnp.uint32
NT = (((1,), (1,)), ((), ()))
T = 128
EPS = 1e-5
LOG2E = math.log2(math.e)

GRP = 4
LEAD = 10
PROW = 3
RES = 32
LAT_A = 16
LAT_B = 20
ALEAD = 32
MID = 40
SD0, SDS = 60, 3
RB = 256
PC = 32
P0, PSTEP, PD = 440, 30, 52
NLN, LN0, LNS = 4, 4, 5
LP = 16
PROLOGUE = ('|kva|Z; |b|; kva|wc|K0123; bw|xdn|C0@56 N0123@52 K4567; cx|mq|N4567@52 K89ab; '
            'd|y|C1@56 Kcdef; nmq|zo|M H01 H234567@30 Q0123; y||H89ab@30 Q4567; '
            'zo||L Hcdef@30 Q89ab S01 Qcdef')


def _dot(a, b):
    return jnp.dot(a, b, preferred_element_type=F32)


def _dot_nt(a, b):
    return jax.lax.dot_general(a, b, NT, preferred_element_type=F32)


def _ln(x):
    m = jnp.mean(x, axis=-1, keepdims=True)
    xc = x - m
    v = jnp.mean(xc * xc, axis=-1, keepdims=True)
    return xc * jnp.exp2(jnp.log(v + EPS) * (-0.5 * LOG2E))


def _rows(v, n):
    return jnp.broadcast_to(v[None], (n // 8, 8, v.shape[1])).reshape(n, v.shape[1])


def _gelu(x):
    c0 = math.sqrt(2.0 / math.pi)
    return 0.5 * x * (1.0 + jnp.tanh(c0 * (x + 0.044715 * (x * x * x))))


def _after(x, dep):
    return jnp.where(dep > jnp.inf, dep, x)


def _tie(x, dep):
    xu = pltpu.bitcast(x, U32)
    first = jnp.where(dep > jnp.inf, jnp.uint32(0), xu[:8])
    return pltpu.bitcast(jnp.concatenate([first, xu[8:]], axis=0), BF16)


def _tile(j):
    return slice(j * T, (j + 1) * T)


def _ld(ref, *idx):
    return pltpu.bitcast(ref[idx], BF16)


def _pk(x):
    return pltpu.bitcast(x, U32)


def _a_ops(a11, a12, a21, a22):
    return [a11 + a22, a21 + a22, a11, a22, a11 + a12, a21 - a11, a12 - a22]


def _b_ops(b11, b12, b21, b22):
    return [b11 + b22, b11, b12 - b22, b21 - b11, b22, b11 + b12, b21 + b22]


def _strassen(prod, col1=None, col2=None):
    m4 = prod(3)
    m2 = prod(1)
    c21 = m2 + m4
    if col1 is not None:
        e11, e21 = col1()
        m4, c21 = m4 + e11, c21 + e21
    m3 = prod(2)
    m5 = prod(4)
    c12 = m3 + m5
    if col2 is not None:
        e12, e22 = col2()
        c12, m3 = c12 + e12, m3 + e22
    m1 = prod(0)
    c11 = prod(6) + (m1 + (m4 - m5))
    c22 = prod(5) + (m1 + (m3 - m2))
    return c11, c12, c21, c22


def _group(rows, cols, pairs):
    xs, ys = dict.fromkeys(x for x, _ in pairs), dict.fromkeys(y for _, y in pairs)
    used = set(xs) | set(ys) | {(x[0], y[1]) for x, y in pairs} | {(y[0], x[1]) for x, y in pairs}
    prods = []
    for n, r in enumerate(rows):
        for i, k in [x for x in xs if x[0] == r]:
            mates = [y for x, y in pairs if x == (i, k)]
            prods.append((((1, i, k),) + tuple((1, i, k2) for _, k2 in mates), ((1, k, 0),),
                          ((1, i, 0), (-1, i, 1))))
            prods.append((((1, i, k),) + tuple((-1, i2, k) for i2, _ in mates), ((1, k, 0), (1, k, 1)),
                          ((1, i, 1),)))
        for i2, k2 in [y for y in ys if y[0] == r]:
            mates = [x for x, y in pairs if y == (i2, k2)]
            prods.append((((1, i2, k2),) + tuple((1, i2, k) for _, k in mates), ((1, k2, 1),),
                          ((1, i2, 1), (-1, i2, 0))))
            prods.append((((1, i2, k2),) + tuple((-1, i, k2) for i, _ in mates), ((1, k2, 0), (1, k2, 1)),
                          ((1, i2, 0),)))
        prods += [(((1, r, k),), ((1, k, h),), ((1, r, h),)) for k in cols if (r, k) not in used for h in (0, 1)]
        for (i, k), (i2, k2) in pairs:
            if r in (i, i2) and i + i2 - r in rows[n + 1:]:
                prods.append((((1, i, k2),), ((1, k2, 0), (-1, k, 0)), ((1, i2, 0), (1, i, 0))))
                prods.append((((1, i2, k), (1, i, k2)), ((1, k, 0), (1, k2, 1)), ((1, i2, 0), (1, i, 1))))
                prods.append((((1, i2, k),), ((1, k, 1), (-1, k2, 1)), ((1, i2, 1), (1, i, 1))))
    return prods


def _all_pairs(xrows, yrows):
    return [((x, a), (y, b)) for a, x in enumerate(xrows) for b, y in enumerate(yrows) if a != b]


_PAIRS65 = [((x[0] + 10, x[1]), (y[0] + 10, y[1])) for x, y in (
    ((0, 1), (1, 0)), ((0, 1), (5, 2)), ((2, 3), (1, 0)), ((2, 3), (3, 1)), ((2, 3), (5, 2)), ((3, 2), (1, 0)),
    ((4, 4), (0, 3)), ((4, 4), (1, 0)), ((4, 4), (3, 1)), ((4, 4), (5, 2)))]
_C_GROUPS = [_group(range(r, r + 8), range(4), _all_pairs(range(r, r + 4), range(r + 4, r + 8))) for r in (0, 8)]
_H_GROUPS = [_group(range(10), range(5), _all_pairs(range(5), range(5, 10))),
             _group(range(10, 16), range(5), _PAIRS65)]
_sum_index = lambda groups: {f: n for n, f in enumerate(
    dict.fromkeys(t[0] for g in groups for t in g if len(t[0]) > 1))}
_C_SUMS, _H_SUMS = _sum_index(_C_GROUPS), _sum_index(_H_GROUPS)


def _form(form, get):
    acc = None
    for sign, i, j in form:
        v = get(i, j)
        acc = v if acc is None else (acc + v if sign > 0 else acc - v)
    return acc


def _gap_items(bufs, gap_scr):
    items = []
    for n, buf in enumerate(bufs):
        acc = []

        def part(r0, buf=buf, acc=acc):
            def fn(dep):
                wu = jnp.concatenate([buf[r:r + 8, :] for r in range(r0, r0 + T, 32)])
                mask = jnp.full((8, T), 0x7FFF0000, U32)
                if dep is not None:
                    mask = jnp.where(dep > jnp.inf, jnp.uint32(0), mask)
                mask = _rows(mask, 32)
                new = [jnp.sum(pltpu.bitcast(v & mask, F32).reshape(4, 8, T), axis=0) for v in (wu << 16, wu)]
                acc[:] = [u + v for u, v in zip(acc, new)] if acc else new
            return fn

        def last(_, n=n, acc=acc):
            bits = []
            for v in acc:
                l1 = jnp.sum(jnp.sum(v, axis=1, keepdims=True), axis=0, keepdims=True)
                bits.append(pltpu.bitcast(jnp.broadcast_to(l1, (8, T)), jnp.int32) >> 8)
            gap_scr[n] = jnp.clip((bits[0] - bits[1] + (1 << 14)) >> 15, -8, 8) << 23

        items += [part(r0) for r0 in range(0, buf.shape[0], T)] + [last]
    return items


class _PairWeights:
    def __init__(self, w_ref, transpose=False, shift=None):
        self.base = {}
        if shift is not None:
            fac = _rows(pltpu.bitcast(0x3F800000 + shift, F32), T)
            self.inv = pltpu.bitcast(0x3F800000 - shift, F32)
        for j in range(w_ref.shape[0] // T):
            wu = w_ref[_tile(j), :]
            if transpose:
                wu = wu.T
            hi = pltpu.bitcast(wu & jnp.uint32(0xFFFF0000), F32)
            self.base[j, 0] = pltpu.bitcast(wu << 16, F32)
            self.base[j, 1] = hi if shift is None else hi * fac
        self.cache = {}

    def __call__(self, form):
        sign = 1
        if form[-1][0] < 0 and form[0][1:] > form[1][1:]:
            sign, form = -1, ((1,) + form[1][1:], (-1,) + form[0][1:])
        if form not in self.cache:
            self.cache[form] = _form(form, lambda k, h: self.base[k, h]).astype(BF16)
        return sign, self.cache[form]


def _run_group(jobs, prods, a_get, w, transposed, finish):
    left = {}
    for _, _, outs in prods:
        for _, i, h in outs:
            left[i, h] = left.get((i, h), 0) + 1
    acc = {}
    for af, bf, outs in prods:
        sign, wt = w(bf)
        m = jobs.mm([wt], [a_get(af)], _dot_nt) if transposed else jobs.mm([a_get(af)], [wt], _dot)
        for s_, i, h in outs:
            if (i, h) not in acc:
                acc[i, h] = (s_ * sign, m)
            else:
                s0, v = acc[i, h]
                acc[i, h] = (s0, v + m if s0 == s_ * sign else v - m) if s0 > 0 or s_ * sign < 0 else (1, m - v)
            left[i, h] -= 1
            if not left[i, h]:
                s0, v = acc.pop((i, h))
                assert s0 > 0
                finish(2 * i + h, v)


class _Jobs:
    def __init__(self, side=()):
        self.res = []
        self.side = list(side)

    def mm(self, lhs, wt, dot):
        acc = None
        for x, w in zip(lhs, wt):
            v = dot(x, w)
            self.res.append(v)
            acc = v if acc is None else v + acc
            rel = 4 * (len(self.res) % 4)
            while self.side and self.side[0][0] <= len(self.res):
                self.side.pop(0)[1](v[8 * rel:8 * rel + 8, :])
                rel = (rel + 2) % 16
        return acc


def _proj_step(h_scr, hs_scr, c_ref, cs_scr, wq_ref, wuk_ref, wuv_ref, q_scr, k_scr, v_scr, scale, shifts, side):
    wk, wvT, wq = [_PairWeights(w, n == 1, shifts[n]) for n, w in enumerate((wuk_ref, wuv_ref, wq_ref))]
    c_get = lambda f: cs_scr[_C_SUMS[f]] if len(f) > 1 else c_ref[_tile(f[0][1]), _tile(f[0][2])]
    h_get = lambda f: hs_scr[_H_SUMS[f]] if len(f) > 1 else h_scr[f[0][1], f[0][2]]

    def put(dst, w, mul=None):
        muls = [mul, _rows(w.inv if mul is None else w.inv * mul, T)]

        def fn(u, v):
            dst[u] = _pk((v if muls[u % 2] is None else v * muls[u % 2]).astype(BF16))
        return fn

    jobs = _Jobs(side)
    for groups, get, w, transposed, fin in ((_C_GROUPS, c_get, wk, False, put(k_scr, wk)),
                                            (_C_GROUPS, c_get, wvT, True, put(v_scr, wvT)),
                                            (_H_GROUPS, h_get, wq, False, put(q_scr, wq, scale))):
        for prods in groups:
            _run_group(jobs, prods, get, w, transposed, fin)
    assert not jobs.side


def _inner_group(rows, cols, pairs):
    xs, ys = dict.fromkeys(x for x, _ in pairs), dict.fromkeys(y for _, y in pairs)
    used = set(xs) | set(ys) | {(x[0], y[1]) for x, y in pairs} | {(y[0], x[1]) for x, y in pairs}
    prods = []
    for i, j in xs:
        mates = [y for x, y in pairs if x == (i, j)]
        prods.append((((1, i, 0),), ((1, 0, j), (-1, 1, j)), ((1, i, j),) + tuple((1, i2, j) for i2, _ in mates)))
        prods.append((((1, i, 0), (1, i, 1)), ((1, 1, j),), ((1, i, j),) + tuple((-1, i, j2) for _, j2 in mates)))
    for i2, j2 in ys:
        mates = [x for x, y in pairs if y == (i2, j2)]
        prods.append((((1, i2, 0), (1, i2, 1)), ((1, 0, j2),),
                      ((1, i2, j2),) + tuple((-1, i2, j) for _, j in mates)))
        prods.append((((1, i2, 1),), ((1, 0, j2), (-1, 1, j2)),
                      ((-1, i2, j2),) + tuple((-1, i, j2) for i, _ in mates)))
    prods += [(((1, i, h),), ((1, h, j),), ((1, i, j),))
              for i in rows for j in cols if (i, j) not in used for h in (0, 1)]
    for (i, j), (i2, j2) in pairs:
        lo, hi = min(j, j2), max(j, j2)
        prods.append((((1, i2, 0), (-1, i, 0)), ((1, 0, lo), (1, 0, hi)), ((1, i2, j),)))
        prods.append((((1, i, 0), (1, i2, 1)), ((1, 0, j2), (1, 1, j)), ((1, i, j2), (1, i2, j))))
        prods.append((((1, i, 1), (-1, i2, 1)), ((1, 1, lo), (1, 1, hi)), ((1, i, j2),)))
    return prods


def _o_jobs():
    prods = (_inner_group(range(10), range(5), _all_pairs(range(0, 10, 2), range(1, 10, 2)))
             + _inner_group(range(10, 16), range(5), _PAIRS65))
    row = lambda t: max(i for _, i, _ in t[0])
    unit = lambda t: max(2 * i + h for _, i, h in t[0])
    need = lambda t: unit(t) if row(t) == 15 else 2 * row(t) + 1
    return [(need(t), t) for t in sorted(prods, key=need)]


_O_JOBS = _o_jobs()


def _job_order(nb):
    units = range(2 * nb)
    qa = [('a', u, c) for u in units for c in range(u // 2 + 1)]
    qb = [('b', u, c) for u in units for c in range(u // 2 + 1)]
    qo = [('o', u, j) for j, (u, _) in enumerate(_O_JOBS)]
    done = {}
    order = []

    def ready(q, lat, pre):
        return bool(q) and (pre, q[0][1]) in done and done[(pre, q[0][1])] + lat <= len(order)

    def emit(q):
        kind, u, j = job = q.pop(0)
        if kind != 'o' and j == u // 2:
            done[(kind, u)] = len(order)
        order.append(job)

    turn = 0
    while qa or qb or qo:
        pref = 'abo'[turn % 3]
        turn += 1
        for _ in range(GRP):
            b_ok, o_ok = ready(qb, LAT_A, 'a'), ready(qo, LAT_B, 'b')
            if pref == 'a' and qa and (len(qb) - len(qa) < ALEAD or not b_ok):
                emit(qa)
            elif pref == 'b' and b_ok:
                emit(qb)
            elif pref == 'o' and o_ok and (len(qo) > RES or not (qa or b_ok)):
                emit(qo)
            elif not (qa or b_ok or o_ok) and (qb or qo):
                emit(qb or qo)
            else:
                break
    return order


def _attention_step(q_scr, k_scr, v_scr, wo_ref, acc_scr, mid):
    causal = (jax.lax.broadcasted_iota(jnp.int32, (T, T), 0)
              <= jax.lax.broadcasted_iota(jnp.int32, (T, T), 1))
    sv, mx, mfin, lsum, pv, of, lhs = {}, {}, {}, {}, {}, {}, {}
    res = []
    wo, terms = {}, {}
    left = {}
    for _, t in _O_JOBS:
        for _, i, j in t[2]:
            left[i, j] = left.get((i, j), 0) + 1

    def job_a(u, c):
        r, hd = divmod(u, 2)
        s = _dot_nt(_ld(k_scr, 2 * c + hd), _ld(q_scr, u))
        res.append(s)
        if c == r:
            s = jnp.where(causal, s, -1e9 * LOG2E)
        s = s.reshape(T // 8, 8, T)
        sv[(u, c)] = s
        pm = jnp.max(s, axis=0)
        mx[u] = pm if u not in mx else jnp.maximum(mx[u], pm)

    def job_b(u, c):
        r, hd = divmod(u, 2)
        if u not in mfin:
            mfin[u] = jnp.broadcast_to(jnp.max(mx[u], axis=0, keepdims=True), (8, T))
        m = mfin[u]
        if len(res) >= LEAD:
            r0 = 8 * PROW * (c % 4)
            m = _after(m, res[len(res) - LEAD][r0:r0 + 8, :])
        p = jnp.exp2(sv.pop((u, c)) - m[None])
        ls = jnp.sum(p, axis=0)
        lsum[u] = ls if u not in lsum else lsum[u] + ls
        v = _dot(_ld(v_scr, 2 * c + hd), p.reshape(T, T).astype(BF16))
        res.append(v)
        pv[u] = v if u not in pv else v + pv[u]
        if c == r:
            of[u] = pv[u] * (1.0 / jnp.sum(lsum[u], axis=0, keepdims=True))

    def job_o(_, n):
        af, bf, outs = _O_JOBS[n][1]
        if af not in lhs:
            v = _form(af, lambda i, h: of[2 * i + h])
            lhs[af] = _tie(v.astype(BF16).T, v[0:8, :])
        if bf not in wo:
            wo[bf] = (wo_ref[_tile(bf[0][1]), _tile(bf[0][2])] if len(bf) == 1 else
                      _form(bf, lambda h, j: wo_ref[_tile(h), _tile(j)].astype(F32)).astype(BF16))
        v = _dot(lhs[af], wo[bf])
        res.append(v)
        for sign, i, j in outs:
            terms.setdefault((i, j), []).append((sign, v))
            if len(terms[i, j]) == left[i, j]:
                tot = acc_scr[_tile(i), _tile(j)]
                for sg, m in terms.pop((i, j)):
                    tot = tot + m if sg > 0 else tot - m
                acc_scr[_tile(i), _tile(j)] = tot

    fns = dict(a=job_a, b=job_b, o=job_o)
    for n, (kind, u, j) in enumerate(_job_order(q_scr.shape[0] // 2)):
        if n == MID:
            mid()
        fns[kind](u, j)


def _kernel(x_hbm, c_hbm, wq_hbm, wuk_hbm, wuv_hbm, wo_hbm, w1_hbm, w2_hbm, w3_hbm, w4_hbm,
            cond_hbm, wmod_hbm, out_hbm,
            x_ref, c_ref, cond_ref, wma_ref, wmb_ref, w1_ref, w2_ref, w3_ref, w4_ref,
            wq_buf, wk_buf, wv_buf, wo_buf, out_buf, sem, wsem, osem,
            mod_scr, h_scr, cs_scr, hs_scr, w_scr, q_scr, k_scr, v_scr, acc_scr, x1_scr, hb_scr, a1_scr, t_scr,
            ws12, ws3, ws4, pq_buf, pk_buf, pv_buf, gap_scr):
    S, M = x_hbm.shape
    D = wq_hbm.shape[2]
    nattn = wo_hbm.shape[0]
    Fd = w4_hbm.shape[0]
    scale = float(D) ** -0.5 * LOG2E
    nb, nrb = S // T, S // RB
    km, kc = M // T, c_hbm.shape[1] // T
    NX = 4
    XR = S // NX
    CB = XR // T

    work, probe = (wk_buf, wv_buf, wq_buf), (pk_buf, pv_buf, pq_buf)

    def pcopies(g, bufs=work, s0=0):
        return [pltpu.make_async_copy(src.bitcast(U32).at[:, g, :], dst, wsem.at[s0 + j])
                for j, (src, dst) in enumerate(zip((wuk_hbm, wuv_hbm, wq_hbm), bufs))]

    def ocopy(g):
        return pltpu.make_async_copy(wo_hbm.at[g], wo_buf, wsem.at[3])

    def chunk_copy(src, dst, i, s0):
        rows = slice(i * XR, (i + 1) * XR)
        return pltpu.make_async_copy(src.at[rows, :], dst.at[rows, :], sem.at[s0 + i])

    cp_cond = pltpu.make_async_copy(cond_hbm, cond_ref, sem.at[0])
    cp_wma = pltpu.make_async_copy(wmod_hbm.at[:, 0:2 * M], wma_ref, sem.at[1])
    cp_late = [pltpu.make_async_copy(src, dst, sem.at[2 + j]) for j, (src, dst) in enumerate((
        (wmod_hbm.at[:, 2 * M:6 * M], wmb_ref), (w1_hbm, w1_ref), (w2_hbm, w2_ref),
        (w3_hbm, w3_ref), (w4_hbm, w4_ref)))]
    cp_x = [chunk_copy(x_hbm, x_ref, i, 7) for i in range(NX)]
    cp_c = [chunk_copy(c_hbm, c_ref, i, 7 + NX) for i in range(NX)]

    def silu_cond():
        cf = cond_ref[...].astype(F32)
        return jnp.broadcast_to((cf * jax.nn.sigmoid(cf)).astype(BF16), (8, M))

    cp_wk, cp_wv, cp_wq = pcopies(0)
    named = dict(k=cp_wk, v=cp_wv, q=cp_wq, o=ocopy(0), n=cp_cond, m=cp_wma)
    named.update(zip('abcd', cp_c))
    named.update(zip('wxyz', cp_x))
    started, arrived, did = set(), set(), set()

    def zero(r, carry):
        acc_scr[pl.ds(pl.multiple_of(r * T, T), T), :] = jnp.zeros((T, M), F32)
        return carry

    def x_rows(rows, dep):
        xf = x_ref[rows, :].astype(F32)
        if dep is None:
            return xf
        return jnp.concatenate([_after(xf[:, :T], _rows(dep, xf.shape[0])), xf[:, T:]], axis=1)

    def n_item(r, i):
        def fn(dep):
            rows = slice(r * T + i * LP, r * T + (i + 1) * LP)
            x1_scr[rows, :] = _ln(x_rows(rows, dep))
        return fn

    def h_item(r, i, normed):
        def fn(dep):
            rows = slice(i * LP, (i + 1) * LP)
            grows = slice(r * T + i * LP, r * T + (i + 1) * LP)
            sa = mod_scr[:, 0:M]
            if normed and dep is not None:
                sa = jnp.concatenate([_after(sa[:, _tile(j)], dep) for j in range(km)], axis=1)
            hf = ((x1_scr[grows, :] if normed else _ln(x_rows(grows, dep))) * _rows(mod_scr[:, M:2 * M], LP)
                  + _rows(sa, LP))
            for j in range(km):
                h_scr[r, j, rows, :] = hf[:, _tile(j)].astype(BF16)
            for f, n in _H_SUMS.items():
                if all(t[1] == r for t in f):
                    hs_scr[n, rows, :] = _form(f, lambda _, k: hf[:, _tile(k)]).astype(BF16)
            did.add(('h', r, i))
        return fn

    def release(jobs, span, items):
        if span and items:
            jobs.side += [(len(jobs.res) + 1 + i * span // len(items), fn) for i, fn in enumerate(items)]
            jobs.side.sort(key=lambda e: e[0])
        else:
            for fn in items:
                fn(None)

    def sum_items(n, group, index, dst, get, skip_rows):
        forms = [f for f in dict.fromkeys(t[0] for t in group)
                 if len(f) > 1 and not (skip_rows and len({t[1] for t in f}) == 1)]

        def item(f, rows):
            def fn(dep):
                def term(r, k):
                    v = get(r, k, rows).astype(F32)
                    return v if dep is None or (r, k) != f[0][1:] else _after(v, _rows(dep, v.shape[0]))
                dst[index[f], rows, :] = _form(f, term).astype(BF16)
            return fn

        return [item(f, slice(i, i + n)) for i in range(0, T, n) for f in forms]

    h_sums = lambda n, gi: sum_items(n, _H_GROUPS[gi], _H_SUMS, hs_scr,
                                     lambda r_, k, rows: h_scr[r_, k, rows, :], True)

    def stash(key, buf, j0, transpose=False):
        n = buf.shape[0] // T
        if key not in did:
            assert key in arrived
            did.add(key)
            w = _PairWeights(buf, transpose)
            for j in range(n):
                for hd in range(2):
                    w_scr[hd, j0 + j] = _pk(w(((1, j, hd),))[1])
        return lambda hd: [_ld(w_scr, hd, j0 + j) for j in range(n)]

    def kv_tile(jobs, r):
        wk, wvT = stash('k', wk_buf, 0), stash('v', wv_buf, kc, True)
        ct = [c_ref[_tile(r), _tile(j)] for j in range(kc)]
        for hd in range(2):
            k_scr[2 * r + hd] = _pk(jobs.mm(ct, wk(hd), _dot).astype(BF16))
        for hd in range(2):
            v_scr[2 * r + hd] = _pk(jobs.mm(wvT(hd), ct, _dot_nt).astype(BF16))

    def q_tile(jobs, r):
        wq = stash('q', wq_buf, 2 * kc)
        ht = [h_scr[r, j] for j in range(km)]
        for hd in range(2):
            q_scr[2 * r + hd] = _pk((jobs.mm(ht, wq(hd), _dot) * scale).astype(BF16))

    for blk in PROLOGUE.split(';'):
        waits, starts, acts = blk.split('|')
        for ch in waits.strip():
            assert ch in started and ch not in arrived
            arrived.add(ch)
            named[ch].wait()
        for ch in starts.strip():
            assert ch not in started
            started.add(ch)
            named[ch].start()
        jobs = _Jobs()
        for act in acts.split():
            if act == 'Z':
                jax.lax.fori_loop(0, nb, zero, 0)
                acc_scr[S:, :] = jnp.zeros((acc_scr.shape[0] - S, M), F32)
                x_ref[S:, :] = jnp.zeros((x_ref.shape[0] - S, M), BF16)
            elif act == 'L':
                did.add('L')
                for cp in cp_late[1:] + cp_late[:1]:
                    cp.start()
            elif act == 'M':
                assert arrived >= set('nm')
                mod = _dot(silu_cond(), wma_ref[...])
                mod_scr[:, 0:M] = mod[:, 0:M]
                mod_scr[:, M:2 * M] = 1.0 + mod[:, M:2 * M]
                did.add('M')
            else:
                act, _, span = act.partition('@')
                span = int(span or 0)
                items = []
                for r in [int(ch, 16) for ch in act[1:]]:
                    did.add((act[0], r))
                    if act[0] == 'K':
                        assert 'abcd'[r // CB] in arrived
                        kv_tile(jobs, r)
                    elif act[0] == 'H':
                        assert 'wxyz'[r // CB] in arrived and 'M' in did
                        items += [h_item(r, i, ('N', r) in did) for i in range(T // LP)]
                    elif act[0] == 'N':
                        assert 'wxyz'[r // CB] in arrived
                        items += [n_item(r, i) for i in range(T // LP)]
                    elif act[0] == 'Q':
                        assert all(('h', r, i) in did for i in range(T // LP))
                        q_tile(jobs, r)
                    elif act[0] == 'C':
                        assert all('abcd'[t[1] // CB] in arrived for p_ in _C_GROUPS[r] for t in p_[0])
                        items += sum_items(
                            32, _C_GROUPS[r], _C_SUMS, cs_scr,
                            lambda r_, k, rows: c_ref[r_ * T + rows.start:r_ * T + rows.stop, _tile(k)], False)
                    else:
                        assert act[0] == 'S' and all(('h', t[1], T // LP - 1) in did for p_ in _H_GROUPS[r] for t in p_[0])
                        items += h_sums(32 if span else 16, r)
                release(jobs, span, items)
        assert not jobs.side
    assert arrived == set(named) and all((k_, r) in did for k_ in 'KHQ' for r in range(nb))
    assert all((k_, r) in did for k_ in 'CS' for r in range(2)) and 'L' in did

    FH = ws3.shape[0] * T
    assert nattn - 1 >= FH // 64

    def mixer_prep(g):
        def blocks(w_ref, r0, n, half, c0, c1, dep):
            lo, hi = pl.ds(r0, n), pl.ds(r0 + half, n)
            return [_after(w_ref[rows, _tile(c)].astype(F32), _rows(dep, n)) if (rows is lo) == (c == c0)
                    else w_ref[rows, _tile(c)].astype(F32) for rows in (lo, hi) for c in (c0, c1)]

        def rows_items(w_ref, dst, per_step, half, n=16):
            gi = jnp.minimum(g, half // per_step - 1)
            src = w_ref.at[pl.ds(pl.multiple_of(gi * per_step, per_step), half + per_step), :]
            hs = per_step // 2

            def item(c, o):
                def fn(dep):
                    for i, v in enumerate(_b_ops(*blocks(src, o, n, half, c, c + 2, dep))):
                        dst[i, c, pl.ds(pl.multiple_of(gi * hs, hs) + o // 2, n // 2), :] = _pk(v.astype(BF16))
                return fn
            return [item(c, o) for c in range(2) for o in range(0, per_step, n)]

        def w3_item(k, i):
            def fn(dep):
                n = jnp.minimum(g, FH // T - 1)
                b11, b21, b12, b22 = blocks(w3_ref, pl.multiple_of(n * T, T), T, FH, k, k + 2, dep)
                ws3[n, i, k] = _pk(_b_ops(b11, b12, b21, b22)[i].astype(BF16).T)
            return fn

        return (rows_items(w1_ref, ws12.at[0], 32, 2 * T) + rows_items(w2_ref, ws12.at[1], 32, 2 * T)
                + rows_items(w4_ref, ws4, 64, FH) + [w3_item(k, i) for k in range(2) for i in range(7)])

    def attn_body(g, carry):
        copies = pcopies(jnp.minimum(g + 1, nattn - 1)) + pcopies(jnp.minimum(g + 2, nattn - 1), probe, 4)

        def mid():
            for cp in copies:
                cp.start()

        _attention_step(q_scr, k_scr, v_scr, wo_buf, acc_scr, mid)
        for cp in copies:
            cp.wait()

        @pl.when(g == 0)
        def _():
            for cp in cp_late[1:]:
                cp.wait()
            for fn in _gap_items(work, gap_scr):
                fn(None)

        @pl.when(g + 1 < nattn)
        def _():
            ocopy(g + 1).start()
            side = [(SD0 + i * SDS, fn) for i, fn in enumerate(mixer_prep(g) + _gap_items(probe, gap_scr))]
            _proj_step(h_scr, hs_scr, c_ref, cs_scr, wq_buf, wk_buf, wv_buf, q_scr, k_scr, v_scr, scale,
                       gap_scr, side)
            ocopy(g + 1).wait()

        return carry

    jax.lax.fori_loop(0, nattn, attn_body, 0)

    cp_late[0].wait()
    mod = _dot(silu_cond(), wmb_ref[...])
    mod_scr[:, 2 * M:4 * M] = mod[:, 0:2 * M]
    mod_scr[:, 4 * M:5 * M] = 1.0 + mod[:, 2 * M:3 * M]
    mod_scr[:, 5 * M:6 * M] = mod[:, 3 * M:4 * M]
    ftiles = [(f, min(f + T, Fd)) for f in range(0, Fd, T)]
    OFF = x_ref.shape[0] - S
    CAR = t_scr.shape[0] - RB

    def p1(r0, n, dep=None):
        ga = mod_scr[:, 2 * M:3 * M]
        if dep is not None:
            ga = jnp.concatenate([_after(ga[:, 0:T], dep), ga[:, T:]], axis=1)
        rows = pl.ds(r0, n)
        x1 = x_ref[rows, :].astype(F32) + _rows(ga, n) * acc_scr[rows, :]
        x1_scr[rows, :] = x1
        hb = _ln(x1) * _rows(mod_scr[:, 4 * M:5 * M], n) + _rows(mod_scr[:, 3 * M:4 * M], n)
        hb_scr[rows, :] = hb
        return _ln(hb)

    HT = T // 2

    def p1_store(r0, c, dep=None):
        v = p1(r0 + c * PC, PC, dep)
        a1_scr[c * PC:(c + 1) * PC, :] = v
        return jnp.max(v[:, M - T:].reshape(PC // 8, 8, T), axis=0)

    t_scr[RB:RB + CAR - OFF, :] = jnp.zeros((CAR - OFF, M), F32)
    t_scr[RB + CAR - OFF:RB + CAR, :] = _gelu(_dot(p1(0, OFF).astype(BF16), w1_ref[...]))
    for c in range(RB // PC):
        p1_store(OFF, c)

    def out_copy(i):
        rows = pl.ds(i * T if isinstance(i, int) else pl.multiple_of(i * T, T), T)
        return pltpu.make_async_copy(out_buf.at[rows, :], out_hbm.at[rows, :], osem.at[i])

    def b_body(r, carry):
        gb = _rows(mod_scr[:, 5 * M:6 * M], T)
        r0 = pl.multiple_of(r * RB, RB)
        n0 = pl.multiple_of(jnp.minimum(r0 + RB, S - RB) + OFF, OFF)
        nh = RB // T
        now = [0]
        due = []
        pace = []

        def p1_item(c):
            return lambda dep: due.append((now[0] + PD, p1_store(n0, c, dep)))

        pace += [(P0 + i * PSTEP, p1_item(i)) for i in range(RB // PC)]
        wt = lambda ref, f0, f1, n: ref[f0:f1, _tile(n)]

        def mm(lhs, wts, dot=_dot):
            acc = None
            for x, w in zip(lhs, wts):
                if due and due[0][0] <= now[0]:
                    w = _tie(w, due.pop(0)[1])
                v = dot(x, w)
                now[0] += x.shape[0] // HT
                acc = v if acc is None else v + acc
                if pace and pace[0][0] <= now[0]:
                    pace.pop(0)[1](v[0:8, :])
            return acc

        def split_ops(lo, hi):
            return [v.astype(BF16) for v in _a_ops(lo[:HT], hi[:HT], lo[HT:], hi[HT:])]

        def two_tiles(aops, wsel, rest):
            def col(w):
                v = mm(rest[0], w, rest[3])
                return v[:HT], v[HT:]

            c11, c12, c21, c22 = _strassen(
                lambda i: mm([a[i] for a in aops], [wsel(i, k) for k in range(len(aops))]),
                lambda: col(rest[1]), lambda: col(rest[2]))
            return jnp.concatenate([c11, c21], axis=0), jnp.concatenate([c12, c22], axis=0)

        def square(full, aops, w_ref, ws_ref):
            out = {}
            for n in range(2):
                out[n], out[n + 2] = two_tiles(
                    aops, lambda i, k: _ld(ws_ref, i, n, slice(k * HT, (k + 1) * HT)),
                    (full[4:], [wt(w_ref, 4 * T, M, n)], [wt(w_ref, 4 * T, M, n + 2)], _dot))
            out[4] = mm(full, [wt(w_ref, j * T, (j + 1) * T, 4) for j in range(km)])
            return out

        t_scr[0:CAR, :] = t_scr[RB:RB + CAR, :]
        for hf in range(nh):
            a1 = [a1_scr[_tile(hf), _tile(j)] for j in range(km)]
            full = [v.astype(BF16) for v in a1]
            aops = [split_ops(a1[k], a1[2 + k]) for k in range(2)]
            for n, v in square(full, aops, w1_ref, ws12.at[0]).items():
                t = _gelu(v)
                if hf == nh - 1:
                    t = jnp.concatenate([t[:T - OFF], jnp.where(r < nrb - 1, t[T - OFF:], 0.0)], axis=0)
                t_scr[CAR + hf * T:CAR + (hf + 1) * T, _tile(n)] = t
        cq = M // 4
        shifts = (-1, 1, -2, 2)
        lane = jax.lax.broadcasted_iota(jnp.int32, (T, T), 1)
        y1, a3 = [], []
        for hf in range(nh):
            base = CAR - OFF + hf * T
            sh = []
            for j in range(km):
                g_lo, g_hi = (j * T) // cq, ((j + 1) * T - 1) // cq
                assert g_hi - g_lo <= 1
                v = t_scr[base + shifts[g_lo]:base + shifts[g_lo] + T, _tile(j)]
                if g_hi != g_lo:
                    v2 = t_scr[base + shifts[g_hi]:base + shifts[g_hi] + T, _tile(j)]
                    v = jnp.where(lane < g_hi * cq - j * T, v, v2)
                sh.append(v)
            hs = square([v.astype(BF16) for v in sh], [split_ops(sh[k], sh[2 + k]) for k in range(2)],
                        w2_ref, ws12.at[1])
            hs = jnp.concatenate([hs[n] for n in range(km)], axis=1)
            y1.append(hs + hb_scr[pl.ds(pl.multiple_of(r0 + hf * T, T), T), :])
            a3.append({})

            def ln_item(hf, c):
                def item(dep):
                    n = HT // NLN
                    for d in (0, HT):
                        v = y1[hf][d + c * n:d + (c + 1) * n]
                        if dep is not None:
                            v = jnp.concatenate([_after(v[:, :T], _rows(dep, n)), v[:, T:]], axis=1)
                        a3[hf][d + c * n] = _ln(v)
                return item

            ln_item(hf, 0)(None)
            pace += [(now[0] + LN0 + (c - 1) * LNS * (1 + hf), ln_item(hf, c)) for c in range(1, NLN)]
            pace.sort(key=lambda e: e[0])
        nf = FH // T
        h3, h3ops = [], []
        for hf in range(nh):
            assert len(a3[hf]) == 2 * NLN
            af = jnp.concatenate([a3[hf][key] for key in sorted(a3[hf])], axis=0)
            full = [af[:, _tile(j)].astype(BF16) for j in range(km)]
            aops = [split_ops(af[:, _tile(k)], af[:, _tile(2 + k)]) for k in range(2)]
            row, ops = {}, []
            narrow = None
            for n in range(nf):
                lo, hi = two_tiles(aops, lambda i, k: _ld(ws3, n, i, k),
                                   (full[4:], [wt(w3_ref, *ftiles[n], 4)],
                                    [wt(w3_ref, *ftiles[nf + n], 4)], _dot_nt))
                lo, hi = _gelu(lo), _gelu(hi)
                row[n], row[nf + n] = lo.astype(BF16), hi.astype(BF16)
                ops.append(split_ops(lo, hi))
                if n < km:
                    v = mm([wt(w3_ref, *ftiles[-1], n)], [full[n]], _dot_nt)
                    narrow = v if narrow is None else v + narrow
            row[2 * nf] = _gelu(mm(full, [wt(w3_ref, *ftiles[2 * nf], j) for j in range(km)],
                                   _dot_nt)).astype(BF16)
            fw = Fd - ftiles[-1][0]
            gT = jnp.concatenate([_gelu(narrow), jnp.zeros((T - fw, T), F32)], axis=0)
            row[2 * nf + 1] = _tie(gT.astype(BF16).T, gT[0:8, :])[:, :fw]
            h3.append([row[i] for i in range(len(ftiles))])
            h3ops.append(ops)
        for hf in range(nh):
            rows = pl.ds(pl.multiple_of(r0 + hf * T, T), T)

            def finish(n, v):
                out_buf[rows, _tile(n)] = (
                    x1_scr[rows, _tile(n)] + gb[:, _tile(n)] * (v + y1[hf][:, _tile(n)])
                ).astype(out_buf.dtype)

            w4t = lambda n, f_: [wt(w4_ref, f0, f1, n) for f0, f1 in f_]
            finish(4, mm(h3[hf], w4t(4, ftiles)))
            for n in range(2):
                lo, hi = two_tiles(h3ops[hf], lambda i, k: _ld(ws4, i, n, slice(k * HT, (k + 1) * HT)),
                                   (h3[hf][2 * nf:], w4t(n, ftiles[2 * nf:]), w4t(n + 2, ftiles[2 * nf:]), _dot))
                finish(n, lo)
                finish(n + 2, hi)
            out_copy(r * nh + hf).start()
        assert not pace
        return carry

    jax.lax.fori_loop(0, nrb, b_body, 0)
    for i in range(nb):
        out_copy(i).wait()


@jax.jit
def pallas_adaLN_cond__compressed_kv_cla__mixer_s_mlp__prompt_kernel(
    A_x: jax.Array,
    A_c_kv: jax.Array,
    A_w_q: jax.Array,
    A_w_uk: jax.Array,
    A_w_uv: jax.Array,
    A_w_o: jax.Array,
    B_x: jax.Array,
    B_w1: jax.Array,
    B_w2: jax.Array,
    B_w3: jax.Array,
    B_w4: jax.Array,
    c: jax.Array,
    w_mod: jax.Array,
):
    _, S, M = A_x.shape
    Dc = A_c_kv.shape[2]
    H, D = A_w_q.shape[1], A_w_q.shape[2]
    Fd = B_w3.shape[1]
    assert D == T and A_c_kv.shape[1] == S and Dc == 4 * T and M == 5 * T and 13 * T < Fd < 14 * T and S == 16 * T
    vmem = pltpu.VMEM
    packed = lambda *lead: vmem(lead + (T // 2, T), U32)
    out = pl.pallas_call(
        _kernel,
        in_specs=[pl.BlockSpec(memory_space=pltpu.HBM)] * 12,
        out_specs=pl.BlockSpec(memory_space=pltpu.HBM),
        out_shape=jax.ShapeDtypeStruct((S, M), A_x.dtype),
        scratch_shapes=[
            vmem((S + 16, M), BF16),
            vmem((S, Dc), BF16),
            vmem((1, M), BF16),
            vmem((M, 2 * M), BF16),
            vmem((M, 4 * M), BF16),
            vmem((M, M), BF16),
            vmem((M, M), BF16),
            vmem((Fd, M), BF16),
            vmem((Fd, M), BF16),
            vmem((M, D), U32),
            vmem((Dc, D), U32),
            vmem((Dc, D), U32),
            vmem((2 * D, M), BF16),
            vmem((S, M), A_x.dtype),
            pltpu.SemaphoreType.DMA((15,)),
            pltpu.SemaphoreType.DMA((7,)),
            pltpu.SemaphoreType.DMA((S // T,)),
            vmem((8, 6 * M), F32),
            vmem((S // T, M // T, T, T), BF16),
            vmem((len(_C_SUMS), T, T), BF16),
            vmem((len(_H_SUMS), T, T), BF16),
            packed(2, M // T + 2 * (Dc // T)),
            packed(2 * S // T),
            packed(2 * S // T),
            packed(2 * S // T),
            vmem((S + 16, M), F32),
            vmem((S + 16, M), F32),
            vmem((S + 16, M), F32),
            vmem((RB, M), F32),
            vmem((RB + 32, M), F32),
            vmem((2, 7, 2, T, T), U32),
            packed(6, 7, 2),
            vmem((7, 2, 3 * T, T), U32),
            vmem((M, D), U32),
            vmem((Dc, D), U32),
            vmem((Dc, D), U32),
            vmem((3, 8, T), jnp.int32),
        ],
        compiler_params=pltpu.CompilerParams(
            vmem_limit_bytes=100 * 1024 * 1024,
            disable_bounds_checks=True,
        ),
    )(
        A_x.reshape(S, M), A_c_kv.reshape(S, Dc),
        A_w_q, A_w_uk, A_w_uv,
        A_w_o.reshape(H // 2, 2 * D, M),
        B_w1, B_w2, B_w3.T, B_w4, c, w_mod,
    )
    return out.reshape(1, S, M)
```

```python
import math

import jax
import jax.numpy as jnp
import jax.experimental.pallas as pl
import jax.experimental.pallas.tpu as pltpu

F32 = jnp.float32
BF16 = jnp.bfloat16
U32 = jnp.uint32
NT = (((1,), (1,)), ((), ()))
T = 128
EPS = 1e-5
LOG2E = math.log2(math.e)

GRP = 4
LEAD = 10
PROW = 3
RES = 32
LAT_A = 16
LAT_B = 20
ALEAD = 32
MID = 40
SD0, SDS, SDN, SDJ = 158, 2, 20, 30
QT = 3
RB = 256
PC = 32
P0, PSTEP, PD = 440, 30, 52
NLN, LN0, LNS = 4, 4, 5
LP = 16
PROLOGUE = ('|kva|Z; |b|; kva|wc|K0123; bw|xdn|C0@56 N0123@52 K4567; cx|mq|N4567@52 K89ab; '
            'd|y|C1@56 Kcdef; nmq|zo|M H01 H234567@30 Q0123; y||H89ab@30 Q4567; '
            'zo||L Hcdef@30 Q89ab S01 Qcdef')


def _dot(a, b):
    return jnp.dot(a, b, preferred_element_type=F32)


def _dot_nt(a, b):
    return jax.lax.dot_general(a, b, NT, preferred_element_type=F32)


def _ln(x):
    m = jnp.mean(x, axis=-1, keepdims=True)
    xc = x - m
    v = jnp.mean(xc * xc, axis=-1, keepdims=True)
    return xc * jnp.exp2(jnp.log(v + EPS) * (-0.5 * LOG2E))


def _rows(v, n):
    return jnp.broadcast_to(v[None], (n // 8, 8, v.shape[1])).reshape(n, v.shape[1])


def _gelu(x):
    c0 = math.sqrt(2.0 / math.pi)
    return 0.5 * x * (1.0 + jnp.tanh(c0 * (x + 0.044715 * (x * x * x))))


def _after(x, dep):
    return jnp.where(dep > jnp.inf, dep, x)


def _tie(x, dep):
    xu = pltpu.bitcast(x, U32)
    first = jnp.where(dep > jnp.inf, jnp.uint32(0), xu[:8])
    return pltpu.bitcast(jnp.concatenate([first, xu[8:]], axis=0), BF16)


def _tile(j):
    return slice(j * T, (j + 1) * T)


def _ld(ref, *idx):
    return pltpu.bitcast(ref[idx], BF16)


def _pk(x):
    return pltpu.bitcast(x, U32)


def _a_ops(a11, a12, a21, a22):
    return [a11 + a22, a21 + a22, a11, a22, a11 + a12, a21 - a11, a12 - a22]


def _b_ops(b11, b12, b21, b22):
    return [b11 + b22, b11, b12 - b22, b21 - b11, b22, b11 + b12, b21 + b22]


def _strassen(prod, col1=None, col2=None):
    m4 = prod(3)
    m2 = prod(1)
    c21 = m2 + m4
    if col1 is not None:
        e11, e21 = col1()
        m4, c21 = m4 + e11, c21 + e21
    m3 = prod(2)
    m5 = prod(4)
    c12 = m3 + m5
    if col2 is not None:
        e12, e22 = col2()
        c12, m3 = c12 + e12, m3 + e22
    m1 = prod(0)
    c11 = prod(6) + (m1 + (m4 - m5))
    c22 = prod(5) + (m1 + (m3 - m2))
    return c11, c12, c21, c22


def _group(rows, cols, pairs):
    xs, ys = dict.fromkeys(x for x, _ in pairs), dict.fromkeys(y for _, y in pairs)
    used = set(xs) | set(ys) | {(x[0], y[1]) for x, y in pairs} | {(y[0], x[1]) for x, y in pairs}
    prods = []
    for n, r in enumerate(rows):
        for i, k in [x for x in xs if x[0] == r]:
            mates = [y for x, y in pairs if x == (i, k)]
            prods.append((((1, i, k),) + tuple((1, i, k2) for _, k2 in mates), ((1, k, 0),),
                          ((1, i, 0), (-1, i, 1))))
            prods.append((((1, i, k),) + tuple((-1, i2, k) for i2, _ in mates), ((1, k, 0), (1, k, 1)),
                          ((1, i, 1),)))
        for i2, k2 in [y for y in ys if y[0] == r]:
            mates = [x for x, y in pairs if y == (i2, k2)]
            prods.append((((1, i2, k2),) + tuple((1, i2, k) for _, k in mates), ((1, k2, 1),),
                          ((1, i2, 1), (-1, i2, 0))))
            prods.append((((1, i2, k2),) + tuple((-1, i, k2) for i, _ in mates), ((1, k2, 0), (1, k2, 1)),
                          ((1, i2, 0),)))
        prods += [(((1, r, k),), ((1, k, h),), ((1, r, h),)) for k in cols if (r, k) not in used for h in (0, 1)]
        for (i, k), (i2, k2) in pairs:
            if r in (i, i2) and i + i2 - r in rows[n + 1:]:
                prods.append((((1, i, k2),), ((1, k2, 0), (-1, k, 0)), ((1, i2, 0), (1, i, 0))))
                prods.append((((1, i2, k), (1, i, k2)), ((1, k, 0), (1, k2, 1)), ((1, i2, 0), (1, i, 1))))
                prods.append((((1, i2, k),), ((1, k, 1), (-1, k2, 1)), ((1, i2, 1), (1, i, 1))))
    return prods


def _all_pairs(xrows, yrows):
    return [((x, a), (y, b)) for a, x in enumerate(xrows) for b, y in enumerate(yrows) if a != b]


_PAIRS65 = [((x[0] + 10, x[1]), (y[0] + 10, y[1])) for x, y in (
    ((0, 1), (1, 0)), ((0, 1), (5, 2)), ((2, 3), (1, 0)), ((2, 3), (3, 1)), ((2, 3), (5, 2)), ((3, 2), (1, 0)),
    ((4, 4), (0, 3)), ((4, 4), (1, 0)), ((4, 4), (3, 1)), ((4, 4), (5, 2)))]
_C_GROUPS = [_group(range(r, r + 8), range(4), _all_pairs(range(r, r + 4), range(r + 4, r + 8))) for r in (0, 8)]
_H_GROUPS = [_group(range(10), range(5), _all_pairs(range(5), range(5, 10))),
             _group(range(10, 16), range(5), _PAIRS65)]
_sum_index = lambda groups: {f: n for n, f in enumerate(
    dict.fromkeys(t[0] for g in groups for t in g if len(t[0]) > 1))}
_C_SUMS, _H_SUMS = _sum_index(_C_GROUPS), _sum_index(_H_GROUPS)


def _form(form, get):
    acc = None
    for sign, i, j in form:
        v = get(i, j)
        acc = v if acc is None else (acc + v if sign > 0 else acc - v)
    return acc


def _gap_items(bufs, gap_scr):
    items = []
    for n, buf in enumerate(bufs):
        acc = []

        def part(r0, buf=buf, acc=acc):
            def fn(dep):
                wu = jnp.concatenate([buf[r:r + 8, :] for r in range(r0, r0 + T, 32)])
                mask = jnp.full((8, T), 0x7FFF0000, U32)
                if dep is not None:
                    mask = jnp.where(dep > jnp.inf, jnp.uint32(0), mask)
                mask = _rows(mask, 32)
                new = [jnp.sum(pltpu.bitcast(v & mask, F32).reshape(4, 8, T), axis=0) for v in (wu << 16, wu)]
                acc[:] = [u + v for u, v in zip(acc, new)] if acc else new
            return fn

        def last(_, n=n, acc=acc):
            bits = []
            for v in acc:
                l1 = jnp.sum(jnp.sum(v, axis=1, keepdims=True), axis=0, keepdims=True)
                bits.append(pltpu.bitcast(jnp.broadcast_to(l1, (8, T)), jnp.int32) >> 8)
            gap_scr[n] = jnp.clip((bits[0] - bits[1] + (1 << 14)) >> 15, -8, 8) << 23

        items += [part(r0) for r0 in range(0, buf.shape[0], T)] + [last]
    return items


class _PairWeights:
    def __init__(self, w_ref, transpose=False, shift=None):
        self.base = {}
        if shift is not None:
            fac = _rows(pltpu.bitcast(0x3F800000 + shift, F32), T)
            self.inv = pltpu.bitcast(0x3F800000 - shift, F32)
        for j in range(w_ref.shape[0] // T):
            wu = w_ref[_tile(j), :]
            if transpose:
                wu = wu.T
            hi = pltpu.bitcast(wu & jnp.uint32(0xFFFF0000), F32)
            self.base[j, 0] = pltpu.bitcast(wu << 16, F32)
            self.base[j, 1] = hi if shift is None else hi * fac
        self.cache = {}

    def __call__(self, form):
        sign = 1
        if form[-1][0] < 0 and form[0][1:] > form[1][1:]:
            sign, form = -1, ((1,) + form[1][1:], (-1,) + form[0][1:])
        if form not in self.cache:
            self.cache[form] = _form(form, lambda k, h: self.base[k, h]).astype(BF16)
        return sign, self.cache[form]


def _run_group(jobs, prods, a_get, w, transposed, finish):
    left = {}
    for _, _, outs in prods:
        for _, i, h in outs:
            left[i, h] = left.get((i, h), 0) + 1
    acc = {}
    for af, bf, outs in prods:
        sign, wt = w(bf)
        m = jobs.mm([wt], [a_get(af)], _dot_nt) if transposed else jobs.mm([a_get(af)], [wt], _dot)
        for s_, i, h in outs:
            if (i, h) not in acc:
                acc[i, h] = (s_ * sign, m)
            else:
                s0, v = acc[i, h]
                acc[i, h] = (s0, v + m if s0 == s_ * sign else v - m) if s0 > 0 or s_ * sign < 0 else (1, m - v)
            left[i, h] -= 1
            if not left[i, h]:
                s0, v = acc.pop((i, h))
                assert s0 > 0
                finish(2 * i + h, v)


class _Jobs:
    def __init__(self, side=()):
        self.res = []
        self.side = list(side)

    def mm(self, lhs, wt, dot):
        acc = None
        for x, w in zip(lhs, wt):
            v = dot(x, w)
            self.res.append(v)
            acc = v if acc is None else v + acc
            rel = 4 * (len(self.res) % 4)
            while self.side and self.side[0][0] <= len(self.res):
                self.side.pop(0)[1](v[8 * rel:8 * rel + 8, :])
                rel = (rel + 2) % 16
        return acc


def _proj_step(h_scr, hs_scr, c_ref, cs_scr, wq_ref, wuk_ref, wuv_ref, q_scr, k_scr, v_scr, scale, shifts, side):
    wk, wvT, wq = [_PairWeights(w, n == 1, shifts[n]) for n, w in enumerate((wuk_ref, wuv_ref, wq_ref))]
    c_get = lambda f: cs_scr[_C_SUMS[f]] if len(f) > 1 else c_ref[_tile(f[0][1]), _tile(f[0][2])]
    h_get = lambda f: hs_scr[_H_SUMS[f]] if len(f) > 1 else h_scr[f[0][1], f[0][2]]

    def put(dst, w, mul=None):
        muls = [mul, _rows(w.inv if mul is None else w.inv * mul, T)]

        def fn(u, v):
            v = (v if muls[u % 2] is None else v * muls[u % 2]).astype(BF16)
            dst[u] = _pk(v.T if mul is not None and u < QT else v)
        return fn

    jobs = _Jobs(side)
    for groups, get, w, transposed, fin in ((_C_GROUPS, c_get, wk, False, put(k_scr, wk)),
                                            (_C_GROUPS, c_get, wvT, True, put(v_scr, wvT)),
                                            (_H_GROUPS, h_get, wq, False, put(q_scr, wq, scale))):
        for prods in groups:
            _run_group(jobs, prods, get, w, transposed, fin)
    assert not jobs.side


def _inner_group(rows, cols, pairs):
    xs, ys = dict.fromkeys(x for x, _ in pairs), dict.fromkeys(y for _, y in pairs)
    used = set(xs) | set(ys) | {(x[0], y[1]) for x, y in pairs} | {(y[0], x[1]) for x, y in pairs}
    prods = []
    for i, j in xs:
        mates = [y for x, y in pairs if x == (i, j)]
        prods.append((((1, i, 0),), ((1, 0, j), (-1, 1, j)), ((1, i, j),) + tuple((1, i2, j) for i2, _ in mates)))
        prods.append((((1, i, 0), (1, i, 1)), ((1, 1, j),), ((1, i, j),) + tuple((-1, i, j2) for _, j2 in mates)))
    for i2, j2 in ys:
        mates = [x for x, y in pairs if y == (i2, j2)]
        prods.append((((1, i2, 0), (1, i2, 1)), ((1, 0, j2),),
                      ((1, i2, j2),) + tuple((-1, i2, j) for _, j in mates)))
        prods.append((((1, i2, 1),), ((1, 0, j2), (-1, 1, j2)),
                      ((-1, i2, j2),) + tuple((-1, i, j2) for i, _ in mates)))
    prods += [(((1, i, h),), ((1, h, j),), ((1, i, j),))
              for i in rows for j in cols if (i, j) not in used for h in (0, 1)]
    for (i, j), (i2, j2) in pairs:
        lo, hi = min(j, j2), max(j, j2)
        prods.append((((1, i2, 0), (-1, i, 0)), ((1, 0, lo), (1, 0, hi)), ((1, i2, j),)))
        prods.append((((1, i, 0), (1, i2, 1)), ((1, 0, j2), (1, 1, j)), ((1, i, j2), (1, i2, j))))
        prods.append((((1, i, 1), (-1, i2, 1)), ((1, 1, lo), (1, 1, hi)), ((1, i, j2),)))
    return prods


def _o_jobs():
    prods = (_inner_group(range(10), range(5), _all_pairs(range(0, 10, 2), range(1, 10, 2)))
             + _inner_group(range(10, 16), range(5), _PAIRS65))
    row = lambda t: max(i for _, i, _ in t[0])
    unit = lambda t: max(2 * i + h for _, i, h in t[0])
    need = lambda t: unit(t) if row(t) == 15 else 2 * row(t) + 1
    return [(need(t), t) for t in sorted(prods, key=need)]


_O_JOBS = _o_jobs()


def _job_order(nb):
    units = range(2 * nb)
    qa = [('a', u, c) for u in units for c in range(u // 2 + 1)]
    qb = [('b', u, c) for u in units for c in range(u // 2 + 1)]
    qo = [('o', u, j) for j, (u, _) in enumerate(_O_JOBS)]
    done = {}
    order = []

    def ready(q, lat, pre):
        return bool(q) and (pre, q[0][1]) in done and done[(pre, q[0][1])] + lat <= len(order)

    def emit(q):
        kind, u, j = job = q.pop(0)
        if kind != 'o' and j == u // 2:
            done[(kind, u)] = len(order)
        order.append(job)

    turn = 0
    while qa or qb or qo:
        pref = 'abo'[turn % 3]
        turn += 1
        for _ in range(GRP):
            b_ok, o_ok = ready(qb, LAT_A, 'a'), ready(qo, LAT_B, 'b')
            if pref == 'a' and qa and (len(qb) - len(qa) < ALEAD or not b_ok):
                emit(qa)
            elif pref == 'b' and b_ok:
                emit(qb)
            elif pref == 'o' and o_ok and (len(qo) > RES or not (qa or b_ok)):
                emit(qo)
            elif not (qa or b_ok or o_ok) and (qb or qo):
                emit(qb or qo)
            else:
                break
    return order


def _attention_step(q_scr, k_scr, v_scr, wo_ref, acc_scr, mid):
    causal = (jax.lax.broadcasted_iota(jnp.int32, (T, T), 0)
              <= jax.lax.broadcasted_iota(jnp.int32, (T, T), 1))
    sv, mx, mfin, lsum, pv, of, lhs = {}, {}, {}, {}, {}, {}, {}
    res = []
    wo, terms = {}, {}
    left = {}
    for _, t in _O_JOBS:
        for _, i, j in t[2]:
            left[i, j] = left.get((i, j), 0) + 1

    def job_a(u, c):
        r, hd = divmod(u, 2)
        s = (_dot if u < QT else _dot_nt)(_ld(k_scr, 2 * c + hd), _ld(q_scr, u))
        res.append(s)
        if c == r:
            s = jnp.where(causal, s, -1e9 * LOG2E)
        s = s.reshape(T // 8, 8, T)
        sv[(u, c)] = s
        pm = jnp.max(s, axis=0)
        mx[u] = pm if u not in mx else jnp.maximum(mx[u], pm)

    def job_b(u, c):
        r, hd = divmod(u, 2)
        if u not in mfin:
            mfin[u] = jnp.broadcast_to(jnp.max(mx[u], axis=0, keepdims=True), (8, T))
        m = mfin[u]
        if len(res) >= LEAD:
            r0 = 8 * PROW * (c % 4)
            m = _after(m, res[len(res) - LEAD][r0:r0 + 8, :])
        p = jnp.exp2(sv.pop((u, c)) - m[None])
        ls = jnp.sum(p, axis=0)
        lsum[u] = ls if u not in lsum else lsum[u] + ls
        v = _dot(_ld(v_scr, 2 * c + hd), p.reshape(T, T).astype(BF16))
        res.append(v)
        pv[u] = v if u not in pv else v + pv[u]
        if c == r:
            of[u] = pv[u] * (1.0 / jnp.sum(lsum[u], axis=0, keepdims=True))

    def job_o(_, n):
        af, bf, outs = _O_JOBS[n][1]
        if af not in lhs:
            v = _form(af, lambda i, h: of[2 * i + h])
            lhs[af] = _tie(v.astype(BF16).T, v[0:8, :])
        if bf not in wo:
            wo[bf] = (wo_ref[_tile(bf[0][1]), _tile(bf[0][2])] if len(bf) == 1 else
                      _form(bf, lambda h, j: wo_ref[_tile(h), _tile(j)].astype(F32)).astype(BF16))
        v = _dot(lhs[af], wo[bf])
        res.append(v)
        for sign, i, j in outs:
            terms.setdefault((i, j), []).append((sign, v))
            if len(terms[i, j]) == left[i, j]:
                tot = acc_scr[_tile(i), _tile(j)]
                for sg, m in terms.pop((i, j)):
                    tot = tot + m if sg > 0 else tot - m
                acc_scr[_tile(i), _tile(j)] = tot

    fns = dict(a=job_a, b=job_b, o=job_o)
    for n, (kind, u, j) in enumerate(_job_order(q_scr.shape[0] // 2)):
        if n == MID:
            mid()
        fns[kind](u, j)


def _kernel(x_hbm, c_hbm, wq_hbm, wuk_hbm, wuv_hbm, wo_hbm, w1_hbm, w2_hbm, w3_hbm, w4_hbm,
            cond_hbm, wmod_hbm, out_hbm,
            x_ref, c_ref, cond_ref, wma_ref, wmb_ref, w1_ref, w2_ref, w3_ref, w4_ref,
            wq_buf, wk_buf, wv_buf, wo_buf, out_buf, sem, wsem, osem,
            mod_scr, h_scr, cs_scr, hs_scr, w_scr, q_scr, k_scr, v_scr, acc_scr, x1_scr, hb_scr, a1_scr, t_scr,
            ws12, ws3, ws4, pq_buf, pk_buf, pv_buf, gap_scr):
    S, M = x_hbm.shape
    D = wq_hbm.shape[2]
    nattn = wo_hbm.shape[0]
    Fd = w4_hbm.shape[0]
    scale = float(D) ** -0.5 * LOG2E
    nb, nrb = S // T, S // RB
    km, kc = M // T, c_hbm.shape[1] // T
    NX = 4
    XR = S // NX
    CB = XR // T

    work, probe = (wk_buf, wv_buf, wq_buf), (pk_buf, pv_buf, pq_buf)

    def pcopies(g, bufs=work, s0=0):
        return [pltpu.make_async_copy(src.bitcast(U32).at[:, g, :], dst, wsem.at[s0 + j])
                for j, (src, dst) in enumerate(zip((wuk_hbm, wuv_hbm, wq_hbm), bufs))]

    def ocopy(g):
        return pltpu.make_async_copy(wo_hbm.at[g], wo_buf, wsem.at[3])

    def chunk_copy(src, dst, i, s0):
        rows = slice(i * XR, (i + 1) * XR)
        return pltpu.make_async_copy(src.at[rows, :], dst.at[rows, :], sem.at[s0 + i])

    cp_cond = pltpu.make_async_copy(cond_hbm, cond_ref, sem.at[0])
    cp_wma = pltpu.make_async_copy(wmod_hbm.at[:, 0:2 * M], wma_ref, sem.at[1])
    cp_late = [pltpu.make_async_copy(src, dst, sem.at[2 + j]) for j, (src, dst) in enumerate((
        (wmod_hbm.at[:, 2 * M:6 * M], wmb_ref), (w1_hbm, w1_ref), (w2_hbm, w2_ref),
        (w3_hbm, w3_ref), (w4_hbm, w4_ref)))]
    cp_x = [chunk_copy(x_hbm, x_ref, i, 7) for i in range(NX)]
    cp_c = [chunk_copy(c_hbm, c_ref, i, 7 + NX) for i in range(NX)]

    def silu_cond():
        cf = cond_ref[...].astype(F32)
        return jnp.broadcast_to((cf * jax.nn.sigmoid(cf)).astype(BF16), (8, M))

    cp_wk, cp_wv, cp_wq = pcopies(0)
    named = dict(k=cp_wk, v=cp_wv, q=cp_wq, o=ocopy(0), n=cp_cond, m=cp_wma)
    named.update(zip('abcd', cp_c))
    named.update(zip('wxyz', cp_x))
    started, arrived, did = set(), set(), set()

    def zero(r, carry):
        acc_scr[pl.ds(pl.multiple_of(r * T, T), T), :] = jnp.zeros((T, M), F32)
        return carry

    def x_rows(rows, dep):
        xf = x_ref[rows, :].astype(F32)
        if dep is None:
            return xf
        return jnp.concatenate([_after(xf[:, :T], _rows(dep, xf.shape[0])), xf[:, T:]], axis=1)

    def n_item(r, i):
        def fn(dep):
            rows = slice(r * T + i * LP, r * T + (i + 1) * LP)
            x1_scr[rows, :] = _ln(x_rows(rows, dep))
        return fn

    def h_item(r, i, normed):
        def fn(dep):
            rows = slice(i * LP, (i + 1) * LP)
            grows = slice(r * T + i * LP, r * T + (i + 1) * LP)
            sa = mod_scr[:, 0:M]
            if normed and dep is not None:
                sa = jnp.concatenate([_after(sa[:, _tile(j)], dep) for j in range(km)], axis=1)
            hf = ((x1_scr[grows, :] if normed else _ln(x_rows(grows, dep))) * _rows(mod_scr[:, M:2 * M], LP)
                  + _rows(sa, LP))
            for j in range(km):
                h_scr[r, j, rows, :] = hf[:, _tile(j)].astype(BF16)
            for f, n in _H_SUMS.items():
                if all(t[1] == r for t in f):
                    hs_scr[n, rows, :] = _form(f, lambda _, k: hf[:, _tile(k)]).astype(BF16)
            did.add(('h', r, i))
        return fn

    def release(jobs, span, items):
        if span and items:
            jobs.side += [(len(jobs.res) + 1 + i * span // len(items), fn) for i, fn in enumerate(items)]
            jobs.side.sort(key=lambda e: e[0])
        else:
            for fn in items:
                fn(None)

    def sum_items(n, group, index, dst, get, skip_rows):
        forms = [f for f in dict.fromkeys(t[0] for t in group)
                 if len(f) > 1 and not (skip_rows and len({t[1] for t in f}) == 1)]

        def item(f, rows):
            def fn(dep):
                def term(r, k):
                    v = get(r, k, rows).astype(F32)
                    return v if dep is None or (r, k) != f[0][1:] else _after(v, _rows(dep, v.shape[0]))
                dst[index[f], rows, :] = _form(f, term).astype(BF16)
            return fn

        return [item(f, slice(i, i + n)) for i in range(0, T, n) for f in forms]

    h_sums = lambda n, gi: sum_items(n, _H_GROUPS[gi], _H_SUMS, hs_scr,
                                     lambda r_, k, rows: h_scr[r_, k, rows, :], True)

    def stash(key, buf, j0, transpose=False):
        n = buf.shape[0] // T
        if key not in did:
            assert key in arrived
            did.add(key)
            w = _PairWeights(buf, transpose)
            for j in range(n):
                for hd in range(2):
                    w_scr[hd, j0 + j] = _pk(w(((1, j, hd),))[1])
        return lambda hd: [_ld(w_scr, hd, j0 + j) for j in range(n)]

    def kv_tile(jobs, r):
        wk, wvT = stash('k', wk_buf, 0), stash('v', wv_buf, kc, True)
        ct = [c_ref[_tile(r), _tile(j)] for j in range(kc)]
        for hd in range(2):
            k_scr[2 * r + hd] = _pk(jobs.mm(ct, wk(hd), _dot).astype(BF16))
        for hd in range(2):
            v_scr[2 * r + hd] = _pk(jobs.mm(wvT(hd), ct, _dot_nt).astype(BF16))

    def q_tile(jobs, r):
        wq = stash('q', wq_buf, 2 * kc)
        ht = [h_scr[r, j] for j in range(km)]
        for hd in range(2):
            v = (jobs.mm(ht, wq(hd), _dot) * scale).astype(BF16)
            q_scr[2 * r + hd] = _pk(v.T if 2 * r + hd < QT else v)

    for blk in PROLOGUE.split(';'):
        waits, starts, acts = blk.split('|')
        for ch in waits.strip():
            assert ch in started and ch not in arrived
            arrived.add(ch)
            named[ch].wait()
        for ch in starts.strip():
            assert ch not in started
            started.add(ch)
            named[ch].start()
        jobs = _Jobs()
        for act in acts.split():
            if act == 'Z':
                jax.lax.fori_loop(0, nb, zero, 0)
                acc_scr[S:, :] = jnp.zeros((acc_scr.shape[0] - S, M), F32)
                x_ref[S:, :] = jnp.zeros((x_ref.shape[0] - S, M), BF16)
            elif act == 'L':
                did.add('L')
                for cp in cp_late[1:] + cp_late[:1]:
                    cp.start()
            elif act == 'M':
                assert arrived >= set('nm')
                mod = _dot(silu_cond(), wma_ref[...])
                mod_scr[:, 0:M] = mod[:, 0:M]
                mod_scr[:, M:2 * M] = 1.0 + mod[:, M:2 * M]
                did.add('M')
            else:
                act, _, span = act.partition('@')
                span = int(span or 0)
                items = []
                for r in [int(ch, 16) for ch in act[1:]]:
                    did.add((act[0], r))
                    if act[0] == 'K':
                        assert 'abcd'[r // CB] in arrived
                        kv_tile(jobs, r)
                    elif act[0] == 'H':
                        assert 'wxyz'[r // CB] in arrived and 'M' in did
                        items += [h_item(r, i, ('N', r) in did) for i in range(T // LP)]
                    elif act[0] == 'N':
                        assert 'wxyz'[r // CB] in arrived
                        items += [n_item(r, i) for i in range(T // LP)]
                    elif act[0] == 'Q':
                        assert all(('h', r, i) in did for i in range(T // LP))
                        q_tile(jobs, r)
                    elif act[0] == 'C':
                        assert all('abcd'[t[1] // CB] in arrived for p_ in _C_GROUPS[r] for t in p_[0])
                        items += sum_items(
                            32, _C_GROUPS[r], _C_SUMS, cs_scr,
                            lambda r_, k, rows: c_ref[r_ * T + rows.start:r_ * T + rows.stop, _tile(k)], False)
                    else:
                        assert act[0] == 'S' and all(('h', t[1], T // LP - 1) in did for p_ in _H_GROUPS[r] for t in p_[0])
                        items += h_sums(32 if span else 16, r)
                release(jobs, span, items)
        assert not jobs.side
    assert arrived == set(named) and all((k_, r) in did for k_ in 'KHQ' for r in range(nb))
    assert all((k_, r) in did for k_ in 'CS' for r in range(2)) and 'L' in did

    FH = ws3.shape[0] * T
    assert nattn - 1 >= FH // 64

    def mixer_prep(g):
        def blocks(w_ref, r0, n, half, c0, c1, dep):
            lo, hi = pl.ds(r0, n), pl.ds(r0 + half, n)
            return [_after(w_ref[rows, _tile(c)].astype(F32), _rows(dep, n)) if (rows is lo) == (c == c0)
                    else w_ref[rows, _tile(c)].astype(F32) for rows in (lo, hi) for c in (c0, c1)]

        def rows_items(w_ref, dst, per_step, half, n=16):
            gi = jnp.minimum(g, half // per_step - 1)
            src = w_ref.at[pl.ds(pl.multiple_of(gi * per_step, per_step), half + per_step), :]
            hs = per_step // 2

            def item(c, o):
                def fn(dep):
                    for i, v in enumerate(_b_ops(*blocks(src, o, n, half, c, c + 2, dep))):
                        dst[i, c, pl.ds(pl.multiple_of(gi * hs, hs) + o // 2, n // 2), :] = _pk(v.astype(BF16))
                return fn
            return [item(c, o) for c in range(2) for o in range(0, per_step, n)]

        def w3_item(k, i):
            def fn(dep):
                n = jnp.minimum(g, FH // T - 1)
                b11, b21, b12, b22 = blocks(w3_ref, pl.multiple_of(n * T, T), T, FH, k, k + 2, dep)
                ws3[n, i, k] = _pk(_b_ops(b11, b12, b21, b22)[i].astype(BF16).T)
            return fn

        return (rows_items(w1_ref, ws12.at[0], 32, 2 * T) + rows_items(w2_ref, ws12.at[1], 32, 2 * T)
                + rows_items(w4_ref, ws4, 64, FH) + [w3_item(k, i) for k in range(2) for i in range(7)])

    def attn_body(g, carry):
        copies = pcopies(jnp.minimum(g + 1, nattn - 1)) + pcopies(jnp.minimum(g + 2, nattn - 1), probe, 4)

        def mid():
            for cp in copies:
                cp.start()

        _attention_step(q_scr, k_scr, v_scr, wo_buf, acc_scr, mid)
        for cp in copies:
            cp.wait()

        @pl.when(g == 0)
        def _():
            for cp in cp_late[1:]:
                cp.wait()
            for fn in _gap_items(work, gap_scr):
                fn(None)

        @pl.when(g + 1 < nattn)
        def _():
            ocopy(g + 1).start()
            side = mixer_prep(g) + _gap_items(probe, gap_scr)
            side = [(SD0 + i * SDS + (SDJ if i >= SDN else 0), fn) for i, fn in enumerate(side)]
            _proj_step(h_scr, hs_scr, c_ref, cs_scr, wq_buf, wk_buf, wv_buf, q_scr, k_scr, v_scr, scale,
                       gap_scr, side)
            ocopy(g + 1).wait()

        return carry

    jax.lax.fori_loop(0, nattn, attn_body, 0)

    cp_late[0].wait()
    mod = _dot(silu_cond(), wmb_ref[...])
    mod_scr[:, 2 * M:4 * M] = mod[:, 0:2 * M]
    mod_scr[:, 4 * M:5 * M] = 1.0 + mod[:, 2 * M:3 * M]
    mod_scr[:, 5 * M:6 * M] = mod[:, 3 * M:4 * M]
    ftiles = [(f, min(f + T, Fd)) for f in range(0, Fd, T)]
    OFF = x_ref.shape[0] - S
    CAR = t_scr.shape[0] - RB

    def p1(r0, n, dep=None):
        ga = mod_scr[:, 2 * M:3 * M]
        if dep is not None:
            ga = jnp.concatenate([_after(ga[:, 0:T], dep), ga[:, T:]], axis=1)
        rows = pl.ds(r0, n)
        x1 = x_ref[rows, :].astype(F32) + _rows(ga, n) * acc_scr[rows, :]
        x1_scr[rows, :] = x1
        hb = _ln(x1) * _rows(mod_scr[:, 4 * M:5 * M], n) + _rows(mod_scr[:, 3 * M:4 * M], n)
        hb_scr[rows, :] = hb
        return _ln(hb)

    HT = T // 2

    def p1_store(r0, c, dep=None):
        v = p1(r0 + c * PC, PC, dep)
        a1_scr[c * PC:(c + 1) * PC, :] = v
        return jnp.max(v[:, M - T:].reshape(PC // 8, 8, T), axis=0)

    t_scr[RB:RB + CAR - OFF, :] = jnp.zeros((CAR - OFF, M), F32)
    t_scr[RB + CAR - OFF:RB + CAR, :] = _gelu(_dot(p1(0, OFF).astype(BF16), w1_ref[...]))
    for c in range(RB // PC):
        p1_store(OFF, c)

    def out_copy(i):
        rows = pl.ds(i * T if isinstance(i, int) else pl.multiple_of(i * T, T), T)
        return pltpu.make_async_copy(out_buf.at[rows, :], out_hbm.at[rows, :], osem.at[i])

    def b_body(r, carry):
        gb = _rows(mod_scr[:, 5 * M:6 * M], T)
        r0 = pl.multiple_of(r * RB, RB)
        n0 = pl.multiple_of(jnp.minimum(r0 + RB, S - RB) + OFF, OFF)
        nh = RB // T
        now = [0]
        due = []
        pace = []

        def p1_item(c):
            return lambda dep: due.append((now[0] + PD, p1_store(n0, c, dep)))

        pace += [(P0 + i * PSTEP, p1_item(i)) for i in range(RB // PC)]
        wt = lambda ref, f0, f1, n: ref[f0:f1, _tile(n)]

        def mm(lhs, wts, dot=_dot):
            acc = None
            for x, w in zip(lhs, wts):
                if due and due[0][0] <= now[0]:
                    w = _tie(w, due.pop(0)[1])
                v = dot(x, w)
                now[0] += x.shape[0] // HT
                acc = v if acc is None else v + acc
                if pace and pace[0][0] <= now[0]:
                    pace.pop(0)[1](v[0:8, :])
            return acc

        def split_ops(lo, hi):
            return [v.astype(BF16) for v in _a_ops(lo[:HT], hi[:HT], lo[HT:], hi[HT:])]

        def two_tiles(aops, wsel, rest):
            def col(w):
                v = mm(rest[0], w, rest[3])
                return v[:HT], v[HT:]

            c11, c12, c21, c22 = _strassen(
                lambda i: mm([a[i] for a in aops], [wsel(i, k) for k in range(len(aops))]),
                lambda: col(rest[1]), lambda: col(rest[2]))
            return jnp.concatenate([c11, c21], axis=0), jnp.concatenate([c12, c22], axis=0)

        def square(full, aops, w_ref, ws_ref):
            out = {}
            for n in range(2):
                out[n], out[n + 2] = two_tiles(
                    aops, lambda i, k: _ld(ws_ref, i, n, slice(k * HT, (k + 1) * HT)),
                    (full[4:], [wt(w_ref, 4 * T, M, n)], [wt(w_ref, 4 * T, M, n + 2)], _dot))
            out[4] = mm(full, [wt(w_ref, j * T, (j + 1) * T, 4) for j in range(km)])
            return out

        t_scr[0:CAR, :] = t_scr[RB:RB + CAR, :]
        for hf in range(nh):
            a1 = [a1_scr[_tile(hf), _tile(j)] for j in range(km)]
            full = [v.astype(BF16) for v in a1]
            aops = [split_ops(a1[k], a1[2 + k]) for k in range(2)]
            for n, v in square(full, aops, w1_ref, ws12.at[0]).items():
                t = _gelu(v)
                if hf == nh - 1:
                    t = jnp.concatenate([t[:T - OFF], jnp.where(r < nrb - 1, t[T - OFF:], 0.0)], axis=0)
                t_scr[CAR + hf * T:CAR + (hf + 1) * T, _tile(n)] = t
        cq = M // 4
        shifts = (-1, 1, -2, 2)
        lane = jax.lax.broadcasted_iota(jnp.int32, (T, T), 1)
        y1, a3 = [], []
        for hf in range(nh):
            base = CAR - OFF + hf * T
            sh = []
            for j in range(km):
                g_lo, g_hi = (j * T) // cq, ((j + 1) * T - 1) // cq
                assert g_hi - g_lo <= 1
                v = t_scr[base + shifts[g_lo]:base + shifts[g_lo] + T, _tile(j)]
                if g_hi != g_lo:
                    v2 = t_scr[base + shifts[g_hi]:base + shifts[g_hi] + T, _tile(j)]
                    v = jnp.where(lane < g_hi * cq - j * T, v, v2)
                sh.append(v)
            hs = square([v.astype(BF16) for v in sh], [split_ops(sh[k], sh[2 + k]) for k in range(2)],
                        w2_ref, ws12.at[1])
            hs = jnp.concatenate([hs[n] for n in range(km)], axis=1)
            y1.append(hs + hb_scr[pl.ds(pl.multiple_of(r0 + hf * T, T), T), :])
            a3.append({})

            def ln_item(hf, c):
                def item(dep):
                    n = HT // NLN
                    for d in (0, HT):
                        v = y1[hf][d + c * n:d + (c + 1) * n]
                        if dep is not None:
                            v = jnp.concatenate([_after(v[:, :T], _rows(dep, n)), v[:, T:]], axis=1)
                        a3[hf][d + c * n] = _ln(v)
                return item

            ln_item(hf, 0)(None)
            pace += [(now[0] + LN0 + (c - 1) * LNS * (1 + hf), ln_item(hf, c)) for c in range(1, NLN)]
            pace.sort(key=lambda e: e[0])
        nf = FH // T
        h3, h3ops = [], []
        for hf in range(nh):
            assert len(a3[hf]) == 2 * NLN
            af = jnp.concatenate([a3[hf][key] for key in sorted(a3[hf])], axis=0)
            full = [af[:, _tile(j)].astype(BF16) for j in range(km)]
            aops = [split_ops(af[:, _tile(k)], af[:, _tile(2 + k)]) for k in range(2)]
            row, ops = {}, []
            narrow = None
            for n in range(nf):
                lo, hi = two_tiles(aops, lambda i, k: _ld(ws3, n, i, k),
                                   (full[4:], [wt(w3_ref, *ftiles[n], 4)],
                                    [wt(w3_ref, *ftiles[nf + n], 4)], _dot_nt))
                lo, hi = _gelu(lo), _gelu(hi)
                row[n], row[nf + n] = lo.astype(BF16), hi.astype(BF16)
                ops.append(split_ops(lo, hi))
                if n < km:
                    v = mm([wt(w3_ref, *ftiles[-1], n)], [full[n]], _dot_nt)
                    narrow = v if narrow is None else v + narrow
            row[2 * nf] = _gelu(mm(full, [wt(w3_ref, *ftiles[2 * nf], j) for j in range(km)],
                                   _dot_nt)).astype(BF16)
            fw = Fd - ftiles[-1][0]
            gT = jnp.concatenate([_gelu(narrow), jnp.zeros((T - fw, T), F32)], axis=0)
            row[2 * nf + 1] = _tie(gT.astype(BF16).T, gT[0:8, :])[:, :fw]
            h3.append([row[i] for i in range(len(ftiles))])
            h3ops.append(ops)
        for hf in range(nh):
            rows = pl.ds(pl.multiple_of(r0 + hf * T, T), T)

            def finish(n, v):
                out_buf[rows, _tile(n)] = (
                    x1_scr[rows, _tile(n)] + gb[:, _tile(n)] * (v + y1[hf][:, _tile(n)])
                ).astype(out_buf.dtype)

            w4t = lambda n, f_: [wt(w4_ref, f0, f1, n) for f0, f1 in f_]
            finish(4, mm(h3[hf], w4t(4, ftiles)))
            for n in range(2):
                lo, hi = two_tiles(h3ops[hf], lambda i, k: _ld(ws4, i, n, slice(k * HT, (k + 1) * HT)),
                                   (h3[hf][2 * nf:], w4t(n, ftiles[2 * nf:]), w4t(n + 2, ftiles[2 * nf:]), _dot))
                finish(n, lo)
                finish(n + 2, hi)
            out_copy(r * nh + hf).start()
        assert not pace
        return carry

    jax.lax.fori_loop(0, nrb, b_body, 0)
    for i in range(nb):
        out_copy(i).wait()


@jax.jit
def pallas_adaLN_cond__compressed_kv_cla__mixer_s_mlp__prompt_kernel(
    A_x: jax.Array,
    A_c_kv: jax.Array,
    A_w_q: jax.Array,
    A_w_uk: jax.Array,
    A_w_uv: jax.Array,
    A_w_o: jax.Array,
    B_x: jax.Array,
    B_w1: jax.Array,
    B_w2: jax.Array,
    B_w3: jax.Array,
    B_w4: jax.Array,
    c: jax.Array,
    w_mod: jax.Array,
):
    _, S, M = A_x.shape
    Dc = A_c_kv.shape[2]
    H, D = A_w_q.shape[1], A_w_q.shape[2]
    Fd = B_w3.shape[1]
    assert D == T and A_c_kv.shape[1] == S and Dc == 4 * T and M == 5 * T and 13 * T < Fd < 14 * T and S == 16 * T
    vmem = pltpu.VMEM
    packed = lambda *lead: vmem(lead + (T // 2, T), U32)
    out = pl.pallas_call(
        _kernel,
        in_specs=[pl.BlockSpec(memory_space=pltpu.HBM)] * 12,
        out_specs=pl.BlockSpec(memory_space=pltpu.HBM),
        out_shape=jax.ShapeDtypeStruct((S, M), A_x.dtype),
        scratch_shapes=[
            vmem((S + 16, M), BF16),
            vmem((S, Dc), BF16),
            vmem((1, M), BF16),
            vmem((M, 2 * M), BF16),
            vmem((M, 4 * M), BF16),
            vmem((M, M), BF16),
            vmem((M, M), BF16),
            vmem((Fd, M), BF16),
            vmem((Fd, M), BF16),
            vmem((M, D), U32),
            vmem((Dc, D), U32),
            vmem((Dc, D), U32),
            vmem((2 * D, M), BF16),
            vmem((S, M), A_x.dtype),
            pltpu.SemaphoreType.DMA((15,)),
            pltpu.SemaphoreType.DMA((7,)),
            pltpu.SemaphoreType.DMA((S // T,)),
            vmem((8, 6 * M), F32),
            vmem((S // T, M // T, T, T), BF16),
            vmem((len(_C_SUMS), T, T), BF16),
            vmem((len(_H_SUMS), T, T), BF16),
            packed(2, M // T + 2 * (Dc // T)),
            packed(2 * S // T),
            packed(2 * S // T),
            packed(2 * S // T),
            vmem((S + 16, M), F32),
            vmem((S + 16, M), F32),
            vmem((S + 16, M), F32),
            vmem((RB, M), F32),
            vmem((RB + 32, M), F32),
            vmem((2, 7, 2, T, T), U32),
            packed(6, 7, 2),
            vmem((7, 2, 3 * T, T), U32),
            vmem((M, D), U32),
            vmem((Dc, D), U32),
            vmem((Dc, D), U32),
            vmem((3, 8, T), jnp.int32),
        ],
        compiler_params=pltpu.CompilerParams(
            vmem_limit_bytes=100 * 1024 * 1024,
            disable_bounds_checks=True,
        ),
    )(
        A_x.reshape(S, M), A_c_kv.reshape(S, Dc),
        A_w_q, A_w_uk, A_w_uv,
        A_w_o.reshape(H // 2, 2 * D, M),
        B_w1, B_w2, B_w3.T, B_w4, c, w_mod,
    )
    return out.reshape(1, S, M)
```

```python
import math

import jax
import jax.numpy as jnp
import jax.experimental.pallas as pl
import jax.experimental.pallas.tpu as pltpu

F32 = jnp.float32
BF16 = jnp.bfloat16
U32 = jnp.uint32
NT = (((1,), (1,)), ((), ()))
T = 128
EPS = 1e-5
LOG2E = math.log2(math.e)

GRP = 4
LEAD = 10
PROW = 3
RES = 32
LAT_A = 16
LAT_B = 20
ALEAD = 32
MID = 40
SD0, SDS, SDN, SDJ = 158, 2, 20, 30
QT = 3
RB = 256
PC = 32
P0, PSTEP, PD = 440, 30, 52
NLN, LN0, LNS = 4, 4, 5
LP = 16
PROLOGUE = ('|kva|Z; |b|; kva|wc|K0123; bw|xdn|C0@56 N0123@52 K4567; cx|mq|N4567@52 K89ab; '
            'd|y|C1@56 Kcdef; nmq|zo|M H01 H234567@30 Q0123; y||H89ab@30 Q4567; '
            'zo||L Hcdef@30 Q89ab S01 Qcdef')


def _dot(a, b):
    return jnp.dot(a, b, preferred_element_type=F32)


def _dot_nt(a, b):
    return jax.lax.dot_general(a, b, NT, preferred_element_type=F32)


def _ln(x):
    m = jnp.mean(x, axis=-1, keepdims=True)
    xc = x - m
    v = jnp.mean(xc * xc, axis=-1, keepdims=True)
    return xc * jnp.exp2(jnp.log(v + EPS) * (-0.5 * LOG2E))


def _rows(v, n):
    return jnp.broadcast_to(v[None], (n // 8, 8, v.shape[1])).reshape(n, v.shape[1])


def _gelu(x):
    c0 = math.sqrt(2.0 / math.pi)
    return 0.5 * x * (1.0 + jnp.tanh(c0 * (x + 0.044715 * (x * x * x))))


def _after(x, dep):
    return jnp.where(dep > jnp.inf, dep, x)


def _tie(x, dep):
    xu = pltpu.bitcast(x, U32)
    first = jnp.where(dep > jnp.inf, jnp.uint32(0), xu[:8])
    return pltpu.bitcast(jnp.concatenate([first, xu[8:]], axis=0), BF16)


def _tile(j):
    return slice(j * T, (j + 1) * T)


def _ld(ref, *idx):
    return pltpu.bitcast(ref[idx], BF16)


def _pk(x):
    return pltpu.bitcast(x, U32)


def _a_ops(a11, a12, a21, a22):
    return [a11 + a22, a21 + a22, a11, a22, a11 + a12, a21 - a11, a12 - a22]


def _b_ops(b11, b12, b21, b22):
    return [b11 + b22, b11, b12 - b22, b21 - b11, b22, b11 + b12, b21 + b22]


def _strassen(prod, col1=None, col2=None):
    m4 = prod(3)
    m2 = prod(1)
    c21 = m2 + m4
    if col1 is not None:
        e11, e21 = col1()
        m4, c21 = m4 + e11, c21 + e21
    m3 = prod(2)
    m5 = prod(4)
    c12 = m3 + m5
    if col2 is not None:
        e12, e22 = col2()
        c12, m3 = c12 + e12, m3 + e22
    m1 = prod(0)
    c11 = prod(6) + (m1 + (m4 - m5))
    c22 = prod(5) + (m1 + (m3 - m2))
    return c11, c12, c21, c22


def _group(rows, cols, pairs):
    xs, ys = dict.fromkeys(x for x, _ in pairs), dict.fromkeys(y for _, y in pairs)
    used = set(xs) | set(ys) | {(x[0], y[1]) for x, y in pairs} | {(y[0], x[1]) for x, y in pairs}
    prods = []
    for n, r in enumerate(rows):
        for i, k in [x for x in xs if x[0] == r]:
            mates = [y for x, y in pairs if x == (i, k)]
            prods.append((((1, i, k),) + tuple((1, i, k2) for _, k2 in mates), ((1, k, 0),),
                          ((1, i, 0), (-1, i, 1))))
            prods.append((((1, i, k),) + tuple((-1, i2, k) for i2, _ in mates), ((1, k, 0), (1, k, 1)),
                          ((1, i, 1),)))
        for i2, k2 in [y for y in ys if y[0] == r]:
            mates = [x for x, y in pairs if y == (i2, k2)]
            prods.append((((1, i2, k2),) + tuple((1, i2, k) for _, k in mates), ((1, k2, 1),),
                          ((1, i2, 1), (-1, i2, 0))))
            prods.append((((1, i2, k2),) + tuple((-1, i, k2) for i, _ in mates), ((1, k2, 0), (1, k2, 1)),
                          ((1, i2, 0),)))
        prods += [(((1, r, k),), ((1, k, h),), ((1, r, h),)) for k in cols if (r, k) not in used for h in (0, 1)]
        for (i, k), (i2, k2) in pairs:
            if r in (i, i2) and i + i2 - r in rows[n + 1:]:
                prods.append((((1, i, k2),), ((1, k2, 0), (-1, k, 0)), ((1, i2, 0), (1, i, 0))))
                prods.append((((1, i2, k), (1, i, k2)), ((1, k, 0), (1, k2, 1)), ((1, i2, 0), (1, i, 1))))
                prods.append((((1, i2, k),), ((1, k, 1), (-1, k2, 1)), ((1, i2, 1), (1, i, 1))))
    return prods


def _all_pairs(xrows, yrows):
    return [((x, a), (y, b)) for a, x in enumerate(xrows) for b, y in enumerate(yrows) if a != b]


_PAIRS65 = [((x[0] + 10, x[1]), (y[0] + 10, y[1])) for x, y in (
    ((0, 1), (1, 0)), ((0, 1), (5, 2)), ((2, 3), (1, 0)), ((2, 3), (3, 1)), ((2, 3), (5, 2)), ((3, 2), (1, 0)),
    ((4, 4), (0, 3)), ((4, 4), (1, 0)), ((4, 4), (3, 1)), ((4, 4), (5, 2)))]
_C_GROUPS = [_group(range(r, r + 8), range(4), _all_pairs(range(r, r + 4), range(r + 4, r + 8))) for r in (0, 8)]
_H_GROUPS = [_group(range(10), range(5), _all_pairs(range(5), range(5, 10))),
             _group(range(10, 16), range(5), _PAIRS65)]
_sum_index = lambda groups: {f: n for n, f in enumerate(
    dict.fromkeys(t[0] for g in groups for t in g if len(t[0]) > 1))}
_C_SUMS, _H_SUMS = _sum_index(_C_GROUPS), _sum_index(_H_GROUPS)


def _form(form, get):
    acc = None
    for sign, i, j in form:
        v = get(i, j)
        acc = v if acc is None else (acc + v if sign > 0 else acc - v)
    return acc


def _gap_items(bufs, gap_scr):
    items = []
    for n, buf in enumerate(bufs):
        acc = []

        def part(r0, buf=buf, acc=acc):
            def fn(dep):
                wu = jnp.concatenate([buf[r:r + 8, :] for r in range(r0, r0 + T, 32)])
                mask = jnp.full((8, T), 0x7FFF0000, U32)
                if dep is not None:
                    mask = jnp.where(dep > jnp.inf, jnp.uint32(0), mask)
                mask = _rows(mask, 32)
                new = [jnp.sum(pltpu.bitcast(v & mask, F32).reshape(4, 8, T), axis=0) for v in (wu << 16, wu)]
                acc[:] = [u + v for u, v in zip(acc, new)] if acc else new
            return fn

        def last(_, n=n, acc=acc):
            bits = []
            for v in acc:
                l1 = jnp.sum(jnp.sum(v, axis=1, keepdims=True), axis=0, keepdims=True)
                bits.append(pltpu.bitcast(jnp.broadcast_to(l1, (8, T)), jnp.int32) >> 8)
            gap_scr[n] = jnp.clip((bits[0] - bits[1] + (1 << 14)) >> 15, -8, 8) << 23

        items += [part(r0) for r0 in range(0, buf.shape[0], T)] + [last]
    return items


class _PairWeights:
    def __init__(self, w_ref, transpose=False, shift=None):
        self.base = {}
        if shift is not None:
            fac = _rows(pltpu.bitcast(0x3F800000 + shift, F32), T)
            self.inv = pltpu.bitcast(0x3F800000 - shift, F32)
        for j in range(w_ref.shape[0] // T):
            wu = w_ref[_tile(j), :]
            if transpose:
                wu = wu.T
            hi = pltpu.bitcast(wu & jnp.uint32(0xFFFF0000), F32)
            self.base[j, 0] = pltpu.bitcast(wu << 16, F32)
            self.base[j, 1] = hi if shift is None else hi * fac
        self.cache = {}

    def __call__(self, form):
        sign = 1
        if form[-1][0] < 0 and form[0][1:] > form[1][1:]:
            sign, form = -1, ((1,) + form[1][1:], (-1,) + form[0][1:])
        if form not in self.cache:
            self.cache[form] = _form(form, lambda k, h: self.base[k, h]).astype(BF16)
        return sign, self.cache[form]


def _run_group(jobs, prods, a_get, w, transposed, finish):
    left = {}
    for _, _, outs in prods:
        for _, i, h in outs:
            left[i, h] = left.get((i, h), 0) + 1
    acc = {}
    for af, bf, outs in prods:
        sign, wt = w(bf)
        m = jobs.mm([wt], [a_get(af)], _dot_nt) if transposed else jobs.mm([a_get(af)], [wt], _dot)
        for s_, i, h in outs:
            if (i, h) not in acc:
                acc[i, h] = (s_ * sign, m)
            else:
                s0, v = acc[i, h]
                acc[i, h] = (s0, v + m if s0 == s_ * sign else v - m) if s0 > 0 or s_ * sign < 0 else (1, m - v)
            left[i, h] -= 1
            if not left[i, h]:
                s0, v = acc.pop((i, h))
                assert s0 > 0
                finish(2 * i + h, v)


class _Jobs:
    def __init__(self, side=()):
        self.res = []
        self.side = list(side)

    def mm(self, lhs, wt, dot):
        acc = None
        for x, w in zip(lhs, wt):
            v = dot(x, w)
            self.res.append(v)
            acc = v if acc is None else v + acc
            rel = 4 * (len(self.res) % 4)
            while self.side and self.side[0][0] <= len(self.res):
                self.side.pop(0)[1](v[8 * rel:8 * rel + 8, :])
                rel = (rel + 2) % 16
        return acc


def _proj_step(h_scr, hs_scr, c_ref, cs_scr, wq_ref, wuk_ref, wuv_ref, q_scr, k_scr, v_scr, scale, shifts, side):
    wk, wvT, wq = [_PairWeights(w, n == 1, shifts[n]) for n, w in enumerate((wuk_ref, wuv_ref, wq_ref))]
    c_get = lambda f: cs_scr[_C_SUMS[f]] if len(f) > 1 else c_ref[_tile(f[0][1]), _tile(f[0][2])]
    h_get = lambda f: hs_scr[_H_SUMS[f]] if len(f) > 1 else h_scr[f[0][1], f[0][2]]

    def put(dst, w, mul=None):
        muls = [mul, _rows(w.inv if mul is None else w.inv * mul, T)]

        def fn(u, v):
            v = (v if muls[u % 2] is None else v * muls[u % 2]).astype(BF16)
            dst[u] = _pk(v.T if mul is not None and u < QT else v)
        return fn

    jobs = _Jobs(side)
    for groups, get, w, transposed, fin in ((_C_GROUPS, c_get, wk, False, put(k_scr, wk)),
                                            (_C_GROUPS, c_get, wvT, True, put(v_scr, wvT)),
                                            (_H_GROUPS, h_get, wq, False, put(q_scr, wq, scale))):
        for prods in groups:
            _run_group(jobs, prods, get, w, transposed, fin)
    assert not jobs.side


def _inner_group(rows, cols, pairs):
    xs, ys = dict.fromkeys(x for x, _ in pairs), dict.fromkeys(y for _, y in pairs)
    used = set(xs) | set(ys) | {(x[0], y[1]) for x, y in pairs} | {(y[0], x[1]) for x, y in pairs}
    prods = []
    for i, j in xs:
        mates = [y for x, y in pairs if x == (i, j)]
        prods.append((((1, i, 0),), ((1, 0, j), (-1, 1, j)), ((1, i, j),) + tuple((1, i2, j) for i2, _ in mates)))
        prods.append((((1, i, 0), (1, i, 1)), ((1, 1, j),), ((1, i, j),) + tuple((-1, i, j2) for _, j2 in mates)))
    for i2, j2 in ys:
        mates = [x for x, y in pairs if y == (i2, j2)]
        prods.append((((1, i2, 0), (1, i2, 1)), ((1, 0, j2),),
                      ((1, i2, j2),) + tuple((-1, i2, j) for _, j in mates)))
        prods.append((((1, i2, 1),), ((1, 0, j2), (-1, 1, j2)),
                      ((-1, i2, j2),) + tuple((-1, i, j2) for i, _ in mates)))
    prods += [(((1, i, h),), ((1, h, j),), ((1, i, j),))
              for i in rows for j in cols if (i, j) not in used for h in (0, 1)]
    for (i, j), (i2, j2) in pairs:
        lo, hi = min(j, j2), max(j, j2)
        prods.append((((1, i2, 0), (-1, i, 0)), ((1, 0, lo), (1, 0, hi)), ((1, i2, j),)))
        prods.append((((1, i, 0), (1, i2, 1)), ((1, 0, j2), (1, 1, j)), ((1, i, j2), (1, i2, j))))
        prods.append((((1, i, 1), (-1, i2, 1)), ((1, 1, lo), (1, 1, hi)), ((1, i, j2),)))
    return prods


def _o_jobs():
    prods = (_inner_group(range(10), range(5), _all_pairs(range(0, 10, 2), range(1, 10, 2)))
             + _inner_group(range(10, 16), range(5), _PAIRS65))
    row = lambda t: max(i for _, i, _ in t[0])
    unit = lambda t: max(2 * i + h for _, i, h in t[0])
    need = lambda t: unit(t) if row(t) == 15 else 2 * row(t) + 1
    return [(need(t), t) for t in sorted(prods, key=need)]


_O_JOBS = _o_jobs()


def _job_order(nb):
    units = range(2 * nb)
    qa = [('a', u, c) for u in units for c in range(u // 2 + 1)]
    qb = [('b', u, c) for u in units for c in range(u // 2 + 1)]
    qo = [('o', u, j) for j, (u, _) in enumerate(_O_JOBS)]
    done = {}
    order = []

    def ready(q, lat, pre):
        return bool(q) and (pre, q[0][1]) in done and done[(pre, q[0][1])] + lat <= len(order)

    def emit(q):
        kind, u, j = job = q.pop(0)
        if kind != 'o' and j == u // 2:
            done[(kind, u)] = len(order)
        order.append(job)

    turn = 0
    while qa or qb or qo:
        pref = 'abo'[turn % 3]
        turn += 1
        for _ in range(GRP):
            b_ok, o_ok = ready(qb, LAT_A, 'a'), ready(qo, LAT_B, 'b')
            if pref == 'a' and qa and (len(qb) - len(qa) < ALEAD or not b_ok):
                emit(qa)
            elif pref == 'b' and b_ok:
                emit(qb)
            elif pref == 'o' and o_ok and (len(qo) > RES or not (qa or b_ok)):
                emit(qo)
            elif not (qa or b_ok or o_ok) and (qb or qo):
                emit(qb or qo)
            else:
                break
    return order


def _attention_step(q_scr, k_scr, v_scr, wo_ref, acc_scr, mid):
    causal = (jax.lax.broadcasted_iota(jnp.int32, (T, T), 0)
              <= jax.lax.broadcasted_iota(jnp.int32, (T, T), 1))
    sv, mx, mfin, lsum, pv, of, lhs = {}, {}, {}, {}, {}, {}, {}
    res = []
    wo, terms = {}, {}
    left = {}
    for _, t in _O_JOBS:
        for _, i, j in t[2]:
            left[i, j] = left.get((i, j), 0) + 1

    def job_a(u, c):
        r, hd = divmod(u, 2)
        s = (_dot if u < QT else _dot_nt)(_ld(k_scr, 2 * c + hd), _ld(q_scr, u))
        res.append(s)
        if c == r:
            s = jnp.where(causal, s, -1e9 * LOG2E)
        s = s.reshape(T // 8, 8, T)
        sv[(u, c)] = s
        pm = jnp.max(s, axis=0)
        mx[u] = pm if u not in mx else jnp.maximum(mx[u], pm)

    def job_b(u, c):
        r, hd = divmod(u, 2)
        if u not in mfin:
            mfin[u] = jnp.broadcast_to(jnp.max(mx[u], axis=0, keepdims=True), (8, T))
        m = mfin[u]
        if len(res) >= LEAD:
            r0 = 8 * PROW * (c % 4)
            m = _after(m, res[len(res) - LEAD][r0:r0 + 8, :])
        p = jnp.exp2(sv.pop((u, c)) - m[None])
        ls = jnp.sum(p, axis=0)
        lsum[u] = ls if u not in lsum else lsum[u] + ls
        v = _dot(_ld(v_scr, 2 * c + hd), p.reshape(T, T).astype(BF16))
        res.append(v)
        pv[u] = v if u not in pv else v + pv[u]
        if c == r:
            of[u] = pv[u] * (1.0 / jnp.sum(lsum[u], axis=0, keepdims=True))

    def job_o(_, n):
        af, bf, outs = _O_JOBS[n][1]
        if af not in lhs:
            v = _form(af, lambda i, h: of[2 * i + h])
            lhs[af] = _tie(v.astype(BF16).T, v[0:8, :])
        if bf not in wo:
            wo[bf] = (wo_ref[_tile(bf[0][1]), _tile(bf[0][2])] if len(bf) == 1 else
                      _form(bf, lambda h, j: wo_ref[_tile(h), _tile(j)].astype(F32)).astype(BF16))
        v = _dot(lhs[af], wo[bf])
        res.append(v)
        for sign, i, j in outs:
            terms.setdefault((i, j), []).append((sign, v))
            if len(terms[i, j]) == left[i, j]:
                tot = acc_scr[_tile(i), _tile(j)]
                for sg, m in terms.pop((i, j)):
                    tot = tot + m if sg > 0 else tot - m
                acc_scr[_tile(i), _tile(j)] = tot

    fns = dict(a=job_a, b=job_b, o=job_o)
    for n, (kind, u, j) in enumerate(_job_order(q_scr.shape[0] // 2)):
        if n == MID:
            mid()
        fns[kind](u, j)


def _kernel(x_hbm, c_hbm, wq_hbm, wuk_hbm, wuv_hbm, wo_hbm, w1_hbm, w2_hbm, w3_hbm, w4_hbm,
            cond_hbm, wmod_hbm, out_hbm,
            x_ref, c_ref, cond_ref, wma_ref, wmb_ref, w1_ref, w2_ref, w3_ref, w4_ref,
            wq_buf, wk_buf, wv_buf, wo_buf, out_buf, sem, wsem, osem,
            mod_scr, h_scr, cs_scr, hs_scr, w_scr, q_scr, k_scr, v_scr, acc_scr, x1_scr, hb_scr, a1_scr, t_scr,
            ws12, ws3, ws4, pq_buf, pk_buf, pv_buf, gap_scr, st_in):
    S, M = x_hbm.shape
    D = wq_hbm.shape[2]
    nattn = wo_hbm.shape[0]
    Fd = w4_hbm.shape[0]
    scale = float(D) ** -0.5 * LOG2E
    nb, nrb = S // T, S // RB
    km, kc = M // T, c_hbm.shape[1] // T
    NX = 4
    XR = S // NX
    CB = XR // T

    work, probe = (wk_buf, wv_buf, wq_buf), (pk_buf, pv_buf, pq_buf)

    def pcopies(g, bufs=work, s0=0):
        return [pltpu.make_async_copy(src.bitcast(U32).at[:, g, :], dst, wsem.at[s0 + j])
                for j, (src, dst) in enumerate(zip((wuk_hbm, wuv_hbm, wq_hbm), bufs))]

    def ocopy(g):
        return pltpu.make_async_copy(wo_hbm.at[g], wo_buf, wsem.at[3])

    def chunk_copy(src, dst, i, s0):
        rows = slice(i * XR, (i + 1) * XR)
        return pltpu.make_async_copy(src.at[rows, :], dst.at[rows, :], sem.at[s0 + i])

    cp_cond = pltpu.make_async_copy(cond_hbm, cond_ref, sem.at[0])
    cp_wma = pltpu.make_async_copy(wmod_hbm.at[:, 0:2 * M], wma_ref, sem.at[1])
    cp_late = [pltpu.make_async_copy(src, dst, sem.at[2 + j]) for j, (src, dst) in enumerate((
        (wmod_hbm.at[:, 2 * M:6 * M], wmb_ref), (w1_hbm, w1_ref), (w2_hbm, w2_ref),
        (w3_hbm, w3_ref), (w4_hbm, w4_ref)))]
    cp_x = [chunk_copy(x_hbm, x_ref, i, 7) for i in range(NX)]
    cp_c = [chunk_copy(c_hbm, c_ref, i, 7 + NX) for i in range(NX)]

    def silu_cond():
        cf = cond_ref[...].astype(F32)
        return jnp.broadcast_to((cf * jax.nn.sigmoid(cf)).astype(BF16), (8, M))

    cp_wk, cp_wv, cp_wq = pcopies(0)
    named = dict(k=cp_wk, v=cp_wv, q=cp_wq, o=ocopy(0), n=cp_cond, m=cp_wma)
    named.update(zip('abcd', cp_c))
    named.update(zip('wxyz', cp_x))
    started, arrived, did = set(), set(), set()

    def zero(r, carry):
        acc_scr[pl.ds(pl.multiple_of(r * T, T), T), :] = jnp.zeros((T, M), F32)
        return carry

    def x_rows(rows, dep):
        xf = x_ref[rows, :].astype(F32)
        if dep is None:
            return xf
        return jnp.concatenate([_after(xf[:, :T], _rows(dep, xf.shape[0])), xf[:, T:]], axis=1)

    def n_item(r, i):
        def fn(dep):
            rows = slice(r * T + i * LP, r * T + (i + 1) * LP)
            x1_scr[rows, :] = _ln(x_rows(rows, dep))
        return fn

    def h_item(r, i, normed):
        def fn(dep):
            rows = slice(i * LP, (i + 1) * LP)
            grows = slice(r * T + i * LP, r * T + (i + 1) * LP)
            sa = mod_scr[:, 0:M]
            if normed and dep is not None:
                sa = jnp.concatenate([_after(sa[:, _tile(j)], dep) for j in range(km)], axis=1)
            hf = ((x1_scr[grows, :] if normed else _ln(x_rows(grows, dep))) * _rows(mod_scr[:, M:2 * M], LP)
                  + _rows(sa, LP))
            for j in range(km):
                h_scr[r, j, rows, :] = hf[:, _tile(j)].astype(BF16)
            for f, n in _H_SUMS.items():
                if all(t[1] == r for t in f):
                    hs_scr[n, rows, :] = _form(f, lambda _, k: hf[:, _tile(k)]).astype(BF16)
            did.add(('h', r, i))
        return fn

    def release(jobs, span, items):
        if span and items:
            jobs.side += [(len(jobs.res) + 1 + i * span // len(items), fn) for i, fn in enumerate(items)]
            jobs.side.sort(key=lambda e: e[0])
        else:
            for fn in items:
                fn(None)

    def sum_items(n, group, index, dst, get, skip_rows):
        forms = [f for f in dict.fromkeys(t[0] for t in group)
                 if len(f) > 1 and not (skip_rows and len({t[1] for t in f}) == 1)]

        def item(f, rows):
            def fn(dep):
                def term(r, k):
                    v = get(r, k, rows).astype(F32)
                    return v if dep is None or (r, k) != f[0][1:] else _after(v, _rows(dep, v.shape[0]))
                dst[index[f], rows, :] = _form(f, term).astype(BF16)
            return fn

        return [item(f, slice(i, i + n)) for i in range(0, T, n) for f in forms]

    h_sums = lambda n, gi: sum_items(n, _H_GROUPS[gi], _H_SUMS, hs_scr,
                                     lambda r_, k, rows: h_scr[r_, k, rows, :], True)

    def stash(key, buf, j0, transpose=False):
        n = buf.shape[0] // T
        if key not in did:
            assert key in arrived
            did.add(key)
            w = _PairWeights(buf, transpose)
            for j in range(n):
                for hd in range(2):
                    w_scr[hd, j0 + j] = _pk(w(((1, j, hd),))[1])
        return lambda hd: [_ld(w_scr, hd, j0 + j) for j in range(n)]

    def kv_tile(jobs, r):
        wk, wvT = stash('k', wk_buf, 0), stash('v', wv_buf, kc, True)
        ct = [c_ref[_tile(r), _tile(j)] for j in range(kc)]
        for hd in range(2):
            k_scr[2 * r + hd] = _pk(jobs.mm(ct, wk(hd), _dot).astype(BF16))
        for hd in range(2):
            v_scr[2 * r + hd] = _pk(jobs.mm(wvT(hd), ct, _dot_nt).astype(BF16))

    def q_tile(jobs, r):
        wq = stash('q', wq_buf, 2 * kc)
        ht = [h_scr[r, j] for j in range(km)]
        for hd in range(2):
            v = (jobs.mm(ht, wq(hd), _dot) * scale).astype(BF16)
            q_scr[2 * r + hd] = _pk(v.T if 2 * r + hd < QT else v)

    for blk in PROLOGUE.split(';'):
        waits, starts, acts = blk.split('|')
        for ch in waits.strip():
            assert ch in started and ch not in arrived
            arrived.add(ch)
            named[ch].wait()
        for ch in starts.strip():
            assert ch not in started
            started.add(ch)
            named[ch].start()
        jobs = _Jobs()
        for act in acts.split():
            if act == 'Z':
                jax.lax.fori_loop(0, nb, zero, 0)
                acc_scr[S:, :] = jnp.zeros((acc_scr.shape[0] - S, M), F32)
                x_ref[S:, :] = jnp.zeros((x_ref.shape[0] - S, M), BF16)
            elif act == 'L':
                did.add('L')
                for cp in cp_late:
                    cp.start()
            elif act == 'M':
                assert arrived >= set('nm')
                mod = _dot(silu_cond(), wma_ref[...])
                mod_scr[:, 0:M] = mod[:, 0:M]
                mod_scr[:, M:2 * M] = 1.0 + mod[:, M:2 * M]
                did.add('M')
            else:
                act, _, span = act.partition('@')
                span = int(span or 0)
                items = []
                for r in [int(ch, 16) for ch in act[1:]]:
                    did.add((act[0], r))
                    if act[0] == 'K':
                        assert 'abcd'[r // CB] in arrived
                        kv_tile(jobs, r)
                    elif act[0] == 'H':
                        assert 'wxyz'[r // CB] in arrived and 'M' in did
                        items += [h_item(r, i, ('N', r) in did) for i in range(T // LP)]
                    elif act[0] == 'N':
                        assert 'wxyz'[r // CB] in arrived
                        items += [n_item(r, i) for i in range(T // LP)]
                    elif act[0] == 'Q':
                        assert all(('h', r, i) in did for i in range(T // LP))
                        q_tile(jobs, r)
                    elif act[0] == 'C':
                        assert all('abcd'[t[1] // CB] in arrived for p_ in _C_GROUPS[r] for t in p_[0])
                        items += sum_items(
                            32, _C_GROUPS[r], _C_SUMS, cs_scr,
                            lambda r_, k, rows: c_ref[r_ * T + rows.start:r_ * T + rows.stop, _tile(k)], False)
                    else:
                        assert act[0] == 'S' and all(('h', t[1], T // LP - 1) in did for p_ in _H_GROUPS[r] for t in p_[0])
                        items += h_sums(32 if span else 16, r)
                release(jobs, span, items)
        assert not jobs.side
    assert arrived == set(named) and all((k_, r) in did for k_ in 'KHQ' for r in range(nb))
    assert all((k_, r) in did for k_ in 'CS' for r in range(2)) and 'L' in did

    FH = ws3.shape[0] * T
    assert nattn - 1 >= FH // 64

    slices = ((w1_hbm, 32, 2 * T, 0), (w2_hbm, 32, 2 * T, 64), (w4_hbm, 64, FH, 128), (w3_hbm, T, FH, 256))
    slice_of = lambda g, n, half: jnp.minimum(g, half // n - 1)

    def prep_in(g):
        return [pltpu.make_async_copy(
            w.at[pl.ds(pl.multiple_of(slice_of(g, n, half) * n + x * half, n), n), 0:4 * T],
            st_in.at[r0 + x * n:r0 + (x + 1) * n, :], wsem.at[7]) for w, n, half, r0 in slices for x in range(2)]

    def mixer_prep(g):
        def blocks(r0, n, half, c0, c1, dep):
            get = lambda x, c: st_in[r0 + x * half:r0 + x * half + n, _tile(c)].astype(F32)
            return [_after(get(0, c0), _rows(dep, n)), get(0, c1), get(1, c0), _after(get(1, c1), _rows(dep, n))]

        def rows_item(dst, per, half, r0, c, o, n=16):
            def fn(dep):
                rows = pl.ds(pl.multiple_of(slice_of(g, per, half) * (per // 2), per // 2) + o // 2, n // 2)
                for i, v in enumerate(_b_ops(*blocks(r0 + o, n, per, c, c + 2, dep))):
                    dst[i, c, rows, :] = _pk(v.astype(BF16))
            return fn

        def w3_item(k, i):
            def fn(dep):
                b11, b21, b12, b22 = blocks(slices[3][3], T, T, k, k + 2, dep)
                ws3[slice_of(g, T, FH), i, k] = _pk(_b_ops(b11, b12, b21, b22)[i].astype(BF16).T)
            return fn

        return ([rows_item(dst, *sl[1:], c, o) for dst, sl in zip((ws12.at[0], ws12.at[1], ws4), slices)
                 for c in range(2) for o in range(0, sl[1], 16)]
                + [w3_item(k, i) for k in range(2) for i in range(7)])

    def attn_body(g, carry):
        copies = pcopies(jnp.minimum(g + 1, nattn - 1)) + pcopies(jnp.minimum(g + 2, nattn - 1), probe, 4)

        def mid():
            for cp in copies + prep_in(g):
                cp.start()

        _attention_step(q_scr, k_scr, v_scr, wo_buf, acc_scr, mid)
        for cp in copies:
            cp.wait()
        pltpu.make_async_copy(st_in, st_in, wsem.at[7]).wait()

        @pl.when(g == 0)
        def _():
            for fn in _gap_items(work, gap_scr):
                fn(None)

        @pl.when(g + 1 < nattn)
        def _():
            ocopy(g + 1).start()
            side = mixer_prep(g) + _gap_items(probe, gap_scr)
            side = [(SD0 + i * SDS + (SDJ if i >= SDN else 0), fn) for i, fn in enumerate(side)]
            _proj_step(h_scr, hs_scr, c_ref, cs_scr, wq_buf, wk_buf, wv_buf, q_scr, k_scr, v_scr, scale,
                       gap_scr, side)
            ocopy(g + 1).wait()

        return carry

    jax.lax.fori_loop(0, nattn, attn_body, 0)

    for cp in cp_late:
        cp.wait()
    mod = _dot(silu_cond(), wmb_ref[...])
    mod_scr[:, 2 * M:4 * M] = mod[:, 0:2 * M]
    mod_scr[:, 4 * M:5 * M] = 1.0 + mod[:, 2 * M:3 * M]
    mod_scr[:, 5 * M:6 * M] = mod[:, 3 * M:4 * M]
    ftiles = [(f, min(f + T, Fd)) for f in range(0, Fd, T)]
    OFF = x_ref.shape[0] - S
    CAR = t_scr.shape[0] - RB

    def p1(r0, n, dep=None):
        ga = mod_scr[:, 2 * M:3 * M]
        if dep is not None:
            ga = jnp.concatenate([_after(ga[:, 0:T], dep), ga[:, T:]], axis=1)
        rows = pl.ds(r0, n)
        x1 = x_ref[rows, :].astype(F32) + _rows(ga, n) * acc_scr[rows, :]
        x1_scr[rows, :] = x1
        hb = _ln(x1) * _rows(mod_scr[:, 4 * M:5 * M], n) + _rows(mod_scr[:, 3 * M:4 * M], n)
        hb_scr[rows, :] = hb
        return _ln(hb)

    HT = T // 2

    def p1_store(r0, c, dep=None):
        v = p1(r0 + c * PC, PC, dep)
        a1_scr[c * PC:(c + 1) * PC, :] = v
        return jnp.max(v[:, M - T:].reshape(PC // 8, 8, T), axis=0)

    t_scr[RB:RB + CAR - OFF, :] = jnp.zeros((CAR - OFF, M), F32)
    t_scr[RB + CAR - OFF:RB + CAR, :] = _gelu(_dot(p1(0, OFF).astype(BF16), w1_ref[...]))
    for c in range(RB // PC):
        p1_store(OFF, c)

    def out_copy(i):
        rows = pl.ds(i * T if isinstance(i, int) else pl.multiple_of(i * T, T), T)
        return pltpu.make_async_copy(out_buf.at[rows, :], out_hbm.at[rows, :], osem.at[i])

    def b_body(r, carry):
        gb = _rows(mod_scr[:, 5 * M:6 * M], T)
        r0 = pl.multiple_of(r * RB, RB)
        n0 = pl.multiple_of(jnp.minimum(r0 + RB, S - RB) + OFF, OFF)
        nh = RB // T
        now = [0]
        due = []
        pace = []

        def p1_item(c):
            return lambda dep: due.append((now[0] + PD, p1_store(n0, c, dep)))

        pace += [(P0 + i * PSTEP, p1_item(i)) for i in range(RB // PC)]
        wt = lambda ref, f0, f1, n: ref[f0:f1, _tile(n)]

        def mm(lhs, wts, dot=_dot):
            acc = None
            for x, w in zip(lhs, wts):
                if due and due[0][0] <= now[0]:
                    w = _tie(w, due.pop(0)[1])
                v = dot(x, w)
                now[0] += x.shape[0] // HT
                acc = v if acc is None else v + acc
                if pace and pace[0][0] <= now[0]:
                    pace.pop(0)[1](v[0:8, :])
            return acc

        def split_ops(lo, hi):
            return [v.astype(BF16) for v in _a_ops(lo[:HT], hi[:HT], lo[HT:], hi[HT:])]

        def two_tiles(aops, wsel, rest):
            def col(w):
                v = mm(rest[0], w, rest[3])
                return v[:HT], v[HT:]

            c11, c12, c21, c22 = _strassen(
                lambda i: mm([a[i] for a in aops], [wsel(i, k) for k in range(len(aops))]),
                lambda: col(rest[1]), lambda: col(rest[2]))
            return jnp.concatenate([c11, c21], axis=0), jnp.concatenate([c12, c22], axis=0)

        def square(full, aops, w_ref, ws_ref):
            out = {}
            for n in range(2):
                out[n], out[n + 2] = two_tiles(
                    aops, lambda i, k: _ld(ws_ref, i, n, slice(k * HT, (k + 1) * HT)),
                    (full[4:], [wt(w_ref, 4 * T, M, n)], [wt(w_ref, 4 * T, M, n + 2)], _dot))
            out[4] = mm(full, [wt(w_ref, j * T, (j + 1) * T, 4) for j in range(km)])
            return out

        t_scr[0:CAR, :] = t_scr[RB:RB + CAR, :]
        for hf in range(nh):
            a1 = [a1_scr[_tile(hf), _tile(j)] for j in range(km)]
            full = [v.astype(BF16) for v in a1]
            aops = [split_ops(a1[k], a1[2 + k]) for k in range(2)]
            for n, v in square(full, aops, w1_ref, ws12.at[0]).items():
                t = _gelu(v)
                if hf == nh - 1:
                    t = jnp.concatenate([t[:T - OFF], jnp.where(r < nrb - 1, t[T - OFF:], 0.0)], axis=0)
                t_scr[CAR + hf * T:CAR + (hf + 1) * T, _tile(n)] = t
        cq = M // 4
        shifts = (-1, 1, -2, 2)
        lane = jax.lax.broadcasted_iota(jnp.int32, (T, T), 1)
        y1, a3 = [], []
        for hf in range(nh):
            base = CAR - OFF + hf * T
            sh = []
            for j in range(km):
                g_lo, g_hi = (j * T) // cq, ((j + 1) * T - 1) // cq
                assert g_hi - g_lo <= 1
                v = t_scr[base + shifts[g_lo]:base + shifts[g_lo] + T, _tile(j)]
                if g_hi != g_lo:
                    v2 = t_scr[base + shifts[g_hi]:base + shifts[g_hi] + T, _tile(j)]
                    v = jnp.where(lane < g_hi * cq - j * T, v, v2)
                sh.append(v)
            hs = square([v.astype(BF16) for v in sh], [split_ops(sh[k], sh[2 + k]) for k in range(2)],
                        w2_ref, ws12.at[1])
            hs = jnp.concatenate([hs[n] for n in range(km)], axis=1)
            y1.append(hs + hb_scr[pl.ds(pl.multiple_of(r0 + hf * T, T), T), :])
            a3.append({})

            def ln_item(hf, c):
                def item(dep):
                    n = HT // NLN
                    for d in (0, HT):
                        v = y1[hf][d + c * n:d + (c + 1) * n]
                        if dep is not None:
                            v = jnp.concatenate([_after(v[:, :T], _rows(dep, n)), v[:, T:]], axis=1)
                        a3[hf][d + c * n] = _ln(v)
                return item

            ln_item(hf, 0)(None)
            pace += [(now[0] + LN0 + (c - 1) * LNS * (1 + hf), ln_item(hf, c)) for c in range(1, NLN)]
            pace.sort(key=lambda e: e[0])
        nf = FH // T
        h3, h3ops = [], []
        for hf in range(nh):
            assert len(a3[hf]) == 2 * NLN
            af = jnp.concatenate([a3[hf][key] for key in sorted(a3[hf])], axis=0)
            full = [af[:, _tile(j)].astype(BF16) for j in range(km)]
            aops = [split_ops(af[:, _tile(k)], af[:, _tile(2 + k)]) for k in range(2)]
            row, ops = {}, []
            narrow = None
            for n in range(nf):
                lo, hi = two_tiles(aops, lambda i, k: _ld(ws3, n, i, k),
                                   (full[4:], [wt(w3_ref, *ftiles[n], 4)],
                                    [wt(w3_ref, *ftiles[nf + n], 4)], _dot_nt))
                lo, hi = _gelu(lo), _gelu(hi)
                row[n], row[nf + n] = lo.astype(BF16), hi.astype(BF16)
                ops.append(split_ops(lo, hi))
                if n < km:
                    v = mm([wt(w3_ref, *ftiles[-1], n)], [full[n]], _dot_nt)
                    narrow = v if narrow is None else v + narrow
            row[2 * nf] = _gelu(mm(full, [wt(w3_ref, *ftiles[2 * nf], j) for j in range(km)],
                                   _dot_nt)).astype(BF16)
            fw = Fd - ftiles[-1][0]
            gT = jnp.concatenate([_gelu(narrow), jnp.zeros((T - fw, T), F32)], axis=0)
            row[2 * nf + 1] = _tie(gT.astype(BF16).T, gT[0:8, :])[:, :fw]
            h3.append([row[i] for i in range(len(ftiles))])
            h3ops.append(ops)
        for hf in range(nh):
            rows = pl.ds(pl.multiple_of(r0 + hf * T, T), T)

            def finish(n, v):
                out_buf[rows, _tile(n)] = (
                    x1_scr[rows, _tile(n)] + gb[:, _tile(n)] * (v + y1[hf][:, _tile(n)])
                ).astype(out_buf.dtype)

            w4t = lambda n, f_: [wt(w4_ref, f0, f1, n) for f0, f1 in f_]
            finish(4, mm(h3[hf], w4t(4, ftiles)))
            for n in range(2):
                lo, hi = two_tiles(h3ops[hf], lambda i, k: _ld(ws4, i, n, slice(k * HT, (k + 1) * HT)),
                                   (h3[hf][2 * nf:], w4t(n, ftiles[2 * nf:]), w4t(n + 2, ftiles[2 * nf:]), _dot))
                finish(n, lo)
                finish(n + 2, hi)
            out_copy(r * nh + hf).start()
        assert not pace
        return carry

    jax.lax.fori_loop(0, nrb, b_body, 0)
    for i in range(nb):
        out_copy(i).wait()


@jax.jit
def pallas_adaLN_cond__compressed_kv_cla__mixer_s_mlp__prompt_kernel(
    A_x: jax.Array,
    A_c_kv: jax.Array,
    A_w_q: jax.Array,
    A_w_uk: jax.Array,
    A_w_uv: jax.Array,
    A_w_o: jax.Array,
    B_x: jax.Array,
    B_w1: jax.Array,
    B_w2: jax.Array,
    B_w3: jax.Array,
    B_w4: jax.Array,
    c: jax.Array,
    w_mod: jax.Array,
):
    _, S, M = A_x.shape
    Dc = A_c_kv.shape[2]
    H, D = A_w_q.shape[1], A_w_q.shape[2]
    Fd = B_w3.shape[1]
    assert D == T and A_c_kv.shape[1] == S and Dc == 4 * T and M == 5 * T and 13 * T < Fd < 14 * T and S == 16 * T
    vmem = pltpu.VMEM
    packed = lambda *lead: vmem(lead + (T // 2, T), U32)
    out = pl.pallas_call(
        _kernel,
        in_specs=[pl.BlockSpec(memory_space=pltpu.HBM)] * 12,
        out_specs=pl.BlockSpec(memory_space=pltpu.HBM),
        out_shape=jax.ShapeDtypeStruct((S, M), A_x.dtype),
        scratch_shapes=[
            vmem((S + 16, M), BF16),
            vmem((S, Dc), BF16),
            vmem((1, M), BF16),
            vmem((M, 2 * M), BF16),
            vmem((M, 4 * M), BF16),
            vmem((M, M), BF16),
            vmem((M, M), BF16),
            vmem((Fd, M), BF16),
            vmem((Fd, M), BF16),
            vmem((M, D), U32),
            vmem((Dc, D), U32),
            vmem((Dc, D), U32),
            vmem((2 * D, M), BF16),
            vmem((S, M), A_x.dtype),
            pltpu.SemaphoreType.DMA((15,)),
            pltpu.SemaphoreType.DMA((8,)),
            pltpu.SemaphoreType.DMA((S // T,)),
            vmem((8, 6 * M), F32),
            vmem((S // T, M // T, T, T), BF16),
            vmem((len(_C_SUMS), T, T), BF16),
            vmem((len(_H_SUMS), T, T), BF16),
            packed(2, M // T + 2 * (Dc // T)),
            packed(2 * S // T),
            packed(2 * S // T),
            packed(2 * S // T),
            vmem((S + 16, M), F32),
            vmem((S + 16, M), F32),
            vmem((S + 16, M), F32),
            vmem((RB, M), F32),
            vmem((RB + 32, M), F32),
            vmem((2, 7, 2, T, T), U32),
            packed(6, 7, 2),
            vmem((7, 2, 3 * T, T), U32),
            vmem((M, D), U32),
            vmem((Dc, D), U32),
            vmem((Dc, D), U32),
            vmem((3, 8, T), jnp.int32),
            vmem((4 * T, 4 * T), BF16),
        ],
        compiler_params=pltpu.CompilerParams(
            vmem_limit_bytes=100 * 1024 * 1024,
            disable_bounds_checks=True,
        ),
    )(
        A_x.reshape(S, M), A_c_kv.reshape(S, Dc),
        A_w_q, A_w_uk, A_w_uv,
        A_w_o.reshape(H // 2, 2 * D, M),
        B_w1, B_w2, B_w3.T, B_w4, c, w_mod,
    )
    return out.reshape(1, S, M)
```

```python
import math

import jax
import jax.numpy as jnp
import jax.experimental.pallas as pl
import jax.experimental.pallas.tpu as pltpu

F32 = jnp.float32
BF16 = jnp.bfloat16
U32 = jnp.uint32
NT = (((1,), (1,)), ((), ()))
T = 128
EPS = 1e-5
LOG2E = math.log2(math.e)

GRP = 4
LEAD = 10
PROW = 3
RES = 32
LAT_A = 16
LAT_B = 20
ALEAD = 32
MID = 40
SD0, SDS, SDN, SDJ = 158, 2, 20, 30
QT = 3
RB = 256
PC = 32
P0, PSTEP, PD = 440, 30, 52
NLN, LN0, LNS = 4, 4, 5
LP = 16
PROLOGUE = ('|kva|Z; |b|; kva|wc|K0123; bw|xdn|C0@56 N0123@52 K4567; cx|mq|N4567@52 K89ab; '
            'd|y|C1@56 Kcdef; nmq|zo|M H01 H234567@30 Q0123; y||H89ab@30 Q4567; '
            'zo||L Hcdef@30 Q89ab S01 Qcdef')


def _dot(a, b):
    return jnp.dot(a, b, preferred_element_type=F32)


def _dot_nt(a, b):
    return jax.lax.dot_general(a, b, NT, preferred_element_type=F32)


def _ln(x):
    m = jnp.mean(x, axis=-1, keepdims=True)
    xc = x - m
    v = jnp.mean(xc * xc, axis=-1, keepdims=True)
    return xc * jnp.exp2(jnp.log(v + EPS) * (-0.5 * LOG2E))


def _rows(v, n):
    return jnp.broadcast_to(v[None], (n // 8, 8, v.shape[1])).reshape(n, v.shape[1])


def _gelu(x):
    c0 = math.sqrt(2.0 / math.pi)
    return 0.5 * x * (1.0 + jnp.tanh(c0 * (x + 0.044715 * (x * x * x))))


def _after(x, dep):
    return jnp.where(dep > jnp.inf, dep, x)


def _tie(x, dep):
    xu = pltpu.bitcast(x, U32)
    first = jnp.where(dep > jnp.inf, jnp.uint32(0), xu[:8])
    return pltpu.bitcast(jnp.concatenate([first, xu[8:]], axis=0), BF16)


def _tile(j):
    return slice(j * T, (j + 1) * T)


def _ld(ref, *idx):
    return pltpu.bitcast(ref[idx], BF16)


def _pk(x):
    return pltpu.bitcast(x, U32)


def _a_ops(a11, a12, a21, a22):
    return [a11 + a22, a21 + a22, a11, a22, a11 + a12, a21 - a11, a12 - a22]


def _b_ops(b11, b12, b21, b22):
    return [b11 + b22, b11, b12 - b22, b21 - b11, b22, b11 + b12, b21 + b22]


def _strassen(prod, col1=None, col2=None):
    m4 = prod(3)
    m2 = prod(1)
    c21 = m2 + m4
    if col1 is not None:
        e11, e21 = col1()
        m4, c21 = m4 + e11, c21 + e21
    m3 = prod(2)
    m5 = prod(4)
    c12 = m3 + m5
    if col2 is not None:
        e12, e22 = col2()
        c12, m3 = c12 + e12, m3 + e22
    m1 = prod(0)
    c11 = prod(6) + (m1 + (m4 - m5))
    c22 = prod(5) + (m1 + (m3 - m2))
    return c11, c12, c21, c22


def _group(rows, cols, pairs):
    xs, ys = dict.fromkeys(x for x, _ in pairs), dict.fromkeys(y for _, y in pairs)
    used = set(xs) | set(ys) | {(x[0], y[1]) for x, y in pairs} | {(y[0], x[1]) for x, y in pairs}
    prods = []
    for n, r in enumerate(rows):
        for i, k in [x for x in xs if x[0] == r]:
            mates = [y for x, y in pairs if x == (i, k)]
            prods.append((((1, i, k),) + tuple((1, i, k2) for _, k2 in mates), ((1, k, 0),),
                          ((1, i, 0), (-1, i, 1))))
            prods.append((((1, i, k),) + tuple((-1, i2, k) for i2, _ in mates), ((1, k, 0), (1, k, 1)),
                          ((1, i, 1),)))
        for i2, k2 in [y for y in ys if y[0] == r]:
            mates = [x for x, y in pairs if y == (i2, k2)]
            prods.append((((1, i2, k2),) + tuple((1, i2, k) for _, k in mates), ((1, k2, 1),),
                          ((1, i2, 1), (-1, i2, 0))))
            prods.append((((1, i2, k2),) + tuple((-1, i, k2) for i, _ in mates), ((1, k2, 0), (1, k2, 1)),
                          ((1, i2, 0),)))
        prods += [(((1, r, k),), ((1, k, h),), ((1, r, h),)) for k in cols if (r, k) not in used for h in (0, 1)]
        for (i, k), (i2, k2) in pairs:
            if r in (i, i2) and i + i2 - r in rows[n + 1:]:
                prods.append((((1, i, k2),), ((1, k2, 0), (-1, k, 0)), ((1, i2, 0), (1, i, 0))))
                prods.append((((1, i2, k), (1, i, k2)), ((1, k, 0), (1, k2, 1)), ((1, i2, 0), (1, i, 1))))
                prods.append((((1, i2, k),), ((1, k, 1), (-1, k2, 1)), ((1, i2, 1), (1, i, 1))))
    return prods


def _all_pairs(xrows, yrows):
    return [((x, a), (y, b)) for a, x in enumerate(xrows) for b, y in enumerate(yrows) if a != b]


_PAIRS65 = [((x[0] + 10, x[1]), (y[0] + 10, y[1])) for x, y in (
    ((0, 1), (1, 0)), ((0, 1), (5, 2)), ((2, 3), (1, 0)), ((2, 3), (3, 1)), ((2, 3), (5, 2)), ((3, 2), (1, 0)),
    ((4, 4), (0, 3)), ((4, 4), (1, 0)), ((4, 4), (3, 1)), ((4, 4), (5, 2)))]
_C_GROUPS = [_group(range(r, r + 8), range(4), _all_pairs(range(r, r + 4), range(r + 4, r + 8))) for r in (0, 8)]
_H_GROUPS = [_group(range(10), range(5), _all_pairs(range(5), range(5, 10))),
             _group(range(10, 16), range(5), _PAIRS65)]
_sum_index = lambda groups: {f: n for n, f in enumerate(
    dict.fromkeys(t[0] for g in groups for t in g if len(t[0]) > 1))}
_C_SUMS, _H_SUMS = _sum_index(_C_GROUPS), _sum_index(_H_GROUPS)


def _form(form, get):
    acc = None
    for sign, i, j in form:
        v = get(i, j)
        acc = v if acc is None else (acc + v if sign > 0 else acc - v)
    return acc


def _gap_items(bufs, gap_scr):
    items = []
    for n, buf in enumerate(bufs):
        acc = []

        def part(r0, buf=buf, acc=acc):
            def fn(dep):
                wu = jnp.concatenate([buf[r:r + 8, :] for r in range(r0, r0 + T, 32)])
                mask = jnp.full((8, T), 0x7FFF0000, U32)
                if dep is not None:
                    mask = jnp.where(dep > jnp.inf, jnp.uint32(0), mask)
                mask = _rows(mask, 32)
                new = [jnp.sum(pltpu.bitcast(v & mask, F32).reshape(4, 8, T), axis=0) for v in (wu << 16, wu)]
                acc[:] = [u + v for u, v in zip(acc, new)] if acc else new
            return fn

        def last(_, n=n, acc=acc):
            bits = []
            for v in acc:
                l1 = jnp.sum(jnp.sum(v, axis=1, keepdims=True), axis=0, keepdims=True)
                bits.append(pltpu.bitcast(jnp.broadcast_to(l1, (8, T)), jnp.int32) >> 8)
            gap_scr[n] = jnp.clip((bits[0] - bits[1] + (1 << 14)) >> 15, -8, 8) << 23

        items += [part(r0) for r0 in range(0, buf.shape[0], T)] + [last]
    return items


class _PairWeights:
    def __init__(self, w_ref, transpose=False, shift=None):
        self.base = {}
        if shift is not None:
            fac = _rows(pltpu.bitcast(0x3F800000 + shift, F32), T)
            self.inv = pltpu.bitcast(0x3F800000 - shift, F32)
        for j in range(w_ref.shape[0] // T):
            wu = w_ref[_tile(j), :]
            if transpose:
                wu = wu.T
            hi = pltpu.bitcast(wu & jnp.uint32(0xFFFF0000), F32)
            self.base[j, 0] = pltpu.bitcast(wu << 16, F32)
            self.base[j, 1] = hi if shift is None else hi * fac
        self.cache = {}

    def __call__(self, form):
        sign = 1
        if form[-1][0] < 0 and form[0][1:] > form[1][1:]:
            sign, form = -1, ((1,) + form[1][1:], (-1,) + form[0][1:])
        if form not in self.cache:
            self.cache[form] = _form(form, lambda k, h: self.base[k, h]).astype(BF16)
        return sign, self.cache[form]


def _run_group(jobs, prods, a_get, w, transposed, finish):
    left = {}
    for _, _, outs in prods:
        for _, i, h in outs:
            left[i, h] = left.get((i, h), 0) + 1
    acc = {}
    for af, bf, outs in prods:
        sign, wt = w(bf)
        m = jobs.mm([wt], [a_get(af)], _dot_nt) if transposed else jobs.mm([a_get(af)], [wt], _dot)
        for s_, i, h in outs:
            if (i, h) not in acc:
                acc[i, h] = (s_ * sign, m)
            else:
                s0, v = acc[i, h]
                acc[i, h] = (s0, v + m if s0 == s_ * sign else v - m) if s0 > 0 or s_ * sign < 0 else (1, m - v)
            left[i, h] -= 1
            if not left[i, h]:
                s0, v = acc.pop((i, h))
                assert s0 > 0
                finish(2 * i + h, v)


class _Jobs:
    def __init__(self, side=()):
        self.res = []
        self.side = list(side)

    def mm(self, lhs, wt, dot):
        acc = None
        for x, w in zip(lhs, wt):
            v = dot(x, w)
            self.res.append(v)
            acc = v if acc is None else v + acc
            rel = 4 * (len(self.res) % 4)
            while self.side and self.side[0][0] <= len(self.res):
                self.side.pop(0)[1](v[8 * rel:8 * rel + 8, :])
                rel = (rel + 2) % 16
        return acc


def _proj_step(h_scr, hs_scr, c_ref, cs_scr, wq_ref, wuk_ref, wuv_ref, q_scr, k_scr, v_scr, scale, shifts, side):
    wk, wvT, wq = [_PairWeights(w, n == 1, shifts[n]) for n, w in enumerate((wuk_ref, wuv_ref, wq_ref))]
    c_get = lambda f: cs_scr[_C_SUMS[f]] if len(f) > 1 else c_ref[_tile(f[0][1]), _tile(f[0][2])]
    h_get = lambda f: hs_scr[_H_SUMS[f]] if len(f) > 1 else h_scr[f[0][1], f[0][2]]

    def put(dst, w, mul=None):
        muls = [mul, _rows(w.inv if mul is None else w.inv * mul, T)]

        def fn(u, v):
            v = (v if muls[u % 2] is None else v * muls[u % 2]).astype(BF16)
            dst[u] = _pk(v.T if mul is not None and u < QT else v)
        return fn

    jobs = _Jobs(side)
    for groups, get, w, transposed, fin in ((_C_GROUPS, c_get, wk, False, put(k_scr, wk)),
                                            (_C_GROUPS, c_get, wvT, True, put(v_scr, wvT)),
                                            (_H_GROUPS, h_get, wq, False, put(q_scr, wq, scale))):
        for prods in groups:
            _run_group(jobs, prods, get, w, transposed, fin)
    assert not jobs.side


def _inner_group(rows, cols, pairs):
    xs, ys = dict.fromkeys(x for x, _ in pairs), dict.fromkeys(y for _, y in pairs)
    used = set(xs) | set(ys) | {(x[0], y[1]) for x, y in pairs} | {(y[0], x[1]) for x, y in pairs}
    prods = []
    for i, j in xs:
        mates = [y for x, y in pairs if x == (i, j)]
        prods.append((((1, i, 0),), ((1, 0, j), (-1, 1, j)), ((1, i, j),) + tuple((1, i2, j) for i2, _ in mates)))
        prods.append((((1, i, 0), (1, i, 1)), ((1, 1, j),), ((1, i, j),) + tuple((-1, i, j2) for _, j2 in mates)))
    for i2, j2 in ys:
        mates = [x for x, y in pairs if y == (i2, j2)]
        prods.append((((1, i2, 0), (1, i2, 1)), ((1, 0, j2),),
                      ((1, i2, j2),) + tuple((-1, i2, j) for _, j in mates)))
        prods.append((((1, i2, 1),), ((1, 0, j2), (-1, 1, j2)),
                      ((-1, i2, j2),) + tuple((-1, i, j2) for i, _ in mates)))
    prods += [(((1, i, h),), ((1, h, j),), ((1, i, j),))
              for i in rows for j in cols if (i, j) not in used for h in (0, 1)]
    for (i, j), (i2, j2) in pairs:
        lo, hi = min(j, j2), max(j, j2)
        prods.append((((1, i2, 0), (-1, i, 0)), ((1, 0, lo), (1, 0, hi)), ((1, i2, j),)))
        prods.append((((1, i, 0), (1, i2, 1)), ((1, 0, j2), (1, 1, j)), ((1, i, j2), (1, i2, j))))
        prods.append((((1, i, 1), (-1, i2, 1)), ((1, 1, lo), (1, 1, hi)), ((1, i, j2),)))
    return prods


def _o_jobs():
    prods = (_inner_group(range(10), range(5), _all_pairs(range(0, 10, 2), range(1, 10, 2)))
             + _inner_group(range(10, 16), range(5), _PAIRS65))
    row = lambda t: max(i for _, i, _ in t[0])
    unit = lambda t: max(2 * i + h for _, i, h in t[0])
    need = lambda t: unit(t) if row(t) == 15 else 2 * row(t) + 1
    return [(need(t), t) for t in sorted(prods, key=need)]


_O_JOBS = _o_jobs()


def _job_order(nb):
    units = range(2 * nb)
    qa = [('a', u, c) for u in units for c in range(u // 2 + 1)]
    qb = [('b', u, c) for u in units for c in range(u // 2 + 1)]
    qo = [('o', u, j) for j, (u, _) in enumerate(_O_JOBS)]
    done = {}
    order = []

    def ready(q, lat, pre):
        return bool(q) and (pre, q[0][1]) in done and done[(pre, q[0][1])] + lat <= len(order)

    def emit(q):
        kind, u, j = job = q.pop(0)
        if kind != 'o' and j == u // 2:
            done[(kind, u)] = len(order)
        order.append(job)

    turn = 0
    while qa or qb or qo:
        pref = 'abo'[turn % 3]
        turn += 1
        for _ in range(GRP):
            b_ok, o_ok = ready(qb, LAT_A, 'a'), ready(qo, LAT_B, 'b')
            if pref == 'a' and qa and (len(qb) - len(qa) < ALEAD or not b_ok):
                emit(qa)
            elif pref == 'b' and b_ok:
                emit(qb)
            elif pref == 'o' and o_ok and (len(qo) > RES or not (qa or b_ok)):
                emit(qo)
            elif not (qa or b_ok or o_ok) and (qb or qo):
                emit(qb or qo)
            else:
                break
    return order


def _attention_step(q_scr, k_scr, v_scr, wo_ref, acc_scr, mid):
    causal = (jax.lax.broadcasted_iota(jnp.int32, (T, T), 0)
              <= jax.lax.broadcasted_iota(jnp.int32, (T, T), 1))
    sv, mx, mfin, lsum, pv, of, lhs = {}, {}, {}, {}, {}, {}, {}
    res = []
    wo, terms = {}, {}
    left = {}
    for _, t in _O_JOBS:
        for _, i, j in t[2]:
            left[i, j] = left.get((i, j), 0) + 1

    def job_a(u, c):
        r, hd = divmod(u, 2)
        s = (_dot if u < QT else _dot_nt)(_ld(k_scr, 2 * c + hd), _ld(q_scr, u))
        res.append(s)
        if c == r:
            s = jnp.where(causal, s, -1e9 * LOG2E)
        s = s.reshape(T // 8, 8, T)
        sv[(u, c)] = s
        pm = jnp.max(s, axis=0)
        mx[u] = pm if u not in mx else jnp.maximum(mx[u], pm)

    def job_b(u, c):
        r, hd = divmod(u, 2)
        if u not in mfin:
            mfin[u] = jnp.broadcast_to(jnp.max(mx[u], axis=0, keepdims=True), (8, T))
        m = mfin[u]
        if len(res) >= LEAD:
            r0 = 8 * PROW * (c % 4)
            m = _after(m, res[len(res) - LEAD][r0:r0 + 8, :])
        p = jnp.exp2(sv.pop((u, c)) - m[None])
        ls = jnp.sum(p, axis=0)
        lsum[u] = ls if u not in lsum else lsum[u] + ls
        v = _dot(_ld(v_scr, 2 * c + hd), p.reshape(T, T).astype(BF16))
        res.append(v)
        pv[u] = v if u not in pv else v + pv[u]
        if c == r:
            of[u] = pv[u] * (1.0 / jnp.sum(lsum[u], axis=0, keepdims=True))

    def job_o(_, n):
        af, bf, outs = _O_JOBS[n][1]
        if af not in lhs:
            v = _form(af, lambda i, h: of[2 * i + h])
            lhs[af] = _tie(v.astype(BF16).T, v[0:8, :])
        if bf not in wo:
            wo[bf] = (wo_ref[_tile(bf[0][1]), _tile(bf[0][2])] if len(bf) == 1 else
                      _form(bf, lambda h, j: wo_ref[_tile(h), _tile(j)].astype(F32)).astype(BF16))
        v = _dot(lhs[af], wo[bf])
        res.append(v)
        for sign, i, j in outs:
            terms.setdefault((i, j), []).append((sign, v))
            if len(terms[i, j]) == left[i, j]:
                tot = acc_scr[_tile(i), _tile(j)]
                for sg, m in terms.pop((i, j)):
                    tot = tot + m if sg > 0 else tot - m
                acc_scr[_tile(i), _tile(j)] = tot

    fns = dict(a=job_a, b=job_b, o=job_o)
    for n, (kind, u, j) in enumerate(_job_order(q_scr.shape[0] // 2)):
        if n == MID:
            mid()
        fns[kind](u, j)


def _kernel(x_hbm, c_hbm, wq_hbm, wuk_hbm, wuv_hbm, wo_hbm, w1_hbm, w2_hbm, w3_hbm, w4_hbm,
            cond_hbm, wmod_hbm, out_hbm,
            x_ref, c_ref, cond_ref, wma_ref, wmb_ref, w1_ref, w2_ref, w3_ref, w4_ref,
            wq_buf, wk_buf, wv_buf, wo_buf, out_buf, sem, wsem, osem,
            mod_scr, h_scr, cs_scr, hs_scr, w_scr, q_scr, k_scr, v_scr, acc_scr, xn_scr, xh_scr, a1_scr, t_scr,
            ws12, ws3, ws4, pq_buf, pk_buf, pv_buf, gap_scr, st_in):
    S, M = x_hbm.shape
    D = wq_hbm.shape[2]
    nattn = wo_hbm.shape[0]
    Fd = w4_hbm.shape[0]
    scale = float(D) ** -0.5 * LOG2E
    nb, nrb = S // T, S // RB
    km, kc = M // T, c_hbm.shape[1] // T
    NX = 4
    XR = S // NX
    CB = XR // T

    work, probe = (wk_buf, wv_buf, wq_buf), (pk_buf, pv_buf, pq_buf)

    def pcopies(g, bufs=work, s0=0):
        return [pltpu.make_async_copy(src.bitcast(U32).at[:, g, :], dst, wsem.at[s0 + j])
                for j, (src, dst) in enumerate(zip((wuk_hbm, wuv_hbm, wq_hbm), bufs))]

    def ocopy(g):
        return pltpu.make_async_copy(wo_hbm.at[g], wo_buf, wsem.at[3])

    def chunk_copy(src, dst, i, s0):
        rows = slice(i * XR, (i + 1) * XR)
        return pltpu.make_async_copy(src.at[rows, :], dst.at[rows, :], sem.at[s0 + i])

    cp_cond = pltpu.make_async_copy(cond_hbm, cond_ref, sem.at[0])
    cp_wma = pltpu.make_async_copy(wmod_hbm.at[:, 0:2 * M], wma_ref, sem.at[1])
    cp_late = [pltpu.make_async_copy(src, dst, sem.at[2 + j]) for j, (src, dst) in enumerate((
        (wmod_hbm.at[:, 2 * M:6 * M], wmb_ref), (w1_hbm, w1_ref), (w2_hbm, w2_ref),
        (w3_hbm, w3_ref), (w4_hbm, w4_ref)))]
    cp_x = [chunk_copy(x_hbm, x_ref, i, 7) for i in range(NX)]
    cp_c = [chunk_copy(c_hbm, c_ref, i, 7 + NX) for i in range(NX)]

    def silu_cond():
        cf = cond_ref[...].astype(F32)
        return jnp.broadcast_to((cf * jax.nn.sigmoid(cf)).astype(BF16), (8, M))

    cp_wk, cp_wv, cp_wq = pcopies(0)
    named = dict(k=cp_wk, v=cp_wv, q=cp_wq, o=ocopy(0), n=cp_cond, m=cp_wma)
    named.update(zip('abcd', cp_c))
    named.update(zip('wxyz', cp_x))
    started, arrived, did = set(), set(), set()

    def zero(r, carry):
        acc_scr[pl.ds(pl.multiple_of(r * T, T), T), :] = jnp.zeros((T, M), F32)
        return carry

    def x_rows(rows, dep):
        xf = x_ref[rows, :].astype(F32)
        if dep is None:
            return xf
        return jnp.concatenate([_after(xf[:, :T], _rows(dep, xf.shape[0])), xf[:, T:]], axis=1)

    def n_item(r, i):
        def fn(dep):
            rows = slice(r * T + i * LP, r * T + (i + 1) * LP)
            xn_scr[rows, :] = _ln(x_rows(rows, dep))
        return fn

    def h_item(r, i, normed):
        def fn(dep):
            rows = slice(i * LP, (i + 1) * LP)
            grows = slice(r * T + i * LP, r * T + (i + 1) * LP)
            sa = mod_scr[:, 0:M]
            if normed and dep is not None:
                sa = jnp.concatenate([_after(sa[:, _tile(j)], dep) for j in range(km)], axis=1)
            hf = ((xn_scr[grows, :] if normed else _ln(x_rows(grows, dep))) * _rows(mod_scr[:, M:2 * M], LP)
                  + _rows(sa, LP))
            for j in range(km):
                h_scr[r, j, rows, :] = hf[:, _tile(j)].astype(BF16)
            for f, n in _H_SUMS.items():
                if all(t[1] == r for t in f):
                    hs_scr[n, rows, :] = _form(f, lambda _, k: hf[:, _tile(k)]).astype(BF16)
            did.add(('h', r, i))
        return fn

    def release(jobs, span, items):
        if span and items:
            jobs.side += [(len(jobs.res) + 1 + i * span // len(items), fn) for i, fn in enumerate(items)]
            jobs.side.sort(key=lambda e: e[0])
        else:
            for fn in items:
                fn(None)

    def sum_items(n, group, index, dst, get, skip_rows):
        forms = [f for f in dict.fromkeys(t[0] for t in group)
                 if len(f) > 1 and not (skip_rows and len({t[1] for t in f}) == 1)]

        def item(f, rows):
            def fn(dep):
                def term(r, k):
                    v = get(r, k, rows).astype(F32)
                    return v if dep is None or (r, k) != f[0][1:] else _after(v, _rows(dep, v.shape[0]))
                dst[index[f], rows, :] = _form(f, term).astype(BF16)
            return fn

        return [item(f, slice(i, i + n)) for i in range(0, T, n) for f in forms]

    h_sums = lambda n, gi: sum_items(n, _H_GROUPS[gi], _H_SUMS, hs_scr,
                                     lambda r_, k, rows: h_scr[r_, k, rows, :], True)

    def stash(key, buf, j0, transpose=False):
        n = buf.shape[0] // T
        if key not in did:
            assert key in arrived
            did.add(key)
            w = _PairWeights(buf, transpose)
            for j in range(n):
                for hd in range(2):
                    w_scr[hd, j0 + j] = _pk(w(((1, j, hd),))[1])
        return lambda hd: [_ld(w_scr, hd, j0 + j) for j in range(n)]

    def kv_tile(jobs, r):
        wk, wvT = stash('k', wk_buf, 0), stash('v', wv_buf, kc, True)
        ct = [c_ref[_tile(r), _tile(j)] for j in range(kc)]
        for hd in range(2):
            k_scr[2 * r + hd] = _pk(jobs.mm(ct, wk(hd), _dot).astype(BF16))
        for hd in range(2):
            v_scr[2 * r + hd] = _pk(jobs.mm(wvT(hd), ct, _dot_nt).astype(BF16))

    def q_tile(jobs, r):
        wq = stash('q', wq_buf, 2 * kc)
        ht = [h_scr[r, j] for j in range(km)]
        for hd in range(2):
            v = (jobs.mm(ht, wq(hd), _dot) * scale).astype(BF16)
            q_scr[2 * r + hd] = _pk(v.T if 2 * r + hd < QT else v)

    for blk in PROLOGUE.split(';'):
        waits, starts, acts = blk.split('|')
        for ch in waits.strip():
            assert ch in started and ch not in arrived
            arrived.add(ch)
            named[ch].wait()
        for ch in starts.strip():
            assert ch not in started
            started.add(ch)
            named[ch].start()
        jobs = _Jobs()
        for act in acts.split():
            if act == 'Z':
                jax.lax.fori_loop(0, nb, zero, 0)
                acc_scr[S:, :] = jnp.zeros((acc_scr.shape[0] - S, M), F32)
                x_ref[S:, :] = jnp.zeros((x_ref.shape[0] - S, M), BF16)
            elif act == 'L':
                did.add('L')
                for cp in cp_late:
                    cp.start()
            elif act == 'M':
                assert arrived >= set('nm')
                mod = _dot(silu_cond(), wma_ref[...])
                mod_scr[:, 0:M] = mod[:, 0:M]
                mod_scr[:, M:2 * M] = 1.0 + mod[:, M:2 * M]
                did.add('M')
            else:
                act, _, span = act.partition('@')
                span = int(span or 0)
                items = []
                for r in [int(ch, 16) for ch in act[1:]]:
                    did.add((act[0], r))
                    if act[0] == 'K':
                        assert 'abcd'[r // CB] in arrived
                        kv_tile(jobs, r)
                    elif act[0] == 'H':
                        assert 'wxyz'[r // CB] in arrived and 'M' in did
                        items += [h_item(r, i, ('N', r) in did) for i in range(T // LP)]
                    elif act[0] == 'N':
                        assert 'wxyz'[r // CB] in arrived
                        items += [n_item(r, i) for i in range(T // LP)]
                    elif act[0] == 'Q':
                        assert all(('h', r, i) in did for i in range(T // LP))
                        q_tile(jobs, r)
                    elif act[0] == 'C':
                        assert all('abcd'[t[1] // CB] in arrived for p_ in _C_GROUPS[r] for t in p_[0])
                        items += sum_items(
                            32, _C_GROUPS[r], _C_SUMS, cs_scr,
                            lambda r_, k, rows: c_ref[r_ * T + rows.start:r_ * T + rows.stop, _tile(k)], False)
                    else:
                        assert act[0] == 'S' and all(('h', t[1], T // LP - 1) in did for p_ in _H_GROUPS[r] for t in p_[0])
                        items += h_sums(32 if span else 16, r)
                release(jobs, span, items)
        assert not jobs.side
    assert arrived == set(named) and all((k_, r) in did for k_ in 'KHQ' for r in range(nb))
    assert all((k_, r) in did for k_ in 'CS' for r in range(2)) and 'L' in did

    FH = ws3.shape[0] * T
    assert nattn - 1 >= FH // 64

    slices = ((w1_hbm, 32, 2 * T, 0), (w2_hbm, 32, 2 * T, 64), (w4_hbm, 64, FH, 128), (w3_hbm, T, FH, 256))
    slice_of = lambda g, n, half: jnp.minimum(g, half // n - 1)

    def prep_in(g):
        return [pltpu.make_async_copy(
            w.at[pl.ds(pl.multiple_of(slice_of(g, n, half) * n + x * half, n), n), 0:4 * T],
            st_in.at[r0 + x * n:r0 + (x + 1) * n, :], wsem.at[7]) for w, n, half, r0 in slices for x in range(2)]

    def mixer_prep(g):
        def blocks(r0, n, half, c0, c1, dep):
            get = lambda x, c: st_in[r0 + x * half:r0 + x * half + n, _tile(c)].astype(F32)
            return [_after(get(0, c0), _rows(dep, n)), get(0, c1), get(1, c0), _after(get(1, c1), _rows(dep, n))]

        def rows_item(dst, per, half, r0, c, o, n=16):
            def fn(dep):
                rows = pl.ds(pl.multiple_of(slice_of(g, per, half) * (per // 2), per // 2) + o // 2, n // 2)
                for i, v in enumerate(_b_ops(*blocks(r0 + o, n, per, c, c + 2, dep))):
                    dst[i, c, rows, :] = _pk(v.astype(BF16))
            return fn

        def w3_item(k, i):
            def fn(dep):
                b11, b21, b12, b22 = blocks(slices[3][3], T, T, k, k + 2, dep)
                ws3[slice_of(g, T, FH), i, k] = _pk(_b_ops(b11, b12, b21, b22)[i].astype(BF16).T)
            return fn

        return ([rows_item(dst, *sl[1:], c, o) for dst, sl in zip((ws12.at[0], ws12.at[1], ws4), slices)
                 for c in range(2) for o in range(0, sl[1], 16)]
                + [w3_item(k, i) for k in range(2) for i in range(7)])

    def attn_body(g, carry):
        copies = pcopies(jnp.minimum(g + 1, nattn - 1)) + pcopies(jnp.minimum(g + 2, nattn - 1), probe, 4)

        def mid():
            for cp in copies + prep_in(g):
                cp.start()

        _attention_step(q_scr, k_scr, v_scr, wo_buf, acc_scr, mid)
        for cp in copies:
            cp.wait()
        pltpu.make_async_copy(st_in, st_in, wsem.at[7]).wait()

        @pl.when(g == 0)
        def _():
            for fn in _gap_items(work, gap_scr):
                fn(None)

        @pl.when(g + 1 < nattn)
        def _():
            ocopy(g + 1).start()
            side = mixer_prep(g) + _gap_items(probe, gap_scr)
            side = [(SD0 + i * SDS + (SDJ if i >= SDN else 0), fn) for i, fn in enumerate(side)]
            _proj_step(h_scr, hs_scr, c_ref, cs_scr, wq_buf, wk_buf, wv_buf, q_scr, k_scr, v_scr, scale,
                       gap_scr, side)
            ocopy(g + 1).wait()

        return carry

    jax.lax.fori_loop(0, nattn, attn_body, 0)

    for cp in cp_late:
        cp.wait()
    mod = _dot(silu_cond(), wmb_ref[...])
    mod_scr[:, 2 * M:4 * M] = mod[:, 0:2 * M]
    mod_scr[:, 4 * M:5 * M] = 1.0 + mod[:, 2 * M:3 * M]
    mod_scr[:, 5 * M:6 * M] = mod[:, 3 * M:4 * M]
    ftiles = [(f, min(f + T, Fd)) for f in range(0, Fd, T)]
    OFF = x_ref.shape[0] - S
    CAR = t_scr.shape[0] - RB

    def p1(r0, l0, n, dep=None):
        ga = mod_scr[:, 2 * M:3 * M]
        if dep is not None:
            ga = jnp.concatenate([_after(ga[:, 0:T], dep), ga[:, T:]], axis=1)
        rows = pl.ds(r0, n)
        x1 = x_ref[rows, :].astype(F32) + _rows(ga, n) * acc_scr[rows, :]
        xh_scr[0, l0:l0 + n, :] = x1
        hb = _ln(x1) * _rows(mod_scr[:, 4 * M:5 * M], n) + _rows(mod_scr[:, 3 * M:4 * M], n)
        xh_scr[1, l0:l0 + n, :] = hb
        return _ln(hb)

    HT = T // 2

    def p1_store(r0, c, dep=None):
        v = p1(r0 + c * PC, OFF + c * PC, PC, dep)
        a1_scr[c * PC:(c + 1) * PC, :] = v
        return jnp.max(v[:, M - T:].reshape(PC // 8, 8, T), axis=0)

    t_scr[RB:RB + CAR - OFF, :] = jnp.zeros((CAR - OFF, M), F32)
    t_scr[RB + CAR - OFF:RB + CAR, :] = _gelu(_dot(p1(0, 0, OFF).astype(BF16), w1_ref[...]))
    for c in range(RB // PC):
        p1_store(OFF, c)

    def out_copy(i):
        rows = pl.ds(i * T if isinstance(i, int) else pl.multiple_of(i * T, T), T)
        return pltpu.make_async_copy(out_buf.at[rows, :], out_hbm.at[rows, :], osem.at[i])

    def b_body(r, carry):
        gb = _rows(mod_scr[:, 5 * M:6 * M], T)
        r0 = pl.multiple_of(r * RB, RB)
        n0 = pl.multiple_of(jnp.minimum(r0 + RB, S - RB) + OFF, OFF)
        nh = RB // T
        now = [0]
        due = []
        pace = []

        def p1_item(c):
            return lambda dep: due.append((now[0] + PD, p1_store(n0, c, dep)))

        pace += [(P0 + i * PSTEP, p1_item(i)) for i in range(RB // PC)]
        wt = lambda ref, f0, f1, n: ref[f0:f1, _tile(n)]

        def mm(lhs, wts, dot=_dot):
            acc = None
            for x, w in zip(lhs, wts):
                if due and due[0][0] <= now[0]:
                    w = _tie(w, due.pop(0)[1])
                v = dot(x, w)
                now[0] += x.shape[0] // HT
                acc = v if acc is None else v + acc
                if pace and pace[0][0] <= now[0]:
                    pace.pop(0)[1](v[0:8, :])
            return acc

        def split_ops(lo, hi):
            return [v.astype(BF16) for v in _a_ops(lo[:HT], hi[:HT], lo[HT:], hi[HT:])]

        def two_tiles(aops, wsel, rest):
            def col(w):
                v = mm(rest[0], w, rest[3])
                return v[:HT], v[HT:]

            c11, c12, c21, c22 = _strassen(
                lambda i: mm([a[i] for a in aops], [wsel(i, k) for k in range(len(aops))]),
                lambda: col(rest[1]), lambda: col(rest[2]))
            return jnp.concatenate([c11, c21], axis=0), jnp.concatenate([c12, c22], axis=0)

        def square(full, aops, w_ref, ws_ref):
            out = {}
            for n in range(2):
                out[n], out[n + 2] = two_tiles(
                    aops, lambda i, k: _ld(ws_ref, i, n, slice(k * HT, (k + 1) * HT)),
                    (full[4:], [wt(w_ref, 4 * T, M, n)], [wt(w_ref, 4 * T, M, n + 2)], _dot))
            out[4] = mm(full, [wt(w_ref, j * T, (j + 1) * T, 4) for j in range(km)])
            return out

        t_scr[0:CAR, :] = t_scr[RB:RB + CAR, :]
        for hf in range(nh):
            a1 = [a1_scr[_tile(hf), _tile(j)] for j in range(km)]
            full = [v.astype(BF16) for v in a1]
            aops = [split_ops(a1[k], a1[2 + k]) for k in range(2)]
            for n, v in square(full, aops, w1_ref, ws12.at[0]).items():
                t = _gelu(v)
                if hf == nh - 1:
                    t = jnp.concatenate([t[:T - OFF], jnp.where(r < nrb - 1, t[T - OFF:], 0.0)], axis=0)
                t_scr[CAR + hf * T:CAR + (hf + 1) * T, _tile(n)] = t
        cq = M // 4
        shifts = (-1, 1, -2, 2)
        lane = jax.lax.broadcasted_iota(jnp.int32, (T, T), 1)
        y1, z, a3 = [], [], []
        for hf in range(nh):
            base = CAR - OFF + hf * T
            sh = []
            for j in range(km):
                g_lo, g_hi = (j * T) // cq, ((j + 1) * T - 1) // cq
                assert g_hi - g_lo <= 1
                v = t_scr[base + shifts[g_lo]:base + shifts[g_lo] + T, _tile(j)]
                if g_hi != g_lo:
                    v2 = t_scr[base + shifts[g_hi]:base + shifts[g_hi] + T, _tile(j)]
                    v = jnp.where(lane < g_hi * cq - j * T, v, v2)
                sh.append(v)
            hs = square([v.astype(BF16) for v in sh], [split_ops(sh[k], sh[2 + k]) for k in range(2)],
                        w2_ref, ws12.at[1])
            hs = jnp.concatenate([hs[n] for n in range(km)], axis=1)
            y1.append(hs + xh_scr[1, _tile(hf), :])
            z.append(xh_scr[0, _tile(hf), :] + gb * y1[hf])
            a3.append({})

            def ln_item(hf, c):
                def item(dep):
                    n = HT // NLN
                    for d in (0, HT):
                        v = y1[hf][d + c * n:d + (c + 1) * n]
                        if dep is not None:
                            v = jnp.concatenate([_after(v[:, :T], _rows(dep, n)), v[:, T:]], axis=1)
                        a3[hf][d + c * n] = _ln(v)
                return item

            ln_item(hf, 0)(None)
            pace += [(now[0] + LN0 + (c - 1) * LNS * (1 + hf), ln_item(hf, c)) for c in range(1, NLN)]
            pace.sort(key=lambda e: e[0])
        xh_scr[:, 0:OFF, :] = xh_scr[:, RB:RB + OFF, :]
        nf = FH // T
        h3, h3ops = [], []
        for hf in range(nh):
            assert len(a3[hf]) == 2 * NLN
            af = jnp.concatenate([a3[hf][key] for key in sorted(a3[hf])], axis=0)
            full = [af[:, _tile(j)].astype(BF16) for j in range(km)]
            aops = [split_ops(af[:, _tile(k)], af[:, _tile(2 + k)]) for k in range(2)]
            row, ops = {}, []
            narrow = None
            for n in range(nf):
                lo, hi = two_tiles(aops, lambda i, k: _ld(ws3, n, i, k),
                                   (full[4:], [wt(w3_ref, *ftiles[n], 4)],
                                    [wt(w3_ref, *ftiles[nf + n], 4)], _dot_nt))
                lo, hi = _gelu(lo), _gelu(hi)
                row[n], row[nf + n] = lo.astype(BF16), hi.astype(BF16)
                ops.append(split_ops(lo, hi))
                if n < km:
                    v = mm([wt(w3_ref, *ftiles[-1], n)], [full[n]], _dot_nt)
                    narrow = v if narrow is None else v + narrow
            row[2 * nf] = _gelu(mm(full, [wt(w3_ref, *ftiles[2 * nf], j) for j in range(km)],
                                   _dot_nt)).astype(BF16)
            fw = Fd - ftiles[-1][0]
            gT = jnp.concatenate([_gelu(narrow), jnp.zeros((T - fw, T), F32)], axis=0)
            row[2 * nf + 1] = _tie(gT.astype(BF16).T, gT[0:8, :])[:, :fw]
            h3.append([row[i] for i in range(len(ftiles))])
            h3ops.append(ops)
        for hf in range(nh):
            rows = pl.ds(pl.multiple_of(r0 + hf * T, T), T)

            def finish(n, v):
                out_buf[rows, _tile(n)] = (z[hf][:, _tile(n)] + gb[:, _tile(n)] * v).astype(out_buf.dtype)

            w4t = lambda n, f_: [wt(w4_ref, f0, f1, n) for f0, f1 in f_]
            finish(4, mm(h3[hf], w4t(4, ftiles)))
            for n in range(2):
                lo, hi = two_tiles(h3ops[hf], lambda i, k: _ld(ws4, i, n, slice(k * HT, (k + 1) * HT)),
                                   (h3[hf][2 * nf:], w4t(n, ftiles[2 * nf:]), w4t(n + 2, ftiles[2 * nf:]), _dot))
                finish(n, lo)
                finish(n + 2, hi)
            out_copy(r * nh + hf).start()
        assert not pace
        return carry

    jax.lax.fori_loop(0, nrb, b_body, 0)
    for i in range(nb):
        out_copy(i).wait()


@jax.jit
def pallas_adaLN_cond__compressed_kv_cla__mixer_s_mlp__prompt_kernel(
    A_x: jax.Array,
    A_c_kv: jax.Array,
    A_w_q: jax.Array,
    A_w_uk: jax.Array,
    A_w_uv: jax.Array,
    A_w_o: jax.Array,
    B_x: jax.Array,
    B_w1: jax.Array,
    B_w2: jax.Array,
    B_w3: jax.Array,
    B_w4: jax.Array,
    c: jax.Array,
    w_mod: jax.Array,
):
    _, S, M = A_x.shape
    Dc = A_c_kv.shape[2]
    H, D = A_w_q.shape[1], A_w_q.shape[2]
    Fd = B_w3.shape[1]
    assert D == T and A_c_kv.shape[1] == S and Dc == 4 * T and M == 5 * T and 13 * T < Fd < 14 * T and S == 16 * T
    vmem = pltpu.VMEM
    packed = lambda *lead: vmem(lead + (T // 2, T), U32)
    out = pl.pallas_call(
        _kernel,
        in_specs=[pl.BlockSpec(memory_space=pltpu.HBM)] * 12,
        out_specs=pl.BlockSpec(memory_space=pltpu.HBM),
        out_shape=jax.ShapeDtypeStruct((S, M), A_x.dtype),
        scratch_shapes=[
            vmem((S + 16, M), BF16),
            vmem((S, Dc), BF16),
            vmem((1, M), BF16),
            vmem((M, 2 * M), BF16),
            vmem((M, 4 * M), BF16),
            vmem((M, M), BF16),
            vmem((M, M), BF16),
            vmem((Fd, M), BF16),
            vmem((Fd, M), BF16),
            vmem((M, D), U32),
            vmem((Dc, D), U32),
            vmem((Dc, D), U32),
            vmem((2 * D, M), BF16),
            vmem((S, M), A_x.dtype),
            pltpu.SemaphoreType.DMA((15,)),
            pltpu.SemaphoreType.DMA((8,)),
            pltpu.SemaphoreType.DMA((S // T,)),
            vmem((8, 6 * M), F32),
            vmem((S // T, M // T, T, T), BF16),
            vmem((len(_C_SUMS), T, T), BF16),
            vmem((len(_H_SUMS), T, T), BF16),
            packed(2, M // T + 2 * (Dc // T)),
            packed(2 * S // T),
            packed(2 * S // T),
            packed(2 * S // T),
            vmem((S + 16, M), F32),
            vmem((S, M), F32),
            vmem((2, RB + 16, M), F32),
            vmem((RB, M), F32),
            vmem((RB + 32, M), F32),
            vmem((2, 7, 2, T, T), U32),
            packed(6, 7, 2),
            vmem((7, 2, 3 * T, T), U32),
            vmem((M, D), U32),
            vmem((Dc, D), U32),
            vmem((Dc, D), U32),
            vmem((3, 8, T), jnp.int32),
            vmem((4 * T, 4 * T), BF16),
        ],
        compiler_params=pltpu.CompilerParams(
            vmem_limit_bytes=100 * 1024 * 1024,
            disable_bounds_checks=True,
        ),
    )(
        A_x.reshape(S, M), A_c_kv.reshape(S, Dc),
        A_w_q, A_w_uk, A_w_uv,
        A_w_o.reshape(H // 2, 2 * D, M),
        B_w1, B_w2, B_w3.T, B_w4, c, w_mod,
    )
    return out.reshape(1, S, M)
```
